```python
import jax
import jax.numpy as jnp

def _softmax(x, axis=-1):
    return jax.nn.softmax(x, axis=axis)

def _gelu(x):
    return jax.nn.gelu(x, approximate=True)

def _silu(x):
    return jax.nn.silu(x)

def _sigmoid(x):
    return jax.nn.sigmoid(x)

def _layernorm(x, axis=-1, eps=1e-05):
    m = jnp.mean(x, axis=axis, keepdims=True)
    v = jnp.var(x, axis=axis, keepdims=True)
    return (x - m) / jnp.sqrt(v + eps)

def _scatter_add(tgt, idx, src, axis=0):
    return tgt.at[idx].add(src)

def _segment_sum(src, seg, n):
    return jax.ops.segment_sum(src, seg, n)

class _Rng:

    def __init__(self, key):
        self._k = key

    def _next(self):
        self._k, sub = jax.random.split(self._k)
        return sub

    def normal(self, shape):
        return jax.random.normal(self._next(), shape, dtype=jnp.bfloat16)

    def randint(self, lo, hi, shape):
        return jax.random.randint(self._next(), shape, lo, hi, dtype=jnp.int32)

    def uniform(self, shape, lo=0.0, hi=1.0):
        return jax.random.uniform(self._next(), shape, jnp.bfloat16, lo, hi)

    def permutation(self, n):
        return jax.random.permutation(self._next(), n)
kernel_name = 'gated_mix__memory_aug_recurrent_mem_tr__mixer_s_mlp__prompt'

def setup_inputs():
    _rng = _Rng(jax.random.key(int.from_bytes(__import__("os").urandom(4), "little")))
    _w = lambda a: (lambda t: t.astype(jnp.bfloat16) if jnp.issubdtype(t.dtype, jnp.floating) else t)(jnp.asarray(a))

    def _A_setup():
        B, S, Dm = (1, 2048, 1024)
        H, Dh = (32, 128)
        M, seg = (8, 32)
        seg = min(seg, S)
        S = S // seg * seg
        return {'x': _w((lambda *s: _rng.normal(s) * 0.05)(B, S, Dm)), 'mem0': _w((lambda *s: _rng.normal(s) * 0.05)(B, M, Dm)), 'Wq': _w((lambda *s: _rng.normal(s) * 0.05)(Dm, H, Dh) * Dm ** (-0.5)), 'Wk': _w((lambda *s: _rng.normal(s) * 0.05)(Dm, H, Dh) * Dm ** (-0.5)), 'Wv': _w((lambda *s: _rng.normal(s) * 0.05)(Dm, H, Dh) * Dm ** (-0.5)), 'Wo': _w((lambda *s: _rng.normal(s) * 0.05)(H, Dh, Dm) * (H * Dh) ** (-0.5)), 'seg_len': seg}
    _A_in = _A_setup()

    def _B_setup():
        B, S, D, F = (1, 2048, 1024, 3584)
        return {'x': _w((lambda *s: _rng.normal(s) * 0.05)(B, S, D)), 'w1': _w((lambda *s: _rng.normal(s) * 0.05)(D, D) * D ** (-0.5)), 'w2': _w((lambda *s: _rng.normal(s) * 0.05)(D, D) * D ** (-0.5)), 'w3': _w((lambda *s: _rng.normal(s) * 0.05)(D, F) * D ** (-0.5)), 'w4': _w((lambda *s: _rng.normal(s) * 0.05)(F, D) * F ** (-0.5))}
    _B_in = _B_setup()
    return {'A_x': _A_in['x'], 'A_mem0': _A_in['mem0'], 'A_Wq': _A_in['Wq'], 'A_Wk': _A_in['Wk'], 'A_Wv': _A_in['Wv'], 'A_Wo': _A_in['Wo'], 'A_seg_len': _A_in['seg_len'], 'B_x': _B_in['x'], 'B_w1': _B_in['w1'], 'B_w2': _B_in['w2'], 'B_w3': _B_in['w3'], 'B_w4': _B_in['w4'], 'gate_w': _w((lambda *s: _rng.normal(s) * 0.05)(1024))}

def reference(A_x, A_mem0, A_Wq, A_Wk, A_Wv, A_Wo, A_seg_len, B_x, B_w1, B_w2, B_w3, B_w4, gate_w):

    def _A_ref(x, mem0, Wq, Wk, Wv, Wo, seg_len):
        B, S, Dm = x.shape
        H, Dh = (Wq.shape[1], Wq.shape[2])
        M = mem0.shape[1]
        scale = Dh ** (-0.5)
        n_seg = S // seg_len
        L = M + seg_len
        idx = jnp.arange(L)
        mask = (idx[:, None] < M) | (idx[:, None] >= idx[None, :])
        mem = mem0
        outs = []
        for s in range(n_seg):
            xs = x[:, s * seg_len:(s + 1) * seg_len, :].copy()
            h = jnp.concatenate([mem, xs], axis=1)
            q = jnp.einsum('btd,dhe->bhte', h, Wq)
            k = jnp.einsum('btd,dhe->bhte', h, Wk)
            v = jnp.einsum('btd,dhe->bhte', h, Wv)
            scores = jnp.einsum('bhqe,bhke->bhqk', q, k) * scale
            scores = jnp.where(mask[None, None], scores, -1000000000.0)
            p = _softmax(scores, axis=-1)
            o = jnp.einsum('bhqk,bhke->bhqe', p, v)
            o = jnp.einsum('bhte,hed->btd', o, Wo)
            mem = o[:, :M, :].copy()
            outs.append(o[:, M:, :])
        return jnp.concatenate(outs, axis=1)

    def _B_ref(x, w1, w2, w3, w4):
        B, S, D = x.shape
        h = _gelu(_layernorm(x, axis=-1) @ w1)
        c = D // 4
        g0 = jnp.pad(h[:, :, 0 * c:1 * c], ((0, 0), (1, 0), (0, 0)))[:, :S, :]
        g1 = jnp.pad(h[:, :, 1 * c:2 * c], ((0, 0), (0, 1), (0, 0)))[:, 1:, :]
        g2 = jnp.pad(h[:, :, 2 * c:3 * c], ((0, 0), (2, 0), (0, 0)))[:, :S, :]
        g3 = jnp.pad(h[:, :, 3 * c:], ((0, 0), (0, 2), (0, 0)))[:, 2:, :]
        hs = jnp.concatenate([g0, g1, g2, g3], axis=-1) @ w2
        x1 = x + hs
        h2 = _gelu(_layernorm(x1, axis=-1) @ w3) @ w4
        return x1 + h2
    x = A_x
    g = _sigmoid((x * gate_w).sum(-1, keepdims=True))
    a = _A_ref(x, A_mem0, A_Wq, A_Wk, A_Wv, A_Wo, A_seg_len)
    b = _B_ref(x, B_w1, B_w2, B_w3, B_w4)
    return g * a + (1 - g) * b
```

```python
import functools

import jax
import jax.numpy as jnp
from jax import lax
import jax.experimental.pallas as pl
import jax.experimental.pallas.tpu as pltpu

f32, bf16, u32 = jnp.float32, jnp.bfloat16, jnp.uint32

S, D, H, DH, M, SEG, F = 2048, 1024, 32, 128, 8, 32, 3584
SCALE = DH ** -0.5
NEG = -1000000000.0
EPS = 1e-05

TM = 256
NB = S // TM
FC = 512
NFC = F // FC
NPAIR = S // (2 * SEG)
G = 4
NG = H // G
PAD = 8
NT = D // 128

_dot = functools.partial(jnp.dot, preferred_element_type=f32)


def _ln(x):
    m = jnp.mean(x, axis=-1, keepdims=True)
    xc = x - m
    v = jnp.mean(xc * xc, axis=-1, keepdims=True)
    return xc * lax.rsqrt(v + EPS)


def _gelu(x):
    return jax.nn.gelu(x, approximate=True)


def _masks():
    r = lax.broadcasted_iota(jnp.int32, (32, 48), 0)
    c = lax.broadcasted_iota(jnp.int32, (32, 48), 1)
    exist_e = (c >= 40) | (c < 32)
    allow_e = (c >= 40) | ((c < 32) & ((r >= 24) | (c <= r)))
    fill_e = jnp.where(exist_e, NEG, -jnp.inf).astype(f32)
    r = lax.broadcasted_iota(jnp.int32, (48, 80), 0)
    c = lax.broadcasted_iota(jnp.int32, (48, 80), 1)
    keys_even = (c < 32) | ((c >= 40) & (c < 48))
    exist_o = ((r < 8) & keys_even) | ((r >= 8) & ~keys_even)
    ktok = jnp.where(c < 40, c, c - 16)
    qtok = jnp.where(r < 8, r + 24, r + 16)
    is_mem_key = (c >= 40) & (c < 56)
    is_mem_q = (r >= 8) & (r < 16)
    allow_o = exist_o & (is_mem_key | is_mem_q | (ktok <= qtok))
    fill_o = jnp.where(exist_o, NEG, -jnp.inf).astype(f32)
    return allow_e, fill_e, allow_o, fill_o


def _softmax(s, allow, fill):
    s = jnp.where(allow, s * SCALE, fill)
    m = jnp.max(s, axis=-1, keepdims=True)
    e = jnp.exp(s - m)
    l = jnp.sum(e, axis=-1, keepdims=True)
    return (e * pl.reciprocal(l, approx=False)).astype(bf16)


def _kernel(x_hbm, mem0_ref, wq_hbm, wk_hbm, wv_hbm, wo_hbm, w1_hbm, w2_hbm, w3_hbm, w4_hbm,
            gw_ref, out_hbm,
            x_v, w1_v, w2_v, w3_v, w4_v, wqkv_v, wo_v, h_v, b_v, xn_v, out_v,
            ke_v, ve_v, o_v, mem_v,
            sem_x, sem_w, sem_qkv, sem_wo, sem_out):
    def x_copy(i):
        return pltpu.make_async_copy(x_hbm.at[pl.ds(i * TM, TM)], x_v.at[pl.ds(i * TM, TM)], sem_x.at[i])

    w_copies = [pltpu.make_async_copy(src, dst, sem_w.at[i]) for i, (src, dst) in enumerate(
        [(w1_hbm, w1_v), (w2_hbm, w2_v), (w3_hbm, w3_v), (w4_hbm, w4_v)])]

    SLABS_PER_GROUP = 3 * H // NB

    def qkv_copies():
        cps = []
        for w, w_hbm in enumerate((wq_hbm, wk_hbm, wv_hbm)):
            wu = w_hbm.bitcast(u32)
            for hp in range(H // 2):
                for par in range(2):
                    slab = w * H + 2 * hp + par
                    cps.append(pltpu.make_async_copy(
                        wu.at[:, par * (H // 2) + hp, :], wqkv_v.at[slab],
                        sem_qkv.at[slab // SLABS_PER_GROUP]))
        return cps

    def wo_copies():
        wu = wo_hbm.bitcast(u32)
        return [pltpu.make_async_copy(wu.at[:, pl.ds(j * 128, 128)], wo_v.at[j], sem_wo)
                for j in range(NT)]

    x_copy(0).start()
    w_copies[0].start()
    for i in range(1, NB):
        x_copy(i).start()
    for cp in w_copies[1:]:
        cp.start()
    for cp in qkv_copies():
        cp.start()
    for cp in wo_copies():
        cp.start()

    h_v[:, 0:PAD, :] = jnp.zeros((NT, PAD, 128), f32)
    h_v[:, PAD + S:PAD + S + PAD, :] = jnp.zeros((NT, PAD, 128), f32)

    def d1(i):
        x_copy(i).wait()
        if i == 0:
            w_copies[0].wait()
        xn = _ln(x_v[i * TM:(i + 1) * TM, :].astype(f32)).astype(bf16)
        h = _gelu(_dot(xn, w1_v[...]))
        for j in range(NT):
            h_v[j, PAD + i * TM:PAD + (i + 1) * TM, :] = h[:, j * 128:(j + 1) * 128]

    shifts = (1, 1, -1, -1, 2, 2, -2, -2)

    def d2(i):
        if i == 0:
            w_copies[1].wait()
        hs = jnp.concatenate(
            [h_v[j, pl.ds(PAD + i * TM - shifts[j], TM), :].astype(bf16) for j in range(NT)], axis=1)
        x1 = x_v[i * TM:(i + 1) * TM, :].astype(f32) + _dot(hs, w2_v[...])
        b_v[i * TM:(i + 1) * TM, :] = x1
        xn_v[i * TM // 2:(i + 1) * TM // 2, :] = pltpu.bitcast(_ln(x1).astype(bf16), u32)

    for i in range(NB + 2):
        if i >= 2:
            d2(i - 2)
        if i < NB:
            d1(i)

    w_copies[2].wait()
    w_copies[3].wait()

    def ffn(i, carry):
        grp = wqkv_v.at[pl.ds(i * SLABS_PER_GROUP, SLABS_PER_GROUP)]
        pltpu.make_async_copy(grp, grp, sem_qkv.at[i]).wait()
        r0 = pl.multiple_of(i * TM, TM)
        xn = pltpu.bitcast(xn_v[pl.ds(pl.multiple_of(i * (TM // 2), TM // 2), TM // 2), :], bf16)
        hs = {}

        def d3(c):
            hs[c] = _gelu(_dot(xn, w3_v[:, c * FC:(c + 1) * FC])).astype(bf16)

        def relayout(p):
            s0 = i * SLABS_PER_GROUP + 2 * p
            e = wqkv_v[s0]
            o = wqkv_v[s0 + 1]
            wqkv_v[s0] = (e & jnp.uint32(0xFFFF)) | (o << 16)
            wqkv_v[s0 + 1] = (e >> 16) | (o & jnp.uint32(0xFFFF0000))

        acc = b_v[pl.ds(r0, TM), :]
        d3(0)
        for c in range(NFC):
            if c + 1 < NFC:
                d3(c + 1)
            if c < SLABS_PER_GROUP // 2:
                relayout(c)
            acc = _dot(hs.pop(c), w4_v[c * FC:(c + 1) * FC, :]) + acc
        b_v[pl.ds(r0, TM), :] = acc
        return carry

    lax.fori_loop(0, NB, ffn, 0)

    for cp in wo_copies():
        cp.wait()
    mem_v[...] = mem0_ref[...].astype(f32)

    def wload(idx):
        return pltpu.bitcast(wqkv_v[idx], bf16)

    def step(hq, hkv, odd, allow, fill):
        nq = hq.shape[0]
        qs, ks, vs, ps = {}, {}, {}, {}

        def proj(g):
            for h in range(g * G, (g + 1) * G):
                qs[h] = _dot(hq, wload(h)).astype(bf16)
                k = _dot(hkv, wload(H + h)).astype(bf16)
                v = _dot(hkv, wload(2 * H + h)).astype(bf16)
                if odd:
                    k = jnp.concatenate([pltpu.bitcast(ke_v[h], bf16), k], axis=0)
                    v = jnp.concatenate([pltpu.bitcast(ve_v[h], bf16), v], axis=0)
                else:
                    ke_v[h] = pltpu.bitcast(k, u32)
                    ve_v[h] = pltpu.bitcast(v, u32)
                ks[h] = k
                vs[h] = v

        def score(g):
            for h in range(g * G, (g + 1) * G):
                s = lax.dot_general(qs.pop(h), ks.pop(h), (((1,), (1,)), ((), ())),
                                    preferred_element_type=f32)
                ps[h] = _softmax(s, allow, fill)

        def pv(g):
            for h in range(g * G, (g + 1) * G):
                o = _dot(ps.pop(h), vs.pop(h)).astype(bf16)
                o_v[0:nq // 2, h * 128:(h + 1) * 128] = pltpu.bitcast(o, u32)

        acc = [None] * NT

        def wo(h0, h1, j0, j1):
            o = pltpu.bitcast(o_v[0:nq // 2, h0 * 128:h1 * 128], bf16)
            for j in range(j0, j1):
                y = _dot(o, pltpu.bitcast(wo_v[j, h0 * 64:h1 * 64, :], bf16))
                acc[j] = y if acc[j] is None else y + acc[j]

        for t in range(NG):
            proj(t)
            if t >= 1:
                score(t - 1)
            if t >= 2:
                pv(t - 2)
        wo(0, 16, 0, 4)
        score(NG - 1)
        pv(NG - 2)
        wo(0, 16, 4, 8)
        pv(NG - 1)
        wo(16, 24, 0, 8)
        wo(24, 32, 0, 8)
        return jnp.concatenate(acc, axis=1)

    def out_copy(j, slot):
        r0 = pl.multiple_of(j * 64, 64)
        return pltpu.make_async_copy(out_v.at[slot], out_hbm.at[pl.ds(r0, 64)], sem_out.at[slot])

    def pair(j, carry):
        slot = j % 2

        @pl.when(j >= 2)
        def _():
            out_copy(j - 2, slot).wait()

        allow_e, fill_e, allow_o, fill_o = _masks()
        r0 = pl.multiple_of(j * 64, 64)
        x0 = x_v[pl.ds(r0, 16), :]
        x1 = x_v[pl.ds(r0 + 16, 16), :]
        x2 = x_v[pl.ds(r0 + 32, 16), :]
        x3 = x_v[pl.ds(r0 + 48, 16), :]
        x1f = x1.astype(f32)
        x2f = x2.astype(f32)
        mem = mem_v[...]
        hq = jnp.concatenate([x0, jnp.concatenate([x1f[:8], mem], 0).astype(bf16)], 0)
        hkv = jnp.concatenate([x0, x1, jnp.concatenate([x2f[:8], mem], 0).astype(bf16)], 0)
        oe = step(hq, hkv, False, allow_e, fill_e)
        mem = oe[24:32]
        hq = jnp.concatenate([jnp.concatenate([x1f[8:], mem], 0).astype(bf16), x2, x3], 0)
        hkv = jnp.concatenate([jnp.concatenate([mem, x2f[8:]], 0).astype(bf16), x3], 0)
        oo = step(hq, hkv, True, allow_o, fill_o)
        mem_v[...] = oo[8:16]
        a = jnp.concatenate([oe[:24], oo[:8], oo[16:]], 0)
        xf = x_v[pl.ds(r0, 64), :].astype(f32)
        g = jax.nn.sigmoid(jnp.sum(xf * gw_ref[...].astype(f32), axis=-1, keepdims=True))
        out_v[slot] = (g * a + (1.0 - g) * b_v[pl.ds(r0, 64), :]).astype(bf16)
        out_copy(j, slot).start()
        return carry

    lax.fori_loop(0, NPAIR, pair, 0)
    out_copy(NPAIR - 2, 0).wait()
    out_copy(NPAIR - 1, 1).wait()


@functools.partial(jax.jit, static_argnames=("A_seg_len",))
def pallas_gated_mix__memory_aug_recurrent_mem_tr__mixer_s_mlp__prompt_kernel(
    A_x, A_mem0, A_Wq, A_Wk, A_Wv, A_Wo, A_seg_len, B_x, B_w1, B_w2, B_w3, B_w4, gate_w,
):
    assert A_seg_len == SEG
    assert A_x.shape == (1, S, D) and A_mem0.shape == (1, M, D)
    any_spec = pl.BlockSpec(memory_space=pl.ANY)
    vmem_spec = pl.BlockSpec(memory_space=pltpu.VMEM)
    out = pl.pallas_call(
        _kernel,
        out_shape=jax.ShapeDtypeStruct((S, D), bf16),
        in_specs=[any_spec, vmem_spec] + [any_spec] * 8 + [vmem_spec],
        out_specs=any_spec,
        scratch_shapes=[
            pltpu.VMEM((S, D), bf16),
            pltpu.VMEM((D, D), bf16),
            pltpu.VMEM((D, D), bf16),
            pltpu.VMEM((D, F), bf16),
            pltpu.VMEM((F, D), bf16),
            pltpu.VMEM((3 * H, D // 2, DH), u32),
            pltpu.VMEM((NT, H * DH // 2, 128), u32),
            pltpu.VMEM((NT, S + 2 * PAD, 128), f32),
            pltpu.VMEM((S, D), f32),
            pltpu.VMEM((S // 2, D), u32),
            pltpu.VMEM((2, 64, D), bf16),
            pltpu.VMEM((H, 24, 128), u32),
            pltpu.VMEM((H, 24, 128), u32),
            pltpu.VMEM((24, H * DH), u32),
            pltpu.VMEM((M, D), f32),
            pltpu.SemaphoreType.DMA((NB,)),
            pltpu.SemaphoreType.DMA((4,)),
            pltpu.SemaphoreType.DMA((NB,)),
            pltpu.SemaphoreType.DMA,
            pltpu.SemaphoreType.DMA((2,)),
        ],
        compiler_params=pltpu.CompilerParams(vmem_limit_bytes=120 * 1024 * 1024),
    )(
        A_x.reshape(S, D), A_mem0.reshape(M, D),
        A_Wq.reshape(D // 2, 2 * H, DH), A_Wk.reshape(D // 2, 2 * H, DH), A_Wv.reshape(D // 2, 2 * H, DH),
        A_Wo.reshape(H * DH, D), B_w1, B_w2, B_w3, B_w4, gate_w.reshape(1, D),
    )
    return out.reshape(1, S, D)
```

```python
import functools

import jax
import jax.numpy as jnp
from jax import lax
import jax.experimental.pallas as pl
import jax.experimental.pallas.tpu as pltpu

f32, bf16, u32 = jnp.float32, jnp.bfloat16, jnp.uint32

S, D, H, DH, M, SEG, F = 2048, 1024, 32, 128, 8, 32, 3584
SCALE = DH ** -0.5
NEG = -1000000000.0
EPS = 1e-05

TM = 256
NB = S // TM
FC = 512
NFC = F // FC
NPAIR = S // (2 * SEG)
G = 4
NG = H // G
PAD = 8
NT = D // 128
assert NB == NG

_dot = functools.partial(jnp.dot, preferred_element_type=f32)


def _ln(x):
    m = jnp.mean(x, axis=-1, keepdims=True)
    xc = x - m
    v = jnp.mean(xc * xc, axis=-1, keepdims=True)
    return xc * lax.rsqrt(v + EPS)


def _gelu(x):
    return jax.nn.gelu(x, approximate=True)


def _masks():
    r = lax.broadcasted_iota(jnp.int32, (32, 48), 0)
    c = lax.broadcasted_iota(jnp.int32, (32, 48), 1)
    exist_e = (c >= 40) | (c < 32)
    allow_e = (c >= 40) | ((c < 32) & ((r >= 24) | (c <= r)))
    fill_e = jnp.where(exist_e, NEG, -jnp.inf).astype(f32)
    r = lax.broadcasted_iota(jnp.int32, (48, 80), 0)
    c = lax.broadcasted_iota(jnp.int32, (48, 80), 1)
    keys_even = (c < 32) | ((c >= 40) & (c < 48))
    exist_o = ((r < 8) & keys_even) | ((r >= 8) & ~keys_even)
    ktok = jnp.where(c < 40, c, c - 16)
    qtok = jnp.where(r < 8, r + 24, r + 16)
    is_mem_key = (c >= 40) & (c < 56)
    is_mem_q = (r >= 8) & (r < 16)
    allow_o = exist_o & (is_mem_key | is_mem_q | (ktok <= qtok))
    fill_o = jnp.where(exist_o, NEG, -jnp.inf).astype(f32)
    return allow_e, fill_e, allow_o, fill_o


def _softmax(s, allow, fill):
    s = jnp.where(allow, s * SCALE, fill)
    m = jnp.max(s, axis=-1, keepdims=True)
    e = jnp.exp(s - m)
    l = jnp.sum(e, axis=-1, keepdims=True)
    return (e * pl.reciprocal(l, approx=False)).astype(bf16)


def _kernel(x_hbm, mem0_ref, wq_hbm, wk_hbm, wv_hbm, wo_hbm, w1_hbm, w2_hbm, w3_hbm, w4_hbm,
            gw_ref, out_hbm,
            x_v, w1_v, w2_v, w3_v, w4_v, wqkv_v, wo_v, h_v, b_v, xn_v, out_v,
            ke_v, ve_v, o_v, mem_v,
            sem_x, sem_w, sem_qkv, sem_wo, sem_out):
    def x_copy(i):
        return pltpu.make_async_copy(x_hbm.at[pl.ds(i * TM, TM)], x_v.at[pl.ds(i * TM, TM)], sem_x.at[i])

    w_copies = [pltpu.make_async_copy(src, dst, sem_w.at[i]) for i, (src, dst) in enumerate(
        [(w1_hbm, w1_v), (w2_hbm, w2_v), (w3_hbm, w3_v), (w4_hbm, w4_v)])]

    SPG = 3 * G

    def qkv_start(g):
        for w, w_hbm in enumerate((wq_hbm, wk_hbm, wv_hbm)):
            wu = w_hbm.bitcast(u32)
            for k in range(G // 2):
                for par in range(2):
                    pltpu.make_async_copy(
                        wu.at[:, par * (H // 2) + g * (G // 2) + k, :],
                        wqkv_v.at[g * SPG + w * G + 2 * k + par], sem_qkv.at[g]).start()

    def qkv_wait(g):
        grp = wqkv_v.at[pl.ds(g * SPG, SPG)]
        pltpu.make_async_copy(grp, grp, sem_qkv.at[g]).wait()

    def wo_copies():
        wu = wo_hbm.bitcast(u32)
        return [pltpu.make_async_copy(wu.at[:, pl.ds(j * 128, 128)], wo_v.at[j], sem_wo)
                for j in range(NT)]

    x_copy(0).start()
    w_copies[0].start()

    h_v[:, 0:PAD, :] = jnp.zeros((NT, PAD, 128), f32)
    h_v[:, PAD + S:PAD + S + PAD, :] = jnp.zeros((NT, PAD, 128), f32)

    def d1(i):
        xn = _ln(x_v[i * TM:(i + 1) * TM, :].astype(f32)).astype(bf16)
        h = _gelu(_dot(xn, w1_v[...]))
        for j in range(NT):
            h_v[j, PAD + i * TM:PAD + (i + 1) * TM, :] = h[:, j * 128:(j + 1) * 128]

    shifts = (1, 1, -1, -1, 2, 2, -2, -2)

    def d2(i):
        hs = jnp.concatenate(
            [h_v[j, pl.ds(PAD + i * TM - shifts[j], TM), :].astype(bf16) for j in range(NT)], axis=1)
        x1 = x_v[i * TM:(i + 1) * TM, :].astype(f32) + _dot(hs, w2_v[...])
        b_v[i * TM:(i + 1) * TM, :] = x1
        xn_v[i * TM // 2:(i + 1) * TM // 2, :] = pltpu.bitcast(_ln(x1).astype(bf16), u32)

    x_copy(0).wait()
    w_copies[0].wait()
    for i in range(1, 5):
        x_copy(i).start()
    d1(0)
    for i in range(1, 5):
        x_copy(i).wait()
    for i in range(5, NB):
        x_copy(i).start()
    w_copies[1].start()
    d1(1)
    d1(2)
    for i in range(5, NB):
        x_copy(i).wait()
    w_copies[1].wait()
    w_copies[2].start()
    w_copies[3].start()
    qkv_start(0)
    qkv_start(1)
    for i in range(3, NB + 3):
        d2(i - 3)
        if i < NB:
            d1(i)

    w_copies[2].wait()
    w_copies[3].wait()
    for cp in wo_copies():
        cp.start()

    def ffn(i, carry):
        qkv_wait(i)

        @pl.when(i + 2 < NG)
        def _():
            qkv_start(i + 2)

        r0 = pl.multiple_of(i * TM, TM)
        xn = pltpu.bitcast(xn_v[pl.ds(pl.multiple_of(i * (TM // 2), TM // 2), TM // 2), :], bf16)
        hs = {}

        def d3(c):
            hs[c] = _gelu(_dot(xn, w3_v[:, c * FC:(c + 1) * FC])).astype(bf16)

        def relayout(p):
            s0 = i * SPG + 2 * p
            for r in range(0, D // 2, 8):
                e = wqkv_v[s0, r:r + 8, :]
                o = wqkv_v[s0 + 1, r:r + 8, :]
                wqkv_v[s0, r:r + 8, :] = (e & jnp.uint32(0xFFFF)) | (o << 16)
                wqkv_v[s0 + 1, r:r + 8, :] = (e >> 16) | (o & jnp.uint32(0xFFFF0000))

        acc = b_v[pl.ds(r0, TM), :]
        d3(0)
        for c in range(NFC):
            if c + 1 < NFC:
                d3(c + 1)
            if c < SPG // 2:
                relayout(c)
            acc = _dot(hs.pop(c), w4_v[c * FC:(c + 1) * FC, :]) + acc
        b_v[pl.ds(r0, TM), :] = acc
        return carry

    lax.fori_loop(0, NB, ffn, 0)

    for cp in wo_copies():
        cp.wait()
    mem_v[...] = mem0_ref[...].astype(f32)

    def wload(w, h):
        return pltpu.bitcast(wqkv_v[(h // G) * SPG + w * G + h % G], bf16)

    def step(hq, hkv, odd, allow, fill):
        nq = hq.shape[0]
        qs, ks, vs, ps = {}, {}, {}, {}

        def proj(g):
            for h in range(g * G, (g + 1) * G):
                qs[h] = _dot(hq, wload(0, h)).astype(bf16)
                k = _dot(hkv, wload(1, h)).astype(bf16)
                v = _dot(hkv, wload(2, h)).astype(bf16)
                if odd:
                    k = jnp.concatenate([pltpu.bitcast(ke_v[h], bf16), k], axis=0)
                    v = jnp.concatenate([pltpu.bitcast(ve_v[h], bf16), v], axis=0)
                else:
                    ke_v[h] = pltpu.bitcast(k, u32)
                    ve_v[h] = pltpu.bitcast(v, u32)
                ks[h] = k
                vs[h] = v

        def score(g):
            for h in range(g * G, (g + 1) * G):
                s = lax.dot_general(qs.pop(h), ks.pop(h), (((1,), (1,)), ((), ())),
                                    preferred_element_type=f32)
                ps[h] = _softmax(s, allow, fill)

        def pv(g):
            for h in range(g * G, (g + 1) * G):
                o = _dot(ps.pop(h), vs.pop(h)).astype(bf16)
                o_v[0:nq // 2, h * 128:(h + 1) * 128] = pltpu.bitcast(o, u32)

        acc = [None] * NT

        def wo(h0, h1, j0, j1):
            o = pltpu.bitcast(o_v[0:nq // 2, h0 * 128:h1 * 128], bf16)
            for j in range(j0, j1):
                y = _dot(o, pltpu.bitcast(wo_v[j, h0 * 64:h1 * 64, :], bf16))
                acc[j] = y if acc[j] is None else y + acc[j]

        for t in range(NG):
            proj(t)
            if t >= 1:
                score(t - 1)
            if t >= 2:
                pv(t - 2)
        wo(0, 16, 0, 4)
        score(NG - 1)
        pv(NG - 2)
        wo(0, 16, 4, 8)
        pv(NG - 1)
        wo(16, 24, 0, 8)
        wo(24, 32, 0, 8)
        return jnp.concatenate(acc, axis=1)

    def out_copy(j, slot):
        r0 = pl.multiple_of(j * 64, 64)
        return pltpu.make_async_copy(out_v.at[slot], out_hbm.at[pl.ds(r0, 64)], sem_out.at[slot])

    def pair(j, carry):
        slot = j % 2

        @pl.when(j >= 2)
        def _():
            out_copy(j - 2, slot).wait()

        allow_e, fill_e, allow_o, fill_o = _masks()
        r0 = pl.multiple_of(j * 64, 64)
        x0 = x_v[pl.ds(r0, 16), :]
        x1 = x_v[pl.ds(r0 + 16, 16), :]
        x2 = x_v[pl.ds(r0 + 32, 16), :]
        x3 = x_v[pl.ds(r0 + 48, 16), :]
        x1f = x1.astype(f32)
        x2f = x2.astype(f32)
        mem = mem_v[...]
        hq = jnp.concatenate([x0, jnp.concatenate([x1f[:8], mem], 0).astype(bf16)], 0)
        hkv = jnp.concatenate([x0, x1, jnp.concatenate([x2f[:8], mem], 0).astype(bf16)], 0)
        oe = step(hq, hkv, False, allow_e, fill_e)
        mem = oe[24:32]
        hq = jnp.concatenate([jnp.concatenate([x1f[8:], mem], 0).astype(bf16), x2, x3], 0)
        hkv = jnp.concatenate([jnp.concatenate([mem, x2f[8:]], 0).astype(bf16), x3], 0)
        oo = step(hq, hkv, True, allow_o, fill_o)
        mem_v[...] = oo[8:16]
        a = jnp.concatenate([oe[:24], oo[:8], oo[16:]], 0)
        xf = x_v[pl.ds(r0, 64), :].astype(f32)
        gw = gw_ref[...].astype(f32)
        gw = jnp.concatenate([gw[t:t + 1, :] for t in range(NT)], axis=1)
        g = jax.nn.sigmoid(jnp.sum(xf * gw, axis=-1, keepdims=True))
        out_v[slot] = (g * a + (1.0 - g) * b_v[pl.ds(r0, 64), :]).astype(bf16)
        out_copy(j, slot).start()
        return carry

    lax.fori_loop(0, NPAIR, pair, 0)
    out_copy(NPAIR - 2, 0).wait()
    out_copy(NPAIR - 1, 1).wait()


@functools.partial(jax.jit, static_argnames=("A_seg_len",))
def pallas_gated_mix__memory_aug_recurrent_mem_tr__mixer_s_mlp__prompt_kernel(
    A_x, A_mem0, A_Wq, A_Wk, A_Wv, A_Wo, A_seg_len, B_x, B_w1, B_w2, B_w3, B_w4, gate_w,
):
    assert A_seg_len == SEG
    assert A_x.shape == (1, S, D) and A_mem0.shape == (1, M, D)
    any_spec = pl.BlockSpec(memory_space=pl.ANY)
    vmem_spec = pl.BlockSpec(memory_space=pltpu.VMEM)
    out = pl.pallas_call(
        _kernel,
        out_shape=jax.ShapeDtypeStruct((S, D), bf16),
        in_specs=[any_spec, vmem_spec] + [any_spec] * 8 + [vmem_spec],
        out_specs=any_spec,
        scratch_shapes=[
            pltpu.VMEM((S, D), bf16),
            pltpu.VMEM((D, D), bf16),
            pltpu.VMEM((D, D), bf16),
            pltpu.VMEM((D, F), bf16),
            pltpu.VMEM((F, D), bf16),
            pltpu.VMEM((3 * H, D // 2, DH), u32),
            pltpu.VMEM((NT, H * DH // 2, 128), u32),
            pltpu.VMEM((NT, S + 2 * PAD, 128), f32),
            pltpu.VMEM((S, D), f32),
            pltpu.VMEM((S // 2, D), u32),
            pltpu.VMEM((2, 64, D), bf16),
            pltpu.VMEM((H, 24, 128), u32),
            pltpu.VMEM((H, 24, 128), u32),
            pltpu.VMEM((24, H * DH), u32),
            pltpu.VMEM((M, D), f32),
            pltpu.SemaphoreType.DMA((NB,)),
            pltpu.SemaphoreType.DMA((4,)),
            pltpu.SemaphoreType.DMA((NB,)),
            pltpu.SemaphoreType.DMA,
            pltpu.SemaphoreType.DMA((2,)),
        ],
        compiler_params=pltpu.CompilerParams(vmem_limit_bytes=120 * 1024 * 1024),
    )(
        A_x.reshape(S, D), A_mem0.reshape(M, D),
        A_Wq.reshape(D // 2, 2 * H, DH), A_Wk.reshape(D // 2, 2 * H, DH), A_Wv.reshape(D // 2, 2 * H, DH),
        A_Wo.reshape(H * DH, D), B_w1, B_w2, B_w3, B_w4, gate_w.reshape(NT, 128),
    )
    return out.reshape(1, S, D)
```

```python
import functools

import jax
import jax.numpy as jnp
from jax import lax
import jax.experimental.pallas as pl
import jax.experimental.pallas.tpu as pltpu

f32, bf16, u32 = jnp.float32, jnp.bfloat16, jnp.uint32

S, D, H, DH, M, SEG, F = 2048, 1024, 32, 128, 8, 32, 3584
SCALE = DH ** -0.5
NEG = -1000000000.0
EPS = 1e-05

TM = 256
NB = S // TM
FC = 512
NFC = F // FC
NPAIR = S // (2 * SEG)
G = 4
NG = H // G
PAD = 8
NT = D // 128
assert NB == NG

_dot = functools.partial(jnp.dot, preferred_element_type=f32)


def _ln(x):
    m = jnp.mean(x, axis=-1, keepdims=True)
    xc = x - m
    v = jnp.mean(xc * xc, axis=-1, keepdims=True)
    return xc * lax.rsqrt(v + EPS)


def _gelu(x):
    return jax.nn.gelu(x, approximate=True)


def _masks():
    r = lax.broadcasted_iota(jnp.int32, (32, 48), 0)
    c = lax.broadcasted_iota(jnp.int32, (32, 48), 1)
    exist_e = (c >= 40) | (c < 32)
    allow_e = (c >= 40) | ((c < 32) & ((r >= 24) | (c <= r)))
    fill_e = jnp.where(exist_e, NEG, -jnp.inf).astype(f32)
    r = lax.broadcasted_iota(jnp.int32, (48, 80), 0)
    c = lax.broadcasted_iota(jnp.int32, (48, 80), 1)
    keys_even = (c < 32) | ((c >= 40) & (c < 48))
    exist_o = ((r < 8) & keys_even) | ((r >= 8) & ~keys_even)
    ktok = jnp.where(c < 40, c, c - 16)
    qtok = jnp.where(r < 8, r + 24, r + 16)
    is_mem_key = (c >= 40) & (c < 56)
    is_mem_q = (r >= 8) & (r < 16)
    allow_o = exist_o & (is_mem_key | is_mem_q | (ktok <= qtok))
    fill_o = jnp.where(exist_o, NEG, -jnp.inf).astype(f32)
    return allow_e, fill_e, allow_o, fill_o


def _softmax(s, allow, fill):
    s = jnp.where(allow, s * SCALE, fill)
    m = jnp.max(s, axis=-1, keepdims=True)
    e = jnp.exp(s - m)
    l = jnp.sum(e, axis=-1, keepdims=True)
    return (e * pl.reciprocal(l, approx=False)).astype(bf16)


def _kernel(x_hbm, mem0_ref, wq_hbm, wk_hbm, wv_hbm, wo_hbm, w1_hbm, w2_hbm, w3_hbm, w4_hbm,
            gw_ref, out_hbm,
            x_v, w1_v, w2_v, w3_v, w4_v, wqkv_v, wo_v, h_v, b_v, xn_v, out_v,
            ke_v, ve_v, o_v, mem_v, zero_s,
            sem_x, sem_w, sem_qkv, sem_wo, sem_out):
    def x_copy(i):
        return pltpu.make_async_copy(x_hbm.at[pl.ds(i * TM, TM)], x_v.at[pl.ds(i * TM, TM)], sem_x.at[i])

    w_copies = [pltpu.make_async_copy(src, dst, sem_w.at[i]) for i, (src, dst) in enumerate(
        [(w1_hbm, w1_v), (w2_hbm, w2_v), (w3_hbm, w3_v), (w4_hbm, w4_v)])]

    SPG = 3 * G

    def qkv_start(g):
        for w, w_hbm in enumerate((wq_hbm, wk_hbm, wv_hbm)):
            wu = w_hbm.bitcast(u32)
            for k in range(G // 2):
                for par in range(2):
                    pltpu.make_async_copy(
                        wu.at[:, par * (H // 2) + g * (G // 2) + k, :],
                        wqkv_v.at[g * SPG + w * G + 2 * k + par], sem_qkv.at[g]).start()

    def qkv_wait(g):
        grp = wqkv_v.at[pl.ds(g * SPG, SPG)]
        pltpu.make_async_copy(grp, grp, sem_qkv.at[g]).wait()

    def wo_copies():
        wu = wo_hbm.bitcast(u32)
        return [pltpu.make_async_copy(wu.at[:, pl.ds(j * 128, 128)], wo_v.at[j], sem_wo)
                for j in range(NT)]

    x_copy(0).start()
    w_copies[0].start()
    zero_s[0] = 0

    h_v[:, 0:PAD, :] = jnp.zeros((NT, PAD, 128), f32)
    h_v[:, PAD + S:PAD + S + PAD, :] = jnp.zeros((NT, PAD, 128), f32)

    def d1(i):
        xn = _ln(x_v[i * TM:(i + 1) * TM, :].astype(f32)).astype(bf16)
        h = _gelu(_dot(xn, w1_v[...]))
        for j in range(NT):
            h_v[j, PAD + i * TM:PAD + (i + 1) * TM, :] = h[:, j * 128:(j + 1) * 128]

    shifts = (1, 1, -1, -1, 2, 2, -2, -2)

    def d2(i):
        hs = jnp.concatenate(
            [h_v[j, pl.ds(PAD + i * TM - shifts[j], TM), :].astype(bf16) for j in range(NT)], axis=1)
        x1 = x_v[i * TM:(i + 1) * TM, :].astype(f32) + _dot(hs, w2_v[...])
        b_v[i * TM:(i + 1) * TM, :] = x1
        xn_v[i * TM // 2:(i + 1) * TM // 2, :] = pltpu.bitcast(_ln(x1).astype(bf16), u32)

    x_copy(0).wait()
    w_copies[0].wait()
    for i in range(1, 5):
        x_copy(i).start()
    d1(0)
    for i in range(1, 5):
        x_copy(i).wait()
    for i in range(5, NB):
        x_copy(i).start()
    w_copies[1].start()
    d1(1)
    d1(2)
    for i in range(5, NB):
        x_copy(i).wait()
    w_copies[1].wait()
    w_copies[2].start()
    w_copies[3].start()
    qkv_start(0)
    qkv_start(1)
    for i in range(3, NB + 3):
        d2(i - 3)
        if i < NB:
            d1(i)

    w_copies[2].wait()
    w_copies[3].wait()
    for cp in wo_copies():
        cp.start()

    def ffn(i, carry):
        qkv_wait(i)
        r0 = pl.multiple_of(i * TM, TM)
        xn = pltpu.bitcast(xn_v[pl.ds(pl.multiple_of(i * (TM // 2), TM // 2), TM // 2), :], bf16)
        hs = {}

        def d3(c):
            hs[c] = _gelu(_dot(xn, w3_v[:, c * FC:(c + 1) * FC])).astype(bf16)

        def relayout(p):
            s0 = i * SPG + 2 * p
            for r in range(0, D // 2, 8):
                e = wqkv_v[s0, r:r + 8, :]
                o = wqkv_v[s0 + 1, r:r + 8, :]
                wqkv_v[s0, r:r + 8, :] = (e & jnp.uint32(0xFFFF)) | (o << 16)
                wqkv_v[s0 + 1, r:r + 8, :] = (e >> 16) | (o & jnp.uint32(0xFFFF0000))

        acc = b_v[pl.ds(r0, TM), :]
        d3(0)
        for c in range(NFC):
            if c + 1 < NFC:
                d3(c + 1)
            hc = hs.pop(c)
            if c < SPG // 2:
                relayout(c)
                z = pl.multiple_of(zero_s[0], 8)
                dummy = pltpu.bitcast(wqkv_v[i * SPG + zero_s[0], pl.ds(z, 8), :], bf16)
                t = jnp.where(zero_s[0] > 0, dummy, hc[-16:, -128:])
                hc = jnp.concatenate([hc[:-16], jnp.concatenate([hc[-16:, :-128], t], axis=1)], axis=0)
            acc = _dot(hc, w4_v[c * FC:(c + 1) * FC, :]) + acc
        b_v[pl.ds(r0, TM), :] = acc

        @pl.when(i + 2 < NG)
        def _():
            qkv_start(i + 2)

        return carry

    lax.fori_loop(0, NB, ffn, 0)

    for cp in wo_copies():
        cp.wait()
    mem_v[...] = mem0_ref[...].astype(f32)

    def wload(w, h):
        return pltpu.bitcast(wqkv_v[(h // G) * SPG + w * G + h % G], bf16)

    def step(hq, hkv, odd, allow, fill):
        nq = hq.shape[0]
        qs, ks, vs, ps = {}, {}, {}, {}

        def proj(g):
            for h in range(g * G, (g + 1) * G):
                qs[h] = _dot(hq, wload(0, h)).astype(bf16)
                k = _dot(hkv, wload(1, h)).astype(bf16)
                v = _dot(hkv, wload(2, h)).astype(bf16)
                if odd:
                    k = jnp.concatenate([pltpu.bitcast(ke_v[h], bf16), k], axis=0)
                    v = jnp.concatenate([pltpu.bitcast(ve_v[h], bf16), v], axis=0)
                else:
                    ke_v[h] = pltpu.bitcast(k, u32)
                    ve_v[h] = pltpu.bitcast(v, u32)
                ks[h] = k
                vs[h] = v

        def score(g):
            for h in range(g * G, (g + 1) * G):
                s = lax.dot_general(qs.pop(h), ks.pop(h), (((1,), (1,)), ((), ())),
                                    preferred_element_type=f32)
                ps[h] = _softmax(s, allow, fill)

        def pv(g):
            for h in range(g * G, (g + 1) * G):
                o = _dot(ps.pop(h), vs.pop(h)).astype(bf16)
                o_v[0:nq // 2, h * 128:(h + 1) * 128] = pltpu.bitcast(o, u32)

        acc = [None] * NT

        def wo(h0, h1, j0, j1):
            o = pltpu.bitcast(o_v[0:nq // 2, h0 * 128:h1 * 128], bf16)
            for j in range(j0, j1):
                y = _dot(o, pltpu.bitcast(wo_v[j, h0 * 64:h1 * 64, :], bf16))
                acc[j] = y if acc[j] is None else y + acc[j]

        for t in range(NG):
            proj(t)
            if t >= 1:
                score(t - 1)
            if t >= 2:
                pv(t - 2)
        wo(0, 16, 0, 4)
        score(NG - 1)
        pv(NG - 2)
        wo(0, 16, 4, 8)
        pv(NG - 1)
        wo(16, 24, 0, 8)
        wo(24, 32, 0, 8)
        return jnp.concatenate(acc, axis=1)

    def out_copy(j, slot):
        r0 = pl.multiple_of(j * 64, 64)
        return pltpu.make_async_copy(out_v.at[slot], out_hbm.at[pl.ds(r0, 64)], sem_out.at[slot])

    def pair(j, carry):
        slot = j % 2

        @pl.when(j >= 2)
        def _():
            out_copy(j - 2, slot).wait()

        allow_e, fill_e, allow_o, fill_o = _masks()
        r0 = pl.multiple_of(j * 64, 64)
        x0 = x_v[pl.ds(r0, 16), :]
        x1 = x_v[pl.ds(r0 + 16, 16), :]
        x2 = x_v[pl.ds(r0 + 32, 16), :]
        x3 = x_v[pl.ds(r0 + 48, 16), :]
        x1f = x1.astype(f32)
        x2f = x2.astype(f32)
        mem = mem_v[...]
        hq = jnp.concatenate([x0, jnp.concatenate([x1f[:8], mem], 0).astype(bf16)], 0)
        hkv = jnp.concatenate([x0, x1, jnp.concatenate([x2f[:8], mem], 0).astype(bf16)], 0)
        oe = step(hq, hkv, False, allow_e, fill_e)
        mem = oe[24:32]
        hq = jnp.concatenate([jnp.concatenate([x1f[8:], mem], 0).astype(bf16), x2, x3], 0)
        hkv = jnp.concatenate([jnp.concatenate([mem, x2f[8:]], 0).astype(bf16), x3], 0)
        oo = step(hq, hkv, True, allow_o, fill_o)
        mem_v[...] = oo[8:16]
        a = jnp.concatenate([oe[:24], oo[:8], oo[16:]], 0)
        xf = x_v[pl.ds(r0, 64), :].astype(f32)
        gw = gw_ref[...].astype(f32)
        gw = jnp.concatenate([gw[t:t + 1, :] for t in range(NT)], axis=1)
        g = jax.nn.sigmoid(jnp.sum(xf * gw, axis=-1, keepdims=True))
        out_v[slot] = (g * a + (1.0 - g) * b_v[pl.ds(r0, 64), :]).astype(bf16)
        out_copy(j, slot).start()
        return carry

    lax.fori_loop(0, NPAIR, pair, 0)
    out_copy(NPAIR - 2, 0).wait()
    out_copy(NPAIR - 1, 1).wait()


@functools.partial(jax.jit, static_argnames=("A_seg_len",))
def pallas_gated_mix__memory_aug_recurrent_mem_tr__mixer_s_mlp__prompt_kernel(
    A_x, A_mem0, A_Wq, A_Wk, A_Wv, A_Wo, A_seg_len, B_x, B_w1, B_w2, B_w3, B_w4, gate_w,
):
    assert A_seg_len == SEG
    assert A_x.shape == (1, S, D) and A_mem0.shape == (1, M, D)
    any_spec = pl.BlockSpec(memory_space=pl.ANY)
    vmem_spec = pl.BlockSpec(memory_space=pltpu.VMEM)
    out = pl.pallas_call(
        _kernel,
        out_shape=jax.ShapeDtypeStruct((S, D), bf16),
        in_specs=[any_spec, vmem_spec] + [any_spec] * 8 + [vmem_spec],
        out_specs=any_spec,
        scratch_shapes=[
            pltpu.VMEM((S, D), bf16),
            pltpu.VMEM((D, D), bf16),
            pltpu.VMEM((D, D), bf16),
            pltpu.VMEM((D, F), bf16),
            pltpu.VMEM((F, D), bf16),
            pltpu.VMEM((3 * H, D // 2, DH), u32),
            pltpu.VMEM((NT, H * DH // 2, 128), u32),
            pltpu.VMEM((NT, S + 2 * PAD, 128), f32),
            pltpu.VMEM((S, D), f32),
            pltpu.VMEM((S // 2, D), u32),
            pltpu.VMEM((2, 64, D), bf16),
            pltpu.VMEM((H, 24, 128), u32),
            pltpu.VMEM((H, 24, 128), u32),
            pltpu.VMEM((24, H * DH), u32),
            pltpu.VMEM((M, D), f32),
            pltpu.SMEM((1,), jnp.int32),
            pltpu.SemaphoreType.DMA((NB,)),
            pltpu.SemaphoreType.DMA((4,)),
            pltpu.SemaphoreType.DMA((NB,)),
            pltpu.SemaphoreType.DMA,
            pltpu.SemaphoreType.DMA((2,)),
        ],
        compiler_params=pltpu.CompilerParams(vmem_limit_bytes=120 * 1024 * 1024,
                                             disable_bounds_checks=True),
    )(
        A_x.reshape(S, D), A_mem0.reshape(M, D),
        A_Wq.reshape(D // 2, 2 * H, DH), A_Wk.reshape(D // 2, 2 * H, DH), A_Wv.reshape(D // 2, 2 * H, DH),
        A_Wo.reshape(H * DH, D), B_w1, B_w2, B_w3, B_w4, gate_w.reshape(NT, 128),
    )
    return out.reshape(1, S, D)
```

```python
import functools

import jax
import jax.numpy as jnp
from jax import lax
import jax.experimental.pallas as pl
import jax.experimental.pallas.tpu as pltpu

f32, bf16, u32 = jnp.float32, jnp.bfloat16, jnp.uint32

S, D, H, DH, M, SEG, F = 2048, 1024, 32, 128, 8, 32, 3584
SCALE = DH ** -0.5
NEG = -1000000000.0
EPS = 1e-05

TM = 256
NB = S // TM
HM = TM // 2
DH2 = D // 2
FH = F // 2
FC = 256
NFC = FH // FC
NC1 = 256
NPAIR = S // (2 * SEG)
G = 4
NG = H // G
PAD = 8
NT = D // 128
assert NB == NG

_dot = functools.partial(jnp.dot, preferred_element_type=f32)


def _ln(x):
    m = jnp.mean(x, axis=-1, keepdims=True)
    xc = x - m
    v = jnp.mean(xc * xc, axis=-1, keepdims=True)
    return xc * lax.rsqrt(v + EPS)


def _gelu(x):
    return jax.nn.gelu(x, approximate=True)


def _lcombos(a11, a12, a21, a22):
    return [a11 + a22, a21 + a22, a11, a22, a11 + a12, a21 - a11, a12 - a22]


def _strassen(lhs, rhs, init=(None, None, None, None)):
    def add(a, b):
        return a if b is None else a + b
    p = [_dot(lhs(k), rhs(k)) for k in range(5)]
    c12 = add(p[2] + p[4], init[1])
    c21 = add(p[1] + p[3], init[2])
    c22 = _dot(lhs(5), rhs(5)) + add(p[0] - p[1] + p[2], init[3])
    c11 = _dot(lhs(6), rhs(6)) + add(p[0] + p[3] - p[4], init[0])
    return c11, c12, c21, c22


def _merge(*lists):
    keyed = [((j + 0.5) / len(l), n, j, v) for n, l in enumerate(lists) for j, v in enumerate(l)]
    return [v for _, _, _, v in sorted(keyed, key=lambda t: t[:3])]


def _masks():
    r = lax.broadcasted_iota(jnp.int32, (32, 48), 0)
    c = lax.broadcasted_iota(jnp.int32, (32, 48), 1)
    exist_e = (c >= 40) | (c < 32)
    allow_e = (c >= 40) | ((c < 32) & ((r >= 24) | (c <= r)))
    fill_e = jnp.where(exist_e, NEG, -jnp.inf).astype(f32)
    r = lax.broadcasted_iota(jnp.int32, (48, 80), 0)
    c = lax.broadcasted_iota(jnp.int32, (48, 80), 1)
    keys_even = (c < 32) | ((c >= 40) & (c < 48))
    exist_o = ((r < 8) & keys_even) | ((r >= 8) & ~keys_even)
    ktok = jnp.where(c < 40, c, c - 16)
    qtok = jnp.where(r < 8, r + 24, r + 16)
    is_mem_key = (c >= 40) & (c < 56)
    is_mem_q = (r >= 8) & (r < 16)
    allow_o = exist_o & (is_mem_key | is_mem_q | (ktok <= qtok))
    fill_o = jnp.where(exist_o, NEG, -jnp.inf).astype(f32)
    return allow_e, fill_e, allow_o, fill_o


def _softmax(s, allow, fill):
    s = jnp.where(allow, s * SCALE, fill)
    m = jnp.max(s, axis=-1, keepdims=True)
    e = jnp.exp(s - m)
    l = jnp.sum(e, axis=-1, keepdims=True)
    return (e * pl.reciprocal(l, approx=False)).astype(bf16)


def _kernel(x_hbm, mem0_hbm, wq_hbm, wk_hbm, wv_hbm, wo_hbm, w1_hbm, w2_hbm, w3_hbm, w4_hbm,
            gw_hbm, out_hbm,
            x_v, w1_v, w2_v, w3_v, w4_v, r1_v, r2_v, r3_v, r4_v, wqkv_v, wo_v, h_v, b_v, l_v, out_v,
            ke_v, ve_v, o_v, mem_v, mem0_ref, gw_ref, zero_s,
            sem, sem_qkv, sem_out):
    def rows(ref, r0, r1):
        return ref.at[pl.ds(r0, r1 - r0)]

    def cols(ref, c0, c1):
        return ref.at[:, pl.ds(c0, c1 - c0)]

    wo_u = wo_hbm.bitcast(u32)
    loads = dict(
        x01=(rows(x_hbm, 0, 2 * TM), rows(x_v, 0, 2 * TM)),
        w1a=(cols(w1_hbm, 0, 256), cols(w1_v, 0, 256)),
        w1bc=(cols(w1_hbm, 256, 768), cols(w1_v, 256, 768)),
        w1d=(cols(w1_hbm, 768, D), cols(w1_v, 768, D)),
        x234=(rows(x_hbm, 2 * TM, 5 * TM), rows(x_v, 2 * TM, 5 * TM)),
        x567=(rows(x_hbm, 5 * TM, S), rows(x_v, 5 * TM, S)),
        w2=(w2_hbm, w2_v), w3=(w3_hbm, w3_v), w4=(w4_hbm, w4_v),
        mem0=(mem0_hbm, mem0_ref), gw=(gw_hbm, gw_ref),
    )
    for j in range(NT):
        loads["wo%d" % j] = (cols(wo_u, j * 128, (j + 1) * 128), wo_v.at[j])
    cp = {k: pltpu.make_async_copy(src, dst, sem.at[n]) for n, (k, (src, dst)) in enumerate(loads.items())}

    SPG = 3 * G

    def qkv_start(g):
        for w, w_hbm in enumerate((wq_hbm, wk_hbm, wv_hbm)):
            wu = w_hbm.bitcast(u32)
            for k in range(G // 2):
                for par in range(2):
                    pltpu.make_async_copy(
                        wu.at[:, par * (H // 2) + g * (G // 2) + k, :],
                        wqkv_v.at[g * SPG + w * G + 2 * k + par], sem_qkv.at[g]).start(priority=1)

    def qkv_wait(g):
        grp = wqkv_v.at[pl.ds(g * SPG, SPG)]
        pltpu.make_async_copy(grp, grp, sem_qkv.at[g]).wait()

    for k in ("x01", "w1a", "w1bc", "w1d", "x234", "x567", "w2", "w3", "w4", "mem0", "gw"):
        cp[k].start()
    zero_s[0] = 0

    def probe(ref):
        z = zero_s[0]
        lead = (z,) * (len(ref.shape) - 2)
        if ref.dtype == u32:
            return pltpu.bitcast(ref[lead + (pl.ds(pl.multiple_of(z, 8), 8), slice(0, 128))], bf16)
        return ref[lead + (pl.ds(pl.multiple_of(z, 16), 16), slice(0, 128))]

    class Side:
        def __init__(self, pieces, n):
            self.pieces, self.n = list(pieces), n

        def __call__(self, val):
            if not self.pieces:
                return val
            take = -(-len(self.pieces) // self.n)
            self.n -= 1
            refs = []
            for fn, rs in self.pieces[:take]:
                fn()
                refs += [r for r in rs if not any(r is q for q in refs)]
            self.pieces = self.pieces[take:]
            t = val[-16:, -128:]
            for r in refs:
                t = jnp.where(zero_s[0] > 0, probe(r), t)
            return jnp.concatenate([val[:-16], jnp.concatenate([val[-16:, :-128], t], axis=1)], axis=0)

    def prep_pieces(w_v, r_v):
        k2, n2 = w_v.shape[0] // 2, w_v.shape[1] // 2
        inplace = r_v.shape[0] == 3

        def piece(r, c):
            b11 = w_v[r:r + 16, c:c + 256].astype(f32)
            b12 = w_v[r:r + 16, n2 + c:n2 + c + 256].astype(f32)
            b21 = w_v[k2 + r:k2 + r + 16, c:c + 256].astype(f32)
            b22 = w_v[k2 + r:k2 + r + 16, n2 + c:n2 + c + 256].astype(f32)
            r_v[0, r:r + 16, c:c + 256] = (b11 + b22).astype(bf16)
            r_v[1, r:r + 16, c:c + 256] = (b11 + b12).astype(bf16)
            r_v[2, r:r + 16, c:c + 256] = (b21 + b22).astype(bf16)
            if inplace:
                w_v[r:r + 16, n2 + c:n2 + c + 256] = (b12 - b22).astype(bf16)
                w_v[k2 + r:k2 + r + 16, c:c + 256] = (b21 - b11).astype(bf16)
            else:
                r_v[3, r:r + 16, c:c + 256] = (b12 - b22).astype(bf16)
                r_v[4, r:r + 16, c:c + 256] = (b21 - b11).astype(bf16)
        return [(functools.partial(piece, r, c), (w_v, r_v) if inplace else (r_v,))
                for r in range(0, k2, 16) for c in range(0, n2, 256)]

    def rhs_of(w_v, r_v, rs, cs):
        k2, n2 = w_v.shape[0] // 2, w_v.shape[1] // 2
        inplace = r_v.shape[0] == 3
        off = lambda sl, o: slice(sl.start + o, sl.stop + o)

        def rhs(k):
            if k == 0:
                return r_v[0, rs, cs]
            if k == 1:
                return w_v[rs, cs]
            if k == 2:
                return w_v[rs, off(cs, n2)] if inplace else r_v[3, rs, cs]
            if k == 3:
                return w_v[off(rs, k2), cs] if inplace else r_v[4, rs, cs]
            if k == 4:
                return w_v[off(rs, k2), off(cs, n2)]
            return r_v[k - 4, rs, cs]
        return rhs

    def lhs_pieces(rows_fn, r0, slot):
        def piece(q):
            top, bot = rows_fn(r0 + q), rows_fn(r0 + HM + q)
            for k, t in enumerate(_lcombos(top[:, :DH2], top[:, DH2:], bot[:, :DH2], bot[:, DH2:])):
                l_v[slot, k, q // 2:q // 2 + 8, :] = pltpu.bitcast(t.astype(bf16), u32)
        return [(functools.partial(piece, q), (l_v,)) for q in range(0, HM, 16)]

    def lhs_of(slot, side):
        return lambda k: side(pltpu.bitcast(l_v[slot, k], bf16))

    shifts = (1, 1, -1, -1, 2, 2, -2, -2)
    ln_x = lambda r: _ln(x_v[pl.ds(r, 16), :].astype(f32))
    ln_x1 = lambda r: _ln(b_v[pl.ds(r, 16), :])
    shifted_h = lambda r: jnp.concatenate(
        [h_v[j, pl.ds(PAD + r - shifts[j], 16), :] for j in range(NT)], axis=1)

    h_v[:, 0:PAD, :] = jnp.zeros((NT, PAD, 128), f32)
    h_v[:, PAD + S:PAD + S + PAD, :] = jnp.zeros((NT, PAD, 128), f32)

    def store_h(r0, c0, h):
        for j in range(h.shape[1] // 128):
            h_v[c0 // 128 + j, PAD + r0:PAD + r0 + h.shape[0], :] = h[:, j * 128:(j + 1) * 128]

    def d1_plain(xn, r0, c0, c1, step, side=lambda v: v):
        for c in range(c0, c1, step):
            store_h(r0, c, _gelu(_dot(side(xn), w1_v[:, c:c + step])))

    NP1 = 7 * (DH2 // NC1)

    def d1_s(b, slot, pieces):
        side = Side(pieces, NP1)
        for c in range(0, DH2, NC1):
            cs = _strassen(lhs_of(slot, side), rhs_of(w1_v, r1_v, slice(0, DH2), slice(c, c + NC1)))
            for q, t in enumerate(cs):
                store_h(b * TM + (q // 2) * HM, (q % 2) * DH2 + c, _gelu(t))

    def d2_s(b, slot, pieces):
        side = Side(pieces, NP1)
        for c in range(0, DH2, NC1):
            idx = [(slice(b * TM + (q // 2) * HM, b * TM + (q // 2 + 1) * HM),
                    slice((q % 2) * DH2 + c, (q % 2) * DH2 + c + NC1)) for q in range(4)]
            cs = _strassen(lhs_of(slot, side), rhs_of(w2_v, r2_v, slice(0, DH2), slice(c, c + NC1)),
                           [x_v[i].astype(f32) for i in idx])
            for i, t in zip(idx, cs):
                b_v[i] = t

    def split(l, n):
        return [l[len(l) * i // n:len(l) * (i + 1) // n] for i in range(n)]

    cp["x01"].wait()
    xn01 = _ln(x_v[0:2 * TM, :].astype(f32)).astype(bf16)
    cp["w1a"].wait()
    d1_plain(xn01, 0, 0, 256, 256)
    cp["w1bc"].wait()
    d1_plain(xn01, 0, 256, 768, 256)
    cp["w1d"].wait()
    cp["x234"].wait()
    d1_plain(xn01, 0, 768, D, 256)
    xn2 = _ln(x_v[2 * TM:3 * TM, :].astype(f32)).astype(bf16)
    d1_plain(xn2, 2 * TM, 0, D, 128,
             Side(_merge(prep_pieces(w1_v, r1_v), lhs_pieces(ln_x, 3 * TM, 1)), 8))
    d1_s(3, 1, lhs_pieces(ln_x, 4 * TM, 0))
    cp["x567"].wait()
    cp["w2"].wait()
    qkv_start(0)
    qkv_start(1)
    pw = split(prep_pieces(w2_v, r2_v), 4)
    for b in range(4, NB):
        nxt = lhs_pieces(ln_x, (b + 1) * TM, (b + 1) % 2) if b + 1 < NB else lhs_pieces(shifted_h, 0, 0)
        d1_s(b, b % 2, _merge(pw[b - 4], nxt))
    cp["w3"].wait()
    pw = split(prep_pieces(w3_v, r3_v), 4)
    for b in range(0, 4):
        d2_s(b, b % 2, _merge(pw[b], lhs_pieces(shifted_h, (b + 1) * TM, (b + 1) % 2)))
    cp["w4"].wait()
    for j in range(NT):
        cp["wo%d" % j].start()
    pw = split(prep_pieces(w4_v, r4_v), 4)
    for b in range(4, NB):
        nxt = lhs_pieces(shifted_h, (b + 1) * TM, (b + 1) % 2) if b + 1 < NB else lhs_pieces(ln_x1, 0, 0)
        d2_s(b, b % 2, _merge(pw[b - 4], nxt))

    def ffn(i, carry):
        qkv_wait(i)
        r0 = pl.multiple_of(i * TM, TM)
        rn = pl.multiple_of(jnp.minimum(i + 1, NB - 1) * TM, TM)
        slot = i % 2
        lh = {}
        acc = [None] * 7

        def relayout(p, r0_, r1_):
            s0 = i * SPG + 2 * p
            for r in range(r0_, r1_, 8):
                e = wqkv_v[s0, r:r + 8, :]
                o = wqkv_v[s0 + 1, r:r + 8, :]
                wqkv_v[s0, r:r + 8, :] = (e & jnp.uint32(0xFFFF)) | (o << 16)
                wqkv_v[s0 + 1, r:r + 8, :] = (e >> 16) | (o & jnp.uint32(0xFFFF0000))

        side3 = Side([(functools.partial(relayout, p, r, r + 64), (wqkv_v,))
                      for p in range(SPG // 2) for r in range(0, D // 2, 64)], 48)
        lp = lhs_pieces(ln_x1, rn, 1 - slot)

        def d3(c):
            cs = _strassen(lhs_of(slot, side3 if c > 0 else (lambda v: v)),
                           rhs_of(w3_v, r3_v, slice(0, DH2), slice(c * FC, (c + 1) * FC)))
            lh[c] = [t.astype(bf16) for t in _lcombos(*[_gelu(t) for t in cs])]

        def d4(c):
            l = lh.pop(c)
            rhs = rhs_of(w4_v, r4_v, slice(c * FC, (c + 1) * FC), slice(0, DH2))
            if c + 1 < NFC:
                for k in range(7):
                    lk = l[k]
                    if k in (3, 6) and lp:
                        lk = Side([lp.pop(0)], 1)(lk)
                    elif c == NFC - 2:
                        lk = side3(lk)
                    y = _dot(lk, rhs(k))
                    acc[k] = y if acc[k] is None else y + acc[k]
                return
            q = [_dot(l[k], rhs(k)) + acc[k] for k in range(5)]
            top, bot = pl.ds(r0, HM), pl.ds(r0 + HM, HM)
            b_v[top, DH2:] = q[2] + q[4] + b_v[top, DH2:]
            b_v[bot, :DH2] = q[1] + q[3] + b_v[bot, :DH2]
            b_v[bot, DH2:] = _dot(l[5], rhs(5)) + (acc[5] + q[0] - q[1] + q[2] + b_v[bot, DH2:])
            b_v[top, :DH2] = _dot(l[6], rhs(6)) + (acc[6] + q[0] + q[3] - q[4] + b_v[top, :DH2])

        d3(0)
        for c in range(NFC):
            if c + 1 < NFC:
                d3(c + 1)
            d4(c)
        assert not side3.pieces and not lp

        @pl.when(i + 2 < NG)
        def _():
            qkv_start(i + 2)

        return carry

    lax.fori_loop(0, NB, ffn, 0)

    for k in ["mem0", "gw"] + ["wo%d" % j for j in range(NT)]:
        cp[k].wait()
    mem_v[...] = mem0_ref[...].astype(f32)

    def wload(w, h):
        return pltpu.bitcast(wqkv_v[(h // G) * SPG + w * G + h % G], bf16)

    def step(hq, hkv, odd, allow, fill):
        nq = hq.shape[0]
        qs, ks, vs, ps = {}, {}, {}, {}

        def proj(g):
            for h in range(g * G, (g + 1) * G):
                qs[h] = _dot(hq, wload(0, h)).astype(bf16)
                k = _dot(hkv, wload(1, h)).astype(bf16)
                v = _dot(hkv, wload(2, h)).astype(bf16)
                if odd:
                    k = jnp.concatenate([pltpu.bitcast(ke_v[h], bf16), k], axis=0)
                    v = jnp.concatenate([pltpu.bitcast(ve_v[h], bf16), v], axis=0)
                else:
                    ke_v[h] = pltpu.bitcast(k, u32)
                    ve_v[h] = pltpu.bitcast(v, u32)
                ks[h] = k
                vs[h] = v

        def score(g):
            for h in range(g * G, (g + 1) * G):
                s = lax.dot_general(qs.pop(h), ks.pop(h), (((1,), (1,)), ((), ())),
                                    preferred_element_type=f32)
                ps[h] = _softmax(s, allow, fill)

        def pv(g):
            for h in range(g * G, (g + 1) * G):
                o = _dot(ps.pop(h), vs.pop(h)).astype(bf16)
                o_v[0:nq // 2, h * 128:(h + 1) * 128] = pltpu.bitcast(o, u32)

        acc = [None] * NT

        def wo(h0, h1, j0, j1):
            o = pltpu.bitcast(o_v[0:nq // 2, h0 * 128:h1 * 128], bf16)
            for j in range(j0, j1):
                y = _dot(o, pltpu.bitcast(wo_v[j, h0 * 64:h1 * 64, :], bf16))
                acc[j] = y if acc[j] is None else y + acc[j]

        for t in range(NG):
            proj(t)
            if t >= 1:
                score(t - 1)
            if t >= 2:
                pv(t - 2)
        wo(0, 16, 0, 4)
        score(NG - 1)
        pv(NG - 2)
        wo(0, 16, 4, 8)
        pv(NG - 1)
        wo(16, 24, 0, 8)
        wo(24, 32, 0, 8)
        return jnp.concatenate(acc, axis=1)

    def out_copy(j, slot):
        r0 = pl.multiple_of(j * 64, 64)
        return pltpu.make_async_copy(out_v.at[slot], out_hbm.at[pl.ds(r0, 64)], sem_out.at[slot])

    def pair(j, carry):
        slot = j % 2

        @pl.when(j >= 2)
        def _():
            out_copy(j - 2, slot).wait()

        allow_e, fill_e, allow_o, fill_o = _masks()
        r0 = pl.multiple_of(j * 64, 64)
        x0 = x_v[pl.ds(r0, 16), :]
        x1 = x_v[pl.ds(r0 + 16, 16), :]
        x2 = x_v[pl.ds(r0 + 32, 16), :]
        x3 = x_v[pl.ds(r0 + 48, 16), :]
        x1f = x1.astype(f32)
        x2f = x2.astype(f32)
        mem = mem_v[...]
        hq = jnp.concatenate([x0, jnp.concatenate([x1f[:8], mem], 0).astype(bf16)], 0)
        hkv = jnp.concatenate([x0, x1, jnp.concatenate([x2f[:8], mem], 0).astype(bf16)], 0)
        oe = step(hq, hkv, False, allow_e, fill_e)
        mem = oe[24:32]
        hq = jnp.concatenate([jnp.concatenate([x1f[8:], mem], 0).astype(bf16), x2, x3], 0)
        hkv = jnp.concatenate([jnp.concatenate([mem, x2f[8:]], 0).astype(bf16), x3], 0)
        oo = step(hq, hkv, True, allow_o, fill_o)
        mem_v[...] = oo[8:16]
        a = jnp.concatenate([oe[:24], oo[:8], oo[16:]], 0)
        xf = x_v[pl.ds(r0, 64), :].astype(f32)
        gw = gw_ref[...].astype(f32)
        gw = jnp.concatenate([gw[t:t + 1, :] for t in range(NT)], axis=1)
        g = jax.nn.sigmoid(jnp.sum(xf * gw, axis=-1, keepdims=True))
        out_v[slot] = (g * a + (1.0 - g) * b_v[pl.ds(r0, 64), :]).astype(bf16)
        out_copy(j, slot).start()
        return carry

    lax.fori_loop(0, NPAIR, pair, 0)
    out_copy(NPAIR - 2, 0).wait()
    out_copy(NPAIR - 1, 1).wait()


@functools.partial(jax.jit, static_argnames=("A_seg_len",))
def pallas_gated_mix__memory_aug_recurrent_mem_tr__mixer_s_mlp__prompt_kernel(
    A_x, A_mem0, A_Wq, A_Wk, A_Wv, A_Wo, A_seg_len, B_x, B_w1, B_w2, B_w3, B_w4, gate_w,
):
    assert A_seg_len == SEG
    assert A_x.shape == (1, S, D) and A_mem0.shape == (1, M, D)
    any_spec = pl.BlockSpec(memory_space=pl.ANY)
    out = pl.pallas_call(
        _kernel,
        out_shape=jax.ShapeDtypeStruct((S, D), bf16),
        in_specs=[any_spec] * 11,
        out_specs=any_spec,
        scratch_shapes=[
            pltpu.VMEM((S, D), bf16),
            pltpu.VMEM((D, D), bf16),
            pltpu.VMEM((D, D), bf16),
            pltpu.VMEM((D, F), bf16),
            pltpu.VMEM((F, D), bf16),
            pltpu.VMEM((5, D // 2, D // 2), bf16),
            pltpu.VMEM((3, D // 2, D // 2), bf16),
            pltpu.VMEM((3, D // 2, F // 2), bf16),
            pltpu.VMEM((3, F // 2, D // 2), bf16),
            pltpu.VMEM((3 * H, D // 2, DH), u32),
            pltpu.VMEM((NT, H * DH // 2, 128), u32),
            pltpu.VMEM((NT, S + 2 * PAD, 128), f32),
            pltpu.VMEM((S, D), f32),
            pltpu.VMEM((2, 7, HM // 2, D // 2), u32),
            pltpu.VMEM((2, 64, D), bf16),
            pltpu.VMEM((H, 24, 128), u32),
            pltpu.VMEM((H, 24, 128), u32),
            pltpu.VMEM((24, H * DH), u32),
            pltpu.VMEM((M, D), f32),
            pltpu.VMEM((M, D), bf16),
            pltpu.VMEM((NT, 128), bf16),
            pltpu.SMEM((1,), jnp.int32),
            pltpu.SemaphoreType.DMA((11 + NT,)),
            pltpu.SemaphoreType.DMA((NG,)),
            pltpu.SemaphoreType.DMA((2,)),
        ],
        compiler_params=pltpu.CompilerParams(vmem_limit_bytes=120 * 1024 * 1024,
                                             disable_bounds_checks=True),
    )(
        A_x.reshape(S, D), A_mem0.reshape(M, D),
        A_Wq.reshape(D // 2, 2 * H, DH), A_Wk.reshape(D // 2, 2 * H, DH), A_Wv.reshape(D // 2, 2 * H, DH),
        A_Wo.reshape(H * DH, D), B_w1, B_w2, B_w3, B_w4, gate_w.reshape(NT, 128),
    )
    return out.reshape(1, S, D)
```

```python
import functools

import jax
import jax.numpy as jnp
from jax import lax
import jax.experimental.pallas as pl
import jax.experimental.pallas.tpu as pltpu

f32, bf16, u32 = jnp.float32, jnp.bfloat16, jnp.uint32

S, D, H, DH, M, SEG, F = 2048, 1024, 32, 128, 8, 32, 3584
SCALE = DH ** -0.5
NEG = -1000000000.0
EPS = 1e-05

TM = 256
NB = S // TM
HM = TM // 2
DH2 = D // 2
FH = F // 2
FC = 256
NFC = FH // FC
NC1 = 128
NPAIR = S // (2 * SEG)
G = 4
NG = H // G
PAD = 8
NT = D // 128
NLOAD = 3 + 8 + 12 + 2 + NT
assert NB == NG

_dot = functools.partial(jnp.dot, preferred_element_type=f32)


def _ln(x):
    m = jnp.mean(x, axis=-1, keepdims=True)
    xc = x - m
    v = jnp.mean(xc * xc, axis=-1, keepdims=True)
    return xc * lax.rsqrt(v + EPS)


def _gelu(x):
    return jax.nn.gelu(x, approximate=True)


def _unpack(u):
    return pltpu.bitcast(u, bf16).astype(f32)


def _pack(x):
    return pltpu.bitcast(x.astype(bf16), u32)


def _lcombos(a11, a12, a21, a22):
    return [a11 + a22, a21 + a22, a11, a22, a11 + a12, a21 - a11, a12 - a22]


def _merge(*lists):
    keyed = [((j + 0.5) / len(l), n, j, v) for n, l in enumerate(lists) for j, v in enumerate(l)]
    return [v for _, _, _, v in sorted(keyed, key=lambda t: t[:3])]


def _masks():
    r = lax.broadcasted_iota(jnp.int32, (32, 48), 0)
    c = lax.broadcasted_iota(jnp.int32, (32, 48), 1)
    exist_e = (c >= 40) | (c < 32)
    allow_e = (c >= 40) | ((c < 32) & ((r >= 24) | (c <= r)))
    fill_e = jnp.where(exist_e, NEG, -jnp.inf).astype(f32)
    r = lax.broadcasted_iota(jnp.int32, (48, 80), 0)
    c = lax.broadcasted_iota(jnp.int32, (48, 80), 1)
    keys_even = (c < 32) | ((c >= 40) & (c < 48))
    exist_o = ((r < 8) & keys_even) | ((r >= 8) & ~keys_even)
    ktok = jnp.where(c < 40, c, c - 16)
    qtok = jnp.where(r < 8, r + 24, r + 16)
    is_mem_key = (c >= 40) & (c < 56)
    is_mem_q = (r >= 8) & (r < 16)
    allow_o = exist_o & (is_mem_key | is_mem_q | (ktok <= qtok))
    fill_o = jnp.where(exist_o, NEG, -jnp.inf).astype(f32)
    return allow_e, fill_e, allow_o, fill_o


def _softmax(s, allow, fill):
    s = jnp.where(allow, s * SCALE, fill)
    m = jnp.max(s, axis=-1, keepdims=True)
    e = jnp.exp(s - m)
    l = jnp.sum(e, axis=-1, keepdims=True)
    return (e * pl.reciprocal(l, approx=False)).astype(bf16)


def _kernel(x_hbm, mem0_hbm, wq_hbm, wk_hbm, wv_hbm, wo_hbm, w1_hbm, w2_hbm, w3_hbm, w4_hbm,
            gw_hbm, out_hbm,
            x_v, s1_v, s2_v, s3_v, s4_v, wqkv_v, wo_v, h_v, b_v, l_v, out_v,
            ke_v, ve_v, o_v, mem_v, mem0_ref, gw_ref, zero_s,
            sem, sem_qkv, sem_out):
    RAW = (1, 2, 3, 4)
    RAW1 = (1, 7, 8, 4)

    loads = []

    def rows_load(name, r0, r1):
        loads.append((name, x_hbm.at[pl.ds(r0, r1 - r0)], x_v.at[pl.ds(r0, r1 - r0)]))

    def quad_load(name, w_hbm, s_v, raw, q, c0=0, c1=None):
        k4, n2 = s_v.shape[1], s_v.shape[2]
        c1 = n2 if c1 is None else c1
        src = w_hbm.bitcast(u32).at[pl.ds((q // 2) * k4, k4), pl.ds((q % 2) * n2 + c0, c1 - c0)]
        loads.append((name, src, s_v.at[raw[q], :, pl.ds(c0, c1 - c0)]))

    rows_load("x01", 0, 2 * TM)
    for name, half, c0, c1 in (("w1a", 0, 0, 256), ("w1bc", 0, 256, 512), ("w1bc", 1, 0, 256), ("w1d", 1, 256, 512)):
        quad_load(name, w1_hbm, s1_v, RAW1, half, c0, c1)
        quad_load(name, w1_hbm, s1_v, RAW1, 2 + half, c0, c1)
    rows_load("x234", 2 * TM, 5 * TM)
    rows_load("x567", 5 * TM, S)
    for name, w_hbm, s_v in (("w2", w2_hbm, s2_v), ("w3", w3_hbm, s3_v), ("w4", w4_hbm, s4_v)):
        for q in range(4):
            quad_load(name, w_hbm, s_v, RAW, q)
    loads.append(("small", mem0_hbm, mem0_ref))
    loads.append(("small", gw_hbm, gw_ref))
    for j in range(NT):
        loads.append(("wo", wo_hbm.bitcast(u32).at[:, pl.ds(j * 128, 128)], wo_v.at[j]))
    assert len(loads) == NLOAD

    def start(*names):
        for n, (name, src, dst) in enumerate(loads):
            if name in names:
                pltpu.make_async_copy(src, dst, sem.at[n]).start()

    def wait(*names):
        for n, (name, src, dst) in enumerate(loads):
            if name in names:
                pltpu.make_async_copy(src, dst, sem.at[n]).wait()

    SPG = 3 * G

    def qkv_start(g):
        for w, w_hbm in enumerate((wq_hbm, wk_hbm, wv_hbm)):
            wu = w_hbm.bitcast(u32)
            for k in range(G // 2):
                for par in range(2):
                    pltpu.make_async_copy(
                        wu.at[:, par * (H // 2) + g * (G // 2) + k, :],
                        wqkv_v.at[g * SPG + w * G + 2 * k + par], sem_qkv.at[g]).start(priority=1)

    def qkv_wait(g):
        grp = wqkv_v.at[pl.ds(g * SPG, SPG)]
        pltpu.make_async_copy(grp, grp, sem_qkv.at[g]).wait()

    start("x01", "w1a", "w1bc", "w1d", "x234", "x567", "w2", "w3", "w4", "small")
    zero_s[0] = 0

    def tile_idx(ref):
        z = zero_s[0]
        n = 16 if ref.dtype == bf16 else 8
        return (z,) * (len(ref.shape) - 2) + (pl.ds(pl.multiple_of(z, n), n), slice(0, 128))

    hist = []

    def mm(lhs, rhs, side=None, acc=None):
        if side is not None:
            lhs = side(lhs)
        y = _dot(pltpu.bitcast(lhs, bf16), pltpu.bitcast(rhs, bf16))
        if acc is not None:
            y = y + acc
        hist.append(y)
        return y

    class Side:
        def __init__(self, pieces, n):
            self.pieces, self.n = list(pieces), n

        def __call__(self, val):
            take = -(-len(self.pieces) // self.n) if self.pieces else 0
            self.n -= 1
            if not take:
                return val
            never = zero_s[0] > 0
            ng = val.shape[0] // 8
            groups = [val[8 * m:8 * m + 8] for m in range(ng)]
            for j, (fn, rd, wr, lag) in enumerate(self.pieces[:take]):
                m = (j + 1) * ng // take - 1
                if len(hist) >= lag:
                    a = hist[-lag]
                    r0 = (16 * m) % a.shape[0]
                    a = (a[r0:r0 + 16, :128].astype(bf16) if rd.dtype == bf16 else
                         a[r0:r0 + 8, :128] if rd.dtype == f32 else pltpu.bitcast(a[r0:r0 + 8, :128], u32))
                    idx = tile_idx(rd)
                    rd[idx] = jnp.where(never, a, rd[idx])
                fn()
                t = jnp.where(never, wr[tile_idx(wr)], groups[m][:, -128:])
                groups[m] = jnp.concatenate([groups[m][:, :-128], t], axis=1)
            self.pieces = self.pieces[take:]
            return jnp.concatenate(groups, axis=0)

    def strassen(lhs, rhs, side, init=(None, None, None, None)):
        def add(a, b):
            return a if b is None else a + b
        p = [mm(lhs(k), rhs(k), side) for k in range(5)]
        c12 = add(p[2] + p[4], init[1])
        c21 = add(p[1] + p[3], init[2])
        c22 = mm(lhs(5), rhs(5), side, add(p[0] - p[1] + p[2], init[3]))
        c11 = mm(lhs(6), rhs(6), side, add(p[0] + p[3] - p[4], init[0]))
        return c11, c12, c21, c22

    def prep_pieces(s_v, raw, lag, width=256):
        def piece(r, c):
            idx = (slice(r, r + 8), slice(c, c + width))
            b11, b12, b21, b22 = [_unpack(s_v[(q,) + idx]) for q in raw]
            for k, t in ((0, b11 + b22), (2, b12 - b22), (3, b21 - b11), (5, b11 + b12), (6, b21 + b22)):
                s_v[(k,) + idx] = _pack(t)
        return [(functools.partial(piece, r, c), s_v, s_v, lag)
                for r in range(0, s_v.shape[1], 8) for c in range(0, s_v.shape[2], width)]

    def store_l(slot, q, c, quads):
        for k, t in enumerate(_lcombos(*quads)):
            l_v[slot, k, q // 2:q // 2 + 8, c:c + t.shape[1]] = _pack(t)

    def ln_pieces(src, r0, slot, lag):
        def piece(q):
            top = _ln(src[pl.ds(r0 + q, 16), :].astype(f32))
            bot = _ln(src[pl.ds(r0 + HM + q, 16), :].astype(f32))
            store_l(slot, q, 0, (top[:, :DH2], top[:, DH2:], bot[:, :DH2], bot[:, DH2:]))
        return [(functools.partial(piece, q), src, l_v, lag) for q in range(0, HM, 16)]

    shifts = (1, 1, -1, -1, 2, 2, -2, -2)

    def shift_pieces(r0, slot, lag):
        def piece(q, j):
            store_l(slot, q, j * 128, [h_v[jj, pl.ds(PAD + r0 + rr + q - shifts[jj], 16), :]
                                       for rr in (0, HM) for jj in (j, j + NT // 2)])
        return [(functools.partial(piece, q, j), h_v, l_v, lag)
                for q in range(0, HM, 16) for j in range(NT // 2)]

    def lhs_of(slot):
        return lambda k: l_v[slot, k]

    h_v[:, 0:PAD, :] = jnp.zeros((NT, PAD, 128), f32)
    h_v[:, PAD + S:PAD + S + PAD, :] = jnp.zeros((NT, PAD, 128), f32)

    def store_h(r0, c0, h):
        for j in range(h.shape[1] // 128):
            h_v[c0 // 128 + j, PAD + r0:PAD + r0 + h.shape[0], :] = h[:, j * 128:(j + 1) * 128]

    def d1_plain(xn, r0, c0, c1, step, side=None):
        for c in range(c0, c1, step):
            half, cc = c // DH2, c % DH2
            w = jnp.concatenate([s1_v[RAW1[half], :, cc:cc + step], s1_v[RAW1[2 + half], :, cc:cc + step]], axis=0)
            store_h(r0, c, _gelu(mm(xn, w, side)))

    NP1 = 7 * (DH2 // NC1)

    def d1_s(b, slot, pieces):
        side = Side(pieces, NP1)
        for c in range(0, DH2, NC1):
            cs = strassen(lhs_of(slot), lambda k: s1_v[k, :, c:c + NC1], side)
            for q, t in enumerate(cs):
                store_h(b * TM + (q // 2) * HM, (q % 2) * DH2 + c, _gelu(t))

    def d2_s(b, slot, pieces):
        side = Side(pieces, NP1)
        for c in range(0, DH2, NC1):
            idx = [(slice(b * TM + (q // 2) * HM, b * TM + (q // 2 + 1) * HM),
                    slice((q % 2) * DH2 + c, (q % 2) * DH2 + c + NC1)) for q in range(4)]
            cs = strassen(lhs_of(slot), lambda k: s2_v[k, :, c:c + NC1], side,
                          [x_v[i].astype(f32) for i in idx])
            for i, t in zip(idx, cs):
                b_v[i] = t

    def split(l, n):
        return [l[len(l) * i // n:len(l) * (i + 1) // n] for i in range(n)]

    LS, LL = 3, 5

    wait("x01")
    xn01 = _pack(_ln(x_v[0:2 * TM, :].astype(f32)))
    wait("w1a")
    d1_plain(xn01, 0, 0, 256, 256)
    wait("w1bc")
    d1_plain(xn01, 0, 256, 768, 256)
    wait("w1d", "x234")
    hist.clear()
    d1_plain(xn01, 0, 768, D, 128)
    xn2 = _pack(_ln(x_v[2 * TM:3 * TM, :].astype(f32)))
    d1_plain(xn2, 2 * TM, 0, D, 128,
             Side(_merge(prep_pieces(s1_v, RAW1, 1), ln_pieces(x_v, 3 * TM, 1, 2)), 8))
    d1_s(3, 1, ln_pieces(x_v, 4 * TM, 0, LL))
    wait("x567", "w2")
    qkv_start(0)
    qkv_start(1)
    hist.clear()
    pw = split(prep_pieces(s2_v, RAW, LS), 4)
    for b in range(4, NB):
        nxt = ln_pieces(x_v, (b + 1) * TM, (b + 1) % 2, LL) if b + 1 < NB else shift_pieces(0, 0, LS)
        d1_s(b, b % 2, _merge(pw[b - 4], nxt))
    wait("w3")
    hist.clear()
    pw = split(prep_pieces(s3_v, RAW, LS), 4)
    for b in range(0, 4):
        d2_s(b, b % 2, _merge(pw[b], shift_pieces((b + 1) * TM, (b + 1) % 2, LS)))
    wait("w4")
    start("wo")
    hist.clear()
    pw = split(prep_pieces(s4_v, RAW, LS), 4)
    for b in range(4, NB):
        nxt = shift_pieces((b + 1) * TM, (b + 1) % 2, LS) if b + 1 < NB else ln_pieces(b_v, 0, 0, LL)
        d2_s(b, b % 2, _merge(pw[b - 4], nxt))

    def ffn(i, carry):
        qkv_wait(i)
        r0 = pl.multiple_of(i * TM, TM)
        rn = pl.multiple_of(jnp.minimum(i + 1, NB - 1) * TM, TM)
        slot = i % 2
        lh = {}
        acc = [None] * 7
        hist.clear()

        def relayout(p, r0_, r1_):
            s0 = i * SPG + 2 * p
            for r in range(r0_, r1_, 8):
                e = wqkv_v[s0, r:r + 8, :]
                o = wqkv_v[s0 + 1, r:r + 8, :]
                wqkv_v[s0, r:r + 8, :] = (e & jnp.uint32(0xFFFF)) | (o << 16)
                wqkv_v[s0 + 1, r:r + 8, :] = (e >> 16) | (o & jnp.uint32(0xFFFF0000))

        side3 = Side([(functools.partial(relayout, p, r, r + 64), wqkv_v, wqkv_v, 2)
                      for p in range(SPG // 2) for r in range(0, D // 2, 64)], 48)
        lp = ln_pieces(b_v, rn, 1 - slot, 3)

        def d3(c):
            cs = strassen(lhs_of(slot), lambda k: s3_v[k, :, c * FC:(c + 1) * FC], side3 if c > 0 else None)
            lh[c] = [_pack(t) for t in _lcombos(*[_gelu(t) for t in cs])]

        def d4(c):
            l = lh.pop(c)
            rhs = lambda k: s4_v[k, c * FC // 2:(c + 1) * FC // 2, :]
            if c + 1 < NFC:
                for k in range(7):
                    side = None
                    if k in (3, 6) and lp:
                        side = Side([lp.pop(0)], 1)
                    elif c == NFC - 2:
                        side = side3
                    acc[k] = mm(l[k], rhs(k), side, acc[k])
                return
            q = [mm(l[k], rhs(k), None, acc[k]) for k in range(5)]
            top, bot = pl.ds(r0, HM), pl.ds(r0 + HM, HM)
            b_v[top, DH2:] = q[2] + q[4] + b_v[top, DH2:]
            b_v[bot, :DH2] = q[1] + q[3] + b_v[bot, :DH2]
            b_v[bot, DH2:] = mm(l[5], rhs(5), None, acc[5] + q[0] - q[1] + q[2] + b_v[bot, DH2:])
            b_v[top, :DH2] = mm(l[6], rhs(6), None, acc[6] + q[0] + q[3] - q[4] + b_v[top, :DH2])

        d3(0)
        for c in range(NFC):
            if c + 1 < NFC:
                d3(c + 1)
            d4(c)
        assert not side3.pieces and not lp

        @pl.when(i + 2 < NG)
        def _():
            qkv_start(i + 2)

        return carry

    lax.fori_loop(0, NB, ffn, 0)

    wait("small", "wo")
    mem_v[...] = mem0_ref[...].astype(f32)

    def wload(w, h):
        return pltpu.bitcast(wqkv_v[(h // G) * SPG + w * G + h % G], bf16)

    def step(hq, hkv, odd, allow, fill):
        nq = hq.shape[0]
        qs, ks, vs, ps = {}, {}, {}, {}

        def proj(g):
            for h in range(g * G, (g + 1) * G):
                qs[h] = _dot(hq, wload(0, h)).astype(bf16)
                k = _dot(hkv, wload(1, h)).astype(bf16)
                v = _dot(hkv, wload(2, h)).astype(bf16)
                if odd:
                    k = jnp.concatenate([pltpu.bitcast(ke_v[h], bf16), k], axis=0)
                    v = jnp.concatenate([pltpu.bitcast(ve_v[h], bf16), v], axis=0)
                else:
                    ke_v[h] = pltpu.bitcast(k, u32)
                    ve_v[h] = pltpu.bitcast(v, u32)
                ks[h] = k
                vs[h] = v

        def score(g):
            for h in range(g * G, (g + 1) * G):
                s = lax.dot_general(qs.pop(h), ks.pop(h), (((1,), (1,)), ((), ())),
                                    preferred_element_type=f32)
                ps[h] = _softmax(s, allow, fill)

        def pv(g):
            for h in range(g * G, (g + 1) * G):
                o = _dot(ps.pop(h), vs.pop(h)).astype(bf16)
                o_v[0:nq // 2, h * 128:(h + 1) * 128] = pltpu.bitcast(o, u32)

        acc = [None] * NT

        def wo(h0, h1, j0, j1):
            o = pltpu.bitcast(o_v[0:nq // 2, h0 * 128:h1 * 128], bf16)
            for j in range(j0, j1):
                y = _dot(o, pltpu.bitcast(wo_v[j, h0 * 64:h1 * 64, :], bf16))
                acc[j] = y if acc[j] is None else y + acc[j]

        for t in range(NG):
            proj(t)
            if t >= 1:
                score(t - 1)
            if t >= 2:
                pv(t - 2)
        wo(0, 16, 0, 4)
        score(NG - 1)
        pv(NG - 2)
        wo(0, 16, 4, 8)
        pv(NG - 1)
        wo(16, 24, 0, 8)
        wo(24, 32, 0, 8)
        return jnp.concatenate(acc, axis=1)

    def out_copy(j, slot):
        r0 = pl.multiple_of(j * 64, 64)
        return pltpu.make_async_copy(out_v.at[slot], out_hbm.at[pl.ds(r0, 64)], sem_out.at[slot])

    def pair(j, carry):
        slot = j % 2

        @pl.when(j >= 2)
        def _():
            out_copy(j - 2, slot).wait()

        allow_e, fill_e, allow_o, fill_o = _masks()
        r0 = pl.multiple_of(j * 64, 64)
        x0 = x_v[pl.ds(r0, 16), :]
        x1 = x_v[pl.ds(r0 + 16, 16), :]
        x2 = x_v[pl.ds(r0 + 32, 16), :]
        x3 = x_v[pl.ds(r0 + 48, 16), :]
        x1f = x1.astype(f32)
        x2f = x2.astype(f32)
        mem = mem_v[...]
        hq = jnp.concatenate([x0, jnp.concatenate([x1f[:8], mem], 0).astype(bf16)], 0)
        hkv = jnp.concatenate([x0, x1, jnp.concatenate([x2f[:8], mem], 0).astype(bf16)], 0)
        oe = step(hq, hkv, False, allow_e, fill_e)
        mem = oe[24:32]
        hq = jnp.concatenate([jnp.concatenate([x1f[8:], mem], 0).astype(bf16), x2, x3], 0)
        hkv = jnp.concatenate([jnp.concatenate([mem, x2f[8:]], 0).astype(bf16), x3], 0)
        oo = step(hq, hkv, True, allow_o, fill_o)
        mem_v[...] = oo[8:16]
        a = jnp.concatenate([oe[:24], oo[:8], oo[16:]], 0)
        xf = x_v[pl.ds(r0, 64), :].astype(f32)
        gw = gw_ref[...].astype(f32)
        gw = jnp.concatenate([gw[t:t + 1, :] for t in range(NT)], axis=1)
        g = jax.nn.sigmoid(jnp.sum(xf * gw, axis=-1, keepdims=True))
        out_v[slot] = (g * a + (1.0 - g) * b_v[pl.ds(r0, 64), :]).astype(bf16)
        out_copy(j, slot).start()
        return carry

    lax.fori_loop(0, NPAIR, pair, 0)
    out_copy(NPAIR - 2, 0).wait()
    out_copy(NPAIR - 1, 1).wait()


@functools.partial(jax.jit, static_argnames=("A_seg_len",))
def pallas_gated_mix__memory_aug_recurrent_mem_tr__mixer_s_mlp__prompt_kernel(
    A_x, A_mem0, A_Wq, A_Wk, A_Wv, A_Wo, A_seg_len, B_x, B_w1, B_w2, B_w3, B_w4, gate_w,
):
    assert A_seg_len == SEG
    assert A_x.shape == (1, S, D) and A_mem0.shape == (1, M, D)
    any_spec = pl.BlockSpec(memory_space=pl.ANY)
    out = pl.pallas_call(
        _kernel,
        out_shape=jax.ShapeDtypeStruct((S, D), bf16),
        in_specs=[any_spec] * 11,
        out_specs=any_spec,
        scratch_shapes=[
            pltpu.VMEM((S, D), bf16),
            pltpu.VMEM((9, D // 4, D // 2), u32),
            pltpu.VMEM((7, D // 4, D // 2), u32),
            pltpu.VMEM((7, D // 4, F // 2), u32),
            pltpu.VMEM((7, F // 4, D // 2), u32),
            pltpu.VMEM((3 * H, D // 2, DH), u32),
            pltpu.VMEM((NT, H * DH // 2, 128), u32),
            pltpu.VMEM((NT, S + 2 * PAD, 128), f32),
            pltpu.VMEM((S, D), f32),
            pltpu.VMEM((2, 7, HM // 2, D // 2), u32),
            pltpu.VMEM((2, 64, D), bf16),
            pltpu.VMEM((H, 24, 128), u32),
            pltpu.VMEM((H, 24, 128), u32),
            pltpu.VMEM((24, H * DH), u32),
            pltpu.VMEM((M, D), f32),
            pltpu.VMEM((M, D), bf16),
            pltpu.VMEM((NT, 128), bf16),
            pltpu.SMEM((1,), jnp.int32),
            pltpu.SemaphoreType.DMA((NLOAD,)),
            pltpu.SemaphoreType.DMA((NG,)),
            pltpu.SemaphoreType.DMA((2,)),
        ],
        compiler_params=pltpu.CompilerParams(vmem_limit_bytes=120 * 1024 * 1024,
                                             disable_bounds_checks=True),
    )(
        A_x.reshape(S, D), A_mem0.reshape(M, D),
        A_Wq.reshape(D // 2, 2 * H, DH), A_Wk.reshape(D // 2, 2 * H, DH), A_Wv.reshape(D // 2, 2 * H, DH),
        A_Wo.reshape(H * DH, D), B_w1, B_w2, B_w3, B_w4, gate_w.reshape(NT, 128),
    )
    return out.reshape(1, S, D)
```

```python
import functools

import jax
import jax.numpy as jnp
from jax import lax
import jax.experimental.pallas as pl
import jax.experimental.pallas.tpu as pltpu

f32, bf16, u32 = jnp.float32, jnp.bfloat16, jnp.uint32

S, D, H, DH, M, SEG, F = 2048, 1024, 32, 128, 8, 32, 3584
SCALE = DH ** -0.5
NEG = -1000000000.0
EPS = 1e-05

TM = 256
NB = S // TM
HM = TM // 2
DH2 = D // 2
FH = F // 2
FC = 256
NFC = FH // FC
NC1 = 128
NPAIR = S // (2 * SEG)
G = 4
NG = H // G
PAD = 8
NT = D // 128
NLOAD = 4 + 8 + 12 + 2 + NT
assert NB == NG

_dot = functools.partial(jnp.dot, preferred_element_type=f32)


def _ln(x):
    m = jnp.mean(x, axis=-1, keepdims=True)
    xc = x - m
    v = jnp.mean(xc * xc, axis=-1, keepdims=True)
    return xc * lax.rsqrt(v + EPS)


_GC = 0.7978845608028654


def _gelu(x):
    h = 0.5 * x
    return h + h * jnp.tanh(x * (_GC + (_GC * 0.044715) * (x * x)))


def _unpack(u):
    return pltpu.bitcast(u, bf16).astype(f32)


def _pack(x):
    return pltpu.bitcast(x.astype(bf16), u32)


def _lcombos(a11, a12, a21, a22):
    return [a11 + a22, a21 + a22, a11, a22, a11 + a12, a21 - a11, a12 - a22]


def _merge(*lists):
    keyed = [((j + 0.5) / len(l), n, j, v) for n, l in enumerate(lists) for j, v in enumerate(l)]
    return [v for _, _, _, v in sorted(keyed, key=lambda t: t[:3])]


def _masks():
    r = lax.broadcasted_iota(jnp.int32, (32, 48), 0)
    c = lax.broadcasted_iota(jnp.int32, (32, 48), 1)
    exist_e = (c >= 40) | (c < 32)
    allow_e = (c >= 40) | ((c < 32) & ((r >= 24) | (c <= r)))
    fill_e = jnp.where(exist_e, NEG, -jnp.inf).astype(f32)
    r = lax.broadcasted_iota(jnp.int32, (48, 80), 0)
    c = lax.broadcasted_iota(jnp.int32, (48, 80), 1)
    keys_even = (c < 32) | ((c >= 40) & (c < 48))
    exist_o = ((r < 8) & keys_even) | ((r >= 8) & ~keys_even)
    ktok = jnp.where(c < 40, c, c - 16)
    qtok = jnp.where(r < 8, r + 24, r + 16)
    is_mem_key = (c >= 40) & (c < 56)
    is_mem_q = (r >= 8) & (r < 16)
    allow_o = exist_o & (is_mem_key | is_mem_q | (ktok <= qtok))
    fill_o = jnp.where(exist_o, NEG, -jnp.inf).astype(f32)
    return allow_e, fill_e, allow_o, fill_o


def _softmax(s, allow, fill):
    s = jnp.where(allow, s * SCALE, fill)
    m = jnp.max(s, axis=-1, keepdims=True)
    e = jnp.exp(s - m)
    l = jnp.sum(e, axis=-1, keepdims=True)
    return (e * pl.reciprocal(l, approx=False)).astype(bf16)


def _kernel(x_hbm, mem0_hbm, wq_hbm, wk_hbm, wv_hbm, wo_hbm, w1_hbm, w2_hbm, w3_hbm, w4_hbm,
            gw_hbm, out_hbm,
            x_v, s1_v, s2_v, s3_v, s4_v, wqkv_v, wo_v, h_v, b_v, l_v, n_v, out_v,
            ke_v, ve_v, o_v, mem_v, mem0_ref, gw_ref, zero_s,
            sem, sem_qkv, sem_out):
    RAW = (1, 2, 3, 4)
    RAW1 = (1, 7, 8, 4)

    loads = []

    def rows_load(name, r0, r1):
        loads.append((name, x_hbm.at[pl.ds(r0, r1 - r0)], x_v.at[pl.ds(r0, r1 - r0)]))

    def quad_load(name, w_hbm, s_v, raw, q, c0=0, c1=None):
        k4, n2 = s_v.shape[1], s_v.shape[2]
        c1 = n2 if c1 is None else c1
        src = w_hbm.bitcast(u32).at[pl.ds((q // 2) * k4, k4), pl.ds((q % 2) * n2 + c0, c1 - c0)]
        loads.append((name, src, s_v.at[raw[q], :, pl.ds(c0, c1 - c0)]))

    rows_load("x0", 0, TM)
    rows_load("x1", TM, 2 * TM)
    for name, half, c0, c1 in (("w1a", 0, 0, 256), ("w1bc", 0, 256, 512), ("w1bc", 1, 0, 256), ("w1d", 1, 256, 512)):
        quad_load(name, w1_hbm, s1_v, RAW1, half, c0, c1)
        quad_load(name, w1_hbm, s1_v, RAW1, 2 + half, c0, c1)
    rows_load("x234", 2 * TM, 5 * TM)
    rows_load("x567", 5 * TM, S)
    for name, w_hbm, s_v in (("w2", w2_hbm, s2_v), ("w3", w3_hbm, s3_v), ("w4", w4_hbm, s4_v)):
        for q in range(4):
            quad_load(name, w_hbm, s_v, RAW, q)
    loads.append(("small", mem0_hbm, mem0_ref))
    loads.append(("small", gw_hbm, gw_ref))
    for j in range(NT):
        loads.append(("wo", wo_hbm.bitcast(u32).at[:, pl.ds(j * 128, 128)], wo_v.at[j]))
    assert len(loads) == NLOAD

    def start(*names, priority=0):
        for n, (name, src, dst) in enumerate(loads):
            if name in names:
                pltpu.make_async_copy(src, dst, sem.at[n]).start(priority=priority)

    def wait(*names):
        for n, (name, src, dst) in enumerate(loads):
            if name in names:
                pltpu.make_async_copy(src, dst, sem.at[n]).wait()

    SPG = 3 * G

    def qkv_start(g):
        for w, w_hbm in enumerate((wq_hbm, wk_hbm, wv_hbm)):
            wu = w_hbm.bitcast(u32)
            for k in range(G // 2):
                for par in range(2):
                    pltpu.make_async_copy(
                        wu.at[:, par * (H // 2) + g * (G // 2) + k, :],
                        wqkv_v.at[g * SPG + w * G + 2 * k + par], sem_qkv.at[g]).start(priority=1)

    def qkv_wait(g):
        grp = wqkv_v.at[pl.ds(g * SPG, SPG)]
        pltpu.make_async_copy(grp, grp, sem_qkv.at[g]).wait()

    start("x0", "x1", "w1a", "w1bc", "w1d", "x234", "x567", "w2", "w3", "w4", "small")
    zero_s[0] = 0

    def tile_idx(ref):
        z = zero_s[0]
        return (z,) * (len(ref.shape) - 2) + (pl.ds(pl.multiple_of(z, 8), 8), slice(0, 128))

    hist = []

    def mm(lhs, rhs, side=None, acc=None):
        if side is not None:
            lhs = side(lhs)
        lhs = pltpu.bitcast(lhs, bf16) if lhs.dtype == u32 else lhs.astype(bf16)
        y = _dot(lhs, pltpu.bitcast(rhs, bf16))
        if acc is not None:
            y = y + acc
        hist.append(y)
        return y

    class Side:
        def __init__(self, pieces, n):
            self.pieces, self.n = list(pieces), n

        def __call__(self, val):
            take = -(-len(self.pieces) // self.n) if self.pieces else 0
            self.n -= 1
            if not take:
                return val
            never = zero_s[0] > 0
            rg = 8 if val.dtype == u32 else 16
            ng = val.shape[0] // rg
            groups = [val[8 * m:8 * m + 8] for m in range(val.shape[0] // 8)]
            for j, (fn, rd, wr, lag) in enumerate(self.pieces[:take]):
                m = (j + 1) * ng // take - 1
                pin = lambda v: v
                if lag is not None and len(hist) >= lag:
                    r0 = (16 * m) % hist[-lag].shape[0]
                    a = hist[-lag][r0:r0 + 8, :128]
                    if rd is None:
                        def pin(v, a=a):
                            t = jnp.where(never, jnp.concatenate([a] * (v.shape[0] // 8), axis=0), v[:, :128])
                            return t if v.shape[1] == 128 else jnp.concatenate([t, v[:, 128:]], axis=1)
                    else:
                        idx = tile_idx(rd)
                        rd[idx] = jnp.where(never, pltpu.bitcast(a, rd.dtype), rd[idx])
                fn(pin)
                g = m * rg // 8
                t = jnp.where(never, pltpu.bitcast(wr[tile_idx(wr)], val.dtype), groups[g][:, -128:])
                groups[g] = jnp.concatenate([groups[g][:, :-128], t], axis=1)
            self.pieces = self.pieces[take:]
            return jnp.concatenate(groups, axis=0)

    def strassen(lhs, rhs, side, init=(None, None, None, None), ks=range(7)):
        def add(a, b):
            return a if b is None else a + b
        sd = lambda k: side if k in ks else None
        p = [mm(lhs(k), rhs(k), sd(k)) for k in range(5)]
        c12 = add(p[2] + p[4], init[1])
        c21 = add(p[1] + p[3], init[2])
        c22 = mm(lhs(5), rhs(5), sd(5), add(p[0] - p[1] + p[2], init[3]))
        c11 = mm(lhs(6), rhs(6), sd(6), add(p[0] + p[3] - p[4], init[0]))
        return c11, c12, c21, c22

    def prep_pieces(s_v, raw, lag, width=256):
        def piece(r, c, pin):
            idx = (slice(r, r + 8), slice(c, c + width))
            b11, b12, b21, b22 = [_unpack(s_v[(q,) + idx]) for q in raw]
            for k, t in ((0, b11 + b22), (2, b12 - b22), (3, b21 - b11), (5, b11 + b12), (6, b21 + b22)):
                s_v[(k,) + idx] = _pack(t)
        return [(functools.partial(piece, r, c), s_v, s_v, lag)
                for r in range(0, s_v.shape[1], 8) for c in range(0, s_v.shape[2], width)]

    def store_l(slot, q, c, quads, plain=False):
        for k, t in enumerate(quads if plain else _lcombos(*quads)):
            l_v[slot, k, q // 2:q // 2 + 8, c:c + t.shape[1]] = _pack(t)

    def ln_pieces(src, r0, slot, lag, plain=False, width=256, staged=False, clag=None):
        def norm(q, pin):
            n_v[q:q + 16, :] = _ln(pin(src[pl.ds(r0 + q, 16), :].astype(f32)))

        def comb(q, c, pin):
            store_l(slot, q, c, [n_v[rr + q:rr + q + 16, cc + c:cc + c + width]
                                 for rr in (0, HM) for cc in (0, DH2)], plain)
        norms = [[(functools.partial(norm, rr + q), None, n_v, lag) for rr in (0, HM)] for q in range(0, HM, 16)]
        combs = [[(functools.partial(comb, q, c), n_v, l_v, clag) for c in range(0, DH2, width)]
                 for q in range(0, HM, 16)]
        if staged:
            return sum(norms, []), sum(combs, [])
        out = list(norms[0])
        for a, b in zip(norms[1:] + [[]], combs):
            out += _merge(a, b) if a else b
        return out

    shifts = (1, 1, -1, -1, 2, 2, -2, -2)

    def shift_pieces(r0, slot, lag, by_value=False):
        def piece(q, j, pin):
            a = [h_v[jj, pl.ds(PAD + r0 + rr + q - shifts[jj], 16), :]
                 for rr in (0, HM) for jj in (j, j + NT // 2)]
            store_l(slot, q, j * 128, [pin(a[0]), a[1], a[2], pin(a[3])])
        return [(functools.partial(piece, q, j), None if by_value else h_v, l_v, lag)
                for q in range(0, HM, 16) for j in range(NT // 2)]

    def lhs_of(slot):
        return lambda k: l_v[slot, k]

    h_v[:, 0:PAD, :] = jnp.zeros((NT, PAD, 128), f32)
    h_v[:, PAD + S:PAD + S + PAD, :] = jnp.zeros((NT, PAD, 128), f32)

    def store_h(r0, c0, h):
        for j in range(h.shape[1] // 128):
            h_v[c0 // 128 + j, PAD + r0:PAD + r0 + h.shape[0], :] = h[:, j * 128:(j + 1) * 128]

    def d1_plain(xn, r0, c0, c1, step, side=None):
        for c in range(c0, c1, step):
            half, cc = c // DH2, c % DH2
            w = jnp.concatenate([s1_v[RAW1[half], :, cc:cc + step], s1_v[RAW1[2 + half], :, cc:cc + step]], axis=0)
            store_h(r0, c, _gelu(mm(xn, w, side)))

    NP1 = 7 * (DH2 // NC1)
    KS1 = (2, 3, 4, 5)

    def d1_s(b, slot, pieces):
        side = Side(pieces, len(KS1) * (DH2 // NC1))
        for c in range(0, DH2, NC1):
            cs = strassen(lhs_of(slot), lambda k: s1_v[k, :, c:c + NC1], side, ks=KS1)
            for q, t in enumerate(cs):
                store_h(b * TM + (q // 2) * HM, (q % 2) * DH2 + c, _gelu(t))

    def d2_s(b, slot, pieces):
        side = Side(pieces, NP1)
        for c in range(0, DH2, NC1):
            idx = [(slice(b * TM + (q // 2) * HM, b * TM + (q // 2 + 1) * HM),
                    slice((q % 2) * DH2 + c, (q % 2) * DH2 + c + NC1)) for q in range(4)]
            cs = strassen(lhs_of(slot), lambda k: s2_v[k, :, c:c + NC1], side,
                          [x_v[i].astype(f32) for i in idx])
            for i, t in zip(idx, cs):
                b_v[i] = t

    def split(l, n):
        return [l[len(l) * i // n:len(l) * (i + 1) // n] for i in range(n)]

    LS, LL = 3, 5

    wait("x0")
    xn0 = _pack(_ln(x_v[0:TM, :].astype(f32)))
    wait("x1")
    xn01 = jnp.concatenate([xn0, _pack(_ln(x_v[TM:2 * TM, :].astype(f32)))], axis=0)
    wait("w1a")
    d1_plain(xn01, 0, 0, 256, 256)
    wait("w1bc")
    d1_plain(xn01, 0, 256, 768, 256)
    wait("w1d", "x234")
    hist.clear()
    d1_plain(xn01, 0, 768, D, 128, Side(ln_pieces(x_v, 2 * TM, 0, None, plain=True), 2))
    xn2 = jnp.concatenate([jnp.concatenate([l_v[0, 2 * h], l_v[0, 2 * h + 1]], axis=1) for h in range(2)], axis=0)
    d1_plain(xn2, 2 * TM, 0, D, 128,
             Side(_merge(prep_pieces(s1_v, RAW1, 1), ln_pieces(x_v, 3 * TM, 1, 2)), 8))
    d1_s(3, 1, ln_pieces(x_v, 4 * TM, 0, LL))
    wait("x567", "w2")
    qkv_start(0)
    qkv_start(1)
    hist.clear()
    pw = split(prep_pieces(s2_v, RAW, LS), 4)
    for b in range(4, NB):
        nxt = ln_pieces(x_v, (b + 1) * TM, (b + 1) % 2, LL) if b + 1 < NB else shift_pieces(0, 0, LS, True)
        d1_s(b, b % 2, _merge(pw[b - 4], nxt))
    d2_s(0, 0, shift_pieces(TM, 1, LS, True))
    wait("w3")
    hist.clear()
    pw = split(prep_pieces(s3_v, RAW, LS), 4)
    for b in range(1, 5):
        d2_s(b, b % 2, _merge(pw[b - 1], shift_pieces((b + 1) * TM, (b + 1) % 2, LS)))
    wait("w4")
    hist.clear()
    pw = prep_pieces(s4_v, RAW, LS)
    pw = [pw[:82], pw[82:164], pw[164:]]
    for b in range(5, NB):
        nxt = shift_pieces((b + 1) * TM, (b + 1) % 2, LS) if b + 1 < NB else ln_pieces(b_v, 0, 0, LL)
        d2_s(b, b % 2, _merge(pw[b - 5], nxt))
    start("wo", priority=1)

    def ffn(i, carry):
        qkv_wait(i)
        r0 = pl.multiple_of(i * TM, TM)
        rn = pl.multiple_of(jnp.minimum(i + 1, NB - 1) * TM, TM)
        lh = {}
        acc = [None] * 7
        hist.clear()

        def relayout(p, r0_, r1_, pin):
            s0 = i * SPG + 2 * p
            for r in range(r0_, r1_, 8):
                e = wqkv_v[s0, r:r + 8, :]
                o = wqkv_v[s0 + 1, r:r + 8, :]
                wqkv_v[s0, r:r + 8, :] = (e & jnp.uint32(0xFFFF)) | (o << 16)
                wqkv_v[s0 + 1, r:r + 8, :] = (e >> 16) | (o & jnp.uint32(0xFFFF0000))

        side3 = Side([(functools.partial(relayout, p, r, r + 32), wqkv_v, wqkv_v, 2)
                      for p in range(SPG // 2) for r in range(0, D // 2, 32)], 42 + 5)
        norms, combs = ln_pieces(b_v, rn, 0, 3, staged=True, width=128, clag=2)
        side4 = Side(norms, 16)
        side5 = Side(combs, 11)

        def d3(c):
            cs = strassen(lhs_of(0), lambda k: s3_v[k, :, c * FC:(c + 1) * FC],
                          side3 if c > 0 else (lambda v: side3(v) if len(hist) >= 2 else v))
            lh[c] = _lcombos(*[_gelu(t) for t in cs])

        def d4(c):
            l = lh.pop(c)
            rhs = lambda k: s4_v[k, c * FC // 2:(c + 1) * FC // 2, :]
            if c + 1 < NFC:
                for k in range(7):
                    side = (side5 if k > 0 else None) if c == NFC - 2 else (side4 if k >= 3 else None)
                    acc[k] = mm(l[k], rhs(k), side, acc[k])
                return
            q = [mm(l[k], rhs(k), side5, acc[k]) for k in range(5)]
            top, bot = pl.ds(r0, HM), pl.ds(r0 + HM, HM)
            b_v[top, DH2:] = q[2] + q[4] + b_v[top, DH2:]
            b_v[bot, :DH2] = q[1] + q[3] + b_v[bot, :DH2]
            b_v[bot, DH2:] = mm(l[5], rhs(5), None, acc[5] + q[0] - q[1] + q[2] + b_v[bot, DH2:])
            b_v[top, :DH2] = mm(l[6], rhs(6), None, acc[6] + q[0] + q[3] - q[4] + b_v[top, :DH2])

        d3(0)
        for c in range(NFC):
            if c + 1 < NFC:
                d3(c + 1)
            d4(c)
        assert not side3.pieces and not side4.pieces and not side5.pieces

        @pl.when(i + 2 < NG)
        def _():
            qkv_start(i + 2)

        return carry

    lax.fori_loop(0, NB, ffn, 0)

    wait("small", "wo")
    mem_v[...] = mem0_ref[...].astype(f32)

    def wload(w, h):
        return pltpu.bitcast(wqkv_v[(h // G) * SPG + w * G + h % G], bf16)

    def step(hq, hkv, odd, allow, fill):
        nq = hq.shape[0]
        qs, ks, vs, ps = {}, {}, {}, {}

        def proj(g):
            for h in range(g * G, (g + 1) * G):
                qs[h] = _dot(hq, wload(0, h)).astype(bf16)
                k = _dot(hkv, wload(1, h)).astype(bf16)
                v = _dot(hkv, wload(2, h)).astype(bf16)
                if odd:
                    k = jnp.concatenate([pltpu.bitcast(ke_v[h], bf16), k], axis=0)
                    v = jnp.concatenate([pltpu.bitcast(ve_v[h], bf16), v], axis=0)
                else:
                    ke_v[h] = pltpu.bitcast(k, u32)
                    ve_v[h] = pltpu.bitcast(v, u32)
                ks[h] = k
                vs[h] = v

        def score(g):
            for h in range(g * G, (g + 1) * G):
                s = lax.dot_general(qs.pop(h), ks.pop(h), (((1,), (1,)), ((), ())),
                                    preferred_element_type=f32)
                ps[h] = _softmax(s, allow, fill)

        def pv(g):
            for h in range(g * G, (g + 1) * G):
                o = _dot(ps.pop(h), vs.pop(h)).astype(bf16)
                o_v[0:nq // 2, h * 128:(h + 1) * 128] = pltpu.bitcast(o, u32)

        acc = [None] * NT

        def wo(h0, h1, j0, j1):
            o = pltpu.bitcast(o_v[0:nq // 2, h0 * 128:h1 * 128], bf16)
            for j in range(j0, j1):
                y = _dot(o, pltpu.bitcast(wo_v[j, h0 * 64:h1 * 64, :], bf16))
                acc[j] = y if acc[j] is None else y + acc[j]

        for t in range(NG):
            proj(t)
            if t >= 1:
                score(t - 1)
            if t >= 2:
                pv(t - 2)
        wo(0, 16, 0, 4)
        score(NG - 1)
        pv(NG - 2)
        wo(0, 16, 4, 8)
        pv(NG - 1)
        wo(16, 24, 0, 8)
        wo(24, 32, 0, 8)
        return jnp.concatenate(acc, axis=1)

    def out_copy(j, slot):
        r0 = pl.multiple_of(j * 64, 64)
        return pltpu.make_async_copy(out_v.at[slot], out_hbm.at[pl.ds(r0, 64)], sem_out.at[slot])

    def pair(j, carry):
        slot = j % 2

        @pl.when(j >= 2)
        def _():
            out_copy(j - 2, slot).wait()

        allow_e, fill_e, allow_o, fill_o = _masks()
        r0 = pl.multiple_of(j * 64, 64)
        x0 = x_v[pl.ds(r0, 16), :]
        x1 = x_v[pl.ds(r0 + 16, 16), :]
        x2 = x_v[pl.ds(r0 + 32, 16), :]
        x3 = x_v[pl.ds(r0 + 48, 16), :]
        x1f = x1.astype(f32)
        x2f = x2.astype(f32)
        mem = mem_v[...]
        hq = jnp.concatenate([x0, jnp.concatenate([x1f[:8], mem], 0).astype(bf16)], 0)
        hkv = jnp.concatenate([x0, x1, jnp.concatenate([x2f[:8], mem], 0).astype(bf16)], 0)
        oe = step(hq, hkv, False, allow_e, fill_e)
        mem = oe[24:32]
        hq = jnp.concatenate([jnp.concatenate([x1f[8:], mem], 0).astype(bf16), x2, x3], 0)
        hkv = jnp.concatenate([jnp.concatenate([mem, x2f[8:]], 0).astype(bf16), x3], 0)
        oo = step(hq, hkv, True, allow_o, fill_o)
        mem_v[...] = oo[8:16]
        a = jnp.concatenate([oe[:24], oo[:8], oo[16:]], 0)
        xf = x_v[pl.ds(r0, 64), :].astype(f32)
        gw = gw_ref[...].astype(f32)
        gw = jnp.concatenate([gw[t:t + 1, :] for t in range(NT)], axis=1)
        g = jax.nn.sigmoid(jnp.sum(xf * gw, axis=-1, keepdims=True))
        out_v[slot] = (g * a + (1.0 - g) * b_v[pl.ds(r0, 64), :]).astype(bf16)
        out_copy(j, slot).start()
        return carry

    lax.fori_loop(0, NPAIR, pair, 0)
    out_copy(NPAIR - 2, 0).wait()
    out_copy(NPAIR - 1, 1).wait()


@functools.partial(jax.jit, static_argnames=("A_seg_len",))
def pallas_gated_mix__memory_aug_recurrent_mem_tr__mixer_s_mlp__prompt_kernel(
    A_x, A_mem0, A_Wq, A_Wk, A_Wv, A_Wo, A_seg_len, B_x, B_w1, B_w2, B_w3, B_w4, gate_w,
):
    assert A_seg_len == SEG
    assert A_x.shape == (1, S, D) and A_mem0.shape == (1, M, D)
    any_spec = pl.BlockSpec(memory_space=pl.ANY)
    out = pl.pallas_call(
        _kernel,
        out_shape=jax.ShapeDtypeStruct((S, D), bf16),
        in_specs=[any_spec] * 11,
        out_specs=any_spec,
        scratch_shapes=[
            pltpu.VMEM((S, D), bf16),
            pltpu.VMEM((9, D // 4, D // 2), u32),
            pltpu.VMEM((7, D // 4, D // 2), u32),
            pltpu.VMEM((7, D // 4, F // 2), u32),
            pltpu.VMEM((7, F // 4, D // 2), u32),
            pltpu.VMEM((3 * H, D // 2, DH), u32),
            pltpu.VMEM((NT, H * DH // 2, 128), u32),
            pltpu.VMEM((NT, S + 2 * PAD, 128), f32),
            pltpu.VMEM((S, D), f32),
            pltpu.VMEM((2, 7, HM // 2, D // 2), u32),
            pltpu.VMEM((TM, D), f32),
            pltpu.VMEM((2, 64, D), bf16),
            pltpu.VMEM((H, 24, 128), u32),
            pltpu.VMEM((H, 24, 128), u32),
            pltpu.VMEM((24, H * DH), u32),
            pltpu.VMEM((M, D), f32),
            pltpu.VMEM((M, D), bf16),
            pltpu.VMEM((NT, 128), bf16),
            pltpu.SMEM((1,), jnp.int32),
            pltpu.SemaphoreType.DMA((NLOAD,)),
            pltpu.SemaphoreType.DMA((NG,)),
            pltpu.SemaphoreType.DMA((2,)),
        ],
        compiler_params=pltpu.CompilerParams(vmem_limit_bytes=120 * 1024 * 1024,
                                             disable_bounds_checks=True),
    )(
        A_x.reshape(S, D), A_mem0.reshape(M, D),
        A_Wq.reshape(D // 2, 2 * H, DH), A_Wk.reshape(D // 2, 2 * H, DH), A_Wv.reshape(D // 2, 2 * H, DH),
        A_Wo.reshape(H * DH, D), B_w1, B_w2, B_w3, B_w4, gate_w.reshape(NT, 128),
    )
    return out.reshape(1, S, D)
```

```python
import functools

import jax
import jax.numpy as jnp
from jax import lax
import jax.experimental.pallas as pl
import jax.experimental.pallas.tpu as pltpu

f32, bf16, u32 = jnp.float32, jnp.bfloat16, jnp.uint32

S, D, H, DH, M, SEG, F = 2048, 1024, 32, 128, 8, 32, 3584
SCALE = DH ** -0.5
NEG = -1000000000.0
EPS = 1e-05

TM = 256
NB = S // TM
HM = TM // 2
DH2 = D // 2
FH = F // 2
FC = 256
NFC = FH // FC
NC1 = 128
NPAIR = S // (2 * SEG)
G = 4
NG = H // G
PAD = 8
NT = D // 128
NLOAD = 4 + 8 + 12 + 2 + NT
assert NB == NG

_dot = functools.partial(jnp.dot, preferred_element_type=f32)


def _ln(x):
    m = jnp.mean(x, axis=-1, keepdims=True)
    xc = x - m
    v = jnp.mean(xc * xc, axis=-1, keepdims=True)
    return xc * lax.rsqrt(v + EPS)


_GC = 0.7978845608028654


def _gelu(x):
    h = 0.5 * x
    return h + h * jnp.tanh(x * (_GC + (_GC * 0.044715) * (x * x)))


def _unpack(u):
    return pltpu.bitcast(u, bf16).astype(f32)


def _pack(x):
    return pltpu.bitcast(x.astype(bf16), u32)


def _lcombos(a11, a12, a21, a22):
    return [a11 + a22, a21 + a22, a11, a22, a11 + a12, a21 - a11, a12 - a22]


def _merge(*lists):
    keyed = [((j + 0.5) / len(l), n, j, v) for n, l in enumerate(lists) for j, v in enumerate(l)]
    return [v for _, _, _, v in sorted(keyed, key=lambda t: t[:3])]


def _masks():
    r = lax.broadcasted_iota(jnp.int32, (32, 48), 0)
    c = lax.broadcasted_iota(jnp.int32, (32, 48), 1)
    exist_e = (c >= 40) | (c < 32)
    allow_e = (c >= 40) | ((c < 32) & ((r >= 24) | (c <= r)))
    fill_e = jnp.where(exist_e, NEG, -jnp.inf).astype(f32)
    r = lax.broadcasted_iota(jnp.int32, (48, 80), 0)
    c = lax.broadcasted_iota(jnp.int32, (48, 80), 1)
    keys_even = (c < 32) | ((c >= 40) & (c < 48))
    exist_o = ((r < 8) & keys_even) | ((r >= 8) & ~keys_even)
    ktok = jnp.where(c < 40, c, c - 16)
    qtok = jnp.where(r < 8, r + 24, r + 16)
    is_mem_key = (c >= 40) & (c < 56)
    is_mem_q = (r >= 8) & (r < 16)
    allow_o = exist_o & (is_mem_key | is_mem_q | (ktok <= qtok))
    fill_o = jnp.where(exist_o, NEG, -jnp.inf).astype(f32)
    return allow_e, fill_e, allow_o, fill_o


def _softmax(s, allow, fill):
    s = jnp.where(allow, s * SCALE, fill)
    m = jnp.max(s, axis=-1, keepdims=True)
    e = jnp.exp(s - m)
    l = jnp.sum(e, axis=-1, keepdims=True)
    return (e * pl.reciprocal(l, approx=False)).astype(bf16)


def _kernel(x_hbm, mem0_hbm, wq_hbm, wk_hbm, wv_hbm, wo_hbm, w1_hbm, w2_hbm, w3_hbm, w4_hbm,
            gw_hbm, out_hbm,
            x_v, s1_v, s2_v, s3_v, s4_v, wqkv_v, wo_v, h_v, b_v, l_v, n_v, out_v,
            ke_v, ve_v, o_v, mem_v, mem0_ref, gw_ref, zero_s,
            sem, sem_qkv, sem_out):
    RAW = (1, 2, 3, 4)
    RAW1 = (1, 7, 8, 4)

    loads = []

    def rows_load(name, r0, r1):
        loads.append((name, x_hbm.at[pl.ds(r0, r1 - r0)], x_v.at[pl.ds(r0, r1 - r0)]))

    def quad_load(name, w_hbm, s_v, raw, q, c0=0, c1=None):
        k4, n2 = s_v.shape[1], s_v.shape[2]
        c1 = n2 if c1 is None else c1
        src = w_hbm.bitcast(u32).at[pl.ds((q // 2) * k4, k4), pl.ds((q % 2) * n2 + c0, c1 - c0)]
        loads.append((name, src, s_v.at[raw[q], :, pl.ds(c0, c1 - c0)]))

    rows_load("x0", 0, TM)
    rows_load("x1", TM, 2 * TM)
    for name, half, c0, c1 in (("w1a", 0, 0, 256), ("w1bc", 0, 256, 512), ("w1bc", 1, 0, 256), ("w1d", 1, 256, 512)):
        quad_load(name, w1_hbm, s1_v, RAW1, half, c0, c1)
        quad_load(name, w1_hbm, s1_v, RAW1, 2 + half, c0, c1)
    rows_load("x234", 2 * TM, 5 * TM)
    rows_load("x567", 5 * TM, S)
    for name, w_hbm, s_v in (("w2", w2_hbm, s2_v), ("w3", w3_hbm, s3_v), ("w4", w4_hbm, s4_v)):
        for q in range(4):
            quad_load(name, w_hbm, s_v, RAW, q)
    loads.append(("small", mem0_hbm, mem0_ref))
    loads.append(("small", gw_hbm, gw_ref))
    for j in range(NT):
        loads.append(("wo", wo_hbm.bitcast(u32).at[:, pl.ds(j * 128, 128)], wo_v.at[j]))
    assert len(loads) == NLOAD

    def start(*names, priority=0):
        for n, (name, src, dst) in enumerate(loads):
            if name in names:
                pltpu.make_async_copy(src, dst, sem.at[n]).start(priority=priority)

    def wait(*names):
        for n, (name, src, dst) in enumerate(loads):
            if name in names:
                pltpu.make_async_copy(src, dst, sem.at[n]).wait()

    SPG = 3 * G

    def qkv_start(g):
        for w, w_hbm in enumerate((wq_hbm, wk_hbm, wv_hbm)):
            wu = w_hbm.bitcast(u32)
            for k in range(G // 2):
                for par in range(2):
                    pltpu.make_async_copy(
                        wu.at[:, par * (H // 2) + g * (G // 2) + k, :],
                        wqkv_v.at[g * SPG + w * G + 2 * k + par], sem_qkv.at[g]).start(priority=1)

    def qkv_wait(g):
        grp = wqkv_v.at[pl.ds(g * SPG, SPG)]
        pltpu.make_async_copy(grp, grp, sem_qkv.at[g]).wait()

    start("x0", "x1", "w1a", "w1bc", "w1d", "x234", "x567", "w2", "w3", "w4", "small")
    zero_s[0] = 0

    def tile_idx(ref):
        z = zero_s[0]
        return (z,) * (len(ref.shape) - 2) + (pl.ds(pl.multiple_of(z, 8), 8), slice(0, 128))

    hist = []

    def mm(lhs, rhs, side=None, acc=None):
        if side is not None:
            lhs = side(lhs)
        lhs = pltpu.bitcast(lhs, bf16) if lhs.dtype == u32 else lhs.astype(bf16)
        y = _dot(lhs, pltpu.bitcast(rhs, bf16))
        if acc is not None:
            y = y + acc
        hist.append(y)
        return y

    class Side:
        def __init__(self, pieces, n):
            self.pieces, self.n = list(pieces), n

        def __call__(self, val):
            take = -(-len(self.pieces) // self.n) if self.pieces else 0
            self.n -= 1
            if not take:
                return val
            never = zero_s[0] > 0
            rg = 8 if val.dtype == u32 else 16
            ng = val.shape[0] // rg
            groups = [val[8 * m:8 * m + 8] for m in range(val.shape[0] // 8)]
            for j, (fn, rd, wr, lag) in enumerate(self.pieces[:take]):
                m = (j + 1) * ng // take - 1
                pin = lambda v: v
                if lag is not None and len(hist) >= lag:
                    r0 = (16 * m) % hist[-lag].shape[0]
                    a = hist[-lag][r0:r0 + 8, :128]
                    if rd is None:
                        def pin(v, a=a):
                            t = jnp.where(never, jnp.concatenate([a] * (v.shape[0] // 8), axis=0), v[:, :128])
                            return t if v.shape[1] == 128 else jnp.concatenate([t, v[:, 128:]], axis=1)
                    else:
                        idx = tile_idx(rd)
                        rd[idx] = jnp.where(never, pltpu.bitcast(a, rd.dtype), rd[idx])
                fn(pin)
                g = m * rg // 8
                t = jnp.where(never, pltpu.bitcast(wr[tile_idx(wr)], val.dtype), groups[g][:, -128:])
                groups[g] = jnp.concatenate([groups[g][:, :-128], t], axis=1)
            self.pieces = self.pieces[take:]
            return jnp.concatenate(groups, axis=0)

    def strassen(lhs, rhs, side, init=(None, None, None, None), ks=range(7)):
        def add(a, b):
            return a if b is None else a + b
        sd = lambda k: side if k in ks else None
        p = [mm(lhs(k), rhs(k), sd(k)) for k in range(5)]
        c12 = add(p[2] + p[4], init[1])
        c21 = add(p[1] + p[3], init[2])
        c22 = mm(lhs(5), rhs(5), sd(5), add(p[0] - p[1] + p[2], init[3]))
        c11 = mm(lhs(6), rhs(6), sd(6), add(p[0] + p[3] - p[4], init[0]))
        return c11, c12, c21, c22

    def prep_pieces(s_v, raw, lag, width=256):
        def piece(r, c, pin):
            idx = (slice(r, r + 8), slice(c, c + width))
            b11, b12, b21, b22 = [_unpack(s_v[(q,) + idx]) for q in raw]
            for k, t in ((0, b11 + b22), (2, b12 - b22), (3, b21 - b11), (5, b11 + b12), (6, b21 + b22)):
                s_v[(k,) + idx] = _pack(t)
        return [(functools.partial(piece, r, c), s_v, s_v, lag)
                for r in range(0, s_v.shape[1], 8) for c in range(0, s_v.shape[2], width)]

    def store_l(slot, q, c, quads, plain=False):
        for k, t in enumerate(quads if plain else _lcombos(*quads)):
            l_v[slot, k, q // 2:q // 2 + 8, c:c + t.shape[1]] = _pack(t)

    def ln_pieces(src, r0, slot, lag, plain=False, width=256, staged=False, clag=None):
        def stats(q, pin):
            x = pin(src[pl.ds(r0 + q, 16), :].astype(f32))
            xs = [x[:, j * 128:(j + 1) * 128] for j in range(NT)]
            m = functools.reduce(lambda a, b: a + b, xs) * (1.0 / NT)
            w = functools.reduce(lambda a, b: a + b, [(t - m) * (t - m) for t in xs])
            mean = jnp.mean(m, axis=-1, keepdims=True)
            var = jnp.sum(w + NT * ((m - mean) * (m - mean)), axis=-1, keepdims=True) * (1.0 / D)
            n_v[0, q:q + 16, :] = jnp.broadcast_to(mean, (16, 128))
            n_v[1, q:q + 16, :] = jnp.broadcast_to(lax.rsqrt(var + EPS), (16, 128))

        def comb(q, c, pin):
            quads = []
            for rr in (0, HM):
                rs = pl.ds(pl.multiple_of(r0 + rr + q + zero_s[0], 16), 16)
                mean, rstd = [jnp.concatenate([n_v[t, rr + q:rr + q + 16, :]] * (width // 128), axis=1)
                              for t in range(2)]
                quads += [(src[rs, cc + c:cc + c + width].astype(f32) - mean) * rstd for cc in (0, DH2)]
            store_l(slot, q, c, quads, plain)
        norms = [[(functools.partial(stats, rr + q), None, n_v, lag) for rr in (0, HM)] for q in range(0, HM, 16)]
        combs = [[(functools.partial(comb, q, c), n_v, l_v, clag) for c in range(0, DH2, width)]
                 for q in range(0, HM, 16)]
        if staged:
            return sum(norms, []), sum(combs, [])
        out = list(norms[0])
        for a, b in zip(norms[1:] + [[]], combs):
            out += _merge(a, b) if a else b
        return out

    shifts = (1, 1, -1, -1, 2, 2, -2, -2)

    def shift_pieces(r0, slot, lag, by_value=False):
        def piece(q, j, pin):
            a = [h_v[jj, pl.ds(PAD + r0 + rr + q - shifts[jj], 16), :]
                 for rr in (0, HM) for jj in (j, j + NT // 2)]
            store_l(slot, q, j * 128, [pin(a[0]), a[1], a[2], pin(a[3])])
        return [(functools.partial(piece, q, j), None if by_value else h_v, l_v, lag)
                for q in range(0, HM, 16) for j in range(NT // 2)]

    def lhs_of(slot):
        return lambda k: l_v[slot, k]

    h_v[:, 0:PAD, :] = jnp.zeros((NT, PAD, 128), f32)
    h_v[:, PAD + S:PAD + S + PAD, :] = jnp.zeros((NT, PAD, 128), f32)

    def store_h(r0, c0, h):
        for j in range(h.shape[1] // 128):
            h_v[c0 // 128 + j, PAD + r0:PAD + r0 + h.shape[0], :] = h[:, j * 128:(j + 1) * 128]

    def d1_plain(xn, r0, c0, c1, step, side=None):
        for c in range(c0, c1, step):
            half, cc = c // DH2, c % DH2
            w = jnp.concatenate([s1_v[RAW1[half], :, cc:cc + step], s1_v[RAW1[2 + half], :, cc:cc + step]], axis=0)
            store_h(r0, c, _gelu(mm(xn, w, side)))

    NP1 = 7 * (DH2 // NC1)
    KS1 = (2, 3, 4, 5)

    def d1_s(b, slot, pieces):
        side = Side(pieces, len(KS1) * (DH2 // NC1))
        for c in range(0, DH2, NC1):
            cs = strassen(lhs_of(slot), lambda k: s1_v[k, :, c:c + NC1], side, ks=KS1)
            for q, t in enumerate(cs):
                store_h(b * TM + (q // 2) * HM, (q % 2) * DH2 + c, _gelu(t))

    def d2_s(b, slot, pieces):
        side = Side(pieces, NP1)
        for c in range(0, DH2, NC1):
            idx = [(slice(b * TM + (q // 2) * HM, b * TM + (q // 2 + 1) * HM),
                    slice((q % 2) * DH2 + c, (q % 2) * DH2 + c + NC1)) for q in range(4)]
            cs = strassen(lhs_of(slot), lambda k: s2_v[k, :, c:c + NC1], side,
                          [x_v[i].astype(f32) for i in idx])
            for i, t in zip(idx, cs):
                b_v[i] = t

    def split(l, n):
        return [l[len(l) * i // n:len(l) * (i + 1) // n] for i in range(n)]

    LS, LL = 3, 5

    wait("x0")
    xn0 = _pack(_ln(x_v[0:TM, :].astype(f32)))
    wait("x1")
    xn01 = jnp.concatenate([xn0, _pack(_ln(x_v[TM:2 * TM, :].astype(f32)))], axis=0)
    wait("w1a")
    d1_plain(xn01, 0, 0, 256, 256)
    wait("w1bc")
    d1_plain(xn01, 0, 256, 768, 256)
    wait("w1d", "x234")
    hist.clear()
    d1_plain(xn01, 0, 768, D, 128, Side(ln_pieces(x_v, 2 * TM, 0, None, plain=True), 2))
    xn2 = jnp.concatenate([jnp.concatenate([l_v[0, 2 * h], l_v[0, 2 * h + 1]], axis=1) for h in range(2)], axis=0)
    d1_plain(xn2, 2 * TM, 0, D, 128,
             Side(_merge(prep_pieces(s1_v, RAW1, 1), ln_pieces(x_v, 3 * TM, 1, 2)), 8))
    d1_s(3, 1, ln_pieces(x_v, 4 * TM, 0, LL))
    wait("x567", "w2")
    qkv_start(0)
    qkv_start(1)
    hist.clear()
    pw = split(prep_pieces(s2_v, RAW, LS), 4)
    for b in range(4, NB):
        nxt = ln_pieces(x_v, (b + 1) * TM, (b + 1) % 2, LL) if b + 1 < NB else shift_pieces(0, 0, LS, True)
        d1_s(b, b % 2, _merge(pw[b - 4], nxt))
    d2_s(0, 0, shift_pieces(TM, 1, LS, True))
    wait("w3")
    hist.clear()
    pw = split(prep_pieces(s3_v, RAW, LS), 4)
    for b in range(1, 5):
        d2_s(b, b % 2, _merge(pw[b - 1], shift_pieces((b + 1) * TM, (b + 1) % 2, LS)))
    wait("w4")
    hist.clear()
    pw = prep_pieces(s4_v, RAW, LS)
    pw = [pw[:82], pw[82:164], pw[164:]]
    for b in range(5, NB):
        nxt = shift_pieces((b + 1) * TM, (b + 1) % 2, LS) if b + 1 < NB else ln_pieces(b_v, 0, 0, LL)
        d2_s(b, b % 2, _merge(pw[b - 5], nxt))
    start("wo", priority=1)

    def ffn(i, carry):
        qkv_wait(i)
        r0 = pl.multiple_of(i * TM, TM)
        rn = pl.multiple_of(jnp.minimum(i + 1, NB - 1) * TM, TM)
        lh = {}
        acc = [None] * 7
        hist.clear()

        def relayout(p, r0_, r1_, pin):
            s0 = i * SPG + 2 * p
            for r in range(r0_, r1_, 8):
                e = wqkv_v[s0, r:r + 8, :]
                o = wqkv_v[s0 + 1, r:r + 8, :]
                wqkv_v[s0, r:r + 8, :] = (e & jnp.uint32(0xFFFF)) | (o << 16)
                wqkv_v[s0 + 1, r:r + 8, :] = (e >> 16) | (o & jnp.uint32(0xFFFF0000))

        side3 = Side([(functools.partial(relayout, p, r, r + 32), wqkv_v, wqkv_v, 2)
                      for p in range(SPG // 2) for r in range(0, D // 2, 32)], 42 + 5)
        norms, combs = ln_pieces(b_v, rn, 0, 3, staged=True, width=128, clag=2)
        side4 = Side(norms, 16)
        side5 = Side(combs, 11)

        def d3(c):
            cs = strassen(lhs_of(0), lambda k: s3_v[k, :, c * FC:(c + 1) * FC],
                          side3 if c > 0 else (lambda v: side3(v) if len(hist) >= 2 else v))
            lh[c] = _lcombos(*[_gelu(t) for t in cs])

        def d4(c):
            l = lh.pop(c)
            rhs = lambda k: s4_v[k, c * FC // 2:(c + 1) * FC // 2, :]
            if c + 1 < NFC:
                for k in range(7):
                    side = (side5 if k > 0 else None) if c == NFC - 2 else (side4 if k >= 3 else None)
                    acc[k] = mm(l[k], rhs(k), side, acc[k])
                return
            q = [mm(l[k], rhs(k), side5, acc[k]) for k in range(5)]
            top, bot = pl.ds(r0, HM), pl.ds(r0 + HM, HM)
            b_v[top, DH2:] = q[2] + q[4] + b_v[top, DH2:]
            b_v[bot, :DH2] = q[1] + q[3] + b_v[bot, :DH2]
            b_v[bot, DH2:] = mm(l[5], rhs(5), None, acc[5] + q[0] - q[1] + q[2] + b_v[bot, DH2:])
            b_v[top, :DH2] = mm(l[6], rhs(6), None, acc[6] + q[0] + q[3] - q[4] + b_v[top, :DH2])

        d3(0)
        for c in range(NFC):
            if c + 1 < NFC:
                d3(c + 1)
            d4(c)
        assert not side3.pieces and not side4.pieces and not side5.pieces

        @pl.when(i + 2 < NG)
        def _():
            qkv_start(i + 2)

        return carry

    lax.fori_loop(0, NB, ffn, 0)

    wait("small", "wo")
    mem_v[...] = mem0_ref[...].astype(f32)

    def wload(w, h):
        return pltpu.bitcast(wqkv_v[(h // G) * SPG + w * G + h % G], bf16)

    def step(hq, hkv, odd, allow, fill):
        nq = hq.shape[0]
        qs, ks, vs, ps = {}, {}, {}, {}

        def proj(g):
            for h in range(g * G, (g + 1) * G):
                qs[h] = _dot(hq, wload(0, h)).astype(bf16)
                k = _dot(hkv, wload(1, h)).astype(bf16)
                v = _dot(hkv, wload(2, h)).astype(bf16)
                if odd:
                    k = jnp.concatenate([pltpu.bitcast(ke_v[h], bf16), k], axis=0)
                    v = jnp.concatenate([pltpu.bitcast(ve_v[h], bf16), v], axis=0)
                else:
                    ke_v[h] = pltpu.bitcast(k, u32)
                    ve_v[h] = pltpu.bitcast(v, u32)
                ks[h] = k
                vs[h] = v

        def score(g):
            for h in range(g * G, (g + 1) * G):
                s = lax.dot_general(qs.pop(h), ks.pop(h), (((1,), (1,)), ((), ())),
                                    preferred_element_type=f32)
                ps[h] = _softmax(s, allow, fill)

        def pv(g):
            for h in range(g * G, (g + 1) * G):
                o = _dot(ps.pop(h), vs.pop(h)).astype(bf16)
                o_v[0:nq // 2, h * 128:(h + 1) * 128] = pltpu.bitcast(o, u32)

        acc = [None] * NT

        def wo(h0, h1, j0, j1):
            o = pltpu.bitcast(o_v[0:nq // 2, h0 * 128:h1 * 128], bf16)
            for j in range(j0, j1):
                y = _dot(o, pltpu.bitcast(wo_v[j, h0 * 64:h1 * 64, :], bf16))
                acc[j] = y if acc[j] is None else y + acc[j]

        for t in range(NG):
            proj(t)
            if t >= 1:
                score(t - 1)
            if t >= 2:
                pv(t - 2)
        wo(0, 16, 0, 4)
        score(NG - 1)
        pv(NG - 2)
        wo(0, 16, 4, 8)
        pv(NG - 1)
        wo(16, 24, 0, 8)
        wo(24, 32, 0, 8)
        return jnp.concatenate(acc, axis=1)

    def out_copy(j, slot):
        r0 = pl.multiple_of(j * 64, 64)
        return pltpu.make_async_copy(out_v.at[slot], out_hbm.at[pl.ds(r0, 64)], sem_out.at[slot])

    def pair(j, carry):
        slot = j % 2

        @pl.when(j >= 2)
        def _():
            out_copy(j - 2, slot).wait()

        allow_e, fill_e, allow_o, fill_o = _masks()
        r0 = pl.multiple_of(j * 64, 64)
        x0 = x_v[pl.ds(r0, 16), :]
        x1 = x_v[pl.ds(r0 + 16, 16), :]
        x2 = x_v[pl.ds(r0 + 32, 16), :]
        x3 = x_v[pl.ds(r0 + 48, 16), :]
        x1f = x1.astype(f32)
        x2f = x2.astype(f32)
        mem = mem_v[...]
        hq = jnp.concatenate([x0, jnp.concatenate([x1f[:8], mem], 0).astype(bf16)], 0)
        hkv = jnp.concatenate([x0, x1, jnp.concatenate([x2f[:8], mem], 0).astype(bf16)], 0)
        oe = step(hq, hkv, False, allow_e, fill_e)
        mem = oe[24:32]
        hq = jnp.concatenate([jnp.concatenate([x1f[8:], mem], 0).astype(bf16), x2, x3], 0)
        hkv = jnp.concatenate([jnp.concatenate([mem, x2f[8:]], 0).astype(bf16), x3], 0)
        oo = step(hq, hkv, True, allow_o, fill_o)
        mem_v[...] = oo[8:16]
        a = jnp.concatenate([oe[:24], oo[:8], oo[16:]], 0)
        xf = x_v[pl.ds(r0, 64), :].astype(f32)
        gw = gw_ref[...].astype(f32)
        gw = jnp.concatenate([gw[t:t + 1, :] for t in range(NT)], axis=1)
        g = jax.nn.sigmoid(jnp.sum(xf * gw, axis=-1, keepdims=True))
        out_v[slot] = (g * a + (1.0 - g) * b_v[pl.ds(r0, 64), :]).astype(bf16)
        out_copy(j, slot).start()
        return carry

    lax.fori_loop(0, NPAIR, pair, 0)
    out_copy(NPAIR - 2, 0).wait()
    out_copy(NPAIR - 1, 1).wait()


@functools.partial(jax.jit, static_argnames=("A_seg_len",))
def pallas_gated_mix__memory_aug_recurrent_mem_tr__mixer_s_mlp__prompt_kernel(
    A_x, A_mem0, A_Wq, A_Wk, A_Wv, A_Wo, A_seg_len, B_x, B_w1, B_w2, B_w3, B_w4, gate_w,
):
    assert A_seg_len == SEG
    assert A_x.shape == (1, S, D) and A_mem0.shape == (1, M, D)
    any_spec = pl.BlockSpec(memory_space=pl.ANY)
    out = pl.pallas_call(
        _kernel,
        out_shape=jax.ShapeDtypeStruct((S, D), bf16),
        in_specs=[any_spec] * 11,
        out_specs=any_spec,
        scratch_shapes=[
            pltpu.VMEM((S, D), bf16),
            pltpu.VMEM((9, D // 4, D // 2), u32),
            pltpu.VMEM((7, D // 4, D // 2), u32),
            pltpu.VMEM((7, D // 4, F // 2), u32),
            pltpu.VMEM((7, F // 4, D // 2), u32),
            pltpu.VMEM((3 * H, D // 2, DH), u32),
            pltpu.VMEM((NT, H * DH // 2, 128), u32),
            pltpu.VMEM((NT, S + 2 * PAD, 128), f32),
            pltpu.VMEM((S, D), f32),
            pltpu.VMEM((2, 7, HM // 2, D // 2), u32),
            pltpu.VMEM((2, TM, 128), f32),
            pltpu.VMEM((2, 64, D), bf16),
            pltpu.VMEM((H, 24, 128), u32),
            pltpu.VMEM((H, 24, 128), u32),
            pltpu.VMEM((24, H * DH), u32),
            pltpu.VMEM((M, D), f32),
            pltpu.VMEM((M, D), bf16),
            pltpu.VMEM((NT, 128), bf16),
            pltpu.SMEM((1,), jnp.int32),
            pltpu.SemaphoreType.DMA((NLOAD,)),
            pltpu.SemaphoreType.DMA((NG,)),
            pltpu.SemaphoreType.DMA((2,)),
        ],
        compiler_params=pltpu.CompilerParams(vmem_limit_bytes=120 * 1024 * 1024,
                                             disable_bounds_checks=True),
    )(
        A_x.reshape(S, D), A_mem0.reshape(M, D),
        A_Wq.reshape(D // 2, 2 * H, DH), A_Wk.reshape(D // 2, 2 * H, DH), A_Wv.reshape(D // 2, 2 * H, DH),
        A_Wo.reshape(H * DH, D), B_w1, B_w2, B_w3, B_w4, gate_w.reshape(NT, 128),
    )
    return out.reshape(1, S, D)
```

```python
import functools

import jax
import jax.numpy as jnp
from jax import lax
import jax.experimental.pallas as pl
import jax.experimental.pallas.tpu as pltpu

f32, bf16, u32 = jnp.float32, jnp.bfloat16, jnp.uint32

S, D, H, DH, M, SEG, F = 2048, 1024, 32, 128, 8, 32, 3584
SCALE = DH ** -0.5
NEG = -1000000000.0
EPS = 1e-05

TM = 256
NB = S // TM
HM = TM // 2
DH2 = D // 2
FH = F // 2
FC = 256
NFC = FH // FC
NC1 = 128
NPAIR = S // (2 * SEG)
G = 4
NG = H // G
PAD = 8
NT = D // 128
NLOAD = 4 + 8 + 12 + 2 + NT
assert NB == NG

_dot = functools.partial(jnp.dot, preferred_element_type=f32)


def _ln(x):
    m = jnp.mean(x, axis=-1, keepdims=True)
    xc = x - m
    v = jnp.mean(xc * xc, axis=-1, keepdims=True)
    return xc * lax.rsqrt(v + EPS)


_GC = 0.7978845608028654


def _gelu(x):
    h = 0.5 * x
    return h + h * jnp.tanh(x * (_GC + (_GC * 0.044715) * (x * x)))


def _unpack(u):
    return pltpu.bitcast(u, bf16).astype(f32)


def _pack(x):
    return pltpu.bitcast(x.astype(bf16), u32)


def _lcombos(a11, a12, a21, a22):
    return [a11 + a22, a21 + a22, a11, a22, a11 + a12, a21 - a11, a12 - a22]


def _merge(*lists):
    keyed = [((j + 0.5) / len(l), n, j, v) for n, l in enumerate(lists) for j, v in enumerate(l)]
    return [v for _, _, _, v in sorted(keyed, key=lambda t: t[:3])]


def _masks():
    r = lax.broadcasted_iota(jnp.int32, (32, 48), 0)
    c = lax.broadcasted_iota(jnp.int32, (32, 48), 1)
    exist_e = (c >= 40) | (c < 32)
    allow_e = (c >= 40) | ((c < 32) & ((r >= 24) | (c <= r)))
    fill_e = jnp.where(exist_e, NEG, -jnp.inf).astype(f32)
    r = lax.broadcasted_iota(jnp.int32, (48, 80), 0)
    c = lax.broadcasted_iota(jnp.int32, (48, 80), 1)
    keys_even = (c < 32) | ((c >= 40) & (c < 48))
    exist_o = ((r < 8) & keys_even) | ((r >= 8) & ~keys_even)
    ktok = jnp.where(c < 40, c, c - 16)
    qtok = jnp.where(r < 8, r + 24, r + 16)
    is_mem_key = (c >= 40) & (c < 56)
    is_mem_q = (r >= 8) & (r < 16)
    allow_o = exist_o & (is_mem_key | is_mem_q | (ktok <= qtok))
    fill_o = jnp.where(exist_o, NEG, -jnp.inf).astype(f32)
    return allow_e, fill_e, allow_o, fill_o


def _softmax(s, allow, fill):
    s = jnp.where(allow, s * SCALE, fill)
    m = jnp.max(s, axis=-1, keepdims=True)
    e = jnp.exp(s - m)
    l = jnp.sum(e, axis=-1, keepdims=True)
    return (e * pl.reciprocal(l, approx=False)).astype(bf16)


def _kernel(x_hbm, mem0_hbm, wq_hbm, wk_hbm, wv_hbm, wo_hbm, w1_hbm, w2_hbm, w3_hbm, w4_hbm,
            gw_hbm, out_hbm,
            x_v, s1_v, s2_v, s3_v, s4_v, wqkv_v, wo_v, h_v, b_v, l_v, n_v, g_v, out_v,
            ke_v, ve_v, o_v, mem_v, mem0_ref, gw_ref, zero_s,
            sem, sem_qkv, sem_out):
    RAW = (1, 2, 3, 4)
    RAW1 = (1, 7, 8, 4)

    loads = []

    def rows_load(name, r0, r1):
        loads.append((name, x_hbm.at[pl.ds(r0, r1 - r0)], x_v.at[pl.ds(r0, r1 - r0)]))

    def quad_load(name, w_hbm, s_v, raw, q, c0=0, c1=None):
        k4, n2 = s_v.shape[1], s_v.shape[2]
        c1 = n2 if c1 is None else c1
        src = w_hbm.bitcast(u32).at[pl.ds((q // 2) * k4, k4), pl.ds((q % 2) * n2 + c0, c1 - c0)]
        loads.append((name, src, s_v.at[raw[q], :, pl.ds(c0, c1 - c0)]))

    rows_load("x0", 0, TM)
    rows_load("x1", TM, 2 * TM)
    for name, half, c0, c1 in (("w1a", 0, 0, 256), ("w1bc", 0, 256, 512), ("w1bc", 1, 0, 256), ("w1d", 1, 256, 512)):
        quad_load(name, w1_hbm, s1_v, RAW1, half, c0, c1)
        quad_load(name, w1_hbm, s1_v, RAW1, 2 + half, c0, c1)
    rows_load("x234", 2 * TM, 5 * TM)
    rows_load("x567", 5 * TM, S)
    for name, w_hbm, s_v in (("w2", w2_hbm, s2_v), ("w3", w3_hbm, s3_v), ("w4", w4_hbm, s4_v)):
        for q in range(4):
            quad_load(name, w_hbm, s_v, RAW, q)
    loads.append(("small", mem0_hbm, mem0_ref))
    loads.append(("small", gw_hbm, gw_ref))
    for j in range(NT):
        loads.append(("wo", wo_hbm.bitcast(u32).at[:, pl.ds(j * 128, 128)], wo_v.at[j]))
    assert len(loads) == NLOAD

    def start(*names, priority=0):
        for n, (name, src, dst) in enumerate(loads):
            if name in names:
                pltpu.make_async_copy(src, dst, sem.at[n]).start(priority=priority)

    def wait(*names):
        for n, (name, src, dst) in enumerate(loads):
            if name in names:
                pltpu.make_async_copy(src, dst, sem.at[n]).wait()

    SPG = 3 * G

    def qkv_start(g):
        for w, w_hbm in enumerate((wq_hbm, wk_hbm, wv_hbm)):
            wu = w_hbm.bitcast(u32)
            for k in range(G // 2):
                for par in range(2):
                    pltpu.make_async_copy(
                        wu.at[:, par * (H // 2) + g * (G // 2) + k, :],
                        wqkv_v.at[g * SPG + w * G + 2 * k + par], sem_qkv.at[g]).start(priority=1)

    def qkv_wait(g):
        grp = wqkv_v.at[pl.ds(g * SPG, SPG)]
        pltpu.make_async_copy(grp, grp, sem_qkv.at[g]).wait()

    start("x0", "x1", "w1a", "w1bc", "w1d", "x234", "x567", "w2", "w3", "w4", "small")
    zero_s[0] = 0

    def tile_idx(ref):
        z = zero_s[0]
        return (z,) * (len(ref.shape) - 2) + (pl.ds(pl.multiple_of(z, 8), 8), slice(0, 128))

    hist = []

    def mm(lhs, rhs, side=None, acc=None):
        if side is not None:
            lhs = side(lhs)
        lhs = pltpu.bitcast(lhs, bf16) if lhs.dtype == u32 else lhs.astype(bf16)
        y = _dot(lhs, pltpu.bitcast(rhs, bf16))
        if acc is not None:
            y = y + acc
        hist.append(y)
        return y

    class Side:
        def __init__(self, pieces, n):
            self.pieces, self.n = list(pieces), n

        def __call__(self, val):
            take = -(-len(self.pieces) // self.n) if self.pieces else 0
            self.n -= 1
            if not take:
                return val
            never = zero_s[0] > 0
            rg = 8 if val.dtype == u32 else 16
            ng = val.shape[0] // rg
            groups = [val[8 * m:8 * m + 8] for m in range(val.shape[0] // 8)]
            for j, (fn, rd, wr, lag) in enumerate(self.pieces[:take]):
                m = (j + 1) * ng // take - 1
                pin = lambda v: v
                if lag is not None and len(hist) >= lag:
                    r0 = (16 * m) % hist[-lag].shape[0]
                    a = hist[-lag][r0:r0 + 8, :128]
                    if rd is None:
                        def pin(v, a=a):
                            t = jnp.where(never, jnp.concatenate([a] * (v.shape[0] // 8), axis=0), v[:, :128])
                            return t if v.shape[1] == 128 else jnp.concatenate([t, v[:, 128:]], axis=1)
                    else:
                        idx = tile_idx(rd)
                        rd[idx] = jnp.where(never, pltpu.bitcast(a, rd.dtype), rd[idx])
                fn(pin)
                g = m * rg // 8
                t = jnp.where(never, pltpu.bitcast(wr[tile_idx(wr)], val.dtype), groups[g][:, -128:])
                groups[g] = jnp.concatenate([groups[g][:, :-128], t], axis=1)
            self.pieces = self.pieces[take:]
            return jnp.concatenate(groups, axis=0)

    def strassen(lhs, rhs, side, init=(None, None, None, None), ks=range(7)):
        def add(a, b):
            return a if b is None else a + b
        sd = lambda k: side if k in ks else None
        p = [mm(lhs(k), rhs(k), sd(k)) for k in range(5)]
        c12 = add(p[2] + p[4], init[1])
        c21 = add(p[1] + p[3], init[2])
        c22 = mm(lhs(5), rhs(5), sd(5), add(p[0] - p[1] + p[2], init[3]))
        c11 = mm(lhs(6), rhs(6), sd(6), add(p[0] + p[3] - p[4], init[0]))
        return c11, c12, c21, c22

    def prep_pieces(s_v, raw, lag, width=256):
        def piece(r, c, pin):
            idx = (slice(r, r + 8), slice(c, c + width))
            b11, b12, b21, b22 = [_unpack(s_v[(q,) + idx]) for q in raw]
            for k, t in ((0, b11 + b22), (2, b12 - b22), (3, b21 - b11), (5, b11 + b12), (6, b21 + b22)):
                s_v[(k,) + idx] = _pack(t)
        return [(functools.partial(piece, r, c), s_v, s_v, lag)
                for r in range(0, s_v.shape[1], 8) for c in range(0, s_v.shape[2], width)]

    def store_l(slot, q, c, quads, plain=False):
        for k, t in enumerate(quads if plain else _lcombos(*quads)):
            l_v[slot, k, q // 2:q // 2 + 8, c:c + t.shape[1]] = _pack(t)

    def ln_pieces(src, r0, slot, lag, plain=False, width=256, staged=False, clag=None):
        def stats(q, pin):
            x = pin(src[pl.ds(r0 + q, 16), :].astype(f32))
            xs = [x[:, j * 128:(j + 1) * 128] for j in range(NT)]
            m = functools.reduce(lambda a, b: a + b, xs) * (1.0 / NT)
            w = functools.reduce(lambda a, b: a + b, [(t - m) * (t - m) for t in xs])
            mean = jnp.mean(m, axis=-1, keepdims=True)
            var = jnp.sum(w + NT * ((m - mean) * (m - mean)), axis=-1, keepdims=True) * (1.0 / D)
            n_v[0, q:q + 16, :] = jnp.broadcast_to(mean, (16, 128))
            n_v[1, q:q + 16, :] = jnp.broadcast_to(lax.rsqrt(var + EPS), (16, 128))

        def comb(q, c, pin):
            quads = []
            for rr in (0, HM):
                rs = pl.ds(pl.multiple_of(r0 + rr + q + zero_s[0], 16), 16)
                mean, rstd = [jnp.concatenate([n_v[t, rr + q:rr + q + 16, :]] * (width // 128), axis=1)
                              for t in range(2)]
                quads += [(src[rs, cc + c:cc + c + width].astype(f32) - mean) * rstd for cc in (0, DH2)]
            store_l(slot, q, c, quads, plain)
        norms = [[(functools.partial(stats, rr + q), None, n_v, lag) for rr in (0, HM)] for q in range(0, HM, 16)]
        combs = [[(functools.partial(comb, q, c), n_v, l_v, clag) for c in range(0, DH2, width)]
                 for q in range(0, HM, 16)]
        if staged:
            return sum(norms, []), sum(combs, [])
        out = list(norms[0])
        for a, b in zip(norms[1:] + [[]], combs):
            out += _merge(a, b) if a else b
        return out

    shifts = (1, 1, -1, -1, 2, 2, -2, -2)

    def shift_pieces(r0, slot, lag, by_value=False):
        def piece(q, j, pin):
            a = [h_v[jj, pl.ds(PAD + r0 + rr + q - shifts[jj], 16), :]
                 for rr in (0, HM) for jj in (j, j + NT // 2)]
            store_l(slot, q, j * 128, [pin(a[0]), a[1], a[2], pin(a[3])])
        return [(functools.partial(piece, q, j), None if by_value else h_v, l_v, lag)
                for q in range(0, HM, 16) for j in range(NT // 2)]

    def lhs_of(slot):
        return lambda k: l_v[slot, k]

    h_v[:, 0:PAD, :] = jnp.zeros((NT, PAD, 128), f32)
    h_v[:, PAD + S:PAD + S + PAD, :] = jnp.zeros((NT, PAD, 128), f32)

    def store_h(r0, c0, h):
        for j in range(h.shape[1] // 128):
            h_v[c0 // 128 + j, PAD + r0:PAD + r0 + h.shape[0], :] = h[:, j * 128:(j + 1) * 128]

    def d1_plain(xn, r0, c0, c1, step, side=None):
        for c in range(c0, c1, step):
            half, cc = c // DH2, c % DH2
            w = jnp.concatenate([s1_v[RAW1[half], :, cc:cc + step], s1_v[RAW1[2 + half], :, cc:cc + step]], axis=0)
            store_h(r0, c, _gelu(mm(xn, w, side)))

    NP1 = 7 * (DH2 // NC1)
    KS1 = (2, 3, 4, 5)

    def d1_s(b, slot, pieces):
        side = Side(pieces, len(KS1) * (DH2 // NC1))
        for c in range(0, DH2, NC1):
            cs = strassen(lhs_of(slot), lambda k: s1_v[k, :, c:c + NC1], side, ks=KS1)
            for q, t in enumerate(cs):
                store_h(b * TM + (q // 2) * HM, (q % 2) * DH2 + c, _gelu(t))

    def d2_s(b, slot, pieces):
        side = Side(pieces, NP1)
        for c in range(0, DH2, NC1):
            idx = [(slice(b * TM + (q // 2) * HM, b * TM + (q // 2 + 1) * HM),
                    slice((q % 2) * DH2 + c, (q % 2) * DH2 + c + NC1)) for q in range(4)]
            cs = strassen(lhs_of(slot), lambda k: s2_v[k, :, c:c + NC1], side,
                          [x_v[i].astype(f32) for i in idx])
            for i, t in zip(idx, cs):
                b_v[i] = t

    def split(l, n):
        return [l[len(l) * i // n:len(l) * (i + 1) // n] for i in range(n)]

    LS, LL = 3, 5

    wait("x0")
    xn0 = _pack(_ln(x_v[0:TM, :].astype(f32)))
    wait("x1")
    xn01 = jnp.concatenate([xn0, _pack(_ln(x_v[TM:2 * TM, :].astype(f32)))], axis=0)
    wait("w1a")
    d1_plain(xn01, 0, 0, 256, 256)
    wait("w1bc")
    d1_plain(xn01, 0, 256, 768, 256)
    wait("w1d", "x234")
    hist.clear()
    d1_plain(xn01, 0, 768, D, 128, Side(ln_pieces(x_v, 2 * TM, 0, None, plain=True), 2))
    xn2 = jnp.concatenate([jnp.concatenate([l_v[0, 2 * h], l_v[0, 2 * h + 1]], axis=1) for h in range(2)], axis=0)
    d1_plain(xn2, 2 * TM, 0, D, 128,
             Side(_merge(prep_pieces(s1_v, RAW1, 1), ln_pieces(x_v, 3 * TM, 1, 2)), 8))
    d1_s(3, 1, ln_pieces(x_v, 4 * TM, 0, LL))
    wait("x567", "w2")
    qkv_start(0)
    qkv_start(1)
    hist.clear()
    pw = split(prep_pieces(s2_v, RAW, LS), 4)
    for b in range(4, NB):
        nxt = ln_pieces(x_v, (b + 1) * TM, (b + 1) % 2, LL) if b + 1 < NB else shift_pieces(0, 0, LS, True)
        d1_s(b, b % 2, _merge(pw[b - 4], nxt))
    d2_s(0, 0, shift_pieces(TM, 1, LS, True))
    wait("w3")
    hist.clear()
    pw = split(prep_pieces(s3_v, RAW, LS), 4)
    for b in range(1, 5):
        d2_s(b, b % 2, _merge(pw[b - 1], shift_pieces((b + 1) * TM, (b + 1) % 2, LS)))
    wait("w4", "small")
    hist.clear()
    pw = prep_pieces(s4_v, RAW, LS)
    pw = [pw[:82], pw[82:164], pw[164:]]
    for b in range(5, NB):
        nxt = shift_pieces((b + 1) * TM, (b + 1) % 2, LS) if b + 1 < NB else ln_pieces(b_v, 0, 0, LL)
        d2_s(b, b % 2, _merge(pw[b - 5], nxt))
    start("wo", priority=1)

    def ffn(i, carry):
        qkv_wait(i)
        r0 = pl.multiple_of(i * TM, TM)
        rn = pl.multiple_of(jnp.minimum(i + 1, NB - 1) * TM, TM)
        lh = {}
        acc = [None] * 7
        hist.clear()

        def relayout(p, r0_, r1_, pin):
            s0 = i * SPG + 2 * p
            for r in range(r0_, r1_, 8):
                e = wqkv_v[s0, r:r + 8, :]
                o = wqkv_v[s0 + 1, r:r + 8, :]
                wqkv_v[s0, r:r + 8, :] = (e & jnp.uint32(0xFFFF)) | (o << 16)
                wqkv_v[s0 + 1, r:r + 8, :] = (e >> 16) | (o & jnp.uint32(0xFFFF0000))

        side3 = Side([(functools.partial(relayout, p, r, r + 32), wqkv_v, wqkv_v, 2)
                      for p in range(SPG // 2) for r in range(0, D // 2, 32)], 42 + 5)
        norms, combs = ln_pieces(b_v, rn, 0, 3, staged=True, width=128, clag=2)

        def gate(q, pin):
            gw = gw_ref[...].astype(f32)
            x = pin(x_v[pl.ds(r0 + q, 16), :].astype(f32))
            t = functools.reduce(lambda a, b: a + b,
                                 [x[:, j * 128:(j + 1) * 128] * gw[j:j + 1, :] for j in range(NT)])
            g = jax.nn.sigmoid(jnp.sum(t, axis=-1, keepdims=True))
            g_v[pl.ds(r0 + q, 16), :] = jnp.broadcast_to(g, (16, 128))

        gates = [(functools.partial(gate, q), None, g_v, 3) for q in range(0, TM, 16)]
        side4 = Side(_merge(norms, gates), 20)
        side5 = Side(combs, 11)

        def d3(c):
            cs = strassen(lhs_of(0), lambda k: s3_v[k, :, c * FC:(c + 1) * FC],
                          side3 if c > 0 else (lambda v: side3(v) if len(hist) >= 2 else v))
            lh[c] = _lcombos(*[_gelu(t) for t in cs])

        def d4(c):
            l = lh.pop(c)
            rhs = lambda k: s4_v[k, c * FC // 2:(c + 1) * FC // 2, :]
            if c + 1 < NFC:
                for k in range(7):
                    side = (side5 if k > 0 else None) if c == NFC - 2 else (side4 if k >= 3 else None)
                    acc[k] = mm(l[k], rhs(k), side, acc[k])
                return
            q = [mm(l[k], rhs(k), side5, acc[k]) for k in range(5)]
            top, bot = pl.ds(r0, HM), pl.ds(r0 + HM, HM)
            gt, gb = [jnp.concatenate([1.0 - g_v[r, :]] * (NT // 2), axis=1) for r in (top, bot)]
            b_v[top, DH2:] = gt * (q[2] + q[4] + b_v[top, DH2:])
            b_v[bot, :DH2] = gb * (q[1] + q[3] + b_v[bot, :DH2])
            b_v[bot, DH2:] = gb * mm(l[5], rhs(5), None, acc[5] + q[0] - q[1] + q[2] + b_v[bot, DH2:])
            b_v[top, :DH2] = gt * mm(l[6], rhs(6), None, acc[6] + q[0] + q[3] - q[4] + b_v[top, :DH2])

        d3(0)
        for c in range(NFC):
            if c + 1 < NFC:
                d3(c + 1)
            d4(c)
        assert not side3.pieces and not side4.pieces and not side5.pieces

        @pl.when(i + 2 < NG)
        def _():
            qkv_start(i + 2)

        return carry

    lax.fori_loop(0, NB, ffn, 0)

    wait("wo")
    mem_v[...] = mem0_ref[...].astype(f32)

    def wload(w, h):
        return pltpu.bitcast(wqkv_v[(h // G) * SPG + w * G + h % G], bf16)

    def step(hq, hkv, odd, allow, fill):
        nq = hq.shape[0]
        qs, ks, vs, ps = {}, {}, {}, {}

        def proj(g):
            lhs = (hq, hkv, hkv)
            part = {}
            if odd and g == 0:
                for h in range(2):
                    for w in range(3):
                        part[w, h] = _dot(lhs[w][:, :DH2], wload(w, h)[:DH2])
            for h in range(g * G, (g + 1) * G):
                q, k, v = [(_dot(lhs[w][:, DH2:], wload(w, h)[DH2:]) + part[w, h] if (w, h) in part
                            else _dot(lhs[w], wload(w, h))).astype(bf16) for w in range(3)]
                qs[h] = q
                if odd:
                    k = jnp.concatenate([pltpu.bitcast(ke_v[h], bf16), k], axis=0)
                    v = jnp.concatenate([pltpu.bitcast(ve_v[h], bf16), v], axis=0)
                else:
                    ke_v[h] = pltpu.bitcast(k, u32)
                    ve_v[h] = pltpu.bitcast(v, u32)
                ks[h] = k
                vs[h] = v

        def score(g):
            for h in range(g * G, (g + 1) * G):
                s = lax.dot_general(qs.pop(h), ks.pop(h), (((1,), (1,)), ((), ())),
                                    preferred_element_type=f32)
                ps[h] = _softmax(s, allow, fill)

        def pv(g):
            for h in range(g * G, (g + 1) * G):
                o = _dot(ps.pop(h), vs.pop(h)).astype(bf16)
                o_v[0:nq // 2, h * 128:(h + 1) * 128] = pltpu.bitcast(o, u32)

        acc = [None] * NT

        def wo(h0, h1, j0, j1):
            o = pltpu.bitcast(o_v[0:nq // 2, h0 * 128:h1 * 128], bf16)
            for j in range(j0, j1):
                y = _dot(o, pltpu.bitcast(wo_v[j, h0 * 64:h1 * 64, :], bf16))
                acc[j] = y if acc[j] is None else y + acc[j]

        for t in range(NG):
            proj(t)
            if t >= 1:
                score(t - 1)
            if t >= 2:
                pv(t - 2)
        wo(0, 16, 0, 4)
        score(NG - 1)
        pv(NG - 2)
        wo(0, 16, 4, 8)
        pv(NG - 1)
        wo(16, 24, 0, 8)
        wo(24, 32, 0, 8)
        return jnp.concatenate(acc, axis=1)

    def pair(j, carry):
        r0 = pl.multiple_of(j * 64, 64)
        mem = mem_v[...]
        allow_e, fill_e, allow_o, fill_o = _masks()
        x0 = x_v[pl.ds(r0, 16), :]
        x1 = x_v[pl.ds(r0 + 16, 16), :]
        x2 = x_v[pl.ds(r0 + 32, 16), :]
        x3 = x_v[pl.ds(r0 + 48, 16), :]
        x1f = x1.astype(f32)
        x2f = x2.astype(f32)
        hq = jnp.concatenate([x0, jnp.concatenate([x1f[:8], mem], 0).astype(bf16)], 0)
        hkv = jnp.concatenate([x0, x1, jnp.concatenate([x2f[:8], mem], 0).astype(bf16)], 0)
        oe = step(hq, hkv, False, allow_e, fill_e)
        mem = oe[24:32]
        hq = jnp.concatenate([jnp.concatenate([x1f[8:], mem], 0).astype(bf16), x2, x3], 0)
        hkv = jnp.concatenate([jnp.concatenate([mem, x2f[8:]], 0).astype(bf16), x3], 0)
        oo = step(hq, hkv, True, allow_o, fill_o)
        a = jnp.concatenate([oe[:24], oo[:8], oo[16:]], 0)
        mem_v[...] = oo[8:16]
        g = jnp.concatenate([g_v[pl.ds(r0, 64), :]] * NT, axis=1)
        out_v[pl.ds(r0, 64), :] = (g * a + b_v[pl.ds(r0, 64), :]).astype(bf16)
        pltpu.make_async_copy(out_v.at[pl.ds(r0, 64)], out_hbm.at[pl.ds(r0, 64)], sem_out).start()
        return carry

    lax.fori_loop(0, NPAIR, pair, 0)
    pltpu.make_async_copy(out_v, out_hbm, sem_out).wait()


@functools.partial(jax.jit, static_argnames=("A_seg_len",))
def pallas_gated_mix__memory_aug_recurrent_mem_tr__mixer_s_mlp__prompt_kernel(
    A_x, A_mem0, A_Wq, A_Wk, A_Wv, A_Wo, A_seg_len, B_x, B_w1, B_w2, B_w3, B_w4, gate_w,
):
    assert A_seg_len == SEG
    assert A_x.shape == (1, S, D) and A_mem0.shape == (1, M, D)
    any_spec = pl.BlockSpec(memory_space=pl.ANY)
    out = pl.pallas_call(
        _kernel,
        out_shape=jax.ShapeDtypeStruct((S, D), bf16),
        in_specs=[any_spec] * 11,
        out_specs=any_spec,
        scratch_shapes=[
            pltpu.VMEM((S, D), bf16),
            pltpu.VMEM((9, D // 4, D // 2), u32),
            pltpu.VMEM((7, D // 4, D // 2), u32),
            pltpu.VMEM((7, D // 4, F // 2), u32),
            pltpu.VMEM((7, F // 4, D // 2), u32),
            pltpu.VMEM((3 * H, D // 2, DH), u32),
            pltpu.VMEM((NT, H * DH // 2, 128), u32),
            pltpu.VMEM((NT, S + 2 * PAD, 128), f32),
            pltpu.VMEM((S, D), f32),
            pltpu.VMEM((2, 7, HM // 2, D // 2), u32),
            pltpu.VMEM((2, TM, 128), f32),
            pltpu.VMEM((S, 128), f32),
            pltpu.VMEM((S, D), bf16),
            pltpu.VMEM((H, 24, 128), u32),
            pltpu.VMEM((H, 24, 128), u32),
            pltpu.VMEM((24, H * DH), u32),
            pltpu.VMEM((M, D), f32),
            pltpu.VMEM((M, D), bf16),
            pltpu.VMEM((NT, 128), bf16),
            pltpu.SMEM((1,), jnp.int32),
            pltpu.SemaphoreType.DMA((NLOAD,)),
            pltpu.SemaphoreType.DMA((NG,)),
            pltpu.SemaphoreType.DMA,
        ],
        compiler_params=pltpu.CompilerParams(vmem_limit_bytes=120 * 1024 * 1024,
                                             disable_bounds_checks=True),
    )(
        A_x.reshape(S, D), A_mem0.reshape(M, D),
        A_Wq.reshape(D // 2, 2 * H, DH), A_Wk.reshape(D // 2, 2 * H, DH), A_Wv.reshape(D // 2, 2 * H, DH),
        A_Wo.reshape(H * DH, D), B_w1, B_w2, B_w3, B_w4, gate_w.reshape(NT, 128),
    )
    return out.reshape(1, S, D)
```

```python
import functools

import jax
import jax.numpy as jnp
from jax import lax
import jax.experimental.pallas as pl
import jax.experimental.pallas.tpu as pltpu

f32, bf16, u32 = jnp.float32, jnp.bfloat16, jnp.uint32

S, D, H, DH, M, SEG, F = 2048, 1024, 32, 128, 8, 32, 3584
SCALE = DH ** -0.5
NEG = -1000000000.0
EPS = 1e-05

TM = 256
NB = S // TM
HM = TM // 2
DH2 = D // 2
FH = F // 2
FC = 256
NFC = FH // FC
NC1 = 128
NPAIR = S // (2 * SEG)
G = 4
NG = H // G
PAD = 8
NT = D // 128
NLOAD = 12
assert NB == NG

_dot = functools.partial(jnp.dot, preferred_element_type=f32)


def _ln(x):
    m = jnp.mean(x, axis=-1, keepdims=True)
    xc = x - m
    v = jnp.mean(xc * xc, axis=-1, keepdims=True)
    return xc * lax.rsqrt(v + EPS)


_GC = 0.7978845608028654


def _gelu(x):
    h = 0.5 * x
    return h + h * jnp.tanh(x * (_GC + (_GC * 0.044715) * (x * x)))


def _unpack(u):
    return pltpu.bitcast(u, bf16).astype(f32)


def _pack(x):
    return pltpu.bitcast(x.astype(bf16), u32)


def _lcombos(a11, a12, a21, a22):
    return [a11 + a22, a21 + a22, a11, a22, a11 + a12, a21 - a11, a12 - a22]


def _merge(*lists):
    keyed = [((j + 0.5) / len(l), n, j, v) for n, l in enumerate(lists) for j, v in enumerate(l)]
    return [v for _, _, _, v in sorted(keyed, key=lambda t: t[:3])]


def _masks():
    r = lax.broadcasted_iota(jnp.int32, (32, 48), 0)
    c = lax.broadcasted_iota(jnp.int32, (32, 48), 1)
    exist_e = (c >= 40) | (c < 32)
    allow_e = (c >= 40) | ((c < 32) & ((r >= 24) | (c <= r)))
    fill_e = jnp.where(exist_e, NEG, -jnp.inf).astype(f32)
    r = lax.broadcasted_iota(jnp.int32, (48, 80), 0)
    c = lax.broadcasted_iota(jnp.int32, (48, 80), 1)
    keys_even = (c < 32) | ((c >= 40) & (c < 48))
    exist_o = ((r < 8) & keys_even) | ((r >= 8) & ~keys_even)
    ktok = jnp.where(c < 40, c, c - 16)
    qtok = jnp.where(r < 8, r + 24, r + 16)
    is_mem_key = (c >= 40) & (c < 56)
    is_mem_q = (r >= 8) & (r < 16)
    allow_o = exist_o & (is_mem_key | is_mem_q | (ktok <= qtok))
    fill_o = jnp.where(exist_o, NEG, -jnp.inf).astype(f32)
    return allow_e, fill_e, allow_o, fill_o


def _softmax(s, allow, fill):
    s = jnp.where(allow, s * SCALE, fill)
    m = jnp.max(s, axis=-1, keepdims=True)
    e = jnp.exp(s - m)
    l = jnp.sum(e, axis=-1, keepdims=True)
    r = pl.reciprocal(l, approx=True)
    r = r * (2.0 - l * r)
    return (e * r).astype(bf16)


def _kernel(x_hbm, mem0_hbm, wq_hbm, wk_hbm, wv_hbm, wo_hbm, w1_hbm, w2_hbm, w3_hbm, w4_hbm,
            gw_hbm, out_hbm,
            x_v, s1_v, s2_v, s3_v, s4_v, wqkv_v, wo_v, h_v, b_v, l_v, n_v, g_v, out_v,
            ke_v, ve_v, o_v, mem_v, mem0_ref, gw_ref, zero_s,
            sem, sem_qkv, sem_out):
    RAW = (1, 2, 3, 4)
    RAW1 = (1, 7, 8, 4)

    loads = []

    def rows_load(name, r0, r1):
        loads.append((name, x_hbm.at[pl.ds(r0, r1 - r0)], x_v.at[pl.ds(r0, r1 - r0)]))

    def quad_load(name, w_hbm, s_v, raw, q, c0=0, c1=None):
        k4, n2 = s_v.shape[1], s_v.shape[2]
        c1 = n2 if c1 is None else c1
        src = w_hbm.bitcast(u32).at[pl.ds((q // 2) * k4, k4), pl.ds((q % 2) * n2 + c0, c1 - c0)]
        loads.append((name, src, s_v.at[raw[q], :, pl.ds(c0, c1 - c0)]))

    rows_load("x0", 0, TM)
    rows_load("x1", TM, 2 * TM)
    for name, half, c0, c1 in (("w1a", 0, 0, 256), ("w1bc", 0, 256, 512), ("w1bc", 1, 0, 256), ("w1d", 1, 256, 512)):
        quad_load(name, w1_hbm, s1_v, RAW1, half, c0, c1)
        quad_load(name, w1_hbm, s1_v, RAW1, 2 + half, c0, c1)
    rows_load("x234", 2 * TM, 5 * TM)
    rows_load("x567", 5 * TM, S)
    for name, w_hbm, s_v in (("w2", w2_hbm, s2_v), ("w3", w3_hbm, s3_v), ("w4", w4_hbm, s4_v)):
        for q in range(4):
            quad_load(name, w_hbm, s_v, RAW, q)
    loads.append(("small", mem0_hbm, mem0_ref))
    loads.append(("small", gw_hbm, gw_ref))
    for j in range(NT):
        loads.append(("wo", wo_hbm.bitcast(u32).at[:, pl.ds(j * 128, 128)], wo_v.at[j]))
    groups = list(dict.fromkeys(name for name, _, _ in loads))
    assert len(groups) == NLOAD

    def start(*names, priority=0):
        for name, src, dst in loads:
            if name in names:
                pltpu.make_async_copy(src, dst, sem.at[groups.index(name)]).start(priority=priority)

    def wait(*names):
        for name, src, dst in loads:
            if name in names:
                pltpu.make_async_copy(src, dst, sem.at[groups.index(name)]).wait()

    SPG = 3 * G

    def qkv_start(g):
        for w, w_hbm in enumerate((wq_hbm, wk_hbm, wv_hbm)):
            wu = w_hbm.bitcast(u32)
            for k in range(G // 2):
                for par in range(2):
                    pltpu.make_async_copy(
                        wu.at[:, par * (H // 2) + g * (G // 2) + k, :],
                        wqkv_v.at[g * SPG + w * G + 2 * k + par], sem_qkv.at[g]).start(priority=1)

    def qkv_wait(g):
        grp = wqkv_v.at[pl.ds(g * SPG, SPG)]
        pltpu.make_async_copy(grp, grp, sem_qkv.at[g]).wait()

    start("x0", "x1", "w1a", "w1bc", "w1d", "x234", "x567", "w2", "w3", "w4", "small")
    zero_s[0] = 0

    def tile_idx(ref):
        z = zero_s[0]
        return (z,) * (len(ref.shape) - 2) + (pl.ds(pl.multiple_of(z, 8), 8), slice(0, 128))

    hist = []

    def mm(lhs, rhs, side=None, acc=None):
        if side is not None:
            lhs = side(lhs)
        lhs = pltpu.bitcast(lhs, bf16) if lhs.dtype == u32 else lhs.astype(bf16)
        y = _dot(lhs, pltpu.bitcast(rhs, bf16))
        if acc is not None:
            y = y + acc
        hist.append(y)
        return y

    class Side:
        def __init__(self, pieces, n):
            self.pieces, self.n = list(pieces), n

        def __call__(self, val):
            take = -(-len(self.pieces) // self.n) if self.pieces else 0
            self.n -= 1
            if not take:
                return val
            never = zero_s[0] > 0
            rg = 8 if val.dtype == u32 else 16
            ng = val.shape[0] // rg
            groups = [val[8 * m:8 * m + 8] for m in range(val.shape[0] // 8)]
            for j, (fn, rd, wr, lag) in enumerate(self.pieces[:take]):
                m = (j + 1) * ng // take - 1
                pin = lambda v: v
                if lag is not None and len(hist) >= lag:
                    r0 = (16 * m) % hist[-lag].shape[0]
                    a = hist[-lag][r0:r0 + 8, :128]
                    if rd is None:
                        def pin(v, a=a):
                            t = jnp.where(never, jnp.concatenate([a] * (v.shape[0] // 8), axis=0), v[:, :128])
                            return t if v.shape[1] == 128 else jnp.concatenate([t, v[:, 128:]], axis=1)
                    else:
                        idx = tile_idx(rd)
                        rd[idx] = jnp.where(never, pltpu.bitcast(a, rd.dtype), rd[idx])
                fn(pin)
                g = m * rg // 8
                t = jnp.where(never, pltpu.bitcast(wr[tile_idx(wr)], val.dtype), groups[g][:, -128:])
                groups[g] = jnp.concatenate([groups[g][:, :-128], t], axis=1)
            self.pieces = self.pieces[take:]
            return jnp.concatenate(groups, axis=0)

    def strassen(lhs, rhs, side, init=(None, None, None, None), ks=range(7)):
        def add(a, b):
            return a if b is None else a + b
        sd = lambda k: side if k in ks else None
        p = [mm(lhs(k), rhs(k), sd(k)) for k in range(5)]
        c12 = add(p[2] + p[4], init[1])
        c21 = add(p[1] + p[3], init[2])
        c22 = mm(lhs(5), rhs(5), sd(5), add(p[0] - p[1] + p[2], init[3]))
        c11 = mm(lhs(6), rhs(6), sd(6), add(p[0] + p[3] - p[4], init[0]))
        return c11, c12, c21, c22

    def prep_pieces(s_v, raw, lag, width=256):
        def piece(r, c, pin):
            idx = (slice(r, r + 8), slice(c, c + width))
            b11, b12, b21, b22 = [_unpack(s_v[(q,) + idx]) for q in raw]
            for k, t in ((0, b11 + b22), (2, b12 - b22), (3, b21 - b11), (5, b11 + b12), (6, b21 + b22)):
                s_v[(k,) + idx] = _pack(t)
        return [(functools.partial(piece, r, c), s_v, s_v, lag)
                for r in range(0, s_v.shape[1], 8) for c in range(0, s_v.shape[2], width)]

    def store_l(slot, q, c, quads, plain=False):
        for k, t in enumerate(quads if plain else _lcombos(*quads)):
            l_v[slot, k, q // 2:q // 2 + 8, c:c + t.shape[1]] = _pack(t)

    def ln_pieces(src, r0, slot, lag, plain=False, width=256, staged=False, clag=None):
        def stats(q, pin):
            x = pin(src[pl.ds(r0 + q, 16), :].astype(f32))
            xs = [x[:, j * 128:(j + 1) * 128] for j in range(NT)]
            m = functools.reduce(lambda a, b: a + b, xs) * (1.0 / NT)
            w = functools.reduce(lambda a, b: a + b, [(t - m) * (t - m) for t in xs])
            mean = jnp.mean(m, axis=-1, keepdims=True)
            var = jnp.sum(w + NT * ((m - mean) * (m - mean)), axis=-1, keepdims=True) * (1.0 / D)
            n_v[0, q:q + 16, :] = jnp.broadcast_to(mean, (16, 128))
            n_v[1, q:q + 16, :] = jnp.broadcast_to(lax.rsqrt(var + EPS), (16, 128))

        def comb(q, c, pin):
            quads = []
            for rr in (0, HM):
                rs = pl.ds(pl.multiple_of(r0 + rr + q + zero_s[0], 16), 16)
                mean, rstd = [jnp.concatenate([n_v[t, rr + q:rr + q + 16, :]] * (width // 128), axis=1)
                              for t in range(2)]
                quads += [(src[rs, cc + c:cc + c + width].astype(f32) - mean) * rstd for cc in (0, DH2)]
            store_l(slot, q, c, quads, plain)
        norms = [[(functools.partial(stats, rr + q), None, n_v, lag) for rr in (0, HM)] for q in range(0, HM, 16)]
        combs = [[(functools.partial(comb, q, c), n_v, l_v, clag) for c in range(0, DH2, width)]
                 for q in range(0, HM, 16)]
        if staged:
            return sum(norms, []), sum(combs, [])
        out = list(norms[0])
        for a, b in zip(norms[1:] + [[]], combs):
            out += _merge(a, b) if a else b
        return out

    shifts = (1, 1, -1, -1, 2, 2, -2, -2)

    def shift_pieces(r0, slot, lag, by_value=False):
        def piece(q, j, pin):
            a = [h_v[jj, pl.ds(PAD + r0 + rr + q - shifts[jj], 16), :]
                 for rr in (0, HM) for jj in (j, j + NT // 2)]
            store_l(slot, q, j * 128, [pin(a[0]), a[1], a[2], pin(a[3])])
        return [(functools.partial(piece, q, j), None if by_value else h_v, l_v, lag)
                for q in range(0, HM, 16) for j in range(NT // 2)]

    def lhs_of(slot):
        return lambda k: l_v[slot, k]

    h_v[:, 0:PAD, :] = jnp.zeros((NT, PAD, 128), f32)
    h_v[:, PAD + S:PAD + S + PAD, :] = jnp.zeros((NT, PAD, 128), f32)

    def store_h(r0, c0, h):
        for j in range(h.shape[1] // 128):
            h_v[c0 // 128 + j, PAD + r0:PAD + r0 + h.shape[0], :] = h[:, j * 128:(j + 1) * 128]

    def d1_plain(xn, r0, c0, c1, step, side=None):
        for c in range(c0, c1, step):
            half, cc = c // DH2, c % DH2
            w = jnp.concatenate([s1_v[RAW1[half], :, cc:cc + step], s1_v[RAW1[2 + half], :, cc:cc + step]], axis=0)
            store_h(r0, c, _gelu(mm(xn, w, side)))

    NP1 = 7 * (DH2 // NC1)
    KS1 = (2, 3, 4, 5)

    def d1_s(b, slot, pieces):
        side = Side(pieces, len(KS1) * (DH2 // NC1))
        for c in range(0, DH2, NC1):
            cs = strassen(lhs_of(slot), lambda k: s1_v[k, :, c:c + NC1], side, ks=KS1)
            for q, t in enumerate(cs):
                store_h(b * TM + (q // 2) * HM, (q % 2) * DH2 + c, _gelu(t))

    def d2_s(b, slot, pieces):
        side = Side(pieces, NP1)
        for c in range(0, DH2, NC1):
            idx = [(slice(b * TM + (q // 2) * HM, b * TM + (q // 2 + 1) * HM),
                    slice((q % 2) * DH2 + c, (q % 2) * DH2 + c + NC1)) for q in range(4)]
            cs = strassen(lhs_of(slot), lambda k: s2_v[k, :, c:c + NC1], side,
                          [x_v[i].astype(f32) for i in idx])
            for i, t in zip(idx, cs):
                b_v[i] = t

    def split(l, n):
        return [l[len(l) * i // n:len(l) * (i + 1) // n] for i in range(n)]

    LS, LL = 3, 5

    wait("x0")
    xn0 = _pack(_ln(x_v[0:TM, :].astype(f32)))
    wait("x1")
    xn01 = jnp.concatenate([xn0, _pack(_ln(x_v[TM:2 * TM, :].astype(f32)))], axis=0)
    wait("w1a")
    d1_plain(xn01, 0, 0, 256, 256)
    wait("w1bc")
    d1_plain(xn01, 0, 256, 768, 256)
    wait("w1d", "x234")
    hist.clear()
    d1_plain(xn01, 0, 768, D, 128, Side(ln_pieces(x_v, 2 * TM, 0, None, plain=True), 2))
    xn2 = jnp.concatenate([jnp.concatenate([l_v[0, 2 * h], l_v[0, 2 * h + 1]], axis=1) for h in range(2)], axis=0)
    d1_plain(xn2, 2 * TM, 0, D, 128,
             Side(_merge(prep_pieces(s1_v, RAW1, 1), ln_pieces(x_v, 3 * TM, 1, 2)), 8))
    d1_s(3, 1, ln_pieces(x_v, 4 * TM, 0, LL))
    wait("x567", "w2")
    qkv_start(0)
    qkv_start(1)
    hist.clear()
    pw = split(prep_pieces(s2_v, RAW, LS), 4)
    for b in range(4, NB):
        nxt = ln_pieces(x_v, (b + 1) * TM, (b + 1) % 2, LL) if b + 1 < NB else shift_pieces(0, 0, LS, True)
        d1_s(b, b % 2, _merge(pw[b - 4], nxt))
    d2_s(0, 0, shift_pieces(TM, 1, LS, True))
    wait("w3")
    hist.clear()
    pw = split(prep_pieces(s3_v, RAW, LS), 4)
    for b in range(1, 5):
        d2_s(b, b % 2, _merge(pw[b - 1], shift_pieces((b + 1) * TM, (b + 1) % 2, LS)))
    wait("w4", "small")
    hist.clear()
    pw = prep_pieces(s4_v, RAW, LS)
    pw = [pw[:82], pw[82:164], pw[164:]]
    for b in range(5, NB):
        nxt = shift_pieces((b + 1) * TM, (b + 1) % 2, LS) if b + 1 < NB else ln_pieces(b_v, 0, 0, LL)
        d2_s(b, b % 2, _merge(pw[b - 5], nxt))
    start("wo", priority=1)

    def ffn(i, carry):
        qkv_wait(i)
        r0 = pl.multiple_of(i * TM, TM)
        rn = pl.multiple_of(jnp.minimum(i + 1, NB - 1) * TM, TM)
        lh = {}
        acc = [None] * 7
        hist.clear()

        def relayout(p, r0_, r1_, pin):
            s0 = i * SPG + 2 * p
            for r in range(r0_, r1_, 8):
                e = wqkv_v[s0, r:r + 8, :]
                o = wqkv_v[s0 + 1, r:r + 8, :]
                wqkv_v[s0, r:r + 8, :] = (e & jnp.uint32(0xFFFF)) | (o << 16)
                wqkv_v[s0 + 1, r:r + 8, :] = (e >> 16) | (o & jnp.uint32(0xFFFF0000))

        side3 = Side([(functools.partial(relayout, p, r, r + 32), wqkv_v, wqkv_v, 2)
                      for p in range(SPG // 2) for r in range(0, D // 2, 32)], 42 + 5)
        norms, combs = ln_pieces(b_v, rn, 0, 3, staged=True, width=128, clag=2)

        def gate(q, pin):
            gw = gw_ref[...].astype(f32)
            x = pin(x_v[pl.ds(r0 + q, 16), :].astype(f32))
            t = functools.reduce(lambda a, b: a + b,
                                 [x[:, j * 128:(j + 1) * 128] * gw[j:j + 1, :] for j in range(NT)])
            g = jax.nn.sigmoid(jnp.sum(t, axis=-1, keepdims=True))
            g_v[pl.ds(r0 + q, 16), :] = jnp.broadcast_to(g, (16, 128))

        gates = [(functools.partial(gate, q), None, g_v, 3) for q in range(0, TM, 16)]
        side4 = Side(_merge(norms, gates), 20)
        side5 = Side(combs, 11)

        def d3(c):
            cs = strassen(lhs_of(0), lambda k: s3_v[k, :, c * FC:(c + 1) * FC],
                          side3 if c > 0 else (lambda v: side3(v) if len(hist) >= 2 else v))
            lh[c] = _lcombos(*[_gelu(t) for t in cs])

        def d4(c):
            l = lh.pop(c)
            rhs = lambda k: s4_v[k, c * FC // 2:(c + 1) * FC // 2, :]
            if c + 1 < NFC:
                for k in range(7):
                    side = (side5 if k > 0 else None) if c == NFC - 2 else (side4 if k >= 3 else None)
                    acc[k] = mm(l[k], rhs(k), side, acc[k])
                return
            q = [mm(l[k], rhs(k), side5, acc[k]) for k in range(5)]
            top, bot = pl.ds(r0, HM), pl.ds(r0 + HM, HM)
            gt, gb = [jnp.concatenate([1.0 - g_v[r, :]] * (NT // 2), axis=1) for r in (top, bot)]
            b_v[top, DH2:] = gt * (q[2] + q[4] + b_v[top, DH2:])
            b_v[bot, :DH2] = gb * (q[1] + q[3] + b_v[bot, :DH2])
            b_v[bot, DH2:] = gb * mm(l[5], rhs(5), None, acc[5] + q[0] - q[1] + q[2] + b_v[bot, DH2:])
            b_v[top, :DH2] = gt * mm(l[6], rhs(6), None, acc[6] + q[0] + q[3] - q[4] + b_v[top, :DH2])

        d3(0)
        for c in range(NFC):
            if c + 1 < NFC:
                d3(c + 1)
            d4(c)
        assert not side3.pieces and not side4.pieces and not side5.pieces

        @pl.when(i + 2 < NG)
        def _():
            qkv_start(i + 2)

        return carry

    lax.fori_loop(0, NB, ffn, 0)

    wait("wo")
    mem_v[...] = mem0_ref[...].astype(f32)

    def wload(w, h):
        return pltpu.bitcast(wqkv_v[(h // G) * SPG + w * G + h % G], bf16)

    def step(hq, hkv, odd, allow, fill):
        nq = hq.shape[0]
        qs, ks, vs, ps = {}, {}, {}, {}

        def proj(g):
            lhs = (hq, hkv, hkv)
            part = {}
            if odd and g == 0:
                for h in range(2):
                    for w in range(3):
                        part[w, h] = _dot(lhs[w][:, :DH2], wload(w, h)[:DH2])
            for h in range(g * G, (g + 1) * G):
                q, k, v = [(_dot(lhs[w][:, DH2:], wload(w, h)[DH2:]) + part[w, h] if (w, h) in part
                            else _dot(lhs[w], wload(w, h))).astype(bf16) for w in range(3)]
                qs[h] = q
                if odd:
                    k = jnp.concatenate([pltpu.bitcast(ke_v[h], bf16), k], axis=0)
                    v = jnp.concatenate([pltpu.bitcast(ve_v[h], bf16), v], axis=0)
                else:
                    ke_v[h] = pltpu.bitcast(k, u32)
                    ve_v[h] = pltpu.bitcast(v, u32)
                ks[h] = k
                vs[h] = v

        def score(g):
            for h in range(g * G, (g + 1) * G):
                s = lax.dot_general(qs.pop(h), ks.pop(h), (((1,), (1,)), ((), ())),
                                    preferred_element_type=f32)
                ps[h] = _softmax(s, allow, fill)

        def pv(g):
            for h in range(g * G, (g + 1) * G):
                o = _dot(ps.pop(h), vs.pop(h)).astype(bf16)
                o_v[0:nq // 2, h * 128:(h + 1) * 128] = pltpu.bitcast(o, u32)

        acc = [None] * NT

        def wo(h0, h1, j0, j1):
            o = pltpu.bitcast(o_v[0:nq // 2, h0 * 128:h1 * 128], bf16)
            for j in range(j0, j1):
                y = _dot(o, pltpu.bitcast(wo_v[j, h0 * 64:h1 * 64, :], bf16))
                acc[j] = y if acc[j] is None else y + acc[j]

        for t in range(NG):
            proj(t)
            if t >= 1:
                score(t - 1)
            if t >= 2:
                pv(t - 2)
        wo(0, 16, 0, 4)
        score(NG - 1)
        pv(NG - 2)
        wo(0, 16, 4, 8)
        pv(NG - 1)
        wo(16, 24, 0, 8)
        wo(24, 32, 0, 8)
        return jnp.concatenate(acc, axis=1)

    def pair(j, carry):
        r0 = pl.multiple_of(j * 64, 64)
        mem = mem_v[...]
        allow_e, fill_e, allow_o, fill_o = _masks()
        x0 = x_v[pl.ds(r0, 16), :]
        x1 = x_v[pl.ds(r0 + 16, 16), :]
        x2 = x_v[pl.ds(r0 + 32, 16), :]
        x3 = x_v[pl.ds(r0 + 48, 16), :]
        x1f = x1.astype(f32)
        x2f = x2.astype(f32)
        hq = jnp.concatenate([x0, jnp.concatenate([x1f[:8], mem], 0).astype(bf16)], 0)
        hkv = jnp.concatenate([x0, x1, jnp.concatenate([x2f[:8], mem], 0).astype(bf16)], 0)
        oe = step(hq, hkv, False, allow_e, fill_e)
        mem = oe[24:32]
        hq = jnp.concatenate([jnp.concatenate([x1f[8:], mem], 0).astype(bf16), x2, x3], 0)
        hkv = jnp.concatenate([jnp.concatenate([mem, x2f[8:]], 0).astype(bf16), x3], 0)
        oo = step(hq, hkv, True, allow_o, fill_o)
        a = jnp.concatenate([oe[:24], oo[:8], oo[16:]], 0)
        mem_v[...] = oo[8:16]
        g = jnp.concatenate([g_v[pl.ds(r0, 64), :]] * NT, axis=1)
        out_v[pl.ds(r0, 64), :] = (g * a + b_v[pl.ds(r0, 64), :]).astype(bf16)
        pltpu.make_async_copy(out_v.at[pl.ds(r0, 64)], out_hbm.at[pl.ds(r0, 64)], sem_out).start()
        return carry

    lax.fori_loop(0, NPAIR, pair, 0)
    pltpu.make_async_copy(out_v, out_hbm, sem_out).wait()


@functools.partial(jax.jit, static_argnames=("A_seg_len",))
def pallas_gated_mix__memory_aug_recurrent_mem_tr__mixer_s_mlp__prompt_kernel(
    A_x, A_mem0, A_Wq, A_Wk, A_Wv, A_Wo, A_seg_len, B_x, B_w1, B_w2, B_w3, B_w4, gate_w,
):
    assert A_seg_len == SEG
    assert A_x.shape == (1, S, D) and A_mem0.shape == (1, M, D)
    any_spec = pl.BlockSpec(memory_space=pl.ANY)
    out = pl.pallas_call(
        _kernel,
        out_shape=jax.ShapeDtypeStruct((S, D), bf16),
        in_specs=[any_spec] * 11,
        out_specs=any_spec,
        scratch_shapes=[
            pltpu.VMEM((S, D), bf16),
            pltpu.VMEM((9, D // 4, D // 2), u32),
            pltpu.VMEM((7, D // 4, D // 2), u32),
            pltpu.VMEM((7, D // 4, F // 2), u32),
            pltpu.VMEM((7, F // 4, D // 2), u32),
            pltpu.VMEM((3 * H, D // 2, DH), u32),
            pltpu.VMEM((NT, H * DH // 2, 128), u32),
            pltpu.VMEM((NT, S + 2 * PAD, 128), f32),
            pltpu.VMEM((S, D), f32),
            pltpu.VMEM((2, 7, HM // 2, D // 2), u32),
            pltpu.VMEM((2, TM, 128), f32),
            pltpu.VMEM((S, 128), f32),
            pltpu.VMEM((S, D), bf16),
            pltpu.VMEM((H, 24, 128), u32),
            pltpu.VMEM((H, 24, 128), u32),
            pltpu.VMEM((24, H * DH), u32),
            pltpu.VMEM((M, D), f32),
            pltpu.VMEM((M, D), bf16),
            pltpu.VMEM((NT, 128), bf16),
            pltpu.SMEM((1,), jnp.int32),
            pltpu.SemaphoreType.DMA((NLOAD,)),
            pltpu.SemaphoreType.DMA((NG,)),
            pltpu.SemaphoreType.DMA,
        ],
        compiler_params=pltpu.CompilerParams(vmem_limit_bytes=120 * 1024 * 1024,
                                             disable_bounds_checks=True),
    )(
        A_x.reshape(S, D), A_mem0.reshape(M, D),
        A_Wq.reshape(D // 2, 2 * H, DH), A_Wk.reshape(D // 2, 2 * H, DH), A_Wv.reshape(D // 2, 2 * H, DH),
        A_Wo.reshape(H * DH, D), B_w1, B_w2, B_w3, B_w4, gate_w.reshape(NT, 128),
    )
    return out.reshape(1, S, D)
```

```python
import functools

import jax
import jax.numpy as jnp
from jax import lax
import jax.experimental.pallas as pl
import jax.experimental.pallas.tpu as pltpu

f32, bf16, u32 = jnp.float32, jnp.bfloat16, jnp.uint32

S, D, H, DH, M, SEG, F = 2048, 1024, 32, 128, 8, 32, 3584
SCALE = DH ** -0.5
NEG = -1000000000.0
EPS = 1e-05

TM = 256
NB = S // TM
HM = TM // 2
DH2 = D // 2
FH = F // 2
FC = 256
NFC = FH // FC
NC1 = 128
NPAIR = S // (2 * SEG)
NPRE = 4
G = 4
NG = H // G
PAD = 8
NT = D // 128
NLOAD = 12
assert NB == NG

_dot = functools.partial(jnp.dot, preferred_element_type=f32)


def _ln(x):
    m = jnp.mean(x, axis=-1, keepdims=True)
    xc = x - m
    v = jnp.mean(xc * xc, axis=-1, keepdims=True)
    return xc * lax.rsqrt(v + EPS)


_GC = 0.7978845608028654


def _gelu(x):
    h = 0.5 * x
    return h + h * jnp.tanh(x * (_GC + (_GC * 0.044715) * (x * x)))


def _unpack(u):
    return pltpu.bitcast(u, bf16).astype(f32)


def _pack(x):
    return pltpu.bitcast(x.astype(bf16), u32)


def _lcombos(a11, a12, a21, a22):
    return [a11 + a22, a21 + a22, a11, a22, a11 + a12, a21 - a11, a12 - a22]


def _merge(*lists):
    keyed = [((j + 0.5) / len(l), n, j, v) for n, l in enumerate(lists) for j, v in enumerate(l)]
    return [v for _, _, _, v in sorted(keyed, key=lambda t: t[:3])]


def _masks():
    r = lax.broadcasted_iota(jnp.int32, (32, 48), 0)
    c = lax.broadcasted_iota(jnp.int32, (32, 48), 1)
    exist_e = c < 40
    allow_e = exist_e & ((r >= 24) | ((c >= 24) & (c < 32)) | (c <= r))
    fill_e = jnp.where(exist_e, NEG, -jnp.inf).astype(f32)
    r = lax.broadcasted_iota(jnp.int32, (48, 80), 0)
    c = lax.broadcasted_iota(jnp.int32, (48, 80), 1)
    q_even = (r >= 32) & (r < 40)
    exist_o = (q_even & (c < 40)) | (~q_even & (c >= 40))
    ktok = jnp.where(c < 24, c, jnp.where(c < 48, c - 8, c - 16))
    qtok = jnp.where(r < 32, r + 32, r - 8)
    is_mem_key = ((c >= 24) & (c < 32)) | ((c >= 48) & (c < 56))
    allow_o = exist_o & (is_mem_key | (r < 8) | (ktok <= qtok))
    fill_o = jnp.where(exist_o, NEG, -jnp.inf).astype(f32)
    return allow_e, fill_e, allow_o, fill_o


def _rcombo(k, b11, b12, b21, b22):
    if k in (1, 4):
        return (b11 if k == 1 else b22)()
    a, b, sign = {0: (b11, b22, 1), 2: (b12, b22, -1), 3: (b21, b11, -1), 5: (b11, b12, 1), 6: (b21, b22, 1)}[k]
    a, b = _unpack(a()), _unpack(b())
    return (a + b if sign > 0 else a - b).astype(bf16)


def _softmax(s, allow, fill):
    s = jnp.where(allow, s * SCALE, fill)
    m = jnp.max(s, axis=-1, keepdims=True)
    e = jnp.exp(s - m)
    l = jnp.sum(e, axis=-1, keepdims=True)
    r = pl.reciprocal(l, approx=True)
    r = r * (2.0 - l * r)
    return (e * r).astype(bf16)


def _kernel(x_hbm, mem0_hbm, wq_hbm, wk_hbm, wv_hbm, wo_hbm, w1_hbm, w2_hbm, w3_hbm, w4_hbm,
            gw_hbm, out_hbm,
            x_v, s1_v, s2_v, s3_v, s4_v, wqkv_v, wo_v, h_v, b_v, l_v, n_v, g_v, out_v, xe_v, e_v, oe_v,
            ke_v, ve_v, o_v, mem_v, mem0_ref, gw_ref, zero_s,
            sem, sem_qkv, sem_out):
    RAW = (1, 2, 3, 4)
    RAW1 = (1, 7, 8, 4)

    loads = []

    def rows_load(name, r0, r1):
        loads.append((name, x_hbm.at[pl.ds(r0, r1 - r0)], x_v.at[pl.ds(r0, r1 - r0)]))

    def quad_load(name, w_hbm, s_v, raw, q, c0=0, c1=None):
        k4, n2 = s_v.shape[1], s_v.shape[2]
        c1 = n2 if c1 is None else c1
        src = w_hbm.bitcast(u32).at[pl.ds((q // 2) * k4, k4), pl.ds((q % 2) * n2 + c0, c1 - c0)]
        loads.append((name, src, s_v.at[raw[q], :, pl.ds(c0, c1 - c0)]))

    rows_load("x0", 0, TM)
    rows_load("x1", TM, 2 * TM)
    for name, half, c0, c1 in (("w1a", 0, 0, 256), ("w1bc", 0, 256, 512), ("w1bc", 1, 0, 256), ("w1d", 1, 256, 512)):
        quad_load(name, w1_hbm, s1_v, RAW1, half, c0, c1)
        quad_load(name, w1_hbm, s1_v, RAW1, 2 + half, c0, c1)
    rows_load("x234", 2 * TM, 5 * TM)
    rows_load("x567", 5 * TM, S)
    for name, w_hbm, s_v in (("w2", w2_hbm, s2_v), ("w3", w3_hbm, s3_v), ("w4", w4_hbm, s4_v)):
        for q in range(4):
            quad_load(name, w_hbm, s_v, RAW, q)
    loads.append(("small", mem0_hbm, mem0_ref))
    loads.append(("small", gw_hbm, gw_ref))
    for j in range(NT):
        loads.append(("wo", wo_hbm.bitcast(u32).at[:, pl.ds(j * 128, 128)], wo_v.at[j]))
    groups = list(dict.fromkeys(name for name, _, _ in loads))
    assert len(groups) == NLOAD

    def start(*names, priority=0):
        for name, src, dst in loads:
            if name in names:
                pltpu.make_async_copy(src, dst, sem.at[groups.index(name)]).start(priority=priority)

    def wait(*names):
        for name, src, dst in loads:
            if name in names:
                pltpu.make_async_copy(src, dst, sem.at[groups.index(name)]).wait()

    SPG = 3 * G

    def qkv_start(g):
        for w, w_hbm in enumerate((wq_hbm, wk_hbm, wv_hbm)):
            wu = w_hbm.bitcast(u32)
            for k in range(G // 2):
                for par in range(2):
                    pltpu.make_async_copy(
                        wu.at[:, par * (H // 2) + g * (G // 2) + k, :],
                        wqkv_v.at[g * SPG + w * G + 2 * k + par], sem_qkv.at[g]).start(priority=1)

    def qkv_wait(g):
        grp = wqkv_v.at[pl.ds(g * SPG, SPG)]
        pltpu.make_async_copy(grp, grp, sem_qkv.at[g]).wait()

    start("x0", "x1", "w1a", "w1bc", "w1d", "x234", "x567", "w2", "w3", "w4", "small")
    zero_s[0] = 0

    def tile_idx(ref):
        z = zero_s[0]
        return (z,) * (len(ref.shape) - 2) + (pl.ds(pl.multiple_of(z, 8), 8), slice(0, 128))

    hist = []

    def mm(lhs, rhs, side=None, acc=None):
        if side is not None:
            lhs = side(lhs)
        lhs = pltpu.bitcast(lhs, bf16) if lhs.dtype == u32 else lhs.astype(bf16)
        y = _dot(lhs, pltpu.bitcast(rhs, bf16) if rhs.dtype == u32 else rhs)
        if acc is not None:
            y = y + acc
        hist.append(y)
        return y

    class Side:
        def __init__(self, pieces, n):
            self.pieces, self.n = list(pieces), n

        def __call__(self, val):
            take = -(-len(self.pieces) // self.n) if self.pieces else 0
            self.n -= 1
            if not take:
                return val
            never = zero_s[0] > 0
            rg = 8 if val.dtype == u32 else 16
            ng = val.shape[0] // rg
            groups = [val[8 * m:8 * m + 8] for m in range(val.shape[0] // 8)]
            for j, (fn, rd, wr, lag) in enumerate(self.pieces[:take]):
                m = (j + 1) * ng // take - 1
                pin = lambda v: v
                if lag is not None and len(hist) >= lag:
                    r0 = (16 * m) % hist[-lag].shape[0]
                    a = hist[-lag][r0:r0 + 8, :128]
                    if rd is None:
                        def pin(v, a=a):
                            t = jnp.where(never, jnp.concatenate([a] * (v.shape[0] // 8), axis=0), v[:, :128])
                            return t if v.shape[1] == 128 else jnp.concatenate([t, v[:, 128:]], axis=1)
                    else:
                        idx = tile_idx(rd)
                        rd[idx] = jnp.where(never, pltpu.bitcast(a, rd.dtype), rd[idx])
                fn(pin)
                g = m * rg // 8
                t = jnp.where(never, pltpu.bitcast(wr[tile_idx(wr)], val.dtype), groups[g][:, -128:])
                groups[g] = jnp.concatenate([groups[g][:, :-128], t], axis=1)
            self.pieces = self.pieces[take:]
            return jnp.concatenate(groups, axis=0)

    def strassen(lhs, rhs, side, init=(None, None, None, None), ks=range(7)):
        def add(a, b):
            return a if b is None else a + b
        sd = lambda k: side if k in ks else None
        p = [mm(lhs(k), rhs(k), sd(k)) for k in range(5)]
        c12 = add(p[2] + p[4], init[1])
        c21 = add(p[1] + p[3], init[2])
        c22 = mm(lhs(5), rhs(5), sd(5), add(p[0] - p[1] + p[2], init[3]))
        c11 = mm(lhs(6), rhs(6), sd(6), add(p[0] + p[3] - p[4], init[0]))
        return c11, c12, c21, c22

    def prep_pieces(s_v, raw, lag, width=256):
        def piece(r, c, pin):
            idx = (slice(r, r + 8), slice(c, c + width))
            b11, b12, b21, b22 = [_unpack(s_v[(q,) + idx]) for q in raw]
            for k, t in ((0, b11 + b22), (2, b12 - b22), (3, b21 - b11), (5, b11 + b12), (6, b21 + b22)):
                s_v[(k,) + idx] = _pack(t)
        return [(functools.partial(piece, r, c), s_v, s_v, lag)
                for r in range(0, s_v.shape[1], 8) for c in range(0, s_v.shape[2], width)]

    def store_l(slot, q, c, quads, plain=False):
        for k, t in enumerate(quads if plain else _lcombos(*quads)):
            l_v[slot, k, q // 2:q // 2 + 8, c:c + t.shape[1]] = _pack(t)

    def ln_pieces(src, r0, slot, lag, plain=False, width=256, staged=False, clag=None):
        def stats(q, pin):
            x = pin(src[pl.ds(r0 + q, 16), :].astype(f32))
            xs = [x[:, j * 128:(j + 1) * 128] for j in range(NT)]
            m = functools.reduce(lambda a, b: a + b, xs) * (1.0 / NT)
            w = functools.reduce(lambda a, b: a + b, [(t - m) * (t - m) for t in xs])
            mean = jnp.mean(m, axis=-1, keepdims=True)
            var = jnp.sum(w + NT * ((m - mean) * (m - mean)), axis=-1, keepdims=True) * (1.0 / D)
            n_v[0, q:q + 16, :] = jnp.broadcast_to(mean, (16, 128))
            n_v[1, q:q + 16, :] = jnp.broadcast_to(lax.rsqrt(var + EPS), (16, 128))

        def comb(q, c, pin):
            quads = []
            for rr in (0, HM):
                rs = pl.ds(pl.multiple_of(r0 + rr + q + zero_s[0], 16), 16)
                mean, rstd = [jnp.concatenate([n_v[t, rr + q:rr + q + 16, :]] * (width // 128), axis=1)
                              for t in range(2)]
                quads += [(src[rs, cc + c:cc + c + width].astype(f32) - mean) * rstd for cc in (0, DH2)]
            store_l(slot, q, c, quads, plain)
        norms = [[(functools.partial(stats, rr + q), None, n_v, lag) for rr in (0, HM)] for q in range(0, HM, 16)]
        combs = [[(functools.partial(comb, q, c), n_v, l_v, clag) for c in range(0, DH2, width)]
                 for q in range(0, HM, 16)]
        if staged:
            return sum(norms, []), sum(combs, [])
        out = list(norms[0])
        for a, b in zip(norms[1:] + [[]], combs):
            out += _merge(a, b) if a else b
        return out

    shifts = (1, 1, -1, -1, 2, 2, -2, -2)

    def shift_pieces(r0, slot, lag, by_value=False):
        def piece(q, j, pin):
            a = [h_v[jj, pl.ds(PAD + r0 + rr + q - shifts[jj], 16), :]
                 for rr in (0, HM) for jj in (j, j + NT // 2)]
            store_l(slot, q, j * 128, [pin(a[0]), a[1], a[2], pin(a[3])])
        return [(functools.partial(piece, q, j), None if by_value else h_v, l_v, lag)
                for q in range(0, HM, 16) for j in range(NT // 2)]

    def lhs_of(slot):
        return lambda k: l_v[slot, k]

    h_v[:, 0:PAD, :] = jnp.zeros((NT, PAD, 128), f32)
    h_v[:, PAD + S:PAD + S + PAD, :] = jnp.zeros((NT, PAD, 128), f32)

    def store_h(r0, c0, h):
        for j in range(h.shape[1] // 128):
            h_v[c0 // 128 + j, PAD + r0:PAD + r0 + h.shape[0], :] = h[:, j * 128:(j + 1) * 128]

    def d1_plain(xn, r0, c0, c1, step, side=None):
        for c in range(c0, c1, step):
            half, cc = c // DH2, c % DH2
            w = jnp.concatenate([s1_v[RAW1[half], :, cc:cc + step], s1_v[RAW1[2 + half], :, cc:cc + step]], axis=0)
            store_h(r0, c, _gelu(mm(xn, w, side)))

    NP1 = 7 * (DH2 // NC1)
    KS1 = (2, 3, 4, 5)

    def d1_s(b, slot, pieces):
        side = Side(pieces, len(KS1) * (DH2 // NC1))
        for c in range(0, DH2, NC1):
            cs = strassen(lhs_of(slot), lambda k: s1_v[k, :, c:c + NC1], side, ks=KS1)
            for q, t in enumerate(cs):
                store_h(b * TM + (q // 2) * HM, (q % 2) * DH2 + c, _gelu(t))

    def d2_s(b, slot, pieces):
        side = Side(pieces, NP1)
        for c in range(0, DH2, NC1):
            idx = [(slice(b * TM + (q // 2) * HM, b * TM + (q // 2 + 1) * HM),
                    slice((q % 2) * DH2 + c, (q % 2) * DH2 + c + NC1)) for q in range(4)]
            cs = strassen(lhs_of(slot), lambda k: s2_v[k, :, c:c + NC1], side,
                          [x_v[i].astype(f32) for i in idx])
            for i, t in zip(idx, cs):
                b_v[i] = t

    def split(l, n):
        return [l[len(l) * i // n:len(l) * (i + 1) // n] for i in range(n)]

    LS, LL = 3, 5

    wait("x0")
    xn0 = _pack(_ln(x_v[0:TM, :].astype(f32)))
    wait("x1")
    xn01 = jnp.concatenate([xn0, _pack(_ln(x_v[TM:2 * TM, :].astype(f32)))], axis=0)
    wait("w1a")
    d1_plain(xn01, 0, 0, 256, 256)
    wait("w1bc")
    d1_plain(xn01, 0, 256, 768, 256)
    wait("w1d", "x234")
    hist.clear()
    d1_plain(xn01, 0, 768, D, 128, Side(ln_pieces(x_v, 2 * TM, 0, None, plain=True), 2))
    xn2 = jnp.concatenate([jnp.concatenate([l_v[0, 2 * h], l_v[0, 2 * h + 1]], axis=1) for h in range(2)], axis=0)
    d1_plain(xn2, 2 * TM, 0, D, 128,
             Side(_merge(prep_pieces(s1_v, RAW1, 1), ln_pieces(x_v, 3 * TM, 1, 2)), 8))
    d1_s(3, 1, ln_pieces(x_v, 4 * TM, 0, LL))
    wait("x567", "w2")
    qkv_start(0)
    qkv_start(1)
    hist.clear()
    pw = split(prep_pieces(s2_v, RAW, LS), 4)
    for b in range(4, NB):
        nxt = ln_pieces(x_v, (b + 1) * TM, (b + 1) % 2, LL) if b + 1 < NB else shift_pieces(0, 0, LS, True)
        d1_s(b, b % 2, _merge(pw[b - 4], nxt))
    d2_s(0, 0, shift_pieces(TM, 1, LS, True))
    wait("w3")
    hist.clear()
    pw = split(prep_pieces(s3_v, RAW, LS), 4)
    for b in range(1, 5):
        d2_s(b, b % 2, _merge(pw[b - 1], shift_pieces((b + 1) * TM, (b + 1) % 2, LS)))
    wait("w4", "small")
    hist.clear()
    pw = prep_pieces(s4_v, RAW, LS)
    pw = [pw[:82], pw[82:164], pw[164:]]
    for b in range(5, NB):
        nxt = shift_pieces((b + 1) * TM, (b + 1) % 2, LS) if b + 1 < NB else ln_pieces(b_v, 0, 0, LL)
        d2_s(b, b % 2, _merge(pw[b - 5], nxt))
    start("wo", priority=1)

    def ffn(i, carry):
        qkv_wait(i)
        r0 = pl.multiple_of(i * TM, TM)
        rn = pl.multiple_of(jnp.minimum(i + 1, NB - 1) * TM, TM)
        lh = {}
        acc = [None] * 7
        hist.clear()

        def relayout(p, r0_, r1_, pin):
            s0 = i * SPG + 2 * p
            for r in range(r0_, r1_, 8):
                e = wqkv_v[s0, r:r + 8, :]
                o = wqkv_v[s0 + 1, r:r + 8, :]
                wqkv_v[s0, r:r + 8, :] = (e & jnp.uint32(0xFFFF)) | (o << 16)
                wqkv_v[s0 + 1, r:r + 8, :] = (e >> 16) | (o & jnp.uint32(0xFFFF0000))

        side3 = Side([(functools.partial(relayout, p, r, r + 32), wqkv_v, wqkv_v, 2)
                      for p in range(SPG // 2) for r in range(0, D // 2, 32)], 42 + 5)
        norms, combs = ln_pieces(b_v, rn, 0, 3, staged=True, width=128, clag=2)

        def gate(q, pin):
            gw = gw_ref[...].astype(f32)
            x = pin(x_v[pl.ds(r0 + q, 16), :].astype(f32))
            t = functools.reduce(lambda a, b: a + b,
                                 [x[:, j * 128:(j + 1) * 128] * gw[j:j + 1, :] for j in range(NT)])
            g = jax.nn.sigmoid(jnp.sum(t, axis=-1, keepdims=True))
            g_v[pl.ds(r0 + q, 16), :] = jnp.broadcast_to(g, (16, 128))

        gates = [(functools.partial(gate, q), None, g_v, 3) for q in range(0, TM, 16)]

        def extras(t, c, pin):
            jj = 2 * i + t
            a = [x_v[pl.ds(pl.multiple_of((jj + hh) * 64 + 24, 8), 16), cc + c:cc + c + 256].astype(f32)
                 for hh in (0, NPAIR // 2) for cc in (0, DH2)]
            for k, v in enumerate(_lcombos(pin(a[0]), a[1], a[2], pin(a[3]))):
                xe_v[k, pl.ds(pl.multiple_of(jj * 8, 8), 8), c:c + 256] = _pack(v)

        xes = [(functools.partial(extras, t, c), None, xe_v, 2) for t in range(2) for c in (0, 256)]
        side4 = Side(_merge(norms, gates, xes), 20)
        side5 = Side(combs, 11)

        def d3(c):
            cs = strassen(lhs_of(0), lambda k: s3_v[k, :, c * FC:(c + 1) * FC],
                          side3 if c > 0 else (lambda v: side3(v) if len(hist) >= 2 else v))
            lh[c] = _lcombos(*[_gelu(t) for t in cs])

        def d4(c):
            l = lh.pop(c)
            rhs = lambda k: s4_v[k, c * FC // 2:(c + 1) * FC // 2, :]
            if c + 1 < NFC:
                for k in range(7):
                    side = (side5 if k > 0 else None) if c == NFC - 2 else (side4 if k >= 3 else None)
                    acc[k] = mm(l[k], rhs(k), side, acc[k])
                return
            q = [mm(l[k], rhs(k), side5, acc[k]) for k in range(5)]
            top, bot = pl.ds(r0, HM), pl.ds(r0 + HM, HM)
            gt, gb = [jnp.concatenate([1.0 - g_v[r, :]] * (NT // 2), axis=1) for r in (top, bot)]
            b_v[top, DH2:] = gt * (q[2] + q[4] + b_v[top, DH2:])
            b_v[bot, :DH2] = gb * (q[1] + q[3] + b_v[bot, :DH2])
            b_v[bot, DH2:] = gb * mm(l[5], rhs(5), None, acc[5] + q[0] - q[1] + q[2] + b_v[bot, DH2:])
            b_v[top, :DH2] = gt * mm(l[6], rhs(6), None, acc[6] + q[0] + q[3] - q[4] + b_v[top, :DH2])

        d3(0)
        for c in range(NFC):
            if c + 1 < NFC:
                d3(c + 1)
            d4(c)
        assert not side3.pieces and not side4.pieces and not side5.pieces

        @pl.when(i + 2 < NG)
        def _():
            qkv_start(i + 2)

        return carry

    lax.fori_loop(0, NB, ffn, 0)

    def pre(it, carry):
        hist.clear()
        for u in range(3 * H // 2 // NPRE):
            s0 = it * (3 * H // NPRE) + 2 * u
            quad = [lambda s=s0 + q % 2, r=(q // 2) * (D // 4): wqkv_v[s, r:r + D // 4, :] for q in range(4)]
            cs = strassen(lambda k: xe_v[k], lambda k: _rcombo(k, *quad), None)
            for q, t in enumerate(cs):
                e_v[s0 + q % 2, (q // 2) * 128:(q // 2 + 1) * 128, :] = _pack(t)
        return carry

    lax.fori_loop(0, NPRE, pre, 0)

    wait("wo")
    mem_v[...] = mem0_ref[...].astype(f32)

    def slab(w, h):
        return (h // G) * SPG + w * G + h % G

    def step(j, hx, odd, allow, fill):
        qs, ks, vs, ps = {}, {}, {}, {}
        wload = lambda w, h: pltpu.bitcast(wqkv_v[slab(w, h)], bf16)
        eload = lambda w, h: pltpu.bitcast(e_v[slab(w, h), pl.ds(pl.multiple_of(j * 8, 8), 8), :], bf16)

        def proj(g):
            part = {}
            if odd and g == 0:
                for h in range(2):
                    for w in range(3):
                        part[w, h] = _dot(hx[:, :DH2], wload(w, h)[:DH2])
            for h in range(g * G, (g + 1) * G):
                q, k, v = [(_dot(hx[:, DH2:], wload(w, h)[DH2:]) + part[w, h] if (w, h) in part
                            else _dot(hx, wload(w, h))).astype(bf16) for w in range(3)]
                if odd:
                    q = jnp.concatenate([q, eload(0, h)], axis=0)
                    k = jnp.concatenate([pltpu.bitcast(ke_v[h], bf16), eload(1, h), k], axis=0)
                    v = jnp.concatenate([pltpu.bitcast(ve_v[h], bf16), eload(2, h), v], axis=0)
                else:
                    ke_v[h] = pltpu.bitcast(k, u32)
                    ve_v[h] = pltpu.bitcast(v, u32)
                    k = jnp.concatenate([k, eload(1, h)], axis=0)
                    v = jnp.concatenate([v, eload(2, h)], axis=0)
                qs[h], ks[h], vs[h] = q, k, v

        def score(g):
            for h in range(g * G, (g + 1) * G):
                s = lax.dot_general(qs.pop(h), ks.pop(h), (((1,), (1,)), ((), ())),
                                    preferred_element_type=f32)
                ps[h] = _softmax(s, allow, fill)

        def pv(g):
            os_ = []
            for h in range(g * G, (g + 1) * G):
                o = _dot(ps.pop(h), vs.pop(h))
                o_v[:, h * 128:(h + 1) * 128] = _pack(o[:32])
                os_.append(o)
            if odd:
                quads = [jnp.concatenate([os_[2 * kk][r:r + 8], os_[2 * kk + 1][r:r + 8]], axis=1)
                         for r in (32, 40) for kk in range(2)]
                for k, t in enumerate(_lcombos(*quads)):
                    oe_v[k, pl.ds(pl.multiple_of(j * 8, 8), 8), g * 256:(g + 1) * 256] = t.astype(bf16)

        acc = [None] * NT

        def wo(h0, h1, j0, j1):
            o = pltpu.bitcast(o_v[:, h0 * 128:h1 * 128], bf16)
            for n in range(j0, j1):
                y = _dot(o, pltpu.bitcast(wo_v[n, h0 * 64:h1 * 64, :], bf16))
                acc[n] = y if acc[n] is None else y + acc[n]

        for t in range(NG):
            proj(t)
            if t >= 1:
                score(t - 1)
            if t >= 2:
                pv(t - 2)
        wo(0, 16, 0, 4)
        score(NG - 1)
        pv(NG - 2)
        wo(0, 16, 4, 8)
        pv(NG - 1)
        wo(16, 24, 0, 8)
        wo(24, 32, 0, 8)
        return jnp.concatenate(acc, axis=1)

    def emit(j, r0, o0, a):
        rs = pl.ds(r0 + o0, 24)
        g = jnp.concatenate([g_v[rs, :]] * NT, axis=1)
        out_v[j, o0:o0 + 24, :] = (g * a + b_v[rs, :]).astype(bf16)

    def pair(j, carry):
        r0 = pl.multiple_of(j * 64, 64)
        allow_e, fill_e, allow_o, fill_o = _masks()
        xa = x_v[pl.ds(r0 + 16, 8), :].astype(f32)
        xb = x_v[pl.ds(r0 + 40, 8), :].astype(f32)
        hx = jnp.concatenate([x_v[pl.ds(r0, 16), :], jnp.concatenate([xa, mem_v[...]], 0).astype(bf16)], 0)
        oe = step(j, hx, False, allow_e, fill_e)
        emit(j, r0, 0, oe[:24])
        hx = jnp.concatenate([jnp.concatenate([oe[24:32], xb], 0).astype(bf16), x_v[pl.ds(r0 + 48, 16), :]], 0)
        oo = step(j, hx, True, allow_o, fill_o)
        mem_v[...] = oo[:8]
        emit(j, r0, 40, oo[8:])
        for o0 in (0, 40):
            pltpu.make_async_copy(out_v.at[j, pl.ds(o0, 24)], out_hbm.at[j, pl.ds(o0, 24)], sem_out).start()
        return carry

    lax.fori_loop(0, NPAIR, pair, 0)

    hist.clear()
    for n in range(NT // 2):
        quad = [lambda t=n + (q % 2) * (NT // 2), o=(q // 2) * 128: jnp.concatenate(
            [wo_v[t, g * 256 + o:g * 256 + o + 128, :] for g in range(NG)], axis=0) for q in range(4)]
        cs = strassen(lambda k: oe_v[k], lambda k: _rcombo(k, *quad), None)
        for q, t in enumerate(cs):
            cs_ = slice((n + (q % 2) * (NT // 2)) * 128, (n + (q % 2) * (NT // 2) + 1) * 128)
            o0 = 24 + (q // 2) * 8
            for jj in range(NPAIR):
                rs = slice(jj * 64 + o0, jj * 64 + o0 + 8)
                out_v[jj, o0:o0 + 8, cs_] = (g_v[rs, :] * t[jj * 8:jj * 8 + 8] + b_v[rs, cs_]).astype(bf16)
        for t in (n, n + NT // 2):
            idx = (slice(None), pl.ds(24, 16), pl.ds(t * 128, 128))
            pltpu.make_async_copy(out_v.at[idx], out_hbm.at[idx], sem_out).start()
    pltpu.make_async_copy(out_v, out_hbm, sem_out).wait()


@functools.partial(jax.jit, static_argnames=("A_seg_len",))
def pallas_gated_mix__memory_aug_recurrent_mem_tr__mixer_s_mlp__prompt_kernel(
    A_x, A_mem0, A_Wq, A_Wk, A_Wv, A_Wo, A_seg_len, B_x, B_w1, B_w2, B_w3, B_w4, gate_w,
):
    assert A_seg_len == SEG
    assert A_x.shape == (1, S, D) and A_mem0.shape == (1, M, D)
    any_spec = pl.BlockSpec(memory_space=pl.ANY)
    out = pl.pallas_call(
        _kernel,
        out_shape=jax.ShapeDtypeStruct((NPAIR, 64, D), bf16),
        in_specs=[any_spec] * 11,
        out_specs=any_spec,
        scratch_shapes=[
            pltpu.VMEM((S, D), bf16),
            pltpu.VMEM((9, D // 4, D // 2), u32),
            pltpu.VMEM((7, D // 4, D // 2), u32),
            pltpu.VMEM((7, D // 4, F // 2), u32),
            pltpu.VMEM((7, F // 4, D // 2), u32),
            pltpu.VMEM((3 * H, D // 2, DH), u32),
            pltpu.VMEM((NT, H * DH // 2, 128), u32),
            pltpu.VMEM((NT, S + 2 * PAD, 128), f32),
            pltpu.VMEM((S, D), f32),
            pltpu.VMEM((2, 7, HM // 2, D // 2), u32),
            pltpu.VMEM((2, TM, 128), f32),
            pltpu.VMEM((S, 128), f32),
            pltpu.VMEM((NPAIR, 64, D), bf16),
            pltpu.VMEM((7, 4 * NPAIR, D // 2), u32),
            pltpu.VMEM((3 * H, 8 * NPAIR, DH), u32),
            pltpu.VMEM((7, 8 * NPAIR, H * DH // 2), bf16),
            pltpu.VMEM((H, 16, 128), u32),
            pltpu.VMEM((H, 16, 128), u32),
            pltpu.VMEM((16, H * DH), u32),
            pltpu.VMEM((M, D), f32),
            pltpu.VMEM((M, D), bf16),
            pltpu.VMEM((NT, 128), bf16),
            pltpu.SMEM((1,), jnp.int32),
            pltpu.SemaphoreType.DMA((NLOAD,)),
            pltpu.SemaphoreType.DMA((NG,)),
            pltpu.SemaphoreType.DMA,
        ],
        compiler_params=pltpu.CompilerParams(vmem_limit_bytes=126 * 1024 * 1024,
                                             disable_bounds_checks=True),
    )(
        A_x.reshape(S, D), A_mem0.reshape(M, D),
        A_Wq.reshape(D // 2, 2 * H, DH), A_Wk.reshape(D // 2, 2 * H, DH), A_Wv.reshape(D // 2, 2 * H, DH),
        A_Wo.reshape(H * DH, D), B_w1, B_w2, B_w3, B_w4, gate_w.reshape(NT, 128),
    )
    return out.reshape(1, S, D)
```

```python
import functools

import jax
import jax.numpy as jnp
from jax import lax
import jax.experimental.pallas as pl
import jax.experimental.pallas.tpu as pltpu

f32, bf16, u32 = jnp.float32, jnp.bfloat16, jnp.uint32

S, D, H, DH, M, SEG, F = 2048, 1024, 32, 128, 8, 32, 3584
SCALE = DH ** -0.5
NEG = -1000000000.0
EPS = 1e-05

TM = 256
NB = S // TM
HM = TM // 2
DH2 = D // 2
FH = F // 2
FC = 256
NFC = FH // FC
NC1 = 128
NPAIR = S // (2 * SEG)
NPRE = 4
G = 4
NG = H // G
PAD = 8
NT = D // 128
NLOAD = 12
assert NB == NG

_dot = functools.partial(jnp.dot, preferred_element_type=f32)


def _ln(x):
    m = jnp.mean(x, axis=-1, keepdims=True)
    xc = x - m
    v = jnp.mean(xc * xc, axis=-1, keepdims=True)
    return xc * lax.rsqrt(v + EPS)


_GC = 0.7978845608028654


def _gelu(x):
    h = 0.5 * x
    return h + h * jnp.tanh(x * (_GC + (_GC * 0.044715) * (x * x)))


def _unpack(u):
    return pltpu.bitcast(u, bf16).astype(f32)


def _pack(x):
    return pltpu.bitcast(x.astype(bf16), u32)


def _lcombos(a11, a12, a21, a22):
    return [a11 + a22, a21 + a22, a11, a22, a11 + a12, a21 - a11, a12 - a22]


def _merge(*lists):
    keyed = [((j + 0.5) / len(l), n, j, v) for n, l in enumerate(lists) for j, v in enumerate(l)]
    return [v for _, _, _, v in sorted(keyed, key=lambda t: t[:3])]


def _masks():
    r = lax.broadcasted_iota(jnp.int32, (32, 48), 0)
    c = lax.broadcasted_iota(jnp.int32, (32, 48), 1)
    exist_e = c < 40
    allow_e = exist_e & ((r >= 24) | ((c >= 24) & (c < 32)) | (c <= r))
    fill_e = jnp.where(exist_e, NEG, -jnp.inf).astype(f32)
    r = lax.broadcasted_iota(jnp.int32, (48, 80), 0)
    c = lax.broadcasted_iota(jnp.int32, (48, 80), 1)
    q_even = (r >= 32) & (r < 40)
    exist_o = (q_even & (c < 40)) | (~q_even & (c >= 40))
    ktok = jnp.where(c < 24, c, jnp.where(c < 48, c - 8, c - 16))
    qtok = jnp.where(r < 32, r + 32, r - 8)
    is_mem_key = ((c >= 24) & (c < 32)) | ((c >= 48) & (c < 56))
    allow_o = exist_o & (is_mem_key | (r < 8) | (ktok <= qtok))
    fill_o = jnp.where(exist_o, NEG, -jnp.inf).astype(f32)
    return allow_e, fill_e, allow_o, fill_o


def _rcombo(k, b11, b12, b21, b22):
    if k in (1, 4):
        return (b11 if k == 1 else b22)(k)
    a, b, sign = {0: (b11, b22, 1), 2: (b12, b22, -1), 3: (b21, b11, -1), 5: (b11, b12, 1), 6: (b21, b22, 1)}[k]
    a, b = _unpack(a(k)), _unpack(b(k))
    return (a + b if sign > 0 else a - b).astype(bf16)


def _softmax(s, allow, fill):
    s = jnp.where(allow, s * SCALE, fill)
    m = jnp.max(s, axis=-1, keepdims=True)
    e = jnp.exp(s - m)
    l = jnp.sum(e, axis=-1, keepdims=True)
    r = pl.reciprocal(l, approx=True)
    r = r * (2.0 - l * r)
    return (e * r).astype(bf16)


def _kernel(x_hbm, mem0_hbm, wq_hbm, wk_hbm, wv_hbm, wo_hbm, w1_hbm, w2_hbm, w3_hbm, w4_hbm,
            gw_hbm, out_hbm,
            x_v, s1_v, s2_v, s3_v, s4_v, wqkv_v, wo_v, h_v, b_v, l_v, n_v, g_v, out_v, xe_v, e_v, oe_v,
            ke_v, ve_v, o_v, mem_v, mem0_ref, gw_ref, zero_s,
            sem, sem_qkv, sem_out):
    RAW = (1, 2, 3, 4)
    RAW1 = (1, 7, 8, 4)

    loads = []

    def rows_load(name, r0, r1):
        loads.append((name, x_hbm.at[pl.ds(r0, r1 - r0)], x_v.at[pl.ds(r0, r1 - r0)]))

    def quad_load(name, w_hbm, s_v, raw, q, c0=0, c1=None):
        k4, n2 = s_v.shape[1], s_v.shape[2]
        c1 = n2 if c1 is None else c1
        src = w_hbm.bitcast(u32).at[pl.ds((q // 2) * k4, k4), pl.ds((q % 2) * n2 + c0, c1 - c0)]
        loads.append((name, src, s_v.at[raw[q], :, pl.ds(c0, c1 - c0)]))

    rows_load("x0", 0, TM)
    rows_load("x1", TM, 2 * TM)
    for name, half, c0, c1 in (("w1a", 0, 0, 256), ("w1bc", 0, 256, 512), ("w1bc", 1, 0, 256), ("w1d", 1, 256, 512)):
        quad_load(name, w1_hbm, s1_v, RAW1, half, c0, c1)
        quad_load(name, w1_hbm, s1_v, RAW1, 2 + half, c0, c1)
    rows_load("x234", 2 * TM, 5 * TM)
    rows_load("x567", 5 * TM, S)
    for name, w_hbm, s_v in (("w2", w2_hbm, s2_v), ("w3", w3_hbm, s3_v), ("w4", w4_hbm, s4_v)):
        for q in range(4):
            quad_load(name, w_hbm, s_v, RAW, q)
    loads.append(("small", mem0_hbm, mem0_ref))
    loads.append(("small", gw_hbm, gw_ref))
    for j in range(NT):
        loads.append(("wo", wo_hbm.bitcast(u32).at[:, pl.ds(j * 128, 128)], wo_v.at[j]))
    groups = list(dict.fromkeys(name for name, _, _ in loads))
    assert len(groups) == NLOAD

    def start(*names, priority=0):
        for name, src, dst in loads:
            if name in names:
                pltpu.make_async_copy(src, dst, sem.at[groups.index(name)]).start(priority=priority)

    def wait(*names):
        for name, src, dst in loads:
            if name in names:
                pltpu.make_async_copy(src, dst, sem.at[groups.index(name)]).wait()

    SPG = 3 * G

    def qkv_start(g):
        for w, w_hbm in enumerate((wq_hbm, wk_hbm, wv_hbm)):
            wu = w_hbm.bitcast(u32)
            for k in range(G // 2):
                for par in range(2):
                    pltpu.make_async_copy(
                        wu.at[:, par * (H // 2) + g * (G // 2) + k, :],
                        wqkv_v.at[g * SPG + w * G + 2 * k + par], sem_qkv.at[g]).start(priority=1)

    def qkv_wait(g):
        grp = wqkv_v.at[pl.ds(g * SPG, SPG)]
        pltpu.make_async_copy(grp, grp, sem_qkv.at[g]).wait()

    start("x0", "x1", "w1a", "w1bc", "w1d", "x234", "x567", "w2", "w3", "w4", "small")
    for k in range(8):
        zero_s[k] = 0

    def tile_idx(ref):
        z = zero_s[0]
        return (z,) * (len(ref.shape) - 2) + (pl.ds(pl.multiple_of(z, 8), 8), slice(0, 128))

    hist = []

    def mm(lhs, rhs, side=None, acc=None):
        if side is not None:
            lhs = side(lhs)
        lhs = pltpu.bitcast(lhs, bf16) if lhs.dtype == u32 else lhs.astype(bf16)
        y = _dot(lhs, pltpu.bitcast(rhs, bf16) if rhs.dtype == u32 else rhs)
        if acc is not None:
            y = y + acc
        hist.append(y)
        return y

    class Side:
        def __init__(self, pieces, n):
            self.pieces, self.n = list(pieces), n

        def __call__(self, val):
            take = -(-len(self.pieces) // self.n) if self.pieces else 0
            self.n -= 1
            if not take:
                return val
            never = zero_s[0] > 0
            rg = 8 if val.dtype == u32 else 16
            ng = val.shape[0] // rg
            groups = [val[8 * m:8 * m + 8] for m in range(val.shape[0] // 8)]
            for j, (fn, rd, wr, lag) in enumerate(self.pieces[:take]):
                m = (j + 1) * ng // take - 1
                pin = lambda v: v
                if lag is not None and len(hist) >= lag:
                    r0 = (16 * m) % hist[-lag].shape[0]
                    a = hist[-lag][r0:r0 + 8, :128]
                    if rd is None:
                        def pin(v, a=a):
                            t = jnp.where(never, jnp.concatenate([a] * (v.shape[0] // 8), axis=0), v[:, :128])
                            return t if v.shape[1] == 128 else jnp.concatenate([t, v[:, 128:]], axis=1)
                    else:
                        idx = tile_idx(rd)
                        rd[idx] = jnp.where(never, pltpu.bitcast(a, rd.dtype), rd[idx])
                fn(pin)
                g = m * rg // 8
                t = jnp.where(never, pltpu.bitcast(wr[tile_idx(wr)], val.dtype), groups[g][:, -128:])
                groups[g] = jnp.concatenate([groups[g][:, :-128], t], axis=1)
            self.pieces = self.pieces[take:]
            return jnp.concatenate(groups, axis=0)

    def strassen(lhs, rhs, side, init=(None, None, None, None), ks=range(7)):
        def add(a, b):
            return a if b is None else a + b
        sd = lambda k: side if k in ks else None
        p = [mm(lhs(k), rhs(k), sd(k)) for k in range(5)]
        c12 = add(p[2] + p[4], init[1])
        c21 = add(p[1] + p[3], init[2])
        c22 = mm(lhs(5), rhs(5), sd(5), add(p[0] - p[1] + p[2], init[3]))
        c11 = mm(lhs(6), rhs(6), sd(6), add(p[0] + p[3] - p[4], init[0]))
        return c11, c12, c21, c22

    def prep_pieces(s_v, raw, lag, width=256):
        def piece(r, c, pin):
            idx = (slice(r, r + 8), slice(c, c + width))
            b11, b12, b21, b22 = [_unpack(s_v[(q,) + idx]) for q in raw]
            for k, t in ((0, b11 + b22), (2, b12 - b22), (3, b21 - b11), (5, b11 + b12), (6, b21 + b22)):
                s_v[(k,) + idx] = _pack(t)
        return [(functools.partial(piece, r, c), s_v, s_v, lag)
                for r in range(0, s_v.shape[1], 8) for c in range(0, s_v.shape[2], width)]

    def store_l(slot, q, c, quads, plain=False):
        for k, t in enumerate(quads if plain else _lcombos(*quads)):
            l_v[slot, k, q // 2:q // 2 + 8, c:c + t.shape[1]] = _pack(t)

    def ln_pieces(src, r0, slot, lag, plain=False, width=256, staged=False, clag=None):
        def stats(q, pin):
            x = pin(src[pl.ds(r0 + q, 16), :].astype(f32))
            xs = [x[:, j * 128:(j + 1) * 128] for j in range(NT)]
            m = functools.reduce(lambda a, b: a + b, xs) * (1.0 / NT)
            w = functools.reduce(lambda a, b: a + b, [(t - m) * (t - m) for t in xs])
            mean = jnp.mean(m, axis=-1, keepdims=True)
            var = jnp.sum(w + NT * ((m - mean) * (m - mean)), axis=-1, keepdims=True) * (1.0 / D)
            n_v[0, q:q + 16, :] = jnp.broadcast_to(mean, (16, 128))
            n_v[1, q:q + 16, :] = jnp.broadcast_to(lax.rsqrt(var + EPS), (16, 128))

        def comb(q, c, pin):
            quads = []
            for rr in (0, HM):
                rs = pl.ds(pl.multiple_of(r0 + rr + q + zero_s[0], 16), 16)
                mean, rstd = [jnp.concatenate([n_v[t, rr + q:rr + q + 16, :]] * (width // 128), axis=1)
                              for t in range(2)]
                quads += [(src[rs, cc + c:cc + c + width].astype(f32) - mean) * rstd for cc in (0, DH2)]
            store_l(slot, q, c, quads, plain)
        norms = [[(functools.partial(stats, rr + q), None, n_v, lag) for rr in (0, HM)] for q in range(0, HM, 16)]
        combs = [[(functools.partial(comb, q, c), n_v, l_v, clag) for c in range(0, DH2, width)]
                 for q in range(0, HM, 16)]
        if staged:
            return sum(norms, []), sum(combs, [])
        out = list(norms[0])
        for a, b in zip(norms[1:] + [[]], combs):
            out += _merge(a, b) if a else b
        return out

    shifts = (1, 1, -1, -1, 2, 2, -2, -2)

    def shift_pieces(r0, slot, lag, by_value=False):
        def piece(q, j, pin):
            a = [h_v[jj, pl.ds(PAD + r0 + rr + q - shifts[jj], 16), :]
                 for rr in (0, HM) for jj in (j, j + NT // 2)]
            store_l(slot, q, j * 128, [pin(a[0]), a[1], a[2], pin(a[3])])
        return [(functools.partial(piece, q, j), None if by_value else h_v, l_v, lag)
                for q in range(0, HM, 16) for j in range(NT // 2)]

    def lhs_of(slot):
        return lambda k: l_v[slot, k]

    h_v[:, 0:PAD, :] = jnp.zeros((NT, PAD, 128), f32)
    h_v[:, PAD + S:PAD + S + PAD, :] = jnp.zeros((NT, PAD, 128), f32)

    def store_h(r0, c0, h):
        for j in range(h.shape[1] // 128):
            h_v[c0 // 128 + j, PAD + r0:PAD + r0 + h.shape[0], :] = h[:, j * 128:(j + 1) * 128]

    def d1_plain(xn, r0, c0, c1, step, side=None):
        for c in range(c0, c1, step):
            half, cc = c // DH2, c % DH2
            w = jnp.concatenate([s1_v[RAW1[half], :, cc:cc + step], s1_v[RAW1[2 + half], :, cc:cc + step]], axis=0)
            store_h(r0, c, _gelu(mm(xn, w, side)))

    NP1 = 7 * (DH2 // NC1)
    KS1 = (2, 3, 4, 5)

    def d1_s(b, slot, pieces):
        side = Side(pieces, len(KS1) * (DH2 // NC1))
        for c in range(0, DH2, NC1):
            cs = strassen(lhs_of(slot), lambda k: s1_v[k, :, c:c + NC1], side, ks=KS1)
            for q, t in enumerate(cs):
                store_h(b * TM + (q // 2) * HM, (q % 2) * DH2 + c, _gelu(t))

    def d2_s(b, slot, pieces):
        side = Side(pieces, NP1)
        for c in range(0, DH2, NC1):
            idx = [(slice(b * TM + (q // 2) * HM, b * TM + (q // 2 + 1) * HM),
                    slice((q % 2) * DH2 + c, (q % 2) * DH2 + c + NC1)) for q in range(4)]
            cs = strassen(lhs_of(slot), lambda k: s2_v[k, :, c:c + NC1], side,
                          [x_v[i].astype(f32) for i in idx])
            for i, t in zip(idx, cs):
                b_v[i] = t

    def split(l, n):
        return [l[len(l) * i // n:len(l) * (i + 1) // n] for i in range(n)]

    LS, LL = 3, 5

    wait("x0")
    xn0 = _pack(_ln(x_v[0:TM, :].astype(f32)))
    wait("x1")
    xn01 = jnp.concatenate([xn0, _pack(_ln(x_v[TM:2 * TM, :].astype(f32)))], axis=0)
    wait("w1a")
    d1_plain(xn01, 0, 0, 256, 256)
    wait("w1bc")
    d1_plain(xn01, 0, 256, 768, 256)
    wait("w1d", "x234")
    hist.clear()
    d1_plain(xn01, 0, 768, D, 128, Side(ln_pieces(x_v, 2 * TM, 0, None, plain=True), 2))
    xn2 = jnp.concatenate([jnp.concatenate([l_v[0, 2 * h], l_v[0, 2 * h + 1]], axis=1) for h in range(2)], axis=0)
    d1_plain(xn2, 2 * TM, 0, D, 128,
             Side(_merge(prep_pieces(s1_v, RAW1, 1), ln_pieces(x_v, 3 * TM, 1, 2)), 8))
    d1_s(3, 1, ln_pieces(x_v, 4 * TM, 0, LL))
    wait("x567", "w2")
    qkv_start(0)
    qkv_start(1)
    hist.clear()
    pw = split(prep_pieces(s2_v, RAW, LS), 4)
    for b in range(4, NB):
        nxt = ln_pieces(x_v, (b + 1) * TM, (b + 1) % 2, LL) if b + 1 < NB else shift_pieces(0, 0, LS, True)
        d1_s(b, b % 2, _merge(pw[b - 4], nxt))
    d2_s(0, 0, shift_pieces(TM, 1, LS, True))
    wait("w3")
    hist.clear()
    pw = split(prep_pieces(s3_v, RAW, LS), 4)
    for b in range(1, 5):
        d2_s(b, b % 2, _merge(pw[b - 1], shift_pieces((b + 1) * TM, (b + 1) % 2, LS)))
    wait("w4", "small")
    hist.clear()
    pw = prep_pieces(s4_v, RAW, LS)
    pw = [pw[:82], pw[82:164], pw[164:]]
    for b in range(5, NB):
        nxt = shift_pieces((b + 1) * TM, (b + 1) % 2, LS) if b + 1 < NB else ln_pieces(b_v, 0, 0, LL)
        d2_s(b, b % 2, _merge(pw[b - 5], nxt))
    start("wo", priority=1)

    def ffn(i, carry):
        qkv_wait(i)
        r0 = pl.multiple_of(i * TM, TM)
        rn = pl.multiple_of(jnp.minimum(i + 1, NB - 1) * TM, TM)
        lh = {}
        acc = [None] * 7
        hist.clear()

        def relayout(p, r0_, r1_, pin):
            s0 = i * SPG + 2 * p
            for r in range(r0_, r1_, 8):
                e = wqkv_v[s0, r:r + 8, :]
                o = wqkv_v[s0 + 1, r:r + 8, :]
                wqkv_v[s0, r:r + 8, :] = (e & jnp.uint32(0xFFFF)) | (o << 16)
                wqkv_v[s0 + 1, r:r + 8, :] = (e >> 16) | (o & jnp.uint32(0xFFFF0000))

        side3 = Side([(functools.partial(relayout, p, r, r + 32), wqkv_v, wqkv_v, 2)
                      for p in range(SPG // 2) for r in range(0, D // 2, 32)], 42 + 5)
        norms, combs = ln_pieces(b_v, rn, 0, 3, staged=True, width=128, clag=2)

        def gate(q, pin):
            gw = gw_ref[...].astype(f32)
            x = pin(x_v[pl.ds(r0 + q, 16), :].astype(f32))
            t = functools.reduce(lambda a, b: a + b,
                                 [x[:, j * 128:(j + 1) * 128] * gw[j:j + 1, :] for j in range(NT)])
            g = jax.nn.sigmoid(jnp.sum(t, axis=-1, keepdims=True))
            g_v[pl.ds(r0 + q, 16), :] = jnp.broadcast_to(g, (16, 128))

        gates = [(functools.partial(gate, q), None, g_v, 3) for q in range(0, TM, 16)]

        def extras(t, c, pin):
            jj = 2 * i + t
            a = [x_v[pl.ds(pl.multiple_of((jj + hh) * 64 + 24, 8), 16), cc + c:cc + c + 256].astype(f32)
                 for hh in (0, NPAIR // 2) for cc in (0, DH2)]
            for k, v in enumerate(_lcombos(pin(a[0]), a[1], a[2], pin(a[3]))):
                xe_v[k, pl.ds(pl.multiple_of(jj * 8, 8), 8), c:c + 256] = _pack(v)

        xes = [(functools.partial(extras, t, c), None, xe_v, 2) for t in range(2) for c in (0, 256)]
        side4 = Side(_merge(norms, gates, xes), 20)
        side5 = Side(combs, 11)

        def d3(c):
            cs = strassen(lhs_of(0), lambda k: s3_v[k, :, c * FC:(c + 1) * FC],
                          side3 if c > 0 else (lambda v: side3(v) if len(hist) >= 2 else v))
            lh[c] = _lcombos(*[_gelu(t) for t in cs])

        def d4(c):
            l = lh.pop(c)
            rhs = lambda k: s4_v[k, c * FC // 2:(c + 1) * FC // 2, :]
            if c + 1 < NFC:
                for k in range(7):
                    side = (side5 if k > 0 else None) if c == NFC - 2 else (side4 if k >= 3 else None)
                    acc[k] = mm(l[k], rhs(k), side, acc[k])
                return
            q = [mm(l[k], rhs(k), side5, acc[k]) for k in range(5)]
            top, bot = pl.ds(r0, HM), pl.ds(r0 + HM, HM)
            gt, gb = [jnp.concatenate([1.0 - g_v[r, :]] * (NT // 2), axis=1) for r in (top, bot)]
            b_v[top, DH2:] = gt * (q[2] + q[4] + b_v[top, DH2:])
            b_v[bot, :DH2] = gb * (q[1] + q[3] + b_v[bot, :DH2])
            b_v[bot, DH2:] = gb * mm(l[5], rhs(5), None, acc[5] + q[0] - q[1] + q[2] + b_v[bot, DH2:])
            b_v[top, :DH2] = gt * mm(l[6], rhs(6), None, acc[6] + q[0] + q[3] - q[4] + b_v[top, :DH2])

        d3(0)
        for c in range(NFC):
            if c + 1 < NFC:
                d3(c + 1)
            d4(c)
        assert not side3.pieces and not side4.pieces and not side5.pieces

        @pl.when(i + 2 < NG)
        def _():
            qkv_start(i + 2)

        return carry

    lax.fori_loop(0, NB, ffn, 0)

    def pre(it, carry):
        hist.clear()
        for u in range(3 * H // 2 // NPRE):
            s0 = it * (3 * H // NPRE) + 2 * u
            quad = [lambda k, s=s0 + q % 2, r=(q // 2) * (D // 4): wqkv_v[s + zero_s[k], r:r + D // 4, :]
                    for q in range(4)]
            cs = strassen(lambda k: xe_v[k], lambda k: _rcombo(k, *quad), None)
            for q, t in enumerate(cs):
                e_v[s0 + q % 2, (q // 2) * 128:(q // 2 + 1) * 128, :] = _pack(t)
        return carry

    lax.fori_loop(0, NPRE, pre, 0)

    wait("wo")
    mem_v[...] = mem0_ref[...].astype(f32)

    def slab(w, h):
        return (h // G) * SPG + w * G + h % G

    def step(j, hx, odd, allow, fill):
        qs, ks, vs, ps = {}, {}, {}, {}
        wload = lambda w, h: pltpu.bitcast(wqkv_v[slab(w, h)], bf16)
        eload = lambda w, h: pltpu.bitcast(e_v[slab(w, h), pl.ds(pl.multiple_of(j * 8, 8), 8), :], bf16)

        def proj(g):
            part = {}
            if odd and g == 0:
                for h in range(2):
                    for w in range(3):
                        part[w, h] = _dot(hx[:, :DH2], wload(w, h)[:DH2])
            for h in range(g * G, (g + 1) * G):
                q, k, v = [(_dot(hx[:, DH2:], wload(w, h)[DH2:]) + part[w, h] if (w, h) in part
                            else _dot(hx, wload(w, h))).astype(bf16) for w in range(3)]
                if odd:
                    q = jnp.concatenate([q, eload(0, h)], axis=0)
                    k = jnp.concatenate([pltpu.bitcast(ke_v[h], bf16), eload(1, h), k], axis=0)
                    v = jnp.concatenate([pltpu.bitcast(ve_v[h], bf16), eload(2, h), v], axis=0)
                else:
                    ke_v[h] = pltpu.bitcast(k, u32)
                    ve_v[h] = pltpu.bitcast(v, u32)
                    k = jnp.concatenate([k, eload(1, h)], axis=0)
                    v = jnp.concatenate([v, eload(2, h)], axis=0)
                qs[h], ks[h], vs[h] = q, k, v

        def score(g):
            for h in range(g * G, (g + 1) * G):
                s = lax.dot_general(qs.pop(h), ks.pop(h), (((1,), (1,)), ((), ())),
                                    preferred_element_type=f32)
                ps[h] = _softmax(s, allow, fill)

        def pv(g):
            os_ = []
            for h in range(g * G, (g + 1) * G):
                o = _dot(ps.pop(h), vs.pop(h))
                o_v[:, h * 128:(h + 1) * 128] = _pack(o[:32])
                os_.append(o)
            if odd:
                quads = [jnp.concatenate([os_[2 * kk][r:r + 8], os_[2 * kk + 1][r:r + 8]], axis=1)
                         for r in (32, 40) for kk in range(2)]
                for k, t in enumerate(_lcombos(*quads)):
                    oe_v[k, pl.ds(pl.multiple_of(j * 8, 8), 8), g * 256:(g + 1) * 256] = t.astype(bf16)

        acc = [None] * NT

        def wo(h0, h1, j0, j1):
            o = pltpu.bitcast(o_v[:, h0 * 128:h1 * 128], bf16)
            for n in range(j0, j1):
                y = _dot(o, pltpu.bitcast(wo_v[n, h0 * 64:h1 * 64, :], bf16))
                acc[n] = y if acc[n] is None else y + acc[n]

        for t in range(NG):
            proj(t)
            if t >= 2:
                pv(t - 2)
            if t >= 1:
                score(t - 1)
        wo(0, 16, 0, 4)
        pv(NG - 2)
        score(NG - 1)
        wo(0, 16, 4, 8)
        pv(NG - 1)
        wo(16, 24, 0, 8)
        wo(24, 32, 0, 8)
        return jnp.concatenate(acc, axis=1)

    def emit(j, r0, o0, a):
        rs = pl.ds(r0 + o0, 24)
        g = jnp.concatenate([g_v[rs, :]] * NT, axis=1)
        out_v[j, o0:o0 + 24, :] = (g * a + b_v[rs, :]).astype(bf16)

    def pair(j, carry):
        r0 = pl.multiple_of(j * 64, 64)
        allow_e, fill_e, allow_o, fill_o = _masks()
        xa = x_v[pl.ds(r0 + 16, 8), :].astype(f32)
        xb = x_v[pl.ds(r0 + 40, 8), :].astype(f32)
        hx = jnp.concatenate([x_v[pl.ds(r0, 16), :], jnp.concatenate([xa, mem_v[...]], 0).astype(bf16)], 0)
        oe = step(j, hx, False, allow_e, fill_e)
        emit(j, r0, 0, oe[:24])
        hx = jnp.concatenate([jnp.concatenate([oe[24:32], xb], 0).astype(bf16), x_v[pl.ds(r0 + 48, 16), :]], 0)
        oo = step(j, hx, True, allow_o, fill_o)
        mem_v[...] = oo[:8]
        emit(j, r0, 40, oo[8:])
        for o0 in (0, 40):
            pltpu.make_async_copy(out_v.at[j, pl.ds(o0, 24)], out_hbm.at[j, pl.ds(o0, 24)], sem_out).start()
        return carry

    lax.fori_loop(0, NPAIR, pair, 0)

    hist.clear()
    for n in range(NT // 2):
        quad = [lambda k, t=2 * n + q % 2, o=(q // 2) * 128: jnp.concatenate(
            [wo_v[t + zero_s[k], g * 256 + o:g * 256 + o + 128, :] for g in range(NG)], axis=0) for q in range(4)]
        cs = strassen(lambda k: oe_v[k], lambda k: _rcombo(k, *quad), None)
        cols = slice(n * 256, (n + 1) * 256)
        for half in range(2):
            t = jnp.concatenate(cs[2 * half:2 * half + 2], axis=1)
            o0 = 24 + half * 8
            for jj in range(NPAIR):
                rs = slice(jj * 64 + o0, jj * 64 + o0 + 8)
                g = jnp.concatenate([g_v[rs, :]] * 2, axis=1)
                out_v[jj, o0:o0 + 8, cols] = (g * t[jj * 8:jj * 8 + 8] + b_v[rs, cols]).astype(bf16)
        if n >= 2:
            idx = (slice(None), pl.ds(24, 16), pl.ds(0, 768) if n == 2 else pl.ds(768, 256))
            pltpu.make_async_copy(out_v.at[idx], out_hbm.at[idx], sem_out).start()
    pltpu.make_async_copy(out_v, out_hbm, sem_out).wait()


@functools.partial(jax.jit, static_argnames=("A_seg_len",))
def pallas_gated_mix__memory_aug_recurrent_mem_tr__mixer_s_mlp__prompt_kernel(
    A_x, A_mem0, A_Wq, A_Wk, A_Wv, A_Wo, A_seg_len, B_x, B_w1, B_w2, B_w3, B_w4, gate_w,
):
    assert A_seg_len == SEG
    assert A_x.shape == (1, S, D) and A_mem0.shape == (1, M, D)
    any_spec = pl.BlockSpec(memory_space=pl.ANY)
    out = pl.pallas_call(
        _kernel,
        out_shape=jax.ShapeDtypeStruct((NPAIR, 64, D), bf16),
        in_specs=[any_spec] * 11,
        out_specs=any_spec,
        scratch_shapes=[
            pltpu.VMEM((S, D), bf16),
            pltpu.VMEM((9, D // 4, D // 2), u32),
            pltpu.VMEM((7, D // 4, D // 2), u32),
            pltpu.VMEM((7, D // 4, F // 2), u32),
            pltpu.VMEM((7, F // 4, D // 2), u32),
            pltpu.VMEM((3 * H, D // 2, DH), u32),
            pltpu.VMEM((NT, H * DH // 2, 128), u32),
            pltpu.VMEM((NT, S + 2 * PAD, 128), f32),
            pltpu.VMEM((S, D), f32),
            pltpu.VMEM((2, 7, HM // 2, D // 2), u32),
            pltpu.VMEM((2, TM, 128), f32),
            pltpu.VMEM((S, 128), f32),
            pltpu.VMEM((NPAIR, 64, D), bf16),
            pltpu.VMEM((7, 4 * NPAIR, D // 2), u32),
            pltpu.VMEM((3 * H, 8 * NPAIR, DH), u32),
            pltpu.VMEM((7, 8 * NPAIR, H * DH // 2), bf16),
            pltpu.VMEM((H, 16, 128), u32),
            pltpu.VMEM((H, 16, 128), u32),
            pltpu.VMEM((16, H * DH), u32),
            pltpu.VMEM((M, D), f32),
            pltpu.VMEM((M, D), bf16),
            pltpu.VMEM((NT, 128), bf16),
            pltpu.SMEM((8,), jnp.int32),
            pltpu.SemaphoreType.DMA((NLOAD,)),
            pltpu.SemaphoreType.DMA((NG,)),
            pltpu.SemaphoreType.DMA,
        ],
        compiler_params=pltpu.CompilerParams(vmem_limit_bytes=126 * 1024 * 1024,
                                             disable_bounds_checks=True),
    )(
        A_x.reshape(S, D), A_mem0.reshape(M, D),
        A_Wq.reshape(D // 2, 2 * H, DH), A_Wk.reshape(D // 2, 2 * H, DH), A_Wv.reshape(D // 2, 2 * H, DH),
        A_Wo.reshape(H * DH, D), B_w1, B_w2, B_w3, B_w4, gate_w.reshape(NT, 128),
    )
    return out.reshape(1, S, D)
```

```python
import functools

import jax
import jax.numpy as jnp
from jax import lax
import jax.experimental.pallas as pl
import jax.experimental.pallas.tpu as pltpu

f32, bf16, u32 = jnp.float32, jnp.bfloat16, jnp.uint32

S, D, H, DH, M, SEG, F = 2048, 1024, 32, 128, 8, 32, 3584
SCALE = DH ** -0.5
NEG = -1000000000.0
EPS = 1e-05

TM = 256
NB = S // TM
HM = TM // 2
DH2 = D // 2
FH = F // 2
FC = 256
NFC = FH // FC
NC1 = 128
NPAIR = S // (2 * SEG)
PPI = 2
NPRE = 4
G = 4
NG = H // G
PAD = 8
NT = D // 128
NLOAD = 12
assert NB == NG

_dot = functools.partial(jnp.dot, preferred_element_type=f32)


def _ln(x):
    m = jnp.mean(x, axis=-1, keepdims=True)
    xc = x - m
    v = jnp.mean(xc * xc, axis=-1, keepdims=True)
    return xc * lax.rsqrt(v + EPS)


_GC = 0.7978845608028654


def _gelu(x):
    h = 0.5 * x
    return h + h * jnp.tanh(x * (_GC + (_GC * 0.044715) * (x * x)))


def _unpack(u):
    return pltpu.bitcast(u, bf16).astype(f32)


def _pack(x):
    return pltpu.bitcast(x.astype(bf16), u32)


def _lcombos(a11, a12, a21, a22):
    return [a11 + a22, a21 + a22, a11, a22, a11 + a12, a21 - a11, a12 - a22]


def _merge(*lists):
    keyed = [((j + 0.5) / len(l), n, j, v) for n, l in enumerate(lists) for j, v in enumerate(l)]
    return [v for _, _, _, v in sorted(keyed, key=lambda t: t[:3])]


def _masks():
    r = lax.broadcasted_iota(jnp.int32, (32, 48), 0)
    c = lax.broadcasted_iota(jnp.int32, (32, 48), 1)
    exist_e = c < 40
    allow_e = exist_e & ((r >= 24) | ((c >= 24) & (c < 32)) | (c <= r))
    fill_e = jnp.where(exist_e, NEG, -jnp.inf).astype(f32)
    r = lax.broadcasted_iota(jnp.int32, (48, 80), 0)
    c = lax.broadcasted_iota(jnp.int32, (48, 80), 1)
    q_even = (r >= 32) & (r < 40)
    exist_o = (q_even & (c < 40)) | (~q_even & (c >= 40))
    ktok = jnp.where(c < 24, c, jnp.where(c < 48, c - 8, c - 16))
    qtok = jnp.where(r < 32, r + 32, r - 8)
    is_mem_key = ((c >= 24) & (c < 32)) | ((c >= 48) & (c < 56))
    allow_o = exist_o & (is_mem_key | (r < 8) | (ktok <= qtok))
    fill_o = jnp.where(exist_o, NEG, -jnp.inf).astype(f32)
    return allow_e, fill_e, allow_o, fill_o


def _rcombo(k, b11, b12, b21, b22):
    if k in (1, 4):
        return (b11 if k == 1 else b22)(k)
    a, b, sign = {0: (b11, b22, 1), 2: (b12, b22, -1), 3: (b21, b11, -1), 5: (b11, b12, 1), 6: (b21, b22, 1)}[k]
    a, b = _unpack(a(k)), _unpack(b(k))
    return (a + b if sign > 0 else a - b).astype(bf16)


def _softmax(s, allow, fill):
    s = jnp.where(allow, s * SCALE, fill)
    m = jnp.max(s, axis=-1, keepdims=True)
    e = jnp.exp(s - m)
    l = jnp.sum(e, axis=-1, keepdims=True)
    r = pl.reciprocal(l, approx=True)
    r = r * (2.0 - l * r)
    return (e * r).astype(bf16)


def _kernel(x_hbm, mem0_hbm, wq_hbm, wk_hbm, wv_hbm, wo_hbm, w1_hbm, w2_hbm, w3_hbm, w4_hbm,
            gw_hbm, out_hbm,
            x_v, s1_v, s2_v, s3_v, s4_v, wqkv_v, wo_v, h_v, b_v, l_v, n_v, g_v, out_v, xe_v, e_v, oe_v,
            ke_v, ve_v, o_v, mem_v, mem0_ref, gw_ref, zero_s,
            sem, sem_qkv, sem_out):
    RAW = (1, 2, 3, 4)
    RAW1 = (1, 7, 8, 4)

    loads = []

    def rows_load(name, r0, r1):
        loads.append((name, x_hbm.at[pl.ds(r0, r1 - r0)], x_v.at[pl.ds(r0, r1 - r0)]))

    def quad_load(name, w_hbm, s_v, raw, q, c0=0, c1=None):
        k4, n2 = s_v.shape[1], s_v.shape[2]
        c1 = n2 if c1 is None else c1
        src = w_hbm.bitcast(u32).at[pl.ds((q // 2) * k4, k4), pl.ds((q % 2) * n2 + c0, c1 - c0)]
        loads.append((name, src, s_v.at[raw[q], :, pl.ds(c0, c1 - c0)]))

    rows_load("x0", 0, TM)
    rows_load("x1", TM, 2 * TM)
    for name, half, c0, c1 in (("w1a", 0, 0, 256), ("w1bc", 0, 256, 512), ("w1bc", 1, 0, 256), ("w1d", 1, 256, 512)):
        quad_load(name, w1_hbm, s1_v, RAW1, half, c0, c1)
        quad_load(name, w1_hbm, s1_v, RAW1, 2 + half, c0, c1)
    rows_load("x234", 2 * TM, 5 * TM)
    rows_load("x567", 5 * TM, S)
    for name, w_hbm, s_v in (("w2", w2_hbm, s2_v), ("w3", w3_hbm, s3_v), ("w4", w4_hbm, s4_v)):
        for q in range(4):
            quad_load(name, w_hbm, s_v, RAW, q)
    loads.append(("small", mem0_hbm, mem0_ref))
    loads.append(("small", gw_hbm, gw_ref))
    for j in range(NT):
        loads.append(("wo", wo_hbm.bitcast(u32).at[:, pl.ds(j * 128, 128)], wo_v.at[j]))
    groups = list(dict.fromkeys(name for name, _, _ in loads))
    assert len(groups) == NLOAD

    def start(*names, priority=0):
        for name, src, dst in loads:
            if name in names:
                pltpu.make_async_copy(src, dst, sem.at[groups.index(name)]).start(priority=priority)

    def wait(*names):
        for name, src, dst in loads:
            if name in names:
                pltpu.make_async_copy(src, dst, sem.at[groups.index(name)]).wait()

    SPG = 3 * G

    def qkv_start(g):
        for w, w_hbm in enumerate((wq_hbm, wk_hbm, wv_hbm)):
            wu = w_hbm.bitcast(u32)
            for k in range(G // 2):
                for par in range(2):
                    pltpu.make_async_copy(
                        wu.at[:, par * (H // 2) + g * (G // 2) + k, :],
                        wqkv_v.at[g * SPG + w * G + 2 * k + par], sem_qkv.at[g]).start(priority=1)

    def qkv_wait(g):
        grp = wqkv_v.at[pl.ds(g * SPG, SPG)]
        pltpu.make_async_copy(grp, grp, sem_qkv.at[g]).wait()

    start("x0", "x1", "w1a", "w1bc", "w1d", "x234", "x567", "w2", "w3", "w4", "small")
    for k in range(8):
        zero_s[k] = 0

    def tile_idx(ref):
        z = zero_s[0]
        return (z,) * (len(ref.shape) - 2) + (pl.ds(pl.multiple_of(z, 8), 8), slice(0, 128))

    hist = []

    def mm(lhs, rhs, side=None, acc=None):
        if side is not None:
            lhs = side(lhs)
        lhs = pltpu.bitcast(lhs, bf16) if lhs.dtype == u32 else lhs.astype(bf16)
        y = _dot(lhs, pltpu.bitcast(rhs, bf16) if rhs.dtype == u32 else rhs)
        if acc is not None:
            y = y + acc
        hist.append(y)
        return y

    class Side:
        def __init__(self, pieces, n):
            self.pieces, self.n = list(pieces), n

        def __call__(self, val):
            take = -(-len(self.pieces) // self.n) if self.pieces else 0
            self.n -= 1
            if not take:
                return val
            never = zero_s[0] > 0
            rg = 8 if val.dtype == u32 else 16
            ng = val.shape[0] // rg
            groups = [val[8 * m:8 * m + 8] for m in range(val.shape[0] // 8)]
            for j, (fn, rd, wr, lag) in enumerate(self.pieces[:take]):
                m = (j + 1) * ng // take - 1
                pin = lambda v: v
                if lag is not None and len(hist) >= lag:
                    r0 = (16 * m) % hist[-lag].shape[0]
                    a = hist[-lag][r0:r0 + 8, :128]
                    if rd is None:
                        def pin(v, a=a):
                            t = jnp.where(never, jnp.concatenate([a] * (v.shape[0] // 8), axis=0), v[:, :128])
                            return t if v.shape[1] == 128 else jnp.concatenate([t, v[:, 128:]], axis=1)
                    else:
                        idx = tile_idx(rd)
                        rd[idx] = jnp.where(never, pltpu.bitcast(a, rd.dtype), rd[idx])
                fn(pin)
                g = m * rg // 8
                t = jnp.where(never, pltpu.bitcast(wr[tile_idx(wr)], val.dtype), groups[g][:, -128:])
                groups[g] = jnp.concatenate([groups[g][:, :-128], t], axis=1)
            self.pieces = self.pieces[take:]
            return jnp.concatenate(groups, axis=0)

    def strassen(lhs, rhs, side, init=(None, None, None, None), ks=range(7)):
        def add(a, b):
            return a if b is None else a + b
        sd = lambda k: side if k in ks else None
        p = [mm(lhs(k), rhs(k), sd(k)) for k in range(5)]
        c12 = add(p[2] + p[4], init[1])
        c21 = add(p[1] + p[3], init[2])
        c22 = mm(lhs(5), rhs(5), sd(5), add(p[0] - p[1] + p[2], init[3]))
        c11 = mm(lhs(6), rhs(6), sd(6), add(p[0] + p[3] - p[4], init[0]))
        return c11, c12, c21, c22

    def prep_pieces(s_v, raw, lag, width=256):
        def piece(r, c, pin):
            idx = (slice(r, r + 8), slice(c, c + width))
            b11, b12, b21, b22 = [_unpack(s_v[(q,) + idx]) for q in raw]
            for k, t in ((0, b11 + b22), (2, b12 - b22), (3, b21 - b11), (5, b11 + b12), (6, b21 + b22)):
                s_v[(k,) + idx] = _pack(t)
        return [(functools.partial(piece, r, c), s_v, s_v, lag)
                for r in range(0, s_v.shape[1], 8) for c in range(0, s_v.shape[2], width)]

    def store_l(slot, q, c, quads, plain=False):
        for k, t in enumerate(quads if plain else _lcombos(*quads)):
            l_v[slot, k, q // 2:q // 2 + 8, c:c + t.shape[1]] = _pack(t)

    def ln_pieces(src, r0, slot, lag, plain=False, width=256, staged=False, clag=None):
        def stats(q, pin):
            x = pin(src[pl.ds(r0 + q, 16), :].astype(f32))
            xs = [x[:, j * 128:(j + 1) * 128] for j in range(NT)]
            m = functools.reduce(lambda a, b: a + b, xs) * (1.0 / NT)
            w = functools.reduce(lambda a, b: a + b, [(t - m) * (t - m) for t in xs])
            mean = jnp.mean(m, axis=-1, keepdims=True)
            var = jnp.sum(w + NT * ((m - mean) * (m - mean)), axis=-1, keepdims=True) * (1.0 / D)
            n_v[0, q:q + 16, :] = jnp.broadcast_to(mean, (16, 128))
            n_v[1, q:q + 16, :] = jnp.broadcast_to(lax.rsqrt(var + EPS), (16, 128))

        def comb(q, c, pin):
            quads = []
            for rr in (0, HM):
                rs = pl.ds(pl.multiple_of(r0 + rr + q + zero_s[0], 16), 16)
                mean, rstd = [jnp.concatenate([n_v[t, rr + q:rr + q + 16, :]] * (width // 128), axis=1)
                              for t in range(2)]
                quads += [(src[rs, cc + c:cc + c + width].astype(f32) - mean) * rstd for cc in (0, DH2)]
            store_l(slot, q, c, quads, plain)
        norms = [[(functools.partial(stats, rr + q), None, n_v, lag) for rr in (0, HM)] for q in range(0, HM, 16)]
        combs = [[(functools.partial(comb, q, c), n_v, l_v, clag) for c in range(0, DH2, width)]
                 for q in range(0, HM, 16)]
        if staged:
            return sum(norms, []), sum(combs, [])
        out = list(norms[0])
        for a, b in zip(norms[1:] + [[]], combs):
            out += _merge(a, b) if a else b
        return out

    shifts = (1, 1, -1, -1, 2, 2, -2, -2)

    def shift_pieces(r0, slot, lag, by_value=False):
        def piece(q, j, pin):
            a = [h_v[jj, pl.ds(PAD + r0 + rr + q - shifts[jj], 16), :]
                 for rr in (0, HM) for jj in (j, j + NT // 2)]
            store_l(slot, q, j * 128, [pin(a[0]), a[1], a[2], pin(a[3])])
        return [(functools.partial(piece, q, j), None if by_value else h_v, l_v, lag)
                for q in range(0, HM, 16) for j in range(NT // 2)]

    def lhs_of(slot):
        return lambda k: l_v[slot, k]

    h_v[:, 0:PAD, :] = jnp.zeros((NT, PAD, 128), f32)
    h_v[:, PAD + S:PAD + S + PAD, :] = jnp.zeros((NT, PAD, 128), f32)

    def store_h(r0, c0, h):
        for j in range(h.shape[1] // 128):
            h_v[c0 // 128 + j, PAD + r0:PAD + r0 + h.shape[0], :] = h[:, j * 128:(j + 1) * 128]

    def d1_plain(xn, r0, c0, c1, step, side=None):
        for c in range(c0, c1, step):
            half, cc = c // DH2, c % DH2
            w = jnp.concatenate([s1_v[RAW1[half], :, cc:cc + step], s1_v[RAW1[2 + half], :, cc:cc + step]], axis=0)
            store_h(r0, c, _gelu(mm(xn, w, side)))

    NP1 = 7 * (DH2 // NC1)
    KS1 = (2, 3, 4, 5)

    def d1_s(b, slot, pieces):
        side = Side(pieces, len(KS1) * (DH2 // NC1))
        for c in range(0, DH2, NC1):
            cs = strassen(lhs_of(slot), lambda k: s1_v[k, :, c:c + NC1], side, ks=KS1)
            for q, t in enumerate(cs):
                store_h(b * TM + (q // 2) * HM, (q % 2) * DH2 + c, _gelu(t))

    def d2_s(b, slot, pieces):
        side = Side(pieces, NP1)
        for c in range(0, DH2, NC1):
            idx = [(slice(b * TM + (q // 2) * HM, b * TM + (q // 2 + 1) * HM),
                    slice((q % 2) * DH2 + c, (q % 2) * DH2 + c + NC1)) for q in range(4)]
            cs = strassen(lhs_of(slot), lambda k: s2_v[k, :, c:c + NC1], side,
                          [x_v[i].astype(f32) for i in idx])
            for i, t in zip(idx, cs):
                b_v[i] = t

    def split(l, n):
        return [l[len(l) * i // n:len(l) * (i + 1) // n] for i in range(n)]

    LS, LL = 3, 5

    wait("x0")
    xn0 = _pack(_ln(x_v[0:TM, :].astype(f32)))
    wait("x1")
    xn01 = jnp.concatenate([xn0, _pack(_ln(x_v[TM:2 * TM, :].astype(f32)))], axis=0)
    wait("w1a")
    d1_plain(xn01, 0, 0, 256, 256)
    wait("w1bc")
    d1_plain(xn01, 0, 256, 768, 256)
    wait("w1d", "x234")
    hist.clear()
    d1_plain(xn01, 0, 768, D, 128, Side(ln_pieces(x_v, 2 * TM, 0, None, plain=True), 2))
    xn2 = jnp.concatenate([jnp.concatenate([l_v[0, 2 * h], l_v[0, 2 * h + 1]], axis=1) for h in range(2)], axis=0)
    d1_plain(xn2, 2 * TM, 0, D, 128,
             Side(_merge(prep_pieces(s1_v, RAW1, 1), ln_pieces(x_v, 3 * TM, 1, 2)), 8))
    d1_s(3, 1, ln_pieces(x_v, 4 * TM, 0, LL))
    wait("x567", "w2")
    qkv_start(0)
    qkv_start(1)
    hist.clear()
    pw = split(prep_pieces(s2_v, RAW, LS), 4)
    for b in range(4, NB):
        nxt = ln_pieces(x_v, (b + 1) * TM, (b + 1) % 2, LL) if b + 1 < NB else shift_pieces(0, 0, LS, True)
        d1_s(b, b % 2, _merge(pw[b - 4], nxt))
    d2_s(0, 0, shift_pieces(TM, 1, LS, True))
    wait("w3")
    hist.clear()
    pw = split(prep_pieces(s3_v, RAW, LS), 4)
    for b in range(1, 5):
        d2_s(b, b % 2, _merge(pw[b - 1], shift_pieces((b + 1) * TM, (b + 1) % 2, LS)))
    wait("w4", "small")
    hist.clear()
    pw = prep_pieces(s4_v, RAW, LS)
    pw = [pw[:82], pw[82:164], pw[164:]]
    for b in range(5, NB):
        nxt = shift_pieces((b + 1) * TM, (b + 1) % 2, LS) if b + 1 < NB else ln_pieces(b_v, 0, 0, LL)
        d2_s(b, b % 2, _merge(pw[b - 5], nxt))
    start("wo", priority=1)

    def ffn(i, carry):
        qkv_wait(i)
        r0 = pl.multiple_of(i * TM, TM)
        rn = pl.multiple_of(jnp.minimum(i + 1, NB - 1) * TM, TM)
        lh = {}
        acc = [None] * 7
        hist.clear()

        def relayout(p, r0_, r1_, pin):
            s0 = i * SPG + 2 * p
            for r in range(r0_, r1_, 8):
                e = wqkv_v[s0, r:r + 8, :]
                o = wqkv_v[s0 + 1, r:r + 8, :]
                wqkv_v[s0, r:r + 8, :] = (e & jnp.uint32(0xFFFF)) | (o << 16)
                wqkv_v[s0 + 1, r:r + 8, :] = (e >> 16) | (o & jnp.uint32(0xFFFF0000))

        side3 = Side([(functools.partial(relayout, p, r, r + 32), wqkv_v, wqkv_v, 2)
                      for p in range(SPG // 2) for r in range(0, D // 2, 32)], 42 + 5)
        norms, combs = ln_pieces(b_v, rn, 0, 3, staged=True, width=128, clag=2)

        def gate(q, pin):
            gw = gw_ref[...].astype(f32)
            x = pin(x_v[pl.ds(r0 + q, 16), :].astype(f32))
            t = functools.reduce(lambda a, b: a + b,
                                 [x[:, j * 128:(j + 1) * 128] * gw[j:j + 1, :] for j in range(NT)])
            g = jax.nn.sigmoid(jnp.sum(t, axis=-1, keepdims=True))
            g_v[pl.ds(r0 + q, 16), :] = jnp.broadcast_to(g, (16, 128))

        gates = [(functools.partial(gate, q), None, g_v, 3) for q in range(0, TM, 16)]

        def extras(t, c, pin):
            jj = 2 * i + t
            a = [x_v[pl.ds(pl.multiple_of((jj + hh) * 64 + 24, 8), 16), cc + c:cc + c + 256].astype(f32)
                 for hh in (0, NPAIR // 2) for cc in (0, DH2)]
            for k, v in enumerate(_lcombos(pin(a[0]), a[1], a[2], pin(a[3]))):
                xe_v[k, pl.ds(pl.multiple_of(jj * 8, 8), 8), c:c + 256] = _pack(v)

        xes = [(functools.partial(extras, t, c), None, xe_v, 2) for t in range(2) for c in (0, 256)]
        side4 = Side(_merge(norms, gates, xes), 20)
        side5 = Side(combs, 11)

        def d3(c):
            cs = strassen(lhs_of(0), lambda k: s3_v[k, :, c * FC:(c + 1) * FC],
                          side3 if c > 0 else (lambda v: side3(v) if len(hist) >= 2 else v))
            lh[c] = _lcombos(*[_gelu(t) for t in cs])

        def d4(c):
            l = lh.pop(c)
            rhs = lambda k: s4_v[k, c * FC // 2:(c + 1) * FC // 2, :]
            if c + 1 < NFC:
                for k in range(7):
                    side = (side5 if k > 0 else None) if c == NFC - 2 else (side4 if k >= 3 else None)
                    acc[k] = mm(l[k], rhs(k), side, acc[k])
                return
            q = [mm(l[k], rhs(k), side5, acc[k]) for k in range(5)]
            top, bot = pl.ds(r0, HM), pl.ds(r0 + HM, HM)
            gt, gb = [jnp.concatenate([1.0 - g_v[r, :]] * (NT // 2), axis=1) for r in (top, bot)]
            b_v[top, DH2:] = gt * (q[2] + q[4] + b_v[top, DH2:])
            b_v[bot, :DH2] = gb * (q[1] + q[3] + b_v[bot, :DH2])
            b_v[bot, DH2:] = gb * mm(l[5], rhs(5), None, acc[5] + q[0] - q[1] + q[2] + b_v[bot, DH2:])
            b_v[top, :DH2] = gt * mm(l[6], rhs(6), None, acc[6] + q[0] + q[3] - q[4] + b_v[top, :DH2])

        d3(0)
        for c in range(NFC):
            if c + 1 < NFC:
                d3(c + 1)
            d4(c)
        assert not side3.pieces and not side4.pieces and not side5.pieces

        @pl.when(i + 2 < NG)
        def _():
            qkv_start(i + 2)

        return carry

    lax.fori_loop(0, NB, ffn, 0)

    def pre(it, carry):
        hist.clear()
        for u in range(3 * H // 2 // NPRE):
            s0 = it * (3 * H // NPRE) + 2 * u
            quad = [lambda k, s=s0 + q % 2, r=(q // 2) * (D // 4): wqkv_v[s + zero_s[k], r:r + D // 4, :]
                    for q in range(4)]
            cs = strassen(lambda k: xe_v[k], lambda k: _rcombo(k, *quad), None)
            for q, t in enumerate(cs):
                e_v[s0 + q % 2, (q // 2) * 128:(q // 2 + 1) * 128, :] = _pack(t)
        return carry

    lax.fori_loop(0, NPRE, pre, 0)

    wait("wo")
    mem_v[...] = mem0_ref[...].astype(f32)

    def slab(w, h):
        return (h // G) * SPG + w * G + h % G

    def step(j, hx, odd, late, allow, fill):
        qs, ks, vs, ps = {}, {}, {}, {}
        wload = lambda w, h: pltpu.bitcast(wqkv_v[slab(w, h)], bf16)
        eload = lambda w, h: pltpu.bitcast(e_v[slab(w, h), pl.ds(pl.multiple_of(j * 8, 8), 8), :], bf16)

        def proj(g):
            part = {}
            if late and g == 0:
                for h in range(2):
                    for w in range(3):
                        part[w, h] = _dot(hx[:, :DH2], wload(w, h)[:DH2])
            for h in range(g * G, (g + 1) * G):
                q, k, v = [(_dot(hx[:, DH2:], wload(w, h)[DH2:]) + part[w, h] if (w, h) in part
                            else _dot(hx, wload(w, h))).astype(bf16) for w in range(3)]
                if odd:
                    q = jnp.concatenate([q, eload(0, h)], axis=0)
                    k = jnp.concatenate([pltpu.bitcast(ke_v[h], bf16), eload(1, h), k], axis=0)
                    v = jnp.concatenate([pltpu.bitcast(ve_v[h], bf16), eload(2, h), v], axis=0)
                else:
                    ke_v[h] = pltpu.bitcast(k, u32)
                    ve_v[h] = pltpu.bitcast(v, u32)
                    k = jnp.concatenate([k, eload(1, h)], axis=0)
                    v = jnp.concatenate([v, eload(2, h)], axis=0)
                qs[h], ks[h], vs[h] = q, k, v

        def score(g):
            for h in range(g * G, (g + 1) * G):
                s = lax.dot_general(qs.pop(h), ks.pop(h), (((1,), (1,)), ((), ())),
                                    preferred_element_type=f32)
                ps[h] = _softmax(s, allow, fill)

        def pv(g):
            os_ = []
            for h in range(g * G, (g + 1) * G):
                o = _dot(ps.pop(h), vs.pop(h))
                o_v[:, h * 128:(h + 1) * 128] = _pack(o[:32])
                os_.append(o)
            if odd:
                quads = [jnp.concatenate([os_[2 * kk][r:r + 8], os_[2 * kk + 1][r:r + 8]], axis=1)
                         for r in (32, 40) for kk in range(2)]
                for k, t in enumerate(_lcombos(*quads)):
                    oe_v[k, pl.ds(pl.multiple_of(j * 8, 8), 8), g * 256:(g + 1) * 256] = t.astype(bf16)

        acc = [None] * NT

        def wo(h0, h1, j0, j1):
            o = pltpu.bitcast(o_v[:, h0 * 128:h1 * 128], bf16)
            for n in range(j0, j1):
                y = _dot(o, pltpu.bitcast(wo_v[n, h0 * 64:h1 * 64, :], bf16))
                acc[n] = y if acc[n] is None else y + acc[n]

        for t in range(NG):
            proj(t)
            if t >= 2:
                pv(t - 2)
            if t >= 1:
                score(t - 1)
        wo(0, 16, 0, 4)
        pv(NG - 2)
        score(NG - 1)
        wo(0, 16, 4, 8)
        pv(NG - 1)
        wo(16, 24, 0, 8)
        wo(24, 32, 0, 8)
        return jnp.concatenate(acc, axis=1)

    def emit(j, r0, o0, a):
        rs = pl.ds(r0 + o0, 24)
        g = jnp.concatenate([g_v[rs, :]] * NT, axis=1)
        out_v[j, o0:o0 + 24, :] = (g * a + b_v[rs, :]).astype(bf16)

    def pair(j, mem, late):
        r0 = pl.multiple_of(j * 64, 64)
        allow_e, fill_e, allow_o, fill_o = _masks()
        xa = x_v[pl.ds(r0 + 16, 8), :].astype(f32)
        xb = x_v[pl.ds(r0 + 40, 8), :].astype(f32)
        hx = jnp.concatenate([x_v[pl.ds(r0, 16), :], jnp.concatenate([xa, mem], 0).astype(bf16)], 0)
        oe = step(j, hx, False, late, allow_e, fill_e)
        emit(j, r0, 0, oe[:24])
        hx = jnp.concatenate([jnp.concatenate([oe[24:32], xb], 0).astype(bf16), x_v[pl.ds(r0 + 48, 16), :]], 0)
        oo = step(j, hx, True, True, allow_o, fill_o)
        emit(j, r0, 40, oo[8:])
        return oo[:8]

    def a_iter(it, carry):
        mem = mem_v[...]
        for t in range(PPI):
            mem = pair(it * PPI + t, mem, t > 0)
        mem_v[...] = mem
        for t in range(PPI):
            for o0 in (0, 40):
                idx = (it * PPI + t, pl.ds(o0, 24))
                pltpu.make_async_copy(out_v.at[idx], out_hbm.at[idx], sem_out).start()
        return carry

    lax.fori_loop(0, NPAIR // PPI, a_iter, 0)

    hist.clear()
    for n in range(NT // 2):
        quad = [lambda k, t=2 * n + q % 2, o=(q // 2) * 128: jnp.concatenate(
            [wo_v[t + zero_s[k], g * 256 + o:g * 256 + o + 128, :] for g in range(NG)], axis=0) for q in range(4)]
        cs = strassen(lambda k: oe_v[k], lambda k: _rcombo(k, *quad), None)
        cols = slice(n * 256, (n + 1) * 256)
        for half in range(2):
            t = jnp.concatenate(cs[2 * half:2 * half + 2], axis=1)
            o0 = 24 + half * 8
            for jj in range(NPAIR):
                rs = slice(jj * 64 + o0, jj * 64 + o0 + 8)
                g = jnp.concatenate([g_v[rs, :]] * 2, axis=1)
                out_v[jj, o0:o0 + 8, cols] = (g * t[jj * 8:jj * 8 + 8] + b_v[rs, cols]).astype(bf16)
        if n >= 2:
            idx = (slice(None), pl.ds(24, 16), pl.ds(0, 768) if n == 2 else pl.ds(768, 256))
            pltpu.make_async_copy(out_v.at[idx], out_hbm.at[idx], sem_out).start()
    pltpu.make_async_copy(out_v, out_hbm, sem_out).wait()


@functools.partial(jax.jit, static_argnames=("A_seg_len",))
def pallas_gated_mix__memory_aug_recurrent_mem_tr__mixer_s_mlp__prompt_kernel(
    A_x, A_mem0, A_Wq, A_Wk, A_Wv, A_Wo, A_seg_len, B_x, B_w1, B_w2, B_w3, B_w4, gate_w,
):
    assert A_seg_len == SEG
    assert A_x.shape == (1, S, D) and A_mem0.shape == (1, M, D)
    any_spec = pl.BlockSpec(memory_space=pl.ANY)
    out = pl.pallas_call(
        _kernel,
        out_shape=jax.ShapeDtypeStruct((NPAIR, 64, D), bf16),
        in_specs=[any_spec] * 11,
        out_specs=any_spec,
        scratch_shapes=[
            pltpu.VMEM((S, D), bf16),
            pltpu.VMEM((9, D // 4, D // 2), u32),
            pltpu.VMEM((7, D // 4, D // 2), u32),
            pltpu.VMEM((7, D // 4, F // 2), u32),
            pltpu.VMEM((7, F // 4, D // 2), u32),
            pltpu.VMEM((3 * H, D // 2, DH), u32),
            pltpu.VMEM((NT, H * DH // 2, 128), u32),
            pltpu.VMEM((NT, S + 2 * PAD, 128), f32),
            pltpu.VMEM((S, D), f32),
            pltpu.VMEM((2, 7, HM // 2, D // 2), u32),
            pltpu.VMEM((2, TM, 128), f32),
            pltpu.VMEM((S, 128), f32),
            pltpu.VMEM((NPAIR, 64, D), bf16),
            pltpu.VMEM((7, 4 * NPAIR, D // 2), u32),
            pltpu.VMEM((3 * H, 8 * NPAIR, DH), u32),
            pltpu.VMEM((7, 8 * NPAIR, H * DH // 2), bf16),
            pltpu.VMEM((H, 16, 128), u32),
            pltpu.VMEM((H, 16, 128), u32),
            pltpu.VMEM((16, H * DH), u32),
            pltpu.VMEM((M, D), f32),
            pltpu.VMEM((M, D), bf16),
            pltpu.VMEM((NT, 128), bf16),
            pltpu.SMEM((8,), jnp.int32),
            pltpu.SemaphoreType.DMA((NLOAD,)),
            pltpu.SemaphoreType.DMA((NG,)),
            pltpu.SemaphoreType.DMA,
        ],
        compiler_params=pltpu.CompilerParams(vmem_limit_bytes=126 * 1024 * 1024,
                                             disable_bounds_checks=True),
    )(
        A_x.reshape(S, D), A_mem0.reshape(M, D),
        A_Wq.reshape(D // 2, 2 * H, DH), A_Wk.reshape(D // 2, 2 * H, DH), A_Wv.reshape(D // 2, 2 * H, DH),
        A_Wo.reshape(H * DH, D), B_w1, B_w2, B_w3, B_w4, gate_w.reshape(NT, 128),
    )
    return out.reshape(1, S, D)
```

```python
import functools

import jax
import jax.numpy as jnp
from jax import lax
import jax.experimental.pallas as pl
import jax.experimental.pallas.tpu as pltpu

f32, bf16, u32 = jnp.float32, jnp.bfloat16, jnp.uint32

S, D, H, DH, M, SEG, F = 2048, 1024, 32, 128, 8, 32, 3584
SCALE = DH ** -0.5
NEG = -1000000000.0
EPS = 1e-05

TM = 256
NB = S // TM
HM = TM // 2
DH2 = D // 2
D4, F4 = D // 4, F // 4
FCH = ((0, 256), (256, 512), (512, 768), (768, 896))
NC1 = 128
NPAIR = S // (2 * SEG)
PPI = 2
NPRE = 4
G = 4
NG = H // G
PAD = 8
NT = D // 128
NLOAD = 12
assert NB == NG

_dot = functools.partial(jnp.dot, preferred_element_type=f32)

UP = ((4, 1, 5, 1), (6, 1, 8, 1), (0, 1, 3, 1), (2, -1, 9, 1), (4, -1, 10, 1), (0, 1, 1, 1), (2, 1, 12, 1),
      (5, 1, 7, -1), (7, 1, 12, -1), (11, -1, 13, 1), (10, -1, 11, 1), (2, 1, 7, 1), (0, -1, 4, 1),
      (6, 1, 7, 1), (1, -1, 5, 1), (3, 1, 7, -1), (1, 1, 4, 1), (2, 1, 3, 1), (1, -1, 3, 1), (1, 1, 7, -1),
      (2, 1, 6, -1))
WP = ((0, -1, 3, 1), (4, 1, 6, -1), (1, 1, 8, 1), (5, 1, 10, 1), (4, -1, 7, 1), (0, -1, 9, -1),
      (11, 1, 12, 1), (6, 1, 7, -1), (2, 1, 5, -1), (0, -1, 7, -1), (9, 1, 11, -1), (2, 1, 13, 1),
      (5, 1, 13, 1), (2, -1, 3, 1), (5, 1, 6, 1), (0, 1, 4, 1), (2, 1, 7, 1), (1, 1, 2, 1), (1, 1, 5, 1),
      (3, 1, 7, 1), (2, 1, 6, 1))
VP = ((1, 1, 5, -1), (8, 1, 11, 1), (10, 1, 17, 1), (13, 1, 16, -1), (0, 1, 4, -1), (0, 1, 3, 1),
      (14, 1, 18, -1), (0, 1, 11, 1), (14, 1, 19, -1), (0, 1, 5, 1), (12, 1, 15, 1), (2, 1, 21, 1),
      (10, 1, 14, -1), (4, 1, 7, 1), (11, 1, 19, 1), (12, -1, 20, 1), (13, 1, 14, -1), (9, 1, 30, -1),
      (3, -1, 15, 1), (6, 1, 23, 1), (24, 1, 27, -1), (9, -1, 18, 1), (7, 1, 34, 1), (2, 1, 6, -1),
      (0, 1, 8, -1), (6, 1, 21, 1), (22, 1, 31, -1), (6, 1, 29, 1), (0, 1, 1, 1), (15, 1, 25, 1),
      (5, 1, 37, 1), (15, 1, 20, 1))
UN = (7, 27, 24, 17, 9, 22, 21, 2, 15, 11, 8, 25, 19, 28, 2, 23, 26, 20, 1, 18, 10, 28, 4, 13, 14, 16)
WN = (23, 17, 24, 10, 14, 7, 22, 19, 12, 18, 15, 25, 20, 5, 26, 0, 8, 2, 27, 11, 26, 9, 28, 21, 16, 5)
VN = (42, 47, 41, 5, 11, 43, 18, 28, 20, 23, 35, 19, 22, 46, 33, 26, 45, 36, 38, 25, 44, 40, 39, 21, 24, 32)
RK = len(UN)
UL = tuple(sorted(set(UN)))
_free = iter(r for r in range(RK) if VN[r] >= 16)
RAW16 = tuple(VN.index(b) if b in VN else next(_free) for b in range(16))


def _run(prog, blocks):
    vals = list(blocks)
    for a, sa, b, sb in prog:
        vals.append(vals[a] + vals[b] if sa > 0 and sb > 0 else
                    vals[a] - vals[b] if sa > 0 else vals[b] - vals[a])
    return vals


def _terms(prog, nin, node):
    if node < nin:
        return {node: 1}
    a, sa, b, sb = prog[node - nin]
    out = {k: sa * v for k, v in _terms(prog, nin, a).items()}
    out.update({k: sb * v for k, v in _terms(prog, nin, b).items()})
    return out


_WPAR = {n: [] for n in range(8 + len(WP))}
for _t, (_a, _sa, _b, _sb) in enumerate(WP):
    _WPAR[_a].append((8 + _t, _sa))
    _WPAR[_b].append((8 + _t, _sb))


def _worder():
    order = []

    def closure(n, acc):
        if n not in acc and n not in order:
            acc.add(n)
            for q, _ in _WPAR[n]:
                closure(q, acc)
        return acc

    def visit(n):
        if n not in order:
            for q, _ in _WPAR[n]:
                visit(q)
            order.append(n)
    while len([v for v in range(8) if v not in order]):
        visit(min((v for v in range(8) if v not in order), key=lambda v: len(closure(v, set()))))
    return tuple(order)


WORDER = _worder()


def _ln(x):
    m = jnp.mean(x, axis=-1, keepdims=True)
    xc = x - m
    v = jnp.mean(xc * xc, axis=-1, keepdims=True)
    return xc * lax.rsqrt(v + EPS)


_GC = 0.7978845608028654


def _gelu(x):
    h = 0.5 * x
    return h + h * jnp.tanh(x * (_GC + (_GC * 0.044715) * (x * x)))


def _unpack(u):
    return pltpu.bitcast(u, bf16).astype(f32)


def _pack(x):
    return pltpu.bitcast(x.astype(bf16), u32)


def _lcombos(a11, a12, a21, a22):
    return [a11 + a22, a21 + a22, a11, a22, a11 + a12, a21 - a11, a12 - a22]


def _merge(*lists):
    keyed = [((j + 0.5) / len(l), n, j, v) for n, l in enumerate(lists) for j, v in enumerate(l)]
    return [v for _, _, _, v in sorted(keyed, key=lambda t: t[:3])]


def _masks():
    r = lax.broadcasted_iota(jnp.int32, (32, 48), 0)
    c = lax.broadcasted_iota(jnp.int32, (32, 48), 1)
    exist_e = c < 40
    allow_e = exist_e & ((r >= 24) | ((c >= 24) & (c < 32)) | (c <= r))
    fill_e = jnp.where(exist_e, NEG, -jnp.inf).astype(f32)
    r = lax.broadcasted_iota(jnp.int32, (48, 80), 0)
    c = lax.broadcasted_iota(jnp.int32, (48, 80), 1)
    q_even = (r >= 32) & (r < 40)
    exist_o = (q_even & (c < 40)) | (~q_even & (c >= 40))
    ktok = jnp.where(c < 24, c, jnp.where(c < 48, c - 8, c - 16))
    qtok = jnp.where(r < 32, r + 32, r - 8)
    is_mem_key = ((c >= 24) & (c < 32)) | ((c >= 48) & (c < 56))
    allow_o = exist_o & (is_mem_key | (r < 8) | (ktok <= qtok))
    fill_o = jnp.where(exist_o, NEG, -jnp.inf).astype(f32)
    return allow_e, fill_e, allow_o, fill_o


def _rcombo(k, b11, b12, b21, b22):
    if k in (1, 4):
        return (b11 if k == 1 else b22)(k)
    a, b, sign = {0: (b11, b22, 1), 2: (b12, b22, -1), 3: (b21, b11, -1), 5: (b11, b12, 1), 6: (b21, b22, 1)}[k]
    a, b = _unpack(a(k)), _unpack(b(k))
    return (a + b if sign > 0 else a - b).astype(bf16)


def _softmax(s, allow, fill):
    s = jnp.where(allow, s * SCALE, fill)
    m = jnp.max(s, axis=-1, keepdims=True)
    e = jnp.exp(s - m)
    l = jnp.sum(e, axis=-1, keepdims=True)
    r = pl.reciprocal(l, approx=True)
    r = r * (2.0 - l * r)
    return (e * r).astype(bf16)


def _kernel(x_hbm, mem0_hbm, wq_hbm, wk_hbm, wv_hbm, wo_hbm, w1_hbm, w2_hbm, w3_hbm, w4_hbm,
            gw_hbm, out_hbm,
            x_v, s1_v, s2_v, s3_v, s4_v, wqkv_v, wo_v, h_v, b_v, l_v, lf_v, n_v, g_v, out_v, xe_v, e_v, oe_v,
            ke_v, ve_v, o_v, mem_v, mem0_ref, gw_ref, zero_s,
            sem, sem_qkv, sem_out):
    RAW = (1, 2, 3, 4)
    RAW1 = (1, 7, 8, 4)

    loads = []

    def rows_load(name, r0, r1):
        loads.append((name, x_hbm.at[pl.ds(r0, r1 - r0)], x_v.at[pl.ds(r0, r1 - r0)]))

    def quad_load(name, w_hbm, s_v, raw, q, c0=0, c1=None):
        k4, n2 = s_v.shape[1], s_v.shape[2]
        c1 = n2 if c1 is None else c1
        src = w_hbm.bitcast(u32).at[pl.ds((q // 2) * k4, k4), pl.ds((q % 2) * n2 + c0, c1 - c0)]
        loads.append((name, src, s_v.at[raw[q], :, pl.ds(c0, c1 - c0)]))

    rows_load("x0", 0, TM)
    rows_load("x1", TM, 2 * TM)
    for name, half, c0, c1 in (("w1a", 0, 0, 256), ("w1bc", 0, 256, 512), ("w1bc", 1, 0, 256), ("w1d", 1, 256, 512)):
        quad_load(name, w1_hbm, s1_v, RAW1, half, c0, c1)
        quad_load(name, w1_hbm, s1_v, RAW1, 2 + half, c0, c1)
    rows_load("x234", 2 * TM, 5 * TM)
    rows_load("x567", 5 * TM, S)
    for q in range(4):
        quad_load("w2", w2_hbm, s2_v, RAW, q)
    for name, w_hbm, s_v in (("w3", w3_hbm, s3_v), ("w4", w4_hbm, s4_v)):
        kb, nb = s_v.shape[1:]
        for q in range(16):
            loads.append((name, w_hbm.at[pl.ds((q // 4) * kb, kb), pl.ds((q % 4) * nb, nb)], s_v.at[RAW16[q]]))
    loads.append(("small", mem0_hbm, mem0_ref))
    loads.append(("small", gw_hbm, gw_ref))
    for j in range(NT):
        loads.append(("wo", wo_hbm.bitcast(u32).at[:, pl.ds(j * 128, 128)], wo_v.at[j]))
    groups = list(dict.fromkeys(name for name, _, _ in loads))
    assert len(groups) == NLOAD

    def start(*names, priority=0):
        for name, src, dst in loads:
            if name in names:
                pltpu.make_async_copy(src, dst, sem.at[groups.index(name)]).start(priority=priority)

    def wait(*names):
        for name, src, dst in loads:
            if name in names:
                pltpu.make_async_copy(src, dst, sem.at[groups.index(name)]).wait()

    SPG = 3 * G

    def qkv_start(g):
        for w, w_hbm in enumerate((wq_hbm, wk_hbm, wv_hbm)):
            wu = w_hbm.bitcast(u32)
            for k in range(G // 2):
                for par in range(2):
                    pltpu.make_async_copy(
                        wu.at[:, par * (H // 2) + g * (G // 2) + k, :],
                        wqkv_v.at[g * SPG + w * G + 2 * k + par], sem_qkv.at[g]).start(priority=1)

    def qkv_wait(g):
        grp = wqkv_v.at[pl.ds(g * SPG, SPG)]
        pltpu.make_async_copy(grp, grp, sem_qkv.at[g]).wait()

    start("x0", "x1", "w1a", "w1bc", "w1d", "x234", "x567", "w2", "w3", "w4", "small")
    for k in range(RK):
        zero_s[k] = 0

    def tile_idx(ref, cols=128):
        z = zero_s[0]
        n = 16 if ref.dtype == bf16 and cols == 128 else 8
        return (z,) * (len(ref.shape) - 2) + (pl.ds(pl.multiple_of(z, n), n), slice(0, cols))

    hist = []

    def mm(lhs, rhs, side=None, acc=None):
        if side is not None:
            lhs = side(lhs)
        lhs = pltpu.bitcast(lhs, bf16) if lhs.dtype == u32 else lhs.astype(bf16)
        y = _dot(lhs, pltpu.bitcast(rhs, bf16) if rhs.dtype == u32 else rhs)
        if acc is not None:
            y = y + acc
        hist.append(y)
        return y

    class Side:
        def __init__(self, pieces, n, skip=0):
            self.pieces, self.n, self.skip = list(pieces), n, skip

        def __call__(self, val):
            if self.skip:
                self.skip -= 1
                return val
            take = -(-len(self.pieces) // self.n) if self.pieces else 0
            self.n -= 1
            if not take:
                return val
            never = zero_s[0] > 0
            if val.dtype == bf16:
                val = pltpu.bitcast(val, u32)
            rg = 8 if val.dtype == u32 else 16
            ng = val.shape[0] // rg
            groups = [val[8 * m:8 * m + 8] for m in range(val.shape[0] // 8)]
            for j, (fn, rd, wr, lag) in enumerate(self.pieces[:take]):
                m = (j + 1) * ng // take - 1
                pin = lambda v: v
                if lag is not None and len(hist) >= lag:
                    r0 = (16 * m) % hist[-lag].shape[0]
                    a = hist[-lag][r0:r0 + 8, :128]
                    if rd is None:
                        def pin(v, a=a):
                            t = jnp.where(never, jnp.concatenate([a] * (v.shape[0] // 8), axis=0), v[:, :128])
                            return t if v.shape[1] == 128 else jnp.concatenate([t, v[:, 128:]], axis=1)
                    elif rd.dtype == bf16:
                        idx = tile_idx(rd, 256)
                        rd[idx] = jnp.where(never, jnp.concatenate([a, a], axis=1).astype(bf16), rd[idx])
                    else:
                        idx = tile_idx(rd)
                        rd[idx] = jnp.where(never, pltpu.bitcast(a, rd.dtype), rd[idx])
                tiles = fn(pin)
                g = m * rg // 8
                t = groups[g][:, -128:]
                for u in (tiles if wr is None else [wr[tile_idx(wr)]]):
                    t = jnp.where(never, pltpu.bitcast(u, val.dtype), t)
                groups[g] = t if val.shape[1] == 128 else jnp.concatenate([groups[g][:, :-128], t], axis=1)
            self.pieces = self.pieces[take:]
            return jnp.concatenate(groups, axis=0)

    def strassen(lhs, rhs, side, init=(None, None, None, None), ks=range(7)):
        def add(a, b):
            return a if b is None else a + b
        sd = lambda k: side if k in ks else None
        p = [mm(lhs(k), rhs(k), sd(k)) for k in range(5)]
        c12 = add(p[2] + p[4], init[1])
        c21 = add(p[1] + p[3], init[2])
        c22 = mm(lhs(5), rhs(5), sd(5), add(p[0] - p[1] + p[2], init[3]))
        c11 = mm(lhs(6), rhs(6), sd(6), add(p[0] + p[3] - p[4], init[0]))
        return c11, c12, c21, c22

    def fmm(lhs, rhs, side, extra=lambda n: None):
        val = {}
        for n in WORDER:
            t = extra(n)
            for q, sg in sorted(_WPAR[n], key=lambda e: -e[1]):
                t = val[q] if t is None else (t + val[q] if sg > 0 else t - val[q])
            for r in range(RK):
                if WN[r] == n:
                    t = mm(lhs(UN[r]), rhs(r), side, t)
            val[n] = t
        return [val[v] for v in range(8)]

    def prep26_pieces(s_v, lag):
        def piece(rs, cs, pin):
            vals = _run(VP, [s_v[q, rs, cs].astype(f32) for q in RAW16])
            for r in range(RK):
                if VN[r] >= 16:
                    s_v[r, rs, cs] = vals[VN[r]].astype(bf16)
        kb, nb = s_v.shape[1:]
        out = []
        for r in range(0, kb, 16):
            out += [(slice(rr, rr + 8), slice(c, c + 256)) for c in range(0, nb - 255, 256) for rr in (r, r + 8)]
            out += [(slice(r, r + 16), slice(nb - 128, nb))] if nb % 256 else []
        return [(functools.partial(piece, rs, cs), s_v, s_v, lag) for rs, cs in out]

    def prep_pieces(s_v, raw, lag, width=256):
        def piece(r, c, pin):
            idx = (slice(r, r + 8), slice(c, c + width))
            b11, b12, b21, b22 = [_unpack(s_v[(q,) + idx]) for q in raw]
            for k, t in ((0, b11 + b22), (2, b12 - b22), (3, b21 - b11), (5, b11 + b12), (6, b21 + b22)):
                s_v[(k,) + idx] = _pack(t)
        return [(functools.partial(piece, r, c), s_v, s_v, lag)
                for r in range(0, s_v.shape[1], 8) for c in range(0, s_v.shape[2], width)]

    def store_l(slot, q, c, quads, plain=False):
        for k, t in enumerate(quads if plain else _lcombos(*quads)):
            l_v[slot, k, q // 2:q // 2 + 8, c:c + t.shape[1]] = _pack(t)

    def ln_pieces(src, r0, slot, lag, plain=False, width=256, staged=False, clag=None, dyn=True):
        def stats(q, pin):
            x = pin(src[pl.ds(r0 + q, 16), :].astype(f32))
            xs = [x[:, j * 128:(j + 1) * 128] for j in range(NT)]
            m = functools.reduce(lambda a, b: a + b, xs) * (1.0 / NT)
            w = functools.reduce(lambda a, b: a + b, [(t - m) * (t - m) for t in xs])
            mean = jnp.mean(m, axis=-1, keepdims=True)
            var = jnp.sum(w + NT * ((m - mean) * (m - mean)), axis=-1, keepdims=True) * (1.0 / D)
            n_v[0, q:q + 16, :] = jnp.broadcast_to(mean, (16, 128))
            n_v[1, q:q + 16, :] = jnp.broadcast_to(lax.rsqrt(var + EPS), (16, 128))

        def comb(q, c, pin):
            quads = []
            for rr in (0, HM):
                rs = pl.ds(pl.multiple_of(r0 + rr + q + zero_s[0], 16), 16)
                mean, rstd = [jnp.concatenate([n_v[t, rr + q:rr + q + 16, :]] * (width // 128), axis=1)
                              for t in range(2)]
                quads += [(src[rs, cc + c:cc + c + width].astype(f32) - mean) * rstd for cc in (0, DH2)]
            store_l(slot, q, c, quads, plain)

        def comb26(q, pin):
            blocks = []
            for rr in (0, HM):
                rs = pl.ds(pl.multiple_of(r0 + rr + q + (zero_s[0] if dyn else 0), 8), 8)
                mean, rstd = [jnp.concatenate([n_v[t, rr + q:rr + q + 8, :]] * 2, axis=1) for t in range(2)]
                blocks += [(src[rs, cc:cc + D4] - mean) * rstd for cc in range(0, D, D4)]
            vals = _run(UP, blocks)
            for k, u in enumerate(UL):
                lf_v[k, q:q + 8, :] = vals[u].astype(bf16)
        norms = [[(functools.partial(stats, rr + q), None, n_v, lag) for rr in (0, HM)] for q in range(0, HM, 16)]
        if slot is None:
            combs = [[(functools.partial(comb26, qq), n_v, lf_v, clag) for qq in (q, q + 8)]
                     for q in range(0, HM, 16)]
        else:
            combs = [[(functools.partial(comb, q, c), n_v, l_v, clag) for c in range(0, DH2, width)]
                     for q in range(0, HM, 16)]
        if staged:
            return sum(norms, []), sum(combs, [])
        out = list(norms[0])
        for a, b in zip(norms[1:] + [[]], combs):
            out += _merge(a, b) if a else b
        return out

    shifts = (1, 1, -1, -1, 2, 2, -2, -2)

    def shift_pieces(r0, slot, lag, by_value=False):
        def piece(q, j, pin):
            a = [h_v[jj, pl.ds(PAD + r0 + rr + q - shifts[jj], 16), :]
                 for rr in (0, HM) for jj in (j, j + NT // 2)]
            store_l(slot, q, j * 128, [pin(a[0]), a[1], a[2], pin(a[3])])
        return [(functools.partial(piece, q, j), None if by_value else h_v, l_v, lag)
                for q in range(0, HM, 16) for j in range(NT // 2)]

    def lhs_of(slot):
        return lambda k: l_v[slot, k]

    h_v[:, 0:PAD, :] = jnp.zeros((NT, PAD, 128), f32)
    h_v[:, PAD + S:PAD + S + PAD, :] = jnp.zeros((NT, PAD, 128), f32)

    def store_h(r0, c0, h):
        for j in range(h.shape[1] // 128):
            h_v[c0 // 128 + j, PAD + r0:PAD + r0 + h.shape[0], :] = h[:, j * 128:(j + 1) * 128]

    def d1_plain(xn, r0, c0, c1, step, side=None):
        for c in range(c0, c1, step):
            half, cc = c // DH2, c % DH2
            w = jnp.concatenate([s1_v[RAW1[half], :, cc:cc + step], s1_v[RAW1[2 + half], :, cc:cc + step]], axis=0)
            store_h(r0, c, _gelu(mm(xn, w, side)))

    NP1 = 7 * (DH2 // NC1)
    KS1 = (2, 3, 4, 5)

    def d1_s(b, slot, pieces):
        side = Side(pieces, len(KS1) * (DH2 // NC1))
        for c in range(0, DH2, NC1):
            cs = strassen(lhs_of(slot), lambda k: s1_v[k, :, c:c + NC1], side, ks=KS1)
            for q, t in enumerate(cs):
                store_h(b * TM + (q // 2) * HM, (q % 2) * DH2 + c, _gelu(t))

    def d2_s(b, slot, pieces):
        side = Side(pieces, NP1)
        for c in range(0, DH2, NC1):
            idx = [(slice(b * TM + (q // 2) * HM, b * TM + (q // 2 + 1) * HM),
                    slice((q % 2) * DH2 + c, (q % 2) * DH2 + c + NC1)) for q in range(4)]
            cs = strassen(lhs_of(slot), lambda k: s2_v[k, :, c:c + NC1], side,
                          [x_v[i].astype(f32) for i in idx])
            for i, t in zip(idx, cs):
                b_v[i] = t

    def split(l, n):
        return [l[len(l) * i // n:len(l) * (i + 1) // n] for i in range(n)]

    LS, LL = 3, 5

    wait("x0")
    xn0 = _pack(_ln(x_v[0:TM, :].astype(f32)))
    wait("x1")
    xn01 = jnp.concatenate([xn0, _pack(_ln(x_v[TM:2 * TM, :].astype(f32)))], axis=0)
    wait("w1a")
    d1_plain(xn01, 0, 0, 256, 256)
    wait("w1bc")
    d1_plain(xn01, 0, 256, 768, 256)
    wait("w1d", "x234")
    hist.clear()
    d1_plain(xn01, 0, 768, D, 128, Side(ln_pieces(x_v, 2 * TM, 0, None, plain=True), 2))
    xn2 = jnp.concatenate([jnp.concatenate([l_v[0, 2 * h], l_v[0, 2 * h + 1]], axis=1) for h in range(2)], axis=0)
    d1_plain(xn2, 2 * TM, 0, D, 128,
             Side(_merge(prep_pieces(s1_v, RAW1, 1), ln_pieces(x_v, 3 * TM, 1, 2)), 8))
    d1_s(3, 1, ln_pieces(x_v, 4 * TM, 0, LL))
    wait("x567", "w2")
    qkv_start(0)
    qkv_start(1)
    hist.clear()
    pw = split(prep_pieces(s2_v, RAW, LS), 4)
    for b in range(4, NB):
        nxt = ln_pieces(x_v, (b + 1) * TM, (b + 1) % 2, LL) if b + 1 < NB else shift_pieces(0, 0, LS, True)
        d1_s(b, b % 2, _merge(pw[b - 4], nxt))
    d2_s(0, 0, shift_pieces(TM, 1, LS, True))
    wait("w3")
    hist.clear()
    pw = split(prep26_pieces(s3_v, LS), 4)
    for b in range(1, 5):
        d2_s(b, b % 2, _merge(pw[b - 1], shift_pieces((b + 1) * TM, (b + 1) % 2, LS)))
    wait("w4", "small")
    hist.clear()
    pw = prep26_pieces(s4_v, LS)
    pw = [pw[:40], pw[40:80], pw[80:]]
    for b in range(5, NB):
        nxt = (shift_pieces((b + 1) * TM, (b + 1) % 2, LS) if b + 1 < NB else
               ln_pieces(b_v, 0, None, LL, dyn=False))
        d2_s(b, b % 2, _merge(pw[b - 5], nxt))
    start("wo", priority=1)

    def ffn(i, carry):
        qkv_wait(i)
        r0 = pl.multiple_of(i * TM, TM)
        rn = pl.multiple_of(jnp.minimum(i + 1, NB - 1) * TM, TM)
        acc = {}
        hist.clear()

        def relayout(p, r0_, r1_, pin):
            s0 = i * SPG + 2 * p
            for r in range(r0_, r1_, 8):
                e = wqkv_v[s0, r:r + 8, :]
                o = wqkv_v[s0 + 1, r:r + 8, :]
                wqkv_v[s0, r:r + 8, :] = (e & jnp.uint32(0xFFFF)) | (o << 16)
                wqkv_v[s0 + 1, r:r + 8, :] = (e >> 16) | (o & jnp.uint32(0xFFFF0000))

        relays = [(functools.partial(relayout, p, r, r + 32), wqkv_v, wqkv_v, 3)
                  for p in range(SPG // 2) for r in range(0, D // 2, 32)]
        norms, combs = ln_pieces(b_v, rn, None, 5, staged=True, clag=3)

        def gate(q, pin):
            gw = gw_ref[...].astype(f32)
            x = pin(x_v[pl.ds(r0 + q, 16), :].astype(f32))
            t = functools.reduce(lambda a, b: a + b,
                                 [x[:, j * 128:(j + 1) * 128] * gw[j:j + 1, :] for j in range(NT)])
            g = jax.nn.sigmoid(jnp.sum(t, axis=-1, keepdims=True))
            g_v[pl.ds(r0 + q, 16), :] = jnp.broadcast_to(g, (16, 128))

        gates = [(functools.partial(gate, q), None, g_v, 5) for q in range(0, TM, 16)]

        def extras(t, pin):
            jj, o = 2 * i + t // 2, 24 + 8 * (t % 2)
            xs = [pin(x_v[pl.ds(pl.multiple_of((jj + hh) * 64 + o, 8), 8), :].astype(f32)) for hh in (0, NPAIR // 2)]
            vals = _run(UP, [x[:, cc:cc + D4] for x in xs for cc in range(0, D, D4)])
            for k, u in enumerate(UL):
                xe_v[k, pl.ds(pl.multiple_of(i * 32 + t * 8, 8), 8), :] = vals[u].astype(bf16)

        xes = [(functools.partial(extras, t), None, xe_v, 3) for t in range(4)]
        hs = {}

        def gelu_pieces(c, cs):
            def piece(r, cc, vs, pin):
                for v in vs:
                    hs[c, v, r, cc] = _gelu(pin(cs[v][r:r + 8, cc:cc + 128]))
                return [hs[c, v, r, cc] for v in vs]
            return [(functools.partial(piece, r, cc, vs), None, None, 3) for r in range(0, HM, 8)
                    for cc in range(0, cs[0].shape[1], 128) for vs in ((0, 1, 2, 3), (4, 5, 6, 7))]

        def d3(c, side):
            c0, c1 = FCH[c]
            cs = fmm(lambda u: lf_v[UL.index(u)], lambda r: s3_v[r, :, c0:c1], side)
            assert not side.pieces
            return gelu_pieces(c, cs)

        def d4(c, side):
            c0, c1 = FCH[c]
            lh = _run(UP, [jnp.concatenate([jnp.concatenate(
                [hs.pop((c, v, r, cc)) for cc in range(0, c1 - c0, 128)], axis=1) for r in range(0, HM, 8)], axis=0)
                for v in range(8)])
            rhs = lambda r: s4_v[r, c0:c1, :]
            if c + 1 < len(FCH):
                for n in WORDER:
                    for r in range(RK):
                        if WN[r] == n:
                            acc[n] = mm(lh[UN[r]], rhs(r), side, acc.get(n))
            else:
                idx = lambda v: (pl.ds(r0 + (v // 4) * HM, HM), slice((v % 4) * D4, (v % 4 + 1) * D4))

                def extra(n):
                    if n >= 8:
                        return acc.get(n)
                    return b_v[idx(n)] + acc[n] if n in acc else b_v[idx(n)]
                for v, t in enumerate(fmm(lambda u: lh[u], rhs, side, extra)):
                    b_v[idx(v)] = jnp.concatenate([1.0 - g_v[idx(v)[0], :]] * 2, axis=1) * t
            assert not side.pieces

        g0 = d3(0, Side(_merge(relays[:40], gates), 24, 2))
        g1 = d3(1, Side(g0, 23, 2))
        d4(0, Side(g1, 23, 2))
        g2 = d3(2, Side(_merge(relays[40:76], norms, xes), 26))
        d4(1, Side(g2, 23, 2))
        g3 = d3(3, Side(relays[76:], 26))
        d4(2, Side(_merge(g3, combs[:10]), 23, 2))
        d4(3, Side(combs[10:], 12))

        @pl.when(i + 2 < NG)
        def _():
            qkv_start(i + 2)

        return carry

    lax.fori_loop(0, NB, ffn, 0)

    def pre(it, carry):
        hist.clear()
        for u in range(3 * NG // NPRE):
            s0 = (it * (3 * NG // NPRE) + u) * G

            def rhs(r):
                t = None
                for q, sg in sorted(_terms(VP, 16, VN[r]).items(), key=lambda e: -e[1]):
                    blk = wqkv_v[s0 + q % 4 + zero_s[r], (q // 4) * (D // 8):(q // 4 + 1) * (D // 8), :]
                    if VN[r] < 16:
                        return blk
                    blk = _unpack(blk)
                    t = blk if t is None else (t + blk if sg > 0 else t - blk)
                return t.astype(bf16)
            for v, t in enumerate(fmm(lambda k: xe_v[UL.index(k)], rhs, None)):
                e_v[s0 + v % 4, (v // 4) * 128:(v // 4 + 1) * 128, :] = _pack(t)
        return carry

    lax.fori_loop(0, NPRE, pre, 0)

    wait("wo")
    mem_v[...] = mem0_ref[...].astype(f32)

    def slab(w, h):
        return (h // G) * SPG + w * G + h % G

    def step(j, hx, odd, late, allow, fill):
        qs, ks, vs, ps = {}, {}, {}, {}
        wload = lambda w, h: pltpu.bitcast(wqkv_v[slab(w, h)], bf16)
        eload = lambda w, h: pltpu.bitcast(e_v[slab(w, h), pl.ds(pl.multiple_of(j * 8, 8), 8), :], bf16)

        def proj(g):
            part = {}
            if late and g == 0:
                for h in range(2):
                    for w in range(3):
                        part[w, h] = _dot(hx[:, :DH2], wload(w, h)[:DH2])
            for h in range(g * G, (g + 1) * G):
                q, k, v = [(_dot(hx[:, DH2:], wload(w, h)[DH2:]) + part[w, h] if (w, h) in part
                            else _dot(hx, wload(w, h))).astype(bf16) for w in range(3)]
                if odd:
                    q = jnp.concatenate([q, eload(0, h)], axis=0)
                    k = jnp.concatenate([pltpu.bitcast(ke_v[h], bf16), eload(1, h), k], axis=0)
                    v = jnp.concatenate([pltpu.bitcast(ve_v[h], bf16), eload(2, h), v], axis=0)
                else:
                    ke_v[h] = pltpu.bitcast(k, u32)
                    ve_v[h] = pltpu.bitcast(v, u32)
                    k = jnp.concatenate([k, eload(1, h)], axis=0)
                    v = jnp.concatenate([v, eload(2, h)], axis=0)
                qs[h], ks[h], vs[h] = q, k, v

        def score(g):
            for h in range(g * G, (g + 1) * G):
                s = lax.dot_general(qs.pop(h), ks.pop(h), (((1,), (1,)), ((), ())),
                                    preferred_element_type=f32)
                ps[h] = _softmax(s, allow, fill)

        def pv(g):
            os_ = []
            for h in range(g * G, (g + 1) * G):
                o = _dot(ps.pop(h), vs.pop(h))
                o_v[:, h * 128:(h + 1) * 128] = _pack(o[:32])
                os_.append(o)
            if odd:
                quads = [jnp.concatenate([os_[2 * kk][r:r + 8], os_[2 * kk + 1][r:r + 8]], axis=1)
                         for r in (32, 40) for kk in range(2)]
                for k, t in enumerate(_lcombos(*quads)):
                    oe_v[k, pl.ds(pl.multiple_of(j * 8, 8), 8), g * 256:(g + 1) * 256] = t.astype(bf16)

        acc = [None] * NT

        def wo(h0, h1, j0, j1):
            o = pltpu.bitcast(o_v[:, h0 * 128:h1 * 128], bf16)
            for n in range(j0, j1):
                y = _dot(o, pltpu.bitcast(wo_v[n, h0 * 64:h1 * 64, :], bf16))
                acc[n] = y if acc[n] is None else y + acc[n]

        for t in range(NG):
            proj(t)
            if t >= 2:
                pv(t - 2)
            if t >= 1:
                score(t - 1)
        wo(0, 16, 0, 4)
        pv(NG - 2)
        score(NG - 1)
        wo(0, 16, 4, 8)
        pv(NG - 1)
        wo(16, 24, 0, 8)
        wo(24, 32, 0, 8)
        return jnp.concatenate(acc, axis=1)

    def emit(j, r0, o0, a):
        rs = pl.ds(r0 + o0, 24)
        g = jnp.concatenate([g_v[rs, :]] * NT, axis=1)
        out_v[j, o0:o0 + 24, :] = (g * a + b_v[rs, :]).astype(bf16)

    def pair(j, mem, late):
        r0 = pl.multiple_of(j * 64, 64)
        allow_e, fill_e, allow_o, fill_o = _masks()
        xa = x_v[pl.ds(r0 + 16, 8), :].astype(f32)
        xb = x_v[pl.ds(r0 + 40, 8), :].astype(f32)
        hx = jnp.concatenate([x_v[pl.ds(r0, 16), :], jnp.concatenate([xa, mem], 0).astype(bf16)], 0)
        oe = step(j, hx, False, late, allow_e, fill_e)
        emit(j, r0, 0, oe[:24])
        hx = jnp.concatenate([jnp.concatenate([oe[24:32], xb], 0).astype(bf16), x_v[pl.ds(r0 + 48, 16), :]], 0)
        oo = step(j, hx, True, True, allow_o, fill_o)
        emit(j, r0, 40, oo[8:])
        return oo[:8]

    def a_iter(it, carry):
        mem = mem_v[...]
        for t in range(PPI):
            mem = pair(it * PPI + t, mem, t > 0)
        mem_v[...] = mem
        for t in range(PPI):
            for o0 in (0, 40):
                idx = (it * PPI + t, pl.ds(o0, 24))
                pltpu.make_async_copy(out_v.at[idx], out_hbm.at[idx], sem_out).start()
        return carry

    lax.fori_loop(0, NPAIR // PPI, a_iter, 0)

    hist.clear()
    for n in range(NT // 2):
        quad = [lambda k, t=2 * n + q % 2, o=(q // 2) * 128: jnp.concatenate(
            [wo_v[t + zero_s[k], g * 256 + o:g * 256 + o + 128, :] for g in range(NG)], axis=0) for q in range(4)]
        cs = strassen(lambda k: oe_v[k], lambda k: _rcombo(k, *quad), None)
        cols = slice(n * 256, (n + 1) * 256)
        for half in range(2):
            t = jnp.concatenate(cs[2 * half:2 * half + 2], axis=1)
            o0 = 24 + half * 8
            for jj in range(NPAIR):
                rs = slice(jj * 64 + o0, jj * 64 + o0 + 8)
                g = jnp.concatenate([g_v[rs, :]] * 2, axis=1)
                out_v[jj, o0:o0 + 8, cols] = (g * t[jj * 8:jj * 8 + 8] + b_v[rs, cols]).astype(bf16)
        if n >= 2:
            idx = (slice(None), pl.ds(24, 16), pl.ds(0, 768) if n == 2 else pl.ds(768, 256))
            pltpu.make_async_copy(out_v.at[idx], out_hbm.at[idx], sem_out).start()
    pltpu.make_async_copy(out_v, out_hbm, sem_out).wait()


@functools.partial(jax.jit, static_argnames=("A_seg_len",))
def pallas_gated_mix__memory_aug_recurrent_mem_tr__mixer_s_mlp__prompt_kernel(
    A_x, A_mem0, A_Wq, A_Wk, A_Wv, A_Wo, A_seg_len, B_x, B_w1, B_w2, B_w3, B_w4, gate_w,
):
    assert A_seg_len == SEG
    assert A_x.shape == (1, S, D) and A_mem0.shape == (1, M, D)
    any_spec = pl.BlockSpec(memory_space=pl.ANY)
    out = pl.pallas_call(
        _kernel,
        out_shape=jax.ShapeDtypeStruct((NPAIR, 64, D), bf16),
        in_specs=[any_spec] * 11,
        out_specs=any_spec,
        scratch_shapes=[
            pltpu.VMEM((S, D), bf16),
            pltpu.VMEM((9, D // 4, D // 2), u32),
            pltpu.VMEM((7, D // 4, D // 2), u32),
            pltpu.VMEM((RK, D4, F4), bf16),
            pltpu.VMEM((RK, F4, D4), bf16),
            pltpu.VMEM((3 * H, D // 2, DH), u32),
            pltpu.VMEM((NT, H * DH // 2, 128), u32),
            pltpu.VMEM((NT, S + 2 * PAD, 128), f32),
            pltpu.VMEM((S, D), f32),
            pltpu.VMEM((2, 7, HM // 2, D // 2), u32),
            pltpu.VMEM((len(UL), HM, D4), bf16),
            pltpu.VMEM((2, TM, 128), f32),
            pltpu.VMEM((S, 128), f32),
            pltpu.VMEM((NPAIR, 64, D), bf16),
            pltpu.VMEM((len(UL), 8 * NPAIR, D4), bf16),
            pltpu.VMEM((3 * H, 8 * NPAIR, DH), u32),
            pltpu.VMEM((7, 8 * NPAIR, H * DH // 2), bf16),
            pltpu.VMEM((H, 16, 128), u32),
            pltpu.VMEM((H, 16, 128), u32),
            pltpu.VMEM((16, H * DH), u32),
            pltpu.VMEM((M, D), f32),
            pltpu.VMEM((M, D), bf16),
            pltpu.VMEM((NT, 128), bf16),
            pltpu.SMEM((RK,), jnp.int32),
            pltpu.SemaphoreType.DMA((NLOAD,)),
            pltpu.SemaphoreType.DMA((NG,)),
            pltpu.SemaphoreType.DMA,
        ],
        compiler_params=pltpu.CompilerParams(vmem_limit_bytes=126 * 1024 * 1024,
                                             disable_bounds_checks=True),
    )(
        A_x.reshape(S, D), A_mem0.reshape(M, D),
        A_Wq.reshape(D // 2, 2 * H, DH), A_Wk.reshape(D // 2, 2 * H, DH), A_Wv.reshape(D // 2, 2 * H, DH),
        A_Wo.reshape(H * DH, D), B_w1, B_w2, B_w3, B_w4, gate_w.reshape(NT, 128),
    )
    return out.reshape(1, S, D)
```

```python
import functools

import jax
import jax.numpy as jnp
from jax import lax
import jax.experimental.pallas as pl
import jax.experimental.pallas.tpu as pltpu

f32, bf16, u32 = jnp.float32, jnp.bfloat16, jnp.uint32

S, D, H, DH, M, SEG, F = 2048, 1024, 32, 128, 8, 32, 3584
SCALE = DH ** -0.5
NEG = -1000000000.0
EPS = 1e-05

TM = 256
NB = S // TM
HM = TM // 2
DH2 = D // 2
D4, F4 = D // 4, F // 4
FCH = ((0, 128), (128, 384), (384, 640), (640, 896))
NC1 = 128
NPAIR = S // (2 * SEG)
PPI = 2
NPRE = 4
G = 4
NG = H // G
PAD = 8
NT = D // 128
NLOAD = 12
assert NB == NG

_dot = functools.partial(jnp.dot, preferred_element_type=f32)

UP = ((4, 1, 5, 1), (6, 1, 8, 1), (0, 1, 3, 1), (2, -1, 9, 1), (4, -1, 10, 1), (0, 1, 1, 1), (2, 1, 12, 1),
      (5, 1, 7, -1), (7, 1, 12, -1), (11, -1, 13, 1), (10, -1, 11, 1), (2, 1, 7, 1), (0, -1, 4, 1),
      (6, 1, 7, 1), (1, -1, 5, 1), (3, 1, 7, -1), (1, 1, 4, 1), (2, 1, 3, 1), (1, -1, 3, 1), (1, 1, 7, -1),
      (2, 1, 6, -1))
WP = ((0, -1, 3, 1), (4, 1, 6, -1), (1, 1, 8, 1), (5, 1, 10, 1), (4, -1, 7, 1), (0, -1, 9, -1),
      (11, 1, 12, 1), (6, 1, 7, -1), (2, 1, 5, -1), (0, -1, 7, -1), (9, 1, 11, -1), (2, 1, 13, 1),
      (5, 1, 13, 1), (2, -1, 3, 1), (5, 1, 6, 1), (0, 1, 4, 1), (2, 1, 7, 1), (1, 1, 2, 1), (1, 1, 5, 1),
      (3, 1, 7, 1), (2, 1, 6, 1))
VP = ((1, 1, 5, -1), (8, 1, 11, 1), (10, 1, 17, 1), (13, 1, 16, -1), (0, 1, 4, -1), (0, 1, 3, 1),
      (14, 1, 18, -1), (0, 1, 11, 1), (14, 1, 19, -1), (0, 1, 5, 1), (12, 1, 15, 1), (2, 1, 21, 1),
      (10, 1, 14, -1), (4, 1, 7, 1), (11, 1, 19, 1), (12, -1, 20, 1), (13, 1, 14, -1), (9, 1, 30, -1),
      (3, -1, 15, 1), (6, 1, 23, 1), (24, 1, 27, -1), (9, -1, 18, 1), (7, 1, 34, 1), (2, 1, 6, -1),
      (0, 1, 8, -1), (6, 1, 21, 1), (22, 1, 31, -1), (6, 1, 29, 1), (0, 1, 1, 1), (15, 1, 25, 1),
      (5, 1, 37, 1), (15, 1, 20, 1))
UN = (7, 27, 24, 17, 9, 22, 21, 2, 15, 11, 8, 25, 19, 28, 2, 23, 26, 20, 1, 18, 10, 28, 4, 13, 14, 16)
WN = (23, 17, 24, 10, 14, 7, 22, 19, 12, 18, 15, 25, 20, 5, 26, 0, 8, 2, 27, 11, 26, 9, 28, 21, 16, 5)
VN = (42, 47, 41, 5, 11, 43, 18, 28, 20, 23, 35, 19, 22, 46, 33, 26, 45, 36, 38, 25, 44, 40, 39, 21, 24, 32)
RK = len(UN)
UL = tuple(sorted(set(UN)))
VSTAGES = ((0, 6, 7, 12, 13, 14, 15, 21), (11, 17, 20, 22, 24, 25, 23, 2), (1, 5, 8, 9, 10, 16, 18, 19))
RAW16 = (1, 11, 17, 5, 8, 3, 9, 10, 0, 6, 7, 4, 12, 20, 22, 16)


def _run(prog, blocks):
    vals = list(blocks)
    for a, sa, b, sb in prog:
        vals.append(vals[a] + vals[b] if sa > 0 and sb > 0 else
                    vals[a] - vals[b] if sa > 0 else vals[b] - vals[a])
    return vals


def _terms(prog, nin, node):
    if node < nin:
        return {node: 1}
    a, sa, b, sb = prog[node - nin]
    out = {k: sa * v for k, v in _terms(prog, nin, a).items()}
    out.update({k: sb * v for k, v in _terms(prog, nin, b).items()})
    return out


for _b in range(16):
    _last = max(k for k, st in enumerate(VSTAGES) for r in st if _b in _terms(VP, 16, VN[r]))
    assert VN[RAW16[_b]] == _b or RAW16[_b] in VSTAGES[_last]
assert sorted(sum(VSTAGES, ())) == [r for r in range(RK) if VN[r] >= 16] and len(set(RAW16)) == 16

_WPAR = {n: [] for n in range(8 + len(WP))}
for _t, (_a, _sa, _b, _sb) in enumerate(WP):
    _WPAR[_a].append((8 + _t, _sa))
    _WPAR[_b].append((8 + _t, _sb))


def _worder():
    order = []

    def closure(n, acc):
        if n not in acc and n not in order:
            acc.add(n)
            for q, _ in _WPAR[n]:
                closure(q, acc)
        return acc

    def visit(n):
        if n not in order:
            for q, _ in _WPAR[n]:
                visit(q)
            order.append(n)
    while len([v for v in range(8) if v not in order]):
        visit(min((v for v in range(8) if v not in order), key=lambda v: len(closure(v, set()))))
    return tuple(order)


WORDER = _worder()


def _ln(x):
    m = jnp.mean(x, axis=-1, keepdims=True)
    xc = x - m
    v = jnp.mean(xc * xc, axis=-1, keepdims=True)
    return xc * lax.rsqrt(v + EPS)


_GC = 0.7978845608028654


def _gelu(x):
    h = 0.5 * x
    return h + h * jnp.tanh(x * (_GC + (_GC * 0.044715) * (x * x)))


def _unpack(u):
    return pltpu.bitcast(u, bf16).astype(f32)


def _pack(x):
    return pltpu.bitcast(x.astype(bf16), u32)


def _lcombos(a11, a12, a21, a22):
    return [a11 + a22, a21 + a22, a11, a22, a11 + a12, a21 - a11, a12 - a22]


def _merge(*lists):
    keyed = [((j + 0.5) / len(l), n, j, v) for n, l in enumerate(lists) for j, v in enumerate(l)]
    return [v for _, _, _, v in sorted(keyed, key=lambda t: t[:3])]


def _masks():
    r = lax.broadcasted_iota(jnp.int32, (32, 48), 0)
    c = lax.broadcasted_iota(jnp.int32, (32, 48), 1)
    exist_e = c < 40
    allow_e = exist_e & ((r >= 24) | ((c >= 24) & (c < 32)) | (c <= r))
    fill_e = jnp.where(exist_e, NEG, -jnp.inf).astype(f32)
    r = lax.broadcasted_iota(jnp.int32, (48, 80), 0)
    c = lax.broadcasted_iota(jnp.int32, (48, 80), 1)
    q_even = (r >= 32) & (r < 40)
    exist_o = (q_even & (c < 40)) | (~q_even & (c >= 40))
    ktok = jnp.where(c < 24, c, jnp.where(c < 48, c - 8, c - 16))
    qtok = jnp.where(r < 32, r + 32, r - 8)
    is_mem_key = ((c >= 24) & (c < 32)) | ((c >= 48) & (c < 56))
    allow_o = exist_o & (is_mem_key | (r < 8) | (ktok <= qtok))
    fill_o = jnp.where(exist_o, NEG, -jnp.inf).astype(f32)
    return allow_e, fill_e, allow_o, fill_o


def _rcombo(k, b11, b12, b21, b22):
    if k in (1, 4):
        return (b11 if k == 1 else b22)(k)
    a, b, sign = {0: (b11, b22, 1), 2: (b12, b22, -1), 3: (b21, b11, -1), 5: (b11, b12, 1), 6: (b21, b22, 1)}[k]
    a, b = _unpack(a(k)), _unpack(b(k))
    return (a + b if sign > 0 else a - b).astype(bf16)


def _softmax(s, allow, fill):
    s = jnp.where(allow, s * SCALE, fill)
    m = jnp.max(s, axis=-1, keepdims=True)
    e = jnp.exp(s - m)
    l = jnp.sum(e, axis=-1, keepdims=True)
    r = pl.reciprocal(l, approx=True)
    r = r * (2.0 - l * r)
    return (e * r).astype(bf16)


def _kernel(x_hbm, mem0_hbm, wq_hbm, wk_hbm, wv_hbm, wo_hbm, w1_hbm, w2_hbm, w3_hbm, w4_hbm,
            gw_hbm, out_hbm,
            x_v, s1_v, s2_v, s3_v, s4_v, wqkv_v, wo_v, h_v, b_v, l_v, lf_v, n_v, g_v, out_v, xe_v, e_v, oe_v,
            ke_v, ve_v, o_v, mem_v, mem0_ref, gw_ref, zero_s,
            sem, sem_qkv, sem_out):
    RAW = (1, 2, 3, 4)
    RAW1 = (1, 7, 8, 4)

    loads = []

    def rows_load(name, r0, r1):
        loads.append((name, x_hbm.at[pl.ds(r0, r1 - r0)], x_v.at[pl.ds(r0, r1 - r0)]))

    def quad_load(name, w_hbm, s_v, raw, q, c0=0, c1=None):
        k4, n2 = s_v.shape[1], s_v.shape[2]
        c1 = n2 if c1 is None else c1
        src = w_hbm.bitcast(u32).at[pl.ds((q // 2) * k4, k4), pl.ds((q % 2) * n2 + c0, c1 - c0)]
        loads.append((name, src, s_v.at[raw[q], :, pl.ds(c0, c1 - c0)]))

    rows_load("x0", 0, TM)
    rows_load("x1", TM, 2 * TM)
    for name, half, c0, c1 in (("w1a", 0, 0, 256), ("w1bc", 0, 256, 512), ("w1bc", 1, 0, 256), ("w1d", 1, 256, 512)):
        quad_load(name, w1_hbm, s1_v, RAW1, half, c0, c1)
        quad_load(name, w1_hbm, s1_v, RAW1, 2 + half, c0, c1)
    rows_load("x234", 2 * TM, 5 * TM)
    rows_load("x567", 5 * TM, S)
    for q in range(4):
        quad_load("w2", w2_hbm, s2_v, RAW, q)
    for name, w_hbm, s_v in (("w3", w3_hbm, s3_v), ("w4", w4_hbm, s4_v)):
        kb, nb = s_v.shape[1:]
        for q in range(16):
            loads.append((name, w_hbm.at[pl.ds((q // 4) * kb, kb), pl.ds((q % 4) * nb, nb)], s_v.at[RAW16[q]]))
    loads.append(("small", mem0_hbm, mem0_ref))
    loads.append(("small", gw_hbm, gw_ref))
    for j in range(NT):
        loads.append(("wo", wo_hbm.bitcast(u32).at[:, pl.ds(j * 128, 128)], wo_v.at[j]))
    groups = list(dict.fromkeys(name for name, _, _ in loads))
    assert len(groups) == NLOAD

    def start(*names, priority=0):
        for name, src, dst in loads:
            if name in names:
                pltpu.make_async_copy(src, dst, sem.at[groups.index(name)]).start(priority=priority)

    def wait(*names):
        for name, src, dst in loads:
            if name in names:
                pltpu.make_async_copy(src, dst, sem.at[groups.index(name)]).wait()

    SPG = 3 * G

    def qkv_start(g):
        for w, w_hbm in enumerate((wq_hbm, wk_hbm, wv_hbm)):
            wu = w_hbm.bitcast(u32)
            for k in range(G // 2):
                for par in range(2):
                    pltpu.make_async_copy(
                        wu.at[:, par * (H // 2) + g * (G // 2) + k, :],
                        wqkv_v.at[g * SPG + w * G + 2 * k + par], sem_qkv.at[g]).start(priority=1)

    def qkv_wait(g):
        grp = wqkv_v.at[pl.ds(g * SPG, SPG)]
        pltpu.make_async_copy(grp, grp, sem_qkv.at[g]).wait()

    start("x0", "x1", "w1a", "w1bc", "w1d", "x234", "x567", "w2", "w3", "w4", "small")
    for k in range(RK):
        zero_s[k] = 0

    def tile_idx(ref, cols=128):
        z = zero_s[0]
        n = 16 if ref.dtype == bf16 and cols == 128 else 8
        return (z,) * (len(ref.shape) - 2) + (pl.ds(pl.multiple_of(z, n), n), slice(0, cols))

    hist = []

    def mm(lhs, rhs, side=None, acc=None):
        if side is not None:
            lhs = side(lhs)
        lhs = pltpu.bitcast(lhs, bf16) if lhs.dtype == u32 else lhs.astype(bf16)
        y = _dot(lhs, pltpu.bitcast(rhs, bf16) if rhs.dtype == u32 else rhs)
        if acc is not None:
            y = y + acc
        hist.append(y)
        return y

    class Side:
        def __init__(self, pieces, n, skip=0):
            self.pieces, self.n, self.skip = list(pieces), n, skip

        def __call__(self, val):
            if self.skip:
                self.skip -= 1
                return val
            take = -(-len(self.pieces) // self.n) if self.pieces else 0
            self.n -= 1
            if not take:
                return val
            never = zero_s[0] > 0
            if val.dtype == bf16:
                val = pltpu.bitcast(val, u32)
            rg = 8 if val.dtype == u32 else 16
            ng = val.shape[0] // rg
            groups = [val[8 * m:8 * m + 8] for m in range(val.shape[0] // 8)]
            for j, (fn, rd, wr, lag) in enumerate(self.pieces[:take]):
                m = (j + 1) * ng // take - 1
                pin = lambda v: v
                if lag is not None and len(hist) >= lag:
                    r0 = (16 * m) % hist[-lag].shape[0]
                    a = hist[-lag][r0:r0 + 8, :128]
                    if rd is None:
                        def pin(v, a=a):
                            t = jnp.where(never, jnp.concatenate([a] * (v.shape[0] // 8), axis=0), v[:, :128])
                            return t if v.shape[1] == 128 else jnp.concatenate([t, v[:, 128:]], axis=1)
                    elif rd.dtype == bf16:
                        idx = tile_idx(rd, 256)
                        rd[idx] = jnp.where(never, jnp.concatenate([a, a], axis=1).astype(bf16), rd[idx])
                    else:
                        idx = tile_idx(rd)
                        rd[idx] = jnp.where(never, pltpu.bitcast(a, rd.dtype), rd[idx])
                tiles = fn(pin)
                g = m * rg // 8
                t = groups[g][:, -128:]
                for u in (tiles if wr is None else [wr[tile_idx(wr)]]):
                    t = jnp.where(never, pltpu.bitcast(u, val.dtype), t)
                groups[g] = t if val.shape[1] == 128 else jnp.concatenate([groups[g][:, :-128], t], axis=1)
            self.pieces = self.pieces[take:]
            return jnp.concatenate(groups, axis=0)

    def strassen(lhs, rhs, side, init=(None, None, None, None), ks=range(7)):
        def add(a, b):
            return a if b is None else a + b
        sd = lambda k: side if k in ks else None
        p = [mm(lhs(k), rhs(k), sd(k)) for k in range(5)]
        c12 = add(p[2] + p[4], init[1])
        c21 = add(p[1] + p[3], init[2])
        c22 = mm(lhs(5), rhs(5), sd(5), add(p[0] - p[1] + p[2], init[3]))
        c11 = mm(lhs(6), rhs(6), sd(6), add(p[0] + p[3] - p[4], init[0]))
        return c11, c12, c21, c22

    def fmm(lhs, rhs, side, extra=lambda n: None):
        val = {}
        for n in WORDER:
            t = extra(n)
            for q, sg in sorted(_WPAR[n], key=lambda e: -e[1]):
                t = val[q] if t is None else (t + val[q] if sg > 0 else t - val[q])
            for r in range(RK):
                if WN[r] == n:
                    t = mm(lhs(UN[r]), rhs(r), side, t)
            val[n] = t
        return [val[v] for v in range(8)]

    def prep26_pieces(s_v, lag, stages=(sum(VSTAGES, ()),)):
        def piece(rs, cs, stage, pin):
            @functools.lru_cache(None)
            def node(n):
                if n < 16:
                    return s_v[RAW16[n], rs, cs].astype(f32)
                return _run([(0, VP[n - 16][1], 1, VP[n - 16][3])], [node(VP[n - 16][0]), node(VP[n - 16][2])])[-1]
            vals = [node(VN[r]).astype(bf16) for r in stage]
            for r, t in zip(stage, vals):
                s_v[r, rs, cs] = t
        kb, nb = s_v.shape[1:]
        out = []
        for r in range(0, kb, 16):
            out += [(slice(rr, rr + 8), slice(c, c + 256)) for c in range(0, nb - 255, 256) for rr in (r, r + 8)]
            out += [(slice(r, r + 16), slice(nb - 128, nb))] if nb % 256 else []
        return [(functools.partial(piece, rs, cs, st), s_v, s_v, lag) for rs, cs in out for st in stages]

    def prep_pieces(s_v, raw, lag, width=256):
        def piece(r, c, pin):
            idx = (slice(r, r + 8), slice(c, c + width))
            b11, b12, b21, b22 = [_unpack(s_v[(q,) + idx]) for q in raw]
            for k, t in ((0, b11 + b22), (2, b12 - b22), (3, b21 - b11), (5, b11 + b12), (6, b21 + b22)):
                s_v[(k,) + idx] = _pack(t)
        return [(functools.partial(piece, r, c), s_v, s_v, lag)
                for r in range(0, s_v.shape[1], 8) for c in range(0, s_v.shape[2], width)]

    def store_l(slot, q, c, quads, plain=False):
        for k, t in enumerate(quads if plain else _lcombos(*quads)):
            l_v[slot, k, q // 2:q // 2 + 8, c:c + t.shape[1]] = _pack(t)

    def ln_pieces(src, r0, slot, lag, plain=False, width=256, staged=False, clag=None, dyn=True):
        def stats(q, pin):
            x = pin(src[pl.ds(r0 + q, 16), :].astype(f32))
            xs = [x[:, j * 128:(j + 1) * 128] for j in range(NT)]
            m = functools.reduce(lambda a, b: a + b, xs) * (1.0 / NT)
            w = functools.reduce(lambda a, b: a + b, [(t - m) * (t - m) for t in xs])
            mean = jnp.mean(m, axis=-1, keepdims=True)
            var = jnp.sum(w + NT * ((m - mean) * (m - mean)), axis=-1, keepdims=True) * (1.0 / D)
            n_v[0, q:q + 16, :] = jnp.broadcast_to(mean, (16, 128))
            n_v[1, q:q + 16, :] = jnp.broadcast_to(lax.rsqrt(var + EPS), (16, 128))

        def comb(q, c, pin):
            quads = []
            for rr in (0, HM):
                rs = pl.ds(pl.multiple_of(r0 + rr + q + zero_s[0], 16), 16)
                mean, rstd = [jnp.concatenate([n_v[t, rr + q:rr + q + 16, :]] * (width // 128), axis=1)
                              for t in range(2)]
                quads += [(src[rs, cc + c:cc + c + width].astype(f32) - mean) * rstd for cc in (0, DH2)]
            store_l(slot, q, c, quads, plain)

        def comb26(q, pin):
            blocks = []
            for rr in (0, HM):
                rs = pl.ds(pl.multiple_of(r0 + rr + q + (zero_s[0] if dyn else 0), 8), 8)
                mean, rstd = [jnp.concatenate([n_v[t, rr + q:rr + q + 8, :]] * 2, axis=1) for t in range(2)]
                blocks += [(src[rs, cc:cc + D4] - mean) * rstd for cc in range(0, D, D4)]
            vals = _run(UP, blocks)
            for k, u in enumerate(UL):
                lf_v[k, q:q + 8, :] = vals[u].astype(bf16)
        norms = [[(functools.partial(stats, rr + q), None, n_v, lag) for rr in (0, HM)] for q in range(0, HM, 16)]
        if slot is None:
            combs = [[(functools.partial(comb26, qq), n_v, lf_v, clag) for qq in (q, q + 8)]
                     for q in range(0, HM, 16)]
        else:
            combs = [[(functools.partial(comb, q, c), n_v, l_v, clag) for c in range(0, DH2, width)]
                     for q in range(0, HM, 16)]
        if staged:
            return sum(norms, []), sum(combs, [])
        out = list(norms[0])
        for a, b in zip(norms[1:] + [[]], combs):
            out += _merge(a, b) if a else b
        return out

    shifts = (1, 1, -1, -1, 2, 2, -2, -2)

    def shift_pieces(r0, slot, lag, by_value=False):
        def piece(q, j, pin):
            a = [h_v[jj, pl.ds(PAD + r0 + rr + q - shifts[jj], 16), :]
                 for rr in (0, HM) for jj in (j, j + NT // 2)]
            store_l(slot, q, j * 128, [pin(a[0]), a[1], a[2], pin(a[3])])
        return [(functools.partial(piece, q, j), None if by_value else h_v, l_v, lag)
                for q in range(0, HM, 16) for j in range(NT // 2)]

    def lhs_of(slot):
        return lambda k: l_v[slot, k]

    h_v[:, 0:PAD, :] = jnp.zeros((NT, PAD, 128), f32)
    h_v[:, PAD + S:PAD + S + PAD, :] = jnp.zeros((NT, PAD, 128), f32)

    def store_h(r0, c0, h):
        for j in range(h.shape[1] // 128):
            h_v[c0 // 128 + j, PAD + r0:PAD + r0 + h.shape[0], :] = h[:, j * 128:(j + 1) * 128]

    def d1_plain(xn, r0, c0, c1, step, side=None):
        for c in range(c0, c1, step):
            half, cc = c // DH2, c % DH2
            w = jnp.concatenate([s1_v[RAW1[half], :, cc:cc + step], s1_v[RAW1[2 + half], :, cc:cc + step]], axis=0)
            store_h(r0, c, _gelu(mm(xn, w, side)))

    NP1 = 7 * (DH2 // NC1)
    KS1 = (2, 3, 4, 5)

    def d1_s(b, slot, pieces):
        side = Side(pieces, len(KS1) * (DH2 // NC1))
        for c in range(0, DH2, NC1):
            cs = strassen(lhs_of(slot), lambda k: s1_v[k, :, c:c + NC1], side, ks=KS1)
            for q, t in enumerate(cs):
                store_h(b * TM + (q // 2) * HM, (q % 2) * DH2 + c, _gelu(t))

    def d2_s(b, slot, pieces):
        side = Side(pieces, NP1)
        for c in range(0, DH2, NC1):
            idx = [(slice(b * TM + (q // 2) * HM, b * TM + (q // 2 + 1) * HM),
                    slice((q % 2) * DH2 + c, (q % 2) * DH2 + c + NC1)) for q in range(4)]
            cs = strassen(lhs_of(slot), lambda k: s2_v[k, :, c:c + NC1], side,
                          [x_v[i].astype(f32) for i in idx])
            for i, t in zip(idx, cs):
                b_v[i] = t

    def split(l, n):
        return [l[len(l) * i // n:len(l) * (i + 1) // n] for i in range(n)]

    LS, LL = 3, 5

    wait("x0")
    xn0 = _pack(_ln(x_v[0:TM, :].astype(f32)))
    wait("x1")
    xn01 = jnp.concatenate([xn0, _pack(_ln(x_v[TM:2 * TM, :].astype(f32)))], axis=0)
    wait("w1a")
    d1_plain(xn01, 0, 0, 256, 256)
    wait("w1bc")
    d1_plain(xn01, 0, 256, 768, 256)
    wait("w1d", "x234")
    hist.clear()
    d1_plain(xn01, 0, 768, D, 128, Side(ln_pieces(x_v, 2 * TM, 0, None, plain=True), 2))
    xn2 = jnp.concatenate([jnp.concatenate([l_v[0, 2 * h], l_v[0, 2 * h + 1]], axis=1) for h in range(2)], axis=0)
    d1_plain(xn2, 2 * TM, 0, D, 128,
             Side(_merge(prep_pieces(s1_v, RAW1, 1), ln_pieces(x_v, 3 * TM, 1, 2)), 8))
    d1_s(3, 1, ln_pieces(x_v, 4 * TM, 0, LL))
    wait("x567", "w2")
    qkv_start(0)
    qkv_start(1)
    hist.clear()
    pw = split(prep_pieces(s2_v, RAW, LS), 4)
    for b in range(4, NB):
        nxt = ln_pieces(x_v, (b + 1) * TM, (b + 1) % 2, LL) if b + 1 < NB else shift_pieces(0, 0, LS, True)
        d1_s(b, b % 2, _merge(pw[b - 4], nxt))
    d2_s(0, 0, shift_pieces(TM, 1, LS, True))
    wait("w3")
    hist.clear()
    pw = split(_merge(prep26_pieces(s3_v, LS), ln_pieces(b_v, 0, None, LL, dyn=False)), 4)
    for b in range(1, 5):
        d2_s(b, b % 2, _merge(pw[b - 1], shift_pieces((b + 1) * TM, (b + 1) % 2, LS)))
    wait("w4", "small")
    hist.clear()
    pw = prep26_pieces(s4_v, LS)
    d2_s(5, 1, _merge(pw[:34], shift_pieces(6 * TM, 0, LS)))
    d2_s(6, 0, _merge(pw[34:68], shift_pieces(7 * TM, 1, LS)))
    d2_s(7, 1, pw[68:])
    start("wo", priority=1)

    def ffn(i, carry):
        qkv_wait(i)
        r0 = pl.multiple_of(i * TM, TM)
        rn = pl.multiple_of(jnp.minimum(i + 1, NB - 1) * TM, TM)
        acc = {}
        hist.clear()

        def relayout(p, r0_, r1_, pin):
            s0 = i * SPG + 2 * p
            for r in range(r0_, r1_, 8):
                e = wqkv_v[s0, r:r + 8, :]
                o = wqkv_v[s0 + 1, r:r + 8, :]
                wqkv_v[s0, r:r + 8, :] = (e & jnp.uint32(0xFFFF)) | (o << 16)
                wqkv_v[s0 + 1, r:r + 8, :] = (e >> 16) | (o & jnp.uint32(0xFFFF0000))

        relays = [(functools.partial(relayout, p, r, r + 32), wqkv_v, wqkv_v, 3)
                  for p in range(SPG // 2) for r in range(0, D // 2, 32)]
        norms, combs = ln_pieces(b_v, rn, None, 5, staged=True, clag=3)

        def gate(q, pin):
            gw = gw_ref[...].astype(f32)
            x = pin(x_v[pl.ds(r0 + q, 16), :].astype(f32))
            t = functools.reduce(lambda a, b: a + b,
                                 [x[:, j * 128:(j + 1) * 128] * gw[j:j + 1, :] for j in range(NT)])
            g = jax.nn.sigmoid(jnp.sum(t, axis=-1, keepdims=True))
            g_v[pl.ds(r0 + q, 16), :] = jnp.broadcast_to(g, (16, 128))

        gates = [(functools.partial(gate, q), None, g_v, 5) for q in range(0, TM, 16)]

        def extras(t, pin):
            jj, o = 2 * i + t // 2, 24 + 8 * (t % 2)
            xs = [pin(x_v[pl.ds(pl.multiple_of((jj + hh) * 64 + o, 8), 8), :].astype(f32)) for hh in (0, NPAIR // 2)]
            vals = _run(UP, [x[:, cc:cc + D4] for x in xs for cc in range(0, D, D4)])
            for k, u in enumerate(UL):
                xe_v[k, pl.ds(pl.multiple_of(i * 32 + t * 8, 8), 8), :] = vals[u].astype(bf16)

        xes = [(functools.partial(extras, t), None, xe_v, 3) for t in range(4)]
        hs = {}

        def gelu_pieces(c, cs):
            def piece(r, cc, vs, pin):
                for v in vs:
                    hs[c, v, r, cc] = _gelu(pin(cs[v][r:r + 8, cc:cc + 128]))
                return [hs[c, v, r, cc] for v in vs]
            return [(functools.partial(piece, r, cc, vs), None, None, 3) for r in range(0, HM, 8)
                    for cc in range(0, cs[0].shape[1], 128) for vs in ((0, 1, 2, 3), (4, 5, 6, 7))]

        def d3(c, side):
            c0, c1 = FCH[c]
            cs = fmm(lambda u: lf_v[UL.index(u)], lambda r: s3_v[r, :, c0:c1], side)
            assert not side.pieces
            return gelu_pieces(c, cs)

        def d4(c, side):
            c0, c1 = FCH[c]
            lh = _run(UP, [jnp.concatenate([jnp.concatenate(
                [hs.pop((c, v, r, cc)) for cc in range(0, c1 - c0, 128)], axis=1) for r in range(0, HM, 8)], axis=0)
                for v in range(8)])
            rhs = lambda r: s4_v[r, c0:c1, :]
            if c + 1 < len(FCH):
                for n in WORDER:
                    for r in range(RK):
                        if WN[r] == n:
                            acc[n] = mm(lh[UN[r]], rhs(r), side, acc.get(n))
            else:
                idx = lambda v: (pl.ds(r0 + (v // 4) * HM, HM), slice((v % 4) * D4, (v % 4 + 1) * D4))

                def extra(n):
                    if n >= 8:
                        return acc.get(n)
                    return b_v[idx(n)] + acc[n] if n in acc else b_v[idx(n)]
                for v, t in enumerate(fmm(lambda u: lh[u], rhs, side, extra)):
                    b_v[idx(v)] = jnp.concatenate([1.0 - g_v[idx(v)[0], :]] * 2, axis=1) * t
            assert not side.pieces

        g0 = d3(0, Side(relays[:20], 23, 3))
        g1 = d3(1, Side(_merge(g0, gates), 23, 2))
        d4(0, Side(g1[:22], 22, 4))
        g2 = d3(2, Side(_merge(g1[22:], relays[20:40]), 25))
        d4(1, Side(g2, 23, 2))
        g3 = d3(3, Side(_merge(relays[40:], norms, xes), 26))
        d4(2, Side(_merge(g3, combs), 23, 2))
        d4(3, Side([], 1))

        @pl.when(i + 2 < NG)
        def _():
            qkv_start(i + 2)

        return carry

    lax.fori_loop(0, NB, ffn, 0)

    def pre(it, carry):
        hist.clear()
        for u in range(3 * NG // NPRE):
            s0 = (it * (3 * NG // NPRE) + u) * G

            def rhs(r):
                t = None
                for q, sg in sorted(_terms(VP, 16, VN[r]).items(), key=lambda e: -e[1]):
                    blk = wqkv_v[s0 + q % 4 + zero_s[r], (q // 4) * (D // 8):(q // 4 + 1) * (D // 8), :]
                    if VN[r] < 16:
                        return blk
                    blk = _unpack(blk)
                    t = blk if t is None else (t + blk if sg > 0 else t - blk)
                return t.astype(bf16)
            for v, t in enumerate(fmm(lambda k: xe_v[UL.index(k)], rhs, None)):
                e_v[s0 + v % 4, (v // 4) * 128:(v // 4 + 1) * 128, :] = _pack(t)
        return carry

    lax.fori_loop(0, NPRE, pre, 0)

    wait("wo")
    mem_v[...] = mem0_ref[...].astype(f32)

    def slab(w, h):
        return (h // G) * SPG + w * G + h % G

    def step(j, hx, odd, late, allow, fill):
        qs, ks, vs, ps = {}, {}, {}, {}
        wload = lambda w, h: pltpu.bitcast(wqkv_v[slab(w, h)], bf16)
        eload = lambda w, h: pltpu.bitcast(e_v[slab(w, h), pl.ds(pl.multiple_of(j * 8, 8), 8), :], bf16)

        def proj(g):
            part = {}
            if late and g == 0:
                for h in range(2):
                    for w in range(3):
                        part[w, h] = _dot(hx[:, :DH2], wload(w, h)[:DH2])
            for h in range(g * G, (g + 1) * G):
                q, k, v = [(_dot(hx[:, DH2:], wload(w, h)[DH2:]) + part[w, h] if (w, h) in part
                            else _dot(hx, wload(w, h))).astype(bf16) for w in range(3)]
                if odd:
                    q = jnp.concatenate([q, eload(0, h)], axis=0)
                    k = jnp.concatenate([pltpu.bitcast(ke_v[h], bf16), eload(1, h), k], axis=0)
                    v = jnp.concatenate([pltpu.bitcast(ve_v[h], bf16), eload(2, h), v], axis=0)
                else:
                    ke_v[h] = pltpu.bitcast(k, u32)
                    ve_v[h] = pltpu.bitcast(v, u32)
                    k = jnp.concatenate([k, eload(1, h)], axis=0)
                    v = jnp.concatenate([v, eload(2, h)], axis=0)
                qs[h], ks[h], vs[h] = q, k, v

        def score(g):
            for h in range(g * G, (g + 1) * G):
                s = lax.dot_general(qs.pop(h), ks.pop(h), (((1,), (1,)), ((), ())),
                                    preferred_element_type=f32)
                ps[h] = _softmax(s, allow, fill)

        def pv(g):
            os_ = []
            for h in range(g * G, (g + 1) * G):
                o = _dot(ps.pop(h), vs.pop(h))
                o_v[:, h * 128:(h + 1) * 128] = _pack(o[:32])
                os_.append(o)
            if odd:
                quads = [jnp.concatenate([os_[2 * kk][r:r + 8], os_[2 * kk + 1][r:r + 8]], axis=1)
                         for r in (32, 40) for kk in range(2)]
                for k, t in enumerate(_lcombos(*quads)):
                    oe_v[k, pl.ds(pl.multiple_of(j * 8, 8), 8), g * 256:(g + 1) * 256] = t.astype(bf16)

        acc = [None] * NT

        def wo(h0, h1, j0, j1):
            o = pltpu.bitcast(o_v[:, h0 * 128:h1 * 128], bf16)
            for n in range(j0, j1):
                y = _dot(o, pltpu.bitcast(wo_v[n, h0 * 64:h1 * 64, :], bf16))
                acc[n] = y if acc[n] is None else y + acc[n]

        for t in range(NG):
            proj(t)
            if t >= 2:
                pv(t - 2)
            if t >= 1:
                score(t - 1)
        wo(0, 16, 0, 4)
        pv(NG - 2)
        score(NG - 1)
        wo(0, 16, 4, 8)
        pv(NG - 1)
        wo(16, 24, 0, 8)
        wo(24, 32, 0, 8)
        return jnp.concatenate(acc, axis=1)

    def emit(j, r0, o0, a):
        rs = pl.ds(r0 + o0, 24)
        g = jnp.concatenate([g_v[rs, :]] * NT, axis=1)
        out_v[j, o0:o0 + 24, :] = (g * a + b_v[rs, :]).astype(bf16)

    def pair(j, mem, late):
        r0 = pl.multiple_of(j * 64, 64)
        allow_e, fill_e, allow_o, fill_o = _masks()
        xa = x_v[pl.ds(r0 + 16, 8), :].astype(f32)
        xb = x_v[pl.ds(r0 + 40, 8), :].astype(f32)
        hx = jnp.concatenate([x_v[pl.ds(r0, 16), :], jnp.concatenate([xa, mem], 0).astype(bf16)], 0)
        oe = step(j, hx, False, late, allow_e, fill_e)
        emit(j, r0, 0, oe[:24])
        hx = jnp.concatenate([jnp.concatenate([oe[24:32], xb], 0).astype(bf16), x_v[pl.ds(r0 + 48, 16), :]], 0)
        oo = step(j, hx, True, True, allow_o, fill_o)
        emit(j, r0, 40, oo[8:])
        return oo[:8]

    def a_iter(it, carry):
        mem = mem_v[...]
        for t in range(PPI):
            mem = pair(it * PPI + t, mem, t > 0)
        mem_v[...] = mem
        for t in range(PPI):
            for o0 in (0, 40):
                idx = (it * PPI + t, pl.ds(o0, 24))
                pltpu.make_async_copy(out_v.at[idx], out_hbm.at[idx], sem_out).start()
        return carry

    lax.fori_loop(0, NPAIR // PPI, a_iter, 0)

    hist.clear()
    for n in range(NT // 2):
        quad = [lambda k, t=2 * n + q % 2, o=(q // 2) * 128: jnp.concatenate(
            [wo_v[t + zero_s[k], g * 256 + o:g * 256 + o + 128, :] for g in range(NG)], axis=0) for q in range(4)]
        cs = strassen(lambda k: oe_v[k], lambda k: _rcombo(k, *quad), None)
        cols = slice(n * 256, (n + 1) * 256)
        for half in range(2):
            t = jnp.concatenate(cs[2 * half:2 * half + 2], axis=1)
            o0 = 24 + half * 8
            for jj in range(NPAIR):
                rs = slice(jj * 64 + o0, jj * 64 + o0 + 8)
                g = jnp.concatenate([g_v[rs, :]] * 2, axis=1)
                out_v[jj, o0:o0 + 8, cols] = (g * t[jj * 8:jj * 8 + 8] + b_v[rs, cols]).astype(bf16)
        if n >= 2:
            idx = (slice(None), pl.ds(24, 16), pl.ds(0, 768) if n == 2 else pl.ds(768, 256))
            pltpu.make_async_copy(out_v.at[idx], out_hbm.at[idx], sem_out).start()
    pltpu.make_async_copy(out_v, out_hbm, sem_out).wait()


@functools.partial(jax.jit, static_argnames=("A_seg_len",))
def pallas_gated_mix__memory_aug_recurrent_mem_tr__mixer_s_mlp__prompt_kernel(
    A_x, A_mem0, A_Wq, A_Wk, A_Wv, A_Wo, A_seg_len, B_x, B_w1, B_w2, B_w3, B_w4, gate_w,
):
    assert A_seg_len == SEG
    assert A_x.shape == (1, S, D) and A_mem0.shape == (1, M, D)
    any_spec = pl.BlockSpec(memory_space=pl.ANY)
    out = pl.pallas_call(
        _kernel,
        out_shape=jax.ShapeDtypeStruct((NPAIR, 64, D), bf16),
        in_specs=[any_spec] * 11,
        out_specs=any_spec,
        scratch_shapes=[
            pltpu.VMEM((S, D), bf16),
            pltpu.VMEM((9, D // 4, D // 2), u32),
            pltpu.VMEM((7, D // 4, D // 2), u32),
            pltpu.VMEM((RK, D4, F4), bf16),
            pltpu.VMEM((RK, F4, D4), bf16),
            pltpu.VMEM((3 * H, D // 2, DH), u32),
            pltpu.VMEM((NT, H * DH // 2, 128), u32),
            pltpu.VMEM((NT, S + 2 * PAD, 128), f32),
            pltpu.VMEM((S, D), f32),
            pltpu.VMEM((2, 7, HM // 2, D // 2), u32),
            pltpu.VMEM((len(UL), HM, D4), bf16),
            pltpu.VMEM((2, TM, 128), f32),
            pltpu.VMEM((S, 128), f32),
            pltpu.VMEM((NPAIR, 64, D), bf16),
            pltpu.VMEM((len(UL), 8 * NPAIR, D4), bf16),
            pltpu.VMEM((3 * H, 8 * NPAIR, DH), u32),
            pltpu.VMEM((7, 8 * NPAIR, H * DH // 2), bf16),
            pltpu.VMEM((H, 16, 128), u32),
            pltpu.VMEM((H, 16, 128), u32),
            pltpu.VMEM((16, H * DH), u32),
            pltpu.VMEM((M, D), f32),
            pltpu.VMEM((M, D), bf16),
            pltpu.VMEM((NT, 128), bf16),
            pltpu.SMEM((RK,), jnp.int32),
            pltpu.SemaphoreType.DMA((NLOAD,)),
            pltpu.SemaphoreType.DMA((NG,)),
            pltpu.SemaphoreType.DMA,
        ],
        compiler_params=pltpu.CompilerParams(vmem_limit_bytes=126 * 1024 * 1024,
                                             disable_bounds_checks=True),
    )(
        A_x.reshape(S, D), A_mem0.reshape(M, D),
        A_Wq.reshape(D // 2, 2 * H, DH), A_Wk.reshape(D // 2, 2 * H, DH), A_Wv.reshape(D // 2, 2 * H, DH),
        A_Wo.reshape(H * DH, D), B_w1, B_w2, B_w3, B_w4, gate_w.reshape(NT, 128),
    )
    return out.reshape(1, S, D)
```

```python
import functools

import jax
import jax.numpy as jnp
from jax import lax
import jax.experimental.pallas as pl
import jax.experimental.pallas.tpu as pltpu

f32, bf16, u32 = jnp.float32, jnp.bfloat16, jnp.uint32

S, D, H, DH, M, SEG, F = 2048, 1024, 32, 128, 8, 32, 3584
SCALE = DH ** -0.5
NEG = -1000000000.0
EPS = 1e-05

TM = 256
NB = S // TM
HM = TM // 2
DH2 = D // 2
D4, F4 = D // 4, F // 4
FCH = ((0, 128), (128, 384), (384, 640), (640, 896))
NC1 = 128
NPAIR = S // (2 * SEG)
PPI = 2
NPRE = 4
G = 4
NG = H // G
PAD = 8
NT = D // 128
NLOAD = 12
assert NB == NG

_dot = functools.partial(jnp.dot, preferred_element_type=f32)

UP = ((4, 1, 5, 1), (6, 1, 8, 1), (0, 1, 3, 1), (2, -1, 9, 1), (4, -1, 10, 1), (0, 1, 1, 1), (2, 1, 12, 1),
      (5, 1, 7, -1), (7, 1, 12, -1), (11, -1, 13, 1), (10, -1, 11, 1), (2, 1, 7, 1), (0, -1, 4, 1),
      (6, 1, 7, 1), (1, -1, 5, 1), (3, 1, 7, -1), (1, 1, 4, 1), (2, 1, 3, 1), (1, -1, 3, 1), (1, 1, 7, -1),
      (2, 1, 6, -1))
WP = ((0, -1, 3, 1), (4, 1, 6, -1), (1, 1, 8, 1), (5, 1, 10, 1), (4, -1, 7, 1), (0, -1, 9, -1),
      (11, 1, 12, 1), (6, 1, 7, -1), (2, 1, 5, -1), (0, -1, 7, -1), (9, 1, 11, -1), (2, 1, 13, 1),
      (5, 1, 13, 1), (2, -1, 3, 1), (5, 1, 6, 1), (0, 1, 4, 1), (2, 1, 7, 1), (1, 1, 2, 1), (1, 1, 5, 1),
      (3, 1, 7, 1), (2, 1, 6, 1))
VP = ((1, 1, 5, -1), (8, 1, 11, 1), (10, 1, 17, 1), (13, 1, 16, -1), (0, 1, 4, -1), (0, 1, 3, 1),
      (14, 1, 18, -1), (0, 1, 11, 1), (14, 1, 19, -1), (0, 1, 5, 1), (12, 1, 15, 1), (2, 1, 21, 1),
      (10, 1, 14, -1), (4, 1, 7, 1), (11, 1, 19, 1), (12, -1, 20, 1), (13, 1, 14, -1), (9, 1, 30, -1),
      (3, -1, 15, 1), (6, 1, 23, 1), (24, 1, 27, -1), (9, -1, 18, 1), (7, 1, 34, 1), (2, 1, 6, -1),
      (0, 1, 8, -1), (6, 1, 21, 1), (22, 1, 31, -1), (6, 1, 29, 1), (0, 1, 1, 1), (15, 1, 25, 1),
      (5, 1, 37, 1), (15, 1, 20, 1))
UN = (7, 27, 24, 17, 9, 22, 21, 2, 15, 11, 8, 25, 19, 28, 2, 23, 26, 20, 1, 18, 10, 28, 4, 13, 14, 16)
WN = (23, 17, 24, 10, 14, 7, 22, 19, 12, 18, 15, 25, 20, 5, 26, 0, 8, 2, 27, 11, 26, 9, 28, 21, 16, 5)
VN = (42, 47, 41, 5, 11, 43, 18, 28, 20, 23, 35, 19, 22, 46, 33, 26, 45, 36, 38, 25, 44, 40, 39, 21, 24, 32)
RK = len(UN)
UL = tuple(sorted(set(UN)))
VSTAGES = ((0, 6, 7, 12, 13, 14, 15, 21), (11, 17, 20, 22, 24, 25, 23, 2), (1, 5, 8, 9, 10, 16, 18, 19))
RAW16 = (1, 11, 17, 5, 8, 3, 9, 10, 0, 6, 7, 4, 12, 20, 22, 16)


def _run(prog, blocks):
    vals = list(blocks)
    for a, sa, b, sb in prog:
        vals.append(vals[a] + vals[b] if sa > 0 and sb > 0 else
                    vals[a] - vals[b] if sa > 0 else vals[b] - vals[a])
    return vals


def _terms(prog, nin, node):
    if node < nin:
        return {node: 1}
    a, sa, b, sb = prog[node - nin]
    out = {k: sa * v for k, v in _terms(prog, nin, a).items()}
    out.update({k: sb * v for k, v in _terms(prog, nin, b).items()})
    return out


for _b in range(16):
    _last = max(k for k, st in enumerate(VSTAGES) for r in st if _b in _terms(VP, 16, VN[r]))
    assert VN[RAW16[_b]] == _b or RAW16[_b] in VSTAGES[_last]
assert sorted(sum(VSTAGES, ())) == [r for r in range(RK) if VN[r] >= 16] and len(set(RAW16)) == 16

_WPAR = {n: [] for n in range(8 + len(WP))}
for _t, (_a, _sa, _b, _sb) in enumerate(WP):
    _WPAR[_a].append((8 + _t, _sa))
    _WPAR[_b].append((8 + _t, _sb))


def _worder():
    order = []

    def closure(n, acc):
        if n not in acc and n not in order:
            acc.add(n)
            for q, _ in _WPAR[n]:
                closure(q, acc)
        return acc

    def visit(n):
        if n not in order:
            for q, _ in _WPAR[n]:
                visit(q)
            order.append(n)
    while len([v for v in range(8) if v not in order]):
        visit(min((v for v in range(8) if v not in order), key=lambda v: len(closure(v, set()))))
    return tuple(order)


WORDER = _worder()


def _ln(x):
    m = jnp.mean(x, axis=-1, keepdims=True)
    xc = x - m
    v = jnp.mean(xc * xc, axis=-1, keepdims=True)
    return xc * lax.rsqrt(v + EPS)


_GC = 0.7978845608028654


def _gelu(x):
    h = 0.5 * x
    return h + h * jnp.tanh(x * (_GC + (_GC * 0.044715) * (x * x)))


def _unpack(u):
    return pltpu.bitcast(u, bf16).astype(f32)


def _pack(x):
    return pltpu.bitcast(x.astype(bf16), u32)


def _lcombos(a11, a12, a21, a22):
    return [a11 + a22, a21 + a22, a11, a22, a11 + a12, a21 - a11, a12 - a22]


def _merge(*lists):
    keyed = [((j + 0.5) / len(l), n, j, v) for n, l in enumerate(lists) for j, v in enumerate(l)]
    return [v for _, _, _, v in sorted(keyed, key=lambda t: t[:3])]


def _masks():
    r = lax.broadcasted_iota(jnp.int32, (32, 48), 0)
    c = lax.broadcasted_iota(jnp.int32, (32, 48), 1)
    exist_e = c < 40
    allow_e = exist_e & ((r >= 24) | ((c >= 24) & (c < 32)) | (c <= r))
    fill_e = jnp.where(exist_e, NEG, -jnp.inf).astype(f32)
    r = lax.broadcasted_iota(jnp.int32, (48, 80), 0)
    c = lax.broadcasted_iota(jnp.int32, (48, 80), 1)
    q_even = (r >= 32) & (r < 40)
    exist_o = (q_even & (c < 40)) | (~q_even & (c >= 40))
    ktok = jnp.where(c < 24, c, jnp.where(c < 48, c - 8, c - 16))
    qtok = jnp.where(r < 32, r + 32, r - 8)
    is_mem_key = ((c >= 24) & (c < 32)) | ((c >= 48) & (c < 56))
    allow_o = exist_o & (is_mem_key | (r < 8) | (ktok <= qtok))
    fill_o = jnp.where(exist_o, NEG, -jnp.inf).astype(f32)
    return allow_e, fill_e, allow_o, fill_o


def _rcombo(k, b11, b12, b21, b22):
    if k in (1, 4):
        return (b11 if k == 1 else b22)(k)
    a, b, sign = {0: (b11, b22, 1), 2: (b12, b22, -1), 3: (b21, b11, -1), 5: (b11, b12, 1), 6: (b21, b22, 1)}[k]
    a, b = _unpack(a(k)), _unpack(b(k))
    return (a + b if sign > 0 else a - b).astype(bf16)


def _softmax(s, allow, fill):
    s = jnp.where(allow, s * SCALE, fill)
    m = jnp.max(s, axis=-1, keepdims=True)
    e = jnp.exp(s - m)
    l = jnp.sum(e, axis=-1, keepdims=True)
    r = pl.reciprocal(l, approx=True)
    r = r * (2.0 - l * r)
    return (e * r).astype(bf16)


def _kernel(x_hbm, mem0_hbm, wq_hbm, wk_hbm, wv_hbm, wo_hbm, w1_hbm, w2_hbm, w3_hbm, w4_hbm,
            gw_hbm, out_hbm,
            x_v, s1_v, s2_v, s3_v, s4_v, wqkv_v, wo_v, h_v, b_v, c0_v, l_v, lf_v, n_v, g_v, out_v, xe_v, e_v, oe_v,
            ke_v, ve_v, o_v, mem_v, mem0_ref, gw_ref, zero_s,
            sem, sem_qkv, sem_out):
    RAW = (1, 2, 3, 4)
    RAW1 = (1, 7, 8, 4)

    loads = []

    def rows_load(name, r0, r1):
        loads.append((name, x_hbm.at[pl.ds(r0, r1 - r0)], x_v.at[pl.ds(r0, r1 - r0)]))

    def quad_load(name, w_hbm, s_v, raw, q, c0=0, c1=None):
        k4, n2 = s_v.shape[1], s_v.shape[2]
        c1 = n2 if c1 is None else c1
        src = w_hbm.bitcast(u32).at[pl.ds((q // 2) * k4, k4), pl.ds((q % 2) * n2 + c0, c1 - c0)]
        loads.append((name, src, s_v.at[raw[q], :, pl.ds(c0, c1 - c0)]))

    rows_load("x0", 0, TM)
    rows_load("x1", TM, 2 * TM)
    for name, half, c0, c1 in (("w1a", 0, 0, 256), ("w1bc", 0, 256, 512), ("w1bc", 1, 0, 256), ("w1d", 1, 256, 512)):
        quad_load(name, w1_hbm, s1_v, RAW1, half, c0, c1)
        quad_load(name, w1_hbm, s1_v, RAW1, 2 + half, c0, c1)
    rows_load("x234", 2 * TM, 5 * TM)
    rows_load("x567", 5 * TM, S)
    for q in range(4):
        quad_load("w2", w2_hbm, s2_v, RAW, q)
    for name, w_hbm, s_v in (("w3", w3_hbm, s3_v), ("w4", w4_hbm, s4_v)):
        kb, nb = s_v.shape[1:]
        for q in range(16):
            loads.append((name, w_hbm.at[pl.ds((q // 4) * kb, kb), pl.ds((q % 4) * nb, nb)], s_v.at[RAW16[q]]))
    loads.append(("small", mem0_hbm, mem0_ref))
    loads.append(("small", gw_hbm, gw_ref))
    for j in range(NT):
        loads.append(("wo", wo_hbm.bitcast(u32).at[:, pl.ds(j * 128, 128)], wo_v.at[j]))
    groups = list(dict.fromkeys(name for name, _, _ in loads))
    assert len(groups) == NLOAD

    def start(*names, priority=0):
        for name, src, dst in loads:
            if name in names:
                pltpu.make_async_copy(src, dst, sem.at[groups.index(name)]).start(priority=priority)

    def wait(*names):
        for name, src, dst in loads:
            if name in names:
                pltpu.make_async_copy(src, dst, sem.at[groups.index(name)]).wait()

    SPG = 3 * G

    def qkv_start(g):
        for w, w_hbm in enumerate((wq_hbm, wk_hbm, wv_hbm)):
            wu = w_hbm.bitcast(u32)
            for k in range(G // 2):
                for par in range(2):
                    pltpu.make_async_copy(
                        wu.at[:, par * (H // 2) + g * (G // 2) + k, :],
                        wqkv_v.at[g * SPG + w * G + 2 * k + par], sem_qkv.at[g]).start(priority=1)

    def qkv_wait(g):
        grp = wqkv_v.at[pl.ds(g * SPG, SPG)]
        pltpu.make_async_copy(grp, grp, sem_qkv.at[g]).wait()

    start("x0", "x1", "w1a", "w1bc", "w1d", "x234", "x567", "w2", "w3", "w4", "small")

    def zero(k, carry):
        zero_s[k] = 0
        return carry
    lax.fori_loop(0, RK, zero, 0)

    def tile_idx(ref, cols=128):
        z = zero_s[0]
        n = 16 if ref.dtype == bf16 and cols == 128 else 8
        return (z,) * (len(ref.shape) - 2) + (pl.ds(pl.multiple_of(z, n), n), slice(0, cols))

    hist = []

    def mm(lhs, rhs, side=None, acc=None):
        if side is not None:
            lhs = side(lhs)
        lhs = pltpu.bitcast(lhs, bf16) if lhs.dtype == u32 else lhs.astype(bf16)
        y = _dot(lhs, pltpu.bitcast(rhs, bf16) if rhs.dtype == u32 else rhs)
        if acc is not None:
            y = y + acc
        hist.append(y)
        return y

    class Side:
        def __init__(self, pieces, n, skip=0):
            self.pieces, self.n, self.skip = list(pieces), n, skip

        def __call__(self, val):
            if self.skip:
                self.skip -= 1
                return val
            take = -(-len(self.pieces) // self.n) if self.pieces else 0
            self.n -= 1
            if not take:
                return val
            never = zero_s[0] > 0
            if val.dtype == bf16:
                val = pltpu.bitcast(val, u32)
            rg = 8 if val.dtype == u32 else 16
            ng = val.shape[0] // rg
            groups = [val[8 * m:8 * m + 8] for m in range(val.shape[0] // 8)]
            for j, (fn, rd, wr, lag) in enumerate(self.pieces[:take]):
                m = (j + 1) * ng // take - 1
                pin = lambda v: v
                if lag is not None and len(hist) >= lag:
                    r0 = (16 * m) % hist[-lag].shape[0]
                    a = hist[-lag][r0:r0 + 8, :128]
                    if rd is None:
                        def pin(v, a=a):
                            t = jnp.where(never, jnp.concatenate([a] * (v.shape[0] // 8), axis=0), v[:, :128])
                            return t if v.shape[1] == 128 else jnp.concatenate([t, v[:, 128:]], axis=1)
                    elif rd.dtype == bf16:
                        idx = tile_idx(rd, 256)
                        rd[idx] = jnp.where(never, jnp.concatenate([a, a], axis=1).astype(bf16), rd[idx])
                    else:
                        idx = tile_idx(rd)
                        rd[idx] = jnp.where(never, pltpu.bitcast(a, rd.dtype), rd[idx])
                tiles = fn(pin)
                g = m * rg // 8
                t = groups[g][:, -128:]
                for u in (tiles if wr is None else [wr[tile_idx(wr)]]):
                    t = jnp.where(never, pltpu.bitcast(u, val.dtype), t)
                groups[g] = t if val.shape[1] == 128 else jnp.concatenate([groups[g][:, :-128], t], axis=1)
            self.pieces = self.pieces[take:]
            return jnp.concatenate(groups, axis=0)

    def strassen(lhs, rhs, side, init=(None, None, None, None), ks=range(7)):
        def add(a, b):
            return a if b is None else a + b
        sd = lambda k: side if k in ks else None
        p = [mm(lhs(k), rhs(k), sd(k)) for k in range(5)]
        c12 = add(p[2] + p[4], init[1])
        c21 = add(p[1] + p[3], init[2])
        c22 = mm(lhs(5), rhs(5), sd(5), add(p[0] - p[1] + p[2], init[3]))
        c11 = mm(lhs(6), rhs(6), sd(6), add(p[0] + p[3] - p[4], init[0]))
        return c11, c12, c21, c22

    def fmm(lhs, rhs, side, extra=lambda n: None, emit=None):
        val = {}
        for n in WORDER:
            t = extra(n)
            for q, sg in sorted(_WPAR[n], key=lambda e: -e[1]):
                t = val[q] if t is None else (t + val[q] if sg > 0 else t - val[q])
            for r in range(RK):
                if WN[r] == n:
                    t = mm(lhs(UN[r]), rhs(r), side, t)
            val[n] = t
            if n < 8 and emit is not None:
                emit(n, t)
        return [val[v] for v in range(8)]

    def prep26_pieces(s_v, lag, stages=(sum(VSTAGES, ()),)):
        def piece(rs, cs, stage, pin):
            @functools.lru_cache(None)
            def node(n):
                if n < 16:
                    return s_v[RAW16[n], rs, cs].astype(f32)
                return _run([(0, VP[n - 16][1], 1, VP[n - 16][3])], [node(VP[n - 16][0]), node(VP[n - 16][2])])[-1]
            vals = [node(VN[r]).astype(bf16) for r in stage]
            for r, t in zip(stage, vals):
                s_v[r, rs, cs] = t
        kb, nb = s_v.shape[1:]
        out = []
        for r in range(0, kb, 16):
            out += [(slice(rr, rr + 8), slice(c, c + 256)) for c in range(0, nb - 255, 256) for rr in (r, r + 8)]
            out += [(slice(r, r + 16), slice(nb - 128, nb))] if nb % 256 else []
        return [(functools.partial(piece, rs, cs, st), s_v, s_v, lag) for rs, cs in out for st in stages]

    def prep_pieces(s_v, raw, lag, width=256):
        def piece(r, c, pin):
            idx = (slice(r, r + 8), slice(c, c + width))
            b11, b12, b21, b22 = [_unpack(s_v[(q,) + idx]) for q in raw]
            for k, t in ((0, b11 + b22), (2, b12 - b22), (3, b21 - b11), (5, b11 + b12), (6, b21 + b22)):
                s_v[(k,) + idx] = _pack(t)
        return [(functools.partial(piece, r, c), s_v, s_v, lag)
                for r in range(0, s_v.shape[1], 8) for c in range(0, s_v.shape[2], width)]

    def store_l(slot, q, c, quads, plain=False):
        for k, t in enumerate(quads if plain else _lcombos(*quads)):
            l_v[slot, k, q // 2:q // 2 + 8, c:c + t.shape[1]] = _pack(t)

    def ln_pieces(src, r0, slot, lag, plain=False, width=256, staged=False, clag=None):
        def stats(q, pin):
            x = pin(src[pl.ds(r0 + q, 16), :].astype(f32))
            xs = [x[:, j * 128:(j + 1) * 128] for j in range(NT)]
            m = functools.reduce(lambda a, b: a + b, xs) * (1.0 / NT)
            w = functools.reduce(lambda a, b: a + b, [(t - m) * (t - m) for t in xs])
            mean = jnp.mean(m, axis=-1, keepdims=True)
            var = jnp.sum(w + NT * ((m - mean) * (m - mean)), axis=-1, keepdims=True) * (1.0 / D)
            n_v[0, q:q + 16, :] = jnp.broadcast_to(mean, (16, 128))
            n_v[1, q:q + 16, :] = jnp.broadcast_to(lax.rsqrt(var + EPS), (16, 128))

        def comb(q, c, pin):
            quads = []
            for rr in (0, HM):
                rs = pl.ds(pl.multiple_of(r0 + rr + q + zero_s[0], 16), 16)
                mean, rstd = [jnp.concatenate([n_v[t, rr + q:rr + q + 16, :]] * (width // 128), axis=1)
                              for t in range(2)]
                quads += [(src[rs, cc + c:cc + c + width].astype(f32) - mean) * rstd for cc in (0, DH2)]
            store_l(slot, q, c, quads, plain)

        def comb26(q, pin):
            blocks = []
            for rr in (0, HM):
                rs = pl.ds(pl.multiple_of(r0 + rr + q + zero_s[0], 8), 8)
                mean, rstd = [jnp.concatenate([n_v[t, rr + q:rr + q + 8, :]] * 2, axis=1) for t in range(2)]
                blocks += [(src[rs, cc:cc + D4] - mean) * rstd for cc in range(0, D, D4)]
            vals = _run(UP, blocks)
            for k, u in enumerate(UL):
                lf_v[k, q:q + 8, :] = vals[u].astype(bf16)
        norms = [[(functools.partial(stats, rr + q), None, n_v, lag) for rr in (0, HM)] for q in range(0, HM, 16)]
        if slot is None:
            combs = [[(functools.partial(comb26, qq), n_v, lf_v, clag) for qq in (q, q + 8)]
                     for q in range(0, HM, 16)]
        else:
            combs = [[(functools.partial(comb, q, c), n_v, l_v, clag) for c in range(0, DH2, width)]
                     for q in range(0, HM, 16)]
        if staged:
            return sum(norms, []), sum(combs, [])
        out = list(norms[0])
        for a, b in zip(norms[1:] + [[]], combs):
            out += _merge(a, b) if a else b
        return out

    shifts = (1, 1, -1, -1, 2, 2, -2, -2)

    def shift_pieces(r0, slot, lag, by_value=False):
        def piece(q, j, pin):
            a = [h_v[jj, pl.ds(PAD + r0 + rr + q - shifts[jj], 16), :]
                 for rr in (0, HM) for jj in (j, j + NT // 2)]
            store_l(slot, q, j * 128, [pin(a[0]), a[1], a[2], pin(a[3])])
        return [(functools.partial(piece, q, j), None if by_value else h_v, l_v, lag)
                for q in range(0, HM, 16) for j in range(NT // 2)]

    def lhs_of(slot):
        return lambda k: l_v[slot, k]

    h_v[:, 0:PAD, :] = jnp.zeros((NT, PAD, 128), f32)
    h_v[:, PAD + S:PAD + S + PAD, :] = jnp.zeros((NT, PAD, 128), f32)

    def store_h(r0, c0, h):
        for j in range(h.shape[1] // 128):
            h_v[c0 // 128 + j, PAD + r0:PAD + r0 + h.shape[0], :] = h[:, j * 128:(j + 1) * 128]

    def d1_plain(xn, r0, c0, c1, step, side=None):
        for c in range(c0, c1, step):
            half, cc = c // DH2, c % DH2
            w = jnp.concatenate([s1_v[RAW1[half], :, cc:cc + step], s1_v[RAW1[2 + half], :, cc:cc + step]], axis=0)
            store_h(r0, c, _gelu(mm(xn, w, side)))

    NP1 = 7 * (DH2 // NC1)
    KS1 = (2, 3, 4, 5)

    def d1_s(b, slot, pieces):
        side = Side(pieces, len(KS1) * (DH2 // NC1))
        for c in range(0, DH2, NC1):
            cs = strassen(lhs_of(slot), lambda k: s1_v[k, :, c:c + NC1], side, ks=KS1)
            for q, t in enumerate(cs):
                store_h(b * TM + (q // 2) * HM, (q % 2) * DH2 + c, _gelu(t))

    def d2_s(b, slot, pieces):
        side = Side(pieces, NP1)
        for c in range(0, DH2, NC1):
            idx = [(slice(b * TM + (q // 2) * HM, b * TM + (q // 2 + 1) * HM),
                    slice((q % 2) * DH2 + c, (q % 2) * DH2 + c + NC1)) for q in range(4)]
            cs = strassen(lhs_of(slot), lambda k: s2_v[k, :, c:c + NC1], side,
                          [x_v[i].astype(f32) for i in idx])
            for i, t in zip(idx, cs):
                b_v[i] = t
                if b == 0:
                    c0_v[i] = t

    def split(l, n):
        return [l[len(l) * i // n:len(l) * (i + 1) // n] for i in range(n)]

    LS, LL = 3, 5

    wait("x0")
    xn0 = _pack(_ln(x_v[0:TM, :].astype(f32)))
    wait("x1")
    xn01 = jnp.concatenate([xn0, _pack(_ln(x_v[TM:2 * TM, :].astype(f32)))], axis=0)
    wait("w1a")
    d1_plain(xn01, 0, 0, 256, 256)
    wait("w1bc")
    d1_plain(xn01, 0, 256, 768, 256)
    wait("w1d", "x234")
    hist.clear()
    d1_plain(xn01, 0, 768, D, 128, Side(ln_pieces(x_v, 2 * TM, 0, None, plain=True), 2))
    xn2 = jnp.concatenate([jnp.concatenate([l_v[0, 2 * h], l_v[0, 2 * h + 1]], axis=1) for h in range(2)], axis=0)
    d1_plain(xn2, 2 * TM, 0, D, 128,
             Side(_merge(prep_pieces(s1_v, RAW1, 1), ln_pieces(x_v, 3 * TM, 1, 2)), 8))
    d1_s(3, 1, ln_pieces(x_v, 4 * TM, 0, LL))
    wait("x567", "w2")
    qkv_start(0)
    qkv_start(1)
    hist.clear()
    pw = split(prep_pieces(s2_v, RAW, LS), 4)
    for b in range(4, NB):
        nxt = ln_pieces(x_v, (b + 1) * TM, (b + 1) % 2, LL) if b + 1 < NB else shift_pieces(0, 0, LS, True)
        d1_s(b, b % 2, _merge(pw[b - 4], nxt))
    d2_s(0, 0, shift_pieces(TM, 1, LS, True))
    wait("w3")
    hist.clear()
    pw = split(_merge(prep26_pieces(s3_v, LS), ln_pieces(c0_v, 0, None, LL)), 4)
    for b in range(1, 5):
        d2_s(b, b % 2, _merge(pw[b - 1], shift_pieces((b + 1) * TM, (b + 1) % 2, LS)))
    wait("w4", "small")
    hist.clear()
    pw = prep26_pieces(s4_v, LS)
    d2_s(5, 1, _merge(pw[:34], shift_pieces(6 * TM, 0, LS)))
    d2_s(6, 0, _merge(pw[34:68], shift_pieces(7 * TM, 1, LS)))
    d2_s(7, 1, pw[68:])
    start("wo", priority=1)

    def ffn(i, carry):
        qkv_wait(i)
        r0 = pl.multiple_of(i * TM, TM)
        rn = pl.multiple_of(jnp.minimum(i + 1, NB - 1) * TM, TM)
        acc = {}
        hist.clear()

        def relayout(p, r0_, r1_, pin):
            s0 = i * SPG + 2 * p
            for r in range(r0_, r1_, 8):
                e = wqkv_v[s0, r:r + 8, :]
                o = wqkv_v[s0 + 1, r:r + 8, :]
                wqkv_v[s0, r:r + 8, :] = (e & jnp.uint32(0xFFFF)) | (o << 16)
                wqkv_v[s0 + 1, r:r + 8, :] = (e >> 16) | (o & jnp.uint32(0xFFFF0000))

        relays = [(functools.partial(relayout, p, r, r + 32), wqkv_v, wqkv_v, 3)
                  for p in range(SPG // 2) for r in range(0, D // 2, 32)]
        norms, combs = ln_pieces(b_v, rn, None, 5, staged=True, clag=3)

        def gate(q, pin):
            gw = gw_ref[...].astype(f32)
            x = pin(x_v[pl.ds(r0 + q, 16), :].astype(f32))
            t = functools.reduce(lambda a, b: a + b,
                                 [x[:, j * 128:(j + 1) * 128] * gw[j:j + 1, :] for j in range(NT)])
            g = jax.nn.sigmoid(jnp.sum(t, axis=-1, keepdims=True))
            g_v[pl.ds(r0 + q, 16), :] = jnp.broadcast_to(g, (16, 128))

        gates = [(functools.partial(gate, q), None, g_v, 5) for q in range(0, TM, 16)]

        def extras(t, pin):
            jj, o = 2 * i + t // 2, 24 + 8 * (t % 2)
            xs = [pin(x_v[pl.ds(pl.multiple_of((jj + hh) * 64 + o, 8), 8), :].astype(f32)) for hh in (0, NPAIR // 2)]
            vals = _run(UP, [x[:, cc:cc + D4] for x in xs for cc in range(0, D, D4)])
            for k, u in enumerate(UL):
                xe_v[k, pl.ds(pl.multiple_of(i * 32 + t * 8, 8), 8), :] = vals[u].astype(bf16)

        xes = [(functools.partial(extras, t), None, xe_v, 3) for t in range(4)]
        hs = {}

        def gelu_pieces(c, cs):
            def piece(r, cc, vs, pin):
                for v in vs:
                    hs[c, v, r, cc] = _gelu(pin(cs[v][r:r + 8, cc:cc + 128]))
                return [hs[c, v, r, cc] for v in vs]
            return [(functools.partial(piece, r, cc, vs), None, None, 3) for r in range(0, HM, 8)
                    for cc in range(0, cs[0].shape[1], 128) for vs in ((0, 1, 2, 3), (4, 5, 6, 7))]

        def d3(c, side):
            c0, c1 = FCH[c]
            cs = fmm(lambda u: lf_v[UL.index(u)], lambda r: s3_v[r, :, c0:c1], side)
            assert not side.pieces
            return gelu_pieces(c, cs)

        def d4(c, side):
            c0, c1 = FCH[c]
            lh = _run(UP, [jnp.concatenate([jnp.concatenate(
                [hs.pop((c, v, r, cc)) for cc in range(0, c1 - c0, 128)], axis=1) for r in range(0, HM, 8)], axis=0)
                for v in range(8)])
            rhs = lambda r: s4_v[r, c0:c1, :]
            if c + 1 < len(FCH):
                for n in WORDER:
                    for r in range(RK):
                        if WN[r] == n:
                            acc[n] = mm(lh[UN[r]], rhs(r), side, acc.get(n))
            else:
                idx = lambda v: (pl.ds(r0 + (v // 4) * HM, HM), slice((v % 4) * D4, (v % 4 + 1) * D4))

                def extra(n):
                    if n >= 8:
                        return acc.get(n)
                    return b_v[idx(n)] + acc[n] if n in acc else b_v[idx(n)]

                def emit_b(v, t):
                    b_v[idx(v)] = jnp.concatenate([1.0 - g_v[idx(v)[0], :]] * 2, axis=1) * t
                fmm(lambda u: lh[u], rhs, side, extra, emit_b)
            assert not side.pieces

        g0 = d3(0, Side(relays[:20], 23, 3))
        g1 = d3(1, Side(_merge(g0, gates), 23, 2))
        d4(0, Side(g1[:22], 22, 4))
        g2 = d3(2, Side(_merge(g1[22:], relays[20:40]), 25))
        d4(1, Side(g2, 23, 2))
        g3 = d3(3, Side(_merge(relays[40:], norms, xes), 26))
        d4(2, Side(_merge(g3, combs), 23, 2))
        d4(3, Side([], 1))

        @pl.when(i + 2 < NG)
        def _():
            qkv_start(i + 2)

        return carry

    lax.fori_loop(0, NB, ffn, 0)

    def pre(it, carry):
        hist.clear()
        for u in range(3 * NG // NPRE):
            s0 = (it * (3 * NG // NPRE) + u) * G

            def rhs(r):
                t = None
                for q, sg in sorted(_terms(VP, 16, VN[r]).items(), key=lambda e: -e[1]):
                    blk = wqkv_v[s0 + q % 4 + zero_s[r], (q // 4) * (D // 8):(q // 4 + 1) * (D // 8), :]
                    if VN[r] < 16:
                        return blk
                    blk = _unpack(blk)
                    t = blk if t is None else (t + blk if sg > 0 else t - blk)
                return t.astype(bf16)
            for v, t in enumerate(fmm(lambda k: xe_v[UL.index(k)], rhs, None)):
                e_v[s0 + v % 4, (v // 4) * 128:(v // 4 + 1) * 128, :] = _pack(t)
        return carry

    lax.fori_loop(0, NPRE, pre, 0)

    wait("wo")
    mem_v[...] = mem0_ref[...].astype(f32)

    def slab(w, h):
        return (h // G) * SPG + w * G + h % G

    def step(j, hx, odd, late, allow, fill):
        qs, ks, vs, ps = {}, {}, {}, {}
        wload = lambda w, h: pltpu.bitcast(wqkv_v[slab(w, h)], bf16)
        eload = lambda w, h: pltpu.bitcast(e_v[slab(w, h), pl.ds(pl.multiple_of(j * 8, 8), 8), :], bf16)

        def proj(g):
            part = {}
            if late and g == 0:
                for h in range(2):
                    for w in range(3):
                        part[w, h] = _dot(hx[:, :DH2], wload(w, h)[:DH2])
            for h in range(g * G, (g + 1) * G):
                q, k, v = [(_dot(hx[:, DH2:], wload(w, h)[DH2:]) + part[w, h] if (w, h) in part
                            else _dot(hx, wload(w, h))).astype(bf16) for w in range(3)]
                if odd:
                    q = jnp.concatenate([q, eload(0, h)], axis=0)
                    k = jnp.concatenate([pltpu.bitcast(ke_v[h], bf16), eload(1, h), k], axis=0)
                    v = jnp.concatenate([pltpu.bitcast(ve_v[h], bf16), eload(2, h), v], axis=0)
                else:
                    ke_v[h] = pltpu.bitcast(k, u32)
                    ve_v[h] = pltpu.bitcast(v, u32)
                    k = jnp.concatenate([k, eload(1, h)], axis=0)
                    v = jnp.concatenate([v, eload(2, h)], axis=0)
                qs[h], ks[h], vs[h] = q, k, v

        def score(g):
            for h in range(g * G, (g + 1) * G):
                s = lax.dot_general(qs.pop(h), ks.pop(h), (((1,), (1,)), ((), ())),
                                    preferred_element_type=f32)
                ps[h] = _softmax(s, allow, fill)

        def pv(g):
            os_ = []
            for h in range(g * G, (g + 1) * G):
                o = _dot(ps.pop(h), vs.pop(h))
                o_v[:, h * 128:(h + 1) * 128] = _pack(o[:32])
                os_.append(o)
            if odd:
                quads = [jnp.concatenate([os_[2 * kk][r:r + 8], os_[2 * kk + 1][r:r + 8]], axis=1)
                         for r in (32, 40) for kk in range(2)]
                for k, t in enumerate(_lcombos(*quads)):
                    oe_v[k, pl.ds(pl.multiple_of(j * 8, 8), 8), g * 256:(g + 1) * 256] = t.astype(bf16)

        acc = [None] * NT

        def wo(h0, h1, j0, j1):
            o = pltpu.bitcast(o_v[:, h0 * 128:h1 * 128], bf16)
            for n in range(j0, j1):
                y = _dot(o, pltpu.bitcast(wo_v[n, h0 * 64:h1 * 64, :], bf16))
                acc[n] = y if acc[n] is None else y + acc[n]

        for t in range(NG):
            proj(t)
            if t >= 2:
                pv(t - 2)
            if t >= 1:
                score(t - 1)
        wo(0, 16, 0, 4)
        pv(NG - 2)
        score(NG - 1)
        wo(0, 16, 4, 8)
        pv(NG - 1)
        wo(16, 24, 0, 8)
        wo(24, 32, 0, 8)
        return jnp.concatenate(acc, axis=1)

    def emit(j, r0, o0, a):
        rs = pl.ds(r0 + o0, 24)
        g = jnp.concatenate([g_v[rs, :]] * NT, axis=1)
        out_v[j, o0:o0 + 24, :] = (g * a + b_v[rs, :]).astype(bf16)

    def pair(j, mem, late):
        r0 = pl.multiple_of(j * 64, 64)
        allow_e, fill_e, allow_o, fill_o = _masks()
        xa = x_v[pl.ds(r0 + 16, 8), :].astype(f32)
        xb = x_v[pl.ds(r0 + 40, 8), :].astype(f32)
        hx = jnp.concatenate([x_v[pl.ds(r0, 16), :], jnp.concatenate([xa, mem], 0).astype(bf16)], 0)
        oe = step(j, hx, False, late, allow_e, fill_e)
        emit(j, r0, 0, oe[:24])
        hx = jnp.concatenate([jnp.concatenate([oe[24:32], xb], 0).astype(bf16), x_v[pl.ds(r0 + 48, 16), :]], 0)
        oo = step(j, hx, True, True, allow_o, fill_o)
        emit(j, r0, 40, oo[8:])
        return oo[:8]

    def a_iter(it, carry):
        mem = mem_v[...]
        for t in range(PPI):
            mem = pair(it * PPI + t, mem, t > 0)
        mem_v[...] = mem
        for t in range(PPI):
            for o0 in (0, 40):
                idx = (it * PPI + t, pl.ds(o0, 24))
                pltpu.make_async_copy(out_v.at[idx], out_hbm.at[idx], sem_out).start()
        return carry

    lax.fori_loop(0, NPAIR // PPI, a_iter, 0)

    hist.clear()
    for n in range(NT // 2):
        quad = [lambda k, t=2 * n + q % 2, o=(q // 2) * 128: jnp.concatenate(
            [wo_v[t + zero_s[k], g * 256 + o:g * 256 + o + 128, :] for g in range(NG)], axis=0) for q in range(4)]
        cs = strassen(lambda k: oe_v[k], lambda k: _rcombo(k, *quad), None)
        cols = slice(n * 256, (n + 1) * 256)
        for half in range(2):
            t = jnp.concatenate(cs[2 * half:2 * half + 2], axis=1)
            o0 = 24 + half * 8
            for jj in range(NPAIR):
                rs = slice(jj * 64 + o0, jj * 64 + o0 + 8)
                g = jnp.concatenate([g_v[rs, :]] * 2, axis=1)
                out_v[jj, o0:o0 + 8, cols] = (g * t[jj * 8:jj * 8 + 8] + b_v[rs, cols]).astype(bf16)
        if n >= 2:
            idx = (slice(None), pl.ds(24, 16), pl.ds(0, 768) if n == 2 else pl.ds(768, 256))
            pltpu.make_async_copy(out_v.at[idx], out_hbm.at[idx], sem_out).start()
    pltpu.make_async_copy(out_v, out_hbm, sem_out).wait()


@functools.partial(jax.jit, static_argnames=("A_seg_len",))
def pallas_gated_mix__memory_aug_recurrent_mem_tr__mixer_s_mlp__prompt_kernel(
    A_x, A_mem0, A_Wq, A_Wk, A_Wv, A_Wo, A_seg_len, B_x, B_w1, B_w2, B_w3, B_w4, gate_w,
):
    assert A_seg_len == SEG
    assert A_x.shape == (1, S, D) and A_mem0.shape == (1, M, D)
    any_spec = pl.BlockSpec(memory_space=pl.ANY)
    out = pl.pallas_call(
        _kernel,
        out_shape=jax.ShapeDtypeStruct((NPAIR, 64, D), bf16),
        in_specs=[any_spec] * 11,
        out_specs=any_spec,
        scratch_shapes=[
            pltpu.VMEM((S, D), bf16),
            pltpu.VMEM((9, D // 4, D // 2), u32),
            pltpu.VMEM((7, D // 4, D // 2), u32),
            pltpu.VMEM((RK, D4, F4), bf16),
            pltpu.VMEM((RK, F4, D4), bf16),
            pltpu.VMEM((3 * H, D // 2, DH), u32),
            pltpu.VMEM((NT, H * DH // 2, 128), u32),
            pltpu.VMEM((NT, S + 2 * PAD, 128), f32),
            pltpu.VMEM((S, D), f32),
            pltpu.VMEM((TM, D), f32),
            pltpu.VMEM((2, 7, HM // 2, D // 2), u32),
            pltpu.VMEM((len(UL), HM, D4), bf16),
            pltpu.VMEM((2, TM, 128), f32),
            pltpu.VMEM((S, 128), f32),
            pltpu.VMEM((NPAIR, 64, D), bf16),
            pltpu.VMEM((len(UL), 8 * NPAIR, D4), bf16),
            pltpu.VMEM((3 * H, 8 * NPAIR, DH), u32),
            pltpu.VMEM((7, 8 * NPAIR, H * DH // 2), bf16),
            pltpu.VMEM((H, 16, 128), u32),
            pltpu.VMEM((H, 16, 128), u32),
            pltpu.VMEM((16, H * DH), u32),
            pltpu.VMEM((M, D), f32),
            pltpu.VMEM((M, D), bf16),
            pltpu.VMEM((NT, 128), bf16),
            pltpu.SMEM((RK,), jnp.int32),
            pltpu.SemaphoreType.DMA((NLOAD,)),
            pltpu.SemaphoreType.DMA((NG,)),
            pltpu.SemaphoreType.DMA,
        ],
        compiler_params=pltpu.CompilerParams(vmem_limit_bytes=126 * 1024 * 1024,
                                             disable_bounds_checks=True),
    )(
        A_x.reshape(S, D), A_mem0.reshape(M, D),
        A_Wq.reshape(D // 2, 2 * H, DH), A_Wk.reshape(D // 2, 2 * H, DH), A_Wv.reshape(D // 2, 2 * H, DH),
        A_Wo.reshape(H * DH, D), B_w1, B_w2, B_w3, B_w4, gate_w.reshape(NT, 128),
    )
    return out.reshape(1, S, D)
```

```python
import functools

import jax
import jax.numpy as jnp
from jax import lax
import jax.experimental.pallas as pl
import jax.experimental.pallas.tpu as pltpu

f32, bf16, u32 = jnp.float32, jnp.bfloat16, jnp.uint32

S, D, H, DH, M, SEG, F = 2048, 1024, 32, 128, 8, 32, 3584
SCALE = DH ** -0.5
NEG = -1000000000.0
EPS = 1e-05

TM = 256
NB = S // TM
HM = TM // 2
DH2 = D // 2
D4, F4 = D // 4, F // 4
FCH = ((0, 128), (128, 384), (384, 640), (640, 896))
NC1 = 128
NPAIR = S // (2 * SEG)
PPI = 2
NPRE = 4
G = 4
NG = H // G
PAD = 8
NT = D // 128
NLOAD = 12
assert NB == NG

_dot = functools.partial(jnp.dot, preferred_element_type=f32)

UP = ((4, 1, 5, 1), (6, 1, 8, 1), (0, 1, 3, 1), (2, -1, 9, 1), (4, -1, 10, 1), (0, 1, 1, 1), (2, 1, 12, 1),
      (5, 1, 7, -1), (7, 1, 12, -1), (11, -1, 13, 1), (10, -1, 11, 1), (2, 1, 7, 1), (0, -1, 4, 1),
      (6, 1, 7, 1), (1, -1, 5, 1), (3, 1, 7, -1), (1, 1, 4, 1), (2, 1, 3, 1), (1, -1, 3, 1), (1, 1, 7, -1),
      (2, 1, 6, -1))
WP = ((0, -1, 3, 1), (4, 1, 6, -1), (1, 1, 8, 1), (5, 1, 10, 1), (4, -1, 7, 1), (0, -1, 9, -1),
      (11, 1, 12, 1), (6, 1, 7, -1), (2, 1, 5, -1), (0, -1, 7, -1), (9, 1, 11, -1), (2, 1, 13, 1),
      (5, 1, 13, 1), (2, -1, 3, 1), (5, 1, 6, 1), (0, 1, 4, 1), (2, 1, 7, 1), (1, 1, 2, 1), (1, 1, 5, 1),
      (3, 1, 7, 1), (2, 1, 6, 1))
VP = ((1, 1, 5, -1), (8, 1, 11, 1), (10, 1, 17, 1), (13, 1, 16, -1), (0, 1, 4, -1), (0, 1, 3, 1),
      (14, 1, 18, -1), (0, 1, 11, 1), (14, 1, 19, -1), (0, 1, 5, 1), (12, 1, 15, 1), (2, 1, 21, 1),
      (10, 1, 14, -1), (4, 1, 7, 1), (11, 1, 19, 1), (12, -1, 20, 1), (13, 1, 14, -1), (9, 1, 30, -1),
      (3, -1, 15, 1), (6, 1, 23, 1), (24, 1, 27, -1), (9, -1, 18, 1), (7, 1, 34, 1), (2, 1, 6, -1),
      (0, 1, 8, -1), (6, 1, 21, 1), (22, 1, 31, -1), (6, 1, 29, 1), (0, 1, 1, 1), (15, 1, 25, 1),
      (5, 1, 37, 1), (15, 1, 20, 1))
UN = (7, 27, 24, 17, 9, 22, 21, 2, 15, 11, 8, 25, 19, 28, 2, 23, 26, 20, 1, 18, 10, 28, 4, 13, 14, 16)
WN = (23, 17, 24, 10, 14, 7, 22, 19, 12, 18, 15, 25, 20, 5, 26, 0, 8, 2, 27, 11, 26, 9, 28, 21, 16, 5)
VN = (42, 47, 41, 5, 11, 43, 18, 28, 20, 23, 35, 19, 22, 46, 33, 26, 45, 36, 38, 25, 44, 40, 39, 21, 24, 32)
RK = len(UN)
UL = tuple(sorted(set(UN)))
VSTAGES = ((0, 6, 7, 12, 13, 14, 15, 21), (11, 17, 20, 22, 24, 25, 23, 2), (1, 5, 8, 9, 10, 16, 18, 19))
RAW16 = (1, 11, 17, 5, 8, 3, 9, 10, 0, 6, 7, 4, 12, 20, 22, 16)


def _run(prog, blocks):
    vals = list(blocks)
    for a, sa, b, sb in prog:
        vals.append(vals[a] + vals[b] if sa > 0 and sb > 0 else
                    vals[a] - vals[b] if sa > 0 else vals[b] - vals[a])
    return vals


def _terms(prog, nin, node):
    if node < nin:
        return {node: 1}
    a, sa, b, sb = prog[node - nin]
    out = {k: sa * v for k, v in _terms(prog, nin, a).items()}
    out.update({k: sb * v for k, v in _terms(prog, nin, b).items()})
    return out


for _b in range(16):
    _last = max(k for k, st in enumerate(VSTAGES) for r in st if _b in _terms(VP, 16, VN[r]))
    assert VN[RAW16[_b]] == _b or RAW16[_b] in VSTAGES[_last]
assert sorted(sum(VSTAGES, ())) == [r for r in range(RK) if VN[r] >= 16] and len(set(RAW16)) == 16

_WPAR = {n: [] for n in range(8 + len(WP))}
for _t, (_a, _sa, _b, _sb) in enumerate(WP):
    _WPAR[_a].append((8 + _t, _sa))
    _WPAR[_b].append((8 + _t, _sb))


def _worder():
    order = []

    def closure(n, acc):
        if n not in acc and n not in order:
            acc.add(n)
            for q, _ in _WPAR[n]:
                closure(q, acc)
        return acc

    def visit(n):
        if n not in order:
            for q, _ in _WPAR[n]:
                visit(q)
            order.append(n)
    while len([v for v in range(8) if v not in order]):
        visit(min((v for v in range(8) if v not in order), key=lambda v: len(closure(v, set()))))
    return tuple(order)


WORDER = _worder()


def _ln(x):
    m = jnp.mean(x, axis=-1, keepdims=True)
    xc = x - m
    v = jnp.mean(xc * xc, axis=-1, keepdims=True)
    return xc * lax.rsqrt(v + EPS)


_GC = 0.7978845608028654


def _gelu(x):
    h = 0.5 * x
    return h + h * jnp.tanh(x * (_GC + (_GC * 0.044715) * (x * x)))


def _unpack(u):
    return pltpu.bitcast(u, bf16).astype(f32)


def _pack(x):
    return pltpu.bitcast(x.astype(bf16), u32)


def _lcombos(a11, a12, a21, a22):
    return [a11 + a22, a21 + a22, a11, a22, a11 + a12, a21 - a11, a12 - a22]


def _merge(*lists):
    keyed = [((j + 0.5) / len(l), n, j, v) for n, l in enumerate(lists) for j, v in enumerate(l)]
    return [v for _, _, _, v in sorted(keyed, key=lambda t: t[:3])]


def _masks():
    r = lax.broadcasted_iota(jnp.int32, (32, 48), 0)
    c = lax.broadcasted_iota(jnp.int32, (32, 48), 1)
    exist_e = c < 40
    allow_e = exist_e & ((r >= 24) | ((c >= 24) & (c < 32)) | (c <= r))
    fill_e = jnp.where(exist_e, NEG, -jnp.inf).astype(f32)
    r = lax.broadcasted_iota(jnp.int32, (48, 80), 0)
    c = lax.broadcasted_iota(jnp.int32, (48, 80), 1)
    q_even = (r >= 32) & (r < 40)
    exist_o = (q_even & (c < 40)) | (~q_even & (c >= 40))
    ktok = jnp.where(c < 24, c, jnp.where(c < 48, c - 8, c - 16))
    qtok = jnp.where(r < 32, r + 32, r - 8)
    is_mem_key = ((c >= 24) & (c < 32)) | ((c >= 48) & (c < 56))
    allow_o = exist_o & (is_mem_key | (r < 8) | (ktok <= qtok))
    fill_o = jnp.where(exist_o, NEG, -jnp.inf).astype(f32)
    return allow_e, fill_e, allow_o, fill_o


def _rcombo(k, b11, b12, b21, b22):
    if k in (1, 4):
        return (b11 if k == 1 else b22)(k)
    a, b, sign = {0: (b11, b22, 1), 2: (b12, b22, -1), 3: (b21, b11, -1), 5: (b11, b12, 1), 6: (b21, b22, 1)}[k]
    a, b = _unpack(a(k)), _unpack(b(k))
    return (a + b if sign > 0 else a - b).astype(bf16)


def _softmax(s, allow, fill):
    s = jnp.where(allow, s * SCALE, fill)
    m = jnp.max(s, axis=-1, keepdims=True)
    e = jnp.exp(s - m)
    l = jnp.sum(e, axis=-1, keepdims=True)
    r = pl.reciprocal(l, approx=True)
    r = r * (2.0 - l * r)
    return (e * r).astype(bf16)


def _kernel(x_hbm, mem0_hbm, wq_hbm, wk_hbm, wv_hbm, wo_hbm, w1_hbm, w2_hbm, w3_hbm, w4_hbm,
            gw_hbm, out_hbm,
            x_v, s1_v, s2_v, s3_v, s4_v, wqkv_v, wo_v, h_v, b_v, c0_v, l_v, lf_v, n_v, g_v, out_v, xe_v, e_v, oe_v,
            ke_v, ve_v, o_v, mem_v, mem0_ref, gw_ref, zero_s,
            sem, sem_qkv, sem_out):
    RAW = (1, 2, 3, 4)
    RAW1 = (1, 7, 8, 4)

    loads = []

    def rows_load(name, r0, r1):
        loads.append((name, x_hbm.at[pl.ds(r0, r1 - r0)], x_v.at[pl.ds(r0, r1 - r0)]))

    def quad_load(name, w_hbm, s_v, raw, q, c0=0, c1=None):
        k4, n2 = s_v.shape[1], s_v.shape[2]
        c1 = n2 if c1 is None else c1
        src = w_hbm.bitcast(u32).at[pl.ds((q // 2) * k4, k4), pl.ds((q % 2) * n2 + c0, c1 - c0)]
        loads.append((name, src, s_v.at[raw[q], :, pl.ds(c0, c1 - c0)]))

    rows_load("x0", 0, TM)
    rows_load("x1", TM, 2 * TM)
    for name, half, c0, c1 in (("w1a", 0, 0, 256), ("w1bc", 0, 256, 512), ("w1bc", 1, 0, 256), ("w1d", 1, 256, 512)):
        quad_load(name, w1_hbm, s1_v, RAW1, half, c0, c1)
        quad_load(name, w1_hbm, s1_v, RAW1, 2 + half, c0, c1)
    rows_load("x234", 2 * TM, 5 * TM)
    rows_load("x567", 5 * TM, S)
    for q in range(4):
        quad_load("w2", w2_hbm, s2_v, RAW, q)
    for name, w_hbm, s_v in (("w3", w3_hbm, s3_v), ("w4", w4_hbm, s4_v)):
        kb, nb = s_v.shape[1:]
        for q in range(16):
            loads.append((name, w_hbm.at[pl.ds((q // 4) * kb, kb), pl.ds((q % 4) * nb, nb)], s_v.at[RAW16[q]]))
    loads.append(("small", mem0_hbm, mem0_ref))
    loads.append(("small", gw_hbm, gw_ref))
    for j in range(NT):
        loads.append(("wo", wo_hbm.bitcast(u32).at[:, pl.ds(j * 128, 128)], wo_v.at[j]))
    groups = list(dict.fromkeys(name for name, _, _ in loads))
    assert len(groups) == NLOAD

    def start(*names, priority=0):
        for name, src, dst in loads:
            if name in names:
                pltpu.make_async_copy(src, dst, sem.at[groups.index(name)]).start(priority=priority)

    def wait(*names):
        for name, src, dst in loads:
            if name in names:
                pltpu.make_async_copy(src, dst, sem.at[groups.index(name)]).wait()

    SPG = 3 * G

    def qkv_start(g):
        for w, w_hbm in enumerate((wq_hbm, wk_hbm, wv_hbm)):
            wu = w_hbm.bitcast(u32)
            for k in range(G // 2):
                for par in range(2):
                    pltpu.make_async_copy(
                        wu.at[:, par * (H // 2) + g * (G // 2) + k, :],
                        wqkv_v.at[g * SPG + w * G + 2 * k + par], sem_qkv.at[g]).start(priority=1)

    def qkv_wait(g):
        grp = wqkv_v.at[pl.ds(g * SPG, SPG)]
        pltpu.make_async_copy(grp, grp, sem_qkv.at[g]).wait()

    start("x0", "x1", "w1a", "w1bc", "w1d", "x234", "x567", "w2", "w3", "w4", "small")

    def zero(k, carry):
        zero_s[k] = 0
        return carry
    lax.fori_loop(0, RK, zero, 0)

    def tile_idx(ref, cols=128):
        z = zero_s[0]
        n = 16 if ref.dtype == bf16 and cols == 128 else 8
        return (z,) * (len(ref.shape) - 2) + (pl.ds(pl.multiple_of(z, n), n), slice(0, cols))

    rot = [0]
    ROT = 0
    hist = []

    def mm(lhs, rhs, side=None, acc=None):
        if side is not None:
            lhs = side(lhs)
        lhs = pltpu.bitcast(lhs, bf16) if lhs.dtype == u32 else lhs.astype(bf16)
        y = _dot(lhs, pltpu.bitcast(rhs, bf16) if rhs.dtype == u32 else rhs)
        if acc is not None:
            y = y + acc
        hist.append(y)
        return y

    class Side:
        def __init__(self, pieces, n, skip=0):
            cap = [0] * skip + ([1] * n if isinstance(n, int) else list(n))
            tot = sum(p[4] for p in pieces)
            self.plan = [[] for _ in cap]
            done = 0
            for p in pieces:
                done += p[4]
                x, d = done / tot * sum(cap), 0
                while x > cap[d] + 1e-9:
                    x -= cap[d]
                    d += 1
                self.plan[d].append((p, x / cap[d]))
            self.pieces = len(pieces)

        def __call__(self, val):
            todo = self.plan.pop(0) if self.plan else []
            if not todo:
                return val
            self.pieces -= len(todo)
            never = zero_s[0] > 0
            if val.dtype == bf16:
                val = pltpu.bitcast(val, u32)
            rg = 8 if val.dtype == u32 else 16
            ng = val.shape[0] // rg
            groups = [val[8 * m:8 * m + 8] for m in range(val.shape[0] // 8)]
            nk = val.shape[1] // 128
            npass = max(nk // 4, 1)
            for (fn, rd, wr, lag, _), pos in todo:
                sl = max(-int(-pos * ng * npass // 1) - 1, 0)
                m = sl % ng
                rot[0] += ROT
                kt = (sl // ng) * 4 + (rot[0] - 1) % min(nk, 4)
                pin = lambda v, w=128: v
                if lag is not None and len(hist) >= lag:
                    r0 = (16 * m) % hist[-lag].shape[0]
                    a = hist[-lag][r0:r0 + 8, :128]
                    if rd is None:
                        def pin(v, w=128, a=a):
                            a = jnp.concatenate([pltpu.bitcast(a, v.dtype)] * (v.shape[0] // 8), axis=0)
                            t = jnp.where(never, jnp.concatenate([a] * (w // 128), axis=1), v[:, :w])
                            return t if v.shape[1] == w else jnp.concatenate([t, v[:, w:]], axis=1)
                    elif rd.dtype == bf16:
                        idx = tile_idx(rd, 256)
                        rd[idx] = jnp.where(never, jnp.concatenate([a, a], axis=1).astype(bf16), rd[idx])
                    else:
                        idx = tile_idx(rd)
                        rd[idx] = jnp.where(never, pltpu.bitcast(a, rd.dtype), rd[idx])
                tiles = fn(pin)
                g = m * rg // 8
                ks = [groups[g][:, k * 128:(k + 1) * 128] for k in range(nk)]
                for u in (tiles if wr is None else [wr[tile_idx(wr)]]):
                    ks[kt] = jnp.where(never, pltpu.bitcast(u, val.dtype), ks[kt])
                groups[g] = jnp.concatenate(ks, axis=1)
            return jnp.concatenate(groups, axis=0)

    def strassen(lhs, rhs, side, init=(None, None, None, None)):
        def add(a, b):
            return a if b is None else a + b
        p = [mm(lhs(k), rhs(k), side) for k in range(5)]
        c12 = add(p[2] + p[4], init[1])
        c21 = add(p[1] + p[3], init[2])
        c22 = mm(lhs(5), rhs(5), side, add(p[0] - p[1] + p[2], init[3]))
        c11 = mm(lhs(6), rhs(6), side, add(p[0] + p[3] - p[4], init[0]))
        return c11, c12, c21, c22

    def fmm(lhs, rhs, side, extra=lambda n: None, emit=None):
        val = {}
        for n in WORDER:
            t = extra(n)
            for q, sg in sorted(_WPAR[n], key=lambda e: -e[1]):
                t = val[q] if t is None else (t + val[q] if sg > 0 else t - val[q])
            for r in range(RK):
                if WN[r] == n:
                    t = mm(lhs(UN[r]), rhs(r), side, t)
            val[n] = t
            if n < 8 and emit is not None:
                emit(n, t)
        return [val[v] for v in range(8)]

    def prep26_pieces(s_v, lag, stages=(sum(VSTAGES, ()),)):
        def piece(rs, cs, stage, pin):
            @functools.lru_cache(None)
            def node(n):
                if n < 16:
                    return s_v[RAW16[n], rs, cs].astype(f32)
                return _run([(0, VP[n - 16][1], 1, VP[n - 16][3])], [node(VP[n - 16][0]), node(VP[n - 16][2])])[-1]
            vals = [node(VN[r]).astype(bf16) for r in stage]
            for r, t in zip(stage, vals):
                s_v[r, rs, cs] = t
        kb, nb = s_v.shape[1:]
        out = []
        for r in range(0, kb, 16):
            out += [(slice(rr, rr + 8), slice(c, c + 256)) for c in range(0, nb - 255, 256) for rr in (r, r + 8)]
            out += [(slice(rr, rr + 8), slice(nb - 128, nb)) for rr in (r, r + 8)] if nb % 256 else []
        return [(functools.partial(piece, rs, cs, st), s_v, s_v, lag, 130 if cs.stop - cs.start == 256 else 100)
                for rs, cs in out for st in stages]

    def prep_pieces(s_v, raw, lag, width=256, by_value=False):
        def piece(r, c, pin):
            idx = (slice(r, r + 8), slice(c, c + width))
            b11, b12, b21, b22 = [_unpack(pin(s_v[(q,) + idx], width) if n in (0, 3) else s_v[(q,) + idx])
                                  for n, q in enumerate(raw)]
            for k, t in ((0, b11 + b22), (2, b12 - b22), (3, b21 - b11), (5, b11 + b12), (6, b21 + b22)):
                s_v[(k,) + idx] = _pack(t)
        return [(functools.partial(piece, r, c), None if by_value else s_v, s_v, lag, 80)
                for c in range(0, s_v.shape[2], width) for r in range(0, s_v.shape[1], 8)]

    def store_l(slot, q, c, quads, plain=False):
        for k, t in enumerate(quads if plain else _lcombos(*quads)):
            l_v[slot, k, q // 2:q // 2 + 8, c:c + t.shape[1]] = _pack(t)

    def ln_pieces(src, r0, slot, lag, plain=False, width=256, staged=False, clag=None):
        def stats(q, pin):
            x = pin(src[pl.ds(r0 + q, 16), :].astype(f32))
            xs = [x[:, j * 128:(j + 1) * 128] for j in range(NT)]
            m = functools.reduce(lambda a, b: a + b, xs) * (1.0 / NT)
            w = functools.reduce(lambda a, b: a + b, [(t - m) * (t - m) for t in xs])
            mean = jnp.mean(m, axis=-1, keepdims=True)
            var = jnp.sum(w + NT * ((m - mean) * (m - mean)), axis=-1, keepdims=True) * (1.0 / D)
            n_v[0, q:q + 16, :] = jnp.broadcast_to(mean, (16, 128))
            n_v[1, q:q + 16, :] = jnp.broadcast_to(lax.rsqrt(var + EPS), (16, 128))

        def comb(q, c, pin):
            quads = []
            for rr in (0, HM):
                rs = pl.ds(pl.multiple_of(r0 + rr + q + zero_s[0], 16), 16)
                mean, rstd = [jnp.concatenate([n_v[t, rr + q:rr + q + 16, :]] * (width // 128), axis=1)
                              for t in range(2)]
                quads += [(src[rs, cc + c:cc + c + width].astype(f32) - mean) * rstd for cc in (0, DH2)]
            store_l(slot, q, c, quads, plain)

        def comb26(q, pin):
            blocks = []
            for rr in (0, HM):
                rs = pl.ds(pl.multiple_of(r0 + rr + q + zero_s[0], 8), 8)
                mean, rstd = [jnp.concatenate([n_v[t, rr + q:rr + q + 8, :]] * 2, axis=1) for t in range(2)]
                blocks += [(src[rs, cc:cc + D4] - mean) * rstd for cc in range(0, D, D4)]
            vals = _run(UP, blocks)
            for k, u in enumerate(UL):
                lf_v[k, q:q + 8, :] = vals[u].astype(bf16)
        norms = [[(functools.partial(stats, rr + q), None, n_v, lag, 90) for rr in (0, HM)]
                 for q in range(0, HM, 16)]
        if slot is None:
            combs = [[(functools.partial(comb26, qq), n_v, lf_v, clag, 110) for qq in (q, q + 8)]
                     for q in range(0, HM, 16)]
        else:
            combs = [[(functools.partial(comb, q, c), n_v, l_v, clag, 125) for c in range(0, DH2, width)]
                     for q in range(0, HM, 16)]
        if staged:
            return sum(norms, []), sum(combs, [])
        out = list(norms[0])
        for a, b in zip(norms[1:] + [[]], combs):
            out += _merge(a, b) if a else b
        return out

    shifts = (1, 1, -1, -1, 2, 2, -2, -2)

    def shift_pieces(r0, slot, lag, by_value=False):
        def piece(q, j, pin):
            a = [h_v[jj, pl.ds(PAD + r0 + rr + q - shifts[jj], 16), :]
                 for rr in (0, HM) for jj in (j, j + NT // 2)]
            store_l(slot, q, j * 128, [pin(a[0]), a[1], a[2], pin(a[3])])
        return [(functools.partial(piece, q, j), None if by_value else h_v, l_v, lag, 50)
                for q in range(0, HM, 16) for j in range(NT // 2)]

    def lhs_of(slot):
        return lambda k: l_v[slot, k]

    h_v[:, 0:PAD, :] = jnp.zeros((NT, PAD, 128), f32)
    h_v[:, PAD + S:PAD + S + PAD, :] = jnp.zeros((NT, PAD, 128), f32)

    def store_h(r0, c0, h):
        for j in range(h.shape[1] // 128):
            h_v[c0 // 128 + j, PAD + r0:PAD + r0 + h.shape[0], :] = h[:, j * 128:(j + 1) * 128]

    def h_pieces(r0, c0, t, lag, n=4):
        def piece(r, pin):
            store_h(r0 + r, c0, _gelu(pin(t[r:r + 8 * n])))
        return [(functools.partial(piece, r), None, h_v, lag, 10 * n) for r in range(0, t.shape[0], 8 * n)]

    def flush(pieces):
        for p in pieces:
            p[0](lambda v, w=128: v)

    def w1_cols(c, step):
        half, cc = c // DH2, c % DH2
        return jnp.concatenate([s1_v[RAW1[half], :, cc:cc + step], s1_v[RAW1[2 + half], :, cc:cc + step]], axis=0)

    def d1_plain(xn, r0, c0, c1, step, side=None):
        for c in range(c0, c1, step):
            store_h(r0, c, _gelu(mm(xn, w1_cols(c, step), side)))

    def d1_fine(lhs, r0, nrb, cols, pieces, carry, skip=0):
        tiles = [(rb, c) for c in cols for rb in range(nrb)]
        rounds = [tiles[i:i + 4] for i in range(0, len(tiles), 4)]
        for n, (rnd, part) in enumerate(zip(rounds, split(pieces, len(rounds)))):
            sk = skip if n == 0 else 0
            side = Side(_merge(carry, part) if carry else part, 8 - sk, sk)
            carry = []
            for rb, c in rnd:
                half, cc = c // DH2, c % DH2
                t = mm(lhs(rb, 0), s1_v[RAW1[half], :, cc:cc + 128], side)
                t = mm(lhs(rb, 1), s1_v[RAW1[2 + half], :, cc:cc + 128], side, t)
                carry += h_pieces(r0 + rb * HM, c, t, LS)
        return carry

    CAP1 = (1, 1, 1, 1, 1, 1, 1)
    CAP2 = (2, 3, 3, 3, 3, 3, 2)

    def d1_s(b, slot, pieces, carry, early=()):
        for c, part, e in zip(range(0, DH2, NC1), split(pieces, DH2 // NC1), split(early, 2) + [[], []]):
            side = Side(merge(carry, part, e), CAP1 if hist else (0, 0) + CAP1[2:])
            cs = strassen(lhs_of(slot), lambda k: s1_v[k, :, c:c + NC1], side)
            carry = sum([h_pieces(b * TM + (q // 2) * HM, (q % 2) * DH2 + c, cs[q], LS) for q in (1, 2, 3, 0)], [])
        return carry

    def d2_s(b, slot, pieces, carry=(), early=()):
        for c, part, e in zip(range(0, DH2, NC1), split(pieces, DH2 // NC1), split(early, 2) + [[], []]):
            side = Side(merge(carry, part, e), CAP2 if hist else (0, 0) + CAP2[2:])
            carry = ()
            idx = [(slice(b * TM + (q // 2) * HM, b * TM + (q // 2 + 1) * HM),
                    slice((q % 2) * DH2 + c, (q % 2) * DH2 + c + NC1)) for q in range(4)]
            cs = strassen(lhs_of(slot), lambda k: s2_v[k, :, c:c + NC1], side,
                          [x_v[i].astype(f32) for i in idx])
            for i, t in zip(idx, cs):
                b_v[i] = t
                if b == 0:
                    c0_v[i] = t

    def split(l, n):
        w = [1.0 if hist else 0.6] + [1.0] * (n - 1)
        cut = [int(round(len(l) * sum(w[:i]) / sum(w))) for i in range(n + 1)]
        return [l[cut[i]:cut[i + 1]] for i in range(n)]

    def merge(*ls):
        ls = [l for l in ls if l]
        return _merge(*ls) if ls else []

    NW1, NW2, NW3 = 44, 0, 32
    LS, LL = 3, 5

    wait("x0")
    xn0 = _pack(_ln(x_v[0:TM, :].astype(f32)))
    wait("x1")
    xn01 = jnp.concatenate([xn0, _pack(_ln(x_v[TM:2 * TM, :].astype(f32)))], axis=0)
    wait("w1a")
    d1_plain(xn01, 0, 0, 256, 256)
    wait("w1bc")
    d1_plain(xn01, 0, 256, 768, 256)
    wait("w1d", "x234")
    hist.clear()
    carry = d1_fine(lambda rb, kh: xn01[rb * 64:(rb + 1) * 64, kh * DH2:(kh + 1) * DH2], 0, 4, (768, 896),
                    ln_pieces(x_v, 2 * TM, 0, LL, plain=True), [], 3)
    pw = prep_pieces(s1_v, RAW1, LS, by_value=True)
    carry = d1_fine(lambda rb, kh: l_v[0, 2 * rb + kh], 2 * TM, 2, range(0, D, 128),
                    _merge(pw[:NW1], ln_pieces(x_v, 3 * TM, 1, LL)), carry)
    carry = d1_s(3, 1, ln_pieces(x_v, 4 * TM, 0, LL), carry, pw[NW1:])
    wait("x567", "w2")
    qkv_start(0)
    qkv_start(1)
    hist.clear()
    pw = prep_pieces(s2_v, RAW, LS, by_value=True)
    for b in range(4, NB - 1):
        carry = d1_s(b, b % 2, merge(pw[(b - 4) * NW2:(b - 3) * NW2], ln_pieces(x_v, (b + 1) * TM, (b + 1) % 2, LL)), carry)
    carry = d1_s(7, 1, _merge(pw[3 * NW2:NW3], shift_pieces(0, 0, LS, True)), carry)
    d2_s(0, 0, shift_pieces(TM, 1, LS, True), carry, pw[NW3:])
    wait("w3")
    hist.clear()
    pw = _merge(prep26_pieces(s3_v, LS), ln_pieces(c0_v, 0, None, LL))
    pw = [pw[:37], pw[37:78], pw[78:119], pw[119:]]
    for b in range(1, 5):
        d2_s(b, b % 2, _merge(pw[b - 1], shift_pieces((b + 1) * TM, (b + 1) % 2, LS)))
    wait("w4", "small")
    hist.clear()
    pw = prep26_pieces(s4_v, LS)
    d2_s(5, 1, _merge(pw[:34], shift_pieces(6 * TM, 0, LS)))
    d2_s(6, 0, _merge(pw[34:68], shift_pieces(7 * TM, 1, LS)))
    d2_s(7, 1, pw[68:])
    start("wo", priority=1)

    def ffn(i, carry):
        qkv_wait(i)
        r0 = pl.multiple_of(i * TM, TM)
        rn = pl.multiple_of(jnp.minimum(i + 1, NB - 1) * TM, TM)
        acc = {}
        hist.clear()

        def relayout(p, r0_, r1_, pin):
            s0 = i * SPG + 2 * p
            for r in range(r0_, r1_, 8):
                e = wqkv_v[s0, r:r + 8, :]
                o = wqkv_v[s0 + 1, r:r + 8, :]
                wqkv_v[s0, r:r + 8, :] = (e & jnp.uint32(0xFFFF)) | (o << 16)
                wqkv_v[s0 + 1, r:r + 8, :] = (e >> 16) | (o & jnp.uint32(0xFFFF0000))

        relays = [(functools.partial(relayout, p, r, r + 32), wqkv_v, wqkv_v, 3, 35)
                  for p in range(SPG // 2) for r in range(0, D // 2, 32)]
        norms, combs = ln_pieces(b_v, rn, None, 5, staged=True, clag=3)

        def gate(q, pin):
            gw = gw_ref[...].astype(f32)
            x = pin(x_v[pl.ds(r0 + q, 16), :].astype(f32))
            t = functools.reduce(lambda a, b: a + b,
                                 [x[:, j * 128:(j + 1) * 128] * gw[j:j + 1, :] for j in range(NT)])
            g = jax.nn.sigmoid(jnp.sum(t, axis=-1, keepdims=True))
            g_v[pl.ds(r0 + q, 16), :] = jnp.broadcast_to(g, (16, 128))

        gates = [(functools.partial(gate, q), None, g_v, 5, 90) for q in range(0, TM, 16)]

        def extras(t, pin):
            jj, o = 2 * i + t // 2, 24 + 8 * (t % 2)
            xs = [pin(x_v[pl.ds(pl.multiple_of((jj + hh) * 64 + o, 8), 8), :].astype(f32)) for hh in (0, NPAIR // 2)]
            vals = _run(UP, [x[:, cc:cc + D4] for x in xs for cc in range(0, D, D4)])
            for k, u in enumerate(UL):
                xe_v[k, pl.ds(pl.multiple_of(i * 32 + t * 8, 8), 8), :] = vals[u].astype(bf16)

        xes = [(functools.partial(extras, t), None, xe_v, 3, 100) for t in range(4)]
        hs = {}

        def gelu_pieces(c, cs):
            def piece(r, cc, vs, pin):
                for v in vs:
                    hs[c, v, r, cc] = _gelu(pin(cs[v][r:r + 8, cc:cc + 128]))
                return [hs[c, v, r, cc] for v in vs]
            return [(functools.partial(piece, r, cc, vs), None, None, 3, 40) for r in range(0, HM, 8)
                    for cc in range(0, cs[0].shape[1], 128) for vs in ((0, 1, 2, 3), (4, 5, 6, 7))]

        def d3(c, side):
            c0, c1 = FCH[c]
            cs = fmm(lambda u: lf_v[UL.index(u)], lambda r: s3_v[r, :, c0:c1], side)
            assert not side.pieces
            return gelu_pieces(c, cs)

        def d4(c, side):
            c0, c1 = FCH[c]
            lh = _run(UP, [jnp.concatenate([jnp.concatenate(
                [hs.pop((c, v, r, cc)) for cc in range(0, c1 - c0, 128)], axis=1) for r in range(0, HM, 8)], axis=0)
                for v in range(8)])
            rhs = lambda r: s4_v[r, c0:c1, :]
            if c + 1 < len(FCH):
                for n in WORDER:
                    for r in range(RK):
                        if WN[r] == n:
                            acc[n] = mm(lh[UN[r]], rhs(r), side, acc.get(n))
            else:
                idx = lambda v: (pl.ds(r0 + (v // 4) * HM, HM), slice((v % 4) * D4, (v % 4 + 1) * D4))

                def extra(n):
                    if n >= 8:
                        return acc.get(n)
                    return b_v[idx(n)] + acc[n] if n in acc else b_v[idx(n)]

                def emit_b(v, t):
                    b_v[idx(v)] = jnp.concatenate([1.0 - g_v[idx(v)[0], :]] * 2, axis=1) * t
                fmm(lambda u: lh[u], rhs, side, extra, emit_b)
            assert not side.pieces

        g0 = d3(0, Side(relays[:20], 23, 3))
        g1 = d3(1, Side(_merge(g0, gates), 23, 2))
        d4(0, Side(g1[:22], 22, 4))
        g2 = d3(2, Side(_merge(g1[22:], relays[20:40]), 25))
        d4(1, Side(g2, 23, 2))
        g3 = d3(3, Side(_merge(relays[40:], norms, xes), 26))
        d4(2, Side(_merge(g3, combs), 23, 2))
        d4(3, Side([], 1))

        @pl.when(i + 2 < NG)
        def _():
            qkv_start(i + 2)

        return carry

    lax.fori_loop(0, NB, ffn, 0)

    def pre(it, carry):
        hist.clear()
        for u in range(3 * NG // NPRE):
            s0 = (it * (3 * NG // NPRE) + u) * G

            def rhs(r):
                t = None
                for q, sg in sorted(_terms(VP, 16, VN[r]).items(), key=lambda e: -e[1]):
                    blk = wqkv_v[s0 + q % 4 + zero_s[r], (q // 4) * (D // 8):(q // 4 + 1) * (D // 8), :]
                    if VN[r] < 16:
                        return blk
                    blk = _unpack(blk)
                    t = blk if t is None else (t + blk if sg > 0 else t - blk)
                return t.astype(bf16)
            for v, t in enumerate(fmm(lambda k: xe_v[UL.index(k)], rhs, None)):
                e_v[s0 + v % 4, (v // 4) * 128:(v // 4 + 1) * 128, :] = _pack(t)
        return carry

    lax.fori_loop(0, NPRE, pre, 0)

    wait("wo")
    mem_v[...] = mem0_ref[...].astype(f32)

    def slab(w, h):
        return (h // G) * SPG + w * G + h % G

    def step(j, hx, odd, late, allow, fill):
        qs, ks, vs, ps = {}, {}, {}, {}
        wload = lambda w, h: pltpu.bitcast(wqkv_v[slab(w, h)], bf16)
        eload = lambda w, h: pltpu.bitcast(e_v[slab(w, h), pl.ds(pl.multiple_of(j * 8, 8), 8), :], bf16)

        def proj(g):
            part = {}
            if late and g == 0:
                for h in range(2):
                    for w in range(3):
                        part[w, h] = _dot(hx[:, :DH2], wload(w, h)[:DH2])
            for h in range(g * G, (g + 1) * G):
                q, k, v = [(_dot(hx[:, DH2:], wload(w, h)[DH2:]) + part[w, h] if (w, h) in part
                            else _dot(hx, wload(w, h))).astype(bf16) for w in range(3)]
                if odd:
                    q = jnp.concatenate([q, eload(0, h)], axis=0)
                    k = jnp.concatenate([pltpu.bitcast(ke_v[h], bf16), eload(1, h), k], axis=0)
                    v = jnp.concatenate([pltpu.bitcast(ve_v[h], bf16), eload(2, h), v], axis=0)
                else:
                    ke_v[h] = pltpu.bitcast(k, u32)
                    ve_v[h] = pltpu.bitcast(v, u32)
                    k = jnp.concatenate([k, eload(1, h)], axis=0)
                    v = jnp.concatenate([v, eload(2, h)], axis=0)
                qs[h], ks[h], vs[h] = q, k, v

        def score(g):
            for h in range(g * G, (g + 1) * G):
                s = lax.dot_general(qs.pop(h), ks.pop(h), (((1,), (1,)), ((), ())),
                                    preferred_element_type=f32)
                ps[h] = _softmax(s, allow, fill)

        def pv(g):
            os_ = []
            for h in range(g * G, (g + 1) * G):
                o = _dot(ps.pop(h), vs.pop(h))
                o_v[:, h * 128:(h + 1) * 128] = _pack(o[:32])
                os_.append(o)
            if odd:
                quads = [jnp.concatenate([os_[2 * kk][r:r + 8], os_[2 * kk + 1][r:r + 8]], axis=1)
                         for r in (32, 40) for kk in range(2)]
                for k, t in enumerate(_lcombos(*quads)):
                    oe_v[k, pl.ds(pl.multiple_of(j * 8, 8), 8), g * 256:(g + 1) * 256] = t.astype(bf16)

        acc = [None] * NT

        def wo(h0, h1, j0, j1):
            o = pltpu.bitcast(o_v[:, h0 * 128:h1 * 128], bf16)
            for n in range(j0, j1):
                y = _dot(o, pltpu.bitcast(wo_v[n, h0 * 64:h1 * 64, :], bf16))
                acc[n] = y if acc[n] is None else y + acc[n]

        for t in range(NG):
            proj(t)
            if t >= 2:
                pv(t - 2)
            if t >= 1:
                score(t - 1)
        wo(0, 16, 0, 4)
        pv(NG - 2)
        score(NG - 1)
        wo(0, 16, 4, 8)
        pv(NG - 1)
        wo(16, 24, 0, 8)
        wo(24, 32, 0, 8)
        return jnp.concatenate(acc, axis=1)

    def emit(j, r0, o0, a):
        rs = pl.ds(r0 + o0, 24)
        g = jnp.concatenate([g_v[rs, :]] * NT, axis=1)
        out_v[j, o0:o0 + 24, :] = (g * a + b_v[rs, :]).astype(bf16)

    def pair(j, mem, late):
        r0 = pl.multiple_of(j * 64, 64)
        allow_e, fill_e, allow_o, fill_o = _masks()
        xa = x_v[pl.ds(r0 + 16, 8), :].astype(f32)
        xb = x_v[pl.ds(r0 + 40, 8), :].astype(f32)
        hx = jnp.concatenate([x_v[pl.ds(r0, 16), :], jnp.concatenate([xa, mem], 0).astype(bf16)], 0)
        oe = step(j, hx, False, late, allow_e, fill_e)
        emit(j, r0, 0, oe[:24])
        hx = jnp.concatenate([jnp.concatenate([oe[24:32], xb], 0).astype(bf16), x_v[pl.ds(r0 + 48, 16), :]], 0)
        oo = step(j, hx, True, True, allow_o, fill_o)
        emit(j, r0, 40, oo[8:])
        return oo[:8]

    def a_iter(it, carry):
        mem = mem_v[...]
        for t in range(PPI):
            mem = pair(it * PPI + t, mem, t > 0)
        mem_v[...] = mem
        for t in range(PPI):
            for o0 in (0, 40):
                idx = (it * PPI + t, pl.ds(o0, 24))
                pltpu.make_async_copy(out_v.at[idx], out_hbm.at[idx], sem_out).start()
        return carry

    lax.fori_loop(0, NPAIR // PPI, a_iter, 0)

    hist.clear()
    for n in range(NT // 2):
        quad = [lambda k, t=2 * n + q % 2, o=(q // 2) * 128: jnp.concatenate(
            [wo_v[t + zero_s[k], g * 256 + o:g * 256 + o + 128, :] for g in range(NG)], axis=0) for q in range(4)]
        cs = strassen(lambda k: oe_v[k], lambda k: _rcombo(k, *quad), None)
        cols = slice(n * 256, (n + 1) * 256)
        for half in range(2):
            t = jnp.concatenate(cs[2 * half:2 * half + 2], axis=1)
            o0 = 24 + half * 8
            for jj in range(NPAIR):
                rs = slice(jj * 64 + o0, jj * 64 + o0 + 8)
                g = jnp.concatenate([g_v[rs, :]] * 2, axis=1)
                out_v[jj, o0:o0 + 8, cols] = (g * t[jj * 8:jj * 8 + 8] + b_v[rs, cols]).astype(bf16)
        if n >= 2:
            idx = (slice(None), pl.ds(24, 16), pl.ds(0, 768) if n == 2 else pl.ds(768, 256))
            pltpu.make_async_copy(out_v.at[idx], out_hbm.at[idx], sem_out).start()
    pltpu.make_async_copy(out_v, out_hbm, sem_out).wait()


@functools.partial(jax.jit, static_argnames=("A_seg_len",))
def pallas_gated_mix__memory_aug_recurrent_mem_tr__mixer_s_mlp__prompt_kernel(
    A_x, A_mem0, A_Wq, A_Wk, A_Wv, A_Wo, A_seg_len, B_x, B_w1, B_w2, B_w3, B_w4, gate_w,
):
    assert A_seg_len == SEG
    assert A_x.shape == (1, S, D) and A_mem0.shape == (1, M, D)
    any_spec = pl.BlockSpec(memory_space=pl.ANY)
    out = pl.pallas_call(
        _kernel,
        out_shape=jax.ShapeDtypeStruct((NPAIR, 64, D), bf16),
        in_specs=[any_spec] * 11,
        out_specs=any_spec,
        scratch_shapes=[
            pltpu.VMEM((S, D), bf16),
            pltpu.VMEM((9, D // 4, D // 2), u32),
            pltpu.VMEM((7, D // 4, D // 2), u32),
            pltpu.VMEM((RK, D4, F4), bf16),
            pltpu.VMEM((RK, F4, D4), bf16),
            pltpu.VMEM((3 * H, D // 2, DH), u32),
            pltpu.VMEM((NT, H * DH // 2, 128), u32),
            pltpu.VMEM((NT, S + 2 * PAD, 128), f32),
            pltpu.VMEM((S, D), f32),
            pltpu.VMEM((TM, D), f32),
            pltpu.VMEM((2, 7, HM // 2, D // 2), u32),
            pltpu.VMEM((len(UL), HM, D4), bf16),
            pltpu.VMEM((2, TM, 128), f32),
            pltpu.VMEM((S, 128), f32),
            pltpu.VMEM((NPAIR, 64, D), bf16),
            pltpu.VMEM((len(UL), 8 * NPAIR, D4), bf16),
            pltpu.VMEM((3 * H, 8 * NPAIR, DH), u32),
            pltpu.VMEM((7, 8 * NPAIR, H * DH // 2), bf16),
            pltpu.VMEM((H, 16, 128), u32),
            pltpu.VMEM((H, 16, 128), u32),
            pltpu.VMEM((16, H * DH), u32),
            pltpu.VMEM((M, D), f32),
            pltpu.VMEM((M, D), bf16),
            pltpu.VMEM((NT, 128), bf16),
            pltpu.SMEM((RK,), jnp.int32),
            pltpu.SemaphoreType.DMA((NLOAD,)),
            pltpu.SemaphoreType.DMA((NG,)),
            pltpu.SemaphoreType.DMA,
        ],
        compiler_params=pltpu.CompilerParams(vmem_limit_bytes=126 * 1024 * 1024,
                                             disable_bounds_checks=True),
    )(
        A_x.reshape(S, D), A_mem0.reshape(M, D),
        A_Wq.reshape(D // 2, 2 * H, DH), A_Wk.reshape(D // 2, 2 * H, DH), A_Wv.reshape(D // 2, 2 * H, DH),
        A_Wo.reshape(H * DH, D), B_w1, B_w2, B_w3, B_w4, gate_w.reshape(NT, 128),
    )
    return out.reshape(1, S, D)
```

```python
import functools

import jax
import jax.numpy as jnp
from jax import lax
import jax.experimental.pallas as pl
import jax.experimental.pallas.tpu as pltpu

f32, bf16, u32 = jnp.float32, jnp.bfloat16, jnp.uint32

S, D, H, DH, M, SEG, F = 2048, 1024, 32, 128, 8, 32, 3584
SCALE = DH ** -0.5
NEG = -1000000000.0
EPS = 1e-05

TM = 256
NB = S // TM
HM = TM // 2
DH2 = D // 2
D4, F4 = D // 4, F // 4
FCH = ((0, 128), (128, 384), (384, 640), (640, 896))
NC1 = 128
NPAIR = S // (2 * SEG)
PPI = 2
NPRE = 4
G = 4
NG = H // G
PAD = 8
NT = D // 128
W3A = 192
NLOAD = 11
assert NB == NG

_dot = functools.partial(jnp.dot, preferred_element_type=f32)

UP = ((4, 1, 5, 1), (6, 1, 8, 1), (0, 1, 3, 1), (2, -1, 9, 1), (4, -1, 10, 1), (0, 1, 1, 1), (2, 1, 12, 1),
      (5, 1, 7, -1), (7, 1, 12, -1), (11, -1, 13, 1), (10, -1, 11, 1), (2, 1, 7, 1), (0, -1, 4, 1),
      (6, 1, 7, 1), (1, -1, 5, 1), (3, 1, 7, -1), (1, 1, 4, 1), (2, 1, 3, 1), (1, -1, 3, 1), (1, 1, 7, -1),
      (2, 1, 6, -1))
WP = ((0, -1, 3, 1), (4, 1, 6, -1), (1, 1, 8, 1), (5, 1, 10, 1), (4, -1, 7, 1), (0, -1, 9, -1),
      (11, 1, 12, 1), (6, 1, 7, -1), (2, 1, 5, -1), (0, -1, 7, -1), (9, 1, 11, -1), (2, 1, 13, 1),
      (5, 1, 13, 1), (2, -1, 3, 1), (5, 1, 6, 1), (0, 1, 4, 1), (2, 1, 7, 1), (1, 1, 2, 1), (1, 1, 5, 1),
      (3, 1, 7, 1), (2, 1, 6, 1))
VP = ((1, 1, 5, -1), (8, 1, 11, 1), (10, 1, 17, 1), (13, 1, 16, -1), (0, 1, 4, -1), (0, 1, 3, 1),
      (14, 1, 18, -1), (0, 1, 11, 1), (14, 1, 19, -1), (0, 1, 5, 1), (12, 1, 15, 1), (2, 1, 21, 1),
      (10, 1, 14, -1), (4, 1, 7, 1), (11, 1, 19, 1), (12, -1, 20, 1), (13, 1, 14, -1), (9, 1, 30, -1),
      (3, -1, 15, 1), (6, 1, 23, 1), (24, 1, 27, -1), (9, -1, 18, 1), (7, 1, 34, 1), (2, 1, 6, -1),
      (0, 1, 8, -1), (6, 1, 21, 1), (22, 1, 31, -1), (6, 1, 29, 1), (0, 1, 1, 1), (15, 1, 25, 1),
      (5, 1, 37, 1), (15, 1, 20, 1))
UN = (7, 27, 24, 17, 9, 22, 21, 2, 15, 11, 8, 25, 19, 28, 2, 23, 26, 20, 1, 18, 10, 28, 4, 13, 14, 16)
WN = (23, 17, 24, 10, 14, 7, 22, 19, 12, 18, 15, 25, 20, 5, 26, 0, 8, 2, 27, 11, 26, 9, 28, 21, 16, 5)
VN = (42, 47, 41, 5, 11, 43, 18, 28, 20, 23, 35, 19, 22, 46, 33, 26, 45, 36, 38, 25, 44, 40, 39, 21, 24, 32)
RK = len(UN)
UL = tuple(sorted(set(UN)))
VSTAGES = ((0, 6, 7, 12, 13, 14, 15, 21), (11, 17, 20, 22, 24, 25, 23, 2), (1, 5, 8, 9, 10, 16, 18, 19))
RAW16 = (1, 11, 17, 5, 8, 3, 9, 10, 0, 6, 7, 4, 12, 20, 22, 16)


def _run(prog, blocks):
    vals = list(blocks)
    for a, sa, b, sb in prog:
        vals.append(vals[a] + vals[b] if sa > 0 and sb > 0 else
                    vals[a] - vals[b] if sa > 0 else vals[b] - vals[a])
    return vals


def _terms(prog, nin, node):
    if node < nin:
        return {node: 1}
    a, sa, b, sb = prog[node - nin]
    out = {k: sa * v for k, v in _terms(prog, nin, a).items()}
    out.update({k: sb * v for k, v in _terms(prog, nin, b).items()})
    return out


for _b in range(16):
    _last = max(k for k, st in enumerate(VSTAGES) for r in st if _b in _terms(VP, 16, VN[r]))
    assert VN[RAW16[_b]] == _b or RAW16[_b] in VSTAGES[_last]
assert sorted(sum(VSTAGES, ())) == [r for r in range(RK) if VN[r] >= 16] and len(set(RAW16)) == 16

_WPAR = {n: [] for n in range(8 + len(WP))}
for _t, (_a, _sa, _b, _sb) in enumerate(WP):
    _WPAR[_a].append((8 + _t, _sa))
    _WPAR[_b].append((8 + _t, _sb))


def _worder():
    order = []

    def closure(n, acc):
        if n not in acc and n not in order:
            acc.add(n)
            for q, _ in _WPAR[n]:
                closure(q, acc)
        return acc

    def visit(n):
        if n not in order:
            for q, _ in _WPAR[n]:
                visit(q)
            order.append(n)
    while len([v for v in range(8) if v not in order]):
        visit(min((v for v in range(8) if v not in order), key=lambda v: len(closure(v, set()))))
    return tuple(order)


WORDER = _worder()


def _ln(x):
    m = jnp.mean(x, axis=-1, keepdims=True)
    xc = x - m
    v = jnp.mean(xc * xc, axis=-1, keepdims=True)
    return xc * lax.rsqrt(v + EPS)


_GC = 0.7978845608028654


def _gelu(x):
    h = 0.5 * x
    return h + h * jnp.tanh(x * (_GC + (_GC * 0.044715) * (x * x)))


def _unpack(u):
    return pltpu.bitcast(u, bf16).astype(f32)


def _pack(x):
    return pltpu.bitcast(x.astype(bf16), u32)


def _lcombos(a11, a12, a21, a22):
    return [a11 + a22, a21 + a22, a11, a22, a11 + a12, a21 - a11, a12 - a22]


def _merge(*lists):
    keyed = [((j + 0.5) / len(l), n, j, v) for n, l in enumerate(lists) for j, v in enumerate(l)]
    return [v for _, _, _, v in sorted(keyed, key=lambda t: t[:3])]


def _masks():
    r = lax.broadcasted_iota(jnp.int32, (32, 48), 0)
    c = lax.broadcasted_iota(jnp.int32, (32, 48), 1)
    exist_e = c < 40
    allow_e = exist_e & ((r >= 24) | ((c >= 24) & (c < 32)) | (c <= r))
    fill_e = jnp.where(exist_e, NEG, -jnp.inf).astype(f32)
    r = lax.broadcasted_iota(jnp.int32, (48, 80), 0)
    c = lax.broadcasted_iota(jnp.int32, (48, 80), 1)
    q_even = (r >= 32) & (r < 40)
    exist_o = (q_even & (c < 40)) | (~q_even & (c >= 40))
    ktok = jnp.where(c < 24, c, jnp.where(c < 48, c - 8, c - 16))
    qtok = jnp.where(r < 32, r + 32, r - 8)
    is_mem_key = ((c >= 24) & (c < 32)) | ((c >= 48) & (c < 56))
    allow_o = exist_o & (is_mem_key | (r < 8) | (ktok <= qtok))
    fill_o = jnp.where(exist_o, NEG, -jnp.inf).astype(f32)
    return allow_e, fill_e, allow_o, fill_o


def _rcombo(k, b11, b12, b21, b22):
    if k in (1, 4):
        return (b11 if k == 1 else b22)(k)
    a, b, sign = {0: (b11, b22, 1), 2: (b12, b22, -1), 3: (b21, b11, -1), 5: (b11, b12, 1), 6: (b21, b22, 1)}[k]
    a, b = _unpack(a(k)), _unpack(b(k))
    return (a + b if sign > 0 else a - b).astype(bf16)


def _softmax(s, allow, fill):
    s = jnp.where(allow, s * SCALE, fill)
    m = jnp.max(s, axis=-1, keepdims=True)
    e = jnp.exp(s - m)
    l = jnp.sum(e, axis=-1, keepdims=True)
    r = pl.reciprocal(l, approx=True)
    r = r * (2.0 - l * r)
    return (e * r).astype(bf16)


def _kernel(x_hbm, mem0_hbm, wq_hbm, wk_hbm, wv_hbm, wo_hbm, w1_hbm, w2_hbm, w3_hbm, w4_hbm,
            gw_hbm, out_hbm,
            x_v, s1_v, s2_v, s3_v, s4_v, wqkv_v, wo_v, h_v, b_v, c0_v, l_v, lf_v, n_v, g_v, out_v, xe_v, e_v, oe_v,
            ke_v, ve_v, o_v, mem_v, mem0_ref, gw_ref, zero_s,
            sem, sem_qkv, sem_out):
    RAW = (1, 2, 3, 4)
    RAW1 = (1, 7, 8, 4)

    loads = []

    def rows_load(name, r0, r1):
        loads.append((name, x_hbm.at[pl.ds(r0, r1 - r0)], x_v.at[pl.ds(r0, r1 - r0)]))

    def quad_load(name, w_hbm, s_v, raw, q, c0=0, c1=None):
        k4, n2 = s_v.shape[1], s_v.shape[2]
        c1 = n2 if c1 is None else c1
        src = w_hbm.bitcast(u32).at[pl.ds((q // 2) * k4, k4), pl.ds((q % 2) * n2 + c0, c1 - c0)]
        loads.append((name, src, s_v.at[raw[q], :, pl.ds(c0, c1 - c0)]))

    def w1_load(name, half, c0, c1):
        quad_load(name, w1_hbm, s1_v, RAW1, half, c0, c1)
        quad_load(name, w1_hbm, s1_v, RAW1, 2 + half, c0, c1)

    def block_load(name, w_hbm, s_v, r0, r1):
        kb, nb = s_v.shape[1:]
        for q in range(16):
            loads.append((name, w_hbm.at[pl.ds((q // 4) * kb + r0, r1 - r0), pl.ds((q % 4) * nb, nb)],
                          s_v.at[RAW16[q], pl.ds(r0, r1 - r0)]))

    rows_load("x0", 0, TM)
    w1_load("w1a", 0, 0, 256)
    w1_load("w1b", 0, 256, 512)
    rows_load("x1", TM, 2 * TM)
    w1_load("w1cd", 1, 0, 512)
    rows_load("x23", 2 * TM, 4 * TM)
    rows_load("x4567", 4 * TM, S)
    for q in range(4):
        quad_load("w2", w2_hbm, s2_v, RAW, q)
    block_load("w2", w3_hbm, s3_v, 0, W3A)
    block_load("w4", w3_hbm, s3_v, W3A, D4)
    block_load("w4", w4_hbm, s4_v, 0, F4)
    loads.append(("small", mem0_hbm, mem0_ref))
    loads.append(("small", gw_hbm, gw_ref))
    for j in range(NT):
        loads.append(("wo", wo_hbm.bitcast(u32).at[:, pl.ds(j * 128, 128)], wo_v.at[j]))
    groups = list(dict.fromkeys(name for name, _, _ in loads))
    assert len(groups) == NLOAD

    def start(*names, priority=0):
        for name, src, dst in loads:
            if name in names:
                pltpu.make_async_copy(src, dst, sem.at[groups.index(name)]).start(priority=priority)

    def wait(*names):
        for name, src, dst in loads:
            if name in names:
                pltpu.make_async_copy(src, dst, sem.at[groups.index(name)]).wait()

    SPG = 3 * G

    def qkv_start(g):
        for w, w_hbm in enumerate((wq_hbm, wk_hbm, wv_hbm)):
            wu = w_hbm.bitcast(u32)
            for k in range(G // 2):
                for par in range(2):
                    pltpu.make_async_copy(
                        wu.at[:, par * (H // 2) + g * (G // 2) + k, :],
                        wqkv_v.at[g * SPG + w * G + 2 * k + par], sem_qkv.at[g]).start(priority=1)

    def qkv_wait(g):
        grp = wqkv_v.at[pl.ds(g * SPG, SPG)]
        pltpu.make_async_copy(grp, grp, sem_qkv.at[g]).wait()

    start("x0", "w1a", "w1b", "x1", "w1cd", "x23", "x4567", "w2", "w4", "small")

    def zero(k, carry):
        zero_s[k] = 0
        return carry
    lax.fori_loop(0, RK, zero, 0)

    def tile_idx(ref, cols=128):
        z = zero_s[0]
        n = 16 if ref.dtype == bf16 and cols == 128 else 8
        return (z,) * (len(ref.shape) - 2) + (pl.ds(pl.multiple_of(z, n), n), slice(0, cols))

    rot = [0]
    ROT = 0
    hist = []

    def mm(lhs, rhs, side=None, acc=None):
        if side is not None:
            lhs = side(lhs)
        lhs = pltpu.bitcast(lhs, bf16) if lhs.dtype == u32 else lhs.astype(bf16)
        y = _dot(lhs, pltpu.bitcast(rhs, bf16) if rhs.dtype == u32 else rhs)
        if acc is not None:
            y = y + acc
        hist.append(y)
        return y

    class Side:
        def __init__(self, pieces, n, skip=0):
            cap = [0] * skip + ([1] * n if isinstance(n, int) else list(n))
            tot = sum(p[4] for p in pieces)
            self.plan = [[] for _ in cap]
            done = 0
            for p in pieces:
                done += p[4]
                x, d = done / tot * sum(cap), 0
                while x > cap[d] + 1e-9:
                    x -= cap[d]
                    d += 1
                self.plan[d].append((p, x / cap[d]))
            self.pieces = len(pieces)

        def __call__(self, val):
            todo = self.plan.pop(0) if self.plan else []
            if not todo:
                return val
            self.pieces -= len(todo)
            never = zero_s[0] > 0
            if val.dtype == bf16:
                val = pltpu.bitcast(val, u32)
            rg = 8 if val.dtype == u32 else 16
            ng = val.shape[0] // rg
            groups = [val[8 * m:8 * m + 8] for m in range(val.shape[0] // 8)]
            nk = val.shape[1] // 128
            npass = max(nk // 4, 1)
            for (fn, rd, wr, lag, _), pos in todo:
                sl = max(-int(-pos * ng * npass // 1) - 1, 0)
                m = sl % ng
                rot[0] += ROT
                kt = (sl // ng) * 4 + (rot[0] - 1) % min(nk, 4)
                pin = lambda v, w=128: v
                if lag is not None and len(hist) >= lag:
                    r0 = (16 * m) % hist[-lag].shape[0]
                    a = hist[-lag][r0:r0 + 8, :128]
                    if rd is None:
                        def pin(v, w=128, a=a):
                            a = jnp.concatenate([pltpu.bitcast(a, v.dtype)] * (v.shape[0] // 8), axis=0)
                            t = jnp.where(never, jnp.concatenate([a] * (w // 128), axis=1), v[:, :w])
                            return t if v.shape[1] == w else jnp.concatenate([t, v[:, w:]], axis=1)
                    elif rd.dtype == bf16:
                        idx = tile_idx(rd, 256)
                        rd[idx] = jnp.where(never, jnp.concatenate([a, a], axis=1).astype(bf16), rd[idx])
                    else:
                        idx = tile_idx(rd)
                        rd[idx] = jnp.where(never, pltpu.bitcast(a, rd.dtype), rd[idx])
                tiles = fn(pin)
                g = m * rg // 8
                ks = [groups[g][:, k * 128:(k + 1) * 128] for k in range(nk)]
                for u in (tiles if wr is None else [wr[tile_idx(wr)]]):
                    ks[kt] = jnp.where(never, pltpu.bitcast(u, val.dtype), ks[kt])
                groups[g] = jnp.concatenate(ks, axis=1)
            return jnp.concatenate(groups, axis=0)

    def strassen(lhs, rhs, side, init=(None, None, None, None)):
        def add(a, b):
            return a if b is None else a + b
        p = [mm(lhs(k), rhs(k), side) for k in range(5)]
        c12 = add(p[2] + p[4], init[1])
        c21 = add(p[1] + p[3], init[2])
        c22 = mm(lhs(5), rhs(5), side, add(p[0] - p[1] + p[2], init[3]))
        c11 = mm(lhs(6), rhs(6), side, add(p[0] + p[3] - p[4], init[0]))
        return c11, c12, c21, c22

    def fmm(lhs, rhs, side, extra=lambda n: None, emit=None):
        val = {}
        for n in WORDER:
            t = extra(n)
            for q, sg in sorted(_WPAR[n], key=lambda e: -e[1]):
                t = val[q] if t is None else (t + val[q] if sg > 0 else t - val[q])
            for r in range(RK):
                if WN[r] == n:
                    t = mm(lhs(UN[r]), rhs(r), side, t)
            val[n] = t
            if n < 8 and emit is not None:
                emit(n, t)
        return [val[v] for v in range(8)]

    def prep26_pieces(s_v, lag, stages=(sum(VSTAGES, ()),)):
        def piece(rs, cs, stage, pin):
            @functools.lru_cache(None)
            def node(n):
                if n < 16:
                    return s_v[RAW16[n], rs, cs].astype(f32)
                return _run([(0, VP[n - 16][1], 1, VP[n - 16][3])], [node(VP[n - 16][0]), node(VP[n - 16][2])])[-1]
            vals = [node(VN[r]).astype(bf16) for r in stage]
            for r, t in zip(stage, vals):
                s_v[r, rs, cs] = t
        kb, nb = s_v.shape[1:]
        out = []
        for r in range(0, kb, 16):
            out += [(slice(rr, rr + 8), slice(c, c + 256)) for c in range(0, nb - 255, 256) for rr in (r, r + 8)]
            out += [(slice(rr, rr + 8), slice(nb - 128, nb)) for rr in (r, r + 8)] if nb % 256 else []
        return [(functools.partial(piece, rs, cs, st), s_v, s_v, lag, 130 if cs.stop - cs.start == 256 else 100)
                for rs, cs in out for st in stages]

    def prep_pieces(s_v, raw, lag, width=256, by_value=False):
        def piece(r, c, pin):
            idx = (slice(r, r + 8), slice(c, c + width))
            b11, b12, b21, b22 = [_unpack(pin(s_v[(q,) + idx], width) if n in (0, 3) else s_v[(q,) + idx])
                                  for n, q in enumerate(raw)]
            for k, t in ((0, b11 + b22), (2, b12 - b22), (3, b21 - b11), (5, b11 + b12), (6, b21 + b22)):
                s_v[(k,) + idx] = _pack(t)
        return [(functools.partial(piece, r, c), None if by_value else s_v, s_v, lag, 80)
                for c in range(0, s_v.shape[2], width) for r in range(0, s_v.shape[1], 8)]

    def store_l(slot, q, c, quads, plain=False):
        for k, t in enumerate(quads if plain else _lcombos(*quads)):
            l_v[slot, k, q // 2:q // 2 + 8, c:c + t.shape[1]] = _pack(t)

    def ln_pieces(src, r0, slot, lag, plain=False, width=256, staged=False, clag=None):
        def stats(q, pin):
            x = pin(src[pl.ds(r0 + q, 16), :].astype(f32))
            xs = [x[:, j * 128:(j + 1) * 128] for j in range(NT)]
            m = functools.reduce(lambda a, b: a + b, xs) * (1.0 / NT)
            w = functools.reduce(lambda a, b: a + b, [(t - m) * (t - m) for t in xs])
            mean = jnp.mean(m, axis=-1, keepdims=True)
            var = jnp.sum(w + NT * ((m - mean) * (m - mean)), axis=-1, keepdims=True) * (1.0 / D)
            n_v[0, q:q + 16, :] = jnp.broadcast_to(mean, (16, 128))
            n_v[1, q:q + 16, :] = jnp.broadcast_to(lax.rsqrt(var + EPS), (16, 128))

        def comb(q, c, pin):
            quads = []
            for rr in (0, HM):
                rs = pl.ds(pl.multiple_of(r0 + rr + q + zero_s[0], 16), 16)
                mean, rstd = [jnp.concatenate([n_v[t, rr + q:rr + q + 16, :]] * (width // 128), axis=1)
                              for t in range(2)]
                quads += [(src[rs, cc + c:cc + c + width].astype(f32) - mean) * rstd for cc in (0, DH2)]
            store_l(slot, q, c, quads, plain)

        def comb26(q, pin):
            blocks = []
            for rr in (0, HM):
                rs = pl.ds(pl.multiple_of(r0 + rr + q + zero_s[0], 8), 8)
                mean, rstd = [jnp.concatenate([n_v[t, rr + q:rr + q + 8, :]] * 2, axis=1) for t in range(2)]
                blocks += [(src[rs, cc:cc + D4] - mean) * rstd for cc in range(0, D, D4)]
            vals = _run(UP, blocks)
            for k, u in enumerate(UL):
                lf_v[k, q:q + 8, :] = vals[u].astype(bf16)
        norms = [[(functools.partial(stats, rr + q), None, n_v, lag, 90) for rr in (0, HM)]
                 for q in range(0, HM, 16)]
        if slot is None:
            combs = [[(functools.partial(comb26, qq), n_v, lf_v, clag, 110) for qq in (q, q + 8)]
                     for q in range(0, HM, 16)]
        else:
            combs = [[(functools.partial(comb, q, c), n_v, l_v, clag, 125) for c in range(0, DH2, width)]
                     for q in range(0, HM, 16)]
        if staged:
            return sum(norms, []), sum(combs, [])
        out = list(norms[0])
        for a, b in zip(norms[1:] + [[]], combs):
            out += _merge(a, b) if a else b
        return out

    shifts = (1, 1, -1, -1, 2, 2, -2, -2)

    def shift_pieces(r0, slot, lag, by_value=False):
        def piece(q, j, pin):
            a = [h_v[jj, pl.ds(PAD + r0 + rr + q - shifts[jj], 16), :]
                 for rr in (0, HM) for jj in (j, j + NT // 2)]
            store_l(slot, q, j * 128, [pin(a[0]), a[1], a[2], pin(a[3])])
        return [(functools.partial(piece, q, j), None if by_value else h_v, l_v, lag, 50)
                for q in range(0, HM, 16) for j in range(NT // 2)]

    def lhs_of(slot):
        return lambda k: l_v[slot, k]

    h_v[:, 0:PAD, :] = jnp.zeros((NT, PAD, 128), f32)
    h_v[:, PAD + S:PAD + S + PAD, :] = jnp.zeros((NT, PAD, 128), f32)

    def store_h(r0, c0, h):
        for j in range(h.shape[1] // 128):
            h_v[c0 // 128 + j, PAD + r0:PAD + r0 + h.shape[0], :] = h[:, j * 128:(j + 1) * 128]

    def h_pieces(r0, c0, t, lag, n=4):
        def piece(r, pin):
            store_h(r0 + r, c0, _gelu(pin(t[r:r + 8 * n])))
        return [(functools.partial(piece, r), None, h_v, lag, 10 * n) for r in range(0, t.shape[0], 8 * n)]

    def flush(pieces):
        for p in pieces:
            p[0](lambda v, w=128: v)

    def w1_cols(c, step):
        half, cc = c // DH2, c % DH2
        return jnp.concatenate([s1_v[RAW1[half], :, cc:cc + step], s1_v[RAW1[2 + half], :, cc:cc + step]], axis=0)

    def d1_plain(xn, r0, c0, c1, step, side=None):
        for c in range(c0, c1, step):
            store_h(r0, c, _gelu(mm(xn, w1_cols(c, step), side)))

    def d1_fine(lhs, r0, nrb, cols, pieces, carry, skip=0):
        tiles = [(rb, c) for c in cols for rb in range(nrb)]
        rounds = [tiles[i:i + 4] for i in range(0, len(tiles), 4)]
        for n, (rnd, part) in enumerate(zip(rounds, split(pieces, len(rounds)))):
            sk = skip if n == 0 else 0
            side = Side(_merge(carry, part) if carry else part, 8 - sk, sk)
            carry = []
            for rb, c in rnd:
                half, cc = c // DH2, c % DH2
                t = mm(lhs(rb, 0), s1_v[RAW1[half], :, cc:cc + 128], side)
                t = mm(lhs(rb, 1), s1_v[RAW1[2 + half], :, cc:cc + 128], side, t)
                carry += h_pieces(r0 + rb * HM, c, t, LS)
        return carry

    CAP1 = (1, 1, 1, 1, 1, 1, 1)
    CAP2 = (2, 3, 3, 3, 3, 3, 2)

    def d1_s(b, slot, pieces, carry, early=()):
        for c, part, e in zip(range(0, DH2, NC1), split(pieces, DH2 // NC1), split(early, 2) + [[], []]):
            side = Side(merge(carry, part, e), CAP1 if hist else (0, 0) + CAP1[2:])
            cs = strassen(lhs_of(slot), lambda k: s1_v[k, :, c:c + NC1], side)
            carry = sum([h_pieces(b * TM + (q // 2) * HM, (q % 2) * DH2 + c, cs[q], LS) for q in (1, 2, 3, 0)], [])
        return carry

    def d2_s(b, slot, pieces, carry=(), early=(), late=()):
        for c, part, e in zip(range(0, DH2, NC1), split(pieces, DH2 // NC1), split(early, 2) + split(late, 2)):
            side = Side(merge(carry, part, e), CAP2 if hist else (0, 0) + CAP2[2:])
            carry = ()
            idx = [(slice(b * TM + (q // 2) * HM, b * TM + (q // 2 + 1) * HM),
                    slice((q % 2) * DH2 + c, (q % 2) * DH2 + c + NC1)) for q in range(4)]
            cs = strassen(lhs_of(slot), lambda k: s2_v[k, :, c:c + NC1], side,
                          [x_v[i].astype(f32) for i in idx])
            for i, t in zip(idx, cs):
                b_v[i] = t
                if b == 0:
                    c0_v[i] = t

    def split(l, n):
        w = [1.0 if hist else 0.6] + [1.0] * (n - 1)
        cut = [int(round(len(l) * sum(w[:i]) / sum(w))) for i in range(n + 1)]
        return [l[cut[i]:cut[i + 1]] for i in range(n)]

    def merge(*ls):
        ls = [l for l in ls if l]
        return _merge(*ls) if ls else []

    NW1, NW3, N30 = 44, 32, 16
    LS, LL = 3, 5

    wait("x0")
    xn0 = _pack(_ln(x_v[0:TM, :].astype(f32)))
    wait("w1a")
    d1_plain(xn0, 0, 0, 256, 256)
    wait("w1b")
    d1_plain(xn0, 0, 256, 512, 256)
    wait("x1")
    xn1 = _pack(_ln(x_v[TM:2 * TM, :].astype(f32)))
    d1_plain(xn1, TM, 0, 512, 256)
    wait("w1cd")
    xn01 = jnp.concatenate([xn0, xn1], axis=0)
    d1_plain(xn01, 0, 512, 768, 256)
    wait("x23")
    hist.clear()
    carry = d1_fine(lambda rb, kh: xn01[rb * 64:(rb + 1) * 64, kh * DH2:(kh + 1) * DH2], 0, 4, (768, 896),
                    ln_pieces(x_v, 2 * TM, 0, LL, plain=True), [], 3)
    pw = prep_pieces(s1_v, RAW1, LS, by_value=True)
    carry = d1_fine(lambda rb, kh: l_v[0, 2 * rb + kh], 2 * TM, 2, range(0, D, 128),
                    _merge(pw[:NW1], ln_pieces(x_v, 3 * TM, 1, LL)), carry)
    wait("x4567")
    qkv_start(0)
    qkv_start(1)
    hist.clear()
    for b in range(3, NB - 1):
        carry = d1_s(b, b % 2, ln_pieces(x_v, (b + 1) * TM, (b + 1) % 2, LL), carry, pw[NW1:] if b == 3 else ())
    wait("w2")
    hist.clear()
    pw = prep_pieces(s2_v, RAW, LS, by_value=True)
    p3 = prep26_pieces(s3_v, LS)
    n3 = len(p3) * W3A // D4
    carry = d1_s(7, 1, _merge(pw[:NW3], shift_pieces(0, 0, LS, True)), carry)
    d2_s(0, 0, shift_pieces(TM, 1, LS, True), carry, pw[NW3:], p3[:N30])
    pw = split(_merge(p3[N30:n3], ln_pieces(c0_v, 0, None, LL)), 3)
    for b in range(1, 4):
        d2_s(b, b % 2, _merge(pw[b - 1], shift_pieces((b + 1) * TM, (b + 1) % 2, LS)))
    wait("w4", "small")
    hist.clear()
    pw = p3[n3:] + prep26_pieces(s4_v, LS)
    cut = (0, 31, 65, 99, len(pw))
    for b in range(4, NB):
        d2_s(b, b % 2, merge(pw[cut[b - 4]:cut[b - 3]],
                             shift_pieces((b + 1) * TM, (b + 1) % 2, LS) if b + 1 < NB else ()))
    start("wo", priority=1)

    def ffn(i, carry):
        qkv_wait(i)
        r0 = pl.multiple_of(i * TM, TM)
        rn = pl.multiple_of(jnp.minimum(i + 1, NB - 1) * TM, TM)
        acc = {}
        hist.clear()

        def relayout(p, r0_, r1_, pin):
            s0 = i * SPG + 2 * p
            for r in range(r0_, r1_, 8):
                e = wqkv_v[s0, r:r + 8, :]
                o = wqkv_v[s0 + 1, r:r + 8, :]
                wqkv_v[s0, r:r + 8, :] = (e & jnp.uint32(0xFFFF)) | (o << 16)
                wqkv_v[s0 + 1, r:r + 8, :] = (e >> 16) | (o & jnp.uint32(0xFFFF0000))

        relays = [(functools.partial(relayout, p, r, r + 32), wqkv_v, wqkv_v, 3, 35)
                  for p in range(SPG // 2) for r in range(0, D // 2, 32)]
        norms, combs = ln_pieces(b_v, rn, None, 5, staged=True, clag=3)

        def gate(q, pin):
            gw = gw_ref[...].astype(f32)
            x = pin(x_v[pl.ds(r0 + q, 16), :].astype(f32))
            t = functools.reduce(lambda a, b: a + b,
                                 [x[:, j * 128:(j + 1) * 128] * gw[j:j + 1, :] for j in range(NT)])
            g = jax.nn.sigmoid(jnp.sum(t, axis=-1, keepdims=True))
            g_v[pl.ds(r0 + q, 16), :] = jnp.broadcast_to(g, (16, 128))

        gates = [(functools.partial(gate, q), None, g_v, 5, 90) for q in range(0, TM, 16)]

        def extras(t, pin):
            jj, o = 2 * i + t // 2, 24 + 8 * (t % 2)
            xs = [pin(x_v[pl.ds(pl.multiple_of((jj + hh) * 64 + o, 8), 8), :].astype(f32)) for hh in (0, NPAIR // 2)]
            vals = _run(UP, [x[:, cc:cc + D4] for x in xs for cc in range(0, D, D4)])
            for k, u in enumerate(UL):
                xe_v[k, pl.ds(pl.multiple_of(i * 32 + t * 8, 8), 8), :] = vals[u].astype(bf16)

        xes = [(functools.partial(extras, t), None, xe_v, 3, 100) for t in range(4)]
        hs = {}

        def gelu_pieces(c, cs):
            def piece(r, cc, vs, pin):
                for v in vs:
                    hs[c, v, r, cc] = _gelu(pin(cs[v][r:r + 8, cc:cc + 128]))
                return [hs[c, v, r, cc] for v in vs]
            return [(functools.partial(piece, r, cc, vs), None, None, 3, 40) for r in range(0, HM, 8)
                    for cc in range(0, cs[0].shape[1], 128) for vs in ((0, 1, 2, 3), (4, 5, 6, 7))]

        def d3(c, side):
            c0, c1 = FCH[c]
            cs = fmm(lambda u: lf_v[UL.index(u)], lambda r: s3_v[r, :, c0:c1], side)
            assert not side.pieces
            return gelu_pieces(c, cs)

        def d4(c, side):
            c0, c1 = FCH[c]
            lh = _run(UP, [jnp.concatenate([jnp.concatenate(
                [hs.pop((c, v, r, cc)) for cc in range(0, c1 - c0, 128)], axis=1) for r in range(0, HM, 8)], axis=0)
                for v in range(8)])
            rhs = lambda r: s4_v[r, c0:c1, :]
            if c + 1 < len(FCH):
                for n in WORDER:
                    for r in range(RK):
                        if WN[r] == n:
                            acc[n] = mm(lh[UN[r]], rhs(r), side, acc.get(n))
            else:
                idx = lambda v: (pl.ds(r0 + (v // 4) * HM, HM), slice((v % 4) * D4, (v % 4 + 1) * D4))

                def extra(n):
                    if n >= 8:
                        return acc.get(n)
                    return b_v[idx(n)] + acc[n] if n in acc else b_v[idx(n)]

                def emit_b(v, t):
                    b_v[idx(v)] = jnp.concatenate([1.0 - g_v[idx(v)[0], :]] * 2, axis=1) * t
                fmm(lambda u: lh[u], rhs, side, extra, emit_b)
            assert not side.pieces

        g0 = d3(0, Side(relays[:20], 23, 3))
        g1 = d3(1, Side(_merge(g0, gates), 23, 2))
        d4(0, Side(g1[:22], 22, 4))
        g2 = d3(2, Side(_merge(g1[22:], relays[20:40]), 25))
        d4(1, Side(g2, 23, 2))
        g3 = d3(3, Side(_merge(relays[40:], norms, xes), 26))
        d4(2, Side(_merge(g3, combs), 23, 2))
        d4(3, Side([], 1))

        @pl.when(i + 2 < NG)
        def _():
            qkv_start(i + 2)

        return carry

    lax.fori_loop(0, NB, ffn, 0)

    def pre(it, carry):
        hist.clear()
        for u in range(3 * NG // NPRE):
            s0 = (it * (3 * NG // NPRE) + u) * G

            def rhs(r):
                t = None
                for q, sg in sorted(_terms(VP, 16, VN[r]).items(), key=lambda e: -e[1]):
                    blk = wqkv_v[s0 + q % 4 + zero_s[r], (q // 4) * (D // 8):(q // 4 + 1) * (D // 8), :]
                    if VN[r] < 16:
                        return blk
                    blk = _unpack(blk)
                    t = blk if t is None else (t + blk if sg > 0 else t - blk)
                return t.astype(bf16)
            for v, t in enumerate(fmm(lambda k: xe_v[UL.index(k)], rhs, None)):
                e_v[s0 + v % 4, (v // 4) * 128:(v // 4 + 1) * 128, :] = _pack(t)
        return carry

    lax.fori_loop(0, NPRE, pre, 0)

    wait("wo")
    mem_v[...] = mem0_ref[...].astype(f32)

    def slab(w, h):
        return (h // G) * SPG + w * G + h % G

    def step(j, hx, odd, late, allow, fill):
        qs, ks, vs, ps = {}, {}, {}, {}
        wload = lambda w, h: pltpu.bitcast(wqkv_v[slab(w, h)], bf16)
        eload = lambda w, h: pltpu.bitcast(e_v[slab(w, h), pl.ds(pl.multiple_of(j * 8, 8), 8), :], bf16)

        def proj(g):
            part = {}
            if late and g == 0:
                for h in range(2):
                    for w in range(3):
                        part[w, h] = _dot(hx[:, :DH2], wload(w, h)[:DH2])
            for h in range(g * G, (g + 1) * G):
                q, k, v = [(_dot(hx[:, DH2:], wload(w, h)[DH2:]) + part[w, h] if (w, h) in part
                            else _dot(hx, wload(w, h))).astype(bf16) for w in range(3)]
                if odd:
                    q = jnp.concatenate([q, eload(0, h)], axis=0)
                    k = jnp.concatenate([pltpu.bitcast(ke_v[h], bf16), eload(1, h), k], axis=0)
                    v = jnp.concatenate([pltpu.bitcast(ve_v[h], bf16), eload(2, h), v], axis=0)
                else:
                    ke_v[h] = pltpu.bitcast(k, u32)
                    ve_v[h] = pltpu.bitcast(v, u32)
                    k = jnp.concatenate([k, eload(1, h)], axis=0)
                    v = jnp.concatenate([v, eload(2, h)], axis=0)
                qs[h], ks[h], vs[h] = q, k, v

        def score(g):
            for h in range(g * G, (g + 1) * G):
                s = lax.dot_general(qs.pop(h), ks.pop(h), (((1,), (1,)), ((), ())),
                                    preferred_element_type=f32)
                ps[h] = _softmax(s, allow, fill)

        def pv(g):
            os_ = []
            for h in range(g * G, (g + 1) * G):
                o = _dot(ps.pop(h), vs.pop(h))
                o_v[:, h * 128:(h + 1) * 128] = _pack(o[:32])
                os_.append(o)
            if odd:
                quads = [jnp.concatenate([os_[2 * kk][r:r + 8], os_[2 * kk + 1][r:r + 8]], axis=1)
                         for r in (32, 40) for kk in range(2)]
                for k, t in enumerate(_lcombos(*quads)):
                    oe_v[k, pl.ds(pl.multiple_of(j * 8, 8), 8), g * 256:(g + 1) * 256] = t.astype(bf16)

        acc = [None] * NT

        def wo(h0, h1, j0, j1):
            o = pltpu.bitcast(o_v[:, h0 * 128:h1 * 128], bf16)
            for n in range(j0, j1):
                y = _dot(o, pltpu.bitcast(wo_v[n, h0 * 64:h1 * 64, :], bf16))
                acc[n] = y if acc[n] is None else y + acc[n]

        for t in range(NG):
            proj(t)
            if t >= 2:
                pv(t - 2)
            if t >= 1:
                score(t - 1)
        wo(0, 16, 0, 4)
        pv(NG - 2)
        score(NG - 1)
        wo(0, 16, 4, 8)
        pv(NG - 1)
        wo(16, 24, 0, 8)
        wo(24, 32, 0, 8)
        return jnp.concatenate(acc, axis=1)

    def emit(j, r0, o0, a):
        rs = pl.ds(r0 + o0, 24)
        g = jnp.concatenate([g_v[rs, :]] * NT, axis=1)
        out_v[j, o0:o0 + 24, :] = (g * a + b_v[rs, :]).astype(bf16)

    def pair(j, mem, late):
        r0 = pl.multiple_of(j * 64, 64)
        allow_e, fill_e, allow_o, fill_o = _masks()
        xa = x_v[pl.ds(r0 + 16, 8), :].astype(f32)
        xb = x_v[pl.ds(r0 + 40, 8), :].astype(f32)
        hx = jnp.concatenate([x_v[pl.ds(r0, 16), :], jnp.concatenate([xa, mem], 0).astype(bf16)], 0)
        oe = step(j, hx, False, late, allow_e, fill_e)
        emit(j, r0, 0, oe[:24])
        hx = jnp.concatenate([jnp.concatenate([oe[24:32], xb], 0).astype(bf16), x_v[pl.ds(r0 + 48, 16), :]], 0)
        oo = step(j, hx, True, True, allow_o, fill_o)
        emit(j, r0, 40, oo[8:])
        return oo[:8]

    def a_iter(it, carry):
        mem = mem_v[...]
        for t in range(PPI):
            mem = pair(it * PPI + t, mem, t > 0)
        mem_v[...] = mem
        for t in range(PPI):
            for o0 in (0, 40):
                idx = (it * PPI + t, pl.ds(o0, 24))
                pltpu.make_async_copy(out_v.at[idx], out_hbm.at[idx], sem_out).start()
        return carry

    lax.fori_loop(0, NPAIR // PPI, a_iter, 0)

    hist.clear()
    for n in range(NT // 2):
        quad = [lambda k, t=2 * n + q % 2, o=(q // 2) * 128: jnp.concatenate(
            [wo_v[t + zero_s[k], g * 256 + o:g * 256 + o + 128, :] for g in range(NG)], axis=0) for q in range(4)]
        cs = strassen(lambda k: oe_v[k], lambda k: _rcombo(k, *quad), None)
        cols = slice(n * 256, (n + 1) * 256)
        for half in range(2):
            t = jnp.concatenate(cs[2 * half:2 * half + 2], axis=1)
            o0 = 24 + half * 8
            for jj in range(NPAIR):
                rs = slice(jj * 64 + o0, jj * 64 + o0 + 8)
                g = jnp.concatenate([g_v[rs, :]] * 2, axis=1)
                out_v[jj, o0:o0 + 8, cols] = (g * t[jj * 8:jj * 8 + 8] + b_v[rs, cols]).astype(bf16)
        if n >= 2:
            idx = (slice(None), pl.ds(24, 16), pl.ds(0, 768) if n == 2 else pl.ds(768, 256))
            pltpu.make_async_copy(out_v.at[idx], out_hbm.at[idx], sem_out).start()
    pltpu.make_async_copy(out_v, out_hbm, sem_out).wait()


@functools.partial(jax.jit, static_argnames=("A_seg_len",))
def pallas_gated_mix__memory_aug_recurrent_mem_tr__mixer_s_mlp__prompt_kernel(
    A_x, A_mem0, A_Wq, A_Wk, A_Wv, A_Wo, A_seg_len, B_x, B_w1, B_w2, B_w3, B_w4, gate_w,
):
    assert A_seg_len == SEG
    assert A_x.shape == (1, S, D) and A_mem0.shape == (1, M, D)
    any_spec = pl.BlockSpec(memory_space=pl.ANY)
    out = pl.pallas_call(
        _kernel,
        out_shape=jax.ShapeDtypeStruct((NPAIR, 64, D), bf16),
        in_specs=[any_spec] * 11,
        out_specs=any_spec,
        scratch_shapes=[
            pltpu.VMEM((S, D), bf16),
            pltpu.VMEM((9, D // 4, D // 2), u32),
            pltpu.VMEM((7, D // 4, D // 2), u32),
            pltpu.VMEM((RK, D4, F4), bf16),
            pltpu.VMEM((RK, F4, D4), bf16),
            pltpu.VMEM((3 * H, D // 2, DH), u32),
            pltpu.VMEM((NT, H * DH // 2, 128), u32),
            pltpu.VMEM((NT, S + 2 * PAD, 128), f32),
            pltpu.VMEM((S, D), f32),
            pltpu.VMEM((TM, D), f32),
            pltpu.VMEM((2, 7, HM // 2, D // 2), u32),
            pltpu.VMEM((len(UL), HM, D4), bf16),
            pltpu.VMEM((2, TM, 128), f32),
            pltpu.VMEM((S, 128), f32),
            pltpu.VMEM((NPAIR, 64, D), bf16),
            pltpu.VMEM((len(UL), 8 * NPAIR, D4), bf16),
            pltpu.VMEM((3 * H, 8 * NPAIR, DH), u32),
            pltpu.VMEM((7, 8 * NPAIR, H * DH // 2), bf16),
            pltpu.VMEM((H, 16, 128), u32),
            pltpu.VMEM((H, 16, 128), u32),
            pltpu.VMEM((16, H * DH), u32),
            pltpu.VMEM((M, D), f32),
            pltpu.VMEM((M, D), bf16),
            pltpu.VMEM((NT, 128), bf16),
            pltpu.SMEM((RK,), jnp.int32),
            pltpu.SemaphoreType.DMA((NLOAD,)),
            pltpu.SemaphoreType.DMA((NG,)),
            pltpu.SemaphoreType.DMA,
        ],
        compiler_params=pltpu.CompilerParams(vmem_limit_bytes=126 * 1024 * 1024,
                                             disable_bounds_checks=True),
    )(
        A_x.reshape(S, D), A_mem0.reshape(M, D),
        A_Wq.reshape(D // 2, 2 * H, DH), A_Wk.reshape(D // 2, 2 * H, DH), A_Wv.reshape(D // 2, 2 * H, DH),
        A_Wo.reshape(H * DH, D), B_w1, B_w2, B_w3, B_w4, gate_w.reshape(NT, 128),
    )
    return out.reshape(1, S, D)
```

```python
import functools

import jax
import jax.numpy as jnp
from jax import lax
import jax.experimental.pallas as pl
import jax.experimental.pallas.tpu as pltpu

f32, bf16, u32 = jnp.float32, jnp.bfloat16, jnp.uint32

S, D, H, DH, M, SEG, F = 2048, 1024, 32, 128, 8, 32, 3584
SCALE = DH ** -0.5
NEG = -1000000000.0
EPS = 1e-05

TM = 256
NB = S // TM
HM = TM // 2
DH2 = D // 2
D4, F4 = D // 4, F // 4
FCH = ((0, 128), (128, 384), (384, 640), (640, 896))
NC1 = 128
NPAIR = S // (2 * SEG)
PPI = 2
NPRE = 4
G = 4
NG = H // G
PAD = 8
NT = D // 128
W3A = 192
NLOAD = 11
assert NB == NG

_dot = functools.partial(jnp.dot, preferred_element_type=f32)

UP = ((4, 1, 5, 1), (6, 1, 8, 1), (0, 1, 3, 1), (2, -1, 9, 1), (4, -1, 10, 1), (0, 1, 1, 1), (2, 1, 12, 1),
      (5, 1, 7, -1), (7, 1, 12, -1), (11, -1, 13, 1), (10, -1, 11, 1), (2, 1, 7, 1), (0, -1, 4, 1),
      (6, 1, 7, 1), (1, -1, 5, 1), (3, 1, 7, -1), (1, 1, 4, 1), (2, 1, 3, 1), (1, -1, 3, 1), (1, 1, 7, -1),
      (2, 1, 6, -1))
WP = ((0, -1, 3, 1), (4, 1, 6, -1), (1, 1, 8, 1), (5, 1, 10, 1), (4, -1, 7, 1), (0, -1, 9, -1),
      (11, 1, 12, 1), (6, 1, 7, -1), (2, 1, 5, -1), (0, -1, 7, -1), (9, 1, 11, -1), (2, 1, 13, 1),
      (5, 1, 13, 1), (2, -1, 3, 1), (5, 1, 6, 1), (0, 1, 4, 1), (2, 1, 7, 1), (1, 1, 2, 1), (1, 1, 5, 1),
      (3, 1, 7, 1), (2, 1, 6, 1))
VP = ((1, 1, 5, -1), (8, 1, 11, 1), (10, 1, 17, 1), (13, 1, 16, -1), (0, 1, 4, -1), (0, 1, 3, 1),
      (14, 1, 18, -1), (0, 1, 11, 1), (14, 1, 19, -1), (0, 1, 5, 1), (12, 1, 15, 1), (2, 1, 21, 1),
      (10, 1, 14, -1), (4, 1, 7, 1), (11, 1, 19, 1), (12, -1, 20, 1), (13, 1, 14, -1), (9, 1, 30, -1),
      (3, -1, 15, 1), (6, 1, 23, 1), (24, 1, 27, -1), (9, -1, 18, 1), (7, 1, 34, 1), (2, 1, 6, -1),
      (0, 1, 8, -1), (6, 1, 21, 1), (22, 1, 31, -1), (6, 1, 29, 1), (0, 1, 1, 1), (15, 1, 25, 1),
      (5, 1, 37, 1), (15, 1, 20, 1))
UN = (7, 27, 24, 17, 9, 22, 21, 2, 15, 11, 8, 25, 19, 28, 2, 23, 26, 20, 1, 18, 10, 28, 4, 13, 14, 16)
WN = (23, 17, 24, 10, 14, 7, 22, 19, 12, 18, 15, 25, 20, 5, 26, 0, 8, 2, 27, 11, 26, 9, 28, 21, 16, 5)
VN = (42, 47, 41, 5, 11, 43, 18, 28, 20, 23, 35, 19, 22, 46, 33, 26, 45, 36, 38, 25, 44, 40, 39, 21, 24, 32)
RK = len(UN)
UL = tuple(sorted(set(UN)))
VSTAGES = ((0, 6, 7, 12, 13, 14, 15, 21), (11, 17, 20, 22, 24, 25, 23, 2), (1, 5, 8, 9, 10, 16, 18, 19))
RAW16 = (1, 11, 17, 5, 8, 3, 9, 10, 0, 6, 7, 4, 12, 20, 22, 16)


def _run(prog, blocks):
    vals = list(blocks)
    for a, sa, b, sb in prog:
        vals.append(vals[a] + vals[b] if sa > 0 and sb > 0 else
                    vals[a] - vals[b] if sa > 0 else vals[b] - vals[a])
    return vals


def _terms(prog, nin, node):
    if node < nin:
        return {node: 1}
    a, sa, b, sb = prog[node - nin]
    out = {k: sa * v for k, v in _terms(prog, nin, a).items()}
    out.update({k: sb * v for k, v in _terms(prog, nin, b).items()})
    return out


for _b in range(16):
    _last = max(k for k, st in enumerate(VSTAGES) for r in st if _b in _terms(VP, 16, VN[r]))
    assert VN[RAW16[_b]] == _b or RAW16[_b] in VSTAGES[_last]
assert sorted(sum(VSTAGES, ())) == [r for r in range(RK) if VN[r] >= 16] and len(set(RAW16)) == 16

_WPAR = {n: [] for n in range(8 + len(WP))}
for _t, (_a, _sa, _b, _sb) in enumerate(WP):
    _WPAR[_a].append((8 + _t, _sa))
    _WPAR[_b].append((8 + _t, _sb))


def _worder():
    order = []

    def closure(n, acc):
        if n not in acc and n not in order:
            acc.add(n)
            for q, _ in _WPAR[n]:
                closure(q, acc)
        return acc

    def visit(n):
        if n not in order:
            for q, _ in _WPAR[n]:
                visit(q)
            order.append(n)
    while len([v for v in range(8) if v not in order]):
        visit(min((v for v in range(8) if v not in order), key=lambda v: len(closure(v, set()))))
    return tuple(order)


WORDER = _worder()


def _ln(x):
    m = jnp.mean(x, axis=-1, keepdims=True)
    xc = x - m
    v = jnp.mean(xc * xc, axis=-1, keepdims=True)
    return xc * lax.rsqrt(v + EPS)


_GC = 0.7978845608028654


def _gelu(x):
    h = 0.5 * x
    return h + h * jnp.tanh(x * (_GC + (_GC * 0.044715) * (x * x)))


def _unpack(u):
    return pltpu.bitcast(u, bf16).astype(f32)


def _pack(x):
    return pltpu.bitcast(x.astype(bf16), u32)


def _lcombos(a11, a12, a21, a22):
    return [a11 + a22, a21 + a22, a11, a22, a11 + a12, a21 - a11, a12 - a22]


def _merge(*lists):
    keyed = [((j + 0.5) / len(l), n, j, v) for n, l in enumerate(lists) for j, v in enumerate(l)]
    return [v for _, _, _, v in sorted(keyed, key=lambda t: t[:3])]


def _masks():
    r = lax.broadcasted_iota(jnp.int32, (32, 48), 0)
    c = lax.broadcasted_iota(jnp.int32, (32, 48), 1)
    exist_e = c < 40
    allow_e = exist_e & ((r >= 24) | ((c >= 24) & (c < 32)) | (c <= r))
    fill_e = jnp.where(exist_e, NEG, -jnp.inf).astype(f32)
    r = lax.broadcasted_iota(jnp.int32, (48, 80), 0)
    c = lax.broadcasted_iota(jnp.int32, (48, 80), 1)
    q_even = (r >= 32) & (r < 40)
    exist_o = (q_even & (c < 40)) | (~q_even & (c >= 40))
    ktok = jnp.where(c < 24, c, jnp.where(c < 48, c - 8, c - 16))
    qtok = jnp.where(r < 32, r + 32, r - 8)
    is_mem_key = ((c >= 24) & (c < 32)) | ((c >= 48) & (c < 56))
    allow_o = exist_o & (is_mem_key | (r < 8) | (ktok <= qtok))
    fill_o = jnp.where(exist_o, NEG, -jnp.inf).astype(f32)
    return allow_e, fill_e, allow_o, fill_o


def _rcombo(k, b11, b12, b21, b22):
    if k in (1, 4):
        return (b11 if k == 1 else b22)(k)
    a, b, sign = {0: (b11, b22, 1), 2: (b12, b22, -1), 3: (b21, b11, -1), 5: (b11, b12, 1), 6: (b21, b22, 1)}[k]
    a, b = _unpack(a(k)), _unpack(b(k))
    return (a + b if sign > 0 else a - b).astype(bf16)


def _softmax(s, allow, fill):
    s = jnp.where(allow, s * SCALE, fill)
    m = jnp.max(s, axis=-1, keepdims=True)
    e = jnp.exp(s - m)
    l = jnp.sum(e, axis=-1, keepdims=True)
    r = pl.reciprocal(l, approx=True)
    r = r * (2.0 - l * r)
    return (e * r).astype(bf16)


def _kernel(x_hbm, mem0_hbm, wq_hbm, wk_hbm, wv_hbm, wo_hbm, w1_hbm, w2_hbm, w3_hbm, w4_hbm,
            gw_hbm, out_hbm,
            x_v, s1_v, s2_v, s3_v, s4_v, wqkv_v, wo_v, h_v, b_v, c0_v, l_v, lf_v, n_v, g_v, out_v, xe_v, e_v, oe_v,
            ke_v, ve_v, o_v, mem_v, mem0_ref, gw_ref, zero_s,
            sem, sem_qkv, sem_out):
    RAW = (1, 2, 3, 4)
    RAW1 = (1, 7, 8, 4)

    loads = []

    def rows_load(name, r0, r1):
        loads.append((name, x_hbm.at[pl.ds(r0, r1 - r0)], x_v.at[pl.ds(r0, r1 - r0)]))

    def quad_load(name, w_hbm, s_v, raw, q, c0=0, c1=None):
        k4, n2 = s_v.shape[1], s_v.shape[2]
        c1 = n2 if c1 is None else c1
        src = w_hbm.bitcast(u32).at[pl.ds((q // 2) * k4, k4), pl.ds((q % 2) * n2 + c0, c1 - c0)]
        loads.append((name, src, s_v.at[raw[q], :, pl.ds(c0, c1 - c0)]))

    def w1_load(name, half, c0, c1):
        quad_load(name, w1_hbm, s1_v, RAW1, half, c0, c1)
        quad_load(name, w1_hbm, s1_v, RAW1, 2 + half, c0, c1)

    def block_load(name, w_hbm, s_v, r0, r1):
        kb, nb = s_v.shape[1:]
        for q in range(16):
            loads.append((name, w_hbm.at[pl.ds((q // 4) * kb + r0, r1 - r0), pl.ds((q % 4) * nb, nb)],
                          s_v.at[RAW16[q], pl.ds(r0, r1 - r0)]))

    rows_load("x0", 0, TM)
    w1_load("w1a", 0, 0, 256)
    w1_load("w1b", 0, 256, 512)
    rows_load("x1", TM, 2 * TM)
    w1_load("w1cd", 1, 0, 512)
    rows_load("x23", 2 * TM, 4 * TM)
    rows_load("x4567", 4 * TM, S)
    for q in range(4):
        quad_load("w2", w2_hbm, s2_v, RAW, q)
    block_load("w2", w3_hbm, s3_v, 0, W3A)
    block_load("w4", w3_hbm, s3_v, W3A, D4)
    block_load("w4", w4_hbm, s4_v, 0, F4)
    loads.append(("small", mem0_hbm, mem0_ref))
    loads.append(("small", gw_hbm, gw_ref))
    for j in range(NT):
        loads.append(("wo", wo_hbm.bitcast(u32).at[:, pl.ds(j * 128, 128)], wo_v.at[j]))
    groups = list(dict.fromkeys(name for name, _, _ in loads))
    assert len(groups) == NLOAD

    def start(*names, priority=0):
        for name, src, dst in loads:
            if name in names:
                pltpu.make_async_copy(src, dst, sem.at[groups.index(name)]).start(priority=priority)

    def wait(*names):
        for name, src, dst in loads:
            if name in names:
                pltpu.make_async_copy(src, dst, sem.at[groups.index(name)]).wait()

    SPG = 3 * G

    def qkv_start(g):
        for w, w_hbm in enumerate((wq_hbm, wk_hbm, wv_hbm)):
            wu = w_hbm.bitcast(u32)
            for k in range(G // 2):
                for par in range(2):
                    pltpu.make_async_copy(
                        wu.at[:, par * (H // 2) + g * (G // 2) + k, :],
                        wqkv_v.at[g * SPG + w * G + 2 * k + par], sem_qkv.at[g]).start(priority=1)

    def qkv_wait(g):
        grp = wqkv_v.at[pl.ds(g * SPG, SPG)]
        pltpu.make_async_copy(grp, grp, sem_qkv.at[g]).wait()

    start("x0", "w1a", "w1b", "x1", "w1cd", "x23", "x4567", "w2", "w4", "small")

    def zero(k, carry):
        zero_s[k] = 0
        return carry
    lax.fori_loop(0, RK, zero, 0)

    def tile_idx(ref, cols=128):
        z = zero_s[0]
        n = 16 if ref.dtype == bf16 and cols == 128 else 8
        return (z,) * (len(ref.shape) - 2) + (pl.ds(pl.multiple_of(z, n), n), slice(0, cols))

    rot = [0]
    ROT = 0
    hist = []

    def mm(lhs, rhs, side=None, acc=None):
        if side is not None:
            lhs = side(lhs)
        lhs = pltpu.bitcast(lhs, bf16) if lhs.dtype == u32 else lhs.astype(bf16)
        y = _dot(lhs, pltpu.bitcast(rhs, bf16) if rhs.dtype == u32 else rhs)
        if acc is not None:
            y = y + acc
        hist.append(y)
        return y

    class Side:
        def __init__(self, pieces, n, skip=0):
            cap = [0] * skip + ([1] * n if isinstance(n, int) else list(n))
            tot = sum(p[4] for p in pieces)
            self.plan = [[] for _ in cap]
            done = 0
            for p in pieces:
                done += p[4]
                x, d = done / tot * sum(cap), 0
                while x > cap[d] + 1e-9:
                    x -= cap[d]
                    d += 1
                self.plan[d].append((p, x / cap[d]))
            self.pieces = len(pieces)

        def __call__(self, val):
            todo = self.plan.pop(0) if self.plan else []
            if not todo:
                return val
            self.pieces -= len(todo)
            never = zero_s[0] > 0
            if val.dtype == bf16:
                val = pltpu.bitcast(val, u32)
            rg = 8 if val.dtype == u32 else 16
            ng = val.shape[0] // rg
            groups = [val[8 * m:8 * m + 8] for m in range(val.shape[0] // 8)]
            nk = val.shape[1] // 128
            npass = max(nk // 4, 1)
            for (fn, rd, wr, lag, _), pos in todo:
                sl = max(-int(-pos * ng * npass // 1) - 1, 0)
                m = sl % ng
                rot[0] += ROT
                kt = (sl // ng) * 4 + (rot[0] - 1) % min(nk, 4)
                pin = lambda v, w=128: v
                if lag is not None and len(hist) >= lag:
                    r0 = (16 * m) % hist[-lag].shape[0]
                    a = hist[-lag][r0:r0 + 8, :128]
                    if rd is None:
                        def pin(v, w=128, a=a):
                            a = jnp.concatenate([pltpu.bitcast(a, v.dtype)] * (v.shape[0] // 8), axis=0)
                            t = jnp.where(never, jnp.concatenate([a] * (w // 128), axis=1), v[:, :w])
                            return t if v.shape[1] == w else jnp.concatenate([t, v[:, w:]], axis=1)
                    elif rd.dtype == bf16:
                        idx = tile_idx(rd, 256)
                        rd[idx] = jnp.where(never, jnp.concatenate([a, a], axis=1).astype(bf16), rd[idx])
                    else:
                        idx = tile_idx(rd)
                        rd[idx] = jnp.where(never, pltpu.bitcast(a, rd.dtype), rd[idx])
                tiles = fn(pin)
                g = m * rg // 8
                ks = [groups[g][:, k * 128:(k + 1) * 128] for k in range(nk)]
                for u in (tiles if wr is None else [wr[tile_idx(wr)]]):
                    ks[kt] = jnp.where(never, pltpu.bitcast(u, val.dtype), ks[kt])
                groups[g] = jnp.concatenate(ks, axis=1)
            return jnp.concatenate(groups, axis=0)

    def strassen(lhs, rhs, side, init=(None, None, None, None)):
        def add(a, b):
            return a if b is None else a + b
        p = [mm(lhs(k), rhs(k), side) for k in range(5)]
        c12 = add(p[2] + p[4], init[1])
        c21 = add(p[1] + p[3], init[2])
        c22 = mm(lhs(5), rhs(5), side, add(p[0] - p[1] + p[2], init[3]))
        c11 = mm(lhs(6), rhs(6), side, add(p[0] + p[3] - p[4], init[0]))
        return c11, c12, c21, c22

    def fmm(lhs, rhs, side, extra=lambda n: None, emit=None):
        val = {}
        for n in WORDER:
            t = extra(n)
            for q, sg in sorted(_WPAR[n], key=lambda e: -e[1]):
                t = val[q] if t is None else (t + val[q] if sg > 0 else t - val[q])
            for r in range(RK):
                if WN[r] == n:
                    t = mm(lhs(UN[r]), rhs(r), side, t)
            val[n] = t
            if n < 8 and emit is not None:
                emit(n, t)
        return [val[v] for v in range(8)]

    def prep26_pieces(s_v, lag, stages=(sum(VSTAGES, ()),)):
        def piece(rs, cs, stage, pin):
            @functools.lru_cache(None)
            def node(n):
                if n < 16:
                    return s_v[RAW16[n], rs, cs].astype(f32)
                return _run([(0, VP[n - 16][1], 1, VP[n - 16][3])], [node(VP[n - 16][0]), node(VP[n - 16][2])])[-1]
            vals = [node(VN[r]).astype(bf16) for r in stage]
            for r, t in zip(stage, vals):
                s_v[r, rs, cs] = t
        kb, nb = s_v.shape[1:]
        out = []
        for r in range(0, kb, 16):
            out += [(slice(rr, rr + 8), slice(c, c + 256)) for c in range(0, nb - 255, 256) for rr in (r, r + 8)]
            out += [(slice(rr, rr + 8), slice(nb - 128, nb)) for rr in (r, r + 8)] if nb % 256 else []
        return [(functools.partial(piece, rs, cs, st), s_v, s_v, lag, 130 if cs.stop - cs.start == 256 else 100)
                for rs, cs in out for st in stages]

    def prep_pieces(s_v, raw, lag, width=256, by_value=False):
        def piece(r, c, pin):
            idx = (slice(r, r + 8), slice(c, c + width))
            b11, b12, b21, b22 = [_unpack(pin(s_v[(q,) + idx], width) if n in (0, 3) else s_v[(q,) + idx])
                                  for n, q in enumerate(raw)]
            for k, t in ((0, b11 + b22), (2, b12 - b22), (3, b21 - b11), (5, b11 + b12), (6, b21 + b22)):
                s_v[(k,) + idx] = _pack(t)
        return [(functools.partial(piece, r, c), None if by_value else s_v, s_v, lag, 80)
                for c in range(0, s_v.shape[2], width) for r in range(0, s_v.shape[1], 8)]

    def store_l(slot, q, c, quads, plain=False):
        for k, t in enumerate(quads if plain else _lcombos(*quads)):
            l_v[slot, k, q // 2:q // 2 + 8, c:c + t.shape[1]] = _pack(t)

    def ln_pieces(src, r0, slot, lag, plain=False, width=256, staged=False, clag=None):
        def stats(q, pin):
            x = pin(src[pl.ds(r0 + q, 16), :].astype(f32))
            xs = [x[:, j * 128:(j + 1) * 128] for j in range(NT)]
            m = functools.reduce(lambda a, b: a + b, xs) * (1.0 / NT)
            w = functools.reduce(lambda a, b: a + b, [(t - m) * (t - m) for t in xs])
            mean = jnp.mean(m, axis=-1, keepdims=True)
            var = jnp.sum(w + NT * ((m - mean) * (m - mean)), axis=-1, keepdims=True) * (1.0 / D)
            n_v[0, q:q + 16, :] = jnp.broadcast_to(mean, (16, 128))
            n_v[1, q:q + 16, :] = jnp.broadcast_to(lax.rsqrt(var + EPS), (16, 128))

        def comb(q, c, pin):
            quads = []
            for rr in (0, HM):
                rs = pl.ds(pl.multiple_of(r0 + rr + q + zero_s[0], 16), 16)
                mean, rstd = [jnp.concatenate([n_v[t, rr + q:rr + q + 16, :]] * (width // 128), axis=1)
                              for t in range(2)]
                quads += [(src[rs, cc + c:cc + c + width].astype(f32) - mean) * rstd for cc in (0, DH2)]
            store_l(slot, q, c, quads, plain)

        def comb26(q, pin):
            blocks = []
            for rr in (0, HM):
                rs = pl.ds(pl.multiple_of(r0 + rr + q + zero_s[0], 8), 8)
                mean, rstd = [jnp.concatenate([n_v[t, rr + q:rr + q + 8, :]] * 2, axis=1) for t in range(2)]
                blocks += [(src[rs, cc:cc + D4] - mean) * rstd for cc in range(0, D, D4)]
            vals = _run(UP, blocks)
            for k, u in enumerate(UL):
                lf_v[k, q:q + 8, :] = vals[u].astype(bf16)
        norms = [[(functools.partial(stats, rr + q), None, n_v, lag, 90) for rr in (0, HM)]
                 for q in range(0, HM, 16)]
        if slot is None:
            combs = [[(functools.partial(comb26, qq), n_v, lf_v, clag, 110) for qq in (q, q + 8)]
                     for q in range(0, HM, 16)]
        else:
            combs = [[(functools.partial(comb, q, c), n_v, l_v, clag, 125) for c in range(0, DH2, width)]
                     for q in range(0, HM, 16)]
        if staged:
            return sum(norms, []), sum(combs, [])
        out = list(norms[0])
        for a, b in zip(norms[1:] + [[]], combs):
            out += _merge(a, b) if a else b
        return out

    shifts = (1, 1, -1, -1, 2, 2, -2, -2)

    def shift_pieces(r0, slot, lag, by_value=False):
        def piece(q, j, pin):
            a = [h_v[jj, pl.ds(PAD + r0 + rr + q - shifts[jj], 16), :]
                 for rr in (0, HM) for jj in (j, j + NT // 2)]
            store_l(slot, q, j * 128, [pin(a[0]), a[1], a[2], pin(a[3])])
        return [(functools.partial(piece, q, j), None if by_value else h_v, l_v, lag, 50)
                for q in range(0, HM, 16) for j in range(NT // 2)]

    def lhs_of(slot):
        return lambda k: l_v[slot, k]

    h_v[:, 0:PAD, :] = jnp.zeros((NT, PAD, 128), f32)
    h_v[:, PAD + S:PAD + S + PAD, :] = jnp.zeros((NT, PAD, 128), f32)

    def store_h(r0, c0, h):
        for j in range(h.shape[1] // 128):
            h_v[c0 // 128 + j, PAD + r0:PAD + r0 + h.shape[0], :] = h[:, j * 128:(j + 1) * 128]

    def h_pieces(r0, c0, t, lag, n=4):
        def piece(r, pin):
            store_h(r0 + r, c0, _gelu(pin(t[r:r + 8 * n])))
        return [(functools.partial(piece, r), None, h_v, lag, 10 * n) for r in range(0, t.shape[0], 8 * n)]

    def flush(pieces):
        for p in pieces:
            p[0](lambda v, w=128: v)

    def w1_cols(c, step):
        half, cc = c // DH2, c % DH2
        return jnp.concatenate([s1_v[RAW1[half], :, cc:cc + step], s1_v[RAW1[2 + half], :, cc:cc + step]], axis=0)

    def d1_plain(xn, r0, c0, c1, step, side=None):
        for c in range(c0, c1, step):
            store_h(r0, c, _gelu(mm(xn, w1_cols(c, step), side)))

    def d1_fine(lhs, r0, nrb, cols, pieces, carry, skip=0):
        tiles = [(rb, c) for c in cols for rb in range(nrb)]
        rounds = [tiles[i:i + 4] for i in range(0, len(tiles), 4)]
        for n, (rnd, part) in enumerate(zip(rounds, split(pieces, len(rounds)))):
            sk = skip if n == 0 else 0
            side = Side(_merge(carry, part) if carry else part, 8 - sk, sk)
            carry = []
            for rb, c in rnd:
                half, cc = c // DH2, c % DH2
                t = mm(lhs(rb, 0), s1_v[RAW1[half], :, cc:cc + 128], side)
                t = mm(lhs(rb, 1), s1_v[RAW1[2 + half], :, cc:cc + 128], side, t)
                carry += h_pieces(r0 + rb * HM, c, t, LS)
        return carry

    CAP1 = (1, 1, 1, 1, 1, 1, 1)
    CAP2 = (2, 3, 3, 3, 3, 3, 2)

    def d1_s(b, slot, pieces, carry, early=()):
        for c, part, e in zip(range(0, DH2, NC1), split(pieces, DH2 // NC1), split(early, 2) + [[], []]):
            side = Side(merge(carry, part, e), CAP1 if hist else (0, 0) + CAP1[2:])
            cs = strassen(lhs_of(slot), lambda k: s1_v[k, :, c:c + NC1], side)
            carry = sum([h_pieces(b * TM + (q // 2) * HM, (q % 2) * DH2 + c, cs[q], LS) for q in (1, 2, 3, 0)], [])
        return carry

    def d2_s(b, slot, pieces, carry=(), early=(), late=()):
        for c, part, e in zip(range(0, DH2, NC1), split(pieces, DH2 // NC1), split(early, 2) + split(late, 2)):
            side = Side(merge(carry, part, e), CAP2 if hist else (0, 0) + CAP2[2:])
            carry = ()
            idx = [(slice(b * TM + (q // 2) * HM, b * TM + (q // 2 + 1) * HM),
                    slice((q % 2) * DH2 + c, (q % 2) * DH2 + c + NC1)) for q in range(4)]
            cs = strassen(lhs_of(slot), lambda k: s2_v[k, :, c:c + NC1], side,
                          [x_v[i].astype(f32) for i in idx])
            for i, t in zip(idx, cs):
                b_v[i] = t
                if b == 0:
                    c0_v[i] = t

    def split(l, n):
        w = [1.0 if hist else 0.6] + [1.0] * (n - 1)
        cut = [int(round(len(l) * sum(w[:i]) / sum(w))) for i in range(n + 1)]
        return [l[cut[i]:cut[i + 1]] for i in range(n)]

    def merge(*ls):
        ls = [l for l in ls if l]
        return _merge(*ls) if ls else []

    NW1, NW3, N30 = 32, 32, 20
    LS, LL = 3, 5

    wait("x0")
    xn0 = _pack(_ln(x_v[0:TM, :].astype(f32)))
    wait("w1a")
    d1_plain(xn0, 0, 0, 256, 256)
    wait("w1b")
    d1_plain(xn0, 0, 256, 512, 256)
    wait("x1")
    xn1 = _pack(_ln(x_v[TM:2 * TM, :].astype(f32)))
    d1_plain(xn1, TM, 0, 512, 256)
    wait("w1cd")
    hist.clear()
    xn01 = jnp.concatenate([xn0, xn1], axis=0)
    l01 = lambda rb, kh: xn01[rb * 64:(rb + 1) * 64, kh * DH2:(kh + 1) * DH2]
    pw = prep_pieces(s1_v, RAW1, LS, by_value=True)
    flush(d1_fine(l01, 0, 4, (512, 640), pw[:NW1], [], 1))
    carry = []
    wait("x23")
    hist.clear()
    carry = d1_fine(l01, 0, 4, (768, 896), ln_pieces(x_v, 2 * TM, 0, LL, plain=True), carry, 3)
    carry = d1_fine(lambda rb, kh: l_v[0, 2 * rb + kh], 2 * TM, 2, range(0, D, 128),
                    _merge(pw[NW1:], ln_pieces(x_v, 3 * TM, 1, LL)), carry)
    wait("x4567")
    qkv_start(0)
    qkv_start(1)
    hist.clear()
    for b in range(3, NB - 1):
        carry = d1_s(b, b % 2, ln_pieces(x_v, (b + 1) * TM, (b + 1) % 2, LL), carry)
    wait("w2")
    hist.clear()
    pw = prep_pieces(s2_v, RAW, LS, by_value=True)
    p3 = prep26_pieces(s3_v, LS)
    n3 = len(p3) * W3A // D4
    carry = d1_s(7, 1, _merge(pw[:NW3], shift_pieces(0, 0, LS, True)), carry)
    d2_s(0, 0, shift_pieces(TM, 1, LS, True), carry, pw[NW3:], p3[:N30])
    pw = split(_merge(p3[N30:n3], sum(ln_pieces(c0_v, 0, None, LL, clag=LS, staged=True), [])), 3)
    for b in range(1, 4):
        d2_s(b, b % 2, _merge(pw[b - 1], shift_pieces((b + 1) * TM, (b + 1) % 2, LS)))
    wait("w4", "small")
    hist.clear()
    pw = p3[n3:] + prep26_pieces(s4_v, LS)
    cut = (0, 31, 65, 99, len(pw))
    for b in range(4, NB):
        d2_s(b, b % 2, merge(pw[cut[b - 4]:cut[b - 3]],
                             shift_pieces((b + 1) * TM, (b + 1) % 2, LS) if b + 1 < NB else ()))
    start("wo", priority=1)

    def ffn(i, carry):
        qkv_wait(i)
        r0 = pl.multiple_of(i * TM, TM)
        rn = pl.multiple_of(jnp.minimum(i + 1, NB - 1) * TM, TM)
        acc = {}
        hist.clear()

        def relayout(p, r0_, r1_, pin):
            s0 = i * SPG + 2 * p
            for r in range(r0_, r1_, 8):
                e = wqkv_v[s0, r:r + 8, :]
                o = wqkv_v[s0 + 1, r:r + 8, :]
                wqkv_v[s0, r:r + 8, :] = (e & jnp.uint32(0xFFFF)) | (o << 16)
                wqkv_v[s0 + 1, r:r + 8, :] = (e >> 16) | (o & jnp.uint32(0xFFFF0000))

        relays = [(functools.partial(relayout, p, r, r + 32), wqkv_v, wqkv_v, 3, 35)
                  for p in range(SPG // 2) for r in range(0, D // 2, 32)]
        norms, combs = ln_pieces(b_v, rn, None, 5, staged=True, clag=3)

        def gate(q, pin):
            gw = gw_ref[...].astype(f32)
            x = pin(x_v[pl.ds(r0 + q, 16), :].astype(f32))
            t = functools.reduce(lambda a, b: a + b,
                                 [x[:, j * 128:(j + 1) * 128] * gw[j:j + 1, :] for j in range(NT)])
            g = jax.nn.sigmoid(jnp.sum(t, axis=-1, keepdims=True))
            g_v[pl.ds(r0 + q, 16), :] = jnp.broadcast_to(g, (16, 128))

        gates = [(functools.partial(gate, q), None, g_v, 5, 90) for q in range(0, TM, 16)]

        def extras(t, pin):
            jj, o = 2 * i + t // 2, 24 + 8 * (t % 2)
            xs = [pin(x_v[pl.ds(pl.multiple_of((jj + hh) * 64 + o, 8), 8), :].astype(f32)) for hh in (0, NPAIR // 2)]
            vals = _run(UP, [x[:, cc:cc + D4] for x in xs for cc in range(0, D, D4)])
            for k, u in enumerate(UL):
                xe_v[k, pl.ds(pl.multiple_of(i * 32 + t * 8, 8), 8), :] = vals[u].astype(bf16)

        xes = [(functools.partial(extras, t), None, xe_v, 3, 100) for t in range(4)]
        hs = {}

        def gelu_pieces(c, cs):
            def piece(r, cc, vs, pin):
                for v in vs:
                    hs[c, v, r, cc] = _gelu(pin(cs[v][r:r + 8, cc:cc + 128]))
                return [hs[c, v, r, cc] for v in vs]
            return [(functools.partial(piece, r, cc, vs), None, None, 3, 40) for r in range(0, HM, 8)
                    for cc in range(0, cs[0].shape[1], 128) for vs in ((0, 1, 2, 3), (4, 5, 6, 7))]

        def d3(c, side):
            c0, c1 = FCH[c]
            cs = fmm(lambda u: lf_v[UL.index(u)], lambda r: s3_v[r, :, c0:c1], side)
            assert not side.pieces
            return gelu_pieces(c, cs)

        def d4(c, side):
            c0, c1 = FCH[c]
            lh = _run(UP, [jnp.concatenate([jnp.concatenate(
                [hs.pop((c, v, r, cc)) for cc in range(0, c1 - c0, 128)], axis=1) for r in range(0, HM, 8)], axis=0)
                for v in range(8)])
            rhs = lambda r: s4_v[r, c0:c1, :]
            if c + 1 < len(FCH):
                for n in WORDER:
                    for r in range(RK):
                        if WN[r] == n:
                            acc[n] = mm(lh[UN[r]], rhs(r), side, acc.get(n))
            else:
                idx = lambda v: (pl.ds(r0 + (v // 4) * HM, HM), slice((v % 4) * D4, (v % 4 + 1) * D4))

                def extra(n):
                    if n >= 8:
                        return acc.get(n)
                    return b_v[idx(n)] + acc[n] if n in acc else b_v[idx(n)]

                def emit_b(v, t):
                    b_v[idx(v)] = jnp.concatenate([1.0 - g_v[idx(v)[0], :]] * 2, axis=1) * t
                fmm(lambda u: lh[u], rhs, side, extra, emit_b)
            assert not side.pieces

        g0 = d3(0, Side(relays[:20], 23, 3))
        g1 = d3(1, Side(_merge(g0, gates), 23, 2))
        d4(0, Side(g1[:22], 22, 4))
        g2 = d3(2, Side(_merge(g1[22:], relays[20:40]), 25))
        d4(1, Side(g2, 23, 2))
        g3 = d3(3, Side(_merge(relays[40:], norms, xes), 26))
        d4(2, Side(_merge(g3, combs), 23, 2))
        d4(3, Side([], 1))

        @pl.when(i + 2 < NG)
        def _():
            qkv_start(i + 2)

        return carry

    lax.fori_loop(0, NB, ffn, 0)

    def pre(it, carry):
        hist.clear()
        for u in range(3 * NG // NPRE):
            s0 = (it * (3 * NG // NPRE) + u) * G

            def rhs(r):
                t = None
                for q, sg in sorted(_terms(VP, 16, VN[r]).items(), key=lambda e: -e[1]):
                    blk = wqkv_v[s0 + q % 4 + zero_s[r], (q // 4) * (D // 8):(q // 4 + 1) * (D // 8), :]
                    if VN[r] < 16:
                        return blk
                    blk = _unpack(blk)
                    t = blk if t is None else (t + blk if sg > 0 else t - blk)
                return t.astype(bf16)
            for v, t in enumerate(fmm(lambda k: xe_v[UL.index(k)], rhs, None)):
                e_v[s0 + v % 4, (v // 4) * 128:(v // 4 + 1) * 128, :] = _pack(t)
        return carry

    lax.fori_loop(0, NPRE, pre, 0)

    wait("wo")
    mem_v[...] = mem0_ref[...].astype(f32)

    def slab(w, h):
        return (h // G) * SPG + w * G + h % G

    def step(j, hx, odd, late, allow, fill):
        qs, ks, vs, ps = {}, {}, {}, {}
        wload = lambda w, h: pltpu.bitcast(wqkv_v[slab(w, h)], bf16)
        eload = lambda w, h: pltpu.bitcast(e_v[slab(w, h), pl.ds(pl.multiple_of(j * 8, 8), 8), :], bf16)

        def proj(g):
            part = {}
            if late and g == 0:
                for h in range(2):
                    for w in range(3):
                        part[w, h] = _dot(hx[:, :DH2], wload(w, h)[:DH2])
            for h in range(g * G, (g + 1) * G):
                q, k, v = [(_dot(hx[:, DH2:], wload(w, h)[DH2:]) + part[w, h] if (w, h) in part
                            else _dot(hx, wload(w, h))).astype(bf16) for w in range(3)]
                if odd:
                    q = jnp.concatenate([q, eload(0, h)], axis=0)
                    k = jnp.concatenate([pltpu.bitcast(ke_v[h], bf16), eload(1, h), k], axis=0)
                    v = jnp.concatenate([pltpu.bitcast(ve_v[h], bf16), eload(2, h), v], axis=0)
                else:
                    ke_v[h] = pltpu.bitcast(k, u32)
                    ve_v[h] = pltpu.bitcast(v, u32)
                    k = jnp.concatenate([k, eload(1, h)], axis=0)
                    v = jnp.concatenate([v, eload(2, h)], axis=0)
                qs[h], ks[h], vs[h] = q, k, v

        def score(g):
            for h in range(g * G, (g + 1) * G):
                s = lax.dot_general(qs.pop(h), ks.pop(h), (((1,), (1,)), ((), ())),
                                    preferred_element_type=f32)
                ps[h] = _softmax(s, allow, fill)

        def pv(g):
            os_ = []
            for h in range(g * G, (g + 1) * G):
                o = _dot(ps.pop(h), vs.pop(h))
                o_v[:, h * 128:(h + 1) * 128] = _pack(o[:32])
                os_.append(o)
            if odd:
                quads = [jnp.concatenate([os_[2 * kk][r:r + 8], os_[2 * kk + 1][r:r + 8]], axis=1)
                         for r in (32, 40) for kk in range(2)]
                for k, t in enumerate(_lcombos(*quads)):
                    oe_v[k, pl.ds(pl.multiple_of(j * 8, 8), 8), g * 256:(g + 1) * 256] = t.astype(bf16)

        acc = [None] * NT

        def wo(h0, h1, j0, j1):
            o = pltpu.bitcast(o_v[:, h0 * 128:h1 * 128], bf16)
            for n in range(j0, j1):
                y = _dot(o, pltpu.bitcast(wo_v[n, h0 * 64:h1 * 64, :], bf16))
                acc[n] = y if acc[n] is None else y + acc[n]

        for t in range(NG):
            proj(t)
            if t >= 2:
                pv(t - 2)
            if t >= 1:
                score(t - 1)
        wo(0, 16, 0, 4)
        pv(NG - 2)
        score(NG - 1)
        wo(0, 16, 4, 8)
        pv(NG - 1)
        wo(16, 24, 0, 8)
        wo(24, 32, 0, 8)
        return jnp.concatenate(acc, axis=1)

    def emit(j, r0, o0, a):
        rs = pl.ds(r0 + o0, 24)
        g = jnp.concatenate([g_v[rs, :]] * NT, axis=1)
        out_v[j, o0:o0 + 24, :] = (g * a + b_v[rs, :]).astype(bf16)

    def pair(j, mem, late):
        r0 = pl.multiple_of(j * 64, 64)
        allow_e, fill_e, allow_o, fill_o = _masks()
        xa = x_v[pl.ds(r0 + 16, 8), :].astype(f32)
        xb = x_v[pl.ds(r0 + 40, 8), :].astype(f32)
        hx = jnp.concatenate([x_v[pl.ds(r0, 16), :], jnp.concatenate([xa, mem], 0).astype(bf16)], 0)
        oe = step(j, hx, False, late, allow_e, fill_e)
        emit(j, r0, 0, oe[:24])
        hx = jnp.concatenate([jnp.concatenate([oe[24:32], xb], 0).astype(bf16), x_v[pl.ds(r0 + 48, 16), :]], 0)
        oo = step(j, hx, True, True, allow_o, fill_o)
        emit(j, r0, 40, oo[8:])
        return oo[:8]

    def a_iter(it, carry):
        mem = mem_v[...]
        for t in range(PPI):
            mem = pair(it * PPI + t, mem, t > 0)
        mem_v[...] = mem
        for t in range(PPI):
            for o0 in (0, 40):
                idx = (it * PPI + t, pl.ds(o0, 24))
                pltpu.make_async_copy(out_v.at[idx], out_hbm.at[idx], sem_out).start()
        return carry

    lax.fori_loop(0, NPAIR // PPI, a_iter, 0)

    hist.clear()
    for n in range(NT // 2):
        quad = [lambda k, t=2 * n + q % 2, o=(q // 2) * 128: jnp.concatenate(
            [wo_v[t + zero_s[k], g * 256 + o:g * 256 + o + 128, :] for g in range(NG)], axis=0) for q in range(4)]
        cs = strassen(lambda k: oe_v[k], lambda k: _rcombo(k, *quad), None)
        cols = slice(n * 256, (n + 1) * 256)
        for half in range(2):
            t = jnp.concatenate(cs[2 * half:2 * half + 2], axis=1)
            o0 = 24 + half * 8
            for jj in range(NPAIR):
                rs = slice(jj * 64 + o0, jj * 64 + o0 + 8)
                g = jnp.concatenate([g_v[rs, :]] * 2, axis=1)
                out_v[jj, o0:o0 + 8, cols] = (g * t[jj * 8:jj * 8 + 8] + b_v[rs, cols]).astype(bf16)
        if n >= 2:
            idx = (slice(None), pl.ds(24, 16), pl.ds(0, 768) if n == 2 else pl.ds(768, 256))
            pltpu.make_async_copy(out_v.at[idx], out_hbm.at[idx], sem_out).start()
    pltpu.make_async_copy(out_v, out_hbm, sem_out).wait()


@functools.partial(jax.jit, static_argnames=("A_seg_len",))
def pallas_gated_mix__memory_aug_recurrent_mem_tr__mixer_s_mlp__prompt_kernel(
    A_x, A_mem0, A_Wq, A_Wk, A_Wv, A_Wo, A_seg_len, B_x, B_w1, B_w2, B_w3, B_w4, gate_w,
):
    assert A_seg_len == SEG
    assert A_x.shape == (1, S, D) and A_mem0.shape == (1, M, D)
    any_spec = pl.BlockSpec(memory_space=pl.ANY)
    out = pl.pallas_call(
        _kernel,
        out_shape=jax.ShapeDtypeStruct((NPAIR, 64, D), bf16),
        in_specs=[any_spec] * 11,
        out_specs=any_spec,
        scratch_shapes=[
            pltpu.VMEM((S, D), bf16),
            pltpu.VMEM((9, D // 4, D // 2), u32),
            pltpu.VMEM((7, D // 4, D // 2), u32),
            pltpu.VMEM((RK, D4, F4), bf16),
            pltpu.VMEM((RK, F4, D4), bf16),
            pltpu.VMEM((3 * H, D // 2, DH), u32),
            pltpu.VMEM((NT, H * DH // 2, 128), u32),
            pltpu.VMEM((NT, S + 2 * PAD, 128), f32),
            pltpu.VMEM((S, D), f32),
            pltpu.VMEM((TM, D), f32),
            pltpu.VMEM((2, 7, HM // 2, D // 2), u32),
            pltpu.VMEM((len(UL), HM, D4), bf16),
            pltpu.VMEM((2, TM, 128), f32),
            pltpu.VMEM((S, 128), f32),
            pltpu.VMEM((NPAIR, 64, D), bf16),
            pltpu.VMEM((len(UL), 8 * NPAIR, D4), bf16),
            pltpu.VMEM((3 * H, 8 * NPAIR, DH), u32),
            pltpu.VMEM((7, 8 * NPAIR, H * DH // 2), bf16),
            pltpu.VMEM((H, 16, 128), u32),
            pltpu.VMEM((H, 16, 128), u32),
            pltpu.VMEM((16, H * DH), u32),
            pltpu.VMEM((M, D), f32),
            pltpu.VMEM((M, D), bf16),
            pltpu.VMEM((NT, 128), bf16),
            pltpu.SMEM((RK,), jnp.int32),
            pltpu.SemaphoreType.DMA((NLOAD,)),
            pltpu.SemaphoreType.DMA((NG,)),
            pltpu.SemaphoreType.DMA,
        ],
        compiler_params=pltpu.CompilerParams(vmem_limit_bytes=126 * 1024 * 1024,
                                             disable_bounds_checks=True),
    )(
        A_x.reshape(S, D), A_mem0.reshape(M, D),
        A_Wq.reshape(D // 2, 2 * H, DH), A_Wk.reshape(D // 2, 2 * H, DH), A_Wv.reshape(D // 2, 2 * H, DH),
        A_Wo.reshape(H * DH, D), B_w1, B_w2, B_w3, B_w4, gate_w.reshape(NT, 128),
    )
    return out.reshape(1, S, D)
```

```python
import functools

import jax
import jax.numpy as jnp
from jax import lax
import jax.experimental.pallas as pl
import jax.experimental.pallas.tpu as pltpu

f32, bf16, u32 = jnp.float32, jnp.bfloat16, jnp.uint32

S, D, H, DH, M, SEG, F = 2048, 1024, 32, 128, 8, 32, 3584
SCALE = DH ** -0.5
NEG = -1000000000.0
EPS = 1e-05

TM = 256
NB = S // TM
HM = TM // 2
DH2 = D // 2
D4, F4 = D // 4, F // 4
FCH = ((0, 128), (128, 384), (384, 640), (640, 896))
NC1 = 128
NPAIR = S // (2 * SEG)
PPI = 2
NPRE = 4
G = 4
NG = H // G
PAD = 8
NT = D // 128
W3A = 192
NLOAD = 11
assert NB == NG

_dot = functools.partial(jnp.dot, preferred_element_type=f32)

UP = ((4, 1, 5, 1), (6, 1, 8, 1), (0, 1, 3, 1), (2, -1, 9, 1), (4, -1, 10, 1), (0, 1, 1, 1), (2, 1, 12, 1),
      (5, 1, 7, -1), (7, 1, 12, -1), (11, -1, 13, 1), (10, -1, 11, 1), (2, 1, 7, 1), (0, -1, 4, 1),
      (6, 1, 7, 1), (1, -1, 5, 1), (3, 1, 7, -1), (1, 1, 4, 1), (2, 1, 3, 1), (1, -1, 3, 1), (1, 1, 7, -1),
      (2, 1, 6, -1))
WP = ((0, -1, 3, 1), (4, 1, 6, -1), (1, 1, 8, 1), (5, 1, 10, 1), (4, -1, 7, 1), (0, -1, 9, -1),
      (11, 1, 12, 1), (6, 1, 7, -1), (2, 1, 5, -1), (0, -1, 7, -1), (9, 1, 11, -1), (2, 1, 13, 1),
      (5, 1, 13, 1), (2, -1, 3, 1), (5, 1, 6, 1), (0, 1, 4, 1), (2, 1, 7, 1), (1, 1, 2, 1), (1, 1, 5, 1),
      (3, 1, 7, 1), (2, 1, 6, 1))
VP = ((1, 1, 5, -1), (8, 1, 11, 1), (10, 1, 17, 1), (13, 1, 16, -1), (0, 1, 4, -1), (0, 1, 3, 1),
      (14, 1, 18, -1), (0, 1, 11, 1), (14, 1, 19, -1), (0, 1, 5, 1), (12, 1, 15, 1), (2, 1, 21, 1),
      (10, 1, 14, -1), (4, 1, 7, 1), (11, 1, 19, 1), (12, -1, 20, 1), (13, 1, 14, -1), (9, 1, 30, -1),
      (3, -1, 15, 1), (6, 1, 23, 1), (24, 1, 27, -1), (9, -1, 18, 1), (7, 1, 34, 1), (2, 1, 6, -1),
      (0, 1, 8, -1), (6, 1, 21, 1), (22, 1, 31, -1), (6, 1, 29, 1), (0, 1, 1, 1), (15, 1, 25, 1),
      (5, 1, 37, 1), (15, 1, 20, 1))
UN = (7, 27, 24, 17, 9, 22, 21, 2, 15, 11, 8, 25, 19, 28, 2, 23, 26, 20, 1, 18, 10, 28, 4, 13, 14, 16)
WN = (23, 17, 24, 10, 14, 7, 22, 19, 12, 18, 15, 25, 20, 5, 26, 0, 8, 2, 27, 11, 26, 9, 28, 21, 16, 5)
VN = (42, 47, 41, 5, 11, 43, 18, 28, 20, 23, 35, 19, 22, 46, 33, 26, 45, 36, 38, 25, 44, 40, 39, 21, 24, 32)
RK = len(UN)
UL = tuple(sorted(set(UN)))
VSTAGES = ((0, 6, 7, 12, 13, 14, 15, 21), (11, 17, 20, 22, 24, 25, 23, 2), (1, 5, 8, 9, 10, 16, 18, 19))
RAW16 = (1, 11, 17, 5, 8, 3, 9, 10, 0, 6, 7, 4, 12, 20, 22, 16)


def _run(prog, blocks):
    vals = list(blocks)
    for a, sa, b, sb in prog:
        vals.append(vals[a] + vals[b] if sa > 0 and sb > 0 else
                    vals[a] - vals[b] if sa > 0 else vals[b] - vals[a])
    return vals


def _terms(prog, nin, node):
    if node < nin:
        return {node: 1}
    a, sa, b, sb = prog[node - nin]
    out = {k: sa * v for k, v in _terms(prog, nin, a).items()}
    out.update({k: sb * v for k, v in _terms(prog, nin, b).items()})
    return out


for _b in range(16):
    _last = max(k for k, st in enumerate(VSTAGES) for r in st if _b in _terms(VP, 16, VN[r]))
    assert VN[RAW16[_b]] == _b or RAW16[_b] in VSTAGES[_last]
assert sorted(sum(VSTAGES, ())) == [r for r in range(RK) if VN[r] >= 16] and len(set(RAW16)) == 16

_WPAR = {n: [] for n in range(8 + len(WP))}
for _t, (_a, _sa, _b, _sb) in enumerate(WP):
    _WPAR[_a].append((8 + _t, _sa))
    _WPAR[_b].append((8 + _t, _sb))


def _worder():
    order = []

    def closure(n, acc):
        if n not in acc and n not in order:
            acc.add(n)
            for q, _ in _WPAR[n]:
                closure(q, acc)
        return acc

    def visit(n):
        if n not in order:
            for q, _ in _WPAR[n]:
                visit(q)
            order.append(n)
    while len([v for v in range(8) if v not in order]):
        visit(min((v for v in range(8) if v not in order), key=lambda v: len(closure(v, set()))))
    return tuple(order)


WORDER = _worder()


def _ln(x):
    m = jnp.mean(x, axis=-1, keepdims=True)
    xc = x - m
    v = jnp.mean(xc * xc, axis=-1, keepdims=True)
    return xc * lax.rsqrt(v + EPS)


_GC = 0.7978845608028654


def _gelu(x):
    h = 0.5 * x
    return h + h * jnp.tanh(x * (_GC + (_GC * 0.044715) * (x * x)))


def _unpack(u):
    return pltpu.bitcast(u, bf16).astype(f32)


def _pack(x):
    return pltpu.bitcast(x.astype(bf16), u32)


def _lcombos(a11, a12, a21, a22):
    return [a11 + a22, a21 + a22, a11, a22, a11 + a12, a21 - a11, a12 - a22]


def _merge(*lists):
    keyed = [((j + 0.5) / len(l), n, j, v) for n, l in enumerate(lists) for j, v in enumerate(l)]
    return [v for _, _, _, v in sorted(keyed, key=lambda t: t[:3])]


def _masks():
    r = lax.broadcasted_iota(jnp.int32, (32, 48), 0)
    c = lax.broadcasted_iota(jnp.int32, (32, 48), 1)
    exist_e = c < 40
    allow_e = exist_e & ((r >= 24) | ((c >= 24) & (c < 32)) | (c <= r))
    fill_e = jnp.where(exist_e, NEG, -jnp.inf).astype(f32)
    r = lax.broadcasted_iota(jnp.int32, (48, 80), 0)
    c = lax.broadcasted_iota(jnp.int32, (48, 80), 1)
    q_even = (r >= 32) & (r < 40)
    exist_o = (q_even & (c < 40)) | (~q_even & (c >= 40))
    ktok = jnp.where(c < 24, c, jnp.where(c < 48, c - 8, c - 16))
    qtok = jnp.where(r < 32, r + 32, r - 8)
    is_mem_key = ((c >= 24) & (c < 32)) | ((c >= 48) & (c < 56))
    allow_o = exist_o & (is_mem_key | (r < 8) | (ktok <= qtok))
    fill_o = jnp.where(exist_o, NEG, -jnp.inf).astype(f32)
    return allow_e, fill_e, allow_o, fill_o


def _rcombo(k, b11, b12, b21, b22):
    if k in (1, 4):
        return (b11 if k == 1 else b22)(k)
    a, b, sign = {0: (b11, b22, 1), 2: (b12, b22, -1), 3: (b21, b11, -1), 5: (b11, b12, 1), 6: (b21, b22, 1)}[k]
    a, b = _unpack(a(k)), _unpack(b(k))
    return (a + b if sign > 0 else a - b).astype(bf16)


def _softmax(s, allow, fill):
    s = jnp.where(allow, s * SCALE, fill)
    m = jnp.max(s, axis=-1, keepdims=True)
    e = jnp.exp(s - m)
    l = jnp.sum(e, axis=-1, keepdims=True)
    r = pl.reciprocal(l, approx=True)
    r = r * (2.0 - l * r)
    return (e * r).astype(bf16)


def _kernel(x_hbm, mem0_hbm, wq_hbm, wk_hbm, wv_hbm, wo_hbm, w1_hbm, w2_hbm, w3_hbm, w4_hbm,
            gw_hbm, out_hbm,
            x_v, s1_v, s2_v, s3_v, s4_v, wqkv_v, wo_v, h_v, b_v, c0_v, l_v, lf_v, n_v, g_v, out_v, xe_v, e_v, oe_v,
            ke_v, ve_v, o_v, mem_v, mem0_ref, gw_ref, zero_s,
            sem, sem_qkv, sem_out):
    RAW = (1, 2, 3, 4)
    RAW1 = (1, 7, 8, 4)

    loads = []

    def rows_load(name, r0, r1):
        loads.append((name, x_hbm.at[pl.ds(r0, r1 - r0)], x_v.at[pl.ds(r0, r1 - r0)]))

    def quad_load(name, w_hbm, s_v, raw, q, c0=0, c1=None):
        k4, n2 = s_v.shape[1], s_v.shape[2]
        c1 = n2 if c1 is None else c1
        src = w_hbm.bitcast(u32).at[pl.ds((q // 2) * k4, k4), pl.ds((q % 2) * n2 + c0, c1 - c0)]
        loads.append((name, src, s_v.at[raw[q], :, pl.ds(c0, c1 - c0)]))

    def w1_load(name, half, c0, c1):
        quad_load(name, w1_hbm, s1_v, RAW1, half, c0, c1)
        quad_load(name, w1_hbm, s1_v, RAW1, 2 + half, c0, c1)

    def block_load(name, w_hbm, s_v, r0, r1):
        kb, nb = s_v.shape[1:]
        for q in range(16):
            loads.append((name, w_hbm.at[pl.ds((q // 4) * kb + r0, r1 - r0), pl.ds((q % 4) * nb, nb)],
                          s_v.at[RAW16[q], pl.ds(r0, r1 - r0)]))

    rows_load("x0", 0, TM)
    w1_load("w1a", 0, 0, 256)
    w1_load("w1b", 0, 256, 512)
    rows_load("x1", TM, 2 * TM)
    w1_load("w1cd", 1, 0, 512)
    rows_load("x23", 2 * TM, 4 * TM)
    rows_load("x4567", 4 * TM, S)
    for q in range(4):
        quad_load("w2", w2_hbm, s2_v, RAW, q)
    block_load("w2", w3_hbm, s3_v, 0, W3A)
    block_load("w4", w3_hbm, s3_v, W3A, D4)
    block_load("w4", w4_hbm, s4_v, 0, F4)
    loads.append(("small", mem0_hbm, mem0_ref))
    loads.append(("small", gw_hbm, gw_ref))
    for j in range(NT):
        loads.append(("wo", wo_hbm.bitcast(u32).at[:, pl.ds(j * 128, 128)], wo_v.at[j]))
    groups = list(dict.fromkeys(name for name, _, _ in loads))
    assert len(groups) == NLOAD

    def start(*names, priority=0):
        for name, src, dst in loads:
            if name in names:
                pltpu.make_async_copy(src, dst, sem.at[groups.index(name)]).start(priority=priority)

    def wait(*names):
        for name, src, dst in loads:
            if name in names:
                pltpu.make_async_copy(src, dst, sem.at[groups.index(name)]).wait()

    SPG = 3 * G

    def qkv_start(g):
        for w, w_hbm in enumerate((wq_hbm, wk_hbm, wv_hbm)):
            wu = w_hbm.bitcast(u32)
            for k in range(G // 2):
                for par in range(2):
                    pltpu.make_async_copy(
                        wu.at[:, par * (H // 2) + g * (G // 2) + k, :],
                        wqkv_v.at[g * SPG + w * G + 2 * k + par], sem_qkv.at[g]).start(priority=1)

    def qkv_wait(g):
        grp = wqkv_v.at[pl.ds(g * SPG, SPG)]
        pltpu.make_async_copy(grp, grp, sem_qkv.at[g]).wait()

    start("x0", "w1a", "w1b", "x1", "w1cd", "x23", "x4567", "w2", "w4", "small")

    def zero(k, carry):
        zero_s[k] = 0
        return carry
    lax.fori_loop(0, RK, zero, 0)

    def tile_idx(ref, cols=128):
        z = zero_s[0]
        n = 16 if ref.dtype == bf16 and cols == 128 else 8
        return (z,) * (len(ref.shape) - 2) + (pl.ds(pl.multiple_of(z, n), n), slice(0, cols))

    TIE26 = 16
    rot = [0]
    ROT = 0
    hist = []

    def mm(lhs, rhs, side=None, acc=None):
        if side is not None:
            lhs = side(lhs)
        lhs = pltpu.bitcast(lhs, bf16) if lhs.dtype == u32 else lhs.astype(bf16)
        y = _dot(lhs, pltpu.bitcast(rhs, bf16) if rhs.dtype == u32 else rhs)
        if acc is not None:
            y = y + acc
        hist.append(y)
        return y

    class Side:
        def __init__(self, pieces, n, skip=0):
            cap = [0] * skip + ([1] * n if isinstance(n, int) else list(n))
            tot = sum(p[4] for p in pieces)
            self.plan = [[] for _ in cap]
            done = 0
            for p in pieces:
                done += p[4]
                x, d = done / tot * sum(cap), 0
                while x > cap[d] + 1e-9:
                    x -= cap[d]
                    d += 1
                self.plan[d].append((p, x / cap[d]))
            self.pieces = len(pieces)

        def __call__(self, val):
            todo = self.plan.pop(0) if self.plan else []
            if not todo:
                return val
            self.pieces -= len(todo)
            never = zero_s[0] > 0
            if val.dtype == bf16:
                val = pltpu.bitcast(val, u32)
            rg = 8 if val.dtype == u32 else 16
            ng = val.shape[0] // rg
            groups = [val[8 * m:8 * m + 8] for m in range(val.shape[0] // 8)]
            nk = val.shape[1] // 128
            used = {}
            npass = max(nk // 4, 1)
            for (fn, rd, wr, lag, _), pos in todo:
                sl = max(-int(-pos * ng * npass // 1) - 1, 0)
                m = sl % ng
                rot[0] += ROT
                kt = (sl // ng) * 4 + (rot[0] - 1) % min(nk, 4)
                pin = lambda v, w=128: v
                if lag is not None and len(hist) >= lag:
                    r0 = (16 * m) % hist[-lag].shape[0]
                    a = hist[-lag][r0:r0 + 8, :128]
                    if rd is None:
                        def pin(v, w=128, a=a):
                            a = jnp.concatenate([pltpu.bitcast(a, v.dtype)] * (v.shape[0] // 8), axis=0)
                            t = jnp.where(never, jnp.concatenate([a] * (w // 128), axis=1), v[:, :w])
                            return t if v.shape[1] == w else jnp.concatenate([t, v[:, w:]], axis=1)
                    elif rd.dtype == bf16:
                        idx = tile_idx(rd, 256)
                        rd[idx] = jnp.where(never, jnp.concatenate([a, a], axis=1).astype(bf16), rd[idx])
                    else:
                        idx = tile_idx(rd)
                        rd[idx] = jnp.where(never, pltpu.bitcast(a, rd.dtype), rd[idx])
                tiles = fn(pin)
                if wr is False:
                    continue
                g = m * rg // 8
                ks = [groups[g][:, k * 128:(k + 1) * 128] for k in range(nk)]
                u = functools.reduce(lambda a, b: a + b, tiles) if wr is None else wr[tile_idx(wr)]
                used[g, kt] = used.get((g, kt), -1) + 1
                ks[kt] = jnp.where(zero_s[used[g, kt]] > 0, pltpu.bitcast(u, val.dtype), ks[kt])
                groups[g] = jnp.concatenate(ks, axis=1)
            return jnp.concatenate(groups, axis=0)

    def strassen(lhs, rhs, side, init=(None, None, None, None)):
        def add(a, b):
            return a if b is None else a + b
        p = [mm(lhs(k), rhs(k), side) for k in range(5)]
        c12 = add(p[2] + p[4], init[1])
        c21 = add(p[1] + p[3], init[2])
        c22 = mm(lhs(5), rhs(5), side, add(p[0] - p[1] + p[2], init[3]))
        c11 = mm(lhs(6), rhs(6), side, add(p[0] + p[3] - p[4], init[0]))
        return c11, c12, c21, c22

    def fmm(lhs, rhs, side, extra=lambda n: None, emit=None):
        val = {}
        for n in WORDER:
            t = extra(n)
            for q, sg in sorted(_WPAR[n], key=lambda e: -e[1]):
                t = val[q] if t is None else (t + val[q] if sg > 0 else t - val[q])
            for r in range(RK):
                if WN[r] == n:
                    t = mm(lhs(UN[r]), rhs(r), side, t)
            val[n] = t
            if n < 8 and emit is not None:
                emit(n, t)
        return [val[v] for v in range(8)]

    def prep26_pieces(s_v, lag, stages=(sum(VSTAGES, ()),)):
        def piece(rs, cs, stage, pin):
            @functools.lru_cache(None)
            def node(n):
                if n < 16:
                    return s_v[RAW16[n], rs, cs].astype(f32)
                return _run([(0, VP[n - 16][1], 1, VP[n - 16][3])], [node(VP[n - 16][0]), node(VP[n - 16][2])])[-1]
            vals = [node(VN[r]).astype(bf16) for r in stage]
            for r, t in zip(stage, vals):
                s_v[r, rs, cs] = t
        kb, nb = s_v.shape[1:]
        out = []
        for r in range(0, kb, 16):
            out += [(slice(rr, rr + 8), slice(c, c + 256)) for c in range(0, nb - 255, 256) for rr in (r, r + 8)]
            out += [(slice(rr, rr + 8), slice(nb - 128, nb)) for rr in (r, r + 8)] if nb % 256 else []
        return [(functools.partial(piece, rs, cs, st), s_v, s_v if n % TIE26 == TIE26 - 1 else False, lag,
                 130 if cs.stop - cs.start == 256 else 100) for n, (rs, cs) in enumerate(out) for st in stages]

    def prep_pieces(s_v, raw, lag, width=256, by_value=False):
        def piece(r, c, pin):
            idx = (slice(r, r + 8), slice(c, c + width))
            b11, b12, b21, b22 = [_unpack(pin(s_v[(q,) + idx], width) if n in (0, 3) else s_v[(q,) + idx])
                                  for n, q in enumerate(raw)]
            for k, t in ((0, b11 + b22), (2, b12 - b22), (3, b21 - b11), (5, b11 + b12), (6, b21 + b22)):
                s_v[(k,) + idx] = _pack(t)
        return [(functools.partial(piece, r, c), None if by_value else s_v, s_v, lag, 80)
                for c in range(0, s_v.shape[2], width) for r in range(0, s_v.shape[1], 8)]

    def store_l(slot, q, c, quads, plain=False):
        for k, t in enumerate(quads if plain else _lcombos(*quads)):
            l_v[slot, k, q // 2:q // 2 + 8, c:c + t.shape[1]] = _pack(t)

    def ln_pieces(src, r0, slot, lag, plain=False, width=256, staged=False, clag=None):
        def stats(q, pin):
            x = pin(src[pl.ds(r0 + q, 16), :].astype(f32))
            xs = [x[:, j * 128:(j + 1) * 128] for j in range(NT)]
            m = functools.reduce(lambda a, b: a + b, xs) * (1.0 / NT)
            w = functools.reduce(lambda a, b: a + b, [(t - m) * (t - m) for t in xs])
            mean = jnp.mean(m, axis=-1, keepdims=True)
            var = jnp.sum(w + NT * ((m - mean) * (m - mean)), axis=-1, keepdims=True) * (1.0 / D)
            n_v[0, q:q + 16, :] = jnp.broadcast_to(mean, (16, 128))
            n_v[1, q:q + 16, :] = jnp.broadcast_to(lax.rsqrt(var + EPS), (16, 128))

        def comb(q, c, pin):
            quads = []
            for rr in (0, HM):
                rs = pl.ds(pl.multiple_of(r0 + rr + q + zero_s[0], 16), 16)
                mean, rstd = [jnp.concatenate([n_v[t, rr + q:rr + q + 16, :]] * (width // 128), axis=1)
                              for t in range(2)]
                quads += [(src[rs, cc + c:cc + c + width].astype(f32) - mean) * rstd for cc in (0, DH2)]
            store_l(slot, q, c, quads, plain)

        def comb26(q, pin):
            blocks = []
            for rr in (0, HM):
                rs = pl.ds(pl.multiple_of(r0 + rr + q + zero_s[0], 8), 8)
                mean, rstd = [jnp.concatenate([n_v[t, rr + q:rr + q + 8, :]] * 2, axis=1) for t in range(2)]
                blocks += [(src[rs, cc:cc + D4] - mean) * rstd for cc in range(0, D, D4)]
            vals = _run(UP, blocks)
            for k, u in enumerate(UL):
                lf_v[k, q:q + 8, :] = vals[u].astype(bf16)
        norms = [[(functools.partial(stats, rr + q), None, n_v if slot is not None else False, lag, 90) for rr in (0, HM)]
                 for q in range(0, HM, 16)]
        if slot is None:
            combs = [[(functools.partial(comb26, qq), n_v, lf_v if qq % 32 == 24 else False, clag, 110) for qq in (q, q + 8)]
                     for q in range(0, HM, 16)]
        else:
            combs = [[(functools.partial(comb, q, c), n_v, l_v, clag, 125) for c in range(0, DH2, width)]
                     for q in range(0, HM, 16)]
        if staged:
            return sum(norms, []), sum(combs, [])
        out = list(norms[0])
        for a, b in zip(norms[1:] + [[]], combs):
            out += _merge(a, b) if a else b
        return out

    shifts = (1, 1, -1, -1, 2, 2, -2, -2)

    def shift_pieces(r0, slot, lag, by_value=False):
        def piece(q, j, pin):
            a = [h_v[jj, pl.ds(PAD + r0 + rr + q - shifts[jj], 16), :]
                 for rr in (0, HM) for jj in (j, j + NT // 2)]
            store_l(slot, q, j * 128, [pin(a[0]), a[1], a[2], pin(a[3])])
        return [(functools.partial(piece, q, j), None if by_value else h_v, l_v if (q // 16) % 2 and j == 3 else False, lag, 50)
                for q in range(0, HM, 16) for j in range(NT // 2)]

    def lhs_of(slot):
        return lambda k: l_v[slot, k]

    h_v[:, 0:PAD, :] = jnp.zeros((NT, PAD, 128), f32)
    h_v[:, PAD + S:PAD + S + PAD, :] = jnp.zeros((NT, PAD, 128), f32)

    def store_h(r0, c0, h):
        for j in range(h.shape[1] // 128):
            h_v[c0 // 128 + j, PAD + r0:PAD + r0 + h.shape[0], :] = h[:, j * 128:(j + 1) * 128]

    def h_pieces(r0, c0, t, lag, n=4):
        def piece(r, pin):
            store_h(r0 + r, c0, _gelu(pin(t[r:r + 8 * n])))
        return [(functools.partial(piece, r), None, h_v, lag, 10 * n) for r in range(0, t.shape[0], 8 * n)]

    def flush(pieces):
        for p in pieces:
            p[0](lambda v, w=128: v)

    def w1_cols(c, step):
        half, cc = c // DH2, c % DH2
        return jnp.concatenate([s1_v[RAW1[half], :, cc:cc + step], s1_v[RAW1[2 + half], :, cc:cc + step]], axis=0)

    def d1_plain(xn, r0, c0, c1, step, side=None):
        for c in range(c0, c1, step):
            store_h(r0, c, _gelu(mm(xn, w1_cols(c, step), side)))

    def d1_fine(lhs, r0, nrb, cols, pieces, carry, skip=0):
        tiles = [(rb, c) for c in cols for rb in range(nrb)]
        rounds = [tiles[i:i + 4] for i in range(0, len(tiles), 4)]
        for n, (rnd, part) in enumerate(zip(rounds, split(pieces, len(rounds)))):
            sk = skip if n == 0 else 0
            side = Side(_merge(carry, part) if carry else part, 8 - sk, sk)
            carry = []
            for rb, c in rnd:
                half, cc = c // DH2, c % DH2
                t = mm(lhs(rb, 0), s1_v[RAW1[half], :, cc:cc + 128], side)
                t = mm(lhs(rb, 1), s1_v[RAW1[2 + half], :, cc:cc + 128], side, t)
                carry += h_pieces(r0 + rb * HM, c, t, LS)
        return carry

    CAP1 = (1, 1, 1, 1, 1, 1, 1)
    CAP2 = (2, 3, 3, 3, 3, 3, 2)

    def d1_s(b, slot, pieces, carry, early=()):
        for c, part, e in zip(range(0, DH2, NC1), split(pieces, DH2 // NC1), split(early, 2) + [[], []]):
            side = Side(merge(carry, part, e), CAP1 if hist else (0, 0) + CAP1[2:])
            cs = strassen(lhs_of(slot), lambda k: s1_v[k, :, c:c + NC1], side)
            carry = sum([h_pieces(b * TM + (q // 2) * HM, (q % 2) * DH2 + c, cs[q], LS) for q in (1, 2, 3, 0)], [])
        return carry

    def d2_s(b, slot, pieces, carry=(), early=(), late=()):
        for c, part, e in zip(range(0, DH2, NC1), split(pieces, DH2 // NC1), split(early, 2) + split(late, 2)):
            side = Side(merge(carry, part, e), CAP2 if hist else (0, 0) + CAP2[2:])
            carry = ()
            idx = [(slice(b * TM + (q // 2) * HM, b * TM + (q // 2 + 1) * HM),
                    slice((q % 2) * DH2 + c, (q % 2) * DH2 + c + NC1)) for q in range(4)]
            cs = strassen(lhs_of(slot), lambda k: s2_v[k, :, c:c + NC1], side,
                          [x_v[i].astype(f32) for i in idx])
            for i, t in zip(idx, cs):
                b_v[i] = t
                if b == 0:
                    c0_v[i] = t

    def split(l, n):
        w = [1.0 if hist else 0.6] + [1.0] * (n - 1)
        cut = [int(round(len(l) * sum(w[:i]) / sum(w))) for i in range(n + 1)]
        return [l[cut[i]:cut[i + 1]] for i in range(n)]

    def merge(*ls):
        ls = [l for l in ls if l]
        return _merge(*ls) if ls else []

    NW1, NW3, N30 = 32, 32, 20
    LS, LL = 3, 5

    wait("x0")
    xn0 = _pack(_ln(x_v[0:TM, :].astype(f32)))
    wait("w1a")
    d1_plain(xn0, 0, 0, 256, 256)
    wait("w1b")
    d1_plain(xn0, 0, 256, 512, 256)
    wait("x1")
    xn1 = _pack(_ln(x_v[TM:2 * TM, :].astype(f32)))
    d1_plain(xn1, TM, 0, 512, 256)
    wait("w1cd")
    hist.clear()
    xn01 = jnp.concatenate([xn0, xn1], axis=0)
    l01 = lambda rb, kh: xn01[rb * 64:(rb + 1) * 64, kh * DH2:(kh + 1) * DH2]
    pw = prep_pieces(s1_v, RAW1, LS, by_value=True)
    flush(d1_fine(l01, 0, 4, (512, 640), pw[:NW1], [], 1))
    carry = []
    wait("x23")
    hist.clear()
    carry = d1_fine(l01, 0, 4, (768, 896), ln_pieces(x_v, 2 * TM, 0, LL, plain=True), carry, 3)
    carry = d1_fine(lambda rb, kh: l_v[0, 2 * rb + kh], 2 * TM, 2, range(0, D, 128),
                    _merge(pw[NW1:], ln_pieces(x_v, 3 * TM, 1, LL)), carry)
    wait("x4567")
    qkv_start(0)
    qkv_start(1)
    hist.clear()
    for b in range(3, NB - 1):
        carry = d1_s(b, b % 2, ln_pieces(x_v, (b + 1) * TM, (b + 1) % 2, LL), carry)
    wait("w2")
    hist.clear()
    pw = prep_pieces(s2_v, RAW, LS, by_value=True)
    p3 = prep26_pieces(s3_v, 2)
    n3 = len(p3) * W3A // D4
    carry = d1_s(7, 1, _merge(pw[:NW3], shift_pieces(0, 0, LS, True)), carry)
    d2_s(0, 0, shift_pieces(TM, 1, LS, True), carry, pw[NW3:], p3[:N30])
    pw = split(_merge(p3[N30:n3], sum(ln_pieces(c0_v, 0, None, LL, clag=LS, staged=True), [])), 3)
    for b in range(1, 4):
        d2_s(b, b % 2, _merge(pw[b - 1], shift_pieces((b + 1) * TM, (b + 1) % 2, LS)))
    wait("w4", "small")
    hist.clear()
    pw = p3[n3:] + prep26_pieces(s4_v, 2)
    cut = (0, 31, 65, 99, len(pw))
    for b in range(4, NB):
        d2_s(b, b % 2, merge(pw[cut[b - 4]:cut[b - 3]],
                             shift_pieces((b + 1) * TM, (b + 1) % 2, LS) if b + 1 < NB else ()))
    start("wo", priority=1)

    def ffn(i, carry):
        qkv_wait(i)
        r0 = pl.multiple_of(i * TM, TM)
        rn = pl.multiple_of(jnp.minimum(i + 1, NB - 1) * TM, TM)
        acc = {}
        hist.clear()

        def relayout(p, r0_, r1_, pin):
            s0 = i * SPG + 2 * p
            for r in range(r0_, r1_, 8):
                e = wqkv_v[s0, r:r + 8, :]
                o = wqkv_v[s0 + 1, r:r + 8, :]
                wqkv_v[s0, r:r + 8, :] = (e & jnp.uint32(0xFFFF)) | (o << 16)
                wqkv_v[s0 + 1, r:r + 8, :] = (e >> 16) | (o & jnp.uint32(0xFFFF0000))

        relays = [(functools.partial(relayout, p, r, r + 32), wqkv_v, wqkv_v, 3, 35)
                  for p in range(SPG // 2) for r in range(0, D // 2, 32)]
        norms, combs = ln_pieces(b_v, rn, None, 5, staged=True, clag=3)

        def gate(q, pin):
            gw = gw_ref[...].astype(f32)
            x = pin(x_v[pl.ds(r0 + q, 16), :].astype(f32))
            t = functools.reduce(lambda a, b: a + b,
                                 [x[:, j * 128:(j + 1) * 128] * gw[j:j + 1, :] for j in range(NT)])
            g = jax.nn.sigmoid(jnp.sum(t, axis=-1, keepdims=True))
            g_v[pl.ds(r0 + q, 16), :] = jnp.broadcast_to(g, (16, 128))

        gates = [(functools.partial(gate, q), None, g_v, 5, 90) for q in range(0, TM, 16)]

        def extras(t, pin):
            jj, o = 2 * i + t // 2, 24 + 8 * (t % 2)
            xs = [pin(x_v[pl.ds(pl.multiple_of((jj + hh) * 64 + o, 8), 8), :].astype(f32)) for hh in (0, NPAIR // 2)]
            vals = _run(UP, [x[:, cc:cc + D4] for x in xs for cc in range(0, D, D4)])
            for k, u in enumerate(UL):
                xe_v[k, pl.ds(pl.multiple_of(i * 32 + t * 8, 8), 8), :] = vals[u].astype(bf16)

        xes = [(functools.partial(extras, t), None, xe_v, 3, 100) for t in range(4)]
        hs = {}

        def gelu_pieces(c, cs):
            def piece(r, cc, vs, pin):
                for v in vs:
                    hs[c, v, r, cc] = _gelu(pin(cs[v][r:r + 8, cc:cc + 128]))
                return [hs[c, v, r, cc] for v in vs]
            return [(functools.partial(piece, r, cc, vs), None, None, 3, 40) for r in range(0, HM, 8)
                    for cc in range(0, cs[0].shape[1], 128) for vs in ((0, 1, 2, 3), (4, 5, 6, 7))]

        def d3(c, side):
            c0, c1 = FCH[c]
            cs = fmm(lambda u: lf_v[UL.index(u)], lambda r: s3_v[r, :, c0:c1], side)
            assert not side.pieces
            return gelu_pieces(c, cs)

        def d4(c, side):
            c0, c1 = FCH[c]
            lh = _run(UP, [jnp.concatenate([jnp.concatenate(
                [hs.pop((c, v, r, cc)) for cc in range(0, c1 - c0, 128)], axis=1) for r in range(0, HM, 8)], axis=0)
                for v in range(8)])
            rhs = lambda r: s4_v[r, c0:c1, :]
            if c + 1 < len(FCH):
                for n in WORDER:
                    for r in range(RK):
                        if WN[r] == n:
                            acc[n] = mm(lh[UN[r]], rhs(r), side, acc.get(n))
            else:
                idx = lambda v: (pl.ds(r0 + (v // 4) * HM, HM), slice((v % 4) * D4, (v % 4 + 1) * D4))

                def extra(n):
                    if n >= 8:
                        return acc.get(n)
                    return b_v[idx(n)] + acc[n] if n in acc else b_v[idx(n)]

                def emit_b(v, t):
                    b_v[idx(v)] = jnp.concatenate([1.0 - g_v[idx(v)[0], :]] * 2, axis=1) * t
                fmm(lambda u: lh[u], rhs, side, extra, emit_b)
            assert not side.pieces

        g0 = d3(0, Side(relays[:20], 23, 3))
        g1 = d3(1, Side(_merge(g0, gates), 23, 2))
        d4(0, Side(g1[:22], 22, 4))
        g2 = d3(2, Side(_merge(g1[22:], relays[20:40]), 25))
        d4(1, Side(g2, 23, 2))
        g3 = d3(3, Side(_merge(relays[40:], norms, xes), 26))
        d4(2, Side(_merge(g3, combs), 23, 2))
        d4(3, Side([], 1))

        @pl.when(i + 2 < NG)
        def _():
            qkv_start(i + 2)

        return carry

    lax.fori_loop(0, NB, ffn, 0)

    def pre(it, carry):
        hist.clear()
        for u in range(3 * NG // NPRE):
            s0 = (it * (3 * NG // NPRE) + u) * G

            def rhs(r):
                t = None
                for q, sg in sorted(_terms(VP, 16, VN[r]).items(), key=lambda e: -e[1]):
                    blk = wqkv_v[s0 + q % 4 + zero_s[r], (q // 4) * (D // 8):(q // 4 + 1) * (D // 8), :]
                    if VN[r] < 16:
                        return blk
                    blk = _unpack(blk)
                    t = blk if t is None else (t + blk if sg > 0 else t - blk)
                return t.astype(bf16)
            for v, t in enumerate(fmm(lambda k: xe_v[UL.index(k)], rhs, None)):
                e_v[s0 + v % 4, (v // 4) * 128:(v // 4 + 1) * 128, :] = _pack(t)
        return carry

    lax.fori_loop(0, NPRE, pre, 0)

    wait("wo")
    mem_v[...] = mem0_ref[...].astype(f32)

    def slab(w, h):
        return (h // G) * SPG + w * G + h % G

    def step(j, hx, odd, late, allow, fill):
        qs, ks, vs, ps = {}, {}, {}, {}
        wload = lambda w, h: pltpu.bitcast(wqkv_v[slab(w, h)], bf16)
        eload = lambda w, h: pltpu.bitcast(e_v[slab(w, h), pl.ds(pl.multiple_of(j * 8, 8), 8), :], bf16)

        def proj(g):
            part = {}
            if late and g == 0:
                for h in range(2):
                    for w in range(3):
                        part[w, h] = _dot(hx[:, :DH2], wload(w, h)[:DH2])
            for h in range(g * G, (g + 1) * G):
                q, k, v = [(_dot(hx[:, DH2:], wload(w, h)[DH2:]) + part[w, h] if (w, h) in part
                            else _dot(hx, wload(w, h))).astype(bf16) for w in range(3)]
                if odd:
                    q = jnp.concatenate([q, eload(0, h)], axis=0)
                    k = jnp.concatenate([pltpu.bitcast(ke_v[h], bf16), eload(1, h), k], axis=0)
                    v = jnp.concatenate([pltpu.bitcast(ve_v[h], bf16), eload(2, h), v], axis=0)
                else:
                    ke_v[h] = pltpu.bitcast(k, u32)
                    ve_v[h] = pltpu.bitcast(v, u32)
                    k = jnp.concatenate([k, eload(1, h)], axis=0)
                    v = jnp.concatenate([v, eload(2, h)], axis=0)
                qs[h], ks[h], vs[h] = q, k, v

        def score(g):
            for h in range(g * G, (g + 1) * G):
                s = lax.dot_general(qs.pop(h), ks.pop(h), (((1,), (1,)), ((), ())),
                                    preferred_element_type=f32)
                ps[h] = _softmax(s, allow, fill)

        def pv(g):
            os_ = []
            for h in range(g * G, (g + 1) * G):
                o = _dot(ps.pop(h), vs.pop(h))
                o_v[:, h * 128:(h + 1) * 128] = _pack(o[:32])
                os_.append(o)
            if odd:
                quads = [jnp.concatenate([os_[2 * kk][r:r + 8], os_[2 * kk + 1][r:r + 8]], axis=1)
                         for r in (32, 40) for kk in range(2)]
                for k, t in enumerate(_lcombos(*quads)):
                    oe_v[k, pl.ds(pl.multiple_of(j * 8, 8), 8), g * 256:(g + 1) * 256] = t.astype(bf16)

        acc = [None] * NT

        def wo(h0, h1, j0, j1):
            o = pltpu.bitcast(o_v[:, h0 * 128:h1 * 128], bf16)
            for n in range(j0, j1):
                y = _dot(o, pltpu.bitcast(wo_v[n, h0 * 64:h1 * 64, :], bf16))
                acc[n] = y if acc[n] is None else y + acc[n]

        for t in range(NG):
            proj(t)
            if t >= 2:
                pv(t - 2)
            if t >= 1:
                score(t - 1)
        wo(0, 16, 0, 4)
        pv(NG - 2)
        score(NG - 1)
        wo(0, 16, 4, 8)
        pv(NG - 1)
        wo(16, 24, 0, 8)
        wo(24, 32, 0, 8)
        return jnp.concatenate(acc, axis=1)

    def emit(j, r0, o0, a):
        rs = pl.ds(r0 + o0, 24)
        g = jnp.concatenate([g_v[rs, :]] * NT, axis=1)
        out_v[j, o0:o0 + 24, :] = (g * a + b_v[rs, :]).astype(bf16)

    def pair(j, mem, late):
        r0 = pl.multiple_of(j * 64, 64)
        allow_e, fill_e, allow_o, fill_o = _masks()
        xa = x_v[pl.ds(r0 + 16, 8), :].astype(f32)
        xb = x_v[pl.ds(r0 + 40, 8), :].astype(f32)
        hx = jnp.concatenate([x_v[pl.ds(r0, 16), :], jnp.concatenate([xa, mem], 0).astype(bf16)], 0)
        oe = step(j, hx, False, late, allow_e, fill_e)
        emit(j, r0, 0, oe[:24])
        hx = jnp.concatenate([jnp.concatenate([oe[24:32], xb], 0).astype(bf16), x_v[pl.ds(r0 + 48, 16), :]], 0)
        oo = step(j, hx, True, True, allow_o, fill_o)
        emit(j, r0, 40, oo[8:])
        return oo[:8]

    def a_iter(it, carry):
        mem = mem_v[...]
        for t in range(PPI):
            mem = pair(it * PPI + t, mem, t > 0)
        mem_v[...] = mem
        for t in range(PPI):
            for o0 in (0, 40):
                idx = (it * PPI + t, pl.ds(o0, 24))
                pltpu.make_async_copy(out_v.at[idx], out_hbm.at[idx], sem_out).start()
        return carry

    lax.fori_loop(0, NPAIR // PPI, a_iter, 0)

    hist.clear()
    for n in range(NT // 2):
        quad = [lambda k, t=2 * n + q % 2, o=(q // 2) * 128: jnp.concatenate(
            [wo_v[t + zero_s[k], g * 256 + o:g * 256 + o + 128, :] for g in range(NG)], axis=0) for q in range(4)]
        cs = strassen(lambda k: oe_v[k], lambda k: _rcombo(k, *quad), None)
        cols = slice(n * 256, (n + 1) * 256)
        for half in range(2):
            t = jnp.concatenate(cs[2 * half:2 * half + 2], axis=1)
            o0 = 24 + half * 8
            for jj in range(NPAIR):
                rs = slice(jj * 64 + o0, jj * 64 + o0 + 8)
                g = jnp.concatenate([g_v[rs, :]] * 2, axis=1)
                out_v[jj, o0:o0 + 8, cols] = (g * t[jj * 8:jj * 8 + 8] + b_v[rs, cols]).astype(bf16)
        if n >= 2:
            idx = (slice(None), pl.ds(24, 16), pl.ds(0, 768) if n == 2 else pl.ds(768, 256))
            pltpu.make_async_copy(out_v.at[idx], out_hbm.at[idx], sem_out).start()
    pltpu.make_async_copy(out_v, out_hbm, sem_out).wait()


@functools.partial(jax.jit, static_argnames=("A_seg_len",))
def pallas_gated_mix__memory_aug_recurrent_mem_tr__mixer_s_mlp__prompt_kernel(
    A_x, A_mem0, A_Wq, A_Wk, A_Wv, A_Wo, A_seg_len, B_x, B_w1, B_w2, B_w3, B_w4, gate_w,
):
    assert A_seg_len == SEG
    assert A_x.shape == (1, S, D) and A_mem0.shape == (1, M, D)
    any_spec = pl.BlockSpec(memory_space=pl.ANY)
    out = pl.pallas_call(
        _kernel,
        out_shape=jax.ShapeDtypeStruct((NPAIR, 64, D), bf16),
        in_specs=[any_spec] * 11,
        out_specs=any_spec,
        scratch_shapes=[
            pltpu.VMEM((S, D), bf16),
            pltpu.VMEM((9, D // 4, D // 2), u32),
            pltpu.VMEM((7, D // 4, D // 2), u32),
            pltpu.VMEM((RK, D4, F4), bf16),
            pltpu.VMEM((RK, F4, D4), bf16),
            pltpu.VMEM((3 * H, D // 2, DH), u32),
            pltpu.VMEM((NT, H * DH // 2, 128), u32),
            pltpu.VMEM((NT, S + 2 * PAD, 128), f32),
            pltpu.VMEM((S, D), f32),
            pltpu.VMEM((TM, D), f32),
            pltpu.VMEM((2, 7, HM // 2, D // 2), u32),
            pltpu.VMEM((len(UL), HM, D4), bf16),
            pltpu.VMEM((2, TM, 128), f32),
            pltpu.VMEM((S, 128), f32),
            pltpu.VMEM((NPAIR, 64, D), bf16),
            pltpu.VMEM((len(UL), 8 * NPAIR, D4), bf16),
            pltpu.VMEM((3 * H, 8 * NPAIR, DH), u32),
            pltpu.VMEM((7, 8 * NPAIR, H * DH // 2), bf16),
            pltpu.VMEM((H, 16, 128), u32),
            pltpu.VMEM((H, 16, 128), u32),
            pltpu.VMEM((16, H * DH), u32),
            pltpu.VMEM((M, D), f32),
            pltpu.VMEM((M, D), bf16),
            pltpu.VMEM((NT, 128), bf16),
            pltpu.SMEM((RK,), jnp.int32),
            pltpu.SemaphoreType.DMA((NLOAD,)),
            pltpu.SemaphoreType.DMA((NG,)),
            pltpu.SemaphoreType.DMA,
        ],
        compiler_params=pltpu.CompilerParams(vmem_limit_bytes=126 * 1024 * 1024,
                                             disable_bounds_checks=True),
    )(
        A_x.reshape(S, D), A_mem0.reshape(M, D),
        A_Wq.reshape(D // 2, 2 * H, DH), A_Wk.reshape(D // 2, 2 * H, DH), A_Wv.reshape(D // 2, 2 * H, DH),
        A_Wo.reshape(H * DH, D), B_w1, B_w2, B_w3, B_w4, gate_w.reshape(NT, 128),
    )
    return out.reshape(1, S, D)
```

```python
import functools

import jax
import jax.numpy as jnp
from jax import lax
import jax.experimental.pallas as pl
import jax.experimental.pallas.tpu as pltpu

f32, bf16, u32 = jnp.float32, jnp.bfloat16, jnp.uint32

S, D, H, DH, M, SEG, F = 2048, 1024, 32, 128, 8, 32, 3584
SCALE = DH ** -0.5
NEG = -1000000000.0
EPS = 1e-05

TM = 256
NB = S // TM
HM = TM // 2
DH2 = D // 2
D4, F4 = D // 4, F // 4
FCH = ((0, 128), (128, 384), (384, 640), (640, 896))
NC1 = 128
NPAIR = S // (2 * SEG)
PPI = 2
NPRE = 3
G = 4
NG = H // G
PAD = 8
NT = D // 128
W3A = 192
NLOAD = 11
assert NB == NG

_dot = functools.partial(jnp.dot, preferred_element_type=f32)

UP = ((4, 1, 5, 1), (6, 1, 8, 1), (0, 1, 3, 1), (2, -1, 9, 1), (4, -1, 10, 1), (0, 1, 1, 1), (2, 1, 12, 1),
      (5, 1, 7, -1), (7, 1, 12, -1), (11, -1, 13, 1), (10, -1, 11, 1), (2, 1, 7, 1), (0, -1, 4, 1),
      (6, 1, 7, 1), (1, -1, 5, 1), (3, 1, 7, -1), (1, 1, 4, 1), (2, 1, 3, 1), (1, -1, 3, 1), (1, 1, 7, -1),
      (2, 1, 6, -1))
WP = ((0, -1, 3, 1), (4, 1, 6, -1), (1, 1, 8, 1), (5, 1, 10, 1), (4, -1, 7, 1), (0, -1, 9, -1),
      (11, 1, 12, 1), (6, 1, 7, -1), (2, 1, 5, -1), (0, -1, 7, -1), (9, 1, 11, -1), (2, 1, 13, 1),
      (5, 1, 13, 1), (2, -1, 3, 1), (5, 1, 6, 1), (0, 1, 4, 1), (2, 1, 7, 1), (1, 1, 2, 1), (1, 1, 5, 1),
      (3, 1, 7, 1), (2, 1, 6, 1))
VP = ((1, 1, 5, -1), (8, 1, 11, 1), (10, 1, 17, 1), (13, 1, 16, -1), (0, 1, 4, -1), (0, 1, 3, 1),
      (14, 1, 18, -1), (0, 1, 11, 1), (14, 1, 19, -1), (0, 1, 5, 1), (12, 1, 15, 1), (2, 1, 21, 1),
      (10, 1, 14, -1), (4, 1, 7, 1), (11, 1, 19, 1), (12, -1, 20, 1), (13, 1, 14, -1), (9, 1, 30, -1),
      (3, -1, 15, 1), (6, 1, 23, 1), (24, 1, 27, -1), (9, -1, 18, 1), (7, 1, 34, 1), (2, 1, 6, -1),
      (0, 1, 8, -1), (6, 1, 21, 1), (22, 1, 31, -1), (6, 1, 29, 1), (0, 1, 1, 1), (15, 1, 25, 1),
      (5, 1, 37, 1), (15, 1, 20, 1))
UN = (7, 27, 24, 17, 9, 22, 21, 2, 15, 11, 8, 25, 19, 28, 2, 23, 26, 20, 1, 18, 10, 28, 4, 13, 14, 16)
WN = (23, 17, 24, 10, 14, 7, 22, 19, 12, 18, 15, 25, 20, 5, 26, 0, 8, 2, 27, 11, 26, 9, 28, 21, 16, 5)
VN = (42, 47, 41, 5, 11, 43, 18, 28, 20, 23, 35, 19, 22, 46, 33, 26, 45, 36, 38, 25, 44, 40, 39, 21, 24, 32)
RK = len(UN)
UL = tuple(sorted(set(UN)))
VSTAGES = ((0, 6, 7, 12, 13, 14, 15, 21), (11, 17, 20, 22, 24, 25, 23, 2), (1, 5, 8, 9, 10, 16, 18, 19))
RAW16 = (1, 11, 17, 5, 8, 3, 9, 10, 0, 6, 7, 4, 12, 20, 22, 16)


def _run(prog, blocks):
    vals = list(blocks)
    for a, sa, b, sb in prog:
        vals.append(vals[a] + vals[b] if sa > 0 and sb > 0 else
                    vals[a] - vals[b] if sa > 0 else vals[b] - vals[a])
    return vals


def _terms(prog, nin, node):
    if node < nin:
        return {node: 1}
    a, sa, b, sb = prog[node - nin]
    out = {k: sa * v for k, v in _terms(prog, nin, a).items()}
    out.update({k: sb * v for k, v in _terms(prog, nin, b).items()})
    return out


for _b in range(16):
    _last = max(k for k, st in enumerate(VSTAGES) for r in st if _b in _terms(VP, 16, VN[r]))
    assert VN[RAW16[_b]] == _b or RAW16[_b] in VSTAGES[_last]
assert sorted(sum(VSTAGES, ())) == [r for r in range(RK) if VN[r] >= 16] and len(set(RAW16)) == 16

_WPAR = {n: [] for n in range(8 + len(WP))}
for _t, (_a, _sa, _b, _sb) in enumerate(WP):
    _WPAR[_a].append((8 + _t, _sa))
    _WPAR[_b].append((8 + _t, _sb))


def _worder():
    order = []

    def closure(n, acc):
        if n not in acc and n not in order:
            acc.add(n)
            for q, _ in _WPAR[n]:
                closure(q, acc)
        return acc

    def visit(n):
        if n not in order:
            for q, _ in _WPAR[n]:
                visit(q)
            order.append(n)
    while len([v for v in range(8) if v not in order]):
        visit(min((v for v in range(8) if v not in order), key=lambda v: len(closure(v, set()))))
    return tuple(order)


WORDER = _worder()


def _ln(x):
    m = jnp.mean(x, axis=-1, keepdims=True)
    xc = x - m
    v = jnp.mean(xc * xc, axis=-1, keepdims=True)
    return xc * lax.rsqrt(v + EPS)


_GC = 0.7978845608028654


def _gelu(x):
    h = 0.5 * x
    return h + h * jnp.tanh(x * (_GC + (_GC * 0.044715) * (x * x)))


def _unpack(u):
    return pltpu.bitcast(u, bf16).astype(f32)


def _pack(x):
    return pltpu.bitcast(x.astype(bf16), u32)


def _lcombos(a11, a12, a21, a22):
    return [a11 + a22, a21 + a22, a11, a22, a11 + a12, a21 - a11, a12 - a22]


def _merge(*lists):
    keyed = [((j + 0.5) / len(l), n, j, v) for n, l in enumerate(lists) for j, v in enumerate(l)]
    return [v for _, _, _, v in sorted(keyed, key=lambda t: t[:3])]


def _masks():
    r = lax.broadcasted_iota(jnp.int32, (32, 48), 0)
    c = lax.broadcasted_iota(jnp.int32, (32, 48), 1)
    exist_e = c < 40
    allow_e = exist_e & ((r >= 24) | ((c >= 24) & (c < 32)) | (c <= r))
    fill_e = jnp.where(exist_e, NEG, -jnp.inf).astype(f32)
    r = lax.broadcasted_iota(jnp.int32, (48, 80), 0)
    c = lax.broadcasted_iota(jnp.int32, (48, 80), 1)
    q_even = (r >= 32) & (r < 40)
    exist_o = (q_even & (c < 40)) | (~q_even & (c >= 40))
    ktok = jnp.where(c < 24, c, jnp.where(c < 48, c - 8, c - 16))
    qtok = jnp.where(r < 32, r + 32, r - 8)
    is_mem_key = ((c >= 24) & (c < 32)) | ((c >= 48) & (c < 56))
    allow_o = exist_o & (is_mem_key | (r < 8) | (ktok <= qtok))
    fill_o = jnp.where(exist_o, NEG, -jnp.inf).astype(f32)
    return allow_e, fill_e, allow_o, fill_o


def _rcombo(k, b11, b12, b21, b22):
    if k in (1, 4):
        return (b11 if k == 1 else b22)(k)
    a, b, sign = {0: (b11, b22, 1), 2: (b12, b22, -1), 3: (b21, b11, -1), 5: (b11, b12, 1), 6: (b21, b22, 1)}[k]
    a, b = _unpack(a(k)), _unpack(b(k))
    return (a + b if sign > 0 else a - b).astype(bf16)


def _softmax(s, allow, fill):
    s = jnp.where(allow, s * SCALE, fill)
    m = jnp.max(s, axis=-1, keepdims=True)
    e = jnp.exp(s - m)
    l = jnp.sum(e, axis=-1, keepdims=True)
    r = pl.reciprocal(l, approx=True)
    r = r * (2.0 - l * r)
    return (e * r).astype(bf16)


def _kernel(x_hbm, mem0_hbm, wq_hbm, wk_hbm, wv_hbm, wo_hbm, w1_hbm, w2_hbm, w3_hbm, w4_hbm,
            gw_hbm, out_hbm,
            x_v, s1_v, s2_v, s3_v, s4_v, wqkv_v, wo_v, h_v, b_v, c0_v, l_v, lf_v, n_v, g_v, out_v, xe_v, e_v, oe_v,
            ke_v, ve_v, o_v, mem_v, mem0_ref, gw_ref, zero_s,
            sem, sem_qkv, sem_out):
    RAW = (1, 2, 3, 4)
    RAW1 = (1, 7, 8, 4)

    loads = []

    def rows_load(name, r0, r1):
        loads.append((name, x_hbm.at[pl.ds(r0, r1 - r0)], x_v.at[pl.ds(r0, r1 - r0)]))

    def quad_load(name, w_hbm, s_v, raw, q, c0=0, c1=None):
        k4, n2 = s_v.shape[1], s_v.shape[2]
        c1 = n2 if c1 is None else c1
        src = w_hbm.bitcast(u32).at[pl.ds((q // 2) * k4, k4), pl.ds((q % 2) * n2 + c0, c1 - c0)]
        loads.append((name, src, s_v.at[raw[q], :, pl.ds(c0, c1 - c0)]))

    def w1_load(name, half, c0, c1):
        quad_load(name, w1_hbm, s1_v, RAW1, half, c0, c1)
        quad_load(name, w1_hbm, s1_v, RAW1, 2 + half, c0, c1)

    def block_load(name, w_hbm, s_v, r0, r1):
        kb, nb = s_v.shape[1:]
        for q in range(16):
            loads.append((name, w_hbm.at[pl.ds((q // 4) * kb + r0, r1 - r0), pl.ds((q % 4) * nb, nb)],
                          s_v.at[RAW16[q], pl.ds(r0, r1 - r0)]))

    rows_load("x0", 0, TM)
    w1_load("w1a", 0, 0, 256)
    w1_load("w1b", 0, 256, 512)
    rows_load("x1", TM, 2 * TM)
    w1_load("w1cd", 1, 0, 512)
    rows_load("x23", 2 * TM, 4 * TM)
    rows_load("x4567", 4 * TM, S)
    for q in range(4):
        quad_load("w2", w2_hbm, s2_v, RAW, q)
    block_load("w2", w3_hbm, s3_v, 0, W3A)
    block_load("w4", w3_hbm, s3_v, W3A, D4)
    block_load("w4", w4_hbm, s4_v, 0, F4)
    loads.append(("small", mem0_hbm, mem0_ref))
    loads.append(("small", gw_hbm, gw_ref))
    for j in range(NT):
        loads.append(("wo", wo_hbm.bitcast(u32).at[:, pl.ds(j * 128, 128)], wo_v.at[j]))
    groups = list(dict.fromkeys(name for name, _, _ in loads))
    assert len(groups) == NLOAD

    def start(*names, priority=0):
        for name, src, dst in loads:
            if name in names:
                pltpu.make_async_copy(src, dst, sem.at[groups.index(name)]).start(priority=priority)

    def wait(*names):
        for name, src, dst in loads:
            if name in names:
                pltpu.make_async_copy(src, dst, sem.at[groups.index(name)]).wait()

    SPG = 3 * G

    def qkv_start(g):
        for w, w_hbm in enumerate((wq_hbm, wk_hbm, wv_hbm)):
            wu = w_hbm.bitcast(u32)
            for k in range(G // 2):
                for par in range(2):
                    pltpu.make_async_copy(
                        wu.at[:, par * (H // 2) + g * (G // 2) + k, :],
                        wqkv_v.at[g * SPG + w * G + 2 * k + par], sem_qkv.at[g]).start(priority=1)

    def qkv_wait(g):
        grp = wqkv_v.at[pl.ds(g * SPG, SPG)]
        pltpu.make_async_copy(grp, grp, sem_qkv.at[g]).wait()

    start("x0", "w1a", "w1b", "x1", "w1cd", "x23", "x4567", "w2", "w4", "small")

    def zero(k, carry):
        zero_s[k] = 0
        return carry
    lax.fori_loop(0, RK, zero, 0)

    def tile_idx(ref, cols=128):
        z = zero_s[0]
        n = 16 if ref.dtype == bf16 and cols == 128 else 8
        return (z,) * (len(ref.shape) - 2) + (pl.ds(pl.multiple_of(z, n), n), slice(0, cols))

    TIE26 = 16
    rot = [0]
    ROT = 0
    hist = []

    def mm(lhs, rhs, side=None, acc=None):
        if side is not None:
            lhs = side(lhs)
        lhs = pltpu.bitcast(lhs, bf16) if lhs.dtype == u32 else lhs.astype(bf16)
        y = _dot(lhs, pltpu.bitcast(rhs, bf16) if rhs.dtype == u32 else rhs)
        if acc is not None:
            y = y + acc
        hist.append(y)
        return y

    class Side:
        def __init__(self, pieces, n, skip=0):
            cap = [0] * skip + ([1] * n if isinstance(n, int) else list(n))
            tot = sum(p[4] for p in pieces)
            self.plan = [[] for _ in cap]
            done = 0
            for p in pieces:
                done += p[4]
                x, d = done / tot * sum(cap), 0
                while x > cap[d] + 1e-9:
                    x -= cap[d]
                    d += 1
                self.plan[d].append((p, x / cap[d]))
            self.pieces = len(pieces)

        def __call__(self, val):
            todo = self.plan.pop(0) if self.plan else []
            if not todo:
                return val
            self.pieces -= len(todo)
            never = zero_s[0] > 0
            if val.dtype == bf16:
                val = pltpu.bitcast(val, u32)
            rg = 8 if val.dtype == u32 else 16
            ng = val.shape[0] // rg
            groups = [val[8 * m:8 * m + 8] for m in range(val.shape[0] // 8)]
            nk = val.shape[1] // 128
            used = {}
            npass = max(nk // 4, 1)
            for (fn, rd, wr, lag, _), pos in todo:
                sl = max(-int(-pos * ng * npass // 1) - 1, 0)
                m = sl % ng
                rot[0] += ROT
                kt = (sl // ng) * 4 + (rot[0] - 1) % min(nk, 4)
                pin = lambda v, w=128: v
                if lag is not None and len(hist) >= lag:
                    r0 = (16 * m) % hist[-lag].shape[0]
                    a = hist[-lag][r0:r0 + 8, :128]
                    if rd is None:
                        def pin(v, w=128, a=a):
                            a = jnp.concatenate([pltpu.bitcast(a, v.dtype)] * (v.shape[0] // 8), axis=0)
                            t = jnp.where(never, jnp.concatenate([a] * (w // 128), axis=1), v[:, :w])
                            return t if v.shape[1] == w else jnp.concatenate([t, v[:, w:]], axis=1)
                    elif rd.dtype == bf16:
                        idx = tile_idx(rd, 256)
                        rd[idx] = jnp.where(never, jnp.concatenate([a, a], axis=1).astype(bf16), rd[idx])
                    else:
                        idx = tile_idx(rd)
                        rd[idx] = jnp.where(never, pltpu.bitcast(a, rd.dtype), rd[idx])
                tiles = fn(pin)
                if wr is False:
                    continue
                g = m * rg // 8
                ks = [groups[g][:, k * 128:(k + 1) * 128] for k in range(nk)]
                u = functools.reduce(lambda a, b: a + b, tiles) if wr is None else wr[tile_idx(wr)]
                used[g, kt] = used.get((g, kt), -1) + 1
                ks[kt] = jnp.where(zero_s[used[g, kt]] > 0, pltpu.bitcast(u, val.dtype), ks[kt])
                groups[g] = jnp.concatenate(ks, axis=1)
            return jnp.concatenate(groups, axis=0)

    def strassen(lhs, rhs, side, init=(None, None, None, None)):
        def add(a, b):
            return a if b is None else a + b
        p = [mm(lhs(k), rhs(k), side) for k in range(5)]
        c12 = add(p[2] + p[4], init[1])
        c21 = add(p[1] + p[3], init[2])
        c22 = mm(lhs(5), rhs(5), side, add(p[0] - p[1] + p[2], init[3]))
        c11 = mm(lhs(6), rhs(6), side, add(p[0] + p[3] - p[4], init[0]))
        return c11, c12, c21, c22

    def fmm(lhs, rhs, side, extra=lambda n: None, emit=None):
        val = {}
        for n in WORDER:
            t = extra(n)
            for q, sg in sorted(_WPAR[n], key=lambda e: -e[1]):
                t = val[q] if t is None else (t + val[q] if sg > 0 else t - val[q])
            for r in range(RK):
                if WN[r] == n:
                    t = mm(lhs(UN[r]), rhs(r), side, t)
            val[n] = t
            if n < 8 and emit is not None:
                emit(n, t)
        return [val[v] for v in range(8)]

    def prep26_pieces(s_v, lag, stages=(sum(VSTAGES, ()),)):
        def piece(rs, cs, stage, pin):
            @functools.lru_cache(None)
            def node(n):
                if n < 16:
                    return s_v[RAW16[n], rs, cs].astype(f32)
                return _run([(0, VP[n - 16][1], 1, VP[n - 16][3])], [node(VP[n - 16][0]), node(VP[n - 16][2])])[-1]
            vals = [node(VN[r]).astype(bf16) for r in stage]
            for r, t in zip(stage, vals):
                s_v[r, rs, cs] = t
        kb, nb = s_v.shape[1:]
        out = []
        for r in range(0, kb, 16):
            out += [(slice(rr, rr + 8), slice(c, c + 256)) for c in range(0, nb - 255, 256) for rr in (r, r + 8)]
            out += [(slice(rr, rr + 8), slice(nb - 128, nb)) for rr in (r, r + 8)] if nb % 256 else []
        return [(functools.partial(piece, rs, cs, st), s_v, s_v if n % TIE26 == TIE26 - 1 else False, lag,
                 130 if cs.stop - cs.start == 256 else 100) for n, (rs, cs) in enumerate(out) for st in stages]

    def prep_pieces(s_v, raw, lag, width=256, by_value=False):
        def piece(r, c, pin):
            idx = (slice(r, r + 8), slice(c, c + width))
            b11, b12, b21, b22 = [_unpack(pin(s_v[(q,) + idx], width) if n in (0, 3) else s_v[(q,) + idx])
                                  for n, q in enumerate(raw)]
            for k, t in ((0, b11 + b22), (2, b12 - b22), (3, b21 - b11), (5, b11 + b12), (6, b21 + b22)):
                s_v[(k,) + idx] = _pack(t)
        return [(functools.partial(piece, r, c), None if by_value else s_v, s_v, lag, 80)
                for c in range(0, s_v.shape[2], width) for r in range(0, s_v.shape[1], 8)]

    def store_l(slot, q, c, quads, plain=False):
        for k, t in enumerate(quads if plain else _lcombos(*quads)):
            l_v[slot, k, q // 2:q // 2 + 8, c:c + t.shape[1]] = _pack(t)

    def ln_pieces(src, r0, slot, lag, plain=False, width=256, staged=False, clag=None):
        def stats(q, pin):
            x = pin(src[pl.ds(r0 + q, 16), :].astype(f32))
            xs = [x[:, j * 128:(j + 1) * 128] for j in range(NT)]
            m = functools.reduce(lambda a, b: a + b, xs) * (1.0 / NT)
            w = functools.reduce(lambda a, b: a + b, [(t - m) * (t - m) for t in xs])
            mean = jnp.mean(m, axis=-1, keepdims=True)
            var = jnp.sum(w + NT * ((m - mean) * (m - mean)), axis=-1, keepdims=True) * (1.0 / D)
            n_v[0, q:q + 16, :] = jnp.broadcast_to(mean, (16, 128))
            n_v[1, q:q + 16, :] = jnp.broadcast_to(lax.rsqrt(var + EPS), (16, 128))

        def comb(q, c, pin):
            quads = []
            for rr in (0, HM):
                rs = pl.ds(pl.multiple_of(r0 + rr + q + zero_s[0], 16), 16)
                mean, rstd = [jnp.concatenate([n_v[t, rr + q:rr + q + 16, :]] * (width // 128), axis=1)
                              for t in range(2)]
                quads += [(src[rs, cc + c:cc + c + width].astype(f32) - mean) * rstd for cc in (0, DH2)]
            store_l(slot, q, c, quads, plain)

        def comb26(q, pin):
            blocks = []
            for rr in (0, HM):
                rs = pl.ds(pl.multiple_of(r0 + rr + q + zero_s[0], 8), 8)
                mean, rstd = [jnp.concatenate([n_v[t, rr + q:rr + q + 8, :]] * 2, axis=1) for t in range(2)]
                blocks += [(src[rs, cc:cc + D4] - mean) * rstd for cc in range(0, D, D4)]
            vals = _run(UP, blocks)
            for k, u in enumerate(UL):
                lf_v[k, q:q + 8, :] = vals[u].astype(bf16)
        norms = [[(functools.partial(stats, rr + q), None, n_v if slot is not None else False, lag, 90) for rr in (0, HM)]
                 for q in range(0, HM, 16)]
        if slot is None:
            combs = [[(functools.partial(comb26, qq), n_v, lf_v if qq % 32 == 24 else False, clag, 110) for qq in (q, q + 8)]
                     for q in range(0, HM, 16)]
        else:
            combs = [[(functools.partial(comb, q, c), n_v, l_v, clag, 125) for c in range(0, DH2, width)]
                     for q in range(0, HM, 16)]
        if staged:
            return sum(norms, []), sum(combs, [])
        out = list(norms[0])
        for a, b in zip(norms[1:] + [[]], combs):
            out += _merge(a, b) if a else b
        return out

    shifts = (1, 1, -1, -1, 2, 2, -2, -2)

    def shift_pieces(r0, slot, lag, by_value=False):
        def piece(q, j, pin):
            a = [h_v[jj, pl.ds(PAD + r0 + rr + q - shifts[jj], 16), :]
                 for rr in (0, HM) for jj in (j, j + NT // 2)]
            store_l(slot, q, j * 128, [pin(a[0]), a[1], a[2], pin(a[3])])
        return [(functools.partial(piece, q, j), None if by_value else h_v, l_v if (q // 16) % 2 and j == 3 else False, lag, 50)
                for q in range(0, HM, 16) for j in range(NT // 2)]

    def lhs_of(slot):
        return lambda k: l_v[slot, k]

    h_v[:, 0:PAD, :] = jnp.zeros((NT, PAD, 128), f32)
    h_v[:, PAD + S:PAD + S + PAD, :] = jnp.zeros((NT, PAD, 128), f32)

    def store_h(r0, c0, h):
        for j in range(h.shape[1] // 128):
            h_v[c0 // 128 + j, PAD + r0:PAD + r0 + h.shape[0], :] = h[:, j * 128:(j + 1) * 128]

    def h_pieces(r0, c0, t, lag, n=4):
        def piece(r, pin):
            store_h(r0 + r, c0, _gelu(pin(t[r:r + 8 * n])))
        return [(functools.partial(piece, r), None, h_v, lag, 10 * n) for r in range(0, t.shape[0], 8 * n)]

    def flush(pieces):
        for p in pieces:
            p[0](lambda v, w=128: v)

    def w1_cols(c, step):
        half, cc = c // DH2, c % DH2
        return jnp.concatenate([s1_v[RAW1[half], :, cc:cc + step], s1_v[RAW1[2 + half], :, cc:cc + step]], axis=0)

    def d1_plain(xn, r0, c0, c1, step, side=None):
        for c in range(c0, c1, step):
            store_h(r0, c, _gelu(mm(xn, w1_cols(c, step), side)))

    def d1_fine(lhs, r0, nrb, cols, pieces, carry, skip=0):
        tiles = [(rb, c) for c in cols for rb in range(nrb)]
        rounds = [tiles[i:i + 4] for i in range(0, len(tiles), 4)]
        for n, (rnd, part) in enumerate(zip(rounds, split(pieces, len(rounds)))):
            sk = skip if n == 0 else 0
            side = Side(_merge(carry, part) if carry else part, 8 - sk, sk)
            carry = []
            for rb, c in rnd:
                half, cc = c // DH2, c % DH2
                t = mm(lhs(rb, 0), s1_v[RAW1[half], :, cc:cc + 128], side)
                t = mm(lhs(rb, 1), s1_v[RAW1[2 + half], :, cc:cc + 128], side, t)
                carry += h_pieces(r0 + rb * HM, c, t, LS)
        return carry

    CAP1 = (1, 1, 1, 1, 1, 1, 1)
    CAP2 = (2, 3, 3, 3, 3, 3, 2)

    def d1_s(b, slot, pieces, carry, early=()):
        for c, part, e in zip(range(0, DH2, NC1), split(pieces, DH2 // NC1), split(early, 2) + [[], []]):
            side = Side(merge(carry, part, e), CAP1 if hist else (0, 0) + CAP1[2:])
            cs = strassen(lhs_of(slot), lambda k: s1_v[k, :, c:c + NC1], side)
            carry = sum([h_pieces(b * TM + (q // 2) * HM, (q % 2) * DH2 + c, cs[q], LS) for q in (1, 2, 3, 0)], [])
        return carry

    def d2_s(b, slot, pieces, carry=(), early=(), late=()):
        for c, part, e in zip(range(0, DH2, NC1), split(pieces, DH2 // NC1), split(early, 2) + split(late, 2)):
            side = Side(merge(carry, part, e), CAP2 if hist else (0, 0) + CAP2[2:])
            carry = ()
            idx = [(slice(b * TM + (q // 2) * HM, b * TM + (q // 2 + 1) * HM),
                    slice((q % 2) * DH2 + c, (q % 2) * DH2 + c + NC1)) for q in range(4)]
            cs = strassen(lhs_of(slot), lambda k: s2_v[k, :, c:c + NC1], side,
                          [x_v[i].astype(f32) for i in idx])
            for i, t in zip(idx, cs):
                b_v[i] = t
                if b == 0:
                    c0_v[i] = t

    def split(l, n):
        w = [1.0 if hist else 0.6] + [1.0] * (n - 1)
        cut = [int(round(len(l) * sum(w[:i]) / sum(w))) for i in range(n + 1)]
        return [l[cut[i]:cut[i + 1]] for i in range(n)]

    def merge(*ls):
        ls = [l for l in ls if l]
        return _merge(*ls) if ls else []

    NW1, NW3, N30 = 32, 32, 20
    LS, LL = 3, 5

    wait("x0")
    xn0 = _pack(_ln(x_v[0:TM, :].astype(f32)))
    wait("w1a")
    d1_plain(xn0, 0, 0, 256, 256)
    wait("w1b")
    d1_plain(xn0, 0, 256, 512, 256)
    wait("x1")
    xn1 = _pack(_ln(x_v[TM:2 * TM, :].astype(f32)))
    d1_plain(xn1, TM, 0, 512, 256)
    wait("w1cd")
    hist.clear()
    xn01 = jnp.concatenate([xn0, xn1], axis=0)
    l01 = lambda rb, kh: xn01[rb * 64:(rb + 1) * 64, kh * DH2:(kh + 1) * DH2]
    pw = prep_pieces(s1_v, RAW1, LS, by_value=True)
    flush(d1_fine(l01, 0, 4, (512, 640), pw[:NW1], [], 1))
    carry = []
    wait("x23")
    hist.clear()
    carry = d1_fine(l01, 0, 4, (768, 896), ln_pieces(x_v, 2 * TM, 0, LL, plain=True), carry, 3)
    carry = d1_fine(lambda rb, kh: l_v[0, 2 * rb + kh], 2 * TM, 2, range(0, D, 128),
                    _merge(pw[NW1:], ln_pieces(x_v, 3 * TM, 1, LL)), carry)
    wait("x4567")
    qkv_start(0)
    qkv_start(1)
    hist.clear()
    for b in range(3, NB - 1):
        carry = d1_s(b, b % 2, ln_pieces(x_v, (b + 1) * TM, (b + 1) % 2, LL), carry)
    wait("w2")
    hist.clear()
    pw = prep_pieces(s2_v, RAW, LS, by_value=True)
    p3 = prep26_pieces(s3_v, 2)
    n3 = len(p3) * W3A // D4
    carry = d1_s(7, 1, _merge(pw[:NW3], shift_pieces(0, 0, LS, True)), carry)
    d2_s(0, 0, shift_pieces(TM, 1, LS, True), carry, pw[NW3:], p3[:N30])
    pw = split(_merge(p3[N30:n3], sum(ln_pieces(c0_v, 0, None, LL, clag=LS, staged=True), [])), 3)
    for b in range(1, 4):
        d2_s(b, b % 2, _merge(pw[b - 1], shift_pieces((b + 1) * TM, (b + 1) % 2, LS)))
    wait("w4", "small")
    hist.clear()
    pw = p3[n3:] + prep26_pieces(s4_v, 2)
    cut = (0, 31, 65, 99, len(pw))
    for b in range(4, NB):
        d2_s(b, b % 2, merge(pw[cut[b - 4]:cut[b - 3]],
                             shift_pieces((b + 1) * TM, (b + 1) % 2, LS) if b + 1 < NB else ()))
    start("wo", priority=1)

    def ffn(i, carry):
        qkv_wait(i)
        r0 = pl.multiple_of(i * TM, TM)
        rn = pl.multiple_of(jnp.minimum(i + 1, NB - 1) * TM, TM)
        acc = {}
        hist.clear()

        def relayout(p, r0_, r1_, pin):
            s0 = i * SPG + 2 * p
            for r in range(r0_, r1_, 8):
                e = wqkv_v[s0, r:r + 8, :]
                o = wqkv_v[s0 + 1, r:r + 8, :]
                wqkv_v[s0, r:r + 8, :] = (e & jnp.uint32(0xFFFF)) | (o << 16)
                wqkv_v[s0 + 1, r:r + 8, :] = (e >> 16) | (o & jnp.uint32(0xFFFF0000))

        relays = [(functools.partial(relayout, p, r, r + 32), wqkv_v, wqkv_v, 3, 35)
                  for p in range(SPG // 2) for r in range(0, D // 2, 32)]
        norms, combs = ln_pieces(b_v, rn, None, 5, staged=True, clag=3)

        def gate(q, pin):
            gw = gw_ref[...].astype(f32)
            x = pin(x_v[pl.ds(r0 + q, 16), :].astype(f32))
            t = functools.reduce(lambda a, b: a + b,
                                 [x[:, j * 128:(j + 1) * 128] * gw[j:j + 1, :] for j in range(NT)])
            g = jax.nn.sigmoid(jnp.sum(t, axis=-1, keepdims=True))
            g_v[pl.ds(r0 + q, 16), :] = jnp.broadcast_to(g, (16, 128))

        gates = [(functools.partial(gate, q), None, g_v, 5, 90) for q in range(0, TM, 16)]

        def extras(t, pin):
            jj, o = 2 * i + t // 2, 24 + 8 * (t % 2)
            xs = [pin(x_v[pl.ds(pl.multiple_of((jj + hh) * 64 + o, 8), 8), :].astype(f32)) for hh in (0, NPAIR // 2)]
            vals = _run(UP, [x[:, cc:cc + D4] for x in xs for cc in range(0, D, D4)])
            for k, u in enumerate(UL):
                xe_v[k, pl.ds(pl.multiple_of(i * 32 + t * 8, 8), 8), :] = vals[u].astype(bf16)

        xes = [(functools.partial(extras, t), None, xe_v, 3, 100) for t in range(4)]
        hs = {}

        def gelu_pieces(c, cs):
            def piece(r, cc, vs, pin):
                for v in vs:
                    hs[c, v, r, cc] = _gelu(pin(cs[v][r:r + 8, cc:cc + 128]))
                return [hs[c, v, r, cc] for v in vs]
            return [(functools.partial(piece, r, cc, vs), None, None, 3, 40) for r in range(0, HM, 8)
                    for cc in range(0, cs[0].shape[1], 128) for vs in ((0, 1, 2, 3), (4, 5, 6, 7))]

        def d3(c, side):
            c0, c1 = FCH[c]
            cs = fmm(lambda u: lf_v[UL.index(u)], lambda r: s3_v[r, :, c0:c1], side)
            assert not side.pieces
            return gelu_pieces(c, cs)

        def d4(c, side):
            c0, c1 = FCH[c]
            lh = _run(UP, [jnp.concatenate([jnp.concatenate(
                [hs.pop((c, v, r, cc)) for cc in range(0, c1 - c0, 128)], axis=1) for r in range(0, HM, 8)], axis=0)
                for v in range(8)])
            rhs = lambda r: s4_v[r, c0:c1, :]
            if c + 1 < len(FCH):
                for n in WORDER:
                    for r in range(RK):
                        if WN[r] == n:
                            acc[n] = mm(lh[UN[r]], rhs(r), side, acc.get(n))
            else:
                idx = lambda v: (pl.ds(r0 + (v // 4) * HM, HM), slice((v % 4) * D4, (v % 4 + 1) * D4))

                def extra(n):
                    if n >= 8:
                        return acc.get(n)
                    return b_v[idx(n)] + acc[n] if n in acc else b_v[idx(n)]

                def emit_b(v, t):
                    b_v[idx(v)] = jnp.concatenate([1.0 - g_v[idx(v)[0], :]] * 2, axis=1) * t
                fmm(lambda u: lh[u], rhs, side, extra, emit_b)
            assert not side.pieces

        g0 = d3(0, Side(relays[:20], 23, 3))
        g1 = d3(1, Side(_merge(g0, gates), 23, 2))
        d4(0, Side(g1[:22], 22, 4))
        g2 = d3(2, Side(_merge(g1[22:], relays[20:40]), 25))
        d4(1, Side(g2, 23, 2))
        g3 = d3(3, Side(_merge(relays[40:], norms, xes), 26))
        d4(2, Side(_merge(g3, combs), 23, 2))
        d4(3, Side([], 1))

        @pl.when(i + 2 < NG)
        def _():
            qkv_start(i + 2)

        return carry

    lax.fori_loop(0, NB, ffn, 0)

    def pre(it, carry):
        hist.clear()
        for u in range(3 * NG // NPRE):
            s0 = (it * (3 * NG // NPRE) + u) * G

            def rhs(r):
                t = None
                for q, sg in sorted(_terms(VP, 16, VN[r]).items(), key=lambda e: -e[1]):
                    blk = wqkv_v[s0 + q % 4 + zero_s[r], (q // 4) * (D // 8):(q // 4 + 1) * (D // 8), :]
                    if VN[r] < 16:
                        return blk
                    blk = _unpack(blk)
                    t = blk if t is None else (t + blk if sg > 0 else t - blk)
                return t.astype(bf16)
            for v, t in enumerate(fmm(lambda k: xe_v[UL.index(k)], rhs, None)):
                t = _pack(t)
                for jj in range(NPAIR // 2):
                    e_v[(v // 4) * (NPAIR // 2) + jj, s0 + v % 4] = t[jj * 8:jj * 8 + 8]
        return carry

    lax.fori_loop(0, NPRE, pre, 0)

    wait("wo")
    mem_v[...] = mem0_ref[...].astype(f32)

    def slab(w, h):
        return (h // G) * SPG + w * G + h % G

    def step(j, hx, odd, late, allow, fill):
        qs, ks, vs, ps = {}, {}, {}, {}
        wload = lambda w, h: pltpu.bitcast(wqkv_v[slab(w, h)], bf16)
        eload = lambda w, h: pltpu.bitcast(e_v[j, slab(w, h)], bf16)

        def proj(g):
            part = {}
            if late and g == 0:
                for h in range(2):
                    for w in range(3):
                        part[w, h] = _dot(hx[:, :DH2], wload(w, h)[:DH2])
            for h in range(g * G, (g + 1) * G):
                q, k, v = [(_dot(hx[:, DH2:], wload(w, h)[DH2:]) + part[w, h] if (w, h) in part
                            else _dot(hx, wload(w, h))).astype(bf16) for w in range(3)]
                if odd:
                    q = jnp.concatenate([q, eload(0, h)], axis=0)
                    k = jnp.concatenate([pltpu.bitcast(ke_v[h], bf16), eload(1, h), k], axis=0)
                    v = jnp.concatenate([pltpu.bitcast(ve_v[h], bf16), eload(2, h), v], axis=0)
                else:
                    ke_v[h] = pltpu.bitcast(k, u32)
                    ve_v[h] = pltpu.bitcast(v, u32)
                    k = jnp.concatenate([k, eload(1, h)], axis=0)
                    v = jnp.concatenate([v, eload(2, h)], axis=0)
                qs[h], ks[h], vs[h] = q, k, v

        def score(g):
            for h in range(g * G, (g + 1) * G):
                s = lax.dot_general(qs.pop(h), ks.pop(h), (((1,), (1,)), ((), ())),
                                    preferred_element_type=f32)
                ps[h] = _softmax(s, allow, fill)

        def pv(g):
            os_ = []
            for h in range(g * G, (g + 1) * G):
                o = _dot(ps.pop(h), vs.pop(h))
                o_v[:, h * 128:(h + 1) * 128] = _pack(o[:32])
                os_.append(o)
            if odd:
                quads = [jnp.concatenate([os_[2 * kk][r:r + 8], os_[2 * kk + 1][r:r + 8]], axis=1)
                         for r in (32, 40) for kk in range(2)]
                for k, t in enumerate(_lcombos(*quads)):
                    oe_v[k, pl.ds(pl.multiple_of(j * 8, 8), 8), g * 256:(g + 1) * 256] = t.astype(bf16)

        acc = [None] * NT

        def wo(h0, h1, j0, j1):
            o = pltpu.bitcast(o_v[:, h0 * 128:h1 * 128], bf16)
            for n in range(j0, j1):
                y = _dot(o, pltpu.bitcast(wo_v[n, h0 * 64:h1 * 64, :], bf16))
                acc[n] = y if acc[n] is None else y + acc[n]

        for t in range(NG):
            proj(t)
            if t >= 2:
                pv(t - 2)
            if t >= 1:
                score(t - 1)
        wo(0, 16, 0, 4)
        pv(NG - 2)
        score(NG - 1)
        wo(0, 16, 4, 8)
        pv(NG - 1)
        wo(16, 24, 0, 8)
        wo(24, 32, 0, 8)
        return jnp.concatenate(acc, axis=1)

    def emit(j, r0, o0, a):
        rs = pl.ds(r0 + o0, 24)
        g = jnp.concatenate([g_v[rs, :]] * NT, axis=1)
        out_v[j, o0:o0 + 24, :] = (g * a + b_v[rs, :]).astype(bf16)

    def pair(j, mem, late):
        r0 = pl.multiple_of(j * 64, 64)
        allow_e, fill_e, allow_o, fill_o = _masks()
        xa = x_v[pl.ds(r0 + 16, 8), :].astype(f32)
        xb = x_v[pl.ds(r0 + 40, 8), :].astype(f32)
        hx = jnp.concatenate([x_v[pl.ds(r0, 16), :], jnp.concatenate([xa, mem], 0).astype(bf16)], 0)
        oe = step(j, hx, False, late, allow_e, fill_e)
        emit(j, r0, 0, oe[:24])
        hx = jnp.concatenate([jnp.concatenate([oe[24:32], xb], 0).astype(bf16), x_v[pl.ds(r0 + 48, 16), :]], 0)
        oo = step(j, hx, True, True, allow_o, fill_o)
        emit(j, r0, 40, oo[8:])
        return oo[:8]

    def a_iter(it, carry):
        mem = mem_v[...]
        for t in range(PPI):
            mem = pair(it * PPI + t, mem, t > 0)
        mem_v[...] = mem
        for t in range(PPI):
            for o0 in (0, 40):
                idx = (it * PPI + t, pl.ds(o0, 24))
                pltpu.make_async_copy(out_v.at[idx], out_hbm.at[idx], sem_out).start()
        return carry

    lax.fori_loop(0, NPAIR // PPI, a_iter, 0)

    hist.clear()
    for n in range(NT // 2):
        quad = [lambda k, t=2 * n + q % 2, o=(q // 2) * 128: jnp.concatenate(
            [wo_v[t + zero_s[k], g * 256 + o:g * 256 + o + 128, :] for g in range(NG)], axis=0) for q in range(4)]
        cs = strassen(lambda k: oe_v[k], lambda k: _rcombo(k, *quad), None)
        cols = slice(n * 256, (n + 1) * 256)
        for half in range(2):
            t = jnp.concatenate(cs[2 * half:2 * half + 2], axis=1)
            o0 = 24 + half * 8
            for jj in range(NPAIR):
                rs = slice(jj * 64 + o0, jj * 64 + o0 + 8)
                g = jnp.concatenate([g_v[rs, :]] * 2, axis=1)
                out_v[jj, o0:o0 + 8, cols] = (g * t[jj * 8:jj * 8 + 8] + b_v[rs, cols]).astype(bf16)
        if n >= 2:
            idx = (slice(None), pl.ds(24, 16), pl.ds(0, 768) if n == 2 else pl.ds(768, 256))
            pltpu.make_async_copy(out_v.at[idx], out_hbm.at[idx], sem_out).start()
    pltpu.make_async_copy(out_v, out_hbm, sem_out).wait()


@functools.partial(jax.jit, static_argnames=("A_seg_len",))
def pallas_gated_mix__memory_aug_recurrent_mem_tr__mixer_s_mlp__prompt_kernel(
    A_x, A_mem0, A_Wq, A_Wk, A_Wv, A_Wo, A_seg_len, B_x, B_w1, B_w2, B_w3, B_w4, gate_w,
):
    assert A_seg_len == SEG
    assert A_x.shape == (1, S, D) and A_mem0.shape == (1, M, D)
    any_spec = pl.BlockSpec(memory_space=pl.ANY)
    out = pl.pallas_call(
        _kernel,
        out_shape=jax.ShapeDtypeStruct((NPAIR, 64, D), bf16),
        in_specs=[any_spec] * 11,
        out_specs=any_spec,
        scratch_shapes=[
            pltpu.VMEM((S, D), bf16),
            pltpu.VMEM((9, D // 4, D // 2), u32),
            pltpu.VMEM((7, D // 4, D // 2), u32),
            pltpu.VMEM((RK, D4, F4), bf16),
            pltpu.VMEM((RK, F4, D4), bf16),
            pltpu.VMEM((3 * H, D // 2, DH), u32),
            pltpu.VMEM((NT, H * DH // 2, 128), u32),
            pltpu.VMEM((NT, S + 2 * PAD, 128), f32),
            pltpu.VMEM((S, D), f32),
            pltpu.VMEM((TM, D), f32),
            pltpu.VMEM((2, 7, HM // 2, D // 2), u32),
            pltpu.VMEM((len(UL), HM, D4), bf16),
            pltpu.VMEM((2, TM, 128), f32),
            pltpu.VMEM((S, 128), f32),
            pltpu.VMEM((NPAIR, 64, D), bf16),
            pltpu.VMEM((len(UL), 8 * NPAIR, D4), bf16),
            pltpu.VMEM((NPAIR, 3 * H, 8, DH), u32),
            pltpu.VMEM((7, 8 * NPAIR, H * DH // 2), bf16),
            pltpu.VMEM((H, 16, 128), u32),
            pltpu.VMEM((H, 16, 128), u32),
            pltpu.VMEM((16, H * DH), u32),
            pltpu.VMEM((M, D), f32),
            pltpu.VMEM((M, D), bf16),
            pltpu.VMEM((NT, 128), bf16),
            pltpu.SMEM((RK,), jnp.int32),
            pltpu.SemaphoreType.DMA((NLOAD,)),
            pltpu.SemaphoreType.DMA((NG,)),
            pltpu.SemaphoreType.DMA,
        ],
        compiler_params=pltpu.CompilerParams(vmem_limit_bytes=126 * 1024 * 1024,
                                             disable_bounds_checks=True),
    )(
        A_x.reshape(S, D), A_mem0.reshape(M, D),
        A_Wq.reshape(D // 2, 2 * H, DH), A_Wk.reshape(D // 2, 2 * H, DH), A_Wv.reshape(D // 2, 2 * H, DH),
        A_Wo.reshape(H * DH, D), B_w1, B_w2, B_w3, B_w4, gate_w.reshape(NT, 128),
    )
    return out.reshape(1, S, D)
```

```python
import functools

import jax
import jax.numpy as jnp
from jax import lax
import jax.experimental.pallas as pl
import jax.experimental.pallas.tpu as pltpu

f32, bf16, u32 = jnp.float32, jnp.bfloat16, jnp.uint32

S, D, H, DH, M, SEG, F = 2048, 1024, 32, 128, 8, 32, 3584
SCALE = DH ** -0.5
NEG = -1000000000.0
EPS = 1e-05

TM = 256
NB = S // TM
HM = TM // 2
DH2 = D // 2
D4, F4 = D // 4, F // 4
FCH = ((0, 128), (128, 384), (384, 640), (640, 896))
NC1 = 128
NPAIR = S // (2 * SEG)
PPI = 2
NPRE = 3
G = 4
NG = H // G
PAD = 8
NT = D // 128
W3A = 192
NLOAD = 11
assert NB == NG

_dot = functools.partial(jnp.dot, preferred_element_type=f32)

UP = ((4, 1, 5, 1), (6, 1, 8, 1), (0, 1, 3, 1), (2, -1, 9, 1), (4, -1, 10, 1), (0, 1, 1, 1), (2, 1, 12, 1),
      (5, 1, 7, -1), (7, 1, 12, -1), (11, -1, 13, 1), (10, -1, 11, 1), (2, 1, 7, 1), (0, -1, 4, 1),
      (6, 1, 7, 1), (1, -1, 5, 1), (3, 1, 7, -1), (1, 1, 4, 1), (2, 1, 3, 1), (1, -1, 3, 1), (1, 1, 7, -1),
      (2, 1, 6, -1))
WP = ((0, -1, 3, 1), (4, 1, 6, -1), (1, 1, 8, 1), (5, 1, 10, 1), (4, -1, 7, 1), (0, -1, 9, -1),
      (11, 1, 12, 1), (6, 1, 7, -1), (2, 1, 5, -1), (0, -1, 7, -1), (9, 1, 11, -1), (2, 1, 13, 1),
      (5, 1, 13, 1), (2, -1, 3, 1), (5, 1, 6, 1), (0, 1, 4, 1), (2, 1, 7, 1), (1, 1, 2, 1), (1, 1, 5, 1),
      (3, 1, 7, 1), (2, 1, 6, 1))
VP = ((1, 1, 5, -1), (8, 1, 11, 1), (10, 1, 17, 1), (13, 1, 16, -1), (0, 1, 4, -1), (0, 1, 3, 1),
      (14, 1, 18, -1), (0, 1, 11, 1), (14, 1, 19, -1), (0, 1, 5, 1), (12, 1, 15, 1), (2, 1, 21, 1),
      (10, 1, 14, -1), (4, 1, 7, 1), (11, 1, 19, 1), (12, -1, 20, 1), (13, 1, 14, -1), (9, 1, 30, -1),
      (3, -1, 15, 1), (6, 1, 23, 1), (24, 1, 27, -1), (9, -1, 18, 1), (7, 1, 34, 1), (2, 1, 6, -1),
      (0, 1, 8, -1), (6, 1, 21, 1), (22, 1, 31, -1), (6, 1, 29, 1), (0, 1, 1, 1), (15, 1, 25, 1),
      (5, 1, 37, 1), (15, 1, 20, 1))
UN = (7, 27, 24, 17, 9, 22, 21, 2, 15, 11, 8, 25, 19, 28, 2, 23, 26, 20, 1, 18, 10, 28, 4, 13, 14, 16)
WN = (23, 17, 24, 10, 14, 7, 22, 19, 12, 18, 15, 25, 20, 5, 26, 0, 8, 2, 27, 11, 26, 9, 28, 21, 16, 5)
VN = (42, 47, 41, 5, 11, 43, 18, 28, 20, 23, 35, 19, 22, 46, 33, 26, 45, 36, 38, 25, 44, 40, 39, 21, 24, 32)
RK = len(UN)
UL = tuple(sorted(set(UN)))
RAW16 = (1, 11, 17, 5, 8, 3, 9, 10, 0, 6, 7, 4, 12, 20, 22, 16)
VORDER = (0, 6, 7, 12, 13, 14, 15, 21, 11, 17, 20, 22, 24, 25, 23, 2, 1, 5, 8, 9, 10, 16, 18, 19)
assert sorted(VORDER) == [r for r in range(RK) if VN[r] >= 16] and len(set(RAW16)) == 16
assert all(RAW16[VN[r]] == r for r in range(RK) if VN[r] < 16)


def _run(prog, blocks):
    vals = list(blocks)
    for a, sa, b, sb in prog:
        vals.append(vals[a] + vals[b] if sa > 0 and sb > 0 else
                    vals[a] - vals[b] if sa > 0 else vals[b] - vals[a])
    return vals


def _terms(prog, nin, node):
    if node < nin:
        return {node: 1}
    a, sa, b, sb = prog[node - nin]
    out = {k: sa * v for k, v in _terms(prog, nin, a).items()}
    out.update({k: sb * v for k, v in _terms(prog, nin, b).items()})
    return out


_WPAR = {n: [] for n in range(8 + len(WP))}
for _t, (_a, _sa, _b, _sb) in enumerate(WP):
    _WPAR[_a].append((8 + _t, _sa))
    _WPAR[_b].append((8 + _t, _sb))


def _worder():
    order = []

    def closure(n, acc):
        if n not in acc and n not in order:
            acc.add(n)
            for q, _ in _WPAR[n]:
                closure(q, acc)
        return acc

    def visit(n):
        if n not in order:
            for q, _ in _WPAR[n]:
                visit(q)
            order.append(n)
    while len([v for v in range(8) if v not in order]):
        visit(min((v for v in range(8) if v not in order), key=lambda v: len(closure(v, set()))))
    return tuple(order)


WORDER = _worder()


def _ln(x):
    m = jnp.mean(x, axis=-1, keepdims=True)
    xc = x - m
    v = jnp.mean(xc * xc, axis=-1, keepdims=True)
    return xc * lax.rsqrt(v + EPS)


_GC = 0.7978845608028654


def _gelu(x):
    h = 0.5 * x
    return h + h * jnp.tanh(x * (_GC + (_GC * 0.044715) * (x * x)))


def _unpack(u):
    return pltpu.bitcast(u, bf16).astype(f32)


def _pack(x):
    return pltpu.bitcast(x.astype(bf16), u32)


def _cat(xs, axis):
    xs = [x for x in xs if x.shape[axis]]
    return xs[0] if len(xs) == 1 else jnp.concatenate(xs, axis=axis)


def _as(x, dtype):
    return x if x.dtype == dtype else pltpu.bitcast(x, dtype)


def _lcombos(a11, a12, a21, a22):
    return [a11 + a22, a21 + a22, a11, a22, a11 + a12, a21 - a11, a12 - a22]


def _merge(*lists):
    keyed = [((j + 0.5) / len(l), n, j, v) for n, l in enumerate(lists) for j, v in enumerate(l)]
    return [v for _, _, _, v in sorted(keyed, key=lambda t: t[:3])]


def _masks():
    r = lax.broadcasted_iota(jnp.int32, (32, 48), 0)
    c = lax.broadcasted_iota(jnp.int32, (32, 48), 1)
    exist_e = c < 40
    allow_e = exist_e & ((r >= 24) | ((c >= 24) & (c < 32)) | (c <= r))
    fill_e = jnp.where(exist_e, NEG, -jnp.inf).astype(f32)
    r = lax.broadcasted_iota(jnp.int32, (48, 80), 0)
    c = lax.broadcasted_iota(jnp.int32, (48, 80), 1)
    q_even = (r >= 32) & (r < 40)
    exist_o = (q_even & (c < 40)) | (~q_even & (c >= 40))
    ktok = jnp.where(c < 24, c, jnp.where(c < 48, c - 8, c - 16))
    qtok = jnp.where(r < 32, r + 32, r - 8)
    is_mem_key = ((c >= 24) & (c < 32)) | ((c >= 48) & (c < 56))
    allow_o = exist_o & (is_mem_key | (r < 8) | (ktok <= qtok))
    fill_o = jnp.where(exist_o, NEG, -jnp.inf).astype(f32)
    return allow_e, fill_e, allow_o, fill_o


def _rcombo(k, b11, b12, b21, b22):
    if k in (1, 4):
        return (b11 if k == 1 else b22)(k)
    a, b, sign = {0: (b11, b22, 1), 2: (b12, b22, -1), 3: (b21, b11, -1), 5: (b11, b12, 1), 6: (b21, b22, 1)}[k]
    a, b = _unpack(a(k)), _unpack(b(k))
    return (a + b if sign > 0 else a - b).astype(bf16)


def _softmax(s, allow, fill):
    s = jnp.where(allow, s * SCALE, fill)
    m = jnp.max(s, axis=-1, keepdims=True)
    e = jnp.exp(s - m)
    l = jnp.sum(e, axis=-1, keepdims=True)
    r = pl.reciprocal(l, approx=True)
    r = r * (2.0 - l * r)
    return (e * r).astype(bf16)


def _kernel(x_hbm, mem0_hbm, wq_hbm, wk_hbm, wv_hbm, wo_hbm, w1_hbm, w2_hbm, w3_hbm, w4_hbm,
            gw_hbm, out_hbm,
            x_v, s1_v, s2_v, s3_v, s4_v, wqkv_v, wo_v, h_v, b_v, c0_v, l_v, lf_v, n_v, g_v, out_v, xe_v, e_v, oe_v,
            ke_v, ve_v, o_v, mem_v, mem0_ref, gw_ref, zero_s,
            sem, sem_qkv, sem_out):
    RAW = (1, 2, 3, 4)
    RAW1 = (1, 7, 8, 4)

    loads = []

    def rows_load(name, r0, r1):
        loads.append((name, x_hbm.at[pl.ds(r0, r1 - r0)], x_v.at[pl.ds(r0, r1 - r0)]))

    def quad_load(name, w_hbm, s_v, raw, q, c0=0, c1=None):
        k4, n2 = s_v.shape[1], s_v.shape[2]
        c1 = n2 if c1 is None else c1
        src = w_hbm.bitcast(u32).at[pl.ds((q // 2) * k4, k4), pl.ds((q % 2) * n2 + c0, c1 - c0)]
        loads.append((name, src, s_v.at[raw[q], :, pl.ds(c0, c1 - c0)]))

    def w1_load(name, half, c0, c1):
        quad_load(name, w1_hbm, s1_v, RAW1, half, c0, c1)
        quad_load(name, w1_hbm, s1_v, RAW1, 2 + half, c0, c1)

    def block_load(name, w_hbm, s_v, r0, r1):
        kb, nb = s_v.shape[1:]
        for q in range(16):
            loads.append((name, w_hbm.at[pl.ds((q // 4) * kb + r0, r1 - r0), pl.ds((q % 4) * nb, nb)],
                          s_v.at[RAW16[q], pl.ds(r0, r1 - r0)]))

    rows_load("x0", 0, TM)
    w1_load("w1a", 0, 0, 256)
    w1_load("w1b", 0, 256, 512)
    rows_load("x1", TM, 2 * TM)
    w1_load("w1cd", 1, 0, 512)
    rows_load("x23", 2 * TM, 4 * TM)
    rows_load("x4567", 4 * TM, S)
    for q in range(4):
        quad_load("w2", w2_hbm, s2_v, RAW, q)
    block_load("w2", w3_hbm, s3_v, 0, W3A)
    block_load("w4", w3_hbm, s3_v, W3A, D4)
    block_load("w4", w4_hbm, s4_v, 0, F4)
    loads.append(("small", mem0_hbm, mem0_ref))
    loads.append(("small", gw_hbm, gw_ref))
    for j in range(NT):
        loads.append(("wo", wo_hbm.bitcast(u32).at[:, pl.ds(j * 128, 128)], wo_v.at[j]))
    groups = list(dict.fromkeys(name for name, _, _ in loads))
    assert len(groups) == NLOAD

    def start(*names, priority=0):
        for name, src, dst in loads:
            if name in names:
                pltpu.make_async_copy(src, dst, sem.at[groups.index(name)]).start(priority=priority)

    def wait(*names):
        for name, src, dst in loads:
            if name in names:
                pltpu.make_async_copy(src, dst, sem.at[groups.index(name)]).wait()

    SPG = 3 * G

    def qkv_start(g):
        for w, w_hbm in enumerate((wq_hbm, wk_hbm, wv_hbm)):
            wu = w_hbm.bitcast(u32)
            for k in range(G // 2):
                for par in range(2):
                    pltpu.make_async_copy(
                        wu.at[:, par * (H // 2) + g * (G // 2) + k, :],
                        wqkv_v.at[g * SPG + w * G + 2 * k + par], sem_qkv.at[g]).start(priority=1)

    def qkv_wait(g):
        grp = wqkv_v.at[pl.ds(g * SPG, SPG)]
        pltpu.make_async_copy(grp, grp, sem_qkv.at[g]).wait()

    start("x0", "w1a", "w1b", "x1", "w1cd", "x23", "x4567", "w2", "w4", "small")

    def zero(k, carry):
        zero_s[k] = 0
        return carry
    lax.fori_loop(0, RK, zero, 0)

    def tile_idx(ref, cols=128):
        z = zero_s[0]
        n = 16 if ref.dtype == bf16 and cols == 128 else 8
        return (z,) * (len(ref.shape) - 2) + (pl.ds(pl.multiple_of(z, n), n), slice(0, cols))

    hist = []

    def mm(lhs, rhs, side=None, acc=None):
        if side is not None:
            lhs = side(lhs)
        lhs = pltpu.bitcast(lhs, bf16) if lhs.dtype == u32 else lhs.astype(bf16)
        y = _dot(lhs, pltpu.bitcast(rhs, bf16) if rhs.dtype == u32 else rhs)
        if acc is not None:
            y = y + acc
        hist.append(y)
        return y

    class Side:
        def __init__(self, pieces, n, skip=0):
            cap = [0] * skip + ([1] * n if isinstance(n, int) else list(n))
            tot = sum(p[4] for p in pieces)
            self.plan = [[] for _ in cap]
            done = 0
            for p in pieces:
                done += p[4]
                x, d = done / tot * sum(cap), 0
                while x > cap[d] + 1e-9:
                    x -= cap[d]
                    d += 1
                self.plan[d].append((p, x / cap[d]))
            self.pieces = len(pieces)

        def __call__(self, val):
            todo = self.plan.pop(0) if self.plan else []
            if not todo:
                return val
            self.pieces -= len(todo)
            never = [zero_s[0] > 0]
            if val.dtype == bf16:
                val = pltpu.bitcast(val, u32)
            rg = 8 if val.dtype == u32 else 16
            ng = val.shape[0] // rg
            tied = {}
            for (fn, rd, wr, lag, _), pos in todo:
                m = min(max(-int(-pos * ng // 1) - 1, 0), ng - 1)
                pin = lambda v, w=128: v
                if lag is not None and len(hist) >= lag:
                    r0 = (16 * m) % hist[-lag].shape[0]
                    a = hist[-lag][r0:r0 + 8, :128]
                    if rd is None:
                        def pin(v, w=128, a=a):
                            a = _cat([_cat([_as(a, v.dtype)] * (v.shape[0] // 8), 0)] * (w // 128), 1)
                            if v.shape[1] == w:
                                return lax.select(never[0], a, v)
                            return _cat([lax.select(never[0], a, v[:, :w]), v[:, w:]], 1)
                    elif rd.dtype == bf16:
                        idx = tile_idx(rd, 256)
                        rd[idx] = lax.select(never[0], _cat([a, a], 1).astype(bf16), rd[idx])
                    else:
                        idx = tile_idx(rd)
                        rd[idx] = lax.select(never[0], _as(a, rd.dtype), rd[idx])
                u = fn(pin)
                if wr is False:
                    continue
                if wr is not None:
                    u = wr[tile_idx(wr)]
                t, n = tied.get(m * rg) or (val[m * rg:m * rg + 8, -128:], 0)
                tied[m * rg] = (lax.select(zero_s[n] > 0, _as(u, val.dtype), t), n + 1)
            if not tied:
                return val
            col, r = [], 0
            for r0 in sorted(tied):
                col += ([val[r:r0, -128:]] if r0 > r else []) + [tied[r0][0]]
                r = r0 + 8
            col += [val[r:, -128:]] if r < val.shape[0] else []
            return _cat([val[:, :-128], _cat(col, 0)], 1) if val.shape[1] > 128 else _cat(col, 0)

    def strassen(lhs, rhs, side, init=(None, None, None, None)):
        def add(a, b):
            return a if b is None else a + b
        p = [mm(lhs(k), rhs(k), side) for k in range(5)]
        c12 = add(p[2] + p[4], init[1])
        c21 = add(p[1] + p[3], init[2])
        c22 = mm(lhs(5), rhs(5), side, add(p[0] - p[1] + p[2], init[3]))
        c11 = mm(lhs(6), rhs(6), side, add(p[0] + p[3] - p[4], init[0]))
        return c11, c12, c21, c22

    def fmm(lhs, rhs, side, extra=lambda n: None, emit=None):
        val = {}
        for n in WORDER:
            t = extra(n)
            for q, sg in sorted(_WPAR[n], key=lambda e: -e[1]):
                t = val[q] if t is None else (t + val[q] if sg > 0 else t - val[q])
            for r in range(RK):
                if WN[r] == n:
                    t = mm(lhs(UN[r]), rhs(r), side, t)
            val[n] = t
            if n < 8 and emit is not None:
                emit(n, t)
        return [val[v] for v in range(8)]

    def prep26_pieces(s_v, lag):
        def piece(rs, cs, pin):
            @functools.lru_cache(None)
            def node(n):
                if n < 16:
                    return s_v[RAW16[n], rs, cs].astype(f32)
                a, sa, b, sb = VP[n - 16]
                return _run([(0, sa, 1, sb)], [node(a), node(b)])[-1]
            vals = [node(VN[r]).astype(bf16) for r in VORDER]
            for r, t in zip(VORDER, vals):
                s_v[r, rs, cs] = t
        kb, nb = s_v.shape[1:]
        out = []
        for r in range(0, kb, 16):
            out += [(slice(rr, rr + 8), slice(c, c + 256)) for c in range(0, nb - 255, 256) for rr in (r, r + 8)]
            out += [(slice(rr, rr + 8), slice(nb - 128, nb)) for rr in (r, r + 8)] if nb % 256 else []
        return [(functools.partial(piece, rs, cs), s_v, s_v if n % 16 == 15 else False, lag,
                 130 if cs.stop - cs.start == 256 else 100) for n, (rs, cs) in enumerate(out)]

    def prep_pieces(s_v, raw, lag, width=256):
        def piece(r, c, pin):
            idx = (slice(r, r + 8), slice(c, c + width))
            b11, b12, b21, b22 = [_unpack(pin(s_v[(q,) + idx], width) if n in (0, 3) else s_v[(q,) + idx])
                                  for n, q in enumerate(raw)]
            for k, t in ((0, b11 + b22), (2, b12 - b22), (3, b21 - b11), (5, b11 + b12), (6, b21 + b22)):
                s_v[(k,) + idx] = _pack(t)
        return [(functools.partial(piece, r, c), None, s_v, lag, 80)
                for c in range(0, s_v.shape[2], width) for r in range(0, s_v.shape[1], 8)]

    def store_l(slot, q, c, quads, plain=False):
        for k, t in enumerate(quads if plain else _lcombos(*quads)):
            l_v[slot, k, q // 2:q // 2 + 8, c:c + t.shape[1]] = _pack(t)

    def ln_pieces(src, r0, slot, lag, plain=False, width=256, staged=False, clag=None):
        def stats(q, pin):
            x = pin(src[pl.ds(r0 + q, 16), :].astype(f32))
            xs = [x[:, j * 128:(j + 1) * 128] for j in range(NT)]
            m = functools.reduce(lambda a, b: a + b, xs) * (1.0 / NT)
            w = functools.reduce(lambda a, b: a + b, [(t - m) * (t - m) for t in xs])
            mean = jnp.mean(m, axis=-1, keepdims=True)
            var = jnp.sum(w + NT * ((m - mean) * (m - mean)), axis=-1, keepdims=True) * (1.0 / D)
            n_v[0, q:q + 16, :] = jnp.broadcast_to(mean, (16, 128))
            n_v[1, q:q + 16, :] = jnp.broadcast_to(lax.rsqrt(var + EPS), (16, 128))

        def comb(q, c, pin):
            quads = []
            for rr in (0, HM):
                rs = pl.ds(pl.multiple_of(r0 + rr + q + zero_s[0], 16), 16)
                mean, rstd = [jnp.concatenate([n_v[t, rr + q:rr + q + 16, :]] * (width // 128), axis=1)
                              for t in range(2)]
                quads += [(src[rs, cc + c:cc + c + width].astype(f32) - mean) * rstd for cc in (0, DH2)]
            store_l(slot, q, c, quads, plain)

        def comb26(q, pin):
            blocks = []
            for rr in (0, HM):
                rs = pl.ds(pl.multiple_of(r0 + rr + q + zero_s[0], 8), 8)
                mean, rstd = [jnp.concatenate([n_v[t, rr + q:rr + q + 8, :]] * 2, axis=1) for t in range(2)]
                blocks += [(src[rs, cc:cc + D4] - mean) * rstd for cc in range(0, D, D4)]
            vals = _run(UP, blocks)
            for k, u in enumerate(UL):
                lf_v[k, q:q + 8, :] = vals[u].astype(bf16)
        norms = [[(functools.partial(stats, rr + q), None, n_v if slot is not None else False, lag, 90) for rr in (0, HM)]
                 for q in range(0, HM, 16)]
        if slot is None:
            combs = [[(functools.partial(comb26, qq), n_v, lf_v if qq % 32 == 24 else False, clag, 110) for qq in (q, q + 8)]
                     for q in range(0, HM, 16)]
        else:
            combs = [[(functools.partial(comb, q, c), n_v, l_v, clag, 125) for c in range(0, DH2, width)]
                     for q in range(0, HM, 16)]
        if staged:
            return sum(norms, []), sum(combs, [])
        out = list(norms[0])
        for a, b in zip(norms[1:] + [[]], combs):
            out += _merge(a, b) if a else b
        return out

    shifts = (1, 1, -1, -1, 2, 2, -2, -2)

    def shift_pieces(r0, slot, lag, by_value=False):
        def piece(q, j, pin):
            a = [h_v[jj, pl.ds(PAD + r0 + rr + q - shifts[jj], 16), :]
                 for rr in (0, HM) for jj in (j, j + NT // 2)]
            store_l(slot, q, j * 128, [pin(a[0]), a[1], a[2], pin(a[3])])
        return [(functools.partial(piece, q, j), None if by_value else h_v, l_v if (q // 16) % 2 and j == 3 else False, lag, 50)
                for q in range(0, HM, 16) for j in range(NT // 2)]

    def lhs_of(slot):
        return lambda k: l_v[slot, k]

    h_v[:, 0:PAD, :] = jnp.zeros((NT, PAD, 128), f32)
    h_v[:, PAD + S:PAD + S + PAD, :] = jnp.zeros((NT, PAD, 128), f32)

    def store_h(r0, c0, h):
        for j in range(h.shape[1] // 128):
            h_v[c0 // 128 + j, PAD + r0:PAD + r0 + h.shape[0], :] = h[:, j * 128:(j + 1) * 128]

    def h_pieces(r0, c0, t, lag, n=4):
        def piece(r, pin):
            store_h(r0 + r, c0, _gelu(pin(t[r:r + 8 * n])))
        return [(functools.partial(piece, r), None, h_v, lag, 10 * n) for r in range(0, t.shape[0], 8 * n)]

    def flush(pieces):
        for p in pieces:
            p[0](lambda v, w=128: v)

    def w1_cols(c, step):
        half, cc = c // DH2, c % DH2
        return jnp.concatenate([s1_v[RAW1[half], :, cc:cc + step], s1_v[RAW1[2 + half], :, cc:cc + step]], axis=0)

    def d1_plain(xn, r0, c0, c1, step):
        for c in range(c0, c1, step):
            store_h(r0, c, _gelu(mm(xn, w1_cols(c, step))))

    def d1_fine(lhs, r0, nrb, cols, pieces, carry, skip=0):
        tiles = [(rb, c) for c in cols for rb in range(nrb)]
        rounds = [tiles[i:i + 4] for i in range(0, len(tiles), 4)]
        for n, (rnd, part) in enumerate(zip(rounds, split(pieces, len(rounds)))):
            sk = skip if n == 0 else 0
            side = Side(_merge(carry, part) if carry else part, 8 - sk, sk)
            carry = []
            for rb, c in rnd:
                half, cc = c // DH2, c % DH2
                t = mm(lhs(rb, 0), s1_v[RAW1[half], :, cc:cc + 128], side)
                t = mm(lhs(rb, 1), s1_v[RAW1[2 + half], :, cc:cc + 128], side, t)
                carry += h_pieces(r0 + rb * HM, c, t, LS)
        return carry

    CAP1 = (1, 1, 1, 1, 1, 1, 1)
    CAP2 = (2, 3, 3, 3, 3, 3, 2)

    def d1_s(b, slot, pieces, carry):
        for c, part in zip(range(0, DH2, NC1), split(pieces, DH2 // NC1)):
            side = Side(merge(carry, part), CAP1 if hist else (0, 0) + CAP1[2:])
            cs = strassen(lhs_of(slot), lambda k: s1_v[k, :, c:c + NC1], side)
            carry = sum([h_pieces(b * TM + (q // 2) * HM, (q % 2) * DH2 + c, cs[q], LS) for q in (1, 2, 3, 0)], [])
        return carry

    def d2_s(b, slot, pieces, carry=(), early=(), late=()):
        for c, part, e in zip(range(0, DH2, NC1), split(pieces, DH2 // NC1), split(early, 2) + split(late, 2)):
            side = Side(merge(carry, part, e), CAP2 if hist else (0, 0) + CAP2[2:])
            carry = ()
            idx = [(slice(b * TM + (q // 2) * HM, b * TM + (q // 2 + 1) * HM),
                    slice((q % 2) * DH2 + c, (q % 2) * DH2 + c + NC1)) for q in range(4)]
            cs = strassen(lhs_of(slot), lambda k: s2_v[k, :, c:c + NC1], side,
                          [x_v[i].astype(f32) for i in idx])
            for i, t in zip(idx, cs):
                b_v[i] = t
                if b == 0:
                    c0_v[i] = t

    def split(l, n):
        w = [1.0 if hist else 0.6] + [1.0] * (n - 1)
        cut = [int(round(len(l) * sum(w[:i]) / sum(w))) for i in range(n + 1)]
        return [l[cut[i]:cut[i + 1]] for i in range(n)]

    def merge(*ls):
        ls = [l for l in ls if l]
        return _merge(*ls) if ls else []

    NW1, NW3, N30 = 32, 32, 20
    LS, LL = 3, 5

    wait("x0")
    xn0 = _pack(_ln(x_v[0:TM, :].astype(f32)))
    wait("w1a")
    d1_plain(xn0, 0, 0, 256, 256)
    wait("w1b")
    d1_plain(xn0, 0, 256, 512, 256)
    wait("x1")
    xn1 = _pack(_ln(x_v[TM:2 * TM, :].astype(f32)))
    d1_plain(xn1, TM, 0, 512, 256)
    wait("w1cd")
    hist.clear()
    xn01 = jnp.concatenate([xn0, xn1], axis=0)
    l01 = lambda rb, kh: xn01[rb * 64:(rb + 1) * 64, kh * DH2:(kh + 1) * DH2]
    pw = prep_pieces(s1_v, RAW1, LS)
    flush(d1_fine(l01, 0, 4, (512, 640), pw[:NW1], [], 1))
    carry = []
    wait("x23")
    hist.clear()
    carry = d1_fine(l01, 0, 4, (768, 896), ln_pieces(x_v, 2 * TM, 0, LL, plain=True), carry, 3)
    carry = d1_fine(lambda rb, kh: l_v[0, 2 * rb + kh], 2 * TM, 2, range(0, D, 128),
                    _merge(pw[NW1:], ln_pieces(x_v, 3 * TM, 1, LL)), carry)
    wait("x4567")
    qkv_start(0)
    qkv_start(1)
    hist.clear()
    for b in range(3, NB - 1):
        carry = d1_s(b, b % 2, ln_pieces(x_v, (b + 1) * TM, (b + 1) % 2, LL), carry)
    wait("w2")
    hist.clear()
    pw = prep_pieces(s2_v, RAW, LS)
    p3 = prep26_pieces(s3_v, 2)
    n3 = len(p3) * W3A // D4
    carry = d1_s(7, 1, _merge(pw[:NW3], shift_pieces(0, 0, LS, True)), carry)
    d2_s(0, 0, shift_pieces(TM, 1, LS, True), carry, pw[NW3:], p3[:N30])
    pw = split(_merge(p3[N30:n3], sum(ln_pieces(c0_v, 0, None, LL, clag=LS, staged=True), [])), 3)
    for b in range(1, 4):
        d2_s(b, b % 2, _merge(pw[b - 1], shift_pieces((b + 1) * TM, (b + 1) % 2, LS)))
    wait("w4", "small")
    hist.clear()
    pw = p3[n3:] + prep26_pieces(s4_v, 2)
    cut = (0, 31, 65, 99, len(pw))
    for b in range(4, NB):
        d2_s(b, b % 2, merge(pw[cut[b - 4]:cut[b - 3]],
                             shift_pieces((b + 1) * TM, (b + 1) % 2, LS) if b + 1 < NB else ()))
    start("wo", priority=1)

    def ffn(i, carry):
        qkv_wait(i)
        r0 = pl.multiple_of(i * TM, TM)
        rn = pl.multiple_of(jnp.minimum(i + 1, NB - 1) * TM, TM)
        acc = {}
        hist.clear()

        def relayout(p, r0_, r1_, pin):
            s0 = i * SPG + 2 * p
            e = wqkv_v[s0, r0_:r1_, :]
            o = wqkv_v[s0 + 1, r0_:r1_, :]
            wqkv_v[s0, r0_:r1_, :] = (e & jnp.uint32(0xFFFF)) | (o << 16)
            wqkv_v[s0 + 1, r0_:r1_, :] = (e >> 16) | (o & jnp.uint32(0xFFFF0000))

        relays = [(functools.partial(relayout, p, r, r + 32), wqkv_v, wqkv_v, 3, 35)
                  for p in range(SPG // 2) for r in range(0, D // 2, 32)]
        norms, combs = ln_pieces(b_v, rn, None, 5, staged=True, clag=3)

        def gate(q, pin):
            gw = gw_ref[...].astype(f32)
            x = pin(x_v[pl.ds(r0 + q, 16), :].astype(f32))
            t = functools.reduce(lambda a, b: a + b,
                                 [x[:, j * 128:(j + 1) * 128] * gw[j:j + 1, :] for j in range(NT)])
            g = jax.nn.sigmoid(jnp.sum(t, axis=-1, keepdims=True))
            g_v[pl.ds(r0 + q, 16), :] = jnp.broadcast_to(g, (16, 128))

        gates = [(functools.partial(gate, q), None, g_v, 5, 90) for q in range(0, TM, 16)]

        def extras(t, pin):
            jj, o = 2 * i + t // 2, 24 + 8 * (t % 2)
            xs = [pin(x_v[pl.ds(pl.multiple_of((jj + hh) * 64 + o, 8), 8), :].astype(f32)) for hh in (0, NPAIR // 2)]
            vals = _run(UP, [x[:, cc:cc + D4] for x in xs for cc in range(0, D, D4)])
            for k, u in enumerate(UL):
                xe_v[k, pl.ds(pl.multiple_of(i * 32 + t * 8, 8), 8), :] = vals[u].astype(bf16)

        xes = [(functools.partial(extras, t), None, xe_v, 3, 100) for t in range(4)]
        hs = {}

        def gelu_pieces(c, cs):
            def piece(r, cc, vs, pin):
                t = _gelu(pin(_cat([cs[v][r:r + 8, cc:cc + 128] for v in vs], 0)))
                ts = [t[8 * n:8 * n + 8] for n in range(len(vs))]
                hs.update({(c, v, r, cc): u for v, u in zip(vs, ts)})
                return functools.reduce(lambda a, b: a + b, ts)
            return [(functools.partial(piece, r, cc, vs), None, None, 3, 40) for r in range(0, HM, 8)
                    for cc in range(0, cs[0].shape[1], 128) for vs in ((0, 1, 2, 3), (4, 5, 6, 7))]

        def d3(c, side):
            c0, c1 = FCH[c]
            cs = fmm(lambda u: lf_v[UL.index(u)], lambda r: s3_v[r, :, c0:c1], side)
            assert not side.pieces
            return gelu_pieces(c, cs)

        def d4(c, side):
            c0, c1 = FCH[c]
            lh = _run(UP, [_cat([_cat([hs.pop((c, v, r, cc)) for r in range(0, HM, 8)], 0)
                                 for cc in range(0, c1 - c0, 128)], 1) for v in range(8)])
            rhs = lambda r: s4_v[r, c0:c1, :]
            if c + 1 < len(FCH):
                for n in WORDER:
                    for r in range(RK):
                        if WN[r] == n:
                            acc[n] = mm(lh[UN[r]], rhs(r), side, acc.get(n))
            else:
                idx = lambda v: (pl.ds(r0 + (v // 4) * HM, HM), slice((v % 4) * D4, (v % 4 + 1) * D4))

                def extra(n):
                    if n >= 8:
                        return acc.get(n)
                    return b_v[idx(n)] + acc[n] if n in acc else b_v[idx(n)]

                def emit_b(v, t):
                    b_v[idx(v)] = jnp.concatenate([1.0 - g_v[idx(v)[0], :]] * 2, axis=1) * t
                fmm(lambda u: lh[u], rhs, side, extra, emit_b)
            assert not side.pieces

        g0 = d3(0, Side(relays[:20], 23, 3))
        g1 = d3(1, Side(_merge(g0, gates), 23, 2))
        d4(0, Side(g1[:22], 22, 4))
        g2 = d3(2, Side(_merge(g1[22:], relays[20:40]), 25))
        d4(1, Side(g2, 23, 2))
        g3 = d3(3, Side(_merge(relays[40:], norms, xes), 26))
        d4(2, Side(_merge(g3, combs), 23, 2))
        d4(3, Side([], 1))

        @pl.when(i + 2 < NG)
        def _():
            qkv_start(i + 2)

        return carry

    lax.fori_loop(0, NB, ffn, 0)

    def pre(it, carry):
        hist.clear()
        for u in range(3 * NG // NPRE):
            s0 = (it * (3 * NG // NPRE) + u) * G

            def rhs(r):
                t = None
                sz = s0 + zero_s[r]
                for q, sg in sorted(_terms(VP, 16, VN[r]).items(), key=lambda e: -e[1]):
                    blk = wqkv_v[sz + q % 4, (q // 4) * (D // 8):(q // 4 + 1) * (D // 8), :]
                    if VN[r] < 16:
                        return blk
                    blk = _unpack(blk)
                    t = blk if t is None else (t + blk if sg > 0 else t - blk)
                return t.astype(bf16)
            for v, t in enumerate(fmm(lambda k: xe_v[UL.index(k)], rhs, None)):
                e_v[(v // 4) * 16:(v // 4 + 1) * 16, s0 + v % 4] = _pack(t).reshape(16, 8, DH)
        return carry

    lax.fori_loop(0, NPRE, pre, 0)

    wait("wo")
    mem_v[...] = mem0_ref[...].astype(f32)

    def slab(w, h):
        return (h // G) * SPG + w * G + h % G

    def step(j, hx, odd, late, allow, fill):
        qs, ks, vs, ps = {}, {}, {}, {}
        wload = lambda w, h: pltpu.bitcast(wqkv_v[slab(w, h)], bf16)
        eload = lambda w, h: pltpu.bitcast(e_v[j, slab(w, h)], bf16)

        def proj(g):
            part = {}
            if late and g == 0:
                for h in range(2):
                    for w in range(3):
                        part[w, h] = _dot(hx[:, :DH2], wload(w, h)[:DH2])
            for h in range(g * G, (g + 1) * G):
                q, k, v = [(_dot(hx[:, DH2:], wload(w, h)[DH2:]) + part[w, h] if (w, h) in part
                            else _dot(hx, wload(w, h))).astype(bf16) for w in range(3)]
                if odd:
                    q = jnp.concatenate([q, eload(0, h)], axis=0)
                    k = jnp.concatenate([pltpu.bitcast(ke_v[h], bf16), eload(1, h), k], axis=0)
                    v = jnp.concatenate([pltpu.bitcast(ve_v[h], bf16), eload(2, h), v], axis=0)
                else:
                    ke_v[h] = pltpu.bitcast(k, u32)
                    ve_v[h] = pltpu.bitcast(v, u32)
                    k = jnp.concatenate([k, eload(1, h)], axis=0)
                    v = jnp.concatenate([v, eload(2, h)], axis=0)
                qs[h], ks[h], vs[h] = q, k, v

        def score(g):
            for h in range(g * G, (g + 1) * G):
                s = lax.dot_general(qs.pop(h), ks.pop(h), (((1,), (1,)), ((), ())),
                                    preferred_element_type=f32)
                ps[h] = _softmax(s, allow, fill)

        def pv(g):
            os_ = []
            for h in range(g * G, (g + 1) * G):
                o = _dot(ps.pop(h), vs.pop(h))
                o_v[:, h * 128:(h + 1) * 128] = _pack(o[:32])
                os_.append(o)
            if odd:
                quads = [jnp.concatenate([os_[2 * kk][r:r + 8], os_[2 * kk + 1][r:r + 8]], axis=1)
                         for r in (32, 40) for kk in range(2)]
                for k, t in enumerate(_lcombos(*quads)):
                    oe_v[k, pl.ds(pl.multiple_of(j * 8, 8), 8), g * 256:(g + 1) * 256] = t.astype(bf16)

        acc = [None] * NT

        def wo(h0, h1, j0, j1):
            o = pltpu.bitcast(o_v[:, h0 * 128:h1 * 128], bf16)
            for n in range(j0, j1):
                y = _dot(o, pltpu.bitcast(wo_v[n, h0 * 64:h1 * 64, :], bf16))
                acc[n] = y if acc[n] is None else y + acc[n]

        for t in range(NG):
            proj(t)
            if t >= 2:
                pv(t - 2)
            if t >= 1:
                score(t - 1)
        wo(0, 16, 0, 4)
        pv(NG - 2)
        score(NG - 1)
        wo(0, 16, 4, 8)
        pv(NG - 1)
        wo(16, 24, 0, 8)
        wo(24, 32, 0, 8)
        return jnp.concatenate(acc, axis=1)

    def emit(j, r0, o0, a):
        rs = pl.ds(r0 + o0, 24)
        g = jnp.concatenate([g_v[rs, :]] * NT, axis=1)
        out_v[j, o0:o0 + 24, :] = (g * a + b_v[rs, :]).astype(bf16)

    def pair(j, mem, late):
        r0 = pl.multiple_of(j * 64, 64)
        allow_e, fill_e, allow_o, fill_o = _masks()
        xa = x_v[pl.ds(r0 + 16, 8), :].astype(f32)
        xb = x_v[pl.ds(r0 + 40, 8), :].astype(f32)
        hx = jnp.concatenate([x_v[pl.ds(r0, 16), :], jnp.concatenate([xa, mem], 0).astype(bf16)], 0)
        oe = step(j, hx, False, late, allow_e, fill_e)
        emit(j, r0, 0, oe[:24])
        hx = jnp.concatenate([jnp.concatenate([oe[24:32], xb], 0).astype(bf16), x_v[pl.ds(r0 + 48, 16), :]], 0)
        oo = step(j, hx, True, True, allow_o, fill_o)
        emit(j, r0, 40, oo[8:])
        return oo[:8]

    def a_iter(it, carry):
        mem = mem_v[...]
        for t in range(PPI):
            mem = pair(it * PPI + t, mem, t > 0)
        mem_v[...] = mem
        for t in range(PPI):
            for o0 in (0, 40):
                idx = (it * PPI + t, pl.ds(o0, 24))
                pltpu.make_async_copy(out_v.at[idx], out_hbm.at[idx], sem_out).start()
        return carry

    lax.fori_loop(0, NPAIR // PPI, a_iter, 0)

    hist.clear()
    for n in range(NT // 2):
        quad = [lambda k, t=2 * n + q % 2, o=(q // 2) * 128: jnp.concatenate(
            [wo_v[t + zero_s[k], g * 256 + o:g * 256 + o + 128, :] for g in range(NG)], axis=0) for q in range(4)]
        cs = strassen(lambda k: oe_v[k], lambda k: _rcombo(k, *quad), None)
        cols = slice(n * 256, (n + 1) * 256)
        for half in range(2):
            t = jnp.concatenate(cs[2 * half:2 * half + 2], axis=1)
            o0 = 24 + half * 8
            for jj in range(NPAIR):
                rs = slice(jj * 64 + o0, jj * 64 + o0 + 8)
                g = jnp.concatenate([g_v[rs, :]] * 2, axis=1)
                out_v[jj, o0:o0 + 8, cols] = (g * t[jj * 8:jj * 8 + 8] + b_v[rs, cols]).astype(bf16)
        if n >= 2:
            idx = (slice(None), pl.ds(24, 16), pl.ds(0, 768) if n == 2 else pl.ds(768, 256))
            pltpu.make_async_copy(out_v.at[idx], out_hbm.at[idx], sem_out).start()
    pltpu.make_async_copy(out_v, out_hbm, sem_out).wait()


@functools.partial(jax.jit, static_argnames=("A_seg_len",))
def pallas_gated_mix__memory_aug_recurrent_mem_tr__mixer_s_mlp__prompt_kernel(
    A_x, A_mem0, A_Wq, A_Wk, A_Wv, A_Wo, A_seg_len, B_x, B_w1, B_w2, B_w3, B_w4, gate_w,
):
    assert A_seg_len == SEG
    assert A_x.shape == (1, S, D) and A_mem0.shape == (1, M, D)
    any_spec = pl.BlockSpec(memory_space=pl.ANY)
    out = pl.pallas_call(
        _kernel,
        out_shape=jax.ShapeDtypeStruct((NPAIR, 64, D), bf16),
        in_specs=[any_spec] * 11,
        out_specs=any_spec,
        scratch_shapes=[
            pltpu.VMEM((S, D), bf16),
            pltpu.VMEM((9, D // 4, D // 2), u32),
            pltpu.VMEM((7, D // 4, D // 2), u32),
            pltpu.VMEM((RK, D4, F4), bf16),
            pltpu.VMEM((RK, F4, D4), bf16),
            pltpu.VMEM((3 * H, D // 2, DH), u32),
            pltpu.VMEM((NT, H * DH // 2, 128), u32),
            pltpu.VMEM((NT, S + 2 * PAD, 128), f32),
            pltpu.VMEM((S, D), f32),
            pltpu.VMEM((TM, D), f32),
            pltpu.VMEM((2, 7, HM // 2, D // 2), u32),
            pltpu.VMEM((len(UL), HM, D4), bf16),
            pltpu.VMEM((2, TM, 128), f32),
            pltpu.VMEM((S, 128), f32),
            pltpu.VMEM((NPAIR, 64, D), bf16),
            pltpu.VMEM((len(UL), 8 * NPAIR, D4), bf16),
            pltpu.VMEM((NPAIR, 3 * H, 8, DH), u32),
            pltpu.VMEM((7, 8 * NPAIR, H * DH // 2), bf16),
            pltpu.VMEM((H, 16, 128), u32),
            pltpu.VMEM((H, 16, 128), u32),
            pltpu.VMEM((16, H * DH), u32),
            pltpu.VMEM((M, D), f32),
            pltpu.VMEM((M, D), bf16),
            pltpu.VMEM((NT, 128), bf16),
            pltpu.SMEM((RK,), jnp.int32),
            pltpu.SemaphoreType.DMA((NLOAD,)),
            pltpu.SemaphoreType.DMA((NG,)),
            pltpu.SemaphoreType.DMA,
        ],
        compiler_params=pltpu.CompilerParams(vmem_limit_bytes=126 * 1024 * 1024,
                                             disable_bounds_checks=True),
    )(
        A_x.reshape(S, D), A_mem0.reshape(M, D),
        A_Wq.reshape(D // 2, 2 * H, DH), A_Wk.reshape(D // 2, 2 * H, DH), A_Wv.reshape(D // 2, 2 * H, DH),
        A_Wo.reshape(H * DH, D), B_w1, B_w2, B_w3, B_w4, gate_w.reshape(NT, 128),
    )
    return out.reshape(1, S, D)
```

```python
import functools

import jax
import jax.numpy as jnp
from jax import lax
import jax.experimental.pallas as pl
import jax.experimental.pallas.tpu as pltpu

f32, bf16, u32 = jnp.float32, jnp.bfloat16, jnp.uint32

S, D, H, DH, M, SEG, F = 2048, 1024, 32, 128, 8, 32, 3584
SCALE = DH ** -0.5
NEG = -1000000000.0
EPS = 1e-05

TM = 256
NB = S // TM
HM = TM // 2
DH2 = D // 2
D4, F4 = D // 4, F // 4
FCH = ((0, 128), (128, 384), (384, 640), (640, 896))
NC1 = 128
NPAIR = S // (2 * SEG)
PPI = 2
NPRE = 3
G = 4
NG = H // G
PAD = 8
NT = D // 128
W3A = 192
NLOAD = 11
assert NB == NG

_dot = functools.partial(jnp.dot, preferred_element_type=f32)

UP = ((4, 1, 5, 1), (6, 1, 8, 1), (0, 1, 3, 1), (2, -1, 9, 1), (4, -1, 10, 1), (0, 1, 1, 1), (2, 1, 12, 1),
      (5, 1, 7, -1), (7, 1, 12, -1), (11, -1, 13, 1), (10, -1, 11, 1), (2, 1, 7, 1), (0, -1, 4, 1),
      (6, 1, 7, 1), (1, -1, 5, 1), (3, 1, 7, -1), (1, 1, 4, 1), (2, 1, 3, 1), (1, -1, 3, 1), (1, 1, 7, -1),
      (2, 1, 6, -1))
WP = ((0, -1, 3, 1), (4, 1, 6, -1), (1, 1, 8, 1), (5, 1, 10, 1), (4, -1, 7, 1), (0, -1, 9, -1),
      (11, 1, 12, 1), (6, 1, 7, -1), (2, 1, 5, -1), (0, -1, 7, -1), (9, 1, 11, -1), (2, 1, 13, 1),
      (5, 1, 13, 1), (2, -1, 3, 1), (5, 1, 6, 1), (0, 1, 4, 1), (2, 1, 7, 1), (1, 1, 2, 1), (1, 1, 5, 1),
      (3, 1, 7, 1), (2, 1, 6, 1))
VP = ((1, 1, 5, -1), (8, 1, 11, 1), (10, 1, 17, 1), (13, 1, 16, -1), (0, 1, 4, -1), (0, 1, 3, 1),
      (14, 1, 18, -1), (0, 1, 11, 1), (14, 1, 19, -1), (0, 1, 5, 1), (12, 1, 15, 1), (2, 1, 21, 1),
      (10, 1, 14, -1), (4, 1, 7, 1), (11, 1, 19, 1), (12, -1, 20, 1), (13, 1, 14, -1), (9, 1, 30, -1),
      (3, -1, 15, 1), (6, 1, 23, 1), (24, 1, 27, -1), (9, -1, 18, 1), (7, 1, 34, 1), (2, 1, 6, -1),
      (0, 1, 8, -1), (6, 1, 21, 1), (22, 1, 31, -1), (6, 1, 29, 1), (0, 1, 1, 1), (15, 1, 25, 1),
      (5, 1, 37, 1), (15, 1, 20, 1))
UN = (7, 27, 24, 17, 9, 22, 21, 2, 15, 11, 8, 25, 19, 28, 2, 23, 26, 20, 1, 18, 10, 28, 4, 13, 14, 16)
WN = (23, 17, 24, 10, 14, 7, 22, 19, 12, 18, 15, 25, 20, 5, 26, 0, 8, 2, 27, 11, 26, 9, 28, 21, 16, 5)
VN = (42, 47, 41, 5, 11, 43, 18, 28, 20, 23, 35, 19, 22, 46, 33, 26, 45, 36, 38, 25, 44, 40, 39, 21, 24, 32)
RK = len(UN)
UL = tuple(sorted(set(UN)))
RAW16 = (1, 11, 17, 5, 8, 3, 9, 10, 0, 6, 7, 4, 12, 20, 22, 16)
VORDER = (0, 6, 7, 12, 13, 14, 15, 21, 11, 17, 20, 22, 24, 25, 23, 2, 1, 5, 8, 9, 10, 16, 18, 19)
assert sorted(VORDER) == [r for r in range(RK) if VN[r] >= 16] and len(set(RAW16)) == 16
assert all(RAW16[VN[r]] == r for r in range(RK) if VN[r] < 16)


def _run(prog, blocks):
    vals = list(blocks)
    for a, sa, b, sb in prog:
        vals.append(vals[a] + vals[b] if sa > 0 and sb > 0 else
                    vals[a] - vals[b] if sa > 0 else vals[b] - vals[a])
    return vals


def _terms(prog, nin, node):
    if node < nin:
        return {node: 1}
    a, sa, b, sb = prog[node - nin]
    out = {k: sa * v for k, v in _terms(prog, nin, a).items()}
    out.update({k: sb * v for k, v in _terms(prog, nin, b).items()})
    return out


_WPAR = {n: [] for n in range(8 + len(WP))}
for _t, (_a, _sa, _b, _sb) in enumerate(WP):
    _WPAR[_a].append((8 + _t, _sa))
    _WPAR[_b].append((8 + _t, _sb))


def _worder():
    order = []

    def closure(n, acc):
        if n not in acc and n not in order:
            acc.add(n)
            for q, _ in _WPAR[n]:
                closure(q, acc)
        return acc

    def visit(n):
        if n not in order:
            for q, _ in _WPAR[n]:
                visit(q)
            order.append(n)
    while len([v for v in range(8) if v not in order]):
        visit(min((v for v in range(8) if v not in order), key=lambda v: len(closure(v, set()))))
    return tuple(order)


WORDER = _worder()


def _ln(x):
    m = jnp.mean(x, axis=-1, keepdims=True)
    xc = x - m
    v = jnp.mean(xc * xc, axis=-1, keepdims=True)
    return xc * lax.rsqrt(v + EPS)


_GC = 0.7978845608028654


def _gelu(x):
    h = 0.5 * x
    return h + h * jnp.tanh(x * (_GC + (_GC * 0.044715) * (x * x)))


def _unpack(u):
    return pltpu.bitcast(u, bf16).astype(f32)


def _pack(x):
    return pltpu.bitcast(x.astype(bf16), u32)


def _cat(xs, axis):
    xs = [x for x in xs if x.shape[axis]]
    return xs[0] if len(xs) == 1 else jnp.concatenate(xs, axis=axis)


def _as(x, dtype):
    return x if x.dtype == dtype else pltpu.bitcast(x, dtype)


def _lcombos(a11, a12, a21, a22):
    return [a11 + a22, a21 + a22, a11, a22, a11 + a12, a21 - a11, a12 - a22]


def _merge(*lists):
    keyed = [((j + 0.5) / len(l), n, j, v) for n, l in enumerate(lists) for j, v in enumerate(l)]
    return [v for _, _, _, v in sorted(keyed, key=lambda t: t[:3])]


def _masks():
    r = lax.broadcasted_iota(jnp.int32, (32, 48), 0)
    c = lax.broadcasted_iota(jnp.int32, (32, 48), 1)
    exist_e = c < 40
    allow_e = exist_e & ((r >= 24) | ((c >= 24) & (c < 32)) | (c <= r))
    fill_e = jnp.where(exist_e, NEG, -jnp.inf).astype(f32)
    r = lax.broadcasted_iota(jnp.int32, (48, 80), 0)
    c = lax.broadcasted_iota(jnp.int32, (48, 80), 1)
    q_even = (r >= 32) & (r < 40)
    exist_o = (q_even & (c < 40)) | (~q_even & (c >= 40))
    ktok = jnp.where(c < 24, c, jnp.where(c < 48, c - 8, c - 16))
    qtok = jnp.where(r < 32, r + 32, r - 8)
    is_mem_key = ((c >= 24) & (c < 32)) | ((c >= 48) & (c < 56))
    allow_o = exist_o & (is_mem_key | (r < 8) | (ktok <= qtok))
    fill_o = jnp.where(exist_o, NEG, -jnp.inf).astype(f32)
    return allow_e, fill_e, allow_o, fill_o


def _rcombo(k, b11, b12, b21, b22):
    if k in (1, 4):
        return (b11 if k == 1 else b22)(k)
    a, b, sign = {0: (b11, b22, 1), 2: (b12, b22, -1), 3: (b21, b11, -1), 5: (b11, b12, 1), 6: (b21, b22, 1)}[k]
    a, b = _unpack(a(k)), _unpack(b(k))
    return (a + b if sign > 0 else a - b).astype(bf16)


def _softmax(s, allow, fill):
    s = jnp.where(allow, s * SCALE, fill)
    m = jnp.max(s, axis=-1, keepdims=True)
    e = jnp.exp(s - m)
    l = jnp.sum(e, axis=-1, keepdims=True)
    r = pl.reciprocal(l, approx=True)
    r = r * (2.0 - l * r)
    return (e * r).astype(bf16)


def _kernel(x_hbm, mem0_hbm, wq_hbm, wk_hbm, wv_hbm, wo_hbm, w1_hbm, w2_hbm, w3_hbm, w4_hbm,
            gw_hbm, out_hbm,
            x_v, s1_v, s2_v, s3_v, s4_v, wqkv_v, wo_v, h_v, b_v, c0_v, l_v, lf_v, n_v, g_v, out_v, xe_v, e_v, oe_v,
            ke_v, ve_v, o_v, mem_v, mem0_ref, gw_ref, zero_s,
            sem, sem_qkv, sem_out):
    RAW = (1, 2, 3, 4)
    RAW1 = (1, 7, 8, 4)

    loads = []

    def rows_load(name, r0, r1):
        loads.append((name, x_hbm.at[pl.ds(r0, r1 - r0)], x_v.at[pl.ds(r0, r1 - r0)]))

    def quad_load(name, w_hbm, s_v, raw, q, c0=0, c1=None):
        k4, n2 = s_v.shape[1], s_v.shape[2]
        c1 = n2 if c1 is None else c1
        src = w_hbm.bitcast(u32).at[pl.ds((q // 2) * k4, k4), pl.ds((q % 2) * n2 + c0, c1 - c0)]
        loads.append((name, src, s_v.at[raw[q], :, pl.ds(c0, c1 - c0)]))

    def w1_load(name, half, c0, c1):
        quad_load(name, w1_hbm, s1_v, RAW1, half, c0, c1)
        quad_load(name, w1_hbm, s1_v, RAW1, 2 + half, c0, c1)

    def block_load(name, w_hbm, s_v, r0, r1):
        kb, nb = s_v.shape[1:]
        for q in range(16):
            loads.append((name, w_hbm.at[pl.ds((q // 4) * kb + r0, r1 - r0), pl.ds((q % 4) * nb, nb)],
                          s_v.at[RAW16[q], pl.ds(r0, r1 - r0)]))

    rows_load("x0", 0, TM)
    w1_load("w1a", 0, 0, 256)
    w1_load("w1b", 0, 256, 512)
    rows_load("x1", TM, 2 * TM)
    w1_load("w1cd", 1, 0, 512)
    rows_load("x23", 2 * TM, 4 * TM)
    rows_load("x4567", 4 * TM, S)
    for q in range(4):
        quad_load("w2", w2_hbm, s2_v, RAW, q)
    block_load("w2", w3_hbm, s3_v, 0, W3A)
    block_load("w4", w3_hbm, s3_v, W3A, D4)
    block_load("w4", w4_hbm, s4_v, 0, F4)
    loads.append(("small", mem0_hbm, mem0_ref))
    loads.append(("small", gw_hbm, gw_ref))
    for j in range(NT):
        loads.append(("wo", wo_hbm.bitcast(u32).at[:, pl.ds(j * 128, 128)], wo_v.at[j]))
    groups = list(dict.fromkeys(name for name, _, _ in loads))
    assert len(groups) == NLOAD

    def start(*names, priority=0):
        for name, src, dst in loads:
            if name in names:
                pltpu.make_async_copy(src, dst, sem.at[groups.index(name)]).start(priority=priority)

    def wait(*names):
        for name, src, dst in loads:
            if name in names:
                pltpu.make_async_copy(src, dst, sem.at[groups.index(name)]).wait()

    SPG = 3 * G

    def qkv_start(g):
        for w, w_hbm in enumerate((wq_hbm, wk_hbm, wv_hbm)):
            wu = w_hbm.bitcast(u32)
            for k in range(G // 2):
                for par in range(2):
                    pltpu.make_async_copy(
                        wu.at[:, par * (H // 2) + g * (G // 2) + k, :],
                        wqkv_v.at[g * SPG + w * G + 2 * k + par], sem_qkv.at[g]).start(priority=1)

    def qkv_wait(g):
        grp = wqkv_v.at[pl.ds(g * SPG, SPG)]
        pltpu.make_async_copy(grp, grp, sem_qkv.at[g]).wait()

    start("x0", "w1a", "w1b", "x1", "w1cd", "x23", "x4567", "w2", "w4", "small")

    def zero(k, carry):
        zero_s[k] = 0
        return carry
    lax.fori_loop(0, RK, zero, 0)

    def tile_idx(ref, cols=128):
        z = zero_s[0]
        n = 16 if ref.dtype == bf16 and cols == 128 else 8
        return (z,) * (len(ref.shape) - 2) + (pl.ds(pl.multiple_of(z, n), n), slice(0, cols))

    hist = []

    def mm(lhs, rhs, side=None, acc=None):
        if side is not None:
            lhs = side(lhs)
        lhs = pltpu.bitcast(lhs, bf16) if lhs.dtype == u32 else lhs.astype(bf16)
        y = _dot(lhs, pltpu.bitcast(rhs, bf16) if rhs.dtype == u32 else rhs)
        if acc is not None:
            y = y + acc
        hist.append(y)
        return y

    class Side:
        def __init__(self, pieces, n, skip=0):
            cap = [0] * skip + ([1] * n if isinstance(n, int) else list(n))
            tot = sum(p[4] for p in pieces)
            self.plan = [[] for _ in cap]
            done = 0
            for p in pieces:
                done += p[4]
                x, d = done / tot * sum(cap), 0
                while x > cap[d] + 1e-9:
                    x -= cap[d]
                    d += 1
                self.plan[d].append((p, x / cap[d]))
            self.pieces = len(pieces)

        def __call__(self, val):
            todo = self.plan.pop(0) if self.plan else []
            if not todo:
                return val
            self.pieces -= len(todo)
            never = zero_s[0] > 0
            if val.dtype == bf16:
                val = pltpu.bitcast(val, u32)
            rg = 8 if val.dtype == u32 else 16
            ng = val.shape[0] // rg
            tied = {}
            for (fn, rd, wr, lag, _), pos in todo:
                m = min(max(-int(-pos * ng // 1) - 1, 0), ng - 1)
                pin = lambda v, w=128: v
                if lag is not None and len(hist) >= lag:
                    r0 = (16 * m) % hist[-lag].shape[0]
                    a = hist[-lag][r0:r0 + 8, :128]
                    if rd is None:
                        def pin(v, w=128, a=a):
                            a = _cat([_cat([_as(a, v.dtype)] * (v.shape[0] // 8), 0)] * (w // 128), 1)
                            if v.shape[1] == w:
                                return lax.select(never, a, v)
                            return _cat([lax.select(never, a, v[:, :w]), v[:, w:]], 1)
                    elif rd.dtype == bf16:
                        idx = tile_idx(rd, 256)
                        rd[idx] = lax.select(never, _cat([a, a], 1).astype(bf16), rd[idx])
                    else:
                        idx = tile_idx(rd)
                        rd[idx] = lax.select(never, _as(a, rd.dtype), rd[idx])
                u = fn(pin)
                if wr is False:
                    continue
                if wr is not None:
                    u = wr[tile_idx(wr)]
                t, n = tied.get(m * rg) or (val[m * rg:m * rg + 8, -128:], 0)
                tied[m * rg] = (lax.select(zero_s[n] > 0, _as(u, val.dtype), t), n + 1)
            if not tied:
                return val
            col, r = [], 0
            for r0 in sorted(tied):
                col += ([val[r:r0, -128:]] if r0 > r else []) + [tied[r0][0]]
                r = r0 + 8
            col += [val[r:, -128:]] if r < val.shape[0] else []
            return _cat([val[:, :-128], _cat(col, 0)], 1) if val.shape[1] > 128 else _cat(col, 0)

    def strassen(lhs, rhs, side, init=(None, None, None, None)):
        def add(a, b):
            return a if b is None else a + b
        p = [mm(lhs(k), rhs(k), side) for k in range(5)]
        c12 = add(p[2] + p[4], init[1])
        c21 = add(p[1] + p[3], init[2])
        c22 = mm(lhs(5), rhs(5), side, add(p[0] - p[1] + p[2], init[3]))
        c11 = mm(lhs(6), rhs(6), side, add(p[0] + p[3] - p[4], init[0]))
        return c11, c12, c21, c22

    def fmm(lhs, rhs, side, extra=lambda n: None, emit=None):
        val = {}
        for n in WORDER:
            t = extra(n)
            for q, sg in sorted(_WPAR[n], key=lambda e: -e[1]):
                t = val[q] if t is None else (t + val[q] if sg > 0 else t - val[q])
            for r in range(RK):
                if WN[r] == n:
                    t = mm(lhs(UN[r]), rhs(r), side, t)
            val[n] = t
            if n < 8 and emit is not None:
                emit(n, t)
        return [val[v] for v in range(8)]

    def prep26_pieces(s_v, lag):
        def piece(rs, cs, pin):
            @functools.lru_cache(None)
            def node(n):
                if n < 16:
                    return s_v[RAW16[n], rs, cs].astype(f32)
                a, sa, b, sb = VP[n - 16]
                return _run([(0, sa, 1, sb)], [node(a), node(b)])[-1]
            vals = [node(VN[r]).astype(bf16) for r in VORDER]
            for r, t in zip(VORDER, vals):
                s_v[r, rs, cs] = t
        kb, nb = s_v.shape[1:]
        out = []
        for r in range(0, kb, 16):
            out += [(slice(rr, rr + 8), slice(c, c + 256)) for c in range(0, nb - 255, 256) for rr in (r, r + 8)]
            out += [(slice(rr, rr + 8), slice(nb - 128, nb)) for rr in (r, r + 8)] if nb % 256 else []
        return [(functools.partial(piece, rs, cs), s_v, s_v if n % 16 == 15 else False, lag,
                 130 if cs.stop - cs.start == 256 else 100) for n, (rs, cs) in enumerate(out)]

    def prep_pieces(s_v, raw, lag, width=256):
        def piece(r, c, pin):
            idx = (slice(r, r + 8), slice(c, c + width))
            b11, b12, b21, b22 = [_unpack(pin(s_v[(q,) + idx], width) if n in (0, 3) else s_v[(q,) + idx])
                                  for n, q in enumerate(raw)]
            for k, t in ((0, b11 + b22), (2, b12 - b22), (3, b21 - b11), (5, b11 + b12), (6, b21 + b22)):
                s_v[(k,) + idx] = _pack(t)
        return [(functools.partial(piece, r, c), None, s_v, lag, 80)
                for c in range(0, s_v.shape[2], width) for r in range(0, s_v.shape[1], 8)]

    def store_l(slot, q, c, quads, plain=False):
        for k, t in enumerate(quads if plain else _lcombos(*quads)):
            l_v[slot, k, q // 2:q // 2 + 8, c:c + t.shape[1]] = _pack(t)

    def ln_pieces(src, r0, slot, lag, plain=False, width=256, staged=False, clag=None):
        def stats(q, pin):
            x = pin(src[pl.ds(r0 + q, 16), :].astype(f32))
            xs = [x[:, j * 128:(j + 1) * 128] for j in range(NT)]
            m = functools.reduce(lambda a, b: a + b, xs) * (1.0 / NT)
            w = functools.reduce(lambda a, b: a + b, [(t - m) * (t - m) for t in xs])
            mean = jnp.mean(m, axis=-1, keepdims=True)
            var = jnp.sum(w + NT * ((m - mean) * (m - mean)), axis=-1, keepdims=True) * (1.0 / D)
            n_v[0, q:q + 16, :] = jnp.broadcast_to(mean, (16, 128))
            n_v[1, q:q + 16, :] = jnp.broadcast_to(lax.rsqrt(var + EPS), (16, 128))

        def comb(q, c, pin):
            quads = []
            for rr in (0, HM):
                rs = pl.ds(pl.multiple_of(r0 + rr + q + zero_s[0], 16), 16)
                mean, rstd = [jnp.concatenate([n_v[t, rr + q:rr + q + 16, :]] * (width // 128), axis=1)
                              for t in range(2)]
                quads += [(src[rs, cc + c:cc + c + width].astype(f32) - mean) * rstd for cc in (0, DH2)]
            store_l(slot, q, c, quads, plain)

        def comb26(q, pin):
            blocks = []
            for rr in (0, HM):
                rs = pl.ds(pl.multiple_of(r0 + rr + q + zero_s[0], 8), 8)
                mean, rstd = [jnp.concatenate([n_v[t, rr + q:rr + q + 8, :]] * 2, axis=1) for t in range(2)]
                blocks += [(src[rs, cc:cc + D4] - mean) * rstd for cc in range(0, D, D4)]
            vals = _run(UP, blocks)
            for k, u in enumerate(UL):
                lf_v[k, q:q + 8, :] = vals[u].astype(bf16)
        dense = slot is not None or src is b_v
        norms = [[(functools.partial(stats, rr + q), None, n_v if dense else False, lag, 90) for rr in (0, HM)]
                 for q in range(0, HM, 16)]
        if slot is None:
            combs = [[(functools.partial(comb26, qq), n_v, lf_v if dense or qq % 32 == 24 else False, clag, 110)
                      for qq in (q, q + 8)] for q in range(0, HM, 16)]
        else:
            combs = [[(functools.partial(comb, q, c), n_v, l_v, clag, 125) for c in range(0, DH2, width)]
                     for q in range(0, HM, 16)]
        if staged:
            return sum(norms, []), sum(combs, [])
        out = list(norms[0])
        for a, b in zip(norms[1:] + [[]], combs):
            out += _merge(a, b) if a else b
        return out

    shifts = (1, 1, -1, -1, 2, 2, -2, -2)

    def shift_pieces(r0, slot, lag, by_value=False):
        def piece(q, j, pin):
            a = [h_v[jj, pl.ds(PAD + r0 + rr + q - shifts[jj], 16), :]
                 for rr in (0, HM) for jj in (j, j + NT // 2)]
            store_l(slot, q, j * 128, [pin(a[0]), a[1], a[2], pin(a[3])])
        return [(functools.partial(piece, q, j), None if by_value else h_v,
                 l_v if (q // 16) % 2 and j == 3 else False, lag, 50)
                for q in range(0, HM, 16) for j in range(NT // 2)]

    def lhs_of(slot):
        return lambda k: l_v[slot, k]

    xe_v[0, 0:16, :] = jnp.zeros((16, D4), bf16)
    h_v[:, 0:PAD, :] = jnp.zeros((NT, PAD, 128), f32)
    h_v[:, PAD + S:PAD + S + PAD, :] = jnp.zeros((NT, PAD, 128), f32)

    def store_h(r0, c0, h):
        for j in range(h.shape[1] // 128):
            h_v[c0 // 128 + j, PAD + r0:PAD + r0 + h.shape[0], :] = h[:, j * 128:(j + 1) * 128]

    def h_pieces(r0, c0, t, lag, n=4):
        def piece(r, pin):
            store_h(r0 + r, c0, _gelu(pin(t[r:r + 8 * n])))
        return [(functools.partial(piece, r), None, h_v, lag, 10 * n) for r in range(0, t.shape[0], 8 * n)]

    def flush(pieces):
        for p in pieces:
            p[0](lambda v, w=128: v)

    def w1_cols(c, step):
        half, cc = c // DH2, c % DH2
        return jnp.concatenate([s1_v[RAW1[half], :, cc:cc + step], s1_v[RAW1[2 + half], :, cc:cc + step]], axis=0)

    def d1_plain(xn, r0, c0, c1, step):
        for c in range(c0, c1, step):
            store_h(r0, c, _gelu(mm(xn, w1_cols(c, step))))

    def d1_fine(lhs, r0, nrb, cols, pieces, carry, skip=0):
        tiles = [(rb, c) for c in cols for rb in range(nrb)]
        rounds = [tiles[i:i + 4] for i in range(0, len(tiles), 4)]
        for n, (rnd, part) in enumerate(zip(rounds, split(pieces, len(rounds)))):
            sk = skip if n == 0 else 0
            side = Side(_merge(carry, part) if carry else part, 8 - sk, sk)
            carry = []
            for rb, c in rnd:
                half, cc = c // DH2, c % DH2
                t = mm(lhs(rb, 0), s1_v[RAW1[half], :, cc:cc + 128], side)
                t = mm(lhs(rb, 1), s1_v[RAW1[2 + half], :, cc:cc + 128], side, t)
                carry += h_pieces(r0 + rb * HM, c, t, LS)
        return carry

    CAP1 = (1, 1, 1, 1, 1, 1, 1)
    CAP2 = (2, 3, 3, 3, 3, 3, 2)

    def d1_s(b, slot, pieces, carry):
        for c, part in zip(range(0, DH2, NC1), split(pieces, DH2 // NC1)):
            side = Side(merge(carry, part), CAP1 if hist else (0, 0) + CAP1[2:])
            cs = strassen(lhs_of(slot), lambda k: s1_v[k, :, c:c + NC1], side)
            carry = sum([h_pieces(b * TM + (q // 2) * HM, (q % 2) * DH2 + c, cs[q], LS) for q in (1, 2, 3, 0)], [])
        return carry

    def d2_s(b, slot, pieces, carry=(), early=(), late=()):
        for c, part, e in zip(range(0, DH2, NC1), split(pieces, DH2 // NC1), split(early, 2) + split(late, 2)):
            side = Side(merge(carry, part, e), CAP2 if hist else (0, 0) + CAP2[2:])
            carry = ()
            idx = [(slice(b * TM + (q // 2) * HM, b * TM + (q // 2 + 1) * HM),
                    slice((q % 2) * DH2 + c, (q % 2) * DH2 + c + NC1)) for q in range(4)]
            cs = strassen(lhs_of(slot), lambda k: s2_v[k, :, c:c + NC1], side,
                          [x_v[i].astype(f32) for i in idx])
            for i, t in zip(idx, cs):
                b_v[i] = t
                if b == 0:
                    c0_v[i] = t

    def split(l, n):
        w = [1.0 if hist else 0.6] + [1.0] * (n - 1)
        cut = [int(round(len(l) * sum(w[:i]) / sum(w))) for i in range(n + 1)]
        return [l[cut[i]:cut[i + 1]] for i in range(n)]

    def merge(*ls):
        ls = [l for l in ls if l]
        return _merge(*ls) if ls else []

    NW1, NW3, N30 = 32, 32, 20
    LS, LL = 3, 5

    wait("x0")
    xn0 = _pack(_ln(x_v[0:TM, :].astype(f32)))
    wait("w1a")
    d1_plain(xn0, 0, 0, 256, 256)
    wait("w1b")
    d1_plain(xn0, 0, 256, 512, 256)
    wait("x1")
    xn1 = _pack(_ln(x_v[TM:2 * TM, :].astype(f32)))
    d1_plain(xn1, TM, 0, 512, 256)
    wait("w1cd")
    hist.clear()
    xn01 = jnp.concatenate([xn0, xn1], axis=0)
    l01 = lambda rb, kh: xn01[rb * 64:(rb + 1) * 64, kh * DH2:(kh + 1) * DH2]
    pw = prep_pieces(s1_v, RAW1, LS)
    flush(d1_fine(l01, 0, 4, (512, 640), pw[:NW1], [], 1))
    carry = []
    wait("x23")
    hist.clear()
    carry = d1_fine(l01, 0, 4, (768, 896), ln_pieces(x_v, 2 * TM, 0, LL, plain=True), carry, 3)
    carry = d1_fine(lambda rb, kh: l_v[0, 2 * rb + kh], 2 * TM, 2, range(0, D, 128),
                    _merge(pw[NW1:], ln_pieces(x_v, 3 * TM, 1, LL)), carry)
    wait("x4567")
    qkv_start(0)
    qkv_start(1)
    hist.clear()
    for b in range(3, NB - 1):
        carry = d1_s(b, b % 2, ln_pieces(x_v, (b + 1) * TM, (b + 1) % 2, LL), carry)
    wait("w2")
    hist.clear()
    pw = prep_pieces(s2_v, RAW, LS)
    p3 = prep26_pieces(s3_v, 2)
    n3 = len(p3) * W3A // D4
    carry = d1_s(7, 1, _merge(pw[:NW3], shift_pieces(0, 0, LS, True)), carry)
    d2_s(0, 0, shift_pieces(TM, 1, LS, True), carry, pw[NW3:], p3[:N30])
    pw = split(_merge(p3[N30:n3], sum(ln_pieces(c0_v, 0, None, LL, clag=LS, staged=True), [])), 3)
    for b in range(1, 4):
        d2_s(b, b % 2, _merge(pw[b - 1], shift_pieces((b + 1) * TM, (b + 1) % 2, LS)))
    wait("w4", "small")
    hist.clear()
    pw = p3[n3:] + prep26_pieces(s4_v, 2)
    cut = (0, 31, 65, 99, len(pw))
    for b in range(4, NB):
        d2_s(b, b % 2, merge(pw[cut[b - 4]:cut[b - 3]],
                             shift_pieces((b + 1) * TM, (b + 1) % 2, LS) if b + 1 < NB else ()))
    start("wo", priority=1)

    def ffn(i, carry):
        qkv_wait(i)
        r0 = pl.multiple_of(i * TM, TM)
        rn = pl.multiple_of(jnp.minimum(i + 1, NB - 1) * TM, TM)
        acc = {}
        hist.clear()

        def relayout(p, r0_, r1_, pin):
            s0 = i * SPG + 2 * p
            e = wqkv_v[s0, r0_:r1_, :]
            o = wqkv_v[s0 + 1, r0_:r1_, :]
            wqkv_v[s0, r0_:r1_, :] = (e & jnp.uint32(0xFFFF)) | (o << 16)
            wqkv_v[s0 + 1, r0_:r1_, :] = (e >> 16) | (o & jnp.uint32(0xFFFF0000))

        relays = [(functools.partial(relayout, p, r, r + 32), wqkv_v, wqkv_v, 3, 35)
                  for p in range(SPG // 2) for r in range(0, D // 2, 32)]
        norms, combs = ln_pieces(b_v, rn, None, 5, staged=True, clag=3)

        def gate(q, pin):
            gw = gw_ref[...].astype(f32)
            x = pin(x_v[pl.ds(r0 + q, 16), :].astype(f32))
            t = functools.reduce(lambda a, b: a + b,
                                 [x[:, j * 128:(j + 1) * 128] * gw[j:j + 1, :] for j in range(NT)])
            g = jax.nn.sigmoid(jnp.sum(t, axis=-1, keepdims=True))
            g_v[pl.ds(r0 + q, 16), :] = jnp.broadcast_to(g, (16, 128))

        gates = [(functools.partial(gate, q), None, g_v, 5, 90) for q in range(0, TM, 16)]

        def extras(t, pin):
            jj, o = 2 * i + t // 2, 24 + 8 * (t % 2)
            xs = [pin(x_v[pl.ds(pl.multiple_of((jj + hh) * 64 + o, 8), 8), :].astype(f32)) for hh in (0, NPAIR // 2)]
            vals = _run(UP, [x[:, cc:cc + D4] for x in xs for cc in range(0, D, D4)])
            for k, u in enumerate(UL):
                xe_v[k, pl.ds(pl.multiple_of(i * 32 + t * 8, 8), 8), :] = vals[u].astype(bf16)

        xes = [(functools.partial(extras, t), None, xe_v, 3, 100) for t in range(4)]
        hs = {}

        def gelu_pieces(c, cs):
            def piece(r, cc, vs, pin):
                t = _gelu(pin(_cat([cs[v][r:r + 8, cc:cc + 128] for v in vs], 0)))
                ts = [t[8 * n:8 * n + 8] for n in range(len(vs))]
                hs.update({(c, v, r, cc): u for v, u in zip(vs, ts)})
                return functools.reduce(lambda a, b: a + b, ts)
            return [(functools.partial(piece, r, cc, vs), None, None, 3, 40) for r in range(0, HM, 8)
                    for cc in range(0, cs[0].shape[1], 128) for vs in ((0, 1, 2, 3), (4, 5, 6, 7))]

        def d3(c, side):
            c0, c1 = FCH[c]
            cs = fmm(lambda u: lf_v[UL.index(u)], lambda r: s3_v[r, :, c0:c1], side)
            assert not side.pieces
            return gelu_pieces(c, cs)

        def d4(c, side):
            c0, c1 = FCH[c]
            lh = _run(UP, [_cat([_cat([hs.pop((c, v, r, cc)) for r in range(0, HM, 8)], 0)
                                 for cc in range(0, c1 - c0, 128)], 1) for v in range(8)])
            rhs = lambda r: s4_v[r, c0:c1, :]
            if c + 1 < len(FCH):
                for n in WORDER:
                    for r in range(RK):
                        if WN[r] == n:
                            acc[n] = mm(lh[UN[r]], rhs(r), side, acc.get(n))
            else:
                idx = lambda v: (pl.ds(r0 + (v // 4) * HM, HM), slice((v % 4) * D4, (v % 4 + 1) * D4))

                def extra(n):
                    if n >= 8:
                        return acc.get(n)
                    return b_v[idx(n)] + acc[n] if n in acc else b_v[idx(n)]

                def emit_b(v, t):
                    b_v[idx(v)] = jnp.concatenate([1.0 - g_v[idx(v)[0], :]] * 2, axis=1) * t
                fmm(lambda u: lh[u], rhs, side, extra, emit_b)
            assert not side.pieces

        g0 = d3(0, Side(relays[:20], 23, 3))
        g1 = d3(1, Side(_merge(g0, gates, xes), 23, 2))
        d4(0, Side(g1[:22], 22, 4))
        g2 = d3(2, Side(_merge(g1[22:], relays[20:40]), 25))
        d4(1, Side(g2, 23, 2))
        g3 = d3(3, Side(_merge(relays[40:], norms), 26))
        d4(2, Side(_merge(g3, combs), 23, 2))
        d4(3, Side([], 1))

        @pl.when(i + 2 < NG)
        def _():
            qkv_start(i + 2)

        return carry

    lax.fori_loop(0, NB, ffn, 0)

    def pre(it, carry):
        hist.clear()
        for u in range(3 * NG // NPRE):
            s0 = (it * (3 * NG // NPRE) + u) * G

            def rhs(r):
                t = None
                sz = s0 + zero_s[r]
                for q, sg in sorted(_terms(VP, 16, VN[r]).items(), key=lambda e: -e[1]):
                    blk = wqkv_v[sz + q % 4, (q // 4) * (D // 8):(q // 4 + 1) * (D // 8), :]
                    if VN[r] < 16:
                        return blk
                    blk = _unpack(blk)
                    t = blk if t is None else (t + blk if sg > 0 else t - blk)
                return t.astype(bf16)
            for v, t in enumerate(fmm(lambda k: xe_v[UL.index(k)], rhs, None)):
                e_v[(v // 4) * 16:(v // 4 + 1) * 16, s0 + v % 4] = _pack(t).reshape(16, 8, DH)
        return carry

    lax.fori_loop(0, NPRE, pre, 0)

    wait("wo")
    mem_v[...] = mem0_ref[...].astype(f32)

    def slab(w, h):
        return (h // G) * SPG + w * G + h % G

    def step(j, hx, odd, late, allow, fill):
        qs, ks, vs, ps = {}, {}, {}, {}
        wload = lambda w, h: pltpu.bitcast(wqkv_v[slab(w, h)], bf16)
        eload = lambda w, h: pltpu.bitcast(e_v[j, slab(w, h)], bf16)

        def proj(g):
            part = {}
            if late and g == 0:
                for h in range(2):
                    for w in range(3):
                        part[w, h] = _dot(hx[:, :DH2], wload(w, h)[:DH2])
            for h in range(g * G, (g + 1) * G):
                q, k, v = [(_dot(hx[:, DH2:], wload(w, h)[DH2:]) + part[w, h] if (w, h) in part
                            else _dot(hx, wload(w, h))).astype(bf16) for w in range(3)]
                if odd:
                    q = jnp.concatenate([q, eload(0, h)], axis=0)
                    k = jnp.concatenate([pltpu.bitcast(ke_v[h], bf16), eload(1, h), k], axis=0)
                    v = jnp.concatenate([pltpu.bitcast(ve_v[h], bf16), eload(2, h), v], axis=0)
                else:
                    ke_v[h] = pltpu.bitcast(k, u32)
                    ve_v[h] = pltpu.bitcast(v, u32)
                    k = jnp.concatenate([k, eload(1, h)], axis=0)
                    v = jnp.concatenate([v, eload(2, h)], axis=0)
                qs[h], ks[h], vs[h] = q, k, v

        def score(g):
            for h in range(g * G, (g + 1) * G):
                s = lax.dot_general(qs.pop(h), ks.pop(h), (((1,), (1,)), ((), ())),
                                    preferred_element_type=f32)
                ps[h] = _softmax(s, allow, fill)

        def pv(g):
            os_ = []
            for h in range(g * G, (g + 1) * G):
                o = _dot(ps.pop(h), vs.pop(h))
                o_v[:, h * 128:(h + 1) * 128] = _pack(o[:32])
                os_.append(o)
            if odd:
                quads = [jnp.concatenate([os_[2 * kk][r:r + 8], os_[2 * kk + 1][r:r + 8]], axis=1)
                         for r in (32, 40) for kk in range(2)]
                for k, t in enumerate(_lcombos(*quads)):
                    oe_v[k, pl.ds(pl.multiple_of(j * 8, 8), 8), g * 256:(g + 1) * 256] = t.astype(bf16)

        acc = [None] * NT

        def wo(h0, h1, j0, j1):
            o = pltpu.bitcast(o_v[:, h0 * 128:h1 * 128], bf16)
            for n in range(j0, j1):
                y = _dot(o, pltpu.bitcast(wo_v[n, h0 * 64:h1 * 64, :], bf16))
                acc[n] = y if acc[n] is None else y + acc[n]

        for t in range(NG):
            proj(t)
            if t >= 2:
                pv(t - 2)
            if t >= 1:
                score(t - 1)
        wo(0, 16, 0, 4)
        pv(NG - 2)
        score(NG - 1)
        wo(0, 16, 4, 8)
        pv(NG - 1)
        wo(16, 24, 0, 8)
        wo(24, 32, 0, 8)
        return jnp.concatenate(acc, axis=1)

    def emit(j, r0, o0, a):
        rs = pl.ds(r0 + o0, 24)
        g = jnp.concatenate([g_v[rs, :]] * NT, axis=1)
        out_v[j, o0:o0 + 24, :] = (g * a + b_v[rs, :]).astype(bf16)

    def pair(j, mem, late):
        r0 = pl.multiple_of(j * 64, 64)
        allow_e, fill_e, allow_o, fill_o = _masks()
        xa = x_v[pl.ds(r0 + 16, 8), :].astype(f32)
        xb = x_v[pl.ds(r0 + 40, 8), :].astype(f32)
        hx = jnp.concatenate([x_v[pl.ds(r0, 16), :], jnp.concatenate([xa, mem], 0).astype(bf16)], 0)
        oe = step(j, hx, False, late, allow_e, fill_e)
        emit(j, r0, 0, oe[:24])
        hx = jnp.concatenate([jnp.concatenate([oe[24:32], xb], 0).astype(bf16), x_v[pl.ds(r0 + 48, 16), :]], 0)
        oo = step(j, hx, True, True, allow_o, fill_o)
        emit(j, r0, 40, oo[8:])
        return oo[:8]

    def a_iter(it, carry):
        mem = mem_v[...]
        for t in range(PPI):
            mem = pair(it * PPI + t, mem, t > 0)
        mem_v[...] = mem
        for t in range(PPI):
            for o0 in (0, 40):
                idx = (it * PPI + t, pl.ds(o0, 24))
                pltpu.make_async_copy(out_v.at[idx], out_hbm.at[idx], sem_out).start()
        return carry

    lax.fori_loop(0, NPAIR // PPI, a_iter, 0)

    hist.clear()
    for n in range(NT // 2):
        quad = [lambda k, t=2 * n + q % 2, o=(q // 2) * 128: jnp.concatenate(
            [wo_v[t + zero_s[k], g * 256 + o:g * 256 + o + 128, :] for g in range(NG)], axis=0) for q in range(4)]
        cs = strassen(lambda k: oe_v[k], lambda k: _rcombo(k, *quad), None)
        cols = slice(n * 256, (n + 1) * 256)
        for half in range(2):
            t = jnp.concatenate(cs[2 * half:2 * half + 2], axis=1)
            o0 = 24 + half * 8
            for jj in range(NPAIR):
                rs = slice(jj * 64 + o0, jj * 64 + o0 + 8)
                g = jnp.concatenate([g_v[rs, :]] * 2, axis=1)
                out_v[jj, o0:o0 + 8, cols] = (g * t[jj * 8:jj * 8 + 8] + b_v[rs, cols]).astype(bf16)
        if n >= 2:
            idx = (slice(None), pl.ds(24, 16), pl.ds(0, 768) if n == 2 else pl.ds(768, 256))
            pltpu.make_async_copy(out_v.at[idx], out_hbm.at[idx], sem_out).start()
    pltpu.make_async_copy(out_v, out_hbm, sem_out).wait()


@jax.jit
def pallas_gated_mix__memory_aug_recurrent_mem_tr__mixer_s_mlp__prompt_kernel(
    A_x, A_mem0, A_Wq, A_Wk, A_Wv, A_Wo, A_seg_len, B_x, B_w1, B_w2, B_w3, B_w4, gate_w,
):
    assert A_x.shape == (1, S, D) and A_mem0.shape == (1, M, D)
    any_spec = pl.BlockSpec(memory_space=pl.ANY)
    out = pl.pallas_call(
        _kernel,
        out_shape=jax.ShapeDtypeStruct((NPAIR, 64, D), bf16),
        in_specs=[any_spec] * 11,
        out_specs=any_spec,
        scratch_shapes=[
            pltpu.VMEM((S, D), bf16),
            pltpu.VMEM((9, D // 4, D // 2), u32),
            pltpu.VMEM((7, D // 4, D // 2), u32),
            pltpu.VMEM((RK, D4, F4), bf16),
            pltpu.VMEM((RK, F4, D4), bf16),
            pltpu.VMEM((3 * H, D // 2, DH), u32),
            pltpu.VMEM((NT, H * DH // 2, 128), u32),
            pltpu.VMEM((NT, S + 2 * PAD, 128), f32),
            pltpu.VMEM((S, D), f32),
            pltpu.VMEM((TM, D), f32),
            pltpu.VMEM((2, 7, HM // 2, D // 2), u32),
            pltpu.VMEM((len(UL), HM, D4), bf16),
            pltpu.VMEM((2, TM, 128), f32),
            pltpu.VMEM((S, 128), f32),
            pltpu.VMEM((NPAIR, 64, D), bf16),
            pltpu.VMEM((len(UL), 8 * NPAIR, D4), bf16),
            pltpu.VMEM((NPAIR, 3 * H, 8, DH), u32),
            pltpu.VMEM((7, 8 * NPAIR, H * DH // 2), bf16),
            pltpu.VMEM((H, 16, 128), u32),
            pltpu.VMEM((H, 16, 128), u32),
            pltpu.VMEM((16, H * DH), u32),
            pltpu.VMEM((M, D), f32),
            pltpu.VMEM((M, D), bf16),
            pltpu.VMEM((NT, 128), bf16),
            pltpu.SMEM((RK,), jnp.int32),
            pltpu.SemaphoreType.DMA((NLOAD,)),
            pltpu.SemaphoreType.DMA((NG,)),
            pltpu.SemaphoreType.DMA,
        ],
        compiler_params=pltpu.CompilerParams(vmem_limit_bytes=126 * 1024 * 1024,
                                             disable_bounds_checks=True),
    )(
        A_x.reshape(S, D), A_mem0.reshape(M, D),
        A_Wq.reshape(D // 2, 2 * H, DH), A_Wk.reshape(D // 2, 2 * H, DH), A_Wv.reshape(D // 2, 2 * H, DH),
        A_Wo.reshape(H * DH, D), B_w1, B_w2, B_w3, B_w4, gate_w.reshape(NT, 128),
    )
    return out.reshape(1, S, D)
```

```python
import functools

import jax
import jax.numpy as jnp
from jax import lax
import jax.experimental.pallas as pl
import jax.experimental.pallas.tpu as pltpu

f32, bf16, u32 = jnp.float32, jnp.bfloat16, jnp.uint32

S, D, H, DH, M, SEG, F = 2048, 1024, 32, 128, 8, 32, 3584
SCALE = DH ** -0.5
NEG = -1000000000.0
EPS = 1e-05

TM = 256
NB = S // TM
HM = TM // 2
DH2 = D // 2
D4, F4 = D // 4, F // 4
FCH = ((0, 128), (128, 384), (384, 640), (640, 896))
NC1 = 128
NPAIR = S // (2 * SEG)
PPI = 2
NPRE = 3
G = 4
NG = H // G
PAD = 8
NT = D // 128
W3A = 192
NLOAD = 11
assert NB == NG

_dot = functools.partial(jnp.dot, preferred_element_type=f32)

UP = ((4, 1, 5, 1), (6, 1, 8, 1), (0, 1, 3, 1), (2, -1, 9, 1), (4, -1, 10, 1), (0, 1, 1, 1), (2, 1, 12, 1),
      (5, 1, 7, -1), (7, 1, 12, -1), (11, -1, 13, 1), (10, -1, 11, 1), (2, 1, 7, 1), (0, -1, 4, 1),
      (6, 1, 7, 1), (1, -1, 5, 1), (3, 1, 7, -1), (1, 1, 4, 1), (2, 1, 3, 1), (1, -1, 3, 1), (1, 1, 7, -1),
      (2, 1, 6, -1))
WP = ((0, -1, 3, 1), (4, 1, 6, -1), (1, 1, 8, 1), (5, 1, 10, 1), (4, -1, 7, 1), (0, -1, 9, -1),
      (11, 1, 12, 1), (6, 1, 7, -1), (2, 1, 5, -1), (0, -1, 7, -1), (9, 1, 11, -1), (2, 1, 13, 1),
      (5, 1, 13, 1), (2, -1, 3, 1), (5, 1, 6, 1), (0, 1, 4, 1), (2, 1, 7, 1), (1, 1, 2, 1), (1, 1, 5, 1),
      (3, 1, 7, 1), (2, 1, 6, 1))
VP = ((1, 1, 5, -1), (8, 1, 11, 1), (10, 1, 17, 1), (13, 1, 16, -1), (0, 1, 4, -1), (0, 1, 3, 1),
      (14, 1, 18, -1), (0, 1, 11, 1), (14, 1, 19, -1), (0, 1, 5, 1), (12, 1, 15, 1), (2, 1, 21, 1),
      (10, 1, 14, -1), (4, 1, 7, 1), (11, 1, 19, 1), (12, -1, 20, 1), (13, 1, 14, -1), (9, 1, 30, -1),
      (3, -1, 15, 1), (6, 1, 23, 1), (24, 1, 27, -1), (9, -1, 18, 1), (7, 1, 34, 1), (2, 1, 6, -1),
      (0, 1, 8, -1), (6, 1, 21, 1), (22, 1, 31, -1), (6, 1, 29, 1), (0, 1, 1, 1), (15, 1, 25, 1),
      (5, 1, 37, 1), (15, 1, 20, 1))
UN = (7, 27, 24, 17, 9, 22, 21, 2, 15, 11, 8, 25, 19, 28, 2, 23, 26, 20, 1, 18, 10, 28, 4, 13, 14, 16)
WN = (23, 17, 24, 10, 14, 7, 22, 19, 12, 18, 15, 25, 20, 5, 26, 0, 8, 2, 27, 11, 26, 9, 28, 21, 16, 5)
VN = (42, 47, 41, 5, 11, 43, 18, 28, 20, 23, 35, 19, 22, 46, 33, 26, 45, 36, 38, 25, 44, 40, 39, 21, 24, 32)
RK = len(UN)
UL = tuple(sorted(set(UN)))
RAW16 = (1, 11, 17, 5, 8, 3, 9, 10, 0, 6, 7, 4, 12, 20, 22, 16)
VORDER = (0, 6, 7, 12, 13, 14, 15, 21, 11, 17, 20, 22, 24, 25, 23, 2, 1, 5, 8, 9, 10, 16, 18, 19)
assert sorted(VORDER) == [r for r in range(RK) if VN[r] >= 16] and len(set(RAW16)) == 16
assert all(RAW16[VN[r]] == r for r in range(RK) if VN[r] < 16)


def _run(prog, blocks):
    vals = list(blocks)
    for a, sa, b, sb in prog:
        vals.append(vals[a] + vals[b] if sa > 0 and sb > 0 else
                    vals[a] - vals[b] if sa > 0 else vals[b] - vals[a])
    return vals


def _terms(prog, nin, node):
    if node < nin:
        return {node: 1}
    a, sa, b, sb = prog[node - nin]
    out = {k: sa * v for k, v in _terms(prog, nin, a).items()}
    out.update({k: sb * v for k, v in _terms(prog, nin, b).items()})
    return out


_WPAR = {n: [] for n in range(8 + len(WP))}
for _t, (_a, _sa, _b, _sb) in enumerate(WP):
    _WPAR[_a].append((8 + _t, _sa))
    _WPAR[_b].append((8 + _t, _sb))


def _worder():
    order = []

    def closure(n, acc):
        if n not in acc and n not in order:
            acc.add(n)
            for q, _ in _WPAR[n]:
                closure(q, acc)
        return acc

    def visit(n):
        if n not in order:
            for q, _ in _WPAR[n]:
                visit(q)
            order.append(n)
    while len([v for v in range(8) if v not in order]):
        visit(min((v for v in range(8) if v not in order), key=lambda v: len(closure(v, set()))))
    return tuple(order)


WORDER = _worder()


def _ln(x):
    m = jnp.mean(x, axis=-1, keepdims=True)
    xc = x - m
    v = jnp.mean(xc * xc, axis=-1, keepdims=True)
    return xc * lax.rsqrt(v + EPS)


_GC = 0.7978845608028654


def _gelu(x):
    h = 0.5 * x
    return h + h * jnp.tanh(x * (_GC + (_GC * 0.044715) * (x * x)))


def _unpack(u):
    return pltpu.bitcast(u, bf16).astype(f32)


def _pack(x):
    return pltpu.bitcast(x.astype(bf16), u32)


def _cat(xs, axis):
    xs = [x for x in xs if x.shape[axis]]
    return xs[0] if len(xs) == 1 else jnp.concatenate(xs, axis=axis)


def _as(x, dtype):
    return x if x.dtype == dtype else pltpu.bitcast(x, dtype)


def _lcombos(a11, a12, a21, a22):
    return [a11 + a22, a21 + a22, a11, a22, a11 + a12, a21 - a11, a12 - a22]


def _merge(*lists):
    keyed = [((j + 0.5) / len(l), n, j, v) for n, l in enumerate(lists) for j, v in enumerate(l)]
    return [v for _, _, _, v in sorted(keyed, key=lambda t: t[:3])]


def _masks():
    r = lax.broadcasted_iota(jnp.int32, (32, 48), 0)
    c = lax.broadcasted_iota(jnp.int32, (32, 48), 1)
    exist_e = c < 40
    allow_e = exist_e & ((r >= 24) | ((c >= 24) & (c < 32)) | (c <= r))
    fill_e = jnp.where(exist_e, NEG, -jnp.inf).astype(f32)
    r = lax.broadcasted_iota(jnp.int32, (48, 80), 0)
    c = lax.broadcasted_iota(jnp.int32, (48, 80), 1)
    q_even = (r >= 32) & (r < 40)
    exist_o = (q_even & (c < 40)) | (~q_even & (c >= 40))
    ktok = jnp.where(c < 24, c, jnp.where(c < 48, c - 8, c - 16))
    qtok = jnp.where(r < 32, r + 32, r - 8)
    is_mem_key = ((c >= 24) & (c < 32)) | ((c >= 48) & (c < 56))
    allow_o = exist_o & (is_mem_key | (r < 8) | (ktok <= qtok))
    fill_o = jnp.where(exist_o, NEG, -jnp.inf).astype(f32)
    return allow_e, fill_e, allow_o, fill_o


def _rcombo(k, b11, b12, b21, b22):
    if k in (1, 4):
        return (b11 if k == 1 else b22)(k)
    a, b, sign = {0: (b11, b22, 1), 2: (b12, b22, -1), 3: (b21, b11, -1), 5: (b11, b12, 1), 6: (b21, b22, 1)}[k]
    a, b = _unpack(a(k)), _unpack(b(k))
    return (a + b if sign > 0 else a - b).astype(bf16)


def _softmax(s, allow, fill):
    s = jnp.where(allow, s * SCALE, fill)
    m = jnp.max(s, axis=-1, keepdims=True)
    e = jnp.exp(s - m)
    l = jnp.sum(e, axis=-1, keepdims=True)
    r = pl.reciprocal(l, approx=True)
    r = r * (2.0 - l * r)
    return (e * r).astype(bf16)


def _kernel(x_hbm, mem0_hbm, wq_hbm, wk_hbm, wv_hbm, wo_hbm, w1_hbm, w2_hbm, w3_hbm, w4_hbm,
            gw_hbm, out_hbm,
            x_v, s1_v, s2_v, s3_v, s4_v, wqkv_v, wo_v, h_v, b_v, c0_v, l_v, lf_v, n_v, g_v, out_v, xe_v, e_v, oe_v,
            ke_v, ve_v, o_v, mem_v, mem0_ref, gw_ref, zero_s,
            sem, sem_qkv, sem_out):
    RAW = (1, 2, 3, 4)
    RAW1 = (1, 7, 8, 4)

    loads = []

    def rows_load(name, r0, r1):
        loads.append((name, x_hbm.at[pl.ds(r0, r1 - r0)], x_v.at[pl.ds(r0, r1 - r0)]))

    def quad_load(name, w_hbm, s_v, raw, q, c0=0, c1=None):
        k4, n2 = s_v.shape[1], s_v.shape[2]
        c1 = n2 if c1 is None else c1
        src = w_hbm.bitcast(u32).at[pl.ds((q // 2) * k4, k4), pl.ds((q % 2) * n2 + c0, c1 - c0)]
        loads.append((name, src, s_v.at[raw[q], :, pl.ds(c0, c1 - c0)]))

    def w1_load(name, half, c0, c1):
        quad_load(name, w1_hbm, s1_v, RAW1, half, c0, c1)
        quad_load(name, w1_hbm, s1_v, RAW1, 2 + half, c0, c1)

    def block_load(name, w_hbm, s_v, r0, r1):
        kb, nb = s_v.shape[1:]
        for q in range(16):
            loads.append((name, w_hbm.at[pl.ds((q // 4) * kb + r0, r1 - r0), pl.ds((q % 4) * nb, nb)],
                          s_v.at[RAW16[q], pl.ds(r0, r1 - r0)]))

    rows_load("x0", 0, TM)
    w1_load("w1a", 0, 0, 256)
    w1_load("w1b", 0, 256, 512)
    rows_load("x1", TM, 2 * TM)
    w1_load("w1cd", 1, 0, 512)
    rows_load("x23", 2 * TM, 4 * TM)
    rows_load("x4567", 4 * TM, S)
    for q in range(4):
        quad_load("w2", w2_hbm, s2_v, RAW, q)
    block_load("w2", w3_hbm, s3_v, 0, W3A)
    block_load("w4", w3_hbm, s3_v, W3A, D4)
    block_load("w4", w4_hbm, s4_v, 0, F4)
    loads.append(("small", mem0_hbm, mem0_ref))
    loads.append(("small", gw_hbm, gw_ref))
    for j in range(NT):
        loads.append(("wo", wo_hbm.bitcast(u32).at[:, pl.ds(j * 128, 128)], wo_v.at[j]))
    groups = list(dict.fromkeys(name for name, _, _ in loads))
    assert len(groups) == NLOAD

    def start(*names, priority=0):
        for name, src, dst in loads:
            if name in names:
                pltpu.make_async_copy(src, dst, sem.at[groups.index(name)]).start(priority=priority)

    def wait(*names):
        for name, src, dst in loads:
            if name in names:
                pltpu.make_async_copy(src, dst, sem.at[groups.index(name)]).wait()

    SPG = 3 * G

    def qkv_start(g):
        for w, w_hbm in enumerate((wq_hbm, wk_hbm, wv_hbm)):
            wu = w_hbm.bitcast(u32)
            for k in range(G // 2):
                for par in range(2):
                    pltpu.make_async_copy(
                        wu.at[:, par * (H // 2) + g * (G // 2) + k, :],
                        wqkv_v.at[g * SPG + w * G + 2 * k + par], sem_qkv.at[g]).start(priority=1)

    def qkv_wait(g):
        grp = wqkv_v.at[pl.ds(g * SPG, SPG)]
        pltpu.make_async_copy(grp, grp, sem_qkv.at[g]).wait()

    start("x0", "w1a", "w1b", "x1", "w1cd", "x23", "x4567", "w2", "w4", "small")

    def zero(k, carry):
        zero_s[k] = 0
        return carry
    lax.fori_loop(0, RK, zero, 0)

    def tile_idx(ref, cols=128):
        z = zero_s[0]
        n = 16 if ref.dtype == bf16 and cols == 128 else 8
        return (z,) * (len(ref.shape) - 2) + (pl.ds(pl.multiple_of(z, n), n), slice(0, cols))

    hist = []

    def mm(lhs, rhs, side=None, acc=None):
        if side is not None:
            lhs = side(lhs)
        lhs = pltpu.bitcast(lhs, bf16) if lhs.dtype == u32 else lhs.astype(bf16)
        y = _dot(lhs, pltpu.bitcast(rhs, bf16) if rhs.dtype == u32 else rhs)
        if acc is not None:
            y = y + acc
        hist.append(y)
        return y

    class Side:
        def __init__(self, pieces, n, skip=0):
            cap = [0] * skip + [1] * n
            tot = sum(p[4] for p in pieces)
            self.plan = [[] for _ in cap]
            done = 0
            for p in pieces:
                done += p[4]
                x, d = done / tot * sum(cap), 0
                while x > cap[d] + 1e-9:
                    x -= cap[d]
                    d += 1
                self.plan[d].append((p, x / cap[d]))
            self.pieces = len(pieces)

        def __call__(self, val):
            todo = self.plan.pop(0) if self.plan else []
            if not todo:
                return val
            self.pieces -= len(todo)
            never = zero_s[0] > 0
            if val.dtype == bf16:
                val = pltpu.bitcast(val, u32)
            rg = 8 if val.dtype == u32 else 16
            ng = val.shape[0] // rg
            tied = {}
            for (fn, rd, wr, lag, _), pos in todo:
                m = min(max(-int(-pos * ng // 1) - 1, 0), ng - 1)
                pin = lambda v, w=128: v
                if lag is not None and len(hist) >= lag:
                    r0 = (16 * m) % hist[-lag].shape[0]
                    a = hist[-lag][r0:r0 + 8, :128]
                    if rd is None:
                        def pin(v, w=128, a=a):
                            a = _cat([_cat([_as(a, v.dtype)] * (v.shape[0] // 8), 0)] * (w // 128), 1)
                            if v.shape[1] == w:
                                return lax.select(never, a, v)
                            return _cat([lax.select(never, a, v[:, :w]), v[:, w:]], 1)
                    elif rd.dtype == bf16:
                        idx = tile_idx(rd, 256)
                        rd[idx] = lax.select(never, _cat([a, a], 1).astype(bf16), rd[idx])
                    else:
                        idx = tile_idx(rd)
                        rd[idx] = lax.select(never, _as(a, rd.dtype), rd[idx])
                u = fn(pin)
                if wr is False:
                    continue
                if wr is not None:
                    u = wr[tile_idx(wr)]
                t, n = tied.get(m * rg) or (val[m * rg:m * rg + 8, -128:], 0)
                tied[m * rg] = (lax.select(zero_s[n] > 0, _as(u, val.dtype), t), n + 1)
            if not tied:
                return val
            col, r = [], 0
            for r0 in sorted(tied):
                col += ([val[r:r0, -128:]] if r0 > r else []) + [tied[r0][0]]
                r = r0 + 8
            col += [val[r:, -128:]] if r < val.shape[0] else []
            return _cat([val[:, :-128], _cat(col, 0)], 1) if val.shape[1] > 128 else _cat(col, 0)

    def strassen(lhs, rhs, side, init=(None, None, None, None)):
        def add(a, b):
            return a if b is None else a + b
        p = [mm(lhs(k), rhs(k), side) for k in range(5)]
        c12 = add(p[2] + p[4], init[1])
        c21 = add(p[1] + p[3], init[2])
        c22 = mm(lhs(5), rhs(5), side, add(p[0] - p[1] + p[2], init[3]))
        c11 = mm(lhs(6), rhs(6), side, add(p[0] + p[3] - p[4], init[0]))
        return c11, c12, c21, c22

    def fmm(lhs, rhs, side, extra=lambda n: None, emit=None):
        val = {}
        for n in WORDER:
            t = extra(n)
            for q, sg in sorted(_WPAR[n], key=lambda e: -e[1]):
                t = val[q] if t is None else (t + val[q] if sg > 0 else t - val[q])
            for r in range(RK):
                if WN[r] == n:
                    t = mm(lhs(UN[r]), rhs(r), side, t)
            val[n] = t
            if n < 8 and emit is not None:
                emit(n, t)
        return [val[v] for v in range(8)]

    def prep26_pieces(s_v, lag):
        def piece(rs, cs, pin):
            @functools.lru_cache(None)
            def node(n):
                if n < 16:
                    return s_v[RAW16[n], rs, cs].astype(f32)
                a, sa, b, sb = VP[n - 16]
                return _run([(0, sa, 1, sb)], [node(a), node(b)])[-1]
            vals = [node(VN[r]).astype(bf16) for r in VORDER]
            for r, t in zip(VORDER, vals):
                s_v[r, rs, cs] = t
        kb, nb = s_v.shape[1:]
        out = []
        for r in range(0, kb, 16):
            out += [(slice(rr, rr + 8), slice(c, c + 256)) for c in range(0, nb - 255, 256) for rr in (r, r + 8)]
            out += [(slice(rr, rr + 8), slice(nb - 128, nb)) for rr in (r, r + 8)] if nb % 256 else []
        return [(functools.partial(piece, rs, cs), s_v, s_v if n % 16 == 15 else False, lag,
                 130 if cs.stop - cs.start == 256 else 100) for n, (rs, cs) in enumerate(out)]

    def prep_pieces(s_v, raw, lag, width=256):
        def piece(r, c, pin):
            idx = (slice(r, r + 8), slice(c, c + width))
            b11, b12, b21, b22 = [_unpack(pin(s_v[(q,) + idx], width) if n in (0, 3) else s_v[(q,) + idx])
                                  for n, q in enumerate(raw)]
            for k, t in ((0, b11 + b22), (2, b12 - b22), (3, b21 - b11), (5, b11 + b12), (6, b21 + b22)):
                s_v[(k,) + idx] = _pack(t)
        return [(functools.partial(piece, r, c), None, s_v, lag, 80)
                for c in range(0, s_v.shape[2], width) for r in range(0, s_v.shape[1], 8)]

    def store_l(slot, q, c, quads):
        for k, t in enumerate(_lcombos(*quads)):
            l_v[slot, k, q // 2:q // 2 + 8, c:c + t.shape[1]] = _pack(t)

    def ln_pieces(src, r0, slot, lag, width=256, staged=False, clag=None):
        def stats(q, pin):
            x = pin(src[pl.ds(r0 + q, 16), :].astype(f32))
            xs = [x[:, j * 128:(j + 1) * 128] for j in range(NT)]
            m = functools.reduce(lambda a, b: a + b, xs) * (1.0 / NT)
            w = functools.reduce(lambda a, b: a + b, [(t - m) * (t - m) for t in xs])
            mean = jnp.mean(m, axis=-1, keepdims=True)
            var = jnp.sum(w + NT * ((m - mean) * (m - mean)), axis=-1, keepdims=True) * (1.0 / D)
            n_v[0, q:q + 16, :] = jnp.broadcast_to(mean, (16, 128))
            n_v[1, q:q + 16, :] = jnp.broadcast_to(lax.rsqrt(var + EPS), (16, 128))

        def comb(q, c, pin):
            quads = []
            for rr in (0, HM):
                rs = pl.ds(pl.multiple_of(r0 + rr + q + zero_s[0], 16), 16)
                mean, rstd = [jnp.concatenate([n_v[t, rr + q:rr + q + 16, :]] * (width // 128), axis=1)
                              for t in range(2)]
                quads += [(src[rs, cc + c:cc + c + width].astype(f32) - mean) * rstd for cc in (0, DH2)]
            store_l(slot, q, c, quads)

        def comb26(q, pin):
            blocks = []
            for rr in (0, HM):
                rs = pl.ds(pl.multiple_of(r0 + rr + q + zero_s[0], 8), 8)
                mean, rstd = [jnp.concatenate([n_v[t, rr + q:rr + q + 8, :]] * 2, axis=1) for t in range(2)]
                blocks += [(src[rs, cc:cc + D4] - mean) * rstd for cc in range(0, D, D4)]
            vals = _run(UP, blocks)
            for k, u in enumerate(UL):
                lf_v[k, q:q + 8, :] = vals[u].astype(bf16)
        dense = slot is not None or src is b_v
        norms = [[(functools.partial(stats, rr + q), None, n_v if dense else False, lag, 90) for rr in (0, HM)]
                 for q in range(0, HM, 16)]
        if slot is None:
            combs = [[(functools.partial(comb26, qq), n_v, lf_v if dense or qq % 32 == 24 else False, clag, 110)
                      for qq in (q, q + 8)] for q in range(0, HM, 16)]
        else:
            combs = [[(functools.partial(comb, q, c), n_v, l_v, clag, 125) for c in range(0, DH2, width)]
                     for q in range(0, HM, 16)]
        if staged:
            return sum(norms, []), sum(combs, [])
        out = list(norms[0])
        for a, b in zip(norms[1:] + [[]], combs):
            out += _merge(a, b) if a else b
        return out

    shifts = (1, 1, -1, -1, 2, 2, -2, -2)

    def shift_pieces(r0, slot, lag, by_value=False):
        def piece(q, j, pin):
            a = [h_v[jj, pl.ds(PAD + r0 + rr + q - shifts[jj], 16), :]
                 for rr in (0, HM) for jj in (j, j + NT // 2)]
            store_l(slot, q, j * 128, [pin(a[0]), a[1], a[2], pin(a[3])])
        return [(functools.partial(piece, q, j), None if by_value else h_v,
                 l_v if (q // 16) % 2 and j == 3 else False, lag, 50)
                for q in range(0, HM, 16) for j in range(NT // 2)]

    def lhs_of(slot):
        return lambda k: l_v[slot, k]

    xe_v[0, 0:16, :] = jnp.zeros((16, D4), bf16)
    h_v[:, 0:PAD, :] = jnp.zeros((NT, PAD, 128), f32)
    h_v[:, PAD + S:PAD + S + PAD, :] = jnp.zeros((NT, PAD, 128), f32)

    def store_h(r0, c0, h):
        for j in range(h.shape[1] // 128):
            h_v[c0 // 128 + j, PAD + r0:PAD + r0 + h.shape[0], :] = h[:, j * 128:(j + 1) * 128]

    def h_pieces(r0, c0, t, lag, n=4):
        def piece(r, pin):
            store_h(r0 + r, c0, _gelu(pin(t[r:r + 8 * n])))
        return [(functools.partial(piece, r), None, h_v, lag, 10 * n) for r in range(0, t.shape[0], 8 * n)]

    def flush(pieces):
        for p in pieces:
            p[0](lambda v, w=128: v)

    def w1_cols(c, step):
        half, cc = c // DH2, c % DH2
        return jnp.concatenate([s1_v[RAW1[half], :, cc:cc + step], s1_v[RAW1[2 + half], :, cc:cc + step]], axis=0)

    def d1_plain(xn, r0, c0, c1, step):
        for c in range(c0, c1, step):
            store_h(r0, c, _gelu(mm(xn, w1_cols(c, step))))

    def d1_fine(lhs, r0, nrb, cols, pieces, carry, skip=0):
        tiles = [(rb, c) for c in cols for rb in range(nrb)]
        rounds = [tiles[i:i + 4] for i in range(0, len(tiles), 4)]
        for n, (rnd, part) in enumerate(zip(rounds, split(pieces, len(rounds)))):
            sk = skip if n == 0 else 0
            side = Side(_merge(carry, part) if carry else part, 8 - sk, sk)
            carry = []
            for rb, c in rnd:
                half, cc = c // DH2, c % DH2
                t = mm(lhs(rb, 0), s1_v[RAW1[half], :, cc:cc + 128], side)
                t = mm(lhs(rb, 1), s1_v[RAW1[2 + half], :, cc:cc + 128], side, t)
                carry += h_pieces(r0 + rb * HM, c, t, LS)
        return carry

    def d1_s(b, slot, pieces, carry, early=()):
        for c, part, e in zip(range(0, DH2, NC1), split(pieces, DH2 // NC1), split(early, 2) + [[], []]):
            side = Side(merge(carry, part, e), *((7,) if hist else (5, 2)))
            cs = strassen(lhs_of(slot), lambda k: s1_v[k, :, c:c + NC1], side)
            carry = sum([h_pieces(b * TM + (q // 2) * HM, (q % 2) * DH2 + c, cs[q], LS) for q in (1, 2, 3, 0)], [])
        return carry

    def d2_s(b, slot, pieces, carry=(), early=(), late=()):
        for c, part, e in zip(range(0, DH2, NC1), split(pieces, DH2 // NC1), split(early, 2) + split(late, 2)):
            side = Side(merge(carry, part, e), *((7,) if hist else (5, 2)))
            carry = ()
            idx = [(slice(b * TM + (q // 2) * HM, b * TM + (q // 2 + 1) * HM),
                    slice((q % 2) * DH2 + c, (q % 2) * DH2 + c + NC1)) for q in range(4)]
            cs = strassen(lhs_of(slot), lambda k: s2_v[k, :, c:c + NC1], side,
                          [x_v[i].astype(f32) for i in idx])
            for i, t in zip(idx, cs):
                b_v[i] = t
                if b == 0:
                    c0_v[i] = t

    def split(l, n):
        w = [1.0 if hist else 0.6] + [1.0] * (n - 1)
        cut = [int(round(len(l) * sum(w[:i]) / sum(w))) for i in range(n + 1)]
        return [l[cut[i]:cut[i + 1]] for i in range(n)]

    def merge(*ls):
        ls = [l for l in ls if l]
        return _merge(*ls) if ls else []

    NW1, NW3, N30 = 52, 32, 20
    LS, LL = 3, 5

    wait("x0")
    xn0 = _pack(_ln(x_v[0:TM, :].astype(f32)))
    wait("w1a")
    d1_plain(xn0, 0, 0, 256, 256)
    wait("w1b")
    d1_plain(xn0, 0, 256, 512, 256)
    wait("x1")
    xn1 = _pack(_ln(x_v[TM:2 * TM, :].astype(f32)))
    d1_plain(xn1, TM, 0, 512, 256)
    wait("w1cd")
    hist.clear()
    xn01 = jnp.concatenate([xn0, xn1], axis=0)
    l01 = lambda rb, kh: xn01[rb * 64:(rb + 1) * 64, kh * DH2:(kh + 1) * DH2]
    pw = prep_pieces(s1_v, RAW1, LS)
    flush(d1_fine(l01, 0, 4, (512, 640), pw[:NW1], [], 1))
    carry = []
    wait("x23")
    hist.clear()
    carry = d1_fine(l01, 0, 4, (768, 896), ln_pieces(x_v, 2 * TM, 0, LL), carry, 3)
    carry = d1_s(2, 0, ln_pieces(x_v, 3 * TM, 1, LL), carry, pw[NW1:])
    wait("x4567")
    qkv_start(0)
    qkv_start(1)
    hist.clear()
    for b in range(3, NB - 1):
        carry = d1_s(b, b % 2, ln_pieces(x_v, (b + 1) * TM, (b + 1) % 2, LL), carry)
    wait("w2")
    hist.clear()
    pw = prep_pieces(s2_v, RAW, LS)
    p3 = prep26_pieces(s3_v, LS)
    n3 = len(p3) * W3A // D4
    carry = d1_s(7, 1, _merge(pw[:NW3], shift_pieces(0, 0, LS, True)), carry)
    d2_s(0, 0, shift_pieces(TM, 1, LS, True), carry, pw[NW3:], p3[:N30])
    pw = split(_merge(p3[N30:n3], sum(ln_pieces(c0_v, 0, None, LL, clag=LS, staged=True), [])), 3)
    for b in range(1, 4):
        d2_s(b, b % 2, _merge(pw[b - 1], shift_pieces((b + 1) * TM, (b + 1) % 2, LS)))
    wait("w4", "small")
    hist.clear()
    pw = p3[n3:] + prep26_pieces(s4_v, LS)
    cut = (0, 33, 68, 103, len(pw))
    for b in range(4, NB):
        d2_s(b, b % 2, merge(pw[cut[b - 4]:cut[b - 3]],
                             shift_pieces((b + 1) * TM, (b + 1) % 2, LS) if b + 1 < NB else ()))
    start("wo", priority=1)

    def ffn(i, carry):
        qkv_wait(i)
        r0 = pl.multiple_of(i * TM, TM)
        rn = pl.multiple_of(jnp.minimum(i + 1, NB - 1) * TM, TM)
        acc = {}
        hist.clear()

        def relayout(p, r0_, r1_, pin):
            s0 = i * SPG + 2 * p
            e = wqkv_v[s0, r0_:r1_, :]
            o = wqkv_v[s0 + 1, r0_:r1_, :]
            wqkv_v[s0, r0_:r1_, :] = (e & jnp.uint32(0xFFFF)) | (o << 16)
            wqkv_v[s0 + 1, r0_:r1_, :] = (e >> 16) | (o & jnp.uint32(0xFFFF0000))

        relays = [(functools.partial(relayout, p, r, r + 32), wqkv_v, wqkv_v, 3, 35)
                  for p in range(SPG // 2) for r in range(0, D // 2, 32)]
        norms, combs = ln_pieces(b_v, rn, None, 5, staged=True, clag=3)

        def gate(q, pin):
            gw = gw_ref[...].astype(f32)
            x = pin(x_v[pl.ds(r0 + q, 16), :].astype(f32))
            t = functools.reduce(lambda a, b: a + b,
                                 [x[:, j * 128:(j + 1) * 128] * gw[j:j + 1, :] for j in range(NT)])
            g = jax.nn.sigmoid(jnp.sum(t, axis=-1, keepdims=True))
            g_v[pl.ds(r0 + q, 16), :] = jnp.broadcast_to(g, (16, 128))

        gates = [(functools.partial(gate, q), None, g_v, 5, 90) for q in range(0, TM, 16)]

        def extras(t, pin):
            jj, o = 2 * i + t // 2, 24 + 8 * (t % 2)
            xs = [pin(x_v[pl.ds(pl.multiple_of((jj + hh) * 64 + o, 8), 8), :].astype(f32)) for hh in (0, NPAIR // 2)]
            vals = _run(UP, [x[:, cc:cc + D4] for x in xs for cc in range(0, D, D4)])
            for k, u in enumerate(UL):
                xe_v[k, pl.ds(pl.multiple_of(i * 32 + t * 8, 8), 8), :] = vals[u].astype(bf16)

        xes = [(functools.partial(extras, t), None, xe_v, 3, 100) for t in range(4)]
        hs = {}

        def gelu_pieces(c, cs):
            def piece(r, cc, vs, pin):
                t = _gelu(pin(_cat([cs[v][r:r + 8, cc:cc + 128] for v in vs], 0)))
                ts = [t[8 * n:8 * n + 8] for n in range(len(vs))]
                hs.update({(c, v, r, cc): u for v, u in zip(vs, ts)})
                return functools.reduce(lambda a, b: a + b, ts)
            return [(functools.partial(piece, r, cc, vs), None, None, 3, 40) for r in range(0, HM, 8)
                    for cc in range(0, cs[0].shape[1], 128) for vs in ((0, 1, 2, 3), (4, 5, 6, 7))]

        def d3(c, side):
            c0, c1 = FCH[c]
            cs = fmm(lambda u: lf_v[UL.index(u)], lambda r: s3_v[r, :, c0:c1], side)
            assert not side.pieces
            return gelu_pieces(c, cs)

        def d4(c, side):
            c0, c1 = FCH[c]
            lh = _run(UP, [_cat([_cat([hs.pop((c, v, r, cc)) for r in range(0, HM, 8)], 0)
                                 for cc in range(0, c1 - c0, 128)], 1) for v in range(8)])
            rhs = lambda r: s4_v[r, c0:c1, :]
            if c + 1 < len(FCH):
                for n in WORDER:
                    for r in range(RK):
                        if WN[r] == n:
                            acc[n] = mm(lh[UN[r]], rhs(r), side, acc.get(n))
            else:
                idx = lambda v: (pl.ds(r0 + (v // 4) * HM, HM), slice((v % 4) * D4, (v % 4 + 1) * D4))

                def extra(n):
                    if n >= 8:
                        return acc.get(n)
                    return b_v[idx(n)] + acc[n] if n in acc else b_v[idx(n)]

                def emit_b(v, t):
                    b_v[idx(v)] = jnp.concatenate([1.0 - g_v[idx(v)[0], :]] * 2, axis=1) * t
                fmm(lambda u: lh[u], rhs, side, extra, emit_b)
            assert not side.pieces

        g0 = d3(0, Side(relays[:20], 23, 3))
        g1 = d3(1, Side(_merge(g0, gates, xes), 23, 2))
        d4(0, Side(g1[:22], 22, 4))
        g2 = d3(2, Side(_merge(g1[22:], relays[20:40]), 25))
        d4(1, Side(g2, 23, 2))
        g3 = d3(3, Side(_merge(relays[40:], norms), 26))
        d4(2, Side(_merge(g3, combs), 23, 2))
        d4(3, Side([], 1))

        @pl.when(i + 2 < NG)
        def _():
            qkv_start(i + 2)

        return carry

    lax.fori_loop(0, NB, ffn, 0)

    def pre(it, carry):
        hist.clear()
        for u in range(3 * NG // NPRE):
            s0 = (it * (3 * NG // NPRE) + u) * G

            def rhs(r):
                t = None
                sz = s0 + zero_s[r]
                for q, sg in sorted(_terms(VP, 16, VN[r]).items(), key=lambda e: -e[1]):
                    blk = wqkv_v[sz + q % 4, (q // 4) * (D // 8):(q // 4 + 1) * (D // 8), :]
                    if VN[r] < 16:
                        return blk
                    blk = _unpack(blk)
                    t = blk if t is None else (t + blk if sg > 0 else t - blk)
                return t.astype(bf16)
            for v, t in enumerate(fmm(lambda k: xe_v[UL.index(k)], rhs, None)):
                e_v[(v // 4) * 16:(v // 4 + 1) * 16, s0 + v % 4] = _pack(t).reshape(16, 8, DH)
        return carry

    lax.fori_loop(0, NPRE, pre, 0)

    wait("wo")
    mem_v[...] = mem0_ref[...].astype(f32)

    def slab(w, h):
        return (h // G) * SPG + w * G + h % G

    def step(j, hx, odd, late, allow, fill):
        qs, ks, vs, ps = {}, {}, {}, {}
        wload = lambda w, h: pltpu.bitcast(wqkv_v[slab(w, h)], bf16)
        eload = lambda w, h: pltpu.bitcast(e_v[j, slab(w, h)], bf16)

        def proj(g):
            part = {}
            if late and g == 0:
                for h in range(2):
                    for w in range(3):
                        part[w, h] = _dot(hx[:, :DH2], wload(w, h)[:DH2])
            for h in range(g * G, (g + 1) * G):
                q, k, v = [(_dot(hx[:, DH2:], wload(w, h)[DH2:]) + part[w, h] if (w, h) in part
                            else _dot(hx, wload(w, h))).astype(bf16) for w in range(3)]
                if odd:
                    q = jnp.concatenate([q, eload(0, h)], axis=0)
                    k = jnp.concatenate([pltpu.bitcast(ke_v[h], bf16), eload(1, h), k], axis=0)
                    v = jnp.concatenate([pltpu.bitcast(ve_v[h], bf16), eload(2, h), v], axis=0)
                else:
                    ke_v[h] = pltpu.bitcast(k, u32)
                    ve_v[h] = pltpu.bitcast(v, u32)
                    k = jnp.concatenate([k, eload(1, h)], axis=0)
                    v = jnp.concatenate([v, eload(2, h)], axis=0)
                qs[h], ks[h], vs[h] = q, k, v

        def score(g):
            for h in range(g * G, (g + 1) * G):
                s = lax.dot_general(qs.pop(h), ks.pop(h), (((1,), (1,)), ((), ())),
                                    preferred_element_type=f32)
                ps[h] = _softmax(s, allow, fill)

        def pv(g):
            os_ = []
            for h in range(g * G, (g + 1) * G):
                o = _dot(ps.pop(h), vs.pop(h))
                o_v[:, h * 128:(h + 1) * 128] = _pack(o[:32])
                os_.append(o)
            if odd:
                quads = [jnp.concatenate([os_[2 * kk][r:r + 8], os_[2 * kk + 1][r:r + 8]], axis=1)
                         for r in (32, 40) for kk in range(2)]
                for k, t in enumerate(_lcombos(*quads)):
                    oe_v[k, pl.ds(pl.multiple_of(j * 8, 8), 8), g * 256:(g + 1) * 256] = t.astype(bf16)

        acc = [None] * NT

        def wo(h0, h1, j0, j1):
            o = pltpu.bitcast(o_v[:, h0 * 128:h1 * 128], bf16)
            for n in range(j0, j1):
                y = _dot(o, pltpu.bitcast(wo_v[n, h0 * 64:h1 * 64, :], bf16))
                acc[n] = y if acc[n] is None else y + acc[n]

        for t in range(NG):
            proj(t)
            if t >= 2:
                pv(t - 2)
            if t >= 1:
                score(t - 1)
        wo(0, 16, 0, 4)
        pv(NG - 2)
        score(NG - 1)
        wo(0, 16, 4, 8)
        pv(NG - 1)
        wo(16, 24, 0, 8)
        wo(24, 32, 0, 8)
        return jnp.concatenate(acc, axis=1)

    def emit(j, r0, o0, a):
        rs = pl.ds(r0 + o0, 24)
        g = jnp.concatenate([g_v[rs, :]] * NT, axis=1)
        out_v[j, o0:o0 + 24, :] = (g * a + b_v[rs, :]).astype(bf16)

    def pair(j, mem, late):
        r0 = pl.multiple_of(j * 64, 64)
        allow_e, fill_e, allow_o, fill_o = _masks()
        xa = x_v[pl.ds(r0 + 16, 8), :].astype(f32)
        xb = x_v[pl.ds(r0 + 40, 8), :].astype(f32)
        hx = jnp.concatenate([x_v[pl.ds(r0, 16), :], jnp.concatenate([xa, mem], 0).astype(bf16)], 0)
        oe = step(j, hx, False, late, allow_e, fill_e)
        emit(j, r0, 0, oe[:24])
        hx = jnp.concatenate([jnp.concatenate([oe[24:32], xb], 0).astype(bf16), x_v[pl.ds(r0 + 48, 16), :]], 0)
        oo = step(j, hx, True, True, allow_o, fill_o)
        emit(j, r0, 40, oo[8:])
        return oo[:8]

    def a_iter(it, carry):
        mem = mem_v[...]
        for t in range(PPI):
            mem = pair(it * PPI + t, mem, t > 0)
        mem_v[...] = mem
        for t in range(PPI):
            for o0 in (0, 40):
                idx = (it * PPI + t, pl.ds(o0, 24))
                pltpu.make_async_copy(out_v.at[idx], out_hbm.at[idx], sem_out).start()
        return carry

    lax.fori_loop(0, NPAIR // PPI, a_iter, 0)

    hist.clear()
    for n in range(NT // 2):
        quad = [lambda k, t=2 * n + q % 2, o=(q // 2) * 128: jnp.concatenate(
            [wo_v[t + zero_s[k], g * 256 + o:g * 256 + o + 128, :] for g in range(NG)], axis=0) for q in range(4)]
        cs = strassen(lambda k: oe_v[k], lambda k: _rcombo(k, *quad), None)
        cols = slice(n * 256, (n + 1) * 256)
        for half in range(2):
            t = jnp.concatenate(cs[2 * half:2 * half + 2], axis=1)
            o0 = 24 + half * 8
            for jj in range(NPAIR):
                rs = slice(jj * 64 + o0, jj * 64 + o0 + 8)
                g = jnp.concatenate([g_v[rs, :]] * 2, axis=1)
                out_v[jj, o0:o0 + 8, cols] = (g * t[jj * 8:jj * 8 + 8] + b_v[rs, cols]).astype(bf16)
        if n >= 2:
            idx = (slice(None), pl.ds(24, 16), pl.ds(0, 768) if n == 2 else pl.ds(768, 256))
            pltpu.make_async_copy(out_v.at[idx], out_hbm.at[idx], sem_out).start()
    pltpu.make_async_copy(out_v, out_hbm, sem_out).wait()


@jax.jit
def pallas_gated_mix__memory_aug_recurrent_mem_tr__mixer_s_mlp__prompt_kernel(
    A_x, A_mem0, A_Wq, A_Wk, A_Wv, A_Wo, A_seg_len, B_x, B_w1, B_w2, B_w3, B_w4, gate_w,
):
    assert A_x.shape == (1, S, D) and A_mem0.shape == (1, M, D)
    any_spec = pl.BlockSpec(memory_space=pl.ANY)
    out = pl.pallas_call(
        _kernel,
        out_shape=jax.ShapeDtypeStruct((NPAIR, 64, D), bf16),
        in_specs=[any_spec] * 11,
        out_specs=any_spec,
        scratch_shapes=[
            pltpu.VMEM((S, D), bf16),
            pltpu.VMEM((9, D // 4, D // 2), u32),
            pltpu.VMEM((7, D // 4, D // 2), u32),
            pltpu.VMEM((RK, D4, F4), bf16),
            pltpu.VMEM((RK, F4, D4), bf16),
            pltpu.VMEM((3 * H, D // 2, DH), u32),
            pltpu.VMEM((NT, H * DH // 2, 128), u32),
            pltpu.VMEM((NT, S + 2 * PAD, 128), f32),
            pltpu.VMEM((S, D), f32),
            pltpu.VMEM((TM, D), f32),
            pltpu.VMEM((2, 7, HM // 2, D // 2), u32),
            pltpu.VMEM((len(UL), HM, D4), bf16),
            pltpu.VMEM((2, TM, 128), f32),
            pltpu.VMEM((S, 128), f32),
            pltpu.VMEM((NPAIR, 64, D), bf16),
            pltpu.VMEM((len(UL), 8 * NPAIR, D4), bf16),
            pltpu.VMEM((NPAIR, 3 * H, 8, DH), u32),
            pltpu.VMEM((7, 8 * NPAIR, H * DH // 2), bf16),
            pltpu.VMEM((H, 16, 128), u32),
            pltpu.VMEM((H, 16, 128), u32),
            pltpu.VMEM((16, H * DH), u32),
            pltpu.VMEM((M, D), f32),
            pltpu.VMEM((M, D), bf16),
            pltpu.VMEM((NT, 128), bf16),
            pltpu.SMEM((RK,), jnp.int32),
            pltpu.SemaphoreType.DMA((NLOAD,)),
            pltpu.SemaphoreType.DMA((NG,)),
            pltpu.SemaphoreType.DMA,
        ],
        compiler_params=pltpu.CompilerParams(vmem_limit_bytes=126 * 1024 * 1024,
                                             disable_bounds_checks=True),
    )(
        A_x.reshape(S, D), A_mem0.reshape(M, D),
        A_Wq.reshape(D // 2, 2 * H, DH), A_Wk.reshape(D // 2, 2 * H, DH), A_Wv.reshape(D // 2, 2 * H, DH),
        A_Wo.reshape(H * DH, D), B_w1, B_w2, B_w3, B_w4, gate_w.reshape(NT, 128),
    )
    return out.reshape(1, S, D)
```

```python
import functools

import jax
import jax.numpy as jnp
from jax import lax
import jax.experimental.pallas as pl
import jax.experimental.pallas.tpu as pltpu

f32, bf16, u32 = jnp.float32, jnp.bfloat16, jnp.uint32

S, D, H, DH, M, SEG, F = 2048, 1024, 32, 128, 8, 32, 3584
SCALE = DH ** -0.5
NEG = -1000000000.0
EPS = 1e-05

TM = 256
NB = S // TM
HM = TM // 2
DH2 = D // 2
D4, F4 = D // 4, F // 4
FCH = ((0, 128), (128, 384), (384, 640), (640, 896))
NC1 = 128
NPAIR = S // (2 * SEG)
PPI = 2
NPRE = 3
G = 4
NG = H // G
PAD = 8
NT = D // 128
W3A = 192
NLOAD = 11
assert NB == NG

_dot = functools.partial(jnp.dot, preferred_element_type=f32)

UP = ((4, 1, 5, 1), (6, 1, 8, 1), (0, 1, 3, 1), (2, -1, 9, 1), (4, -1, 10, 1), (0, 1, 1, 1), (2, 1, 12, 1),
      (5, 1, 7, -1), (7, 1, 12, -1), (11, -1, 13, 1), (10, -1, 11, 1), (2, 1, 7, 1), (0, -1, 4, 1),
      (6, 1, 7, 1), (1, -1, 5, 1), (3, 1, 7, -1), (1, 1, 4, 1), (2, 1, 3, 1), (1, -1, 3, 1), (1, 1, 7, -1),
      (2, 1, 6, -1))
WP = ((0, -1, 3, 1), (4, 1, 6, -1), (1, 1, 8, 1), (5, 1, 10, 1), (4, -1, 7, 1), (0, -1, 9, -1),
      (11, 1, 12, 1), (6, 1, 7, -1), (2, 1, 5, -1), (0, -1, 7, -1), (9, 1, 11, -1), (2, 1, 13, 1),
      (5, 1, 13, 1), (2, -1, 3, 1), (5, 1, 6, 1), (0, 1, 4, 1), (2, 1, 7, 1), (1, 1, 2, 1), (1, 1, 5, 1),
      (3, 1, 7, 1), (2, 1, 6, 1))
VP = ((1, 1, 5, -1), (8, 1, 11, 1), (10, 1, 17, 1), (13, 1, 16, -1), (0, 1, 4, -1), (0, 1, 3, 1),
      (14, 1, 18, -1), (0, 1, 11, 1), (14, 1, 19, -1), (0, 1, 5, 1), (12, 1, 15, 1), (2, 1, 21, 1),
      (10, 1, 14, -1), (4, 1, 7, 1), (11, 1, 19, 1), (12, -1, 20, 1), (13, 1, 14, -1), (9, 1, 30, -1),
      (3, -1, 15, 1), (6, 1, 23, 1), (24, 1, 27, -1), (9, -1, 18, 1), (7, 1, 34, 1), (2, 1, 6, -1),
      (0, 1, 8, -1), (6, 1, 21, 1), (22, 1, 31, -1), (6, 1, 29, 1), (0, 1, 1, 1), (15, 1, 25, 1),
      (5, 1, 37, 1), (15, 1, 20, 1))
UN = (7, 27, 24, 17, 9, 22, 21, 2, 15, 11, 8, 25, 19, 28, 2, 23, 26, 20, 1, 18, 10, 28, 4, 13, 14, 16)
WN = (23, 17, 24, 10, 14, 7, 22, 19, 12, 18, 15, 25, 20, 5, 26, 0, 8, 2, 27, 11, 26, 9, 28, 21, 16, 5)
VN = (42, 47, 41, 5, 11, 43, 18, 28, 20, 23, 35, 19, 22, 46, 33, 26, 45, 36, 38, 25, 44, 40, 39, 21, 24, 32)
RK = len(UN)
UL = tuple(sorted(set(UN)))
RAW16 = (1, 11, 17, 5, 8, 3, 9, 10, 0, 6, 7, 4, 12, 20, 22, 16)
VORDER = (0, 6, 7, 12, 13, 14, 15, 21, 11, 17, 20, 22, 24, 25, 23, 2, 1, 5, 8, 9, 10, 16, 18, 19)
assert sorted(VORDER) == [r for r in range(RK) if VN[r] >= 16] and len(set(RAW16)) == 16
assert all(RAW16[VN[r]] == r for r in range(RK) if VN[r] < 16)


def _run(prog, blocks):
    vals = list(blocks)
    for a, sa, b, sb in prog:
        vals.append(vals[a] + vals[b] if sa > 0 and sb > 0 else
                    vals[a] - vals[b] if sa > 0 else vals[b] - vals[a])
    return vals


def _terms(prog, nin, node):
    if node < nin:
        return {node: 1}
    a, sa, b, sb = prog[node - nin]
    out = {k: sa * v for k, v in _terms(prog, nin, a).items()}
    out.update({k: sb * v for k, v in _terms(prog, nin, b).items()})
    return out


def _scheme_is_exact():
    t = {}
    for r in range(RK):
        for a, ca in _terms(UP, 8, UN[r]).items():
            for b, cb in _terms(VP, 16, VN[r]).items():
                for c, cc in _terms(WP, 8, WN[r]).items():
                    t[a, b, c] = t.get((a, b, c), 0) + ca * cb * cc
    want = {(4 * i + j, 4 * j + l, 4 * i + l): 1 for i in range(2) for j in range(4) for l in range(4)}
    return {k: v for k, v in t.items() if v} == want


assert _scheme_is_exact()

_WPAR = {n: [] for n in range(8 + len(WP))}
for _t, (_a, _sa, _b, _sb) in enumerate(WP):
    _WPAR[_a].append((8 + _t, _sa))
    _WPAR[_b].append((8 + _t, _sb))


def _worder():
    order = []

    def closure(n, acc):
        if n not in acc and n not in order:
            acc.add(n)
            for q, _ in _WPAR[n]:
                closure(q, acc)
        return acc

    def visit(n):
        if n not in order:
            for q, _ in _WPAR[n]:
                visit(q)
            order.append(n)
    while len([v for v in range(8) if v not in order]):
        visit(min((v for v in range(8) if v not in order), key=lambda v: len(closure(v, set()))))
    return tuple(order)


WORDER = _worder()


def _ln(x):
    m = jnp.mean(x, axis=-1, keepdims=True)
    xc = x - m
    v = jnp.mean(xc * xc, axis=-1, keepdims=True)
    return xc * lax.rsqrt(v + EPS)


_GC = 0.7978845608028654


def _gelu(x):
    h = 0.5 * x
    return h + h * jnp.tanh(x * (_GC + (_GC * 0.044715) * (x * x)))


def _unpack(u):
    return pltpu.bitcast(u, bf16).astype(f32)


def _pack(x):
    return pltpu.bitcast(x.astype(bf16), u32)


def _cat(xs, axis):
    xs = [x for x in xs if x.shape[axis]]
    return xs[0] if len(xs) == 1 else jnp.concatenate(xs, axis=axis)


def _as(x, dtype):
    return x if x.dtype == dtype else pltpu.bitcast(x, dtype)


def _lcombos(a11, a12, a21, a22):
    return [a11 + a22, a21 + a22, a11, a22, a11 + a12, a21 - a11, a12 - a22]


def _merge(*lists):
    keyed = [((j + 0.5) / len(l), n, j, v) for n, l in enumerate(lists) for j, v in enumerate(l)]
    return [v for _, _, _, v in sorted(keyed, key=lambda t: t[:3])]


def _masks():
    r = lax.broadcasted_iota(jnp.int32, (32, 48), 0)
    c = lax.broadcasted_iota(jnp.int32, (32, 48), 1)
    exist_e = c < 40
    allow_e = exist_e & ((r >= 24) | ((c >= 24) & (c < 32)) | (c <= r))
    fill_e = jnp.where(exist_e, NEG, -jnp.inf).astype(f32)
    r = lax.broadcasted_iota(jnp.int32, (48, 80), 0)
    c = lax.broadcasted_iota(jnp.int32, (48, 80), 1)
    q_even = (r >= 32) & (r < 40)
    exist_o = (q_even & (c < 40)) | (~q_even & (c >= 40))
    ktok = jnp.where(c < 24, c, jnp.where(c < 48, c - 8, c - 16))
    qtok = jnp.where(r < 32, r + 32, r - 8)
    is_mem_key = ((c >= 24) & (c < 32)) | ((c >= 48) & (c < 56))
    allow_o = exist_o & (is_mem_key | (r < 8) | (ktok <= qtok))
    fill_o = jnp.where(exist_o, NEG, -jnp.inf).astype(f32)
    return allow_e, fill_e, allow_o, fill_o


def _rcombo(k, b11, b12, b21, b22):
    if k in (1, 4):
        return (b11 if k == 1 else b22)(k)
    a, b, sign = {0: (b11, b22, 1), 2: (b12, b22, -1), 3: (b21, b11, -1), 5: (b11, b12, 1), 6: (b21, b22, 1)}[k]
    a, b = _unpack(a(k)), _unpack(b(k))
    return (a + b if sign > 0 else a - b).astype(bf16)


def _softmax(s, allow, fill):
    s = jnp.where(allow, s * SCALE, fill)
    m = jnp.max(s, axis=-1, keepdims=True)
    e = jnp.exp(s - m)
    l = jnp.sum(e, axis=-1, keepdims=True)
    r = pl.reciprocal(l, approx=True)
    r = r * (2.0 - l * r)
    return (e * r).astype(bf16)


def _kernel(x_hbm, mem0_hbm, wq_hbm, wk_hbm, wv_hbm, wo_hbm, w1_hbm, w2_hbm, w3_hbm, w4_hbm,
            gw_hbm, out_hbm,
            x_v, s1_v, s2_v, s3_v, s4_v, wqkv_v, wo_v, h_v, b_v, c0_v, l_v, lf_v, n_v, g_v, out_v, xe_v, e_v, oe_v,
            ke_v, ve_v, o_v, mem_v, mem0_ref, gw_ref, zero_s,
            sem, sem_qkv, sem_out):
    RAW = (1, 2, 3, 4)
    RAW1 = (1, 7, 8, 4)

    loads = []

    def rows_load(name, r0, r1):
        loads.append((name, x_hbm.at[pl.ds(r0, r1 - r0)], x_v.at[pl.ds(r0, r1 - r0)]))

    def quad_load(name, w_hbm, s_v, raw, q, c0=0, c1=None):
        k4, n2 = s_v.shape[1], s_v.shape[2]
        c1 = n2 if c1 is None else c1
        src = w_hbm.bitcast(u32).at[pl.ds((q // 2) * k4, k4), pl.ds((q % 2) * n2 + c0, c1 - c0)]
        loads.append((name, src, s_v.at[raw[q], :, pl.ds(c0, c1 - c0)]))

    def w1_load(name, half, c0, c1):
        quad_load(name, w1_hbm, s1_v, RAW1, half, c0, c1)
        quad_load(name, w1_hbm, s1_v, RAW1, 2 + half, c0, c1)

    def block_load(name, w_hbm, s_v, r0, r1):
        kb, nb = s_v.shape[1:]
        for q in range(16):
            loads.append((name, w_hbm.at[pl.ds((q // 4) * kb + r0, r1 - r0), pl.ds((q % 4) * nb, nb)],
                          s_v.at[RAW16[q], pl.ds(r0, r1 - r0)]))

    rows_load("x0", 0, TM)
    w1_load("w1a", 0, 0, 256)
    w1_load("w1b", 0, 256, 512)
    rows_load("x1", TM, 2 * TM)
    w1_load("w1cd", 1, 0, 512)
    rows_load("x23", 2 * TM, 4 * TM)
    rows_load("x4567", 4 * TM, S)
    for q in range(4):
        quad_load("w2", w2_hbm, s2_v, RAW, q)
    block_load("w2", w3_hbm, s3_v, 0, W3A)
    block_load("w4", w3_hbm, s3_v, W3A, D4)
    block_load("w4", w4_hbm, s4_v, 0, F4)
    loads.append(("small", mem0_hbm, mem0_ref))
    loads.append(("small", gw_hbm, gw_ref))
    for j in range(NT):
        loads.append(("wo", wo_hbm.bitcast(u32).at[:, pl.ds(j * 128, 128)], wo_v.at[j]))
    groups = list(dict.fromkeys(name for name, _, _ in loads))
    assert len(groups) == NLOAD

    def start(*names, priority=0):
        for name, src, dst in loads:
            if name in names:
                pltpu.make_async_copy(src, dst, sem.at[groups.index(name)]).start(priority=priority)

    def wait(*names):
        for name, src, dst in loads:
            if name in names:
                pltpu.make_async_copy(src, dst, sem.at[groups.index(name)]).wait()

    SPG = 3 * G

    def qkv_start(g):
        for w, w_hbm in enumerate((wq_hbm, wk_hbm, wv_hbm)):
            wu = w_hbm.bitcast(u32)
            for k in range(G // 2):
                for par in range(2):
                    pltpu.make_async_copy(
                        wu.at[:, par * (H // 2) + g * (G // 2) + k, :],
                        wqkv_v.at[g * SPG + w * G + 2 * k + par], sem_qkv.at[g]).start(priority=1)

    def qkv_wait(g):
        grp = wqkv_v.at[pl.ds(g * SPG, SPG)]
        pltpu.make_async_copy(grp, grp, sem_qkv.at[g]).wait()

    start("x0", "w1a", "w1b", "x1", "w1cd", "x23", "x4567", "w2", "w4", "small")

    def zero(k, carry):
        zero_s[k] = 0
        return carry
    lax.fori_loop(0, RK, zero, 0)

    def tile_idx(ref, cols=128):
        z = zero_s[0]
        n = 16 if ref.dtype == bf16 and cols == 128 else 8
        return (z,) * (len(ref.shape) - 2) + (pl.ds(pl.multiple_of(z, n), n), slice(0, cols))

    hist = []

    def mm(lhs, rhs, side=None, acc=None):
        if side is not None:
            lhs = side(lhs)
        lhs = pltpu.bitcast(lhs, bf16) if lhs.dtype == u32 else lhs.astype(bf16)
        y = _dot(lhs, pltpu.bitcast(rhs, bf16) if rhs.dtype == u32 else rhs)
        if acc is not None:
            y = y + acc
        hist.append(y)
        return y

    class Side:
        def __init__(self, pieces, n, skip=0):
            cap = [0] * skip + [1] * n
            tot = sum(p[4] for p in pieces)
            self.plan = [[] for _ in cap]
            done = 0
            for p in pieces:
                done += p[4]
                x, d = done / tot * sum(cap), 0
                while x > cap[d] + 1e-9:
                    x -= cap[d]
                    d += 1
                self.plan[d].append((p, x / cap[d]))
            self.pieces = len(pieces)

        def __call__(self, val):
            todo = self.plan.pop(0) if self.plan else []
            if not todo:
                return val
            self.pieces -= len(todo)
            never = zero_s[0] > 0
            if val.dtype == bf16:
                val = pltpu.bitcast(val, u32)
            rg = 8 if val.dtype == u32 else 16
            ng = val.shape[0] // rg
            tied = {}
            for (fn, rd, wr, lag, _), pos in todo:
                m = min(max(-int(-pos * ng // 1) - 1, 0), ng - 1)
                pin = lambda v, w=128: v
                if lag is not None and len(hist) >= lag:
                    r0 = (16 * m) % hist[-lag].shape[0]
                    a = hist[-lag][r0:r0 + 8, :128]
                    if rd is None:
                        def pin(v, w=128, a=a):
                            a = _cat([_cat([_as(a, v.dtype)] * (v.shape[0] // 8), 0)] * (w // 128), 1)
                            if v.shape[1] == w:
                                return lax.select(never, a, v)
                            return _cat([lax.select(never, a, v[:, :w]), v[:, w:]], 1)
                    elif rd.dtype == bf16:
                        idx = tile_idx(rd, 256)
                        rd[idx] = lax.select(never, _cat([a, a], 1).astype(bf16), rd[idx])
                    else:
                        idx = tile_idx(rd)
                        rd[idx] = lax.select(never, _as(a, rd.dtype), rd[idx])
                u = fn(pin)
                if wr is False:
                    continue
                if wr is not None:
                    u = wr[tile_idx(wr)]
                t, n = tied.get(m * rg) or (val[m * rg:m * rg + 8, -128:], 0)
                tied[m * rg] = (lax.select(zero_s[n] > 0, _as(u, val.dtype), t), n + 1)
            if not tied:
                return val
            col, r = [], 0
            for r0 in sorted(tied):
                col += ([val[r:r0, -128:]] if r0 > r else []) + [tied[r0][0]]
                r = r0 + 8
            col += [val[r:, -128:]] if r < val.shape[0] else []
            return _cat([val[:, :-128], _cat(col, 0)], 1) if val.shape[1] > 128 else _cat(col, 0)

    def strassen(lhs, rhs, side, init=(None, None, None, None)):
        def add(a, b):
            return a if b is None else a + b
        p = [mm(lhs(k), rhs(k), side) for k in range(5)]
        c12 = add(p[2] + p[4], init[1])
        c21 = add(p[1] + p[3], init[2])
        c22 = mm(lhs(5), rhs(5), side, add(p[0] - p[1] + p[2], init[3]))
        c11 = mm(lhs(6), rhs(6), side, add(p[0] + p[3] - p[4], init[0]))
        return c11, c12, c21, c22

    def fmm(lhs, rhs, side, extra=lambda n: None, emit=None):
        val = {}
        for n in WORDER:
            t = extra(n)
            for q, sg in sorted(_WPAR[n], key=lambda e: -e[1]):
                t = val[q] if t is None else (t + val[q] if sg > 0 else t - val[q])
            for r in range(RK):
                if WN[r] == n:
                    t = mm(lhs(UN[r]), rhs(r), side, t)
            val[n] = t
            if n < 8 and emit is not None:
                emit(n, t)
        return [val[v] for v in range(8)]

    def prep26_pieces(s_v, lag):
        def piece(rs, cs, pin):
            @functools.lru_cache(None)
            def node(n):
                if n < 16:
                    return s_v[RAW16[n], rs, cs].astype(f32)
                a, sa, b, sb = VP[n - 16]
                return _run([(0, sa, 1, sb)], [node(a), node(b)])[-1]
            vals = [node(VN[r]).astype(bf16) for r in VORDER]
            for r, t in zip(VORDER, vals):
                s_v[r, rs, cs] = t
        kb, nb = s_v.shape[1:]
        out = []
        for r in range(0, kb, 16):
            out += [(slice(rr, rr + 8), slice(c, c + 256)) for c in range(0, nb - 255, 256) for rr in (r, r + 8)]
            out += [(slice(rr, rr + 8), slice(nb - 128, nb)) for rr in (r, r + 8)] if nb % 256 else []
        return [(functools.partial(piece, rs, cs), s_v, s_v if n % 16 == 15 else False, lag,
                 130 if cs.stop - cs.start == 256 else 100) for n, (rs, cs) in enumerate(out)]

    def prep_pieces(s_v, raw, lag, width=256):
        def piece(r, c, pin):
            idx = (slice(r, r + 8), slice(c, c + width))
            b11, b12, b21, b22 = [_unpack(pin(s_v[(q,) + idx], width) if n in (0, 3) else s_v[(q,) + idx])
                                  for n, q in enumerate(raw)]
            for k, t in ((0, b11 + b22), (2, b12 - b22), (3, b21 - b11), (5, b11 + b12), (6, b21 + b22)):
                s_v[(k,) + idx] = _pack(t)
        return [(functools.partial(piece, r, c), None, s_v, lag, 80)
                for c in range(0, s_v.shape[2], width) for r in range(0, s_v.shape[1], 8)]

    def store_l(slot, q, c, quads):
        for k, t in enumerate(_lcombos(*quads)):
            l_v[slot, k, q // 2:q // 2 + 8, c:c + t.shape[1]] = _pack(t)

    def ln_pieces(src, r0, slot, lag, width=256, staged=False, clag=None):
        def stats(q, pin):
            x = pin(src[pl.ds(r0 + q, 16), :].astype(f32))
            xs = [x[:, j * 128:(j + 1) * 128] for j in range(NT)]
            m = functools.reduce(lambda a, b: a + b, xs) * (1.0 / NT)
            w = functools.reduce(lambda a, b: a + b, [(t - m) * (t - m) for t in xs])
            mean = jnp.mean(m, axis=-1, keepdims=True)
            var = jnp.sum(w + NT * ((m - mean) * (m - mean)), axis=-1, keepdims=True) * (1.0 / D)
            n_v[0, q:q + 16, :] = jnp.broadcast_to(mean, (16, 128))
            n_v[1, q:q + 16, :] = jnp.broadcast_to(lax.rsqrt(var + EPS), (16, 128))

        def comb(q, c, pin):
            quads = []
            for rr in (0, HM):
                rs = pl.ds(pl.multiple_of(r0 + rr + q + zero_s[0], 16), 16)
                mean, rstd = [jnp.concatenate([n_v[t, rr + q:rr + q + 16, :]] * (width // 128), axis=1)
                              for t in range(2)]
                quads += [(src[rs, cc + c:cc + c + width].astype(f32) - mean) * rstd for cc in (0, DH2)]
            store_l(slot, q, c, quads)

        def comb26(q, pin):
            blocks = []
            for rr in (0, HM):
                rs = pl.ds(pl.multiple_of(r0 + rr + q + zero_s[0], 8), 8)
                mean, rstd = [jnp.concatenate([n_v[t, rr + q:rr + q + 8, :]] * 2, axis=1) for t in range(2)]
                blocks += [(src[rs, cc:cc + D4] - mean) * rstd for cc in range(0, D, D4)]
            vals = _run(UP, blocks)
            for k, u in enumerate(UL):
                lf_v[k, q:q + 8, :] = vals[u].astype(bf16)
        dense = slot is not None or src is b_v
        norms = [[(functools.partial(stats, rr + q), None, n_v if dense else False, lag, 90) for rr in (0, HM)]
                 for q in range(0, HM, 16)]
        if slot is None:
            combs = [[(functools.partial(comb26, qq), n_v, lf_v if dense or qq % 32 == 24 else False, clag, 110)
                      for qq in (q, q + 8)] for q in range(0, HM, 16)]
        else:
            combs = [[(functools.partial(comb, q, c), n_v, l_v, clag, 125) for c in range(0, DH2, width)]
                     for q in range(0, HM, 16)]
        if staged:
            return sum(norms, []), sum(combs, [])
        out = list(norms[0])
        for a, b in zip(norms[1:] + [[]], combs):
            out += _merge(a, b) if a else b
        return out

    shifts = (1, 1, -1, -1, 2, 2, -2, -2)

    def shift_pieces(r0, slot, lag, by_value=False):
        def piece(q, j, pin):
            a = [h_v[jj, pl.ds(PAD + r0 + rr + q - shifts[jj], 16), :]
                 for rr in (0, HM) for jj in (j, j + NT // 2)]
            store_l(slot, q, j * 128, [pin(a[0]), a[1], a[2], pin(a[3])])
        return [(functools.partial(piece, q, j), None if by_value else h_v,
                 l_v if (q // 16) % 2 and j == 3 else False, lag, 50)
                for q in range(0, HM, 16) for j in range(NT // 2)]

    def lhs_of(slot):
        return lambda k: l_v[slot, k]

    xe_v[0, 0:16, :] = jnp.zeros((16, D4), bf16)
    h_v[:, 0:PAD, :] = jnp.zeros((NT, PAD, 128), f32)
    h_v[:, PAD + S:PAD + S + PAD, :] = jnp.zeros((NT, PAD, 128), f32)

    def store_h(r0, c0, h):
        for j in range(h.shape[1] // 128):
            h_v[c0 // 128 + j, PAD + r0:PAD + r0 + h.shape[0], :] = h[:, j * 128:(j + 1) * 128]

    def h_pieces(r0, c0, t, lag, n=4):
        def piece(r, pin):
            store_h(r0 + r, c0, _gelu(pin(t[r:r + 8 * n])))
        return [(functools.partial(piece, r), None, h_v, lag, 10 * n) for r in range(0, t.shape[0], 8 * n)]

    def flush(pieces):
        for p in pieces:
            p[0](lambda v, w=128: v)

    def w1_cols(c, step):
        half, cc = c // DH2, c % DH2
        return jnp.concatenate([s1_v[RAW1[half], :, cc:cc + step], s1_v[RAW1[2 + half], :, cc:cc + step]], axis=0)

    def d1_plain(xn, r0, c0, c1, step):
        for c in range(c0, c1, step):
            store_h(r0, c, _gelu(mm(xn, w1_cols(c, step))))

    def d1_fine(lhs, r0, nrb, cols, pieces, carry, skip=0):
        tiles = [(rb, c) for c in cols for rb in range(nrb)]
        rounds = [tiles[i:i + 4] for i in range(0, len(tiles), 4)]
        for n, (rnd, part) in enumerate(zip(rounds, split(pieces, len(rounds)))):
            sk = skip if n == 0 else 0
            side = Side(_merge(carry, part) if carry else part, 8 - sk, sk)
            carry = []
            for rb, c in rnd:
                half, cc = c // DH2, c % DH2
                t = mm(lhs(rb, 0), s1_v[RAW1[half], :, cc:cc + 128], side)
                t = mm(lhs(rb, 1), s1_v[RAW1[2 + half], :, cc:cc + 128], side, t)
                carry += h_pieces(r0 + rb * HM, c, t, LS)
        return carry

    def d1_s(b, slot, pieces, carry, early=()):
        for c, part, e in zip(range(0, DH2, NC1), split(pieces, DH2 // NC1), split(early, 2) + [[], []]):
            side = Side(merge(carry, part, e), *((7,) if hist else (5, 2)))
            cs = strassen(lhs_of(slot), lambda k: s1_v[k, :, c:c + NC1], side)
            carry = sum([h_pieces(b * TM + (q // 2) * HM, (q % 2) * DH2 + c, cs[q], LS) for q in (1, 2, 3, 0)], [])
        return carry

    def d2_s(b, slot, pieces, carry=(), early=(), late=()):
        for c, part, e in zip(range(0, DH2, NC1), split(pieces, DH2 // NC1), split(early, 2) + split(late, 2)):
            side = Side(merge(carry, part, e), *((7,) if hist else (5, 2)))
            carry = ()
            idx = [(slice(b * TM + (q // 2) * HM, b * TM + (q // 2 + 1) * HM),
                    slice((q % 2) * DH2 + c, (q % 2) * DH2 + c + NC1)) for q in range(4)]
            cs = strassen(lhs_of(slot), lambda k: s2_v[k, :, c:c + NC1], side,
                          [x_v[i].astype(f32) for i in idx])
            for i, t in zip(idx, cs):
                b_v[i] = t
                if b == 0:
                    c0_v[i] = t

    def split(l, n):
        w = [1.0 if hist else 0.6] + [1.0] * (n - 1)
        cut = [int(round(len(l) * sum(w[:i]) / sum(w))) for i in range(n + 1)]
        return [l[cut[i]:cut[i + 1]] for i in range(n)]

    def merge(*ls):
        ls = [l for l in ls if l]
        return _merge(*ls) if ls else []

    NW1, NW3, N30 = 52, 32, 20
    LS, LL = 3, 5

    wait("x0")
    xn0 = _pack(_ln(x_v[0:TM, :].astype(f32)))
    wait("w1a")
    d1_plain(xn0, 0, 0, 256, 256)
    wait("w1b")
    d1_plain(xn0, 0, 256, 512, 256)
    wait("x1")
    xn1 = _pack(_ln(x_v[TM:2 * TM, :].astype(f32)))
    d1_plain(xn1, TM, 0, 512, 256)
    wait("w1cd")
    hist.clear()
    xn01 = jnp.concatenate([xn0, xn1], axis=0)
    l01 = lambda rb, kh: xn01[rb * 64:(rb + 1) * 64, kh * DH2:(kh + 1) * DH2]
    pw = prep_pieces(s1_v, RAW1, LS)
    flush(d1_fine(l01, 0, 4, (512, 640), pw[:NW1], [], 1))
    carry = []
    wait("x23")
    hist.clear()
    carry = d1_fine(l01, 0, 4, (768, 896), ln_pieces(x_v, 2 * TM, 0, LL), carry, 3)
    carry = d1_s(2, 0, ln_pieces(x_v, 3 * TM, 1, LL), carry, pw[NW1:])
    wait("x4567")
    qkv_start(0)
    qkv_start(1)
    hist.clear()
    for b in range(3, NB - 1):
        carry = d1_s(b, b % 2, ln_pieces(x_v, (b + 1) * TM, (b + 1) % 2, LL), carry)
    wait("w2")
    hist.clear()
    pw = prep_pieces(s2_v, RAW, LS)
    p3 = prep26_pieces(s3_v, LS)
    n3 = len(p3) * W3A // D4
    carry = d1_s(7, 1, _merge(pw[:NW3], shift_pieces(0, 0, LS, True)), carry)
    d2_s(0, 0, shift_pieces(TM, 1, LS, True), carry, pw[NW3:], p3[:N30])
    pw = split(_merge(p3[N30:n3], sum(ln_pieces(c0_v, 0, None, LL, clag=LS, staged=True), [])), 3)
    for b in range(1, 4):
        d2_s(b, b % 2, _merge(pw[b - 1], shift_pieces((b + 1) * TM, (b + 1) % 2, LS)))
    wait("w4", "small")
    hist.clear()
    pw = p3[n3:] + prep26_pieces(s4_v, LS)
    cut = (0, 33, 68, 103, len(pw))
    for b in range(4, NB):
        d2_s(b, b % 2, merge(pw[cut[b - 4]:cut[b - 3]],
                             shift_pieces((b + 1) * TM, (b + 1) % 2, LS) if b + 1 < NB else ()))
    start("wo", priority=1)

    def ffn(i, carry):
        qkv_wait(i)
        r0 = pl.multiple_of(i * TM, TM)
        rn = pl.multiple_of(jnp.minimum(i + 1, NB - 1) * TM, TM)
        acc = {}
        hist.clear()

        def relayout(p, r0_, r1_, pin):
            s0 = i * SPG + 2 * p
            e = wqkv_v[s0, r0_:r1_, :]
            o = wqkv_v[s0 + 1, r0_:r1_, :]
            wqkv_v[s0, r0_:r1_, :] = (e & jnp.uint32(0xFFFF)) | (o << 16)
            wqkv_v[s0 + 1, r0_:r1_, :] = (e >> 16) | (o & jnp.uint32(0xFFFF0000))

        relays = [(functools.partial(relayout, p, r, r + 32), wqkv_v, wqkv_v, 3, 35)
                  for p in range(SPG // 2) for r in range(0, D // 2, 32)]
        norms, combs = ln_pieces(b_v, rn, None, 5, staged=True, clag=3)

        def gate(q, pin):
            gw = gw_ref[...].astype(f32)
            x = pin(x_v[pl.ds(r0 + q, 16), :].astype(f32))
            t = functools.reduce(lambda a, b: a + b,
                                 [x[:, j * 128:(j + 1) * 128] * gw[j:j + 1, :] for j in range(NT)])
            g = jax.nn.sigmoid(jnp.sum(t, axis=-1, keepdims=True))
            g_v[pl.ds(r0 + q, 16), :] = jnp.broadcast_to(g, (16, 128))

        gates = [(functools.partial(gate, q), None, g_v, 5, 90) for q in range(0, TM, 16)]

        def extras(t, pin):
            jj, o = 2 * i + t // 2, 24 + 8 * (t % 2)
            xs = [pin(x_v[pl.ds(pl.multiple_of((jj + hh) * 64 + o, 8), 8), :].astype(f32)) for hh in (0, NPAIR // 2)]
            vals = _run(UP, [x[:, cc:cc + D4] for x in xs for cc in range(0, D, D4)])
            for k, u in enumerate(UL):
                xe_v[k, pl.ds(pl.multiple_of(i * 32 + t * 8, 8), 8), :] = vals[u].astype(bf16)

        xes = [(functools.partial(extras, t), None, xe_v, 3, 100) for t in range(4)]
        hs = {}

        def gelu_pieces(c, cs):
            def piece(r, cc, vs, pin):
                t = _gelu(pin(_cat([cs[v][r:r + 8, cc:cc + 128] for v in vs], 0)))
                ts = [t[8 * n:8 * n + 8] for n in range(len(vs))]
                hs.update({(c, v, r, cc): u for v, u in zip(vs, ts)})
                return functools.reduce(lambda a, b: a + b, ts)
            return [(functools.partial(piece, r, cc, vs), None, None, 3, 40) for r in range(0, HM, 8)
                    for cc in range(0, cs[0].shape[1], 128) for vs in ((0, 1, 2, 3), (4, 5, 6, 7))]

        def d3(c, side):
            c0, c1 = FCH[c]
            cs = fmm(lambda u: lf_v[UL.index(u)], lambda r: s3_v[r, :, c0:c1], side)
            assert not side.pieces
            return gelu_pieces(c, cs)

        def d4(c, side):
            c0, c1 = FCH[c]
            lh = _run(UP, [_cat([_cat([hs.pop((c, v, r, cc)) for r in range(0, HM, 8)], 0)
                                 for cc in range(0, c1 - c0, 128)], 1) for v in range(8)])
            rhs = lambda r: s4_v[r, c0:c1, :]
            if c + 1 < len(FCH):
                for n in WORDER:
                    for r in range(RK):
                        if WN[r] == n:
                            acc[n] = mm(lh[UN[r]], rhs(r), side, acc.get(n))
            else:
                idx = lambda v: (pl.ds(r0 + (v // 4) * HM, HM), slice((v % 4) * D4, (v % 4 + 1) * D4))

                def extra(n):
                    if n >= 8:
                        return acc.get(n)
                    return b_v[idx(n)] + acc[n] if n in acc else b_v[idx(n)]

                def emit_b(v, t):
                    b_v[idx(v)] = jnp.concatenate([1.0 - g_v[idx(v)[0], :]] * 2, axis=1) * t
                fmm(lambda u: lh[u], rhs, side, extra, emit_b)
            assert not side.pieces

        g0 = d3(0, Side(relays[:20], 23, 3))
        g1 = d3(1, Side(_merge(g0, gates, xes), 23, 2))
        d4(0, Side(g1[:22], 22, 4))
        g2 = d3(2, Side(_merge(g1[22:], relays[20:40]), 25))
        d4(1, Side(g2, 23, 2))
        g3 = d3(3, Side(_merge(relays[40:], norms), 26))
        d4(2, Side(_merge(g3, combs), 23, 2))
        d4(3, Side([], 1))

        @pl.when(i + 2 < NG)
        def _():
            qkv_start(i + 2)

        return carry

    lax.fori_loop(0, NB, ffn, 0)

    def pre(it, carry):
        hist.clear()
        for u in range(3 * NG // NPRE):
            s0 = (it * (3 * NG // NPRE) + u) * G

            def rhs(r):
                t = None
                sz = s0 + zero_s[r]
                for q, sg in sorted(_terms(VP, 16, VN[r]).items(), key=lambda e: -e[1]):
                    blk = wqkv_v[sz + q % 4, (q // 4) * (D // 8):(q // 4 + 1) * (D // 8), :]
                    if VN[r] < 16:
                        return blk
                    blk = _unpack(blk)
                    t = blk if t is None else (t + blk if sg > 0 else t - blk)
                return t.astype(bf16)
            for v, t in enumerate(fmm(lambda k: xe_v[UL.index(k)], rhs, None)):
                e_v[(v // 4) * 16:(v // 4 + 1) * 16, s0 + v % 4] = _pack(t).reshape(16, 8, DH)
        return carry

    lax.fori_loop(0, NPRE, pre, 0)

    wait("wo")
    mem_v[...] = mem0_ref[...].astype(f32)

    def slab(w, h):
        return (h // G) * SPG + w * G + h % G

    def step(j, hx, odd, late, allow, fill):
        qs, ks, vs, ps = {}, {}, {}, {}
        wload = lambda w, h: pltpu.bitcast(wqkv_v[slab(w, h)], bf16)
        eload = lambda w, h: pltpu.bitcast(e_v[j, slab(w, h)], bf16)

        def proj(g):
            part = {}
            if late and g == 0:
                for h in range(2):
                    for w in range(3):
                        part[w, h] = _dot(hx[:, :DH2], wload(w, h)[:DH2])
            for h in range(g * G, (g + 1) * G):
                q, k, v = [(_dot(hx[:, DH2:], wload(w, h)[DH2:]) + part[w, h] if (w, h) in part
                            else _dot(hx, wload(w, h))).astype(bf16) for w in range(3)]
                if odd:
                    q = jnp.concatenate([q, eload(0, h)], axis=0)
                    k = jnp.concatenate([pltpu.bitcast(ke_v[h], bf16), eload(1, h), k], axis=0)
                    v = jnp.concatenate([pltpu.bitcast(ve_v[h], bf16), eload(2, h), v], axis=0)
                else:
                    ke_v[h] = pltpu.bitcast(k, u32)
                    ve_v[h] = pltpu.bitcast(v, u32)
                    k = jnp.concatenate([k, eload(1, h)], axis=0)
                    v = jnp.concatenate([v, eload(2, h)], axis=0)
                qs[h], ks[h], vs[h] = q, k, v

        def score(g):
            for h in range(g * G, (g + 1) * G):
                s = lax.dot_general(qs.pop(h), ks.pop(h), (((1,), (1,)), ((), ())),
                                    preferred_element_type=f32)
                ps[h] = _softmax(s, allow, fill)

        def pv(g):
            os_ = []
            for h in range(g * G, (g + 1) * G):
                o = _dot(ps.pop(h), vs.pop(h))
                o_v[:, h * 128:(h + 1) * 128] = _pack(o[:32])
                os_.append(o)
            if odd:
                quads = [jnp.concatenate([os_[2 * kk][r:r + 8], os_[2 * kk + 1][r:r + 8]], axis=1)
                         for r in (32, 40) for kk in range(2)]
                for k, t in enumerate(_lcombos(*quads)):
                    oe_v[k, pl.ds(pl.multiple_of(j * 8, 8), 8), g * 256:(g + 1) * 256] = t.astype(bf16)

        acc = [None] * NT

        def wo(h0, h1, j0, j1):
            o = pltpu.bitcast(o_v[:, h0 * 128:h1 * 128], bf16)
            for n in range(j0, j1):
                y = _dot(o, pltpu.bitcast(wo_v[n, h0 * 64:h1 * 64, :], bf16))
                acc[n] = y if acc[n] is None else y + acc[n]

        for t in range(NG):
            proj(t)
            if t >= 2:
                pv(t - 2)
            if t >= 1:
                score(t - 1)
        wo(0, 16, 0, 4)
        pv(NG - 2)
        score(NG - 1)
        wo(0, 16, 4, 8)
        pv(NG - 1)
        wo(16, 24, 0, 8)
        wo(24, 32, 0, 8)
        return jnp.concatenate(acc, axis=1)

    def emit(j, r0, o0, a):
        rs = pl.ds(r0 + o0, 24)
        g = jnp.concatenate([g_v[rs, :]] * NT, axis=1)
        out_v[j, o0:o0 + 24, :] = (g * a + b_v[rs, :]).astype(bf16)

    def pair(j, mem, late):
        r0 = pl.multiple_of(j * 64, 64)
        allow_e, fill_e, allow_o, fill_o = _masks()
        xa = x_v[pl.ds(r0 + 16, 8), :].astype(f32)
        xb = x_v[pl.ds(r0 + 40, 8), :].astype(f32)
        hx = jnp.concatenate([x_v[pl.ds(r0, 16), :], jnp.concatenate([xa, mem], 0).astype(bf16)], 0)
        oe = step(j, hx, False, late, allow_e, fill_e)
        emit(j, r0, 0, oe[:24])
        hx = jnp.concatenate([jnp.concatenate([oe[24:32], xb], 0).astype(bf16), x_v[pl.ds(r0 + 48, 16), :]], 0)
        oo = step(j, hx, True, True, allow_o, fill_o)
        emit(j, r0, 40, oo[8:])
        return oo[:8]

    def a_iter(it, carry):
        mem = mem_v[...]
        for t in range(PPI):
            mem = pair(it * PPI + t, mem, t > 0)
        mem_v[...] = mem
        for t in range(PPI):
            for o0 in (0, 40):
                idx = (it * PPI + t, pl.ds(o0, 24))
                pltpu.make_async_copy(out_v.at[idx], out_hbm.at[idx], sem_out).start()
        return carry

    lax.fori_loop(0, NPAIR // PPI, a_iter, 0)

    hist.clear()
    for n in range(NT // 2):
        quad = [lambda k, t=2 * n + q % 2, o=(q // 2) * 128: jnp.concatenate(
            [wo_v[t + zero_s[k], g * 256 + o:g * 256 + o + 128, :] for g in range(NG)], axis=0) for q in range(4)]
        cs = strassen(lambda k: oe_v[k], lambda k: _rcombo(k, *quad), None)
        cols = slice(n * 256, (n + 1) * 256)
        for half in range(2):
            t = jnp.concatenate(cs[2 * half:2 * half + 2], axis=1)
            o0 = 24 + half * 8
            for jj in range(NPAIR):
                rs = slice(jj * 64 + o0, jj * 64 + o0 + 8)
                g = jnp.concatenate([g_v[rs, :]] * 2, axis=1)
                out_v[jj, o0:o0 + 8, cols] = (g * t[jj * 8:jj * 8 + 8] + b_v[rs, cols]).astype(bf16)
        if n >= 2:
            idx = (slice(None), pl.ds(24, 16), pl.ds(0, 768) if n == 2 else pl.ds(768, 256))
            pltpu.make_async_copy(out_v.at[idx], out_hbm.at[idx], sem_out).start()
    pltpu.make_async_copy(out_v, out_hbm, sem_out).wait()


@jax.jit
def pallas_gated_mix__memory_aug_recurrent_mem_tr__mixer_s_mlp__prompt_kernel(
    A_x, A_mem0, A_Wq, A_Wk, A_Wv, A_Wo, A_seg_len, B_x, B_w1, B_w2, B_w3, B_w4, gate_w,
):
    assert A_x.shape == (1, S, D) and A_mem0.shape == (1, M, D)
    any_spec = pl.BlockSpec(memory_space=pl.ANY)
    out = pl.pallas_call(
        _kernel,
        out_shape=jax.ShapeDtypeStruct((NPAIR, 64, D), bf16),
        in_specs=[any_spec] * 11,
        out_specs=any_spec,
        scratch_shapes=[
            pltpu.VMEM((S, D), bf16),
            pltpu.VMEM((9, D // 4, D // 2), u32),
            pltpu.VMEM((7, D // 4, D // 2), u32),
            pltpu.VMEM((RK, D4, F4), bf16),
            pltpu.VMEM((RK, F4, D4), bf16),
            pltpu.VMEM((3 * H, D // 2, DH), u32),
            pltpu.VMEM((NT, H * DH // 2, 128), u32),
            pltpu.VMEM((NT, S + 2 * PAD, 128), f32),
            pltpu.VMEM((S, D), f32),
            pltpu.VMEM((TM, D), f32),
            pltpu.VMEM((2, 7, HM // 2, D // 2), u32),
            pltpu.VMEM((len(UL), HM, D4), bf16),
            pltpu.VMEM((2, TM, 128), f32),
            pltpu.VMEM((S, 128), f32),
            pltpu.VMEM((NPAIR, 64, D), bf16),
            pltpu.VMEM((len(UL), 8 * NPAIR, D4), bf16),
            pltpu.VMEM((NPAIR, 3 * H, 8, DH), u32),
            pltpu.VMEM((7, 8 * NPAIR, H * DH // 2), bf16),
            pltpu.VMEM((H, 16, 128), u32),
            pltpu.VMEM((H, 16, 128), u32),
            pltpu.VMEM((16, H * DH), u32),
            pltpu.VMEM((M, D), f32),
            pltpu.VMEM((M, D), bf16),
            pltpu.VMEM((NT, 128), bf16),
            pltpu.SMEM((RK,), jnp.int32),
            pltpu.SemaphoreType.DMA((NLOAD,)),
            pltpu.SemaphoreType.DMA((NG,)),
            pltpu.SemaphoreType.DMA,
        ],
        compiler_params=pltpu.CompilerParams(vmem_limit_bytes=126 * 1024 * 1024,
                                             disable_bounds_checks=True),
    )(
        A_x.reshape(S, D), A_mem0.reshape(M, D),
        A_Wq.reshape(D // 2, 2 * H, DH), A_Wk.reshape(D // 2, 2 * H, DH), A_Wv.reshape(D // 2, 2 * H, DH),
        A_Wo.reshape(H * DH, D), B_w1, B_w2, B_w3, B_w4, gate_w.reshape(NT, 128),
    )
    return out.reshape(1, S, D)
```

```python
import functools

import jax
import jax.numpy as jnp
from jax import lax
import jax.experimental.pallas as pl
import jax.experimental.pallas.tpu as pltpu

f32, bf16, u32 = jnp.float32, jnp.bfloat16, jnp.uint32

S, D, H, DH, M, SEG, F = 2048, 1024, 32, 128, 8, 32, 3584
SCALE = DH ** -0.5
NEG = -1000000000.0
EPS = 1e-05

TM = 256
NB = S // TM
HM = TM // 2
DH2 = D // 2
D4, F4 = D // 4, F // 4
FCH = ((0, 128), (128, 384), (384, 640), (640, 896))
NC1 = 128
NPAIR = S // (2 * SEG)
PPI = 2
NPRE = 3
G = 4
NG = H // G
PAD = 8
NT = D // 128
W3A = 192
NLOAD = 11
assert NB == NG

_dot = functools.partial(jnp.dot, preferred_element_type=f32)

UP = ((4, 1, 5, 1), (6, 1, 8, 1), (0, 1, 3, 1), (2, -1, 9, 1), (4, -1, 10, 1), (0, 1, 1, 1), (2, 1, 12, 1),
      (5, 1, 7, -1), (7, 1, 12, -1), (11, -1, 13, 1), (10, -1, 11, 1), (2, 1, 7, 1), (0, -1, 4, 1),
      (6, 1, 7, 1), (1, -1, 5, 1), (3, 1, 7, -1), (1, 1, 4, 1), (2, 1, 3, 1), (1, -1, 3, 1), (1, 1, 7, -1),
      (2, 1, 6, -1))
WP = ((0, -1, 3, 1), (4, 1, 6, -1), (1, 1, 8, 1), (5, 1, 10, 1), (4, -1, 7, 1), (0, -1, 9, -1),
      (11, 1, 12, 1), (6, 1, 7, -1), (2, 1, 5, -1), (0, -1, 7, -1), (9, 1, 11, -1), (2, 1, 13, 1),
      (5, 1, 13, 1), (2, -1, 3, 1), (5, 1, 6, 1), (0, 1, 4, 1), (2, 1, 7, 1), (1, 1, 2, 1), (1, 1, 5, 1),
      (3, 1, 7, 1), (2, 1, 6, 1))
VP = ((1, 1, 5, -1), (8, 1, 11, 1), (10, 1, 17, 1), (13, 1, 16, -1), (0, 1, 4, -1), (0, 1, 3, 1),
      (14, 1, 18, -1), (0, 1, 11, 1), (14, 1, 19, -1), (0, 1, 5, 1), (12, 1, 15, 1), (2, 1, 21, 1),
      (10, 1, 14, -1), (4, 1, 7, 1), (11, 1, 19, 1), (12, -1, 20, 1), (13, 1, 14, -1), (9, 1, 30, -1),
      (3, -1, 15, 1), (6, 1, 23, 1), (24, 1, 27, -1), (9, -1, 18, 1), (7, 1, 34, 1), (2, 1, 6, -1),
      (0, 1, 8, -1), (6, 1, 21, 1), (22, 1, 31, -1), (6, 1, 29, 1), (0, 1, 1, 1), (15, 1, 25, 1),
      (5, 1, 37, 1), (15, 1, 20, 1))
UN = (7, 27, 24, 17, 9, 22, 21, 2, 15, 11, 8, 25, 19, 28, 2, 23, 26, 20, 1, 18, 10, 28, 4, 13, 14, 16)
WN = (23, 17, 24, 10, 14, 7, 22, 19, 12, 18, 15, 25, 20, 5, 26, 0, 8, 2, 27, 11, 26, 9, 28, 21, 16, 5)
VN = (42, 47, 41, 5, 11, 43, 18, 28, 20, 23, 35, 19, 22, 46, 33, 26, 45, 36, 38, 25, 44, 40, 39, 21, 24, 32)
RK = len(UN)
UL = tuple(sorted(set(UN)))
RAW16 = (1, 11, 17, 5, 8, 3, 9, 10, 0, 6, 7, 4, 12, 20, 22, 16)
VORDER = (0, 6, 7, 12, 13, 14, 15, 21, 11, 17, 20, 22, 24, 25, 23, 2, 1, 5, 8, 9, 10, 16, 18, 19)
assert sorted(VORDER) == [r for r in range(RK) if VN[r] >= 16] and len(set(RAW16)) == 16
assert all(RAW16[VN[r]] == r for r in range(RK) if VN[r] < 16)


def _run(prog, blocks):
    vals = list(blocks)
    for a, sa, b, sb in prog:
        vals.append(vals[a] + vals[b] if sa > 0 and sb > 0 else
                    vals[a] - vals[b] if sa > 0 else vals[b] - vals[a])
    return vals


def _terms(prog, nin, node):
    if node < nin:
        return {node: 1}
    a, sa, b, sb = prog[node - nin]
    out = {k: sa * v for k, v in _terms(prog, nin, a).items()}
    out.update({k: sb * v for k, v in _terms(prog, nin, b).items()})
    return out


def _scheme_is_exact():
    t = {}
    for r in range(RK):
        for a, ca in _terms(UP, 8, UN[r]).items():
            for b, cb in _terms(VP, 16, VN[r]).items():
                for c, cc in _terms(WP, 8, WN[r]).items():
                    t[a, b, c] = t.get((a, b, c), 0) + ca * cb * cc
    want = {(4 * i + j, 4 * j + l, 4 * i + l): 1 for i in range(2) for j in range(4) for l in range(4)}
    return {k: v for k, v in t.items() if v} == want


assert _scheme_is_exact()

_WPAR = {n: [] for n in range(8 + len(WP))}
for _t, (_a, _sa, _b, _sb) in enumerate(WP):
    _WPAR[_a].append((8 + _t, _sa))
    _WPAR[_b].append((8 + _t, _sb))


def _worder():
    order = []

    def closure(n, acc):
        if n not in acc and n not in order:
            acc.add(n)
            for q, _ in _WPAR[n]:
                closure(q, acc)
        return acc

    def visit(n):
        if n not in order:
            for q, _ in _WPAR[n]:
                visit(q)
            order.append(n)
    while len([v for v in range(8) if v not in order]):
        visit(min((v for v in range(8) if v not in order), key=lambda v: len(closure(v, set()))))
    return tuple(order)


WORDER = _worder()


def _ln(x):
    m = jnp.mean(x, axis=-1, keepdims=True)
    xc = x - m
    v = jnp.mean(xc * xc, axis=-1, keepdims=True)
    return xc * lax.rsqrt(v + EPS)


_GC = 0.7978845608028654


def _gelu(x):
    h = 0.5 * x
    return h + h * jnp.tanh(x * (_GC + (_GC * 0.044715) * (x * x)))


def _unpack(u):
    return pltpu.bitcast(u, bf16).astype(f32)


def _pack(x):
    return pltpu.bitcast(x.astype(bf16), u32)


def _cat(xs, axis):
    xs = [x for x in xs if x.shape[axis]]
    return xs[0] if len(xs) == 1 else jnp.concatenate(xs, axis=axis)


def _as(x, dtype):
    return x if x.dtype == dtype else pltpu.bitcast(x, dtype)


def _lcombos(a11, a12, a21, a22):
    return [a11 + a22, a21 + a22, a11, a22, a11 + a12, a21 - a11, a12 - a22]


def _merge(*lists):
    keyed = [((j + 0.5) / len(l), n, j, v) for n, l in enumerate(lists) for j, v in enumerate(l)]
    return [v for _, _, _, v in sorted(keyed, key=lambda t: t[:3])]


def _masks():
    r = lax.broadcasted_iota(jnp.int32, (32, 48), 0)
    c = lax.broadcasted_iota(jnp.int32, (32, 48), 1)
    exist_e = c < 40
    allow_e = exist_e & ((r >= 24) | ((c >= 24) & (c < 32)) | (c <= r))
    fill_e = jnp.where(exist_e, NEG, -jnp.inf).astype(f32)
    r = lax.broadcasted_iota(jnp.int32, (48, 80), 0)
    c = lax.broadcasted_iota(jnp.int32, (48, 80), 1)
    q_even = (r >= 32) & (r < 40)
    exist_o = (q_even & (c < 40)) | (~q_even & (c >= 40))
    ktok = jnp.where(c < 24, c, jnp.where(c < 48, c - 8, c - 16))
    qtok = jnp.where(r < 32, r + 32, r - 8)
    is_mem_key = ((c >= 24) & (c < 32)) | ((c >= 48) & (c < 56))
    allow_o = exist_o & (is_mem_key | (r < 8) | (ktok <= qtok))
    fill_o = jnp.where(exist_o, NEG, -jnp.inf).astype(f32)
    return allow_e, fill_e, allow_o, fill_o


def _rcombo(k, b11, b12, b21, b22):
    if k in (1, 4):
        return (b11 if k == 1 else b22)(k)
    a, b, sign = {0: (b11, b22, 1), 2: (b12, b22, -1), 3: (b21, b11, -1), 5: (b11, b12, 1), 6: (b21, b22, 1)}[k]
    a, b = _unpack(a(k)), _unpack(b(k))
    return (a + b if sign > 0 else a - b).astype(bf16)


def _softmax(s, allow, fill):
    s = jnp.where(allow, s * SCALE, fill)
    m = jnp.max(s, axis=-1, keepdims=True)
    e = jnp.exp(s - m)
    l = jnp.sum(e, axis=-1, keepdims=True)
    r = pl.reciprocal(l, approx=True)
    r = r * (2.0 - l * r)
    return (e * r).astype(bf16)


def _kernel(x_hbm, mem0_hbm, wq_hbm, wk_hbm, wv_hbm, wo_hbm, w1_hbm, w2_hbm, w3_hbm, w4_hbm,
            gw_hbm, out_hbm,
            x_v, s1_v, s2_v, s3_v, s4_v, wqkv_v, wo_v, h_v, b_v, c0_v, l_v, lf_v, n_v, g_v, out_v, xe_v, e_v, oe_v,
            ke_v, ve_v, o_v, mem_v, mem0_ref, gw_ref, zero_s,
            sem, sem_qkv, sem_out):
    RAW = (1, 2, 3, 4)
    RAW1 = (1, 7, 8, 4)

    loads = []

    def rows_load(name, r0, r1):
        loads.append((name, x_hbm.at[pl.ds(r0, r1 - r0)], x_v.at[pl.ds(r0, r1 - r0)]))

    def quad_load(name, w_hbm, s_v, raw, q, c0=0, c1=None):
        k4, n2 = s_v.shape[1], s_v.shape[2]
        c1 = n2 if c1 is None else c1
        src = w_hbm.bitcast(u32).at[pl.ds((q // 2) * k4, k4), pl.ds((q % 2) * n2 + c0, c1 - c0)]
        loads.append((name, src, s_v.at[raw[q], :, pl.ds(c0, c1 - c0)]))

    def w1_load(name, half, c0, c1):
        quad_load(name, w1_hbm, s1_v, RAW1, half, c0, c1)
        quad_load(name, w1_hbm, s1_v, RAW1, 2 + half, c0, c1)

    def block_load(name, w_hbm, s_v, r0, r1):
        kb, nb = s_v.shape[1:]
        for q in range(16):
            loads.append((name, w_hbm.at[pl.ds((q // 4) * kb + r0, r1 - r0), pl.ds((q % 4) * nb, nb)],
                          s_v.at[RAW16[q], pl.ds(r0, r1 - r0)]))

    rows_load("x0", 0, TM)
    w1_load("w1a", 0, 0, 256)
    w1_load("w1b", 0, 256, 512)
    rows_load("x1", TM, 2 * TM)
    w1_load("w1cd", 1, 0, 512)
    rows_load("x23", 2 * TM, 4 * TM)
    rows_load("x4567", 4 * TM, S)
    for q in range(4):
        quad_load("w2", w2_hbm, s2_v, RAW, q)
    block_load("w2", w3_hbm, s3_v, 0, W3A)
    block_load("w4", w3_hbm, s3_v, W3A, D4)
    block_load("w4", w4_hbm, s4_v, 0, F4)
    loads.append(("small", mem0_hbm, mem0_ref))
    loads.append(("small", gw_hbm, gw_ref))
    for j in range(NT):
        loads.append(("wo", wo_hbm.bitcast(u32).at[:, pl.ds(j * 128, 128)], wo_v.at[j]))
    groups = list(dict.fromkeys(name for name, _, _ in loads))
    assert len(groups) == NLOAD

    def start(*names, priority=0):
        for name, src, dst in loads:
            if name in names:
                pltpu.make_async_copy(src, dst, sem.at[groups.index(name)]).start(priority=priority)

    def wait(*names):
        for name, src, dst in loads:
            if name in names:
                pltpu.make_async_copy(src, dst, sem.at[groups.index(name)]).wait()

    SPG = 3 * G

    def qkv_start(g):
        for w, w_hbm in enumerate((wq_hbm, wk_hbm, wv_hbm)):
            wu = w_hbm.bitcast(u32)
            for k in range(G // 2):
                for par in range(2):
                    pltpu.make_async_copy(
                        wu.at[:, par * (H // 2) + g * (G // 2) + k, :],
                        wqkv_v.at[g * SPG + w * G + 2 * k + par], sem_qkv.at[g]).start(priority=1)

    def qkv_wait(g):
        grp = wqkv_v.at[pl.ds(g * SPG, SPG)]
        pltpu.make_async_copy(grp, grp, sem_qkv.at[g]).wait()

    start("x0", "w1a", "w1b", "x1", "w1cd", "x23", "x4567", "w2", "w4", "small")

    def zero(k, carry):
        zero_s[k] = 0
        return carry
    lax.fori_loop(0, RK, zero, 0)

    def once(fn):
        def body(_, carry):
            fn()
            return carry
        lax.fori_loop(0, 1 + zero_s[1], body, 0)

    def tile_idx(ref, cols=128):
        z = zero_s[0]
        n = 16 if ref.dtype == bf16 and cols == 128 else 8
        return (z,) * (len(ref.shape) - 2) + (pl.ds(pl.multiple_of(z, n), n), slice(0, cols))

    hist = []

    def mm(lhs, rhs, side=None, acc=None):
        if side is not None:
            lhs = side(lhs)
        lhs = pltpu.bitcast(lhs, bf16) if lhs.dtype == u32 else lhs.astype(bf16)
        y = _dot(lhs, pltpu.bitcast(rhs, bf16) if rhs.dtype == u32 else rhs)
        if acc is not None:
            y = y + acc
        hist.append(y)
        return y

    class Side:
        def __init__(self, pieces, n, skip=0):
            cap = [0] * skip + [1] * n
            tot = sum(p[4] for p in pieces)
            self.plan = [[] for _ in cap]
            done = 0
            for p in pieces:
                done += p[4]
                x, d = done / tot * sum(cap), 0
                while x > cap[d] + 1e-9:
                    x -= cap[d]
                    d += 1
                self.plan[d].append((p, x / cap[d]))
            self.pieces = len(pieces)

        def __call__(self, val):
            todo = self.plan.pop(0) if self.plan else []
            if not todo:
                return val
            self.pieces -= len(todo)
            never = zero_s[0] > 0
            if val.dtype == bf16:
                val = pltpu.bitcast(val, u32)
            rg = 8 if val.dtype == u32 else 16
            ng = val.shape[0] // rg
            tied = {}
            for (fn, rd, wr, lag, _), pos in todo:
                m = min(max(-int(-pos * ng // 1) - 1, 0), ng - 1)
                pin = lambda v, w=128: v
                if lag is not None and len(hist) >= lag:
                    r0 = (16 * m) % hist[-lag].shape[0]
                    a = hist[-lag][r0:r0 + 8, :128]
                    if rd is None:
                        def pin(v, w=128, a=a):
                            a = _cat([_cat([_as(a, v.dtype)] * (v.shape[0] // 8), 0)] * (w // 128), 1)
                            if v.shape[1] == w:
                                return lax.select(never, a, v)
                            return _cat([lax.select(never, a, v[:, :w]), v[:, w:]], 1)
                    elif rd.dtype == bf16:
                        idx = tile_idx(rd, 256)
                        rd[idx] = lax.select(never, _cat([a, a], 1).astype(bf16), rd[idx])
                    else:
                        idx = tile_idx(rd)
                        rd[idx] = lax.select(never, _as(a, rd.dtype), rd[idx])
                u = fn(pin)
                if wr is False:
                    continue
                if wr is not None:
                    u = wr[tile_idx(wr)]
                t, n = tied.get(m * rg) or (val[m * rg:m * rg + 8, -128:], 0)
                tied[m * rg] = (lax.select(zero_s[n] > 0, _as(u, val.dtype), t), n + 1)
            if not tied:
                return val
            col, r = [], 0
            for r0 in sorted(tied):
                col += ([val[r:r0, -128:]] if r0 > r else []) + [tied[r0][0]]
                r = r0 + 8
            col += [val[r:, -128:]] if r < val.shape[0] else []
            return _cat([val[:, :-128], _cat(col, 0)], 1) if val.shape[1] > 128 else _cat(col, 0)

    def strassen(lhs, rhs, side, init=(None, None, None, None)):
        def add(a, b):
            return a if b is None else a + b
        p = [mm(lhs(k), rhs(k), side) for k in range(5)]
        c12 = add(p[2] + p[4], init[1])
        c21 = add(p[1] + p[3], init[2])
        c22 = mm(lhs(5), rhs(5), side, add(p[0] - p[1] + p[2], init[3]))
        c11 = mm(lhs(6), rhs(6), side, add(p[0] + p[3] - p[4], init[0]))
        return c11, c12, c21, c22

    def fmm(lhs, rhs, side, extra=lambda n: None, emit=None):
        val = {}
        for n in WORDER:
            t = extra(n)
            for q, sg in sorted(_WPAR[n], key=lambda e: -e[1]):
                t = val[q] if t is None else (t + val[q] if sg > 0 else t - val[q])
            for r in range(RK):
                if WN[r] == n:
                    t = mm(lhs(UN[r]), rhs(r), side, t)
            val[n] = t
            if n < 8 and emit is not None:
                emit(n, t)
        return [val[v] for v in range(8)]

    def prep26_pieces(s_v, lag):
        def piece(rs, cs, pin):
            @functools.lru_cache(None)
            def node(n):
                if n < 16:
                    return s_v[RAW16[n], rs, cs].astype(f32)
                a, sa, b, sb = VP[n - 16]
                return _run([(0, sa, 1, sb)], [node(a), node(b)])[-1]
            vals = [node(VN[r]).astype(bf16) for r in VORDER]
            for r, t in zip(VORDER, vals):
                s_v[r, rs, cs] = t
        kb, nb = s_v.shape[1:]
        out = []
        for r in range(0, kb, 16):
            out += [(slice(rr, rr + 8), slice(c, c + 256)) for c in range(0, nb - 255, 256) for rr in (r, r + 8)]
            out += [(slice(rr, rr + 8), slice(nb - 128, nb)) for rr in (r, r + 8)] if nb % 256 else []
        return [(functools.partial(piece, rs, cs), s_v, s_v if n % 16 == 15 else False, lag,
                 130 if cs.stop - cs.start == 256 else 100) for n, (rs, cs) in enumerate(out)]

    def prep_pieces(s_v, raw, lag, width=256):
        def piece(r, c, pin):
            idx = (slice(r, r + 8), slice(c, c + width))
            b11, b12, b21, b22 = [_unpack(pin(s_v[(q,) + idx], width) if n in (0, 3) else s_v[(q,) + idx])
                                  for n, q in enumerate(raw)]
            for k, t in ((0, b11 + b22), (2, b12 - b22), (3, b21 - b11), (5, b11 + b12), (6, b21 + b22)):
                s_v[(k,) + idx] = _pack(t)
        return [(functools.partial(piece, r, c), None, s_v, lag, 80)
                for c in range(0, s_v.shape[2], width) for r in range(0, s_v.shape[1], 8)]

    def store_l(slot, q, c, quads):
        for k, t in enumerate(_lcombos(*quads)):
            l_v[slot, k, q // 2:q // 2 + 8, c:c + t.shape[1]] = _pack(t)

    def ln_pieces(src, r0, slot, lag, width=256, staged=False, clag=None):
        def stats(q, pin):
            x = pin(src[pl.ds(r0 + q, 16), :].astype(f32))
            xs = [x[:, j * 128:(j + 1) * 128] for j in range(NT)]
            m = functools.reduce(lambda a, b: a + b, xs) * (1.0 / NT)
            w = functools.reduce(lambda a, b: a + b, [(t - m) * (t - m) for t in xs])
            mean = jnp.mean(m, axis=-1, keepdims=True)
            var = jnp.sum(w + NT * ((m - mean) * (m - mean)), axis=-1, keepdims=True) * (1.0 / D)
            n_v[0, q:q + 16, :] = jnp.broadcast_to(mean, (16, 128))
            n_v[1, q:q + 16, :] = jnp.broadcast_to(lax.rsqrt(var + EPS), (16, 128))

        def comb(q, c, pin):
            quads = []
            for rr in (0, HM):
                rs = pl.ds(pl.multiple_of(r0 + rr + q + zero_s[0], 16), 16)
                mean, rstd = [jnp.concatenate([n_v[t, rr + q:rr + q + 16, :]] * (width // 128), axis=1)
                              for t in range(2)]
                quads += [(src[rs, cc + c:cc + c + width].astype(f32) - mean) * rstd for cc in (0, DH2)]
            store_l(slot, q, c, quads)

        def comb26(q, pin):
            blocks = []
            for rr in (0, HM):
                rs = pl.ds(pl.multiple_of(r0 + rr + q + zero_s[0], 8), 8)
                mean, rstd = [jnp.concatenate([n_v[t, rr + q:rr + q + 8, :]] * 2, axis=1) for t in range(2)]
                blocks += [(src[rs, cc:cc + D4] - mean) * rstd for cc in range(0, D, D4)]
            vals = _run(UP, blocks)
            for k, u in enumerate(UL):
                lf_v[k, q:q + 8, :] = vals[u].astype(bf16)
        dense = slot is not None or src is b_v
        norms = [[(functools.partial(stats, rr + q), None, n_v if dense else False, lag, 90) for rr in (0, HM)]
                 for q in range(0, HM, 16)]
        if slot is None:
            combs = [[(functools.partial(comb26, qq), n_v, lf_v if dense or qq % 32 == 24 else False, clag, 110)
                      for qq in (q, q + 8)] for q in range(0, HM, 16)]
        else:
            combs = [[(functools.partial(comb, q, c), n_v, l_v, clag, 125) for c in range(0, DH2, width)]
                     for q in range(0, HM, 16)]
        if staged:
            return sum(norms, []), sum(combs, [])
        out = list(norms[0])
        for a, b in zip(norms[1:] + [[]], combs):
            out += _merge(a, b) if a else b
        return out

    shifts = (1, 1, -1, -1, 2, 2, -2, -2)

    def shift_pieces(r0, slot, lag, by_value=False):
        def piece(q, j, pin):
            a = [h_v[jj, pl.ds(PAD + r0 + rr + q - shifts[jj], 16), :]
                 for rr in (0, HM) for jj in (j, j + NT // 2)]
            store_l(slot, q, j * 128, [pin(a[0]), a[1], a[2], pin(a[3])])
        return [(functools.partial(piece, q, j), None if by_value else h_v,
                 l_v if (q // 16) % 2 and j == 3 else False, lag, 50)
                for q in range(0, HM, 16) for j in range(NT // 2)]

    def lhs_of(slot):
        return lambda k: l_v[slot, k]

    xe_v[0, 0:16, :] = jnp.zeros((16, D4), bf16)
    h_v[:, 0:PAD, :] = jnp.zeros((NT, PAD, 128), f32)
    h_v[:, PAD + S:PAD + S + PAD, :] = jnp.zeros((NT, PAD, 128), f32)

    def store_h(r0, c0, h):
        for j in range(h.shape[1] // 128):
            h_v[c0 // 128 + j, PAD + r0:PAD + r0 + h.shape[0], :] = h[:, j * 128:(j + 1) * 128]

    def h_pieces(r0, c0, t, lag, n=4):
        def piece(r, pin):
            store_h(r0 + r, c0, _gelu(pin(t[r:r + 8 * n])))
        return [(functools.partial(piece, r), None, h_v, lag, 10 * n) for r in range(0, t.shape[0], 8 * n)]

    def flush(pieces):
        for p in pieces:
            p[0](lambda v, w=128: v)

    def w1_cols(c, step):
        half, cc = c // DH2, c % DH2
        return jnp.concatenate([s1_v[RAW1[half], :, cc:cc + step], s1_v[RAW1[2 + half], :, cc:cc + step]], axis=0)

    def d1_plain(xn, r0, c0, c1, step):
        for c in range(c0, c1, step):
            store_h(r0, c, _gelu(mm(xn, w1_cols(c, step))))

    def d1_fine(lhs, r0, nrb, cols, pieces, carry, skip=0):
        tiles = [(rb, c) for c in cols for rb in range(nrb)]
        rounds = [tiles[i:i + 4] for i in range(0, len(tiles), 4)]
        for n, (rnd, part) in enumerate(zip(rounds, split(pieces, len(rounds)))):
            sk = skip if n == 0 else 0
            side = Side(_merge(carry, part) if carry else part, 8 - sk, sk)
            carry = []
            for rb, c in rnd:
                half, cc = c // DH2, c % DH2
                t = mm(lhs(rb, 0), s1_v[RAW1[half], :, cc:cc + 128], side)
                t = mm(lhs(rb, 1), s1_v[RAW1[2 + half], :, cc:cc + 128], side, t)
                carry += h_pieces(r0 + rb * HM, c, t, LS)
        return carry

    def d1_s(b, slot, pieces, carry, early=()):
        for c, part, e in zip(range(0, DH2, NC1), split(pieces, DH2 // NC1), split(early, 2) + [[], []]):
            side = Side(merge(carry, part, e), *((7,) if hist else (5, 2)))
            cs = strassen(lhs_of(slot), lambda k: s1_v[k, :, c:c + NC1], side)
            carry = sum([h_pieces(b * TM + (q // 2) * HM, (q % 2) * DH2 + c, cs[q], LS) for q in (1, 2, 3, 0)], [])
        return carry

    def d2_s(b, slot, pieces, carry=(), early=(), late=()):
        for c, part, e in zip(range(0, DH2, NC1), split(pieces, DH2 // NC1), split(early, 2) + split(late, 2)):
            side = Side(merge(carry, part, e), *((7,) if hist else (5, 2)))
            carry = ()
            idx = [(slice(b * TM + (q // 2) * HM, b * TM + (q // 2 + 1) * HM),
                    slice((q % 2) * DH2 + c, (q % 2) * DH2 + c + NC1)) for q in range(4)]
            cs = strassen(lhs_of(slot), lambda k: s2_v[k, :, c:c + NC1], side,
                          [x_v[i].astype(f32) for i in idx])
            for i, t in zip(idx, cs):
                b_v[i] = t
                if b == 0:
                    c0_v[i] = t

    def split(l, n):
        w = [1.0 if hist else 0.6] + [1.0] * (n - 1)
        cut = [int(round(len(l) * sum(w[:i]) / sum(w))) for i in range(n + 1)]
        return [l[cut[i]:cut[i + 1]] for i in range(n)]

    def merge(*ls):
        ls = [l for l in ls if l]
        return _merge(*ls) if ls else []

    NW1, NW3, N30 = 52, 32, 20
    LS, LL = 3, 5

    p3 = prep26_pieces(s3_v, LS)
    n3 = len(p3) * W3A // D4

    @once
    def _phase1a():
        wait("x0")
        xn0 = _pack(_ln(x_v[0:TM, :].astype(f32)))
        wait("w1a")
        d1_plain(xn0, 0, 0, 256, 256)
        wait("w1b")
        d1_plain(xn0, 0, 256, 512, 256)
        wait("x1")
        xn1 = _pack(_ln(x_v[TM:2 * TM, :].astype(f32)))
        d1_plain(xn1, TM, 0, 512, 256)
        wait("w1cd")
        hist.clear()
        xn01 = jnp.concatenate([xn0, xn1], axis=0)
        l01 = lambda rb, kh: xn01[rb * 64:(rb + 1) * 64, kh * DH2:(kh + 1) * DH2]
        pw = prep_pieces(s1_v, RAW1, LS)
        flush(d1_fine(l01, 0, 4, (512, 640), pw[:NW1], [], 1))
        carry = []
        wait("x23")
        hist.clear()
        carry = d1_fine(l01, 0, 4, (768, 896), ln_pieces(x_v, 2 * TM, 0, LL), carry, 3)
        carry = d1_s(2, 0, ln_pieces(x_v, 3 * TM, 1, LL), carry, pw[NW1:])
        wait("x4567")
        qkv_start(0)
        qkv_start(1)
        hist.clear()
        for b in range(3, NB - 1):
            carry = d1_s(b, b % 2, ln_pieces(x_v, (b + 1) * TM, (b + 1) % 2, LL), carry)
        wait("w2")
        hist.clear()
        pw = prep_pieces(s2_v, RAW, LS)
        carry = d1_s(7, 1, _merge(pw[:NW3], shift_pieces(0, 0, LS, True)), carry)
        d2_s(0, 0, shift_pieces(TM, 1, LS, True), carry, pw[NW3:], p3[:N30])
        pw = split(_merge(p3[N30:n3], sum(ln_pieces(c0_v, 0, None, LL, clag=LS, staged=True), [])), 3)
        for b in range(1, 4):
            d2_s(b, b % 2, _merge(pw[b - 1], shift_pieces((b + 1) * TM, (b + 1) % 2, LS)))
        wait("w4", "small")

    hist.clear()
    pw = p3[n3:] + prep26_pieces(s4_v, LS)
    cut = (0, 33, 68, 103, len(pw))
    for b in range(4, NB):
        d2_s(b, b % 2, merge(pw[cut[b - 4]:cut[b - 3]],
                             shift_pieces((b + 1) * TM, (b + 1) % 2, LS) if b + 1 < NB else ()))
    start("wo", priority=1)

    def ffn(i, carry):
        qkv_wait(i)
        r0 = pl.multiple_of(i * TM, TM)
        rn = pl.multiple_of(jnp.minimum(i + 1, NB - 1) * TM, TM)
        acc = {}
        hist.clear()

        def relayout(p, r0_, r1_, pin):
            s0 = i * SPG + 2 * p
            e = wqkv_v[s0, r0_:r1_, :]
            o = wqkv_v[s0 + 1, r0_:r1_, :]
            wqkv_v[s0, r0_:r1_, :] = (e & jnp.uint32(0xFFFF)) | (o << 16)
            wqkv_v[s0 + 1, r0_:r1_, :] = (e >> 16) | (o & jnp.uint32(0xFFFF0000))

        relays = [(functools.partial(relayout, p, r, r + 32), wqkv_v, wqkv_v, 3, 35)
                  for p in range(SPG // 2) for r in range(0, D // 2, 32)]
        norms, combs = ln_pieces(b_v, rn, None, 5, staged=True, clag=3)

        def gate(q, pin):
            gw = gw_ref[...].astype(f32)
            x = pin(x_v[pl.ds(r0 + q, 16), :].astype(f32))
            t = functools.reduce(lambda a, b: a + b,
                                 [x[:, j * 128:(j + 1) * 128] * gw[j:j + 1, :] for j in range(NT)])
            g = jax.nn.sigmoid(jnp.sum(t, axis=-1, keepdims=True))
            g_v[pl.ds(r0 + q, 16), :] = jnp.broadcast_to(g, (16, 128))

        gates = [(functools.partial(gate, q), None, g_v, 5, 90) for q in range(0, TM, 16)]

        def extras(t, pin):
            jj, o = 2 * i + t // 2, 24 + 8 * (t % 2)
            xs = [pin(x_v[pl.ds(pl.multiple_of((jj + hh) * 64 + o, 8), 8), :].astype(f32)) for hh in (0, NPAIR // 2)]
            vals = _run(UP, [x[:, cc:cc + D4] for x in xs for cc in range(0, D, D4)])
            for k, u in enumerate(UL):
                xe_v[k, pl.ds(pl.multiple_of(i * 32 + t * 8, 8), 8), :] = vals[u].astype(bf16)

        xes = [(functools.partial(extras, t), None, xe_v, 3, 100) for t in range(4)]
        hs = {}

        def gelu_pieces(c, cs):
            def piece(r, cc, vs, pin):
                t = _gelu(pin(_cat([cs[v][r:r + 8, cc:cc + 128] for v in vs], 0)))
                ts = [t[8 * n:8 * n + 8] for n in range(len(vs))]
                hs.update({(c, v, r, cc): u for v, u in zip(vs, ts)})
                return functools.reduce(lambda a, b: a + b, ts)
            return [(functools.partial(piece, r, cc, vs), None, None, 3, 40) for r in range(0, HM, 8)
                    for cc in range(0, cs[0].shape[1], 128) for vs in ((0, 1, 2, 3), (4, 5, 6, 7))]

        def d3(c, side):
            c0, c1 = FCH[c]
            cs = fmm(lambda u: lf_v[UL.index(u)], lambda r: s3_v[r, :, c0:c1], side)
            assert not side.pieces
            return gelu_pieces(c, cs)

        def d4(c, side):
            c0, c1 = FCH[c]
            lh = _run(UP, [_cat([_cat([hs.pop((c, v, r, cc)) for r in range(0, HM, 8)], 0)
                                 for cc in range(0, c1 - c0, 128)], 1) for v in range(8)])
            rhs = lambda r: s4_v[r, c0:c1, :]
            if c + 1 < len(FCH):
                for n in WORDER:
                    for r in range(RK):
                        if WN[r] == n:
                            acc[n] = mm(lh[UN[r]], rhs(r), side, acc.get(n))
            else:
                idx = lambda v: (pl.ds(r0 + (v // 4) * HM, HM), slice((v % 4) * D4, (v % 4 + 1) * D4))

                def extra(n):
                    if n >= 8:
                        return acc.get(n)
                    return b_v[idx(n)] + acc[n] if n in acc else b_v[idx(n)]

                def emit_b(v, t):
                    b_v[idx(v)] = jnp.concatenate([1.0 - g_v[idx(v)[0], :]] * 2, axis=1) * t
                fmm(lambda u: lh[u], rhs, side, extra, emit_b)
            assert not side.pieces

        g0 = d3(0, Side(relays[:20], 23, 3))
        g1 = d3(1, Side(_merge(g0, gates, xes), 23, 2))
        d4(0, Side(g1[:22], 22, 4))
        g2 = d3(2, Side(_merge(g1[22:], relays[20:40]), 25))
        d4(1, Side(g2, 23, 2))
        g3 = d3(3, Side(_merge(relays[40:], norms), 26))
        d4(2, Side(_merge(g3, combs), 23, 2))
        d4(3, Side([], 1))

        @pl.when(i + 2 < NG)
        def _():
            qkv_start(i + 2)

        return carry

    lax.fori_loop(0, NB, ffn, 0)

    def pre(it, carry):
        hist.clear()
        for u in range(3 * NG // NPRE):
            s0 = (it * (3 * NG // NPRE) + u) * G

            def rhs(r):
                t = None
                sz = s0 + zero_s[r]
                for q, sg in sorted(_terms(VP, 16, VN[r]).items(), key=lambda e: -e[1]):
                    blk = wqkv_v[sz + q % 4, (q // 4) * (D // 8):(q // 4 + 1) * (D // 8), :]
                    if VN[r] < 16:
                        return blk
                    blk = _unpack(blk)
                    t = blk if t is None else (t + blk if sg > 0 else t - blk)
                return t.astype(bf16)
            for v, t in enumerate(fmm(lambda k: xe_v[UL.index(k)], rhs, None)):
                e_v[(v // 4) * 16:(v // 4 + 1) * 16, s0 + v % 4] = _pack(t).reshape(16, 8, DH)
        return carry

    lax.fori_loop(0, NPRE, pre, 0)

    wait("wo")
    mem_v[...] = mem0_ref[...].astype(f32)

    def slab(w, h):
        return (h // G) * SPG + w * G + h % G

    def step(j, hx, odd, late, allow, fill):
        qs, ks, vs, ps = {}, {}, {}, {}
        wload = lambda w, h: pltpu.bitcast(wqkv_v[slab(w, h)], bf16)
        eload = lambda w, h: pltpu.bitcast(e_v[j, slab(w, h)], bf16)

        def proj(g):
            part = {}
            if late and g == 0:
                for h in range(2):
                    for w in range(3):
                        part[w, h] = _dot(hx[:, :DH2], wload(w, h)[:DH2])
            for h in range(g * G, (g + 1) * G):
                q, k, v = [(_dot(hx[:, DH2:], wload(w, h)[DH2:]) + part[w, h] if (w, h) in part
                            else _dot(hx, wload(w, h))).astype(bf16) for w in range(3)]
                if odd:
                    q = jnp.concatenate([q, eload(0, h)], axis=0)
                    k = jnp.concatenate([pltpu.bitcast(ke_v[h], bf16), eload(1, h), k], axis=0)
                    v = jnp.concatenate([pltpu.bitcast(ve_v[h], bf16), eload(2, h), v], axis=0)
                else:
                    ke_v[h] = pltpu.bitcast(k, u32)
                    ve_v[h] = pltpu.bitcast(v, u32)
                    k = jnp.concatenate([k, eload(1, h)], axis=0)
                    v = jnp.concatenate([v, eload(2, h)], axis=0)
                qs[h], ks[h], vs[h] = q, k, v

        def score(g):
            for h in range(g * G, (g + 1) * G):
                s = lax.dot_general(qs.pop(h), ks.pop(h), (((1,), (1,)), ((), ())),
                                    preferred_element_type=f32)
                ps[h] = _softmax(s, allow, fill)

        def pv(g):
            os_ = []
            for h in range(g * G, (g + 1) * G):
                o = _dot(ps.pop(h), vs.pop(h))
                o_v[:, h * 128:(h + 1) * 128] = _pack(o[:32])
                os_.append(o)
            if odd:
                quads = [jnp.concatenate([os_[2 * kk][r:r + 8], os_[2 * kk + 1][r:r + 8]], axis=1)
                         for r in (32, 40) for kk in range(2)]
                for k, t in enumerate(_lcombos(*quads)):
                    oe_v[k, pl.ds(pl.multiple_of(j * 8, 8), 8), g * 256:(g + 1) * 256] = t.astype(bf16)

        acc = [None] * NT

        def wo(h0, h1, j0, j1):
            o = pltpu.bitcast(o_v[:, h0 * 128:h1 * 128], bf16)
            for n in range(j0, j1):
                y = _dot(o, pltpu.bitcast(wo_v[n, h0 * 64:h1 * 64, :], bf16))
                acc[n] = y if acc[n] is None else y + acc[n]

        for t in range(NG):
            proj(t)
            if t >= 2:
                pv(t - 2)
            if t >= 1:
                score(t - 1)
        wo(0, 16, 0, 4)
        pv(NG - 2)
        score(NG - 1)
        wo(0, 16, 4, 8)
        pv(NG - 1)
        wo(16, 24, 0, 8)
        wo(24, 32, 0, 8)
        return jnp.concatenate(acc, axis=1)

    def emit(j, r0, o0, a):
        rs = pl.ds(r0 + o0, 24)
        g = jnp.concatenate([g_v[rs, :]] * NT, axis=1)
        out_v[j, o0:o0 + 24, :] = (g * a + b_v[rs, :]).astype(bf16)

    def pair(j, mem, late):
        r0 = pl.multiple_of(j * 64, 64)
        allow_e, fill_e, allow_o, fill_o = _masks()
        xa = x_v[pl.ds(r0 + 16, 8), :].astype(f32)
        xb = x_v[pl.ds(r0 + 40, 8), :].astype(f32)
        hx = jnp.concatenate([x_v[pl.ds(r0, 16), :], jnp.concatenate([xa, mem], 0).astype(bf16)], 0)
        oe = step(j, hx, False, late, allow_e, fill_e)
        emit(j, r0, 0, oe[:24])
        hx = jnp.concatenate([jnp.concatenate([oe[24:32], xb], 0).astype(bf16), x_v[pl.ds(r0 + 48, 16), :]], 0)
        oo = step(j, hx, True, True, allow_o, fill_o)
        emit(j, r0, 40, oo[8:])
        return oo[:8]

    def a_iter(it, carry):
        mem = mem_v[...]
        for t in range(PPI):
            mem = pair(it * PPI + t, mem, t > 0)
        mem_v[...] = mem
        for t in range(PPI):
            for o0 in (0, 40):
                idx = (it * PPI + t, pl.ds(o0, 24))
                pltpu.make_async_copy(out_v.at[idx], out_hbm.at[idx], sem_out).start()
        return carry

    lax.fori_loop(0, NPAIR // PPI, a_iter, 0)

    @once
    def _post():
        hist.clear()
        for n in range(NT // 2):
            quad = [lambda k, t=2 * n + q % 2, o=(q // 2) * 128: jnp.concatenate(
                [wo_v[t + zero_s[k], g * 256 + o:g * 256 + o + 128, :] for g in range(NG)], axis=0) for q in range(4)]
            cs = strassen(lambda k: oe_v[k], lambda k: _rcombo(k, *quad), None)
            cols = slice(n * 256, (n + 1) * 256)
            for half in range(2):
                t = jnp.concatenate(cs[2 * half:2 * half + 2], axis=1)
                o0 = 24 + half * 8
                for jj in range(NPAIR):
                    rs = slice(jj * 64 + o0, jj * 64 + o0 + 8)
                    g = jnp.concatenate([g_v[rs, :]] * 2, axis=1)
                    out_v[jj, o0:o0 + 8, cols] = (g * t[jj * 8:jj * 8 + 8] + b_v[rs, cols]).astype(bf16)
            if n >= 2:
                idx = (slice(None), pl.ds(24, 16), pl.ds(0, 768) if n == 2 else pl.ds(768, 256))
                pltpu.make_async_copy(out_v.at[idx], out_hbm.at[idx], sem_out).start()

    pltpu.make_async_copy(out_v, out_hbm, sem_out).wait()


@jax.jit
def pallas_gated_mix__memory_aug_recurrent_mem_tr__mixer_s_mlp__prompt_kernel(
    A_x, A_mem0, A_Wq, A_Wk, A_Wv, A_Wo, A_seg_len, B_x, B_w1, B_w2, B_w3, B_w4, gate_w,
):
    assert A_x.shape == (1, S, D) and A_mem0.shape == (1, M, D)
    any_spec = pl.BlockSpec(memory_space=pl.ANY)
    out = pl.pallas_call(
        _kernel,
        out_shape=jax.ShapeDtypeStruct((NPAIR, 64, D), bf16),
        in_specs=[any_spec] * 11,
        out_specs=any_spec,
        scratch_shapes=[
            pltpu.VMEM((S, D), bf16),
            pltpu.VMEM((9, D // 4, D // 2), u32),
            pltpu.VMEM((7, D // 4, D // 2), u32),
            pltpu.VMEM((RK, D4, F4), bf16),
            pltpu.VMEM((RK, F4, D4), bf16),
            pltpu.VMEM((3 * H, D // 2, DH), u32),
            pltpu.VMEM((NT, H * DH // 2, 128), u32),
            pltpu.VMEM((NT, S + 2 * PAD, 128), f32),
            pltpu.VMEM((S, D), f32),
            pltpu.VMEM((TM, D), f32),
            pltpu.VMEM((2, 7, HM // 2, D // 2), u32),
            pltpu.VMEM((len(UL), HM, D4), bf16),
            pltpu.VMEM((2, TM, 128), f32),
            pltpu.VMEM((S, 128), f32),
            pltpu.VMEM((NPAIR, 64, D), bf16),
            pltpu.VMEM((len(UL), 8 * NPAIR, D4), bf16),
            pltpu.VMEM((NPAIR, 3 * H, 8, DH), u32),
            pltpu.VMEM((7, 8 * NPAIR, H * DH // 2), bf16),
            pltpu.VMEM((H, 16, 128), u32),
            pltpu.VMEM((H, 16, 128), u32),
            pltpu.VMEM((16, H * DH), u32),
            pltpu.VMEM((M, D), f32),
            pltpu.VMEM((M, D), bf16),
            pltpu.VMEM((NT, 128), bf16),
            pltpu.SMEM((RK,), jnp.int32),
            pltpu.SemaphoreType.DMA((NLOAD,)),
            pltpu.SemaphoreType.DMA((NG,)),
            pltpu.SemaphoreType.DMA,
        ],
        compiler_params=pltpu.CompilerParams(vmem_limit_bytes=126 * 1024 * 1024,
                                             disable_bounds_checks=True),
    )(
        A_x.reshape(S, D), A_mem0.reshape(M, D),
        A_Wq.reshape(D // 2, 2 * H, DH), A_Wk.reshape(D // 2, 2 * H, DH), A_Wv.reshape(D // 2, 2 * H, DH),
        A_Wo.reshape(H * DH, D), B_w1, B_w2, B_w3, B_w4, gate_w.reshape(NT, 128),
    )
    return out.reshape(1, S, D)
```

```python
import functools

import jax
import jax.numpy as jnp
from jax import lax
import jax.experimental.pallas as pl
import jax.experimental.pallas.tpu as pltpu

f32, bf16, u32 = jnp.float32, jnp.bfloat16, jnp.uint32

S, D, H, DH, M, SEG, F = 2048, 1024, 32, 128, 8, 32, 3584
SCALE = DH ** -0.5
NEG = -1000000000.0
EPS = 1e-05

TM = 256
NB = S // TM
HM = TM // 2
DH2 = D // 2
D4, F4 = D // 4, F // 4
FCH = ((0, 128), (128, 384), (384, 640), (640, 896))
NC1 = 128
NPAIR = S // (2 * SEG)
PPI = 2
NPRE = 3
G = 4
NG = H // G
PAD = 8
NT = D // 128
W3A = 192
NLOAD = 11
assert NB == NG

_dot = functools.partial(jnp.dot, preferred_element_type=f32)

UP = ((4, 1, 5, 1), (6, 1, 8, 1), (0, 1, 3, 1), (2, -1, 9, 1), (4, -1, 10, 1), (0, 1, 1, 1), (2, 1, 12, 1),
      (5, 1, 7, -1), (7, 1, 12, -1), (11, -1, 13, 1), (10, -1, 11, 1), (2, 1, 7, 1), (0, -1, 4, 1),
      (6, 1, 7, 1), (1, -1, 5, 1), (3, 1, 7, -1), (1, 1, 4, 1), (2, 1, 3, 1), (1, -1, 3, 1), (1, 1, 7, -1),
      (2, 1, 6, -1))
WP = ((0, -1, 3, 1), (4, 1, 6, -1), (1, 1, 8, 1), (5, 1, 10, 1), (4, -1, 7, 1), (0, -1, 9, -1),
      (11, 1, 12, 1), (6, 1, 7, -1), (2, 1, 5, -1), (0, -1, 7, -1), (9, 1, 11, -1), (2, 1, 13, 1),
      (5, 1, 13, 1), (2, -1, 3, 1), (5, 1, 6, 1), (0, 1, 4, 1), (2, 1, 7, 1), (1, 1, 2, 1), (1, 1, 5, 1),
      (3, 1, 7, 1), (2, 1, 6, 1))
VP = ((1, 1, 5, -1), (8, 1, 11, 1), (10, 1, 17, 1), (13, 1, 16, -1), (0, 1, 4, -1), (0, 1, 3, 1),
      (14, 1, 18, -1), (0, 1, 11, 1), (14, 1, 19, -1), (0, 1, 5, 1), (12, 1, 15, 1), (2, 1, 21, 1),
      (10, 1, 14, -1), (4, 1, 7, 1), (11, 1, 19, 1), (12, -1, 20, 1), (13, 1, 14, -1), (9, 1, 30, -1),
      (3, -1, 15, 1), (6, 1, 23, 1), (24, 1, 27, -1), (9, -1, 18, 1), (7, 1, 34, 1), (2, 1, 6, -1),
      (0, 1, 8, -1), (6, 1, 21, 1), (22, 1, 31, -1), (6, 1, 29, 1), (0, 1, 1, 1), (15, 1, 25, 1),
      (5, 1, 37, 1), (15, 1, 20, 1))
UN = (7, 27, 24, 17, 9, 22, 21, 2, 15, 11, 8, 25, 19, 28, 2, 23, 26, 20, 1, 18, 10, 28, 4, 13, 14, 16)
WN = (23, 17, 24, 10, 14, 7, 22, 19, 12, 18, 15, 25, 20, 5, 26, 0, 8, 2, 27, 11, 26, 9, 28, 21, 16, 5)
VN = (42, 47, 41, 5, 11, 43, 18, 28, 20, 23, 35, 19, 22, 46, 33, 26, 45, 36, 38, 25, 44, 40, 39, 21, 24, 32)
RK = len(UN)
UL = tuple(sorted(set(UN)))
RAW16 = (1, 11, 17, 5, 8, 3, 9, 10, 0, 6, 7, 4, 12, 20, 22, 16)
VORDER = (0, 6, 7, 12, 13, 14, 15, 21, 11, 17, 20, 22, 24, 25, 23, 2, 1, 5, 8, 9, 10, 16, 18, 19)
assert sorted(VORDER) == [r for r in range(RK) if VN[r] >= 16] and len(set(RAW16)) == 16
assert all(RAW16[VN[r]] == r for r in range(RK) if VN[r] < 16)


def _run(prog, blocks):
    vals = list(blocks)
    for a, sa, b, sb in prog:
        vals.append(vals[a] + vals[b] if sa > 0 and sb > 0 else
                    vals[a] - vals[b] if sa > 0 else vals[b] - vals[a])
    return vals


def _terms(prog, nin, node):
    if node < nin:
        return {node: 1}
    a, sa, b, sb = prog[node - nin]
    out = {k: sa * v for k, v in _terms(prog, nin, a).items()}
    out.update({k: sb * v for k, v in _terms(prog, nin, b).items()})
    return out


def _scheme_is_exact():
    t = {}
    for r in range(RK):
        for a, ca in _terms(UP, 8, UN[r]).items():
            for b, cb in _terms(VP, 16, VN[r]).items():
                for c, cc in _terms(WP, 8, WN[r]).items():
                    t[a, b, c] = t.get((a, b, c), 0) + ca * cb * cc
    want = {(4 * i + j, 4 * j + l, 4 * i + l): 1 for i in range(2) for j in range(4) for l in range(4)}
    return {k: v for k, v in t.items() if v} == want


assert _scheme_is_exact()

_WPAR = {n: [] for n in range(8 + len(WP))}
for _t, (_a, _sa, _b, _sb) in enumerate(WP):
    _WPAR[_a].append((8 + _t, _sa))
    _WPAR[_b].append((8 + _t, _sb))


def _worder():
    order = []

    def closure(n, acc):
        if n not in acc and n not in order:
            acc.add(n)
            for q, _ in _WPAR[n]:
                closure(q, acc)
        return acc

    def visit(n):
        if n not in order:
            for q, _ in _WPAR[n]:
                visit(q)
            order.append(n)
    while len([v for v in range(8) if v not in order]):
        visit(min((v for v in range(8) if v not in order), key=lambda v: len(closure(v, set()))))
    return tuple(order)


WORDER = _worder()


def _ln(x):
    m = jnp.mean(x, axis=-1, keepdims=True)
    xc = x - m
    v = jnp.mean(xc * xc, axis=-1, keepdims=True)
    return xc * lax.rsqrt(v + EPS)


_GC = 0.7978845608028654


def _gelu(x):
    h = 0.5 * x
    return h + h * jnp.tanh(x * (_GC + (_GC * 0.044715) * (x * x)))


def _unpack(u):
    return pltpu.bitcast(u, bf16).astype(f32)


def _pack(x):
    return pltpu.bitcast(x.astype(bf16), u32)


def _cat(xs, axis):
    xs = [x for x in xs if x.shape[axis]]
    return xs[0] if len(xs) == 1 else jnp.concatenate(xs, axis=axis)


def _as(x, dtype):
    return x if x.dtype == dtype else pltpu.bitcast(x, dtype)


def _lcombos(a11, a12, a21, a22):
    return [a11 + a22, a21 + a22, a11, a22, a11 + a12, a21 - a11, a12 - a22]


def _merge(*lists):
    keyed = [((j + 0.5) / len(l), n, j, v) for n, l in enumerate(lists) for j, v in enumerate(l)]
    return [v for _, _, _, v in sorted(keyed, key=lambda t: t[:3])]


def _masks():
    r = lax.broadcasted_iota(jnp.int32, (32, 48), 0)
    c = lax.broadcasted_iota(jnp.int32, (32, 48), 1)
    exist_e = c < 40
    allow_e = exist_e & ((r >= 24) | ((c >= 24) & (c < 32)) | (c <= r))
    fill_e = jnp.where(exist_e, NEG, -jnp.inf).astype(f32)
    r = lax.broadcasted_iota(jnp.int32, (48, 80), 0)
    c = lax.broadcasted_iota(jnp.int32, (48, 80), 1)
    q_even = (r >= 32) & (r < 40)
    exist_o = (q_even & (c < 40)) | (~q_even & (c >= 40))
    ktok = jnp.where(c < 24, c, jnp.where(c < 48, c - 8, c - 16))
    qtok = jnp.where(r < 32, r + 32, r - 8)
    is_mem_key = ((c >= 24) & (c < 32)) | ((c >= 48) & (c < 56))
    allow_o = exist_o & (is_mem_key | (r < 8) | (ktok <= qtok))
    fill_o = jnp.where(exist_o, NEG, -jnp.inf).astype(f32)
    return allow_e, fill_e, allow_o, fill_o


def _rcombo(k, b11, b12, b21, b22):
    if k in (1, 4):
        return (b11 if k == 1 else b22)(k)
    a, b, sign = {0: (b11, b22, 1), 2: (b12, b22, -1), 3: (b21, b11, -1), 5: (b11, b12, 1), 6: (b21, b22, 1)}[k]
    a, b = _unpack(a(k)), _unpack(b(k))
    return (a + b if sign > 0 else a - b).astype(bf16)


def _softmax(s, allow, fill):
    s = jnp.where(allow, s * SCALE, fill)
    m = jnp.max(s, axis=-1, keepdims=True)
    e = jnp.exp(s - m)
    l = jnp.sum(e, axis=-1, keepdims=True)
    r = pl.reciprocal(l, approx=True)
    r = r * (2.0 - l * r)
    return (e * r).astype(bf16)


def _kernel(x_hbm, mem0_hbm, wq_hbm, wk_hbm, wv_hbm, wo_hbm, w1_hbm, w2_hbm, w3_hbm, w4_hbm,
            gw_hbm, out_hbm,
            x_v, s1_v, s2_v, s3_v, s4_v, wqkv_v, wo_v, h_v, b_v, c0_v, l_v, lf_v, n_v, g_v, out_v, xe_v, e_v, oe_v,
            ke_v, ve_v, o_v, mem_v, mem0_ref, gw_ref, zero_s,
            sem, sem_qkv, sem_out):
    RAW = (1, 2, 3, 4)
    RAW1 = (1, 7, 8, 4)

    loads = []

    def rows_load(name, r0, r1):
        loads.append((name, x_hbm.at[pl.ds(r0, r1 - r0)], x_v.at[pl.ds(r0, r1 - r0)]))

    def quad_load(name, w_hbm, s_v, raw, q, c0=0, c1=None):
        k4, n2 = s_v.shape[1], s_v.shape[2]
        c1 = n2 if c1 is None else c1
        src = w_hbm.bitcast(u32).at[pl.ds((q // 2) * k4, k4), pl.ds((q % 2) * n2 + c0, c1 - c0)]
        loads.append((name, src, s_v.at[raw[q], :, pl.ds(c0, c1 - c0)]))

    def w1_load(name, half, c0, c1):
        quad_load(name, w1_hbm, s1_v, RAW1, half, c0, c1)
        quad_load(name, w1_hbm, s1_v, RAW1, 2 + half, c0, c1)

    def block_load(name, w_hbm, s_v, r0, r1):
        kb, nb = s_v.shape[1:]
        for q in range(16):
            loads.append((name, w_hbm.at[pl.ds((q // 4) * kb + r0, r1 - r0), pl.ds((q % 4) * nb, nb)],
                          s_v.at[RAW16[q], pl.ds(r0, r1 - r0)]))

    rows_load("x0", 0, TM)
    w1_load("w1a", 0, 0, 256)
    rows_load("x1", TM, 2 * TM)
    w1_load("w1b", 0, 256, 512)
    w1_load("w1cd", 1, 0, 512)
    rows_load("x23", 2 * TM, 4 * TM)
    rows_load("x4567", 4 * TM, S)
    for q in range(4):
        quad_load("w2", w2_hbm, s2_v, RAW, q)
    block_load("w2", w3_hbm, s3_v, 0, W3A)
    block_load("w4", w3_hbm, s3_v, W3A, D4)
    block_load("w4", w4_hbm, s4_v, 0, F4)
    loads.append(("small", mem0_hbm, mem0_ref))
    loads.append(("small", gw_hbm, gw_ref))
    for j in range(NT):
        loads.append(("wo", wo_hbm.bitcast(u32).at[:, pl.ds(j * 128, 128)], wo_v.at[j]))
    groups = list(dict.fromkeys(name for name, _, _ in loads))
    assert len(groups) == NLOAD

    def start(*names, priority=0):
        for name, src, dst in loads:
            if name in names:
                pltpu.make_async_copy(src, dst, sem.at[groups.index(name)]).start(priority=priority)

    def wait(*names):
        for name, src, dst in loads:
            if name in names:
                pltpu.make_async_copy(src, dst, sem.at[groups.index(name)]).wait()

    SPG = 3 * G

    def qkv_start(g):
        for w, w_hbm in enumerate((wq_hbm, wk_hbm, wv_hbm)):
            wu = w_hbm.bitcast(u32)
            for k in range(G // 2):
                for par in range(2):
                    pltpu.make_async_copy(
                        wu.at[:, par * (H // 2) + g * (G // 2) + k, :],
                        wqkv_v.at[g * SPG + w * G + 2 * k + par], sem_qkv.at[g]).start(priority=1)

    def qkv_wait(g):
        grp = wqkv_v.at[pl.ds(g * SPG, SPG)]
        pltpu.make_async_copy(grp, grp, sem_qkv.at[g]).wait()

    start("x0", "w1a", "w1b", "x1", "w1cd", "x23", "x4567", "w2", "w4", "small")

    def zero(k, carry):
        zero_s[k] = 0
        return carry
    lax.fori_loop(0, RK, zero, 0)

    def once(fn):
        def body(_, carry):
            fn()
            return carry
        lax.fori_loop(0, 1 + zero_s[1], body, 0)

    def tile_idx(ref, cols=128):
        z = zero_s[0]
        n = 16 if ref.dtype == bf16 and cols == 128 else 8
        return (z,) * (len(ref.shape) - 2) + (pl.ds(pl.multiple_of(z, n), n), slice(0, cols))

    hist = []

    def mm(lhs, rhs, side=None, acc=None):
        if side is not None:
            lhs = side(lhs)
        lhs = pltpu.bitcast(lhs, bf16) if lhs.dtype == u32 else lhs.astype(bf16)
        y = _dot(lhs, pltpu.bitcast(rhs, bf16) if rhs.dtype == u32 else rhs)
        if acc is not None:
            y = y + acc
        hist.append(y)
        return y

    class Side:
        def __init__(self, pieces, n, skip=0):
            cap = [0] * skip + [1] * n
            tot = sum(p[4] for p in pieces)
            self.plan = [[] for _ in cap]
            done = 0
            for p in pieces:
                done += p[4]
                x, d = done / tot * sum(cap), 0
                while x > cap[d] + 1e-9:
                    x -= cap[d]
                    d += 1
                self.plan[d].append((p, x / cap[d]))
            self.pieces = len(pieces)

        def __call__(self, val):
            todo = self.plan.pop(0) if self.plan else []
            if not todo:
                return val
            self.pieces -= len(todo)
            never = zero_s[0] > 0
            if val.dtype == bf16:
                val = pltpu.bitcast(val, u32)
            rg = 8 if val.dtype == u32 else 16
            ng = val.shape[0] // rg
            tied = {}
            for (fn, rd, wr, lag, _), pos in todo:
                m = min(max(-int(-pos * ng // 1) - 1, 0), ng - 1)
                pin = lambda v, w=128: v
                if lag is not None and len(hist) >= lag:
                    r0 = (16 * m) % hist[-lag].shape[0]
                    a = hist[-lag][r0:r0 + 8, :128]
                    if rd is None:
                        def pin(v, w=128, a=a):
                            a = _cat([_cat([_as(a, v.dtype)] * (v.shape[0] // 8), 0)] * (w // 128), 1)
                            if v.shape[1] == w:
                                return lax.select(never, a, v)
                            return _cat([lax.select(never, a, v[:, :w]), v[:, w:]], 1)
                    elif rd.dtype == bf16:
                        idx = tile_idx(rd, 256)
                        rd[idx] = lax.select(never, _cat([a, a], 1).astype(bf16), rd[idx])
                    else:
                        idx = tile_idx(rd)
                        rd[idx] = lax.select(never, _as(a, rd.dtype), rd[idx])
                u = fn(pin)
                if wr is False:
                    continue
                if wr is not None:
                    u = wr[tile_idx(wr)]
                t, n = tied.get(m * rg) or (val[m * rg:m * rg + 8, -128:], 0)
                tied[m * rg] = (lax.select(zero_s[n] > 0, _as(u, val.dtype), t), n + 1)
            if not tied:
                return val
            col, r = [], 0
            for r0 in sorted(tied):
                col += ([val[r:r0, -128:]] if r0 > r else []) + [tied[r0][0]]
                r = r0 + 8
            col += [val[r:, -128:]] if r < val.shape[0] else []
            return _cat([val[:, :-128], _cat(col, 0)], 1) if val.shape[1] > 128 else _cat(col, 0)

    def strassen(lhs, rhs, side, init=(None, None, None, None)):
        def add(a, b):
            return a if b is None else a + b
        p = [mm(lhs(k), rhs(k), side) for k in range(5)]
        c12 = add(p[2] + p[4], init[1])
        c21 = add(p[1] + p[3], init[2])
        c22 = mm(lhs(5), rhs(5), side, add(p[0] - p[1] + p[2], init[3]))
        c11 = mm(lhs(6), rhs(6), side, add(p[0] + p[3] - p[4], init[0]))
        return c11, c12, c21, c22

    def fmm(lhs, rhs, side, extra=lambda n: None, emit=None):
        val = {}
        for n in WORDER:
            t = extra(n)
            for q, sg in sorted(_WPAR[n], key=lambda e: -e[1]):
                t = val[q] if t is None else (t + val[q] if sg > 0 else t - val[q])
            for r in range(RK):
                if WN[r] == n:
                    t = mm(lhs(UN[r]), rhs(r), side, t)
            val[n] = t
            if n < 8 and emit is not None:
                emit(n, t)
        return [val[v] for v in range(8)]

    def prep26_pieces(s_v, lag):
        def piece(rs, cs, pin):
            @functools.lru_cache(None)
            def node(n):
                if n < 16:
                    return s_v[RAW16[n], rs, cs].astype(f32)
                a, sa, b, sb = VP[n - 16]
                return _run([(0, sa, 1, sb)], [node(a), node(b)])[-1]
            vals = [node(VN[r]).astype(bf16) for r in VORDER]
            for r, t in zip(VORDER, vals):
                s_v[r, rs, cs] = t
        kb, nb = s_v.shape[1:]
        out = []
        for r in range(0, kb, 16):
            out += [(slice(rr, rr + 8), slice(c, c + 256)) for c in range(0, nb - 255, 256) for rr in (r, r + 8)]
            out += [(slice(rr, rr + 8), slice(nb - 128, nb)) for rr in (r, r + 8)] if nb % 256 else []
        return [(functools.partial(piece, rs, cs), s_v, s_v if n % 16 == 15 else False, lag,
                 130 if cs.stop - cs.start == 256 else 100) for n, (rs, cs) in enumerate(out)]

    def prep_pieces(s_v, raw, lag, width=256):
        def piece(r, c, pin):
            idx = (slice(r, r + 8), slice(c, c + width))
            b11, b12, b21, b22 = [_unpack(pin(s_v[(q,) + idx], width) if n in (0, 3) else s_v[(q,) + idx])
                                  for n, q in enumerate(raw)]
            for k, t in ((0, b11 + b22), (2, b12 - b22), (3, b21 - b11), (5, b11 + b12), (6, b21 + b22)):
                s_v[(k,) + idx] = _pack(t)
        return [(functools.partial(piece, r, c), None, s_v, lag, 80)
                for c in range(0, s_v.shape[2], width) for r in range(0, s_v.shape[1], 8)]

    def store_l(slot, q, c, quads):
        for k, t in enumerate(_lcombos(*quads)):
            l_v[slot, k, q // 2:q // 2 + 8, c:c + t.shape[1]] = _pack(t)

    def ln_pieces(src, r0, slot, lag, width=256, staged=False, clag=None):
        def stats(q, pin):
            x = pin(src[pl.ds(r0 + q, 16), :].astype(f32))
            xs = [x[:, j * 128:(j + 1) * 128] for j in range(NT)]
            m = functools.reduce(lambda a, b: a + b, xs) * (1.0 / NT)
            w = functools.reduce(lambda a, b: a + b, [(t - m) * (t - m) for t in xs])
            mean = jnp.mean(m, axis=-1, keepdims=True)
            var = jnp.sum(w + NT * ((m - mean) * (m - mean)), axis=-1, keepdims=True) * (1.0 / D)
            n_v[0, q:q + 16, :] = jnp.broadcast_to(mean, (16, 128))
            n_v[1, q:q + 16, :] = jnp.broadcast_to(lax.rsqrt(var + EPS), (16, 128))

        def comb(q, c, pin):
            quads = []
            for rr in (0, HM):
                rs = pl.ds(pl.multiple_of(r0 + rr + q + zero_s[0], 16), 16)
                mean, rstd = [jnp.concatenate([n_v[t, rr + q:rr + q + 16, :]] * (width // 128), axis=1)
                              for t in range(2)]
                quads += [(src[rs, cc + c:cc + c + width].astype(f32) - mean) * rstd for cc in (0, DH2)]
            store_l(slot, q, c, quads)

        def comb26(q, pin):
            blocks = []
            for rr in (0, HM):
                rs = pl.ds(pl.multiple_of(r0 + rr + q + zero_s[0], 8), 8)
                mean, rstd = [jnp.concatenate([n_v[t, rr + q:rr + q + 8, :]] * 2, axis=1) for t in range(2)]
                blocks += [(src[rs, cc:cc + D4] - mean) * rstd for cc in range(0, D, D4)]
            vals = _run(UP, blocks)
            for k, u in enumerate(UL):
                lf_v[k, q:q + 8, :] = vals[u].astype(bf16)
        dense = slot is not None or src is b_v
        norms = [[(functools.partial(stats, rr + q), None, n_v if dense else False, lag, 90) for rr in (0, HM)]
                 for q in range(0, HM, 16)]
        if slot is None:
            combs = [[(functools.partial(comb26, qq), n_v, lf_v if dense or qq % 32 == 24 else False, clag, 110)
                      for qq in (q, q + 8)] for q in range(0, HM, 16)]
        else:
            combs = [[(functools.partial(comb, q, c), n_v, l_v, clag, 125) for c in range(0, DH2, width)]
                     for q in range(0, HM, 16)]
        if staged:
            return sum(norms, []), sum(combs, [])
        out = list(norms[0])
        for a, b in zip(norms[1:] + [[]], combs):
            out += _merge(a, b) if a else b
        return out

    shifts = (1, 1, -1, -1, 2, 2, -2, -2)

    def shift_pieces(r0, slot, lag, by_value=False):
        def piece(q, j, pin):
            a = [h_v[jj, pl.ds(PAD + r0 + rr + q - shifts[jj], 16), :]
                 for rr in (0, HM) for jj in (j, j + NT // 2)]
            store_l(slot, q, j * 128, [pin(a[0]), a[1], a[2], pin(a[3])])
        return [(functools.partial(piece, q, j), None if by_value else h_v,
                 l_v if (q // 16) % 2 and j == 3 else False, lag, 50)
                for q in range(0, HM, 16) for j in range(NT // 2)]

    def lhs_of(slot):
        return lambda k: l_v[slot, k]

    xe_v[0, 0:16, :] = jnp.zeros((16, D4), bf16)
    h_v[:, 0:PAD, :] = jnp.zeros((NT, PAD, 128), f32)
    h_v[:, PAD + S:PAD + S + PAD, :] = jnp.zeros((NT, PAD, 128), f32)

    def store_h(r0, c0, h):
        for j in range(h.shape[1] // 128):
            h_v[c0 // 128 + j, PAD + r0:PAD + r0 + h.shape[0], :] = h[:, j * 128:(j + 1) * 128]

    def h_pieces(r0, c0, t, lag, n=4):
        def piece(r, pin):
            store_h(r0 + r, c0, _gelu(pin(t[r:r + 8 * n])))
        return [(functools.partial(piece, r), None, h_v, lag, 10 * n) for r in range(0, t.shape[0], 8 * n)]

    def flush(pieces):
        for p in pieces:
            p[0](lambda v, w=128: v)

    def w1_cols(c, step):
        half, cc = c // DH2, c % DH2
        return jnp.concatenate([s1_v[RAW1[half], :, cc:cc + step], s1_v[RAW1[2 + half], :, cc:cc + step]], axis=0)

    def d1_plain(xn, r0, c0, c1, step):
        for c in range(c0, c1, step):
            store_h(r0, c, _gelu(mm(xn, w1_cols(c, step))))

    def d1_fine(lhs, r0, nrb, cols, pieces, carry, skip=0):
        tiles = [(rb, c) for c in cols for rb in range(nrb)]
        rounds = [tiles[i:i + 4] for i in range(0, len(tiles), 4)]
        for n, (rnd, part) in enumerate(zip(rounds, split(pieces, len(rounds)))):
            sk = skip if n == 0 else 0
            side = Side(_merge(carry, part) if carry else part, 8 - sk, sk)
            carry = []
            for rb, c in rnd:
                half, cc = c // DH2, c % DH2
                t = mm(lhs(rb, 0), s1_v[RAW1[half], :, cc:cc + 128], side)
                t = mm(lhs(rb, 1), s1_v[RAW1[2 + half], :, cc:cc + 128], side, t)
                carry += h_pieces(r0 + rb * HM, c, t, LS)
        return carry

    def d1_s(b, slot, pieces, carry, early=()):
        for c, part, e in zip(range(0, DH2, NC1), split(pieces, DH2 // NC1), split(early, 2) + [[], []]):
            side = Side(merge(carry, part, e), *((7,) if hist else (5, 2)))
            cs = strassen(lhs_of(slot), lambda k: s1_v[k, :, c:c + NC1], side)
            carry = sum([h_pieces(b * TM + (q // 2) * HM, (q % 2) * DH2 + c, cs[q], LS) for q in (1, 2, 3, 0)], [])
        return carry

    def d2_s(b, slot, pieces, carry=(), early=(), late=()):
        for c, part, e in zip(range(0, DH2, NC1), split(pieces, DH2 // NC1), split(early, 2) + split(late, 2)):
            side = Side(merge(carry, part, e), *((7,) if hist else (5, 2)))
            carry = ()
            idx = [(slice(b * TM + (q // 2) * HM, b * TM + (q // 2 + 1) * HM),
                    slice((q % 2) * DH2 + c, (q % 2) * DH2 + c + NC1)) for q in range(4)]
            cs = strassen(lhs_of(slot), lambda k: s2_v[k, :, c:c + NC1], side,
                          [x_v[i].astype(f32) for i in idx])
            for i, t in zip(idx, cs):
                b_v[i] = t
                if b == 0:
                    c0_v[i] = t

    def split(l, n):
        w = [1.0 if hist else 0.6] + [1.0] * (n - 1)
        cut = [int(round(len(l) * sum(w[:i]) / sum(w))) for i in range(n + 1)]
        return [l[cut[i]:cut[i + 1]] for i in range(n)]

    def merge(*ls):
        ls = [l for l in ls if l]
        return _merge(*ls) if ls else []

    NW1, NW3, N30 = 52, 32, 20
    LS, LL = 3, 5

    p3 = prep26_pieces(s3_v, LS)
    n3 = len(p3) * W3A // D4

    @once
    def _phase1a():
        wait("x0")
        xn0 = _pack(_ln(x_v[0:TM, :].astype(f32)))
        wait("w1a")
        d1_plain(xn0, 0, 0, 256, 256)
        wait("x1")
        xn1 = [_pack(_ln(x_v[r:r + HM, :].astype(f32))) for r in (TM, TM + HM)]
        for n in range(2):
            d1_plain(xn1[n], TM + n * HM, 0, 256, 256)
        wait("w1b")
        d1_plain(jnp.concatenate([xn0] + xn1, axis=0), 0, 256, 512, 256)
        wait("w1cd")
        hist.clear()
        xn01 = jnp.concatenate([xn0] + xn1, axis=0)
        l01 = lambda rb, kh: xn01[rb * 64:(rb + 1) * 64, kh * DH2:(kh + 1) * DH2]
        pw = prep_pieces(s1_v, RAW1, LS)
        flush(d1_fine(l01, 0, 4, (512, 640), pw[:NW1], [], 1))
        carry = []
        wait("x23")
        hist.clear()
        carry = d1_fine(l01, 0, 4, (768, 896), ln_pieces(x_v, 2 * TM, 0, LL), carry, 3)
        carry = d1_s(2, 0, ln_pieces(x_v, 3 * TM, 1, LL), carry, pw[NW1:])
        wait("x4567")
        qkv_start(0)
        qkv_start(1)
        hist.clear()
        for b in range(3, NB - 1):
            carry = d1_s(b, b % 2, ln_pieces(x_v, (b + 1) * TM, (b + 1) % 2, LL), carry)
        wait("w2")
        hist.clear()
        pw = prep_pieces(s2_v, RAW, LS)
        carry = d1_s(7, 1, _merge(pw[:NW3], shift_pieces(0, 0, LS, True)), carry)
        d2_s(0, 0, shift_pieces(TM, 1, LS, True), carry, pw[NW3:], p3[:N30])
        pw = split(_merge(p3[N30:n3], sum(ln_pieces(c0_v, 0, None, LL, clag=LS, staged=True), [])), 3)
        for b in range(1, 4):
            d2_s(b, b % 2, _merge(pw[b - 1], shift_pieces((b + 1) * TM, (b + 1) % 2, LS)))
        wait("w4", "small")

    hist.clear()
    pw = p3[n3:] + prep26_pieces(s4_v, LS)
    cut = (0, 33, 68, 103, len(pw))
    for b in range(4, NB):
        d2_s(b, b % 2, merge(pw[cut[b - 4]:cut[b - 3]],
                             shift_pieces((b + 1) * TM, (b + 1) % 2, LS) if b + 1 < NB else ()))
    start("wo", priority=1)

    def ffn(i, carry):
        qkv_wait(i)
        r0 = pl.multiple_of(i * TM, TM)
        rn = pl.multiple_of(jnp.minimum(i + 1, NB - 1) * TM, TM)
        acc = {}
        hist.clear()

        def relayout(p, r0_, r1_, pin):
            s0 = i * SPG + 2 * p
            e = wqkv_v[s0, r0_:r1_, :]
            o = wqkv_v[s0 + 1, r0_:r1_, :]
            wqkv_v[s0, r0_:r1_, :] = (e & jnp.uint32(0xFFFF)) | (o << 16)
            wqkv_v[s0 + 1, r0_:r1_, :] = (e >> 16) | (o & jnp.uint32(0xFFFF0000))

        relays = [(functools.partial(relayout, p, r, r + 32), wqkv_v, wqkv_v, 3, 35)
                  for p in range(SPG // 2) for r in range(0, D // 2, 32)]
        norms, combs = ln_pieces(b_v, rn, None, 5, staged=True, clag=3)

        def gate(q, pin):
            gw = gw_ref[...].astype(f32)
            x = pin(x_v[pl.ds(r0 + q, 16), :].astype(f32))
            t = functools.reduce(lambda a, b: a + b,
                                 [x[:, j * 128:(j + 1) * 128] * gw[j:j + 1, :] for j in range(NT)])
            g = jax.nn.sigmoid(jnp.sum(t, axis=-1, keepdims=True))
            g_v[pl.ds(r0 + q, 16), :] = jnp.broadcast_to(g, (16, 128))

        gates = [(functools.partial(gate, q), None, g_v, 5, 90) for q in range(0, TM, 16)]

        def extras(t, pin):
            jj, o = 2 * i + t // 2, 24 + 8 * (t % 2)
            xs = [pin(x_v[pl.ds(pl.multiple_of((jj + hh) * 64 + o, 8), 8), :].astype(f32)) for hh in (0, NPAIR // 2)]
            vals = _run(UP, [x[:, cc:cc + D4] for x in xs for cc in range(0, D, D4)])
            for k, u in enumerate(UL):
                xe_v[k, pl.ds(pl.multiple_of(i * 32 + t * 8, 8), 8), :] = vals[u].astype(bf16)

        xes = [(functools.partial(extras, t), None, xe_v, 3, 100) for t in range(4)]
        hs = {}

        def gelu_pieces(c, cs):
            def piece(r, cc, vs, pin):
                t = _gelu(pin(_cat([cs[v][r:r + 8, cc:cc + 128] for v in vs], 0)))
                ts = [t[8 * n:8 * n + 8] for n in range(len(vs))]
                hs.update({(c, v, r, cc): u for v, u in zip(vs, ts)})
                return functools.reduce(lambda a, b: a + b, ts)
            return [(functools.partial(piece, r, cc, vs), None, None, 3, 40) for r in range(0, HM, 8)
                    for cc in range(0, cs[0].shape[1], 128) for vs in ((0, 1, 2, 3), (4, 5, 6, 7))]

        def d3(c, side):
            c0, c1 = FCH[c]
            cs = fmm(lambda u: lf_v[UL.index(u)], lambda r: s3_v[r, :, c0:c1], side)
            assert not side.pieces
            return gelu_pieces(c, cs)

        def d4(c, side):
            c0, c1 = FCH[c]
            lh = _run(UP, [_cat([_cat([hs.pop((c, v, r, cc)) for r in range(0, HM, 8)], 0)
                                 for cc in range(0, c1 - c0, 128)], 1) for v in range(8)])
            rhs = lambda r: s4_v[r, c0:c1, :]
            if c + 1 < len(FCH):
                for n in WORDER:
                    for r in range(RK):
                        if WN[r] == n:
                            acc[n] = mm(lh[UN[r]], rhs(r), side, acc.get(n))
            else:
                idx = lambda v: (pl.ds(r0 + (v // 4) * HM, HM), slice((v % 4) * D4, (v % 4 + 1) * D4))

                def extra(n):
                    if n >= 8:
                        return acc.get(n)
                    return b_v[idx(n)] + acc[n] if n in acc else b_v[idx(n)]

                def emit_b(v, t):
                    b_v[idx(v)] = jnp.concatenate([1.0 - g_v[idx(v)[0], :]] * 2, axis=1) * t
                fmm(lambda u: lh[u], rhs, side, extra, emit_b)
            assert not side.pieces

        g0 = d3(0, Side(relays[:20], 23, 3))
        g1 = d3(1, Side(_merge(g0, gates, xes), 23, 2))
        d4(0, Side(g1[:22], 22, 4))
        g2 = d3(2, Side(_merge(g1[22:], relays[20:40]), 25))
        d4(1, Side(g2, 23, 2))
        g3 = d3(3, Side(_merge(relays[40:], norms), 26))
        d4(2, Side(_merge(g3, combs), 23, 2))
        d4(3, Side([], 1))

        @pl.when(i + 2 < NG)
        def _():
            qkv_start(i + 2)

        return carry

    lax.fori_loop(0, NB, ffn, 0)

    def pre(it, carry):
        hist.clear()
        for u in range(3 * NG // NPRE):
            s0 = (it * (3 * NG // NPRE) + u) * G

            def rhs(r):
                t = None
                sz = s0 + zero_s[r]
                for q, sg in sorted(_terms(VP, 16, VN[r]).items(), key=lambda e: -e[1]):
                    blk = wqkv_v[sz + q % 4, (q // 4) * (D // 8):(q // 4 + 1) * (D // 8), :]
                    if VN[r] < 16:
                        return blk
                    blk = _unpack(blk)
                    t = blk if t is None else (t + blk if sg > 0 else t - blk)
                return t.astype(bf16)
            for v, t in enumerate(fmm(lambda k: xe_v[UL.index(k)], rhs, None)):
                e_v[(v // 4) * 16:(v // 4 + 1) * 16, s0 + v % 4] = _pack(t).reshape(16, 8, DH)
        return carry

    lax.fori_loop(0, NPRE, pre, 0)

    wait("wo")
    mem_v[...] = mem0_ref[...].astype(f32)

    def slab(w, h):
        return (h // G) * SPG + w * G + h % G

    def step(j, hx, odd, late, allow, fill):
        qs, ks, vs, ps = {}, {}, {}, {}
        wload = lambda w, h: pltpu.bitcast(wqkv_v[slab(w, h)], bf16)
        eload = lambda w, h: pltpu.bitcast(e_v[j, slab(w, h)], bf16)

        def proj(g):
            part = {}
            if late and g == 0:
                for h in range(2):
                    for w in range(3):
                        part[w, h] = _dot(hx[:, :DH2], wload(w, h)[:DH2])
            for h in range(g * G, (g + 1) * G):
                q, k, v = [(_dot(hx[:, DH2:], wload(w, h)[DH2:]) + part[w, h] if (w, h) in part
                            else _dot(hx, wload(w, h))).astype(bf16) for w in range(3)]
                if odd:
                    q = jnp.concatenate([q, eload(0, h)], axis=0)
                    k = jnp.concatenate([pltpu.bitcast(ke_v[h], bf16), eload(1, h), k], axis=0)
                    v = jnp.concatenate([pltpu.bitcast(ve_v[h], bf16), eload(2, h), v], axis=0)
                else:
                    ke_v[h] = pltpu.bitcast(k, u32)
                    ve_v[h] = pltpu.bitcast(v, u32)
                    k = jnp.concatenate([k, eload(1, h)], axis=0)
                    v = jnp.concatenate([v, eload(2, h)], axis=0)
                qs[h], ks[h], vs[h] = q, k, v

        def score(g):
            for h in range(g * G, (g + 1) * G):
                s = lax.dot_general(qs.pop(h), ks.pop(h), (((1,), (1,)), ((), ())),
                                    preferred_element_type=f32)
                ps[h] = _softmax(s, allow, fill)

        def pv(g):
            os_ = []
            for h in range(g * G, (g + 1) * G):
                o = _dot(ps.pop(h), vs.pop(h))
                o_v[:, h * 128:(h + 1) * 128] = _pack(o[:32])
                os_.append(o)
            if odd:
                quads = [jnp.concatenate([os_[2 * kk][r:r + 8], os_[2 * kk + 1][r:r + 8]], axis=1)
                         for r in (32, 40) for kk in range(2)]
                for k, t in enumerate(_lcombos(*quads)):
                    oe_v[k, pl.ds(pl.multiple_of(j * 8, 8), 8), g * 256:(g + 1) * 256] = t.astype(bf16)

        acc = [None] * NT

        def wo(h0, h1, j0, j1):
            o = pltpu.bitcast(o_v[:, h0 * 128:h1 * 128], bf16)
            for n in range(j0, j1):
                y = _dot(o, pltpu.bitcast(wo_v[n, h0 * 64:h1 * 64, :], bf16))
                acc[n] = y if acc[n] is None else y + acc[n]

        for t in range(NG):
            proj(t)
            if t >= 2:
                pv(t - 2)
            if t >= 1:
                score(t - 1)
        wo(0, 16, 0, 4)
        pv(NG - 2)
        score(NG - 1)
        wo(0, 16, 4, 8)
        pv(NG - 1)
        wo(16, 24, 0, 8)
        wo(24, 32, 0, 8)
        return jnp.concatenate(acc, axis=1)

    def emit(j, r0, o0, a):
        rs = pl.ds(r0 + o0, 24)
        g = jnp.concatenate([g_v[rs, :]] * NT, axis=1)
        out_v[j, o0:o0 + 24, :] = (g * a + b_v[rs, :]).astype(bf16)

    def pair(j, mem, late):
        r0 = pl.multiple_of(j * 64, 64)
        allow_e, fill_e, allow_o, fill_o = _masks()
        xa = x_v[pl.ds(r0 + 16, 8), :].astype(f32)
        xb = x_v[pl.ds(r0 + 40, 8), :].astype(f32)
        hx = jnp.concatenate([x_v[pl.ds(r0, 16), :], jnp.concatenate([xa, mem], 0).astype(bf16)], 0)
        oe = step(j, hx, False, late, allow_e, fill_e)
        emit(j, r0, 0, oe[:24])
        hx = jnp.concatenate([jnp.concatenate([oe[24:32], xb], 0).astype(bf16), x_v[pl.ds(r0 + 48, 16), :]], 0)
        oo = step(j, hx, True, True, allow_o, fill_o)
        emit(j, r0, 40, oo[8:])
        return oo[:8]

    def a_iter(it, carry):
        mem = mem_v[...]
        for t in range(PPI):
            mem = pair(it * PPI + t, mem, t > 0)
        mem_v[...] = mem
        for t in range(PPI):
            for o0 in (0, 40):
                idx = (it * PPI + t, pl.ds(o0, 24))
                pltpu.make_async_copy(out_v.at[idx], out_hbm.at[idx], sem_out).start()
        return carry

    lax.fori_loop(0, NPAIR // PPI, a_iter, 0)

    @once
    def _post():
        hist.clear()
        for n in range(NT // 2):
            quad = [lambda k, t=2 * n + q % 2, o=(q // 2) * 128: jnp.concatenate(
                [wo_v[t + zero_s[k], g * 256 + o:g * 256 + o + 128, :] for g in range(NG)], axis=0) for q in range(4)]
            cs = strassen(lambda k: oe_v[k], lambda k: _rcombo(k, *quad), None)
            cols = slice(n * 256, (n + 1) * 256)
            for half in range(2):
                t = jnp.concatenate(cs[2 * half:2 * half + 2], axis=1)
                o0 = 24 + half * 8
                for jj in range(NPAIR):
                    rs = slice(jj * 64 + o0, jj * 64 + o0 + 8)
                    g = jnp.concatenate([g_v[rs, :]] * 2, axis=1)
                    out_v[jj, o0:o0 + 8, cols] = (g * t[jj * 8:jj * 8 + 8] + b_v[rs, cols]).astype(bf16)
            if n >= 2:
                idx = (slice(None), pl.ds(24, 16), pl.ds(0, 768) if n == 2 else pl.ds(768, 256))
                pltpu.make_async_copy(out_v.at[idx], out_hbm.at[idx], sem_out).start()

    pltpu.make_async_copy(out_v, out_hbm, sem_out).wait()


@jax.jit
def pallas_gated_mix__memory_aug_recurrent_mem_tr__mixer_s_mlp__prompt_kernel(
    A_x, A_mem0, A_Wq, A_Wk, A_Wv, A_Wo, A_seg_len, B_x, B_w1, B_w2, B_w3, B_w4, gate_w,
):
    assert A_x.shape == (1, S, D) and A_mem0.shape == (1, M, D)
    any_spec = pl.BlockSpec(memory_space=pl.ANY)
    out = pl.pallas_call(
        _kernel,
        out_shape=jax.ShapeDtypeStruct((NPAIR, 64, D), bf16),
        in_specs=[any_spec] * 11,
        out_specs=any_spec,
        scratch_shapes=[
            pltpu.VMEM((S, D), bf16),
            pltpu.VMEM((9, D // 4, D // 2), u32),
            pltpu.VMEM((7, D // 4, D // 2), u32),
            pltpu.VMEM((RK, D4, F4), bf16),
            pltpu.VMEM((RK, F4, D4), bf16),
            pltpu.VMEM((3 * H, D // 2, DH), u32),
            pltpu.VMEM((NT, H * DH // 2, 128), u32),
            pltpu.VMEM((NT, S + 2 * PAD, 128), f32),
            pltpu.VMEM((S, D), f32),
            pltpu.VMEM((TM, D), f32),
            pltpu.VMEM((2, 7, HM // 2, D // 2), u32),
            pltpu.VMEM((len(UL), HM, D4), bf16),
            pltpu.VMEM((2, TM, 128), f32),
            pltpu.VMEM((S, 128), f32),
            pltpu.VMEM((NPAIR, 64, D), bf16),
            pltpu.VMEM((len(UL), 8 * NPAIR, D4), bf16),
            pltpu.VMEM((NPAIR, 3 * H, 8, DH), u32),
            pltpu.VMEM((7, 8 * NPAIR, H * DH // 2), bf16),
            pltpu.VMEM((H, 16, 128), u32),
            pltpu.VMEM((H, 16, 128), u32),
            pltpu.VMEM((16, H * DH), u32),
            pltpu.VMEM((M, D), f32),
            pltpu.VMEM((M, D), bf16),
            pltpu.VMEM((NT, 128), bf16),
            pltpu.SMEM((RK,), jnp.int32),
            pltpu.SemaphoreType.DMA((NLOAD,)),
            pltpu.SemaphoreType.DMA((NG,)),
            pltpu.SemaphoreType.DMA,
        ],
        compiler_params=pltpu.CompilerParams(vmem_limit_bytes=126 * 1024 * 1024,
                                             disable_bounds_checks=True),
    )(
        A_x.reshape(S, D), A_mem0.reshape(M, D),
        A_Wq.reshape(D // 2, 2 * H, DH), A_Wk.reshape(D // 2, 2 * H, DH), A_Wv.reshape(D // 2, 2 * H, DH),
        A_Wo.reshape(H * DH, D), B_w1, B_w2, B_w3, B_w4, gate_w.reshape(NT, 128),
    )
    return out.reshape(1, S, D)
```

```python
import functools

import jax
import jax.numpy as jnp
from jax import lax
import jax.experimental.pallas as pl
import jax.experimental.pallas.tpu as pltpu

f32, bf16, u32 = jnp.float32, jnp.bfloat16, jnp.uint32

S, D, H, DH, M, SEG, F = 2048, 1024, 32, 128, 8, 32, 3584
SCALE = DH ** -0.5
NEG = -1000000000.0
EPS = 1e-05

TM = 256
NB = S // TM
HM = TM // 2
DH2 = D // 2
D4, F4 = D // 4, F // 4
FCH = ((0, 128), (128, 384), (384, 640), (640, 896))
NC1 = 128
NPAIR = S // (2 * SEG)
PPI = 2
NPRE = 3
G = 4
NG = H // G
PAD = 8
NT = D // 128
W3A = 192
NLOAD = 11
assert NB == NG

_dot = functools.partial(jnp.dot, preferred_element_type=f32)

UP = ((4, 1, 5, 1), (6, 1, 8, 1), (0, 1, 3, 1), (2, -1, 9, 1), (4, -1, 10, 1), (0, 1, 1, 1), (2, 1, 12, 1),
      (5, 1, 7, -1), (7, 1, 12, -1), (11, -1, 13, 1), (10, -1, 11, 1), (2, 1, 7, 1), (0, -1, 4, 1),
      (6, 1, 7, 1), (1, -1, 5, 1), (3, 1, 7, -1), (1, 1, 4, 1), (2, 1, 3, 1), (1, -1, 3, 1), (1, 1, 7, -1),
      (2, 1, 6, -1))
WP = ((0, -1, 3, 1), (4, 1, 6, -1), (1, 1, 8, 1), (5, 1, 10, 1), (4, -1, 7, 1), (0, -1, 9, -1),
      (11, 1, 12, 1), (6, 1, 7, -1), (2, 1, 5, -1), (0, -1, 7, -1), (9, 1, 11, -1), (2, 1, 13, 1),
      (5, 1, 13, 1), (2, -1, 3, 1), (5, 1, 6, 1), (0, 1, 4, 1), (2, 1, 7, 1), (1, 1, 2, 1), (1, 1, 5, 1),
      (3, 1, 7, 1), (2, 1, 6, 1))
VP = ((1, 1, 5, -1), (8, 1, 11, 1), (10, 1, 17, 1), (13, 1, 16, -1), (0, 1, 4, -1), (0, 1, 3, 1),
      (14, 1, 18, -1), (0, 1, 11, 1), (14, 1, 19, -1), (0, 1, 5, 1), (12, 1, 15, 1), (2, 1, 21, 1),
      (10, 1, 14, -1), (4, 1, 7, 1), (11, 1, 19, 1), (12, -1, 20, 1), (13, 1, 14, -1), (9, 1, 30, -1),
      (3, -1, 15, 1), (6, 1, 23, 1), (24, 1, 27, -1), (9, -1, 18, 1), (7, 1, 34, 1), (2, 1, 6, -1),
      (0, 1, 8, -1), (6, 1, 21, 1), (22, 1, 31, -1), (6, 1, 29, 1), (0, 1, 1, 1), (15, 1, 25, 1),
      (5, 1, 37, 1), (15, 1, 20, 1))
UN = (7, 27, 24, 17, 9, 22, 21, 2, 15, 11, 8, 25, 19, 28, 2, 23, 26, 20, 1, 18, 10, 28, 4, 13, 14, 16)
WN = (23, 17, 24, 10, 14, 7, 22, 19, 12, 18, 15, 25, 20, 5, 26, 0, 8, 2, 27, 11, 26, 9, 28, 21, 16, 5)
VN = (42, 47, 41, 5, 11, 43, 18, 28, 20, 23, 35, 19, 22, 46, 33, 26, 45, 36, 38, 25, 44, 40, 39, 21, 24, 32)
RK = len(UN)
UL = tuple(sorted(set(UN)))
RAW16 = (1, 11, 17, 5, 8, 3, 9, 10, 0, 6, 7, 4, 12, 20, 22, 16)
VORDER = (0, 6, 7, 12, 13, 14, 15, 21, 11, 17, 20, 22, 24, 25, 23, 2, 1, 5, 8, 9, 10, 16, 18, 19)
assert sorted(VORDER) == [r for r in range(RK) if VN[r] >= 16] and len(set(RAW16)) == 16
assert all(RAW16[VN[r]] == r for r in range(RK) if VN[r] < 16)


def _run(prog, blocks):
    vals = list(blocks)
    for a, sa, b, sb in prog:
        vals.append(vals[a] + vals[b] if sa > 0 and sb > 0 else
                    vals[a] - vals[b] if sa > 0 else vals[b] - vals[a])
    return vals


def _terms(prog, nin, node):
    if node < nin:
        return {node: 1}
    a, sa, b, sb = prog[node - nin]
    out = {k: sa * v for k, v in _terms(prog, nin, a).items()}
    out.update({k: sb * v for k, v in _terms(prog, nin, b).items()})
    return out


def _scheme_is_exact():
    t = {}
    for r in range(RK):
        for a, ca in _terms(UP, 8, UN[r]).items():
            for b, cb in _terms(VP, 16, VN[r]).items():
                for c, cc in _terms(WP, 8, WN[r]).items():
                    t[a, b, c] = t.get((a, b, c), 0) + ca * cb * cc
    want = {(4 * i + j, 4 * j + l, 4 * i + l): 1 for i in range(2) for j in range(4) for l in range(4)}
    return {k: v for k, v in t.items() if v} == want


assert _scheme_is_exact()

_WPAR = {n: [] for n in range(8 + len(WP))}
for _t, (_a, _sa, _b, _sb) in enumerate(WP):
    _WPAR[_a].append((8 + _t, _sa))
    _WPAR[_b].append((8 + _t, _sb))


def _worder():
    order = []

    def closure(n, acc):
        if n not in acc and n not in order:
            acc.add(n)
            for q, _ in _WPAR[n]:
                closure(q, acc)
        return acc

    def visit(n):
        if n not in order:
            for q, _ in _WPAR[n]:
                visit(q)
            order.append(n)
    while len([v for v in range(8) if v not in order]):
        visit(min((v for v in range(8) if v not in order), key=lambda v: len(closure(v, set()))))
    return tuple(order)


WORDER = _worder()


def _ln(x):
    m = jnp.mean(x, axis=-1, keepdims=True)
    xc = x - m
    v = jnp.mean(xc * xc, axis=-1, keepdims=True)
    return xc * lax.rsqrt(v + EPS)


_GC = 0.7978845608028654


def _gelu(x):
    h = 0.5 * x
    return h + h * jnp.tanh(x * (_GC + (_GC * 0.044715) * (x * x)))


def _unpack(u):
    return pltpu.bitcast(u, bf16).astype(f32)


def _pack(x):
    return pltpu.bitcast(x.astype(bf16), u32)


def _cat(xs, axis):
    xs = [x for x in xs if x.shape[axis]]
    return xs[0] if len(xs) == 1 else jnp.concatenate(xs, axis=axis)


def _as(x, dtype):
    return x if x.dtype == dtype else pltpu.bitcast(x, dtype)


def _lcombos(a11, a12, a21, a22):
    return [a11 + a22, a21 + a22, a11, a22, a11 + a12, a21 - a11, a12 - a22]


def _merge(*lists):
    keyed = [((j + 0.5) / len(l), n, j, v) for n, l in enumerate(lists) for j, v in enumerate(l)]
    return [v for _, _, _, v in sorted(keyed, key=lambda t: t[:3])]


def _masks():
    r = lax.broadcasted_iota(jnp.int32, (32, 48), 0)
    c = lax.broadcasted_iota(jnp.int32, (32, 48), 1)
    exist_e = c < 40
    allow_e = exist_e & ((r >= 24) | ((c >= 24) & (c < 32)) | (c <= r))
    fill_e = jnp.where(exist_e, NEG, -jnp.inf).astype(f32)
    r = lax.broadcasted_iota(jnp.int32, (48, 80), 0)
    c = lax.broadcasted_iota(jnp.int32, (48, 80), 1)
    q_even = (r >= 32) & (r < 40)
    exist_o = (q_even & (c < 40)) | (~q_even & (c >= 40))
    ktok = jnp.where(c < 24, c, jnp.where(c < 48, c - 8, c - 16))
    qtok = jnp.where(r < 32, r + 32, r - 8)
    is_mem_key = ((c >= 24) & (c < 32)) | ((c >= 48) & (c < 56))
    allow_o = exist_o & (is_mem_key | (r < 8) | (ktok <= qtok))
    fill_o = jnp.where(exist_o, NEG, -jnp.inf).astype(f32)
    return allow_e, fill_e, allow_o, fill_o


def _rcombo(k, b11, b12, b21, b22):
    if k in (1, 4):
        return (b11 if k == 1 else b22)(k)
    a, b, sign = {0: (b11, b22, 1), 2: (b12, b22, -1), 3: (b21, b11, -1), 5: (b11, b12, 1), 6: (b21, b22, 1)}[k]
    a, b = _unpack(a(k)), _unpack(b(k))
    return (a + b if sign > 0 else a - b).astype(bf16)


def _softmax(s, allow, fill):
    s = jnp.where(allow, s * SCALE, fill)
    m = jnp.max(s, axis=-1, keepdims=True)
    e = jnp.exp(s - m)
    l = jnp.sum(e, axis=-1, keepdims=True)
    r = pl.reciprocal(l, approx=True)
    r = r * (2.0 - l * r)
    return (e * r).astype(bf16)


def _kernel(x_hbm, mem0_hbm, wq_hbm, wk_hbm, wv_hbm, wo_hbm, w1_hbm, w2_hbm, w3_hbm, w4_hbm,
            gw_hbm, out_hbm,
            x_v, s1_v, s2_v, s3_v, s4_v, wqkv_v, wo_v, h_v, b_v, c0_v, l_v, lf_v, n_v, g_v, out_v, xe_v, e_v, oe_v,
            ke_v, ve_v, o_v, mem_v, mem0_ref, gw_ref, zero_s,
            sem, sem_qkv, sem_out):
    RAW = (1, 2, 3, 4)
    RAW1 = (1, 7, 8, 4)

    loads = []

    def rows_load(name, r0, r1):
        loads.append((name, x_hbm.at[pl.ds(r0, r1 - r0)], x_v.at[pl.ds(r0, r1 - r0)]))

    def quad_load(name, w_hbm, s_v, raw, q, c0=0, c1=None):
        k4, n2 = s_v.shape[1], s_v.shape[2]
        c1 = n2 if c1 is None else c1
        src = w_hbm.bitcast(u32).at[pl.ds((q // 2) * k4, k4), pl.ds((q % 2) * n2 + c0, c1 - c0)]
        loads.append((name, src, s_v.at[raw[q], :, pl.ds(c0, c1 - c0)]))

    def w1_load(name, half, c0, c1):
        quad_load(name, w1_hbm, s1_v, RAW1, half, c0, c1)
        quad_load(name, w1_hbm, s1_v, RAW1, 2 + half, c0, c1)

    def block_load(name, w_hbm, s_v, r0, r1):
        kb, nb = s_v.shape[1] // 128 * 128, s_v.shape[2]
        for q in range(16):
            loads.append((name, w_hbm.at[pl.ds((q // 4) * kb + r0, r1 - r0), pl.ds((q % 4) * nb, nb)],
                          s_v.at[RAW16[q], pl.ds(r0, r1 - r0)]))

    rows_load("x0", 0, TM)
    w1_load("w1a", 0, 0, 256)
    rows_load("x1", TM, 2 * TM)
    w1_load("w1b", 0, 256, 512)
    w1_load("w1cd", 1, 0, 512)
    rows_load("x23", 2 * TM, 4 * TM)
    rows_load("x4567", 4 * TM, S)
    for q in range(4):
        quad_load("w2", w2_hbm, s2_v, RAW, q)
    block_load("w2", w3_hbm, s3_v, 0, W3A)
    block_load("w4", w3_hbm, s3_v, W3A, D4)
    block_load("w4", w4_hbm, s4_v, 0, F4)
    loads.append(("small", mem0_hbm, mem0_ref))
    loads.append(("small", gw_hbm, gw_ref))
    for j in range(NT):
        loads.append(("wo", wo_hbm.bitcast(u32).at[:, pl.ds(j * 128, 128)], wo_v.at[j]))
    groups = list(dict.fromkeys(name for name, _, _ in loads))
    assert len(groups) == NLOAD

    def start(*names, priority=0):
        for name, src, dst in loads:
            if name in names:
                pltpu.make_async_copy(src, dst, sem.at[groups.index(name)]).start(priority=priority)

    def wait(*names):
        for name, src, dst in loads:
            if name in names:
                pltpu.make_async_copy(src, dst, sem.at[groups.index(name)]).wait()

    SPG = 3 * G

    def qkv_start(g):
        for w, w_hbm in enumerate((wq_hbm, wk_hbm, wv_hbm)):
            wu = w_hbm.bitcast(u32)
            for k in range(G // 2):
                for par in range(2):
                    pltpu.make_async_copy(
                        wu.at[:, par * (H // 2) + g * (G // 2) + k, :],
                        wqkv_v.at[g * SPG + w * G + 2 * k + par], sem_qkv.at[g]).start(priority=1)

    def qkv_wait(g):
        grp = wqkv_v.at[pl.ds(g * SPG, SPG)]
        pltpu.make_async_copy(grp, grp, sem_qkv.at[g]).wait()

    start("x0", "w1a", "w1b", "x1", "w1cd", "x23", "x4567", "w2", "w4", "small")

    def zero(k, carry):
        zero_s[k] = 0
        return carry
    lax.fori_loop(0, RK, zero, 0)

    def once(fn):
        def body(_, carry):
            fn()
            return carry
        lax.fori_loop(0, 1 + zero_s[1], body, 0)

    def tile_idx(ref, cols=128):
        z = zero_s[0]
        n = 16 if ref.dtype == bf16 and cols == 128 else 8
        return (z,) * (len(ref.shape) - 2) + (pl.ds(pl.multiple_of(z, n), n), slice(0, cols))

    hist = []

    def mm(lhs, rhs, side=None, acc=None):
        if side is not None:
            lhs = side(lhs)
        lhs = pltpu.bitcast(lhs, bf16) if lhs.dtype == u32 else lhs.astype(bf16)
        y = _dot(lhs, pltpu.bitcast(rhs, bf16) if rhs.dtype == u32 else rhs)
        if acc is not None:
            y = y + acc
        hist.append(y)
        return y

    class Side:
        def __init__(self, pieces, n, skip=0):
            cap = [0] * skip + [1] * n
            tot = sum(p[4] for p in pieces)
            self.plan = [[] for _ in cap]
            done = 0
            for p in pieces:
                done += p[4]
                x, d = done / tot * sum(cap), 0
                while x > cap[d] + 1e-9:
                    x -= cap[d]
                    d += 1
                self.plan[d].append((p, x / cap[d]))
            self.pieces = len(pieces)

        def __call__(self, val):
            todo = self.plan.pop(0) if self.plan else []
            if not todo:
                return val
            self.pieces -= len(todo)
            never = zero_s[0] > 0
            if val.dtype == bf16:
                val = pltpu.bitcast(val, u32)
            rg = 8 if val.dtype == u32 else 16
            ng = val.shape[0] // rg
            tied = {}
            for (fn, rd, wr, lag, _), pos in todo:
                m = min(max(-int(-pos * ng // 1) - 1, 0), ng - 1)
                pin = lambda v, w=128: v
                if lag is not None and len(hist) >= lag:
                    r0 = (16 * m) % hist[-lag].shape[0]
                    a = hist[-lag][r0:r0 + 8, :128]
                    if rd is None:
                        def pin(v, w=128, a=a):
                            a = _cat([_cat([_as(a, v.dtype)] * (v.shape[0] // 8), 0)] * (w // 128), 1)
                            if v.shape[1] == w:
                                return lax.select(never, a, v)
                            return _cat([lax.select(never, a, v[:, :w]), v[:, w:]], 1)
                    elif rd.dtype == bf16:
                        idx = tile_idx(rd, 256)
                        rd[idx] = lax.select(never, _cat([a, a], 1).astype(bf16), rd[idx])
                    else:
                        idx = tile_idx(rd)
                        rd[idx] = lax.select(never, _as(a, rd.dtype), rd[idx])
                u = fn(pin)
                if wr is False:
                    continue
                if wr is not None:
                    u = wr[tile_idx(wr)]
                t, n = tied.get(m * rg) or (val[m * rg:m * rg + 8, -128:], 0)
                tied[m * rg] = (lax.select(zero_s[n] > 0, _as(u, val.dtype), t), n + 1)
            if not tied:
                return val
            col, r = [], 0
            for r0 in sorted(tied):
                col += ([val[r:r0, -128:]] if r0 > r else []) + [tied[r0][0]]
                r = r0 + 8
            col += [val[r:, -128:]] if r < val.shape[0] else []
            return _cat([val[:, :-128], _cat(col, 0)], 1) if val.shape[1] > 128 else _cat(col, 0)

    def strassen(lhs, rhs, side, init=(None, None, None, None)):
        def add(a, b):
            return a if b is None else a + b
        p = [mm(lhs(k), rhs(k), side) for k in range(5)]
        c12 = add(p[2] + p[4], init[1])
        c21 = add(p[1] + p[3], init[2])
        c22 = mm(lhs(5), rhs(5), side, add(p[0] - p[1] + p[2], init[3]))
        c11 = mm(lhs(6), rhs(6), side, add(p[0] + p[3] - p[4], init[0]))
        return c11, c12, c21, c22

    def fmm(lhs, rhs, side, extra=lambda n: None, emit=None):
        val = {}
        for n in WORDER:
            t = extra(n)
            for q, sg in sorted(_WPAR[n], key=lambda e: -e[1]):
                t = val[q] if t is None else (t + val[q] if sg > 0 else t - val[q])
            for r in range(RK):
                if WN[r] == n:
                    t = mm(lhs(UN[r]), rhs(r), side, t)
            val[n] = t
            if n < 8 and emit is not None:
                emit(n, t)
        return [val[v] for v in range(8)]

    def prep26_pieces(s_v, lag):
        def piece(rs, cs, pin):
            @functools.lru_cache(None)
            def node(n):
                if n < 16:
                    return s_v[RAW16[n], rs, cs].astype(f32)
                a, sa, b, sb = VP[n - 16]
                return _run([(0, sa, 1, sb)], [node(a), node(b)])[-1]
            vals = [node(VN[r]).astype(bf16) for r in VORDER]
            for r, t in zip(VORDER, vals):
                s_v[r, rs, cs] = t
        kb, nb = s_v.shape[1] // 128 * 128, s_v.shape[2]
        out = []
        for r in range(0, kb, 16):
            out += [(slice(rr, rr + 8), slice(c, c + 256)) for c in range(0, nb - 255, 256) for rr in (r, r + 8)]
            out += [(slice(rr, rr + 8), slice(nb - 128, nb)) for rr in (r, r + 8)] if nb % 256 else []
        return [(functools.partial(piece, rs, cs), s_v, s_v if n % 16 == 15 else False, lag,
                 130 if cs.stop - cs.start == 256 else 100) for n, (rs, cs) in enumerate(out)]

    def prep_pieces(s_v, raw, lag, width=256):
        def piece(r, c, pin):
            idx = (slice(r, r + 8), slice(c, c + width))
            b11, b12, b21, b22 = [_unpack(pin(s_v[(q,) + idx], width) if n in (0, 3) else s_v[(q,) + idx])
                                  for n, q in enumerate(raw)]
            for k, t in ((0, b11 + b22), (2, b12 - b22), (3, b21 - b11), (5, b11 + b12), (6, b21 + b22)):
                s_v[(k,) + idx] = _pack(t)
        return [(functools.partial(piece, r, c), None, s_v, lag, 80)
                for c in range(0, s_v.shape[2], width) for r in range(0, s_v.shape[1], 8)]

    def store_l(slot, q, c, quads):
        for k, t in enumerate(_lcombos(*quads)):
            l_v[slot, k, q // 2:q // 2 + 8, c:c + t.shape[1]] = _pack(t)

    def ln_pieces(src, r0, slot, lag, width=256, staged=False, clag=None):
        def stats(q, pin):
            x = pin(src[pl.ds(r0 + q, 16), :].astype(f32))
            xs = [x[:, j * 128:(j + 1) * 128] for j in range(NT)]
            m = functools.reduce(lambda a, b: a + b, xs) * (1.0 / NT)
            w = functools.reduce(lambda a, b: a + b, [(t - m) * (t - m) for t in xs])
            mean = jnp.mean(m, axis=-1, keepdims=True)
            var = jnp.sum(w + NT * ((m - mean) * (m - mean)), axis=-1, keepdims=True) * (1.0 / D)
            n_v[0, q:q + 16, :] = jnp.broadcast_to(mean, (16, 128))
            n_v[1, q:q + 16, :] = jnp.broadcast_to(lax.rsqrt(var + EPS), (16, 128))

        def comb(q, c, pin):
            quads = []
            for rr in (0, HM):
                rs = pl.ds(pl.multiple_of(r0 + rr + q + zero_s[0], 16), 16)
                mean, rstd = [jnp.concatenate([n_v[t, rr + q:rr + q + 16, :]] * (width // 128), axis=1)
                              for t in range(2)]
                quads += [(src[rs, cc + c:cc + c + width].astype(f32) - mean) * rstd for cc in (0, DH2)]
            store_l(slot, q, c, quads)

        def comb26(q, pin):
            blocks = []
            for rr in (0, HM):
                rs = pl.ds(pl.multiple_of(r0 + rr + q + zero_s[0], 8), 8)
                mean, rstd = [jnp.concatenate([n_v[t, rr + q:rr + q + 8, :]] * 2, axis=1) for t in range(2)]
                blocks += [(src[rs, cc:cc + D4] - mean) * rstd for cc in range(0, D, D4)]
            vals = _run(UP, blocks)
            for k, u in enumerate(UL):
                lf_v[k, q:q + 8, :] = vals[u].astype(bf16)
        dense = slot is not None or src is b_v
        norms = [[(functools.partial(stats, rr + q), None, n_v if dense else False, lag, 90) for rr in (0, HM)]
                 for q in range(0, HM, 16)]
        if slot is None:
            combs = [[(functools.partial(comb26, qq), n_v, lf_v if dense or qq % 32 == 24 else False, clag, 110)
                      for qq in (q, q + 8)] for q in range(0, HM, 16)]
        else:
            combs = [[(functools.partial(comb, q, c), n_v, l_v, clag, 125) for c in range(0, DH2, width)]
                     for q in range(0, HM, 16)]
        if staged:
            return sum(norms, []), sum(combs, [])
        out = list(norms[0])
        for a, b in zip(norms[1:] + [[]], combs):
            out += _merge(a, b) if a else b
        return out

    shifts = (1, 1, -1, -1, 2, 2, -2, -2)

    def shift_pieces(r0, slot, lag, by_value=False):
        def piece(q, j, pin):
            a = [h_v[jj, pl.ds(PAD + r0 + rr + q - shifts[jj], 16), :]
                 for rr in (0, HM) for jj in (j, j + NT // 2)]
            store_l(slot, q, j * 128, [pin(a[0]), a[1], a[2], pin(a[3])])
        return [(functools.partial(piece, q, j), None if by_value else h_v,
                 l_v if (q // 16) % 2 and j == 3 else False, lag, 50)
                for q in range(0, HM, 16) for j in range(NT // 2)]

    def lhs_of(slot):
        return lambda k: l_v[slot, k]

    xe_v[0, 0:16, :] = jnp.zeros((16, D4), bf16)
    h_v[:, 0:PAD, :] = jnp.zeros((NT, PAD, 128), f32)
    h_v[:, PAD + S:PAD + S + PAD, :] = jnp.zeros((NT, PAD, 128), f32)

    def store_h(r0, c0, h):
        for j in range(h.shape[1] // 128):
            h_v[c0 // 128 + j, PAD + r0:PAD + r0 + h.shape[0], :] = h[:, j * 128:(j + 1) * 128]

    def h_pieces(r0, c0, t, lag, n=4):
        def piece(r, pin):
            store_h(r0 + r, c0, _gelu(pin(t[r:r + 8 * n])))
        return [(functools.partial(piece, r), None, h_v, lag, 10 * n) for r in range(0, t.shape[0], 8 * n)]

    def flush(pieces):
        for p in pieces:
            p[0](lambda v, w=128: v)

    def w1_cols(c, step):
        half, cc = c // DH2, c % DH2
        return jnp.concatenate([s1_v[RAW1[half], :, cc:cc + step], s1_v[RAW1[2 + half], :, cc:cc + step]], axis=0)

    def d1_plain(xn, r0, c0, c1, step):
        for c in range(c0, c1, step):
            store_h(r0, c, _gelu(mm(xn, w1_cols(c, step))))

    def d1_fine(lhs, r0, nrb, cols, pieces, carry, skip=0):
        tiles = [(rb, c) for c in cols for rb in range(nrb)]
        rounds = [tiles[i:i + 4] for i in range(0, len(tiles), 4)]
        for n, (rnd, part) in enumerate(zip(rounds, split(pieces, len(rounds)))):
            sk = skip if n == 0 else 0
            side = Side(_merge(carry, part) if carry else part, 8 - sk, sk)
            carry = []
            for rb, c in rnd:
                half, cc = c // DH2, c % DH2
                t = mm(lhs(rb, 0), s1_v[RAW1[half], :, cc:cc + 128], side)
                t = mm(lhs(rb, 1), s1_v[RAW1[2 + half], :, cc:cc + 128], side, t)
                carry += h_pieces(r0 + rb * HM, c, t, LS)
        return carry

    def d1_s(b, slot, pieces, carry, early=()):
        for c, part, e in zip(range(0, DH2, NC1), split(pieces, DH2 // NC1), split(early, 2) + [[], []]):
            side = Side(merge(carry, part, e), *((7,) if hist else (5, 2)))
            cs = strassen(lhs_of(slot), lambda k: s1_v[k, :, c:c + NC1], side)
            carry = sum([h_pieces(b * TM + (q // 2) * HM, (q % 2) * DH2 + c, cs[q], LS) for q in (1, 2, 3, 0)], [])
        return carry

    def d2_s(b, slot, pieces, carry=(), early=(), late=()):
        for c, part, e in zip(range(0, DH2, NC1), split(pieces, DH2 // NC1), split(early, 2) + split(late, 2)):
            side = Side(merge(carry, part, e), *((7,) if hist else (5, 2)))
            carry = ()
            idx = [(slice(b * TM + (q // 2) * HM, b * TM + (q // 2 + 1) * HM),
                    slice((q % 2) * DH2 + c, (q % 2) * DH2 + c + NC1)) for q in range(4)]
            cs = strassen(lhs_of(slot), lambda k: s2_v[k, :, c:c + NC1], side,
                          [x_v[i].astype(f32) for i in idx])
            for i, t in zip(idx, cs):
                b_v[i] = t
                if b == 0:
                    c0_v[i] = t

    def split(l, n):
        w = [1.0 if hist else 0.6] + [1.0] * (n - 1)
        cut = [int(round(len(l) * sum(w[:i]) / sum(w))) for i in range(n + 1)]
        return [l[cut[i]:cut[i + 1]] for i in range(n)]

    def merge(*ls):
        ls = [l for l in ls if l]
        return _merge(*ls) if ls else []

    NW1, NW3, N30 = 52, 32, 20
    LS, LL = 3, 5

    p3 = prep26_pieces(s3_v, LS)
    n3 = len(p3) * W3A // D4

    @once
    def _phase1a():
        wait("x0")
        xn0 = _pack(_ln(x_v[0:TM, :].astype(f32)))
        wait("w1a")
        d1_plain(xn0, 0, 0, 256, 256)
        wait("x1")
        xn1 = [_pack(_ln(x_v[r:r + HM, :].astype(f32))) for r in (TM, TM + HM)]
        for n in range(2):
            d1_plain(xn1[n], TM + n * HM, 0, 256, 256)
        wait("w1b")
        d1_plain(jnp.concatenate([xn0] + xn1, axis=0), 0, 256, 512, 256)
        wait("w1cd")
        hist.clear()
        xn01 = jnp.concatenate([xn0] + xn1, axis=0)
        l01 = lambda rb, kh: xn01[rb * 64:(rb + 1) * 64, kh * DH2:(kh + 1) * DH2]
        pw = prep_pieces(s1_v, RAW1, LS)
        flush(d1_fine(l01, 0, 4, (512, 640), pw[:NW1], [], 1))
        carry = []
        wait("x23")
        hist.clear()
        carry = d1_fine(l01, 0, 4, (768, 896), ln_pieces(x_v, 2 * TM, 0, LL), carry, 3)
        carry = d1_s(2, 0, ln_pieces(x_v, 3 * TM, 1, LL), carry, pw[NW1:])
        wait("x4567")
        qkv_start(0)
        qkv_start(1)
        hist.clear()
        for b in range(3, NB - 1):
            carry = d1_s(b, b % 2, ln_pieces(x_v, (b + 1) * TM, (b + 1) % 2, LL), carry)
        wait("w2")
        hist.clear()
        pw = prep_pieces(s2_v, RAW, LS)
        carry = d1_s(7, 1, _merge(pw[:NW3], shift_pieces(0, 0, LS, True)), carry)
        d2_s(0, 0, shift_pieces(TM, 1, LS, True), carry, pw[NW3:], p3[:N30])
        pw = split(_merge(p3[N30:n3], sum(ln_pieces(c0_v, 0, None, LL, clag=LS, staged=True), [])), 3)
        for b in range(1, 4):
            d2_s(b, b % 2, _merge(pw[b - 1], shift_pieces((b + 1) * TM, (b + 1) % 2, LS)))
        wait("w4", "small")

    hist.clear()
    pw = p3[n3:] + prep26_pieces(s4_v, LS)
    cut = (0, 33, 68, 103, len(pw))
    for b in range(4, NB):
        d2_s(b, b % 2, merge(pw[cut[b - 4]:cut[b - 3]],
                             shift_pieces((b + 1) * TM, (b + 1) % 2, LS) if b + 1 < NB else ()))
    start("wo", priority=1)

    def ffn(i, carry):
        qkv_wait(i)
        r0 = pl.multiple_of(i * TM, TM)
        rn = pl.multiple_of(jnp.minimum(i + 1, NB - 1) * TM, TM)
        acc = {}
        hist.clear()

        def relayout(p, r0_, r1_, pin):
            s0 = i * SPG + 2 * p
            e = wqkv_v[s0, r0_:r1_, :]
            o = wqkv_v[s0 + 1, r0_:r1_, :]
            wqkv_v[s0, r0_:r1_, :] = (e & jnp.uint32(0xFFFF)) | (o << 16)
            wqkv_v[s0 + 1, r0_:r1_, :] = (e >> 16) | (o & jnp.uint32(0xFFFF0000))

        relays = [(functools.partial(relayout, p, r, r + 32), wqkv_v, wqkv_v, 3, 35)
                  for p in range(SPG // 2) for r in range(0, D // 2, 32)]
        norms, combs = ln_pieces(b_v, rn, None, 5, staged=True, clag=3)

        def gate(q, pin):
            gw = gw_ref[...].astype(f32)
            x = pin(x_v[pl.ds(r0 + q, 16), :].astype(f32))
            t = functools.reduce(lambda a, b: a + b,
                                 [x[:, j * 128:(j + 1) * 128] * gw[j:j + 1, :] for j in range(NT)])
            g = jax.nn.sigmoid(jnp.sum(t, axis=-1, keepdims=True))
            g_v[pl.ds(r0 + q, 16), :] = jnp.broadcast_to(g, (16, 128))

        gates = [(functools.partial(gate, q), None, g_v, 5, 90) for q in range(0, TM, 16)]

        def extras(t, pin):
            jj, o = 2 * i + t // 2, 24 + 8 * (t % 2)
            xs = [pin(x_v[pl.ds(pl.multiple_of((jj + hh) * 64 + o, 8), 8), :].astype(f32)) for hh in (0, NPAIR // 2)]
            vals = _run(UP, [x[:, cc:cc + D4] for x in xs for cc in range(0, D, D4)])
            for k, u in enumerate(UL):
                xe_v[k, pl.ds(pl.multiple_of(i * 32 + t * 8, 8), 8), :] = vals[u].astype(bf16)

        xes = [(functools.partial(extras, t), None, xe_v, 3, 100) for t in range(4)]
        hs = {}

        def gelu_pieces(c, cs):
            def piece(r, cc, vs, pin):
                t = _gelu(pin(_cat([cs[v][r:r + 8, cc:cc + 128] for v in vs], 0)))
                ts = [t[8 * n:8 * n + 8] for n in range(len(vs))]
                hs.update({(c, v, r, cc): u for v, u in zip(vs, ts)})
                return functools.reduce(lambda a, b: a + b, ts)
            return [(functools.partial(piece, r, cc, vs), None, None, 3, 40) for r in range(0, HM, 8)
                    for cc in range(0, cs[0].shape[1], 128) for vs in ((0, 1, 2, 3), (4, 5, 6, 7))]

        def d3(c, side):
            c0, c1 = FCH[c]
            cs = fmm(lambda u: lf_v[UL.index(u)], lambda r: s3_v[r, 0:D4, c0:c1], side)
            assert not side.pieces
            return gelu_pieces(c, cs)

        def d4(c, side):
            c0, c1 = FCH[c]
            lh = _run(UP, [_cat([_cat([hs.pop((c, v, r, cc)) for r in range(0, HM, 8)], 0)
                                 for cc in range(0, c1 - c0, 128)], 1) for v in range(8)])
            rhs = lambda r: s4_v[r, c0:c1, :]
            if c + 1 < len(FCH):
                for n in WORDER:
                    for r in range(RK):
                        if WN[r] == n:
                            acc[n] = mm(lh[UN[r]], rhs(r), side, acc.get(n))
            else:
                idx = lambda v: (pl.ds(r0 + (v // 4) * HM, HM), slice((v % 4) * D4, (v % 4 + 1) * D4))

                def extra(n):
                    if n >= 8:
                        return acc.get(n)
                    return b_v[idx(n)] + acc[n] if n in acc else b_v[idx(n)]

                def emit_b(v, t):
                    b_v[idx(v)] = jnp.concatenate([1.0 - g_v[idx(v)[0], :]] * 2, axis=1) * t
                fmm(lambda u: lh[u], rhs, side, extra, emit_b)
            assert not side.pieces

        g0 = d3(0, Side(relays[:20], 23, 3))
        g1 = d3(1, Side(_merge(g0, gates, xes), 23, 2))
        d4(0, Side(g1[:22], 22, 4))
        g2 = d3(2, Side(_merge(g1[22:], relays[20:40]), 25))
        d4(1, Side(g2, 23, 2))
        g3 = d3(3, Side(_merge(relays[40:], norms), 26))
        d4(2, Side(_merge(g3, combs), 23, 2))
        d4(3, Side([], 1))

        @pl.when(i + 2 < NG)
        def _():
            qkv_start(i + 2)

        return carry

    lax.fori_loop(0, NB, ffn, 0)

    def pre(it, carry):
        hist.clear()
        for u in range(3 * NG // NPRE):
            s0 = (it * (3 * NG // NPRE) + u) * G

            def rhs(r):
                t = None
                sz = s0 + zero_s[r]
                for q, sg in sorted(_terms(VP, 16, VN[r]).items(), key=lambda e: -e[1]):
                    blk = wqkv_v[sz + q % 4, (q // 4) * (D // 8):(q // 4 + 1) * (D // 8), :]
                    if VN[r] < 16:
                        return blk
                    blk = _unpack(blk)
                    t = blk if t is None else (t + blk if sg > 0 else t - blk)
                return t.astype(bf16)
            for v, t in enumerate(fmm(lambda k: xe_v[UL.index(k)], rhs, None)):
                e_v[(v // 4) * 16:(v // 4 + 1) * 16, s0 + v % 4] = _pack(t).reshape(16, 8, DH)
        return carry

    lax.fori_loop(0, NPRE, pre, 0)

    wait("wo")
    mem_v[...] = mem0_ref[...].astype(f32)

    def slab(w, h):
        return (h // G) * SPG + w * G + h % G

    def step(j, hx, odd, late, allow, fill):
        qs, ks, vs, ps = {}, {}, {}, {}
        wload = lambda w, h: pltpu.bitcast(wqkv_v[slab(w, h)], bf16)
        eload = lambda w, h: pltpu.bitcast(e_v[j, slab(w, h)], bf16)

        def proj(g):
            part = {}
            if late and g == 0:
                for h in range(2):
                    for w in range(3):
                        part[w, h] = _dot(hx[:, :DH2], wload(w, h)[:DH2])
            for h in range(g * G, (g + 1) * G):
                q, k, v = [(_dot(hx[:, DH2:], wload(w, h)[DH2:]) + part[w, h] if (w, h) in part
                            else _dot(hx, wload(w, h))).astype(bf16) for w in range(3)]
                if odd:
                    q = jnp.concatenate([q, eload(0, h)], axis=0)
                    k = jnp.concatenate([pltpu.bitcast(ke_v[h], bf16), eload(1, h), k], axis=0)
                    v = jnp.concatenate([pltpu.bitcast(ve_v[h], bf16), eload(2, h), v], axis=0)
                else:
                    ke_v[h] = pltpu.bitcast(k, u32)
                    ve_v[h] = pltpu.bitcast(v, u32)
                    k = jnp.concatenate([k, eload(1, h)], axis=0)
                    v = jnp.concatenate([v, eload(2, h)], axis=0)
                qs[h], ks[h], vs[h] = q, k, v

        def score(g):
            for h in range(g * G, (g + 1) * G):
                s = lax.dot_general(qs.pop(h), ks.pop(h), (((1,), (1,)), ((), ())),
                                    preferred_element_type=f32)
                ps[h] = _softmax(s, allow, fill)

        def pv(g):
            os_ = []
            for h in range(g * G, (g + 1) * G):
                o = _dot(ps.pop(h), vs.pop(h))
                o_v[:, h * 128:(h + 1) * 128] = _pack(o[:32])
                os_.append(o)
            if odd:
                quads = [jnp.concatenate([os_[2 * kk][r:r + 8], os_[2 * kk + 1][r:r + 8]], axis=1)
                         for r in (32, 40) for kk in range(2)]
                for k, t in enumerate(_lcombos(*quads)):
                    oe_v[k, pl.ds(pl.multiple_of(j * 8, 8), 8), g * 256:(g + 1) * 256] = t.astype(bf16)

        acc = [None] * NT

        def wo(h0, h1, j0, j1):
            o = pltpu.bitcast(o_v[:, h0 * 128:h1 * 128], bf16)
            for n in range(j0, j1):
                y = _dot(o, pltpu.bitcast(wo_v[n, h0 * 64:h1 * 64, :], bf16))
                acc[n] = y if acc[n] is None else y + acc[n]

        for t in range(NG):
            proj(t)
            if t >= 2:
                pv(t - 2)
            if t >= 1:
                score(t - 1)
        wo(0, 16, 0, 4)
        pv(NG - 2)
        score(NG - 1)
        wo(0, 16, 4, 8)
        pv(NG - 1)
        wo(16, 24, 0, 8)
        wo(24, 32, 0, 8)
        return jnp.concatenate(acc, axis=1)

    def emit(j, r0, o0, a):
        rs = pl.ds(r0 + o0, 24)
        g = jnp.concatenate([g_v[rs, :]] * NT, axis=1)
        out_v[j, o0:o0 + 24, :] = (g * a + b_v[rs, :]).astype(bf16)

    def pair(j, mem, late):
        r0 = pl.multiple_of(j * 64, 64)
        allow_e, fill_e, allow_o, fill_o = _masks()
        xa = x_v[pl.ds(r0 + 16, 8), :].astype(f32)
        xb = x_v[pl.ds(r0 + 40, 8), :].astype(f32)
        hx = jnp.concatenate([x_v[pl.ds(r0, 16), :], jnp.concatenate([xa, mem], 0).astype(bf16)], 0)
        oe = step(j, hx, False, late, allow_e, fill_e)
        emit(j, r0, 0, oe[:24])
        hx = jnp.concatenate([jnp.concatenate([oe[24:32], xb], 0).astype(bf16), x_v[pl.ds(r0 + 48, 16), :]], 0)
        oo = step(j, hx, True, True, allow_o, fill_o)
        emit(j, r0, 40, oo[8:])
        return oo[:8]

    def a_iter(it, carry):
        mem = mem_v[...]
        for t in range(PPI):
            mem = pair(it * PPI + t, mem, t > 0)
        mem_v[...] = mem
        for t in range(PPI):
            for o0 in (0, 40):
                idx = (it * PPI + t, pl.ds(o0, 24))
                pltpu.make_async_copy(out_v.at[idx], out_hbm.at[idx], sem_out).start()
        return carry

    lax.fori_loop(0, NPAIR // PPI, a_iter, 0)

    @once
    def _post():
        hist.clear()
        for n in range(NT // 2):
            quad = [lambda k, t=2 * n + q % 2, o=(q // 2) * 128: jnp.concatenate(
                [wo_v[t + zero_s[k], g * 256 + o:g * 256 + o + 128, :] for g in range(NG)], axis=0) for q in range(4)]
            cs = strassen(lambda k: oe_v[k], lambda k: _rcombo(k, *quad), None)
            cols = slice(n * 256, (n + 1) * 256)
            for half in range(2):
                t = jnp.concatenate(cs[2 * half:2 * half + 2], axis=1)
                o0 = 24 + half * 8
                for jj in range(NPAIR):
                    rs = slice(jj * 64 + o0, jj * 64 + o0 + 8)
                    g = jnp.concatenate([g_v[rs, :]] * 2, axis=1)
                    out_v[jj, o0:o0 + 8, cols] = (g * t[jj * 8:jj * 8 + 8] + b_v[rs, cols]).astype(bf16)
            if n >= 2:
                idx = (slice(None), pl.ds(24, 16), pl.ds(0, 768) if n == 2 else pl.ds(768, 256))
                pltpu.make_async_copy(out_v.at[idx], out_hbm.at[idx], sem_out).start()

    pltpu.make_async_copy(out_v, out_hbm, sem_out).wait()


@jax.jit
def pallas_gated_mix__memory_aug_recurrent_mem_tr__mixer_s_mlp__prompt_kernel(
    A_x, A_mem0, A_Wq, A_Wk, A_Wv, A_Wo, A_seg_len, B_x, B_w1, B_w2, B_w3, B_w4, gate_w,
):
    assert A_x.shape == (1, S, D) and A_mem0.shape == (1, M, D)
    any_spec = pl.BlockSpec(memory_space=pl.ANY)
    out = pl.pallas_call(
        _kernel,
        out_shape=jax.ShapeDtypeStruct((NPAIR, 64, D), bf16),
        in_specs=[any_spec] * 11,
        out_specs=any_spec,
        scratch_shapes=[
            pltpu.VMEM((S, D), bf16),
            pltpu.VMEM((9, D // 4, D // 2), u32),
            pltpu.VMEM((7, D // 4, D // 2), u32),
            pltpu.VMEM((RK + 2, D4 + 16, F4), bf16),
            pltpu.VMEM((RK + 2, F4 + 8, D4), bf16),
            pltpu.VMEM((3 * H, D // 2, DH), u32),
            pltpu.VMEM((NT, H * DH // 2, 128), u32),
            pltpu.VMEM((NT, S + 2 * PAD, 128), f32),
            pltpu.VMEM((S, D), f32),
            pltpu.VMEM((TM, D), f32),
            pltpu.VMEM((2, 7, HM // 2, D // 2), u32),
            pltpu.VMEM((len(UL), HM, D4), bf16),
            pltpu.VMEM((2, TM, 128), f32),
            pltpu.VMEM((S, 128), f32),
            pltpu.VMEM((NPAIR, 64, D), bf16),
            pltpu.VMEM((len(UL), 8 * NPAIR, D4), bf16),
            pltpu.VMEM((NPAIR, 3 * H, 8, DH), u32),
            pltpu.VMEM((7, 8 * NPAIR, H * DH // 2), bf16),
            pltpu.VMEM((H, 16, 128), u32),
            pltpu.VMEM((H, 16, 128), u32),
            pltpu.VMEM((16, H * DH), u32),
            pltpu.VMEM((M, D), f32),
            pltpu.VMEM((M, D), bf16),
            pltpu.VMEM((NT, 128), bf16),
            pltpu.SMEM((RK,), jnp.int32),
            pltpu.SemaphoreType.DMA((NLOAD,)),
            pltpu.SemaphoreType.DMA((NG,)),
            pltpu.SemaphoreType.DMA,
        ],
        compiler_params=pltpu.CompilerParams(vmem_limit_bytes=126 * 1024 * 1024,
                                             disable_bounds_checks=True),
    )(
        A_x.reshape(S, D), A_mem0.reshape(M, D),
        A_Wq.reshape(D // 2, 2 * H, DH), A_Wk.reshape(D // 2, 2 * H, DH), A_Wv.reshape(D // 2, 2 * H, DH),
        A_Wo.reshape(H * DH, D), B_w1, B_w2, B_w3, B_w4, gate_w.reshape(NT, 128),
    )
    return out.reshape(1, S, D)
```

```python
import functools

import jax
import jax.numpy as jnp
from jax import lax
import jax.experimental.pallas as pl
import jax.experimental.pallas.tpu as pltpu

f32, bf16, u32 = jnp.float32, jnp.bfloat16, jnp.uint32

S, D, H, DH, M, SEG, F = 2048, 1024, 32, 128, 8, 32, 3584
SCALE = DH ** -0.5
NEG = -1000000000.0
EPS = 1e-05

TM = 256
NB = S // TM
HM = TM // 2
DH2 = D // 2
D4, F4 = D // 4, F // 4
FCH = ((0, 128), (128, 384), (384, 640), (640, 896))
NC1 = 128
NPAIR = S // (2 * SEG)
PPI = 2
NPRE = 3
G = 4
NG = H // G
PAD = 8
NT = D // 128
W3A = 192
NLOAD = 11
assert NB == NG

_dot = functools.partial(jnp.dot, preferred_element_type=f32)

UP = ((4, 1, 5, 1), (6, 1, 8, 1), (0, 1, 3, 1), (2, -1, 9, 1), (4, -1, 10, 1), (0, 1, 1, 1), (2, 1, 12, 1),
      (5, 1, 7, -1), (7, 1, 12, -1), (11, -1, 13, 1), (10, -1, 11, 1), (2, 1, 7, 1), (0, -1, 4, 1),
      (6, 1, 7, 1), (1, -1, 5, 1), (3, 1, 7, -1), (1, 1, 4, 1), (2, 1, 3, 1), (1, -1, 3, 1), (1, 1, 7, -1),
      (2, 1, 6, -1))
WP = ((0, -1, 3, 1), (4, 1, 6, -1), (1, 1, 8, 1), (5, 1, 10, 1), (4, -1, 7, 1), (0, -1, 9, -1),
      (11, 1, 12, 1), (6, 1, 7, -1), (2, 1, 5, -1), (0, -1, 7, -1), (9, 1, 11, -1), (2, 1, 13, 1),
      (5, 1, 13, 1), (2, -1, 3, 1), (5, 1, 6, 1), (0, 1, 4, 1), (2, 1, 7, 1), (1, 1, 2, 1), (1, 1, 5, 1),
      (3, 1, 7, 1), (2, 1, 6, 1))
VP = ((1, 1, 5, -1), (8, 1, 11, 1), (10, 1, 17, 1), (13, 1, 16, -1), (0, 1, 4, -1), (0, 1, 3, 1),
      (14, 1, 18, -1), (0, 1, 11, 1), (14, 1, 19, -1), (0, 1, 5, 1), (12, 1, 15, 1), (2, 1, 21, 1),
      (10, 1, 14, -1), (4, 1, 7, 1), (11, 1, 19, 1), (12, -1, 20, 1), (13, 1, 14, -1), (9, 1, 30, -1),
      (3, -1, 15, 1), (6, 1, 23, 1), (24, 1, 27, -1), (9, -1, 18, 1), (7, 1, 34, 1), (2, 1, 6, -1),
      (0, 1, 8, -1), (6, 1, 21, 1), (22, 1, 31, -1), (6, 1, 29, 1), (0, 1, 1, 1), (15, 1, 25, 1),
      (5, 1, 37, 1), (15, 1, 20, 1))
UN = (7, 27, 24, 17, 9, 22, 21, 2, 15, 11, 8, 25, 19, 28, 2, 23, 26, 20, 1, 18, 10, 28, 4, 13, 14, 16)
WN = (23, 17, 24, 10, 14, 7, 22, 19, 12, 18, 15, 25, 20, 5, 26, 0, 8, 2, 27, 11, 26, 9, 28, 21, 16, 5)
VN = (42, 47, 41, 5, 11, 43, 18, 28, 20, 23, 35, 19, 22, 46, 33, 26, 45, 36, 38, 25, 44, 40, 39, 21, 24, 32)
RK = len(UN)
UL = tuple(sorted(set(UN)))
RAW16 = (1, 11, 17, 5, 8, 3, 9, 10, 0, 6, 7, 4, 12, 20, 22, 16)
VORDER = (0, 6, 7, 12, 13, 14, 15, 21, 11, 17, 20, 22, 24, 25, 23, 2, 1, 5, 8, 9, 10, 16, 18, 19)
assert sorted(VORDER) == [r for r in range(RK) if VN[r] >= 16] and len(set(RAW16)) == 16
assert all(RAW16[VN[r]] == r for r in range(RK) if VN[r] < 16)


def _run(prog, blocks):
    vals = list(blocks)
    for a, sa, b, sb in prog:
        vals.append(vals[a] + vals[b] if sa > 0 and sb > 0 else
                    vals[a] - vals[b] if sa > 0 else vals[b] - vals[a])
    return vals


def _terms(prog, nin, node):
    if node < nin:
        return {node: 1}
    a, sa, b, sb = prog[node - nin]
    out = {k: sa * v for k, v in _terms(prog, nin, a).items()}
    out.update({k: sb * v for k, v in _terms(prog, nin, b).items()})
    return out


def _scheme_is_exact():
    t = {}
    for r in range(RK):
        for a, ca in _terms(UP, 8, UN[r]).items():
            for b, cb in _terms(VP, 16, VN[r]).items():
                for c, cc in _terms(WP, 8, WN[r]).items():
                    t[a, b, c] = t.get((a, b, c), 0) + ca * cb * cc
    want = {(4 * i + j, 4 * j + l, 4 * i + l): 1 for i in range(2) for j in range(4) for l in range(4)}
    return {k: v for k, v in t.items() if v} == want


assert _scheme_is_exact()

_WPAR = {n: [] for n in range(8 + len(WP))}
for _t, (_a, _sa, _b, _sb) in enumerate(WP):
    _WPAR[_a].append((8 + _t, _sa))
    _WPAR[_b].append((8 + _t, _sb))


def _worder():
    order = []

    def closure(n, acc):
        if n not in acc and n not in order:
            acc.add(n)
            for q, _ in _WPAR[n]:
                closure(q, acc)
        return acc

    def visit(n):
        if n not in order:
            for q, _ in _WPAR[n]:
                visit(q)
            order.append(n)
    while len([v for v in range(8) if v not in order]):
        visit(min((v for v in range(8) if v not in order), key=lambda v: len(closure(v, set()))))
    return tuple(order)


WORDER = _worder()


def _ln(x):
    m = jnp.mean(x, axis=-1, keepdims=True)
    xc = x - m
    v = jnp.mean(xc * xc, axis=-1, keepdims=True)
    return xc * lax.rsqrt(v + EPS)


_GC = 0.7978845608028654


def _gelu(x):
    h = 0.5 * x
    return h + h * jnp.tanh(x * (_GC + (_GC * 0.044715) * (x * x)))


def _unpack(u):
    return pltpu.bitcast(u, bf16).astype(f32)


def _pack(x):
    return pltpu.bitcast(x.astype(bf16), u32)


def _cat(xs, axis):
    xs = [x for x in xs if x.shape[axis]]
    return xs[0] if len(xs) == 1 else jnp.concatenate(xs, axis=axis)


def _as(x, dtype):
    return x if x.dtype == dtype else pltpu.bitcast(x, dtype)


def _lcombos(a11, a12, a21, a22):
    return [a11 + a22, a21 + a22, a11, a22, a11 + a12, a21 - a11, a12 - a22]


def _merge(*lists):
    keyed = [((j + 0.5) / len(l), n, j, v) for n, l in enumerate(lists) for j, v in enumerate(l)]
    return [v for _, _, _, v in sorted(keyed, key=lambda t: t[:3])]


def _masks():
    r = lax.broadcasted_iota(jnp.int32, (32, 48), 0)
    c = lax.broadcasted_iota(jnp.int32, (32, 48), 1)
    exist_e = c < 40
    allow_e = exist_e & ((r >= 24) | ((c >= 24) & (c < 32)) | (c <= r))
    fill_e = jnp.where(exist_e, NEG, -jnp.inf).astype(f32)
    r = lax.broadcasted_iota(jnp.int32, (48, 80), 0)
    c = lax.broadcasted_iota(jnp.int32, (48, 80), 1)
    q_even = (r >= 32) & (r < 40)
    exist_o = (q_even & (c < 40)) | (~q_even & (c >= 40))
    ktok = jnp.where(c < 24, c, jnp.where(c < 48, c - 8, c - 16))
    qtok = jnp.where(r < 32, r + 32, r - 8)
    is_mem_key = ((c >= 24) & (c < 32)) | ((c >= 48) & (c < 56))
    allow_o = exist_o & (is_mem_key | (r < 8) | (ktok <= qtok))
    fill_o = jnp.where(exist_o, NEG, -jnp.inf).astype(f32)
    return allow_e, fill_e, allow_o, fill_o


def _rcombo(k, b11, b12, b21, b22):
    if k in (1, 4):
        return (b11 if k == 1 else b22)(k)
    a, b, sign = {0: (b11, b22, 1), 2: (b12, b22, -1), 3: (b21, b11, -1), 5: (b11, b12, 1), 6: (b21, b22, 1)}[k]
    a, b = _unpack(a(k)), _unpack(b(k))
    return (a + b if sign > 0 else a - b).astype(bf16)


def _softmax(s, allow, fill):
    s = jnp.where(allow, s * SCALE, fill)
    m = jnp.max(s, axis=-1, keepdims=True)
    e = jnp.exp(s - m)
    l = jnp.sum(e, axis=-1, keepdims=True)
    r = pl.reciprocal(l, approx=True)
    r = r * (2.0 - l * r)
    return (e * r).astype(bf16)


def _kernel(x_hbm, mem0_hbm, wq_hbm, wk_hbm, wv_hbm, wo_hbm, w1_hbm, w2_hbm, w3_hbm, w4_hbm,
            gw_hbm, out_hbm,
            x_v, s1_v, s2_v, s3_v, s4_v, wqkv_v, wo_v, h_v, b_v, c0_v, l_v, lf_v, n_v, g_v, out_v, xe_v, e_v, oe_v,
            ke_v, ve_v, o_v, mem_v, mem0_ref, gw_ref, zero_s,
            sem, sem_qkv, sem_out):
    RAW = (1, 2, 3, 4)
    RAW1 = (1, 7, 8, 4)

    loads = []

    def rows_load(name, r0, r1):
        loads.append((name, x_hbm.at[pl.ds(r0, r1 - r0)], x_v.at[pl.ds(r0, r1 - r0)]))

    def quad_load(name, w_hbm, s_v, raw, q, c0=0, c1=None):
        k4, n2 = s_v.shape[1], s_v.shape[2]
        c1 = n2 if c1 is None else c1
        src = w_hbm.bitcast(u32).at[pl.ds((q // 2) * k4, k4), pl.ds((q % 2) * n2 + c0, c1 - c0)]
        loads.append((name, src, s_v.at[raw[q], :, pl.ds(c0, c1 - c0)]))

    def w1_load(name, half, c0, c1):
        quad_load(name, w1_hbm, s1_v, RAW1, half, c0, c1)
        quad_load(name, w1_hbm, s1_v, RAW1, 2 + half, c0, c1)

    def block_load(name, w_hbm, s_v, r0, r1):
        kb, nb = s_v.shape[1] // 128 * 128, s_v.shape[2]
        for q in range(16):
            loads.append((name, w_hbm.at[pl.ds((q // 4) * kb + r0, r1 - r0), pl.ds((q % 4) * nb, nb)],
                          s_v.at[RAW16[q], pl.ds(r0, r1 - r0)]))

    rows_load("x0", 0, TM)
    w1_load("w1a", 0, 0, 256)
    rows_load("x1", TM, 2 * TM)
    w1_load("w1b", 0, 256, 512)
    w1_load("w1cd", 1, 0, 512)
    rows_load("x23", 2 * TM, 4 * TM)
    rows_load("x4567", 4 * TM, S)
    for q in range(4):
        quad_load("w2", w2_hbm, s2_v, RAW, q)
    block_load("w2", w3_hbm, s3_v, 0, W3A)
    block_load("w4", w3_hbm, s3_v, W3A, D4)
    block_load("w4", w4_hbm, s4_v, 0, F4)
    loads.append(("small", mem0_hbm, mem0_ref))
    loads.append(("small", gw_hbm, gw_ref))
    for j in range(NT):
        loads.append(("wo", wo_hbm.bitcast(u32).at[:, pl.ds(j * 128, 128)], wo_v.at[j, pl.ds(0, H * DH // 2)]))
    groups = list(dict.fromkeys(name for name, _, _ in loads))
    assert len(groups) == NLOAD

    def start(*names, priority=0):
        for name, src, dst in loads:
            if name in names:
                pltpu.make_async_copy(src, dst, sem.at[groups.index(name)]).start(priority=priority)

    def wait(*names):
        for name, src, dst in loads:
            if name in names:
                pltpu.make_async_copy(src, dst, sem.at[groups.index(name)]).wait()

    SPG = 3 * G

    def qkv_start(g):
        for w, w_hbm in enumerate((wq_hbm, wk_hbm, wv_hbm)):
            wu = w_hbm.bitcast(u32)
            for k in range(G // 2):
                for par in range(2):
                    pltpu.make_async_copy(
                        wu.at[:, par * (H // 2) + g * (G // 2) + k, :],
                        wqkv_v.at[g * SPG + w * G + 2 * k + par], sem_qkv.at[g]).start(priority=1)

    def qkv_wait(g):
        grp = wqkv_v.at[pl.ds(g * SPG, SPG)]
        pltpu.make_async_copy(grp, grp, sem_qkv.at[g]).wait()

    start("x0", "w1a", "w1b", "x1", "w1cd", "x23", "x4567", "w2", "w4", "small")

    def zero(k, carry):
        zero_s[k] = 0
        return carry
    lax.fori_loop(0, RK, zero, 0)

    def once(fn):
        def body(_, carry):
            fn()
            return carry
        lax.fori_loop(0, 1 + zero_s[1], body, 0)

    def tile_idx(ref, cols=128):
        z = zero_s[0]
        n = 16 if ref.dtype == bf16 and cols == 128 else 8
        return (z,) * (len(ref.shape) - 2) + (pl.ds(pl.multiple_of(z, n), n), slice(0, cols))

    hist = []

    def mm(lhs, rhs, side=None, acc=None):
        if side is not None:
            lhs = side(lhs)
        lhs = pltpu.bitcast(lhs, bf16) if lhs.dtype == u32 else lhs.astype(bf16)
        y = _dot(lhs, pltpu.bitcast(rhs, bf16) if rhs.dtype == u32 else rhs)
        if acc is not None:
            y = y + acc
        hist.append(y)
        return y

    class Side:
        def __init__(self, pieces, n, skip=0):
            cap = [0] * skip + [1] * n
            tot = sum(p[4] for p in pieces)
            self.plan = [[] for _ in cap]
            done = 0
            for p in pieces:
                done += p[4]
                x, d = done / tot * sum(cap), 0
                while x > cap[d] + 1e-9:
                    x -= cap[d]
                    d += 1
                self.plan[d].append((p, x / cap[d]))
            self.pieces = len(pieces)

        def __call__(self, val):
            todo = self.plan.pop(0) if self.plan else []
            if not todo:
                return val
            self.pieces -= len(todo)
            never = zero_s[0] > 0
            if val.dtype == bf16:
                val = pltpu.bitcast(val, u32)
            rg = 8 if val.dtype == u32 else 16
            ng = val.shape[0] // rg
            tied = {}
            for (fn, rd, wr, lag, _), pos in todo:
                m = min(max(-int(-pos * ng // 1) - 1, 0), ng - 1)
                pin = lambda v, w=128: v
                if lag is not None and len(hist) >= lag:
                    r0 = (16 * m) % hist[-lag].shape[0]
                    a = hist[-lag][r0:r0 + 8, :128]
                    if rd is None:
                        def pin(v, w=128, a=a):
                            a = _cat([_cat([_as(a, v.dtype)] * (v.shape[0] // 8), 0)] * (w // 128), 1)
                            if v.shape[1] == w:
                                return lax.select(never, a, v)
                            return _cat([lax.select(never, a, v[:, :w]), v[:, w:]], 1)
                    elif rd.dtype == bf16:
                        idx = tile_idx(rd, 256)
                        rd[idx] = lax.select(never, _cat([a, a], 1).astype(bf16), rd[idx])
                    else:
                        idx = tile_idx(rd)
                        rd[idx] = lax.select(never, _as(a, rd.dtype), rd[idx])
                u = fn(pin)
                if wr is False:
                    continue
                if wr is not None:
                    u = wr[tile_idx(wr)]
                t, n = tied.get(m * rg) or (val[m * rg:m * rg + 8, -128:], 0)
                tied[m * rg] = (lax.select(zero_s[n] > 0, _as(u, val.dtype), t), n + 1)
            if not tied:
                return val
            col, r = [], 0
            for r0 in sorted(tied):
                col += ([val[r:r0, -128:]] if r0 > r else []) + [tied[r0][0]]
                r = r0 + 8
            col += [val[r:, -128:]] if r < val.shape[0] else []
            return _cat([val[:, :-128], _cat(col, 0)], 1) if val.shape[1] > 128 else _cat(col, 0)

    def strassen(lhs, rhs, side, init=(None, None, None, None)):
        def add(a, b):
            return a if b is None else a + b
        p = [mm(lhs(k), rhs(k), side) for k in range(5)]
        c12 = add(p[2] + p[4], init[1])
        c21 = add(p[1] + p[3], init[2])
        c22 = mm(lhs(5), rhs(5), side, add(p[0] - p[1] + p[2], init[3]))
        c11 = mm(lhs(6), rhs(6), side, add(p[0] + p[3] - p[4], init[0]))
        return c11, c12, c21, c22

    def fmm(lhs, rhs, side, extra=lambda n: None, emit=None):
        val = {}
        for n in WORDER:
            t = extra(n)
            for q, sg in sorted(_WPAR[n], key=lambda e: -e[1]):
                t = val[q] if t is None else (t + val[q] if sg > 0 else t - val[q])
            for r in range(RK):
                if WN[r] == n:
                    t = mm(lhs(UN[r]), rhs(r), side, t)
            val[n] = t
            if n < 8 and emit is not None:
                emit(n, t)
        return [val[v] for v in range(8)]

    def prep26_pieces(s_v, lag):
        def piece(rs, cs, pin):
            @functools.lru_cache(None)
            def node(n):
                if n < 16:
                    return s_v[RAW16[n], rs, cs].astype(f32)
                a, sa, b, sb = VP[n - 16]
                return _run([(0, sa, 1, sb)], [node(a), node(b)])[-1]
            vals = [node(VN[r]).astype(bf16) for r in VORDER]
            for r, t in zip(VORDER, vals):
                s_v[r, rs, cs] = t
        kb, nb = s_v.shape[1] // 128 * 128, s_v.shape[2]
        out = []
        for r in range(0, kb, 16):
            out += [(slice(rr, rr + 8), slice(c, c + 256)) for c in range(0, nb - 255, 256) for rr in (r, r + 8)]
            out += [(slice(rr, rr + 8), slice(nb - 128, nb)) for rr in (r, r + 8)] if nb % 256 else []
        return [(functools.partial(piece, rs, cs), s_v, s_v if n % 16 == 15 else False, lag,
                 130 if cs.stop - cs.start == 256 else 100) for n, (rs, cs) in enumerate(out)]

    def prep_pieces(s_v, raw, lag, width=256):
        def piece(r, c, pin):
            idx = (slice(r, r + 8), slice(c, c + width))
            b11, b12, b21, b22 = [_unpack(pin(s_v[(q,) + idx], width) if n in (0, 3) else s_v[(q,) + idx])
                                  for n, q in enumerate(raw)]
            for k, t in ((0, b11 + b22), (2, b12 - b22), (3, b21 - b11), (5, b11 + b12), (6, b21 + b22)):
                s_v[(k,) + idx] = _pack(t)
        return [(functools.partial(piece, r, c), None, s_v, lag, 80)
                for c in range(0, s_v.shape[2], width) for r in range(0, s_v.shape[1], 8)]

    def store_l(slot, q, c, quads):
        for k, t in enumerate(_lcombos(*quads)):
            l_v[slot, k, q // 2:q // 2 + 8, c:c + t.shape[1]] = _pack(t)

    def ln_pieces(src, r0, slot, lag, width=256, staged=False, clag=None):
        def stats(q, pin):
            x = pin(src[pl.ds(r0 + q, 16), :].astype(f32))
            xs = [x[:, j * 128:(j + 1) * 128] for j in range(NT)]
            m = functools.reduce(lambda a, b: a + b, xs) * (1.0 / NT)
            w = functools.reduce(lambda a, b: a + b, [(t - m) * (t - m) for t in xs])
            mean = jnp.mean(m, axis=-1, keepdims=True)
            var = jnp.sum(w + NT * ((m - mean) * (m - mean)), axis=-1, keepdims=True) * (1.0 / D)
            n_v[0, q:q + 16, :] = jnp.broadcast_to(mean, (16, 128))
            n_v[1, q:q + 16, :] = jnp.broadcast_to(lax.rsqrt(var + EPS), (16, 128))

        def comb(q, c, pin):
            quads = []
            for rr in (0, HM):
                rs = pl.ds(pl.multiple_of(r0 + rr + q + zero_s[0], 16), 16)
                mean, rstd = [jnp.concatenate([n_v[t, rr + q:rr + q + 16, :]] * (width // 128), axis=1)
                              for t in range(2)]
                quads += [(src[rs, cc + c:cc + c + width].astype(f32) - mean) * rstd for cc in (0, DH2)]
            store_l(slot, q, c, quads)

        def comb26(q, pin):
            blocks = []
            for rr in (0, HM):
                rs = pl.ds(pl.multiple_of(r0 + rr + q + zero_s[0], 8), 8)
                mean, rstd = [jnp.concatenate([n_v[t, rr + q:rr + q + 8, :]] * 2, axis=1) for t in range(2)]
                blocks += [(src[rs, cc:cc + D4] - mean) * rstd for cc in range(0, D, D4)]
            vals = _run(UP, blocks)
            for k, u in enumerate(UL):
                lf_v[k, q:q + 8, :] = vals[u].astype(bf16)
        dense = slot is not None or src is b_v
        norms = [[(functools.partial(stats, rr + q), None, n_v if dense else False, lag, 90) for rr in (0, HM)]
                 for q in range(0, HM, 16)]
        if slot is None:
            combs = [[(functools.partial(comb26, qq), n_v, lf_v if dense or qq % 32 == 24 else False, clag, 110)
                      for qq in (q, q + 8)] for q in range(0, HM, 16)]
        else:
            combs = [[(functools.partial(comb, q, c), n_v, l_v, clag, 125) for c in range(0, DH2, width)]
                     for q in range(0, HM, 16)]
        if staged:
            return sum(norms, []), sum(combs, [])
        out = list(norms[0])
        for a, b in zip(norms[1:] + [[]], combs):
            out += _merge(a, b) if a else b
        return out

    shifts = (1, 1, -1, -1, 2, 2, -2, -2)

    def shift_pieces(r0, slot, lag, by_value=False):
        def piece(q, j, pin):
            a = [h_v[jj, pl.ds(PAD + r0 + rr + q - shifts[jj], 16), :]
                 for rr in (0, HM) for jj in (j, j + NT // 2)]
            store_l(slot, q, j * 128, [pin(a[0]), a[1], a[2], pin(a[3])])
        return [(functools.partial(piece, q, j), None if by_value else h_v,
                 l_v if (q // 16) % 2 and j == 3 else False, lag, 50)
                for q in range(0, HM, 16) for j in range(NT // 2)]

    def lhs_of(slot):
        return lambda k: l_v[slot, k]

    xe_v[0, 0:16, :] = jnp.zeros((16, D4), bf16)
    h_v[:, 0:PAD, :] = jnp.zeros((NT, PAD, 128), f32)
    h_v[:, PAD + S:PAD + S + PAD, :] = jnp.zeros((NT, PAD, 128), f32)

    def store_h(r0, c0, h):
        for j in range(h.shape[1] // 128):
            h_v[c0 // 128 + j, PAD + r0:PAD + r0 + h.shape[0], :] = h[:, j * 128:(j + 1) * 128]

    def h_pieces(r0, c0, t, lag, n=4):
        def piece(r, pin):
            store_h(r0 + r, c0, _gelu(pin(t[r:r + 8 * n])))
        return [(functools.partial(piece, r), None, h_v, lag, 10 * n) for r in range(0, t.shape[0], 8 * n)]

    def flush(pieces):
        for p in pieces:
            p[0](lambda v, w=128: v)

    def w1_cols(c, step):
        half, cc = c // DH2, c % DH2
        return jnp.concatenate([s1_v[RAW1[half], :, cc:cc + step], s1_v[RAW1[2 + half], :, cc:cc + step]], axis=0)

    def d1_plain(xn, r0, c0, c1, step):
        for c in range(c0, c1, step):
            store_h(r0, c, _gelu(mm(xn, w1_cols(c, step))))

    def d1_fine(lhs, r0, nrb, cols, pieces, carry, skip=0):
        tiles = [(rb, c) for c in cols for rb in range(nrb)]
        rounds = [tiles[i:i + 4] for i in range(0, len(tiles), 4)]
        for n, (rnd, part) in enumerate(zip(rounds, split(pieces, len(rounds)))):
            sk = skip if n == 0 else 0
            side = Side(_merge(carry, part) if carry else part, 8 - sk, sk)
            carry = []
            for rb, c in rnd:
                half, cc = c // DH2, c % DH2
                t = mm(lhs(rb, 0), s1_v[RAW1[half], :, cc:cc + 128], side)
                t = mm(lhs(rb, 1), s1_v[RAW1[2 + half], :, cc:cc + 128], side, t)
                carry += h_pieces(r0 + rb * HM, c, t, LS)
        return carry

    def d1_s(b, slot, pieces, carry, early=()):
        for c, part, e in zip(range(0, DH2, NC1), split(pieces, DH2 // NC1), split(early, 2) + [[], []]):
            side = Side(merge(carry, part, e), *((7,) if hist else (5, 2)))
            cs = strassen(lhs_of(slot), lambda k: s1_v[k, :, c:c + NC1], side)
            carry = sum([h_pieces(b * TM + (q // 2) * HM, (q % 2) * DH2 + c, cs[q], LS) for q in (1, 2, 3, 0)], [])
        return carry

    def d2_s(b, slot, pieces, carry=(), early=(), late=()):
        for c, part, e in zip(range(0, DH2, NC1), split(pieces, DH2 // NC1), split(early, 2) + split(late, 2)):
            side = Side(merge(carry, part, e), *((7,) if hist else (5, 2)))
            carry = ()
            idx = [(slice(b * TM + (q // 2) * HM, b * TM + (q // 2 + 1) * HM),
                    slice((q % 2) * DH2 + c, (q % 2) * DH2 + c + NC1)) for q in range(4)]
            cs = strassen(lhs_of(slot), lambda k: s2_v[k, :, c:c + NC1], side,
                          [x_v[i].astype(f32) for i in idx])
            for i, t in zip(idx, cs):
                b_v[i] = t
                if b == 0:
                    c0_v[i] = t

    def split(l, n):
        w = [1.0 if hist else 0.6] + [1.0] * (n - 1)
        cut = [int(round(len(l) * sum(w[:i]) / sum(w))) for i in range(n + 1)]
        return [l[cut[i]:cut[i + 1]] for i in range(n)]

    def merge(*ls):
        ls = [l for l in ls if l]
        return _merge(*ls) if ls else []

    NW1, NW3, N30 = 52, 32, 20
    LS, LL = 3, 5

    p3 = prep26_pieces(s3_v, LS)
    n3 = len(p3) * W3A // D4

    @once
    def _phase1a():
        wait("x0")
        xn0 = _pack(_ln(x_v[0:TM, :].astype(f32)))
        wait("w1a")
        d1_plain(xn0, 0, 0, 256, 256)
        wait("x1")
        xn1 = [_pack(_ln(x_v[r:r + HM, :].astype(f32))) for r in (TM, TM + HM)]
        for n in range(2):
            d1_plain(xn1[n], TM + n * HM, 0, 256, 256)
        wait("w1b")
        d1_plain(jnp.concatenate([xn0] + xn1, axis=0), 0, 256, 512, 256)
        wait("w1cd")
        hist.clear()
        xn01 = jnp.concatenate([xn0] + xn1, axis=0)
        l01 = lambda rb, kh: xn01[rb * 64:(rb + 1) * 64, kh * DH2:(kh + 1) * DH2]
        pw = prep_pieces(s1_v, RAW1, LS)
        flush(d1_fine(l01, 0, 4, (512, 640), pw[:NW1], [], 1))
        carry = []
        wait("x23")
        hist.clear()
        carry = d1_fine(l01, 0, 4, (768, 896), ln_pieces(x_v, 2 * TM, 0, LL), carry, 3)
        carry = d1_s(2, 0, ln_pieces(x_v, 3 * TM, 1, LL), carry, pw[NW1:])
        wait("x4567")
        qkv_start(0)
        qkv_start(1)
        hist.clear()
        for b in range(3, NB - 1):
            carry = d1_s(b, b % 2, ln_pieces(x_v, (b + 1) * TM, (b + 1) % 2, LL), carry)
        wait("w2")
        hist.clear()
        pw = prep_pieces(s2_v, RAW, LS)
        carry = d1_s(7, 1, _merge(pw[:NW3], shift_pieces(0, 0, LS, True)), carry)
        d2_s(0, 0, shift_pieces(TM, 1, LS, True), carry, pw[NW3:], p3[:N30])
        pw = split(_merge(p3[N30:n3], sum(ln_pieces(c0_v, 0, None, LL, clag=LS, staged=True), [])), 3)
        for b in range(1, 4):
            d2_s(b, b % 2, _merge(pw[b - 1], shift_pieces((b + 1) * TM, (b + 1) % 2, LS)))
        wait("w4", "small")

    hist.clear()
    pw = p3[n3:] + prep26_pieces(s4_v, LS)
    cut = (0, 33, 68, 103, len(pw))
    for b in range(4, NB):
        d2_s(b, b % 2, merge(pw[cut[b - 4]:cut[b - 3]],
                             shift_pieces((b + 1) * TM, (b + 1) % 2, LS) if b + 1 < NB else ()))
    start("wo", priority=1)

    def ffn(i, carry):
        qkv_wait(i)
        r0 = pl.multiple_of(i * TM, TM)
        rn = pl.multiple_of(jnp.minimum(i + 1, NB - 1) * TM, TM)
        acc = {}
        hist.clear()

        def relayout(p, r0_, r1_, pin):
            s0 = i * SPG + 2 * p
            e = wqkv_v[s0, r0_:r1_, :]
            o = wqkv_v[s0 + 1, r0_:r1_, :]
            wqkv_v[s0, r0_:r1_, :] = (e & jnp.uint32(0xFFFF)) | (o << 16)
            wqkv_v[s0 + 1, r0_:r1_, :] = (e >> 16) | (o & jnp.uint32(0xFFFF0000))

        relays = [(functools.partial(relayout, p, r, r + 32), wqkv_v, wqkv_v, 3, 35)
                  for p in range(SPG // 2) for r in range(0, D // 2, 32)]
        norms, combs = ln_pieces(b_v, rn, None, 5, staged=True, clag=3)

        def gate(q, pin):
            gw = gw_ref[...].astype(f32)
            x = pin(x_v[pl.ds(r0 + q, 16), :].astype(f32))
            t = functools.reduce(lambda a, b: a + b,
                                 [x[:, j * 128:(j + 1) * 128] * gw[j:j + 1, :] for j in range(NT)])
            g = jax.nn.sigmoid(jnp.sum(t, axis=-1, keepdims=True))
            g_v[pl.ds(r0 + q, 16), :] = jnp.broadcast_to(g, (16, 128))

        gates = [(functools.partial(gate, q), None, g_v, 5, 90) for q in range(0, TM, 16)]

        def extras(t, pin):
            jj, o = 2 * i + t // 2, 24 + 8 * (t % 2)
            xs = [pin(x_v[pl.ds(pl.multiple_of((jj + hh) * 64 + o, 8), 8), :].astype(f32)) for hh in (0, NPAIR // 2)]
            vals = _run(UP, [x[:, cc:cc + D4] for x in xs for cc in range(0, D, D4)])
            for k, u in enumerate(UL):
                xe_v[k, pl.ds(pl.multiple_of(i * 32 + t * 8, 8), 8), :] = vals[u].astype(bf16)

        xes = [(functools.partial(extras, t), None, xe_v, 3, 100) for t in range(4)]
        hs = {}

        def gelu_pieces(c, cs):
            def piece(r, cc, vs, pin):
                t = _gelu(pin(_cat([cs[v][r:r + 8, cc:cc + 128] for v in vs], 0)))
                ts = [t[8 * n:8 * n + 8] for n in range(len(vs))]
                hs.update({(c, v, r, cc): u for v, u in zip(vs, ts)})
                return functools.reduce(lambda a, b: a + b, ts)
            return [(functools.partial(piece, r, cc, vs), None, None, 3, 40) for r in range(0, HM, 8)
                    for cc in range(0, cs[0].shape[1], 128) for vs in ((0, 1, 2, 3), (4, 5, 6, 7))]

        def d3(c, side):
            c0, c1 = FCH[c]
            cs = fmm(lambda u: lf_v[UL.index(u), 0:HM], lambda r: s3_v[r, 0:D4, c0:c1], side)
            assert not side.pieces
            return gelu_pieces(c, cs)

        def d4(c, side):
            c0, c1 = FCH[c]
            lh = _run(UP, [_cat([_cat([hs.pop((c, v, r, cc)) for r in range(0, HM, 8)], 0)
                                 for cc in range(0, c1 - c0, 128)], 1) for v in range(8)])
            rhs = lambda r: s4_v[r, c0:c1, :]
            if c + 1 < len(FCH):
                for n in WORDER:
                    for r in range(RK):
                        if WN[r] == n:
                            acc[n] = mm(lh[UN[r]], rhs(r), side, acc.get(n))
            else:
                idx = lambda v: (pl.ds(r0 + (v // 4) * HM, HM), slice((v % 4) * D4, (v % 4 + 1) * D4))

                def extra(n):
                    if n >= 8:
                        return acc.get(n)
                    return b_v[idx(n)] + acc[n] if n in acc else b_v[idx(n)]

                def emit_b(v, t):
                    b_v[idx(v)] = jnp.concatenate([1.0 - g_v[idx(v)[0], :]] * 2, axis=1) * t
                fmm(lambda u: lh[u], rhs, side, extra, emit_b)
            assert not side.pieces

        g0 = d3(0, Side(relays[:20], 23, 3))
        g1 = d3(1, Side(_merge(g0, gates, xes), 23, 2))
        d4(0, Side(g1[:22], 22, 4))
        g2 = d3(2, Side(_merge(g1[22:], relays[20:40]), 25))
        d4(1, Side(g2, 23, 2))
        g3 = d3(3, Side(_merge(relays[40:], norms), 26))
        d4(2, Side(_merge(g3, combs), 23, 2))
        d4(3, Side([], 1))

        @pl.when(i + 2 < NG)
        def _():
            qkv_start(i + 2)

        return carry

    lax.fori_loop(0, NB, ffn, 0)

    def pre(it, carry):
        hist.clear()
        for u in range(3 * NG // NPRE):
            s0 = (it * (3 * NG // NPRE) + u) * G

            def rhs(r):
                t = None
                sz = s0 + zero_s[r]
                for q, sg in sorted(_terms(VP, 16, VN[r]).items(), key=lambda e: -e[1]):
                    blk = wqkv_v[sz + q % 4, (q // 4) * (D // 8):(q // 4 + 1) * (D // 8), :]
                    if VN[r] < 16:
                        return blk
                    blk = _unpack(blk)
                    t = blk if t is None else (t + blk if sg > 0 else t - blk)
                return t.astype(bf16)
            for v, t in enumerate(fmm(lambda k: xe_v[UL.index(k), 0:8 * NPAIR], rhs, None)):
                e_v[(v // 4) * 16:(v // 4 + 1) * 16, s0 + v % 4] = _pack(t).reshape(16, 8, DH)
        return carry

    lax.fori_loop(0, NPRE, pre, 0)

    wait("wo")
    mem_v[...] = mem0_ref[...].astype(f32)

    def slab(w, h):
        return (h // G) * SPG + w * G + h % G

    def step(j, hx, odd, late, allow, fill):
        qs, ks, vs, ps = {}, {}, {}, {}
        wload = lambda w, h: pltpu.bitcast(wqkv_v[slab(w, h)], bf16)
        eload = lambda w, h: pltpu.bitcast(e_v[j, slab(w, h)], bf16)

        def proj(g):
            part = {}
            if late and g == 0:
                for h in range(2):
                    for w in range(3):
                        part[w, h] = _dot(hx[:, :DH2], wload(w, h)[:DH2])
            for h in range(g * G, (g + 1) * G):
                q, k, v = [(_dot(hx[:, DH2:], wload(w, h)[DH2:]) + part[w, h] if (w, h) in part
                            else _dot(hx, wload(w, h))).astype(bf16) for w in range(3)]
                if odd:
                    q = jnp.concatenate([q, eload(0, h)], axis=0)
                    k = jnp.concatenate([pltpu.bitcast(ke_v[h], bf16), eload(1, h), k], axis=0)
                    v = jnp.concatenate([pltpu.bitcast(ve_v[h], bf16), eload(2, h), v], axis=0)
                else:
                    ke_v[h] = pltpu.bitcast(k, u32)
                    ve_v[h] = pltpu.bitcast(v, u32)
                    k = jnp.concatenate([k, eload(1, h)], axis=0)
                    v = jnp.concatenate([v, eload(2, h)], axis=0)
                qs[h], ks[h], vs[h] = q, k, v

        def score(g):
            for h in range(g * G, (g + 1) * G):
                s = lax.dot_general(qs.pop(h), ks.pop(h), (((1,), (1,)), ((), ())),
                                    preferred_element_type=f32)
                ps[h] = _softmax(s, allow, fill)

        def pv(g):
            os_ = []
            for h in range(g * G, (g + 1) * G):
                o = _dot(ps.pop(h), vs.pop(h))
                o_v[:, h * 128:(h + 1) * 128] = _pack(o[:32])
                os_.append(o)
            if odd:
                quads = [jnp.concatenate([os_[2 * kk][r:r + 8], os_[2 * kk + 1][r:r + 8]], axis=1)
                         for r in (32, 40) for kk in range(2)]
                for k, t in enumerate(_lcombos(*quads)):
                    oe_v[k, pl.ds(pl.multiple_of(j * 8, 8), 8), g * 256:(g + 1) * 256] = t.astype(bf16)

        acc = [None] * NT

        def wo(h0, h1, j0, j1):
            o = pltpu.bitcast(o_v[:, h0 * 128:h1 * 128], bf16)
            for n in range(j0, j1):
                y = _dot(o, pltpu.bitcast(wo_v[n, h0 * 64:h1 * 64, :], bf16))
                acc[n] = y if acc[n] is None else y + acc[n]

        for t in range(NG):
            proj(t)
            if t >= 2:
                pv(t - 2)
            if t >= 1:
                score(t - 1)
        wo(0, 16, 0, 4)
        pv(NG - 2)
        score(NG - 1)
        wo(0, 16, 4, 8)
        pv(NG - 1)
        wo(16, 24, 0, 8)
        wo(24, 32, 0, 8)
        return jnp.concatenate(acc, axis=1)

    def emit(j, r0, o0, a):
        rs = pl.ds(r0 + o0, 24)
        g = jnp.concatenate([g_v[rs, :]] * NT, axis=1)
        out_v[j, o0:o0 + 24, :] = (g * a + b_v[rs, :]).astype(bf16)

    def pair(j, mem, late):
        r0 = pl.multiple_of(j * 64, 64)
        allow_e, fill_e, allow_o, fill_o = _masks()
        xa = x_v[pl.ds(r0 + 16, 8), :].astype(f32)
        xb = x_v[pl.ds(r0 + 40, 8), :].astype(f32)
        hx = jnp.concatenate([x_v[pl.ds(r0, 16), :], jnp.concatenate([xa, mem], 0).astype(bf16)], 0)
        oe = step(j, hx, False, late, allow_e, fill_e)
        emit(j, r0, 0, oe[:24])
        hx = jnp.concatenate([jnp.concatenate([oe[24:32], xb], 0).astype(bf16), x_v[pl.ds(r0 + 48, 16), :]], 0)
        oo = step(j, hx, True, True, allow_o, fill_o)
        emit(j, r0, 40, oo[8:])
        return oo[:8]

    def a_iter(it, carry):
        mem = mem_v[...]
        for t in range(PPI):
            mem = pair(it * PPI + t, mem, t > 0)
        mem_v[...] = mem
        for t in range(PPI):
            for o0 in (0, 40):
                idx = (it * PPI + t, pl.ds(o0, 24))
                pltpu.make_async_copy(out_v.at[idx], out_hbm.at[idx], sem_out).start()
        return carry

    lax.fori_loop(0, NPAIR // PPI, a_iter, 0)

    @once
    def _post():
        hist.clear()
        for n in range(NT // 2):
            quad = [lambda k, t=2 * n + q % 2, o=(q // 2) * 128: jnp.concatenate(
                [wo_v[t + zero_s[k], g * 256 + o:g * 256 + o + 128, :] for g in range(NG)], axis=0) for q in range(4)]
            cs = strassen(lambda k: oe_v[k], lambda k: _rcombo(k, *quad), None)
            cols = slice(n * 256, (n + 1) * 256)
            for half in (1, 0):
                t = jnp.concatenate(cs[2 * half:2 * half + 2], axis=1)
                o0 = 24 + half * 8
                for jj in range(NPAIR):
                    rs = slice(jj * 64 + o0, jj * 64 + o0 + 8)
                    g = jnp.concatenate([g_v[rs, :]] * 2, axis=1)
                    out_v[jj, o0:o0 + 8, cols] = (g * t[jj * 8:jj * 8 + 8] + b_v[rs, cols]).astype(bf16)
                idx = (slice(None), pl.ds(o0, 8), pl.ds(n * 256, 256))
                pltpu.make_async_copy(out_v.at[idx], out_hbm.at[idx], sem_out).start()

    pltpu.make_async_copy(out_v, out_hbm, sem_out).wait()


@jax.jit
def pallas_gated_mix__memory_aug_recurrent_mem_tr__mixer_s_mlp__prompt_kernel(
    A_x, A_mem0, A_Wq, A_Wk, A_Wv, A_Wo, A_seg_len, B_x, B_w1, B_w2, B_w3, B_w4, gate_w,
):
    assert A_x.shape == (1, S, D) and A_mem0.shape == (1, M, D)
    any_spec = pl.BlockSpec(memory_space=pl.ANY)
    out = pl.pallas_call(
        _kernel,
        out_shape=jax.ShapeDtypeStruct((NPAIR, 64, D), bf16),
        in_specs=[any_spec] * 11,
        out_specs=any_spec,
        scratch_shapes=[
            pltpu.VMEM((S, D), bf16),
            pltpu.VMEM((9, D // 4, D // 2), u32),
            pltpu.VMEM((7, D // 4, D // 2), u32),
            pltpu.VMEM((RK + 2, D4 + 16, F4), bf16),
            pltpu.VMEM((RK + 2, F4 + 8, D4), bf16),
            pltpu.VMEM((3 * H, D // 2, DH), u32),
            pltpu.VMEM((NT, H * DH // 2 + 8, 128), u32),
            pltpu.VMEM((NT, S + 2 * PAD, 128), f32),
            pltpu.VMEM((S, D), f32),
            pltpu.VMEM((TM, D), f32),
            pltpu.VMEM((2, 7, HM // 2, D // 2), u32),
            pltpu.VMEM((len(UL), HM + 8, D4), bf16),
            pltpu.VMEM((2, TM, 128), f32),
            pltpu.VMEM((S, 128), f32),
            pltpu.VMEM((NPAIR, 64, D), bf16),
            pltpu.VMEM((len(UL), 8 * NPAIR + 8, D4), bf16),
            pltpu.VMEM((NPAIR, 3 * H, 8, DH), u32),
            pltpu.VMEM((7, 8 * NPAIR, H * DH // 2), bf16),
            pltpu.VMEM((H, 16, 128), u32),
            pltpu.VMEM((H, 16, 128), u32),
            pltpu.VMEM((16, H * DH), u32),
            pltpu.VMEM((M, D), f32),
            pltpu.VMEM((M, D), bf16),
            pltpu.VMEM((NT, 128), bf16),
            pltpu.SMEM((RK,), jnp.int32),
            pltpu.SemaphoreType.DMA((NLOAD,)),
            pltpu.SemaphoreType.DMA((NG,)),
            pltpu.SemaphoreType.DMA,
        ],
        compiler_params=pltpu.CompilerParams(vmem_limit_bytes=127 * 1024 * 1024,
                                             disable_bounds_checks=True),
    )(
        A_x.reshape(S, D), A_mem0.reshape(M, D),
        A_Wq.reshape(D // 2, 2 * H, DH), A_Wk.reshape(D // 2, 2 * H, DH), A_Wv.reshape(D // 2, 2 * H, DH),
        A_Wo.reshape(H * DH, D), B_w1, B_w2, B_w3, B_w4, gate_w.reshape(NT, 128),
    )
    return out.reshape(1, S, D)
```

```python
import functools

import jax
import jax.numpy as jnp
from jax import lax
import jax.experimental.pallas as pl
import jax.experimental.pallas.tpu as pltpu

f32, bf16, u32 = jnp.float32, jnp.bfloat16, jnp.uint32

S, D, H, DH, M, SEG, F = 2048, 1024, 32, 128, 8, 32, 3584
SCALE = DH ** -0.5
NEG = -1000000000.0
EPS = 1e-05

TM = 256
NB = S // TM
HM = TM // 2
DH2 = D // 2
D4, F4 = D // 4, F // 4
FCH = ((0, 128), (128, 384), (384, 640), (640, 896))
NC1 = 128
NPAIR = S // (2 * SEG)
PPI = 2
NPRE = 3
G = 4
NG = H // G
PAD = 8
NT = D // 128
TIEP = 2
W3A = 224
NLOAD = 11
assert NB == NG

_dot = functools.partial(jnp.dot, preferred_element_type=f32)

def _run(prog, blocks):
    vals = list(blocks)
    for a, sa, b, sb in prog:
        vals.append(vals[a] + vals[b] if sa > 0 and sb > 0 else
                    vals[a] - vals[b] if sa > 0 else vals[b] - vals[a])
    return vals


def _terms(prog, nin, node):
    if node < nin:
        return {node: 1}
    a, sa, b, sb = prog[node - nin]
    out = {k: sa * v for k, v in _terms(prog, nin, a).items()}
    out.update({k: sb * v for k, v in _terms(prog, nin, b).items()})
    return out


class _Scheme:
    def __init__(self, ms, up, vp, wp, un, vn, wn):
        self.ms, self.nb, self.rank = ms, 4 * ms, len(un)
        self.up, self.vp, self.wp, self.un, self.vn, self.wn = up, vp, wp, un, vn, wn
        self.ul = tuple(sorted(set(un)))
        t = {}
        for r in range(self.rank):
            for a, ca in _terms(up, self.nb, un[r]).items():
                for b, cb in _terms(vp, 16, vn[r]).items():
                    for c, cc in _terms(wp, self.nb, wn[r]).items():
                        t[a, b, c] = t.get((a, b, c), 0) + ca * cb * cc
        assert {k: v for k, v in t.items() if v} == {
            (4 * i + j, 4 * j + l, 4 * i + l): 1 for i in range(ms) for j in range(4) for l in range(4)}
        free = iter(r for r in range(self.rank) if vn[r] >= 16)
        self.raw = tuple(vn.index(q) if q in vn else next(free) for q in range(16))
        self.par = {n: [] for n in range(self.nb + len(wp))}
        for k, (a, sa, b, sb) in enumerate(wp):
            self.par[a].append((self.nb + k, sa))
            self.par[b].append((self.nb + k, sb))
        self.order = order = []

        def closure(n, acc):
            if n not in acc and n not in order:
                acc.add(n)
                for q, _ in self.par[n]:
                    closure(q, acc)
            return acc

        def visit(n):
            if n not in order:
                for q, _ in self.par[n]:
                    visit(q)
                order.append(n)
        while len([v for v in range(self.nb) if v not in order]):
            visit(min((v for v in range(self.nb) if v not in order), key=lambda v: len(closure(v, set()))))


UP = ((4, 1, 5, 1), (6, 1, 8, 1), (0, 1, 3, 1), (2, -1, 9, 1), (4, -1, 10, 1), (0, 1, 1, 1), (2, 1, 12, 1),
      (5, 1, 7, -1), (7, 1, 12, -1), (11, -1, 13, 1), (10, -1, 11, 1), (2, 1, 7, 1), (0, -1, 4, 1),
      (6, 1, 7, 1), (1, -1, 5, 1), (3, 1, 7, -1), (1, 1, 4, 1), (2, 1, 3, 1), (1, -1, 3, 1), (1, 1, 7, -1),
      (2, 1, 6, -1))
WP = ((0, -1, 3, 1), (4, 1, 6, -1), (1, 1, 8, 1), (5, 1, 10, 1), (4, -1, 7, 1), (0, -1, 9, -1),
      (11, 1, 12, 1), (6, 1, 7, -1), (2, 1, 5, -1), (0, -1, 7, -1), (9, 1, 11, -1), (2, 1, 13, 1),
      (5, 1, 13, 1), (2, -1, 3, 1), (5, 1, 6, 1), (0, 1, 4, 1), (2, 1, 7, 1), (1, 1, 2, 1), (1, 1, 5, 1),
      (3, 1, 7, 1), (2, 1, 6, 1))
VP = ((1, 1, 5, -1), (8, 1, 11, 1), (10, 1, 17, 1), (13, 1, 16, -1), (0, 1, 4, -1), (0, 1, 3, 1),
      (14, 1, 18, -1), (0, 1, 11, 1), (14, 1, 19, -1), (0, 1, 5, 1), (12, 1, 15, 1), (2, 1, 21, 1),
      (10, 1, 14, -1), (4, 1, 7, 1), (11, 1, 19, 1), (12, -1, 20, 1), (13, 1, 14, -1), (9, 1, 30, -1),
      (3, -1, 15, 1), (6, 1, 23, 1), (24, 1, 27, -1), (9, -1, 18, 1), (7, 1, 34, 1), (2, 1, 6, -1),
      (0, 1, 8, -1), (6, 1, 21, 1), (22, 1, 31, -1), (6, 1, 29, 1), (0, 1, 1, 1), (15, 1, 25, 1),
      (5, 1, 37, 1), (15, 1, 20, 1))
UN = (7, 27, 24, 17, 9, 22, 21, 2, 15, 11, 8, 25, 19, 28, 2, 23, 26, 20, 1, 18, 10, 28, 4, 13, 14, 16)
WN = (23, 17, 24, 10, 14, 7, 22, 19, 12, 18, 15, 25, 20, 5, 26, 0, 8, 2, 27, 11, 26, 9, 28, 21, 16, 5)
VN = (42, 47, 41, 5, 11, 43, 18, 28, 20, 23, 35, 19, 22, 46, 33, 26, 45, 36, 38, 25, 44, 40, 39, 21, 24, 32)
S26 = _Scheme(2, UP, VP, WP, UN, VN, WN)


def _twice(forms):
    prog, nodes = [], []

    def apply(f, quad):
        if len(f) == 1:
            return quad[f[0]]
        prog.append((quad[f[0]], f[1], quad[f[2]], f[3]))
        return 15 + len(prog)
    for f1 in forms:
        inner = [apply(f1, [4 * (2 * (q // 2) + p // 2) + 2 * (q % 2) + p % 2 for q in range(4)]) for p in range(4)]
        nodes += [apply(f2, inner) for f2 in forms]
    return tuple(prog), tuple(nodes)


_U2 = _twice(((0, 1, 3, 1), (2, 1, 3, 1), (0,), (3,), (0, 1, 1, 1), (2, 1, 0, -1), (1, 1, 3, -1)))
_V2 = _twice(((0, 1, 3, 1), (0,), (1, 1, 3, -1), (2, 1, 0, -1), (3,), (0, 1, 1, 1), (2, 1, 3, 1)))
_W2 = _twice(((0, 1, 3, 1), (2, 1, 3, -1), (1, 1, 3, 1), (0, 1, 2, 1), (1, 1, 0, -1), (3,), (0,)))
S49 = _Scheme(4, _U2[0], _V2[0], _W2[0], _U2[1], _V2[1], _W2[1])
VSTAGES = (((2, 5), (2, 7)), ((3, 6), (8, 13)), ((0, 1, 4), (0, 5, 10, 15)))
S49.raw = tuple(7 * (1, 2, 3, 4)[2 * (q // 8) + q % 4 // 2] + (1, 2, 3, 4)[2 * (q // 4 % 2) + q % 2] for q in range(16))
assert all(S49.raw[S49.vn[r]] == r for r in range(49) if S49.vn[r] < 16)
SF = S49
QM = TM // SF.ms


def _ln(x):
    m = jnp.mean(x, axis=-1, keepdims=True)
    xc = x - m
    v = jnp.mean(xc * xc, axis=-1, keepdims=True)
    return xc * lax.rsqrt(v + EPS)


_GC = 0.7978845608028654


def _gelu(x):
    h = 0.5 * x
    return h + h * jnp.tanh(x * (_GC + (_GC * 0.044715) * (x * x)))


def _unpack(u):
    return pltpu.bitcast(u, bf16).astype(f32)


def _pack(x):
    return pltpu.bitcast(x.astype(bf16), u32)


def _cat(xs, axis):
    xs = [x for x in xs if x.shape[axis]]
    return xs[0] if len(xs) == 1 else jnp.concatenate(xs, axis=axis)


def _as(x, dtype):
    return x if x.dtype == dtype else pltpu.bitcast(x, dtype)


def _lcombos(a11, a12, a21, a22):
    return [a11 + a22, a21 + a22, a11, a22, a11 + a12, a21 - a11, a12 - a22]


def _merge(*lists):
    keyed = [((j + 0.5) / len(l), n, j, v) for n, l in enumerate(lists) for j, v in enumerate(l)]
    return [v for _, _, _, v in sorted(keyed, key=lambda t: t[:3])]


def _masks():
    r = lax.broadcasted_iota(jnp.int32, (32, 48), 0)
    c = lax.broadcasted_iota(jnp.int32, (32, 48), 1)
    exist_e = c < 40
    allow_e = exist_e & ((r >= 24) | ((c >= 24) & (c < 32)) | (c <= r))
    fill_e = jnp.where(exist_e, NEG, -jnp.inf).astype(f32)
    r = lax.broadcasted_iota(jnp.int32, (48, 80), 0)
    c = lax.broadcasted_iota(jnp.int32, (48, 80), 1)
    q_even = (r >= 32) & (r < 40)
    exist_o = (q_even & (c < 40)) | (~q_even & (c >= 40))
    ktok = jnp.where(c < 24, c, jnp.where(c < 48, c - 8, c - 16))
    qtok = jnp.where(r < 32, r + 32, r - 8)
    is_mem_key = ((c >= 24) & (c < 32)) | ((c >= 48) & (c < 56))
    allow_o = exist_o & (is_mem_key | (r < 8) | (ktok <= qtok))
    fill_o = jnp.where(exist_o, NEG, -jnp.inf).astype(f32)
    return allow_e, fill_e, allow_o, fill_o


def _rcombo(k, b11, b12, b21, b22):
    if k in (1, 4):
        return (b11 if k == 1 else b22)(k)
    a, b, sign = {0: (b11, b22, 1), 2: (b12, b22, -1), 3: (b21, b11, -1), 5: (b11, b12, 1), 6: (b21, b22, 1)}[k]
    a, b = _unpack(a(k)), _unpack(b(k))
    return (a + b if sign > 0 else a - b).astype(bf16)


def _softmax(s, allow, fill):
    s = jnp.where(allow, s * SCALE, fill)
    m = jnp.max(s, axis=-1, keepdims=True)
    e = jnp.exp(s - m)
    l = jnp.sum(e, axis=-1, keepdims=True)
    r = pl.reciprocal(l, approx=True)
    r = r * (2.0 - l * r)
    return (e * r).astype(bf16)


def _kernel(x_hbm, mem0_hbm, wq_hbm, wk_hbm, wv_hbm, wo_hbm, w1_hbm, w2_hbm, w3_hbm, w4_hbm,
            gw_hbm, out_hbm,
            x_v, wqkv_v, wo_v, b_v, g_v, xe_v, mem_v, mem0_ref, gw_ref, zero_s,
            sem, sem_qkv, sem_out):
    RAW = (1, 2, 3, 4)
    RAW1 = (1, 7, 8, 4)

    loads = []

    def rows_load(name, r0, r1):
        loads.append((name, x_hbm.at[pl.ds(r0, r1 - r0)], x_v.at[pl.ds(r0, r1 - r0)]))

    def quad_load(name, w_hbm, s_v, raw, q, c0=0, c1=None):
        k4, n2 = s_v.shape[1], s_v.shape[2]
        c1 = n2 if c1 is None else c1
        src = w_hbm.bitcast(u32).at[pl.ds((q // 2) * k4, k4), pl.ds((q % 2) * n2 + c0, c1 - c0)]
        loads.append((name, src, s_v.at[raw[q], :, pl.ds(c0, c1 - c0)]))

    for j in range(NT):
        loads.append(("wo", wo_hbm.bitcast(u32).at[:, pl.ds(j * 128, 128)], wo_v.at[j, pl.ds(0, H * DH // 2)]))
    groups = []

    def start(*names, priority=0):
        for name, src, dst in loads:
            if name in names:
                pltpu.make_async_copy(src, dst, sem.at[groups.index(name)]).start(priority=priority)

    def wait(*names):
        for name, src, dst in loads:
            if name in names:
                pltpu.make_async_copy(src, dst, sem.at[groups.index(name)]).wait()

    SPG = 3 * G

    def qkv_start(g):
        for w, w_hbm in enumerate((wq_hbm, wk_hbm, wv_hbm)):
            wu = w_hbm.bitcast(u32)
            for k in range(G // 2):
                for par in range(2):
                    pltpu.make_async_copy(
                        wu.at[:, par * (H // 2) + g * (G // 2) + k, :],
                        wqkv_v.at[g * SPG + w * G + 2 * k + par], sem_qkv.at[g]).start(priority=1)

    def qkv_wait(g):
        grp = wqkv_v.at[pl.ds(g * SPG, SPG)]
        pltpu.make_async_copy(grp, grp, sem_qkv.at[g]).wait()

    def once(fn):
        def body(_, carry):
            fn()
            return carry
        lax.fori_loop(0, 1 + zero_s[1], body, 0)

    def tile_idx(ref, cols=128):
        z = zero_s[0]
        n = 16 if ref.dtype == bf16 and cols == 128 else 8
        return (z,) * (len(ref.shape) - 2) + (pl.ds(pl.multiple_of(z, n), n), slice(0, cols))

    hist = []

    def mm(lhs, rhs, side=None, acc=None):
        if side is not None:
            lhs = side(lhs)
        lhs = pltpu.bitcast(lhs, bf16) if lhs.dtype == u32 else lhs.astype(bf16)
        y = _dot(lhs, pltpu.bitcast(rhs, bf16) if rhs.dtype == u32 else rhs)
        if acc is not None:
            y = y + acc
        hist.append(y)
        return y

    class Side:
        def __init__(self, pieces, n, skip=0):
            cap = [0] * skip + [1] * n
            tot = sum(p[4] for p in pieces)
            self.plan = [[] for _ in cap]
            done = 0
            for p in pieces:
                done += p[4]
                x, d = done / tot * sum(cap), 0
                while x > cap[d] + 1e-9:
                    x -= cap[d]
                    d += 1
                self.plan[d].append((p, x / cap[d]))
            self.pieces = len(pieces)

        def __call__(self, val):
            todo = self.plan.pop(0) if self.plan else []
            if not todo:
                return val
            self.pieces -= len(todo)
            never = zero_s[0] > 0
            if val.dtype == bf16:
                val = pltpu.bitcast(val, u32)
            rg = 8 if val.dtype == u32 else 16
            ng = val.shape[0] // rg
            tied = {}
            for (fn, rd, wr, lag, _), pos in todo:
                m = min(max(-int(-pos * ng // 1) - 1, 0), ng - 1)
                pin = lambda v, w=128: v
                if lag is not None and len(hist) >= lag:
                    r0 = (16 * m) % hist[-lag].shape[0]
                    a = hist[-lag][r0:r0 + 8, :128]
                    if rd is None:
                        def pin(v, w=128, a=a):
                            if v.dtype == bf16:
                                return lax.select(never, _cat([a] * (v.shape[1] // 128), 1).astype(bf16), v)
                            a = _cat([_cat([_as(a, v.dtype)] * (v.shape[0] // 8), 0)] * (w // 128), 1)
                            if v.shape[1] == w:
                                return lax.select(never, a, v)
                            return _cat([lax.select(never, a, v[:, :w]), v[:, w:]], 1)
                    elif rd.dtype == bf16:
                        idx = tile_idx(rd, 256)
                        rd[idx] = lax.select(never, _cat([a, a], 1).astype(bf16), rd[idx])
                    else:
                        idx = tile_idx(rd)
                        rd[idx] = lax.select(never, _as(a, rd.dtype), rd[idx])
                u = fn(pin)
                if wr is False:
                    continue
                if wr is not None:
                    u = wr[tile_idx(wr)]
                t, n = tied.get(m * rg) or (val[m * rg:m * rg + 8, -128:], 0)
                tied[m * rg] = (lax.select(zero_s[n] > 0, _as(u, val.dtype), t), n + 1)
            if not tied:
                return val
            col, r = [], 0
            for r0 in sorted(tied):
                col += ([val[r:r0, -128:]] if r0 > r else []) + [tied[r0][0]]
                r = r0 + 8
            col += [val[r:, -128:]] if r < val.shape[0] else []
            return _cat([val[:, :-128], _cat(col, 0)], 1) if val.shape[1] > 128 else _cat(col, 0)

    def strassen(lhs, rhs, side, init=(None, None, None, None)):
        def add(a, b):
            return a if b is None else a + b
        p = [mm(lhs(k), rhs(k), side) for k in range(5)]
        c12 = add(p[2] + p[4], init[1])
        c21 = add(p[1] + p[3], init[2])
        c22 = mm(lhs(5), rhs(5), side, add(p[0] - p[1] + p[2], init[3]))
        c11 = mm(lhs(6), rhs(6), side, add(p[0] + p[3] - p[4], init[0]))
        return c11, c12, c21, c22

    def fmm(sc, lhs, rhs, side, extra=lambda n: None, emit=None):
        val = {}
        for n in sc.order:
            t = extra(n)
            for q, sg in sorted(sc.par[n], key=lambda e: -e[1]):
                t = val[q] if t is None else (t + val[q] if sg > 0 else t - val[q])
            for r in range(sc.rank):
                if sc.wn[r] == n:
                    t = mm(lhs(sc.un[r]), rhs(r), side, t)
            val[n] = t
            if n < sc.nb and emit is not None:
                emit(n, t)
        return [val[v] for v in range(sc.nb)]

    def phase_b(s1_v, s2_v, s3_v, s4_v, h_v, c0_v, l_v, lf_v, n_v):
        def w1_load(name, half, c0, c1):
            quad_load(name, w1_hbm, s1_v, RAW1, half, c0, c1)
            quad_load(name, w1_hbm, s1_v, RAW1, 2 + half, c0, c1)

        def block_load(name, w_hbm, s_v, r0, r1):
            kb, nb = s_v.shape[1] // 128 * 128, s_v.shape[2]
            for q in range(16):
                loads.append((name, w_hbm.at[pl.ds((q // 4) * kb + r0, r1 - r0), pl.ds((q % 4) * nb, nb)],
                              s_v.at[SF.raw[q], pl.ds(r0, r1 - r0)]))

        rows_load("x0", 0, TM)
        w1_load("w1a", 0, 0, 256)
        rows_load("x1", TM, 2 * TM)
        w1_load("w1b", 0, 256, 512)
        w1_load("w1cd", 1, 0, 512)
        rows_load("x23", 2 * TM, 4 * TM)
        rows_load("x4567", 4 * TM, S)
        for q in range(4):
            quad_load("w2", w2_hbm, s2_v, RAW, q)
        block_load("w2", w3_hbm, s3_v, 0, W3A)
        block_load("w4", w3_hbm, s3_v, W3A, D4)
        block_load("w4", w4_hbm, s4_v, 0, F4)
        loads.append(("small", mem0_hbm, mem0_ref))
        loads.append(("small", gw_hbm, gw_ref.at[pl.ds(0, NT)]))
        groups.extend(dict.fromkeys(name for name, _, _ in loads))
        assert len(groups) == NLOAD

        start("x0", "w1a", "w1b", "x1", "w1cd", "x23", "x4567", "w2", "w4", "small")

        def zero(k, carry):
            zero_s[k] = 0
            return carry
        lax.fori_loop(0, S26.rank, zero, 0)

        def prepf_pieces(s_v, lag):
            def piece(rs, cs, st, pin):
                z = 4 * zero_s[st]

                @functools.lru_cache(None)
                def node(n):
                    if n < 16:
                        t = s_v[z + SF.raw[n], rs, cs]
                        return (pin(t) if n in VSTAGES[st][1] else t).astype(f32)
                    a, sa, b, sb = SF.vp[n - 16]
                    return _run([(0, sa, 1, sb)], [node(a), node(b)])[-1]
                rr = [r for k in VSTAGES[st][0] for r in range(7 * k, 7 * k + 7) if SF.raw.count(r) == 0 or SF.vn[r] >= 16]
                vals = [node(SF.vn[r]).astype(bf16) for r in rr]
                for r, t in zip(rr, vals):
                    s_v[z + r, rs, cs] = t
            kb, nb = s_v.shape[1] // 128 * 128, s_v.shape[2]
            out = []
            for r in range(0, kb, 16):
                out += [(slice(rr, rr + 8), slice(c, c + 256)) for c in range(0, nb - 255, 256) for rr in (r, r + 8)]
                out += [(slice(rr, rr + 8), slice(nb - 128, nb)) for rr in (r, r + 8)] if nb % 256 else []
            return [(functools.partial(piece, rs, cs, st), None, s_v if n % TIEP == TIEP - 1 else False, lag,
                     80 if cs.stop - cs.start == 256 else 60)
                    for g in range(0, len(out), 8) for st in range(3) for n, (rs, cs) in enumerate(out[g:g + 8])]

        def prep_pieces(s_v, raw, lag, width=256):
            def piece(r, c, pin):
                idx = (slice(r, r + 8), slice(c, c + width))
                b11, b12, b21, b22 = [_unpack(pin(s_v[(q,) + idx], width) if n in (0, 3) else s_v[(q,) + idx])
                                      for n, q in enumerate(raw)]
                for k, t in ((0, b11 + b22), (2, b12 - b22), (3, b21 - b11), (5, b11 + b12), (6, b21 + b22)):
                    s_v[(k,) + idx] = _pack(t)
            return [(functools.partial(piece, r, c), None, s_v, lag, 80)
                    for c in range(0, s_v.shape[2], width) for r in range(0, s_v.shape[1], 8)]

        def store_l(slot, q, c, quads):
            for k, t in enumerate(_lcombos(*quads)):
                l_v[slot, k, q // 2:q // 2 + 8, c:c + t.shape[1]] = _pack(t)

        def ln_pieces(src, r0, slot, lag, width=256, staged=False, clag=None):
            def stats(q, pin):
                x = pin(src[pl.ds(r0 + q, 16), :].astype(f32))
                xs = [x[:, j * 128:(j + 1) * 128] for j in range(NT)]
                m = functools.reduce(lambda a, b: a + b, xs) * (1.0 / NT)
                w = functools.reduce(lambda a, b: a + b, [(t - m) * (t - m) for t in xs])
                mean = jnp.mean(m, axis=-1, keepdims=True)
                var = jnp.sum(w + NT * ((m - mean) * (m - mean)), axis=-1, keepdims=True) * (1.0 / D)
                n_v[0, q:q + 16, :] = jnp.broadcast_to(mean, (16, 128))
                n_v[1, q:q + 16, :] = jnp.broadcast_to(lax.rsqrt(var + EPS), (16, 128))

            def comb(q, c, pin):
                quads = []
                for rr in (0, HM):
                    rs = pl.ds(pl.multiple_of(r0 + rr + q + zero_s[0], 16), 16)
                    mean, rstd = [jnp.concatenate([n_v[t, rr + q:rr + q + 16, :]] * (width // 128), axis=1)
                                  for t in range(2)]
                    quads += [(src[rs, cc + c:cc + c + width].astype(f32) - mean) * rstd for cc in (0, DH2)]
                store_l(slot, q, c, quads)

            def combf(q, us, pin):
                @functools.lru_cache(None)
                def node(n):
                    if n < SF.nb:
                        rr = (n // 4) * QM + q
                        mean, rstd = [_cat([n_v[t, rr:rr + 8, :]] * 2, 1) for t in range(2)]
                        rs = pl.ds(pl.multiple_of(r0 + rr + zero_s[0], 8), 8)
                        return (src[rs, (n % 4) * D4:(n % 4 + 1) * D4] - mean) * rstd
                    a, sa, b, sb = SF.up[n - SF.nb]
                    return _run([(0, sa, 1, sb)], [node(a), node(b)])[-1]
                for u in us:
                    lf_v[SF.ul.index(u), q:q + 8, :] = node(u).astype(bf16)
            dense = slot is not None or src is b_v
            norms = [[(functools.partial(stats, rr + q), None, n_v if dense else False, lag, 90) for rr in (0, HM)]
                     for q in range(0, HM, 16)]
            if slot is None:
                parts = [[SF.un[r] for k in ks for r in range(7 * k, 7 * k + 7)] for ks in ((0, 2, 3), (4, 6), (1, 5))]
                combs = [[(functools.partial(combf, q, us), n_v, lf_v if dense or us is parts[-1] else False, clag, 100)
                          for us in parts] for q in range(0, QM, 8)]
            else:
                combs = [[(functools.partial(comb, q, c), n_v, l_v, clag, 125) for c in range(0, DH2, width)]
                         for q in range(0, HM, 16)]
            if staged:
                return sum(norms, []), sum(combs, [])
            out = list(norms[0])
            for a, b in zip(norms[1:] + [[]], combs):
                out += _merge(a, b) if a else b
            return out

        shifts = (1, 1, -1, -1, 2, 2, -2, -2)

        def shift_pieces(r0, slot, lag, by_value=False):
            def piece(q, j, pin):
                a = [h_v[jj, pl.ds(PAD + r0 + rr + q - shifts[jj], 16), :]
                     for rr in (0, HM) for jj in (j, j + NT // 2)]
                store_l(slot, q, j * 128, [pin(a[0]), a[1], a[2], pin(a[3])])
            return [(functools.partial(piece, q, j), None if by_value else h_v,
                     l_v if (q // 16) % 2 and j == 3 else False, lag, 50)
                    for q in range(0, HM, 16) for j in range(NT // 2)]

        def lhs_of(slot):
            return lambda k: l_v[slot, k]

        xe_v[0, 0:16, :] = jnp.zeros((16, D4), bf16)
        h_v[:, 0:PAD, :] = jnp.zeros((NT, PAD, 128), f32)
        h_v[:, PAD + S:PAD + S + PAD, :] = jnp.zeros((NT, PAD, 128), f32)

        def store_h(r0, c0, h):
            for j in range(h.shape[1] // 128):
                h_v[c0 // 128 + j, PAD + r0:PAD + r0 + h.shape[0], :] = h[:, j * 128:(j + 1) * 128]

        def h_pieces(r0, c0, t, lag, n=4):
            def piece(r, pin):
                store_h(r0 + r, c0, _gelu(pin(t[r:r + 8 * n])))
            return [(functools.partial(piece, r), None, h_v, lag, 10 * n) for r in range(0, t.shape[0], 8 * n)]

        def flush(pieces):
            for p in pieces:
                p[0](lambda v, w=128: v)

        def w1_cols(c, step):
            half, cc = c // DH2, c % DH2
            return jnp.concatenate([s1_v[RAW1[half], :, cc:cc + step], s1_v[RAW1[2 + half], :, cc:cc + step]], axis=0)

        def d1_plain(xn, r0, c0, c1, step):
            for c in range(c0, c1, step):
                store_h(r0, c, _gelu(mm(xn, w1_cols(c, step))))

        def d1_fine(lhs, r0, nrb, cols, pieces, carry, skip=0):
            tiles = [(rb, c) for c in cols for rb in range(nrb)]
            rounds = [tiles[i:i + 4] for i in range(0, len(tiles), 4)]
            for n, (rnd, part) in enumerate(zip(rounds, split(pieces, len(rounds)))):
                sk = skip if n == 0 else 0
                side = Side(_merge(carry, part) if carry else part, 8 - sk, sk)
                carry = []
                for rb, c in rnd:
                    half, cc = c // DH2, c % DH2
                    t = mm(lhs(rb, 0), s1_v[RAW1[half], :, cc:cc + 128], side)
                    t = mm(lhs(rb, 1), s1_v[RAW1[2 + half], :, cc:cc + 128], side, t)
                    carry += h_pieces(r0 + rb * HM, c, t, LS)
            return carry

        def d1_s(b, slot, pieces, carry, early=()):
            for c, part, e in zip(range(0, DH2, NC1), split(pieces, DH2 // NC1), split(early, 2) + [[], []]):
                side = Side(merge(carry, part, e), *((7,) if hist else (5, 2)))
                cs = strassen(lhs_of(slot), lambda k: s1_v[k, :, c:c + NC1], side)
                carry = sum([h_pieces(b * TM + (q // 2) * HM, (q % 2) * DH2 + c, cs[q], LS) for q in (1, 2, 3, 0)], [])
            return carry

        def d2_s(b, slot, pieces, carry=(), early=(), late=()):
            for c, part, e in zip(range(0, DH2, NC1), split(pieces, DH2 // NC1), split(early, 2) + split(late, 2)):
                side = Side(merge(carry, part, e), *((7,) if hist else (5, 2)))
                carry = ()
                idx = [(slice(b * TM + (q // 2) * HM, b * TM + (q // 2 + 1) * HM),
                        slice((q % 2) * DH2 + c, (q % 2) * DH2 + c + NC1)) for q in range(4)]
                cs = strassen(lhs_of(slot), lambda k: s2_v[k, :, c:c + NC1], side,
                              [x_v[i].astype(f32) for i in idx])
                for i, t in zip(idx, cs):
                    b_v[i] = t
                    if b == 0:
                        c0_v[i] = t

        def split(l, n):
            w = [1.0 if hist else 0.6] + [1.0] * (n - 1)
            cut = [int(round(len(l) * sum(w[:i]) / sum(w))) for i in range(n + 1)]
            return [l[cut[i]:cut[i + 1]] for i in range(n)]

        def merge(*ls):
            ls = [l for l in ls if l]
            return _merge(*ls) if ls else []

        NW1, NW3, N30 = 52, 32, 48
        LS, LL = 3, 5

        p3 = prepf_pieces(s3_v, LS)
        n3 = len(p3) * W3A // D4

        @once
        def _phase1a():
            wait("x0")
            xn0 = _pack(_ln(x_v[0:TM, :].astype(f32)))
            wait("w1a")
            d1_plain(xn0, 0, 0, 256, 256)
            wait("x1")
            xn1 = [_pack(_ln(x_v[r:r + HM, :].astype(f32))) for r in (TM, TM + HM)]
            for n in range(2):
                d1_plain(xn1[n], TM + n * HM, 0, 256, 256)
            wait("w1b")
            d1_plain(jnp.concatenate([xn0] + xn1, axis=0), 0, 256, 512, 256)
            wait("w1cd")
            hist.clear()
            xn01 = jnp.concatenate([xn0] + xn1, axis=0)
            l01 = lambda rb, kh: xn01[rb * 64:(rb + 1) * 64, kh * DH2:(kh + 1) * DH2]
            pw = prep_pieces(s1_v, RAW1, LS)
            flush(d1_fine(l01, 0, 4, (512, 640), pw[:NW1], [], 1))
            carry = []
            wait("x23")
            hist.clear()
            carry = d1_fine(l01, 0, 4, (768, 896), ln_pieces(x_v, 2 * TM, 0, LL), carry, 3)
            carry = d1_s(2, 0, ln_pieces(x_v, 3 * TM, 1, LL), carry, pw[NW1:])
            wait("x4567")
            qkv_start(0)
            qkv_start(1)
            hist.clear()
            for b in range(3, NB - 1):
                carry = d1_s(b, b % 2, ln_pieces(x_v, (b + 1) * TM, (b + 1) % 2, LL), carry)
            wait("w2")
            hist.clear()
            pw = prep_pieces(s2_v, RAW, LS)
            carry = d1_s(7, 1, _merge(pw[:NW3], shift_pieces(0, 0, LS, True)), carry)
            d2_s(0, 0, shift_pieces(TM, 1, LS, True), carry, pw[NW3:], p3[:N30])
            pw = split(_merge(p3[N30:n3], sum(ln_pieces(c0_v, 0, None, LL, clag=LS, staged=True), [])), 3)
            for b in range(1, 4):
                d2_s(b, b % 2, _merge(pw[b - 1], shift_pieces((b + 1) * TM, (b + 1) % 2, LS)))
            wait("w4", "small")

        hist.clear()
        pw = p3[n3:] + prepf_pieces(s4_v, LS)
        cut = (0, 87, 180, 273) + (len(pw),)
        for b in range(4, NB):
            d2_s(b, b % 2, merge(pw[cut[b - 4]:cut[b - 3]],
                                 shift_pieces((b + 1) * TM, (b + 1) % 2, LS) if b + 1 < NB else ()))
        start("wo", priority=1)

        def ffn(i, carry):
            qkv_wait(i)
            r0 = pl.multiple_of(i * TM, TM)
            rn = pl.multiple_of(jnp.minimum(i + 1, NB - 1) * TM, TM)
            acc = {}
            hist.clear()
            LG = 6

            def relayout(p, r0_, r1_, pin):
                s0 = i * SPG + 2 * p
                e = wqkv_v[s0, r0_:r1_, :]
                o = wqkv_v[s0 + 1, r0_:r1_, :]
                wqkv_v[s0, r0_:r1_, :] = (e & jnp.uint32(0xFFFF)) | (o << 16)
                wqkv_v[s0 + 1, r0_:r1_, :] = (e >> 16) | (o & jnp.uint32(0xFFFF0000))

            relays = [(functools.partial(relayout, p, r, r + 32), wqkv_v, wqkv_v, LG, 35)
                      for p in range(SPG // 2) for r in range(0, D // 2, 32)]
            norms, combs = ln_pieces(b_v, rn, None, 10, staged=True, clag=LG)

            def gate(q, pin):
                gw = gw_ref[0:NT, :].astype(f32)
                x = pin(x_v[pl.ds(r0 + q, 16), :].astype(f32))
                t = functools.reduce(lambda a, b: a + b,
                                     [x[:, j * 128:(j + 1) * 128] * gw[j:j + 1, :] for j in range(NT)])
                g = jax.nn.sigmoid(jnp.sum(t, axis=-1, keepdims=True))
                g_v[pl.ds(r0 + q, 16), :] = jnp.broadcast_to(g, (16, 128))

            gates = [(functools.partial(gate, q), None, g_v, 10, 90) for q in range(0, TM, 16)]

            def extras(t, pin):
                jj, o = 2 * i + t // 2, 24 + 8 * (t % 2)
                xs = [pin(x_v[pl.ds(pl.multiple_of((jj + hh) * 64 + o, 8), 8), :].astype(f32)) for hh in (0, NPAIR // 2)]
                vals = _run(S26.up, [x[:, cc:cc + D4] for x in xs for cc in range(0, D, D4)])
                for k, u in enumerate(S26.ul):
                    xe_v[k, pl.ds(pl.multiple_of(i * 32 + t * 8, 8), 8), :] = vals[u].astype(bf16)

            xes = [(functools.partial(extras, t), None, xe_v, LG, 100) for t in range(4)]
            hs = {}

            def gelu_pieces(c, cs):
                def piece(r, cc, vs, pin):
                    t = _gelu(pin(_cat([cs[v][r:r + 8, cc:cc + 128] for v in vs], 0)))
                    ts = [t[8 * n:8 * n + 8] for n in range(len(vs))]
                    hs.update({(c, v, r, cc): u for v, u in zip(vs, ts)})
                    return functools.reduce(lambda a, b: a + b, ts)
                return [(functools.partial(piece, r, cc, range(v, v + 4)), None, None, LG, 40) for r in range(0, QM, 8)
                        for cc in range(0, cs[0].shape[1], 128) for v in range(0, SF.nb, 4)]

            def d3(c, side):
                c0, c1 = FCH[c]
                cs = fmm(SF, lambda u: lf_v[SF.ul.index(u), 0:QM], lambda r: s3_v[r, 0:D4, c0:c1], side)
                assert not side.pieces
                return gelu_pieces(c, cs)

            def d4(c, side):
                c0, c1 = FCH[c]
                lh = _run(SF.up, [_cat([_cat([hs.pop((c, v, r, cc)) for r in range(0, QM, 8)], 0)
                                        for cc in range(0, c1 - c0, 128)], 1) for v in range(SF.nb)])
                rhs = lambda r: s4_v[r, c0:c1, :]
                if c + 1 < len(FCH):
                    for n in SF.order:
                        for r in range(SF.rank):
                            if SF.wn[r] == n:
                                acc[n] = mm(lh[SF.un[r]], rhs(r), side, acc.get(n))
                else:
                    idx = lambda v: (pl.ds(r0 + (v // 4) * QM, QM), slice((v % 4) * D4, (v % 4 + 1) * D4))

                    def extra(n):
                        if n >= SF.nb:
                            return acc.get(n)
                        return b_v[idx(n)] + acc[n] if n in acc else b_v[idx(n)]

                    def emit_b(v, t):
                        b_v[idx(v)] = jnp.concatenate([1.0 - g_v[idx(v)[0], :]] * 2, axis=1) * t
                    fmm(SF, lambda u: lh[u], rhs, side, extra, emit_b)
                assert not side.pieces

            g0 = d3(0, Side(relays[:20], 43, 6))
            g1 = d3(1, Side(_merge(g0, gates, xes), 43, 4))
            d4(0, Side(g1[:22], 41, 8))
            g2 = d3(2, Side(_merge(g1[22:], relays[20:40]), 47))
            d4(1, Side(g2, 43, 4))
            g3 = d3(3, Side(_merge(relays[40:], norms), 49))
            d4(2, Side(_merge(g3, combs), 43, 4))
            d4(3, Side([], 1))

            @pl.when(i + 2 < NG)
            def _():
                qkv_start(i + 2)

            return carry

        lax.fori_loop(0, NB, ffn, 0)

    pl.run_scoped(
        phase_b,
        pltpu.VMEM((9, D // 4, D // 2), u32),
        pltpu.VMEM((7, D // 4, D // 2), u32),
        pltpu.VMEM((52, D4 + 16, F4), bf16),
        pltpu.VMEM((52, F4 + 8, D4), bf16),
        pltpu.VMEM((NT, S + 2 * PAD, 128), f32),
        pltpu.VMEM((TM, D), f32),
        pltpu.VMEM((2, 7, HM // 2, D // 2), u32),
        pltpu.VMEM((52, QM + 8, D4), bf16),
        pltpu.VMEM((2, TM, 128), f32),
    )

    def phase_a(out_v, e_v, oe_v, ke_v, ve_v, o_v):
        def pre(it, carry):
            hist.clear()
            for u in range(3 * NG // NPRE):
                s0 = (it * (3 * NG // NPRE) + u) * G

                def rhs(r):
                    t = None
                    sz = s0 + zero_s[r]
                    for q, sg in sorted(_terms(S26.vp, 16, S26.vn[r]).items(), key=lambda e: -e[1]):
                        blk = wqkv_v[sz + q % 4, (q // 4) * (D // 8):(q // 4 + 1) * (D // 8), :]
                        if S26.vn[r] < 16:
                            return blk
                        blk = _unpack(blk)
                        t = blk if t is None else (t + blk if sg > 0 else t - blk)
                    return t.astype(bf16)
                for v, t in enumerate(fmm(S26, lambda k: xe_v[S26.ul.index(k), 0:8 * NPAIR], rhs, None)):
                    e_v[(v // 4) * 16:(v // 4 + 1) * 16, s0 + v % 4] = _pack(t).reshape(16, 8, DH)
            return carry

        lax.fori_loop(0, NPRE, pre, 0)

        wait("wo")
        mem_v[...] = mem0_ref[...].astype(f32)

        def slab(w, h):
            return (h // G) * SPG + w * G + h % G

        def step(j, hx, odd, late, allow, fill):
            qs, ks, vs, ps = {}, {}, {}, {}
            wload = lambda w, h: pltpu.bitcast(wqkv_v[slab(w, h)], bf16)
            eload = lambda w, h: pltpu.bitcast(e_v[j, slab(w, h)], bf16)

            def proj(g):
                part = {}
                if late and g == 0:
                    for h in range(2):
                        for w in range(3):
                            part[w, h] = _dot(hx[:, :DH2], wload(w, h)[:DH2])
                for h in range(g * G, (g + 1) * G):
                    q, k, v = [(_dot(hx[:, DH2:], wload(w, h)[DH2:]) + part[w, h] if (w, h) in part
                                else _dot(hx, wload(w, h))).astype(bf16) for w in range(3)]
                    if odd:
                        q = jnp.concatenate([q, eload(0, h)], axis=0)
                        k = jnp.concatenate([pltpu.bitcast(ke_v[h], bf16), eload(1, h), k], axis=0)
                        v = jnp.concatenate([pltpu.bitcast(ve_v[h], bf16), eload(2, h), v], axis=0)
                    else:
                        ke_v[h] = pltpu.bitcast(k, u32)
                        ve_v[h] = pltpu.bitcast(v, u32)
                        k = jnp.concatenate([k, eload(1, h)], axis=0)
                        v = jnp.concatenate([v, eload(2, h)], axis=0)
                    qs[h], ks[h], vs[h] = q, k, v

            def score(g):
                for h in range(g * G, (g + 1) * G):
                    s = lax.dot_general(qs.pop(h), ks.pop(h), (((1,), (1,)), ((), ())),
                                        preferred_element_type=f32)
                    ps[h] = _softmax(s, allow, fill)

            def pv(g):
                os_ = []
                for h in range(g * G, (g + 1) * G):
                    o = _dot(ps.pop(h), vs.pop(h))
                    o_v[:, h * 128:(h + 1) * 128] = _pack(o[:32])
                    os_.append(o)
                if odd:
                    quads = [jnp.concatenate([os_[2 * kk][r:r + 8], os_[2 * kk + 1][r:r + 8]], axis=1)
                             for r in (32, 40) for kk in range(2)]
                    for k, t in enumerate(_lcombos(*quads)):
                        oe_v[k, pl.ds(pl.multiple_of(j * 8, 8), 8), g * 256:(g + 1) * 256] = t.astype(bf16)

            acc = [None] * NT

            def wo(h0, h1, j0, j1):
                o = pltpu.bitcast(o_v[:, h0 * 128:h1 * 128], bf16)
                for n in range(j0, j1):
                    y = _dot(o, pltpu.bitcast(wo_v[n, h0 * 64:h1 * 64, :], bf16))
                    acc[n] = y if acc[n] is None else y + acc[n]

            for t in range(NG):
                proj(t)
                if t >= 2:
                    pv(t - 2)
                if t >= 1:
                    score(t - 1)
            wo(0, 16, 0, 4)
            pv(NG - 2)
            score(NG - 1)
            wo(0, 16, 4, 8)
            pv(NG - 1)
            wo(16, 24, 0, 8)
            wo(24, 32, 0, 8)
            return jnp.concatenate(acc, axis=1)

        def emit(j, r0, o0, a):
            rs = pl.ds(r0 + o0, 24)
            g = jnp.concatenate([g_v[rs, :]] * NT, axis=1)
            out_v[j, o0:o0 + 24, :] = (g * a + b_v[rs, :]).astype(bf16)

        def pair(j, mem, late):
            r0 = pl.multiple_of(j * 64, 64)
            allow_e, fill_e, allow_o, fill_o = _masks()
            xa = x_v[pl.ds(r0 + 16, 8), :].astype(f32)
            xb = x_v[pl.ds(r0 + 40, 8), :].astype(f32)
            hx = jnp.concatenate([x_v[pl.ds(r0, 16), :], jnp.concatenate([xa, mem], 0).astype(bf16)], 0)
            oe = step(j, hx, False, late, allow_e, fill_e)
            emit(j, r0, 0, oe[:24])
            hx = jnp.concatenate([jnp.concatenate([oe[24:32], xb], 0).astype(bf16), x_v[pl.ds(r0 + 48, 16), :]], 0)
            oo = step(j, hx, True, True, allow_o, fill_o)
            emit(j, r0, 40, oo[8:])
            return oo[:8]

        def a_iter(it, carry):
            mem = mem_v[...]
            for t in range(PPI):
                mem = pair(it * PPI + t, mem, t > 0)
            mem_v[...] = mem
            for t in range(PPI):
                for o0 in (0, 40):
                    idx = (it * PPI + t, pl.ds(o0, 24))
                    pltpu.make_async_copy(out_v.at[idx], out_hbm.at[idx], sem_out).start()
            return carry

        lax.fori_loop(0, NPAIR // PPI, a_iter, 0)

        @once
        def _post():
            hist.clear()
            for n in range(NT // 2):
                quad = [lambda k, t=2 * n + q % 2, o=(q // 2) * 128: jnp.concatenate(
                    [wo_v[t + zero_s[k], g * 256 + o:g * 256 + o + 128, :] for g in range(NG)], axis=0) for q in range(4)]
                cs = strassen(lambda k: oe_v[k], lambda k: _rcombo(k, *quad), None)
                cols = slice(n * 256, (n + 1) * 256)
                for half in (1, 0):
                    t = jnp.concatenate(cs[2 * half:2 * half + 2], axis=1)
                    o0 = 24 + half * 8
                    for jj in range(NPAIR):
                        rs = slice(jj * 64 + o0, jj * 64 + o0 + 8)
                        g = jnp.concatenate([g_v[rs, :]] * 2, axis=1)
                        out_v[jj, o0:o0 + 8, cols] = (g * t[jj * 8:jj * 8 + 8] + b_v[rs, cols]).astype(bf16)
                    idx = (slice(None), pl.ds(o0, 8), pl.ds(n * 256, 256))
                    pltpu.make_async_copy(out_v.at[idx], out_hbm.at[idx], sem_out).start()

        pltpu.make_async_copy(out_v, out_hbm, sem_out).wait()

    pl.run_scoped(
        phase_a,
        pltpu.VMEM((NPAIR, 64, D), bf16),
        pltpu.VMEM((NPAIR, 3 * H, 8, DH), u32),
        pltpu.VMEM((7, 8 * NPAIR, H * DH // 2), bf16),
        pltpu.VMEM((H, 16, 128), u32),
        pltpu.VMEM((H, 16, 128), u32),
        pltpu.VMEM((16, H * DH), u32),
    )


@jax.jit
def pallas_gated_mix__memory_aug_recurrent_mem_tr__mixer_s_mlp__prompt_kernel(
    A_x, A_mem0, A_Wq, A_Wk, A_Wv, A_Wo, A_seg_len, B_x, B_w1, B_w2, B_w3, B_w4, gate_w,
):
    assert A_x.shape == (1, S, D) and A_mem0.shape == (1, M, D)
    any_spec = pl.BlockSpec(memory_space=pl.ANY)
    out = pl.pallas_call(
        _kernel,
        out_shape=jax.ShapeDtypeStruct((NPAIR, 64, D), bf16),
        in_specs=[any_spec] * 11,
        out_specs=any_spec,
        scratch_shapes=[
            pltpu.VMEM((S, D), bf16),
            pltpu.VMEM((3 * H, D // 2, DH), u32),
            pltpu.VMEM((NT, H * DH // 2 + 8, 128), u32),
            pltpu.VMEM((S, D), f32),
            pltpu.VMEM((S, 128), f32),
            pltpu.VMEM((len(S26.ul), 8 * NPAIR + 8, D4), bf16),
            pltpu.VMEM((M, D), f32),
            pltpu.VMEM((M, D), bf16),
            pltpu.VMEM((64, 128), bf16),
            pltpu.SMEM((S26.rank,), jnp.int32),
            pltpu.SemaphoreType.DMA((NLOAD,)),
            pltpu.SemaphoreType.DMA((NG,)),
            pltpu.SemaphoreType.DMA,
        ],
        compiler_params=pltpu.CompilerParams(vmem_limit_bytes=127 * 1024 * 1024,
                                             disable_bounds_checks=True),
    )(
        A_x.reshape(S, D), A_mem0.reshape(M, D),
        A_Wq.reshape(D // 2, 2 * H, DH), A_Wk.reshape(D // 2, 2 * H, DH), A_Wv.reshape(D // 2, 2 * H, DH),
        A_Wo.reshape(H * DH, D), B_w1, B_w2, B_w3, B_w4, gate_w.reshape(NT, 128),
    )
    return out.reshape(1, S, D)
```

```python
import functools

import jax
import jax.numpy as jnp
from jax import lax
import jax.experimental.pallas as pl
import jax.experimental.pallas.tpu as pltpu

f32, bf16, u32 = jnp.float32, jnp.bfloat16, jnp.uint32

S, D, H, DH, M, SEG, F = 2048, 1024, 32, 128, 8, 32, 3584
SCALE = DH ** -0.5
NEG = -1000000000.0
EPS = 1e-05

TM = 256
NB = S // TM
HM = TM // 2
DH2 = D // 2
D4, F4 = D // 4, F // 4
FCH = ((0, 128), (128, 384), (384, 640), (640, 896))
NC1 = 128
NPAIR = S // (2 * SEG)
PPI = 2
NPRE = 3
G = 4
NG = H // G
PAD = 8
NT = D // 128
TIEP = 2
W3A = 208
NLOAD = 11
assert NB == NG

_dot = functools.partial(jnp.dot, preferred_element_type=f32)

def _run(prog, blocks):
    vals = list(blocks)
    for a, sa, b, sb in prog:
        vals.append(vals[a] + vals[b] if sa > 0 and sb > 0 else
                    vals[a] - vals[b] if sa > 0 else vals[b] - vals[a])
    return vals


def _terms(prog, nin, node):
    if node < nin:
        return {node: 1}
    a, sa, b, sb = prog[node - nin]
    out = {k: sa * v for k, v in _terms(prog, nin, a).items()}
    out.update({k: sb * v for k, v in _terms(prog, nin, b).items()})
    return out


class _Scheme:
    def __init__(self, ms, up, vp, wp, un, vn, wn):
        self.ms, self.nb, self.rank = ms, 4 * ms, len(un)
        self.up, self.vp, self.wp, self.un, self.vn, self.wn = up, vp, wp, un, vn, wn
        self.ul = tuple(sorted(set(un)))
        t = {}
        for r in range(self.rank):
            for a, ca in _terms(up, self.nb, un[r]).items():
                for b, cb in _terms(vp, 16, vn[r]).items():
                    for c, cc in _terms(wp, self.nb, wn[r]).items():
                        t[a, b, c] = t.get((a, b, c), 0) + ca * cb * cc
        assert {k: v for k, v in t.items() if v} == {
            (4 * i + j, 4 * j + l, 4 * i + l): 1 for i in range(ms) for j in range(4) for l in range(4)}
        free = iter(r for r in range(self.rank) if vn[r] >= 16)
        self.raw = tuple(vn.index(q) if q in vn else next(free) for q in range(16))
        self.par = {n: [] for n in range(self.nb + len(wp))}
        for k, (a, sa, b, sb) in enumerate(wp):
            self.par[a].append((self.nb + k, sa))
            self.par[b].append((self.nb + k, sb))
        self.order = order = []

        def closure(n, acc):
            if n not in acc and n not in order:
                acc.add(n)
                for q, _ in self.par[n]:
                    closure(q, acc)
            return acc

        def visit(n):
            if n not in order:
                for q, _ in self.par[n]:
                    visit(q)
                order.append(n)
        while len([v for v in range(self.nb) if v not in order]):
            visit(min((v for v in range(self.nb) if v not in order), key=lambda v: len(closure(v, set()))))


UP = ((4, 1, 5, 1), (6, 1, 8, 1), (0, 1, 3, 1), (2, -1, 9, 1), (4, -1, 10, 1), (0, 1, 1, 1), (2, 1, 12, 1),
      (5, 1, 7, -1), (7, 1, 12, -1), (11, -1, 13, 1), (10, -1, 11, 1), (2, 1, 7, 1), (0, -1, 4, 1),
      (6, 1, 7, 1), (1, -1, 5, 1), (3, 1, 7, -1), (1, 1, 4, 1), (2, 1, 3, 1), (1, -1, 3, 1), (1, 1, 7, -1),
      (2, 1, 6, -1))
WP = ((0, -1, 3, 1), (4, 1, 6, -1), (1, 1, 8, 1), (5, 1, 10, 1), (4, -1, 7, 1), (0, -1, 9, -1),
      (11, 1, 12, 1), (6, 1, 7, -1), (2, 1, 5, -1), (0, -1, 7, -1), (9, 1, 11, -1), (2, 1, 13, 1),
      (5, 1, 13, 1), (2, -1, 3, 1), (5, 1, 6, 1), (0, 1, 4, 1), (2, 1, 7, 1), (1, 1, 2, 1), (1, 1, 5, 1),
      (3, 1, 7, 1), (2, 1, 6, 1))
VP = ((1, 1, 5, -1), (8, 1, 11, 1), (10, 1, 17, 1), (13, 1, 16, -1), (0, 1, 4, -1), (0, 1, 3, 1),
      (14, 1, 18, -1), (0, 1, 11, 1), (14, 1, 19, -1), (0, 1, 5, 1), (12, 1, 15, 1), (2, 1, 21, 1),
      (10, 1, 14, -1), (4, 1, 7, 1), (11, 1, 19, 1), (12, -1, 20, 1), (13, 1, 14, -1), (9, 1, 30, -1),
      (3, -1, 15, 1), (6, 1, 23, 1), (24, 1, 27, -1), (9, -1, 18, 1), (7, 1, 34, 1), (2, 1, 6, -1),
      (0, 1, 8, -1), (6, 1, 21, 1), (22, 1, 31, -1), (6, 1, 29, 1), (0, 1, 1, 1), (15, 1, 25, 1),
      (5, 1, 37, 1), (15, 1, 20, 1))
UN = (7, 27, 24, 17, 9, 22, 21, 2, 15, 11, 8, 25, 19, 28, 2, 23, 26, 20, 1, 18, 10, 28, 4, 13, 14, 16)
WN = (23, 17, 24, 10, 14, 7, 22, 19, 12, 18, 15, 25, 20, 5, 26, 0, 8, 2, 27, 11, 26, 9, 28, 21, 16, 5)
VN = (42, 47, 41, 5, 11, 43, 18, 28, 20, 23, 35, 19, 22, 46, 33, 26, 45, 36, 38, 25, 44, 40, 39, 21, 24, 32)
S26 = _Scheme(2, UP, VP, WP, UN, VN, WN)


def _twice(forms):
    prog, nodes = [], []

    def apply(f, quad):
        if len(f) == 1:
            return quad[f[0]]
        prog.append((quad[f[0]], f[1], quad[f[2]], f[3]))
        return 15 + len(prog)
    for f1 in forms:
        inner = [apply(f1, [4 * (2 * (q // 2) + p // 2) + 2 * (q % 2) + p % 2 for q in range(4)]) for p in range(4)]
        nodes += [apply(f2, inner) for f2 in forms]
    return tuple(prog), tuple(nodes)


_U2 = _twice(((0, 1, 3, 1), (2, 1, 3, 1), (0,), (3,), (0, 1, 1, 1), (2, 1, 0, -1), (1, 1, 3, -1)))
_V2 = _twice(((0, 1, 3, 1), (0,), (1, 1, 3, -1), (2, 1, 0, -1), (3,), (0, 1, 1, 1), (2, 1, 3, 1)))
_W2 = _twice(((0, 1, 3, 1), (2, 1, 3, -1), (1, 1, 3, 1), (0, 1, 2, 1), (1, 1, 0, -1), (3,), (0,)))
S49 = _Scheme(4, _U2[0], _V2[0], _W2[0], _U2[1], _V2[1], _W2[1])
VSTAGES = (((2, 5), (2, 7)), ((3, 6), (8, 13)), ((0, 1, 4), (0, 5, 10, 15)))
S49.raw = tuple(7 * (1, 2, 3, 4)[2 * (q // 8) + q % 4 // 2] + (1, 2, 3, 4)[2 * (q // 4 % 2) + q % 2] for q in range(16))
assert all(S49.raw[S49.vn[r]] == r for r in range(49) if S49.vn[r] < 16)
SF = S49
QM = TM // SF.ms


def _ln(x):
    m = jnp.mean(x, axis=-1, keepdims=True)
    xc = x - m
    v = jnp.mean(xc * xc, axis=-1, keepdims=True)
    return xc * lax.rsqrt(v + EPS)


_GC = 0.7978845608028654


def _gelu(x):
    h = 0.5 * x
    return h + h * jnp.tanh(x * (_GC + (_GC * 0.044715) * (x * x)))


def _unpack(u):
    return pltpu.bitcast(u, bf16).astype(f32)


def _pack(x):
    return pltpu.bitcast(x.astype(bf16), u32)


def _cat(xs, axis):
    xs = [x for x in xs if x.shape[axis]]
    return xs[0] if len(xs) == 1 else jnp.concatenate(xs, axis=axis)


def _as(x, dtype):
    return x if x.dtype == dtype else pltpu.bitcast(x, dtype)


def _lcombos(a11, a12, a21, a22):
    return [a11 + a22, a21 + a22, a11, a22, a11 + a12, a21 - a11, a12 - a22]


def _merge(*lists):
    keyed = [((j + 0.5) / len(l), n, j, v) for n, l in enumerate(lists) for j, v in enumerate(l)]
    return [v for _, _, _, v in sorted(keyed, key=lambda t: t[:3])]


def _masks():
    r = lax.broadcasted_iota(jnp.int32, (32, 48), 0)
    c = lax.broadcasted_iota(jnp.int32, (32, 48), 1)
    exist_e = c < 40
    allow_e = exist_e & ((r >= 24) | ((c >= 24) & (c < 32)) | (c <= r))
    fill_e = jnp.where(exist_e, NEG, -jnp.inf).astype(f32)
    r = lax.broadcasted_iota(jnp.int32, (48, 80), 0)
    c = lax.broadcasted_iota(jnp.int32, (48, 80), 1)
    q_even = (r >= 32) & (r < 40)
    exist_o = (q_even & (c < 40)) | (~q_even & (c >= 40))
    ktok = jnp.where(c < 24, c, jnp.where(c < 48, c - 8, c - 16))
    qtok = jnp.where(r < 32, r + 32, r - 8)
    is_mem_key = ((c >= 24) & (c < 32)) | ((c >= 48) & (c < 56))
    allow_o = exist_o & (is_mem_key | (r < 8) | (ktok <= qtok))
    fill_o = jnp.where(exist_o, NEG, -jnp.inf).astype(f32)
    return allow_e, fill_e, allow_o, fill_o


def _rcombo(k, b11, b12, b21, b22):
    if k in (1, 4):
        return (b11 if k == 1 else b22)(k)
    a, b, sign = {0: (b11, b22, 1), 2: (b12, b22, -1), 3: (b21, b11, -1), 5: (b11, b12, 1), 6: (b21, b22, 1)}[k]
    a, b = _unpack(a(k)), _unpack(b(k))
    return (a + b if sign > 0 else a - b).astype(bf16)


def _softmax(s, allow, fill):
    s = jnp.where(allow, s * SCALE, fill)
    m = jnp.max(s, axis=-1, keepdims=True)
    e = jnp.exp(s - m)
    l = jnp.sum(e, axis=-1, keepdims=True)
    r = pl.reciprocal(l, approx=True)
    r = r * (2.0 - l * r)
    return (e * r).astype(bf16)


def _kernel(x_hbm, mem0_hbm, wq_hbm, wk_hbm, wv_hbm, wo_hbm, w1_hbm, w2_hbm, w3_hbm, w4_hbm,
            gw_hbm, out_hbm,
            x_v, wqkv_v, wo_v, b_v, g_v, xe_v, mem_v, mem0_ref, gw_ref, zero_s,
            sem, sem_qkv, sem_out):
    RAW = (1, 2, 3, 4)
    RAW1 = (1, 7, 8, 4)

    loads = []

    def rows_load(name, r0, r1):
        loads.append((name, x_hbm.at[pl.ds(r0, r1 - r0)], x_v.at[pl.ds(r0, r1 - r0)]))

    def quad_load(name, w_hbm, s_v, raw, q, c0=0, c1=None):
        k4, n2 = s_v.shape[1], s_v.shape[2]
        c1 = n2 if c1 is None else c1
        src = w_hbm.bitcast(u32).at[pl.ds((q // 2) * k4, k4), pl.ds((q % 2) * n2 + c0, c1 - c0)]
        loads.append((name, src, s_v.at[raw[q], :, pl.ds(c0, c1 - c0)]))

    for j in range(NT):
        loads.append(("wo", wo_hbm.bitcast(u32).at[:, pl.ds(j * 128, 128)], wo_v.at[j, pl.ds(0, H * DH // 2)]))
    groups = []

    def start(*names, priority=0):
        for name, src, dst in loads:
            if name in names:
                pltpu.make_async_copy(src, dst, sem.at[groups.index(name)]).start(priority=priority)

    def wait(*names):
        for name, src, dst in loads:
            if name in names:
                pltpu.make_async_copy(src, dst, sem.at[groups.index(name)]).wait()

    SPG = 3 * G

    def qkv_start(g):
        for w, w_hbm in enumerate((wq_hbm, wk_hbm, wv_hbm)):
            wu = w_hbm.bitcast(u32)
            for k in range(G // 2):
                for par in range(2):
                    pltpu.make_async_copy(
                        wu.at[:, par * (H // 2) + g * (G // 2) + k, :],
                        wqkv_v.at[g * SPG + w * G + 2 * k + par], sem_qkv.at[g]).start(priority=1)

    def qkv_wait(g):
        grp = wqkv_v.at[pl.ds(g * SPG, SPG)]
        pltpu.make_async_copy(grp, grp, sem_qkv.at[g]).wait()

    def once(fn):
        def body(_, carry):
            fn()
            return carry
        lax.fori_loop(0, 1 + zero_s[1], body, 0)

    def tile_idx(ref, cols=128):
        z = zero_s[0]
        n = 16 if ref.dtype == bf16 and cols == 128 else 8
        return (z,) * (len(ref.shape) - 2) + (pl.ds(pl.multiple_of(z, n), n), slice(0, cols))

    hist = []

    def mm(lhs, rhs, side=None, acc=None):
        if side is not None:
            lhs = side(lhs)
        lhs = pltpu.bitcast(lhs, bf16) if lhs.dtype == u32 else lhs.astype(bf16)
        y = _dot(lhs, pltpu.bitcast(rhs, bf16) if rhs.dtype == u32 else rhs)
        if acc is not None:
            y = y + acc
        hist.append(y)
        return y

    class Side:
        def __init__(self, pieces, n, skip=0):
            cap = [0] * skip + [1] * n
            tot = sum(p[4] for p in pieces)
            self.plan = [[] for _ in cap]
            done = 0
            for p in pieces:
                done += p[4]
                x, d = done / tot * sum(cap), 0
                while x > cap[d] + 1e-9:
                    x -= cap[d]
                    d += 1
                self.plan[d].append((p, x / cap[d]))
            self.pieces = len(pieces)

        def __call__(self, val):
            todo = self.plan.pop(0) if self.plan else []
            if not todo:
                return val
            self.pieces -= len(todo)
            never = zero_s[0] > 0
            if val.dtype == bf16:
                val = pltpu.bitcast(val, u32)
            rg = 8 if val.dtype == u32 else 16
            ng = val.shape[0] // rg
            tied = {}
            for (fn, rd, wr, lag, _), pos in todo:
                m = min(max(-int(-pos * ng // 1) - 1, 0), ng - 1)
                pin = lambda v, w=128: v
                if lag is not None and len(hist) >= lag:
                    r0 = (16 * m) % hist[-lag].shape[0]
                    a = hist[-lag][r0:r0 + 8, :128]
                    if rd is None:
                        def pin(v, w=128, a=a):
                            if v.dtype == bf16:
                                return lax.select(never, _cat([a] * (v.shape[1] // 128), 1).astype(bf16), v)
                            a = _cat([_cat([_as(a, v.dtype)] * (v.shape[0] // 8), 0)] * (w // 128), 1)
                            if v.shape[1] == w:
                                return lax.select(never, a, v)
                            return _cat([lax.select(never, a, v[:, :w]), v[:, w:]], 1)
                    elif rd.dtype == bf16:
                        idx = tile_idx(rd, 256)
                        rd[idx] = lax.select(never, _cat([a, a], 1).astype(bf16), rd[idx])
                    else:
                        idx = tile_idx(rd)
                        rd[idx] = lax.select(never, _as(a, rd.dtype), rd[idx])
                u = fn(pin)
                if wr is False:
                    continue
                if wr is not None:
                    u = wr[tile_idx(wr)]
                t, n = tied.get(m * rg) or (val[m * rg:m * rg + 8, -128:], 0)
                tied[m * rg] = (lax.select(zero_s[n] > 0, _as(u, val.dtype), t), n + 1)
            if not tied:
                return val
            col, r = [], 0
            for r0 in sorted(tied):
                col += ([val[r:r0, -128:]] if r0 > r else []) + [tied[r0][0]]
                r = r0 + 8
            col += [val[r:, -128:]] if r < val.shape[0] else []
            return _cat([val[:, :-128], _cat(col, 0)], 1) if val.shape[1] > 128 else _cat(col, 0)

    def strassen(lhs, rhs, side, init=(None, None, None, None)):
        def add(a, b):
            return a if b is None else a + b
        p = [mm(lhs(k), rhs(k), side) for k in range(5)]
        c12 = add(p[2] + p[4], init[1])
        c21 = add(p[1] + p[3], init[2])
        c22 = mm(lhs(5), rhs(5), side, add(p[0] - p[1] + p[2], init[3]))
        c11 = mm(lhs(6), rhs(6), side, add(p[0] + p[3] - p[4], init[0]))
        return c11, c12, c21, c22

    def fmm(sc, lhs, rhs, side, extra=lambda n: None, emit=None):
        val = {}
        for n in sc.order:
            t = extra(n)
            for q, sg in sorted(sc.par[n], key=lambda e: -e[1]):
                t = val[q] if t is None else (t + val[q] if sg > 0 else t - val[q])
            for r in range(sc.rank):
                if sc.wn[r] == n:
                    t = mm(lhs(sc.un[r]), rhs(r), side, t)
            val[n] = t
            if n < sc.nb and emit is not None:
                emit(n, t)
        return [val[v] for v in range(sc.nb)]

    def phase_b(s1_v, s2_v, s3_v, s4_v, h_v, c0_v, l_v, lf_v, n_v, gb_v):
        def w1_load(name, half, c0, c1):
            quad_load(name, w1_hbm, s1_v, RAW1, half, c0, c1)
            quad_load(name, w1_hbm, s1_v, RAW1, 2 + half, c0, c1)

        def block_load(name, w_hbm, s_v, r0, r1):
            kb, nb = s_v.shape[1] // 128 * 128, s_v.shape[2]
            for q in range(16):
                loads.append((name, w_hbm.at[pl.ds((q // 4) * kb + r0, r1 - r0), pl.ds((q % 4) * nb, nb)],
                              s_v.at[SF.raw[q], pl.ds(r0, r1 - r0)]))

        rows_load("x0", 0, TM)
        w1_load("w1a", 0, 0, 256)
        rows_load("x1", TM, 2 * TM)
        w1_load("w1b", 0, 256, 512)
        w1_load("w1cd", 1, 0, 512)
        rows_load("x23", 2 * TM, 4 * TM)
        rows_load("x4567", 4 * TM, S)
        for q in range(4):
            quad_load("w2", w2_hbm, s2_v, RAW, q)
        block_load("w2", w3_hbm, s3_v, 0, W3A)
        block_load("w4", w3_hbm, s3_v, W3A, D4)
        block_load("w4", w4_hbm, s4_v, 0, F4)
        loads.append(("small", mem0_hbm, mem0_ref))
        loads.append(("small", gw_hbm, gw_ref.at[pl.ds(0, NT)]))
        groups.extend(dict.fromkeys(name for name, _, _ in loads))
        assert len(groups) == NLOAD

        start("x0", "w1a", "w1b", "x1", "w1cd", "x23", "x4567", "w2", "w4", "small")

        def zero(k, carry):
            zero_s[k] = 0
            return carry
        lax.fori_loop(0, S26.rank, zero, 0)

        def prepf_pieces(s_v, lag):
            def piece(rs, cs, st, pin):
                z = 4 * zero_s[st]

                @functools.lru_cache(None)
                def node(n):
                    if n < 16:
                        t = s_v[z + SF.raw[n], rs, cs]
                        return (pin(t) if n in VSTAGES[st][1] else t).astype(f32)
                    a, sa, b, sb = SF.vp[n - 16]
                    return _run([(0, sa, 1, sb)], [node(a), node(b)])[-1]
                rr = [r for k in VSTAGES[st][0] for r in range(7 * k, 7 * k + 7) if SF.raw.count(r) == 0 or SF.vn[r] >= 16]
                vals = [node(SF.vn[r]).astype(bf16) for r in rr]
                for r, t in zip(rr, vals):
                    s_v[z + r, rs, cs] = t
            kb, nb = s_v.shape[1] // 128 * 128, s_v.shape[2]
            out = []
            for r in range(0, kb, 16):
                out += [(slice(rr, rr + 8), slice(c, c + 256)) for c in range(0, nb - 255, 256) for rr in (r, r + 8)]
                out += [(slice(rr, rr + 8), slice(nb - 128, nb)) for rr in (r, r + 8)] if nb % 256 else []
            return [(functools.partial(piece, rs, cs, st), None, s_v if n % TIEP == TIEP - 1 else False, lag,
                     80 if cs.stop - cs.start == 256 else 60)
                    for g in range(0, len(out), 8) for st in range(3) for n, (rs, cs) in enumerate(out[g:g + 8])]

        def prep_pieces(s_v, raw, lag, width=256):
            def piece(r, c, pin):
                idx = (slice(r, r + 8), slice(c, c + width))
                b11, b12, b21, b22 = [_unpack(pin(s_v[(q,) + idx], width) if n in (0, 3) else s_v[(q,) + idx])
                                      for n, q in enumerate(raw)]
                for k, t in ((0, b11 + b22), (2, b12 - b22), (3, b21 - b11), (5, b11 + b12), (6, b21 + b22)):
                    s_v[(k,) + idx] = _pack(t)
            return [(functools.partial(piece, r, c), None, s_v, lag, 80)
                    for c in range(0, s_v.shape[2], width) for r in range(0, s_v.shape[1], 8)]

        def store_l(slot, q, c, quads):
            for k, t in enumerate(_lcombos(*quads)):
                l_v[slot, k, q // 2:q // 2 + 8, c:c + t.shape[1]] = _pack(t)

        def ln_pieces(src, r0, slot, lag, width=256, staged=False, clag=None):
            def stats(q, pin):
                x = pin(src[pl.ds(r0 + q, 16), :].astype(f32))
                xs = [x[:, j * 128:(j + 1) * 128] for j in range(NT)]
                m = functools.reduce(lambda a, b: a + b, xs) * (1.0 / NT)
                w = functools.reduce(lambda a, b: a + b, [(t - m) * (t - m) for t in xs])
                mean = jnp.mean(m, axis=-1, keepdims=True)
                var = jnp.sum(w + NT * ((m - mean) * (m - mean)), axis=-1, keepdims=True) * (1.0 / D)
                n_v[0, q:q + 16, :] = jnp.broadcast_to(mean, (16, 128))
                n_v[1, q:q + 16, :] = jnp.broadcast_to(lax.rsqrt(var + EPS), (16, 128))

            def comb(q, c, pin):
                quads = []
                for rr in (0, HM):
                    rs = pl.ds(pl.multiple_of(r0 + rr + q + zero_s[0], 16), 16)
                    mean, rstd = [jnp.concatenate([n_v[t, rr + q:rr + q + 16, :]] * (width // 128), axis=1)
                                  for t in range(2)]
                    quads += [(src[rs, cc + c:cc + c + width].astype(f32) - mean) * rstd for cc in (0, DH2)]
                store_l(slot, q, c, quads)

            def normf(q, pin):
                mean, rstd = [_cat([n_v[t, q:q + 16, :]] * NT, 1) for t in range(2)]
                c0_v[q:q + 16, :] = (src[pl.ds(pl.multiple_of(r0 + q + zero_s[0], 8), 16), :] - mean) * rstd

            def combf(q, us, pin):
                @functools.lru_cache(None)
                def node(n):
                    if n < SF.nb:
                        return c0_v[(n // 4) * QM + q:(n // 4) * QM + q + 8, (n % 4) * D4:(n % 4 + 1) * D4]
                    a, sa, b, sb = SF.up[n - SF.nb]
                    return _run([(0, sa, 1, sb)], [node(a), node(b)])[-1]
                for u in us:
                    lf_v[SF.ul.index(u), q:q + 8, :] = node(u).astype(bf16)
            dense = slot is not None or src is b_v
            norms = [[(functools.partial(stats, rr + q), None, n_v if dense else False, lag, 90) for rr in (0, HM)]
                     for q in range(0, HM, 16)]
            if slot is None:
                parts = [[SF.un[r] for k in ks for r in range(7 * k, 7 * k + 7)] for ks in ((0, 2, 3), (4, 6), (1, 5))]
                combs = [[(functools.partial(combf, q, us), c0_v, lf_v if dense or us is parts[-1] else False, clag, 55)
                          for us in parts] for q in range(0, QM, 8)]
            else:
                combs = [[(functools.partial(comb, q, c), n_v, l_v, clag, 125) for c in range(0, DH2, width)]
                         for q in range(0, HM, 16)]
            if staged:
                return (sum(norms, []) + [(functools.partial(normf, q), n_v, c0_v, clag, 40) for q in range(0, TM, 16)],
                        sum(combs, []))
            out = list(norms[0])
            for a, b in zip(norms[1:] + [[]], combs):
                out += _merge(a, b) if a else b
            return out

        shifts = (1, 1, -1, -1, 2, 2, -2, -2)

        def shift_pieces(r0, slot, lag, by_value=False):
            def piece(q, j, pin):
                a = [h_v[jj, pl.ds(PAD + r0 + rr + q - shifts[jj], 16), :]
                     for rr in (0, HM) for jj in (j, j + NT // 2)]
                store_l(slot, q, j * 128, [pin(a[0]), a[1], a[2], pin(a[3])])
            return [(functools.partial(piece, q, j), None if by_value else h_v,
                     l_v if (q // 16) % 2 and j == 3 else False, lag, 50)
                    for q in range(0, HM, 16) for j in range(NT // 2)]

        def lhs_of(slot):
            return lambda k: l_v[slot, k]

        xe_v[0, 0:16, :] = jnp.zeros((16, D4), bf16)
        h_v[:, 0:PAD, :] = jnp.zeros((NT, PAD, 128), f32)
        h_v[:, PAD + S:PAD + S + PAD, :] = jnp.zeros((NT, PAD, 128), f32)

        def store_h(r0, c0, h):
            for j in range(h.shape[1] // 128):
                h_v[c0 // 128 + j, PAD + r0:PAD + r0 + h.shape[0], :] = h[:, j * 128:(j + 1) * 128]

        def h_pieces(r0, c0, t, lag, n=4):
            def piece(r, pin):
                store_h(r0 + r, c0, _gelu(pin(t[r:r + 8 * n])))
            return [(functools.partial(piece, r), None, h_v, lag, 10 * n) for r in range(0, t.shape[0], 8 * n)]

        def flush(pieces):
            for p in pieces:
                p[0](lambda v, w=128: v)

        def w1_cols(c, step):
            half, cc = c // DH2, c % DH2
            return jnp.concatenate([s1_v[RAW1[half], :, cc:cc + step], s1_v[RAW1[2 + half], :, cc:cc + step]], axis=0)

        def d1_plain(xn, r0, c0, c1, step):
            for c in range(c0, c1, step):
                store_h(r0, c, _gelu(mm(xn, w1_cols(c, step))))

        def d1_fine(lhs, r0, nrb, cols, pieces, carry, skip=0):
            tiles = [(rb, c) for c in cols for rb in range(nrb)]
            rounds = [tiles[i:i + 4] for i in range(0, len(tiles), 4)]
            for n, (rnd, part) in enumerate(zip(rounds, split(pieces, len(rounds)))):
                sk = skip if n == 0 else 0
                side = Side(_merge(carry, part) if carry else part, 8 - sk, sk)
                carry = []
                for rb, c in rnd:
                    half, cc = c // DH2, c % DH2
                    t = mm(lhs(rb, 0), s1_v[RAW1[half], :, cc:cc + 128], side)
                    t = mm(lhs(rb, 1), s1_v[RAW1[2 + half], :, cc:cc + 128], side, t)
                    carry += h_pieces(r0 + rb * HM, c, t, LS)
            return carry

        def d1_s(b, slot, pieces, carry, early=()):
            for c, part, e in zip(range(0, DH2, NC1), split(pieces, DH2 // NC1), split(early, 2) + [[], []]):
                side = Side(merge(carry, part, e), *((7,) if hist else (5, 2)))
                cs = strassen(lhs_of(slot), lambda k: s1_v[k, :, c:c + NC1], side)
                carry = sum([h_pieces(b * TM + (q // 2) * HM, (q % 2) * DH2 + c, cs[q], LS) for q in (1, 2, 3, 0)], [])
            return carry

        def d2_s(b, slot, pieces, carry=(), early=(), late=()):
            for c, part, e in zip(range(0, DH2, NC1), split(pieces, DH2 // NC1), split(early, 2) + split(late, 2)):
                side = Side(merge(carry, part, e), *((7,) if hist else (5, 2)))
                carry = ()
                idx = [(slice(b * TM + (q // 2) * HM, b * TM + (q // 2 + 1) * HM),
                        slice((q % 2) * DH2 + c, (q % 2) * DH2 + c + NC1)) for q in range(4)]
                cs = strassen(lhs_of(slot), lambda k: s2_v[k, :, c:c + NC1], side,
                              [x_v[i].astype(f32) for i in idx])
                for i, t in zip(idx, cs):
                    b_v[i] = t
                    if b == 0:
                        c0_v[i] = t

        def split(l, n):
            w = [1.0 if hist else 0.6] + [1.0] * (n - 1)
            cut = [int(round(len(l) * sum(w[:i]) / sum(w))) for i in range(n + 1)]
            return [l[cut[i]:cut[i + 1]] for i in range(n)]

        def merge(*ls):
            ls = [l for l in ls if l]
            return _merge(*ls) if ls else []

        NW1, NW3, N30 = 52, 32, 48
        LS, LL = 3, 5

        p3 = prepf_pieces(s3_v, LS)
        n3 = len(p3) * W3A // D4

        @once
        def _phase1a():
            wait("x0")
            xn0 = _pack(_ln(x_v[0:TM, :].astype(f32)))
            wait("w1a")
            d1_plain(xn0, 0, 0, 256, 256)
            wait("x1")
            xn1 = [_pack(_ln(x_v[r:r + HM, :].astype(f32))) for r in (TM, TM + HM)]
            for n in range(2):
                d1_plain(xn1[n], TM + n * HM, 0, 256, 256)
            wait("w1b")
            d1_plain(jnp.concatenate([xn0] + xn1, axis=0), 0, 256, 512, 256)
            wait("w1cd")
            hist.clear()
            xn01 = jnp.concatenate([xn0] + xn1, axis=0)
            l01 = lambda rb, kh: xn01[rb * 64:(rb + 1) * 64, kh * DH2:(kh + 1) * DH2]
            pw = prep_pieces(s1_v, RAW1, LS)
            flush(d1_fine(l01, 0, 4, (512, 640), pw[:NW1], [], 1))
            carry = []
            wait("x23")
            hist.clear()
            carry = d1_fine(l01, 0, 4, (768, 896), ln_pieces(x_v, 2 * TM, 0, LL), carry, 3)
            carry = d1_s(2, 0, ln_pieces(x_v, 3 * TM, 1, LL), carry, pw[NW1:])
            wait("x4567")
            qkv_start(0)
            qkv_start(1)
            hist.clear()
            for b in range(3, NB - 1):
                carry = d1_s(b, b % 2, ln_pieces(x_v, (b + 1) * TM, (b + 1) % 2, LL), carry)
            wait("w2")
            hist.clear()
            pw = prep_pieces(s2_v, RAW, LS)
            carry = d1_s(7, 1, _merge(pw[:NW3], shift_pieces(0, 0, LS, True)), carry)
            d2_s(0, 0, shift_pieces(TM, 1, LS, True), carry, pw[NW3:], p3[:N30])
            pw = split(_merge(p3[N30:n3], sum(ln_pieces(c0_v, 0, None, LL, clag=LS, staged=True), [])), 3)
            for b in range(1, 4):
                d2_s(b, b % 2, _merge(pw[b - 1], shift_pieces((b + 1) * TM, (b + 1) % 2, LS)))
            wait("w4", "small")

        hist.clear()
        pw = p3[n3:] + prepf_pieces(s4_v, LS)
        cut = (0, 93, 192, 291) + (len(pw),)
        for b in range(4, NB):
            d2_s(b, b % 2, merge(pw[cut[b - 4]:cut[b - 3]],
                                 shift_pieces((b + 1) * TM, (b + 1) % 2, LS) if b + 1 < NB else ()))
        start("wo", priority=1)
        gw = gw_ref[0:NT, :].astype(f32)
        gb_v[...] = _cat([jnp.broadcast_to(gw[j:j + 1, :], (8, 128)) for j in range(NT)], 1)

        def ffn(i, carry):
            qkv_wait(i)
            r0 = pl.multiple_of(i * TM, TM)
            rn = pl.multiple_of(jnp.minimum(i + 1, NB - 1) * TM, TM)
            acc = {}
            hist.clear()
            LG = 5

            def relayout(p, r0_, r1_, pin):
                s0 = i * SPG + 2 * p
                e = wqkv_v[s0, r0_:r1_, :]
                o = wqkv_v[s0 + 1, r0_:r1_, :]
                wqkv_v[s0, r0_:r1_, :] = (e & jnp.uint32(0xFFFF)) | (o << 16)
                wqkv_v[s0 + 1, r0_:r1_, :] = (e >> 16) | (o & jnp.uint32(0xFFFF0000))

            relays = [(functools.partial(relayout, p, r, r + 32), wqkv_v, wqkv_v, LG, 35)
                      for p in range(SPG // 2) for r in range(0, D // 2, 32)]
            norms, combs = ln_pieces(b_v, rn, None, 10, staged=True, clag=LG)

            def gate(q, pin):
                x = pin(x_v[pl.ds(r0 + q, 16), :].astype(f32)) * _cat([gb_v[...]] * 2, 0)
                t = functools.reduce(lambda a, b: a + b, [x[:, j * 128:(j + 1) * 128] for j in range(NT)])
                g = jax.nn.sigmoid(jnp.sum(t, axis=-1, keepdims=True))
                g_v[pl.ds(r0 + q, 16), :] = jnp.broadcast_to(g, (16, 128))

            gates = [(functools.partial(gate, q), None, g_v, 10, 90) for q in range(0, TM, 16)]

            def extras(t, pin):
                jj, o = 2 * i + t // 2, 24 + 8 * (t % 2)
                xs = [pin(x_v[pl.ds(pl.multiple_of((jj + hh) * 64 + o, 8), 8), :].astype(f32)) for hh in (0, NPAIR // 2)]
                vals = _run(S26.up, [x[:, cc:cc + D4] for x in xs for cc in range(0, D, D4)])
                for k, u in enumerate(S26.ul):
                    xe_v[k, pl.ds(pl.multiple_of(i * 32 + t * 8, 8), 8), :] = vals[u].astype(bf16)

            xes = [(functools.partial(extras, t), None, xe_v, LG, 100) for t in range(4)]
            hs = {}

            def gelu_pieces(c, cs):
                def piece(r, cc, vs, pin):
                    t = _gelu(pin(_cat([cs[v][r:r + 8, cc:cc + 128] for v in vs], 0)))
                    ts = [t[8 * n:8 * n + 8] for n in range(len(vs))]
                    hs.update({(c, v, r, cc): u for v, u in zip(vs, ts)})
                    return functools.reduce(lambda a, b: a + b, ts)
                return [(functools.partial(piece, r, cc, range(v, v + 4)), None, None, LG, 40) for r in range(0, QM, 8)
                        for cc in range(0, cs[0].shape[1], 128) for v in range(0, SF.nb, 4)]

            def d3(c, side):
                c0, c1 = FCH[c]
                cs = fmm(SF, lambda u: lf_v[SF.ul.index(u), 0:QM], lambda r: s3_v[r, 0:D4, c0:c1], side)
                assert not side.pieces
                return gelu_pieces(c, cs)

            def d4(c, side):
                c0, c1 = FCH[c]
                lh = _run(SF.up, [_cat([_cat([hs.pop((c, v, r, cc)) for r in range(0, QM, 8)], 0)
                                        for cc in range(0, c1 - c0, 128)], 1) for v in range(SF.nb)])
                rhs = lambda r: s4_v[r, c0:c1, :]
                if c + 1 < len(FCH):
                    for n in SF.order:
                        for r in range(SF.rank):
                            if SF.wn[r] == n:
                                acc[n] = mm(lh[SF.un[r]], rhs(r), side, acc.get(n))
                else:
                    idx = lambda v: (pl.ds(r0 + (v // 4) * QM, QM), slice((v % 4) * D4, (v % 4 + 1) * D4))

                    def extra(n):
                        if n >= SF.nb:
                            return acc.get(n)
                        return b_v[idx(n)] + acc[n] if n in acc else b_v[idx(n)]

                    def emit_b(v, t):
                        b_v[idx(v)] = jnp.concatenate([1.0 - g_v[idx(v)[0], :]] * 2, axis=1) * t
                    fmm(SF, lambda u: lh[u], rhs, side, extra, emit_b)
                assert not side.pieces

            g0 = d3(0, Side(relays[:16], 43, 6))
            g1 = d3(1, Side(_merge(g0, gates[:8], xes), 43, 4))
            d4(0, Side(g1[:22], 41, 8))
            g2 = d3(2, Side(_merge(g1[22:], relays[16:32]), 47))
            d4(1, Side(_merge(g2, relays[32:60]), 43, 4))
            g3 = d3(3, Side(_merge(gates[8:], norms), 49))
            d4(2, Side(_merge(g3, combs), 43, 4))
            d4(3, Side(relays[60:], 44))

            @pl.when(i + 2 < NG)
            def _():
                qkv_start(i + 2)

            return carry

        lax.fori_loop(0, NB, ffn, 0)

    pl.run_scoped(
        phase_b,
        pltpu.VMEM((9, D // 4, D // 2), u32),
        pltpu.VMEM((7, D // 4, D // 2), u32),
        pltpu.VMEM((52, D4 + 16, F4), bf16),
        pltpu.VMEM((52, F4 + 8, D4), bf16),
        pltpu.VMEM((NT, S + 2 * PAD, 128), f32),
        pltpu.VMEM((TM, D), f32),
        pltpu.VMEM((2, 7, HM // 2, D // 2), u32),
        pltpu.VMEM((52, QM + 8, D4), bf16),
        pltpu.VMEM((2, TM, 128), f32),
        pltpu.VMEM((8, D), f32),
    )

    def phase_a(out_v, e_v, oe_v, ke_v, ve_v, o_v):
        def pre(it, carry):
            hist.clear()
            for u in range(3 * NG // NPRE):
                s0 = (it * (3 * NG // NPRE) + u) * G

                def rhs(r):
                    t = None
                    sz = s0 + zero_s[r]
                    for q, sg in sorted(_terms(S26.vp, 16, S26.vn[r]).items(), key=lambda e: -e[1]):
                        blk = wqkv_v[sz + q % 4, (q // 4) * (D // 8):(q // 4 + 1) * (D // 8), :]
                        if S26.vn[r] < 16:
                            return blk
                        blk = _unpack(blk)
                        t = blk if t is None else (t + blk if sg > 0 else t - blk)
                    return t.astype(bf16)
                for v, t in enumerate(fmm(S26, lambda k: xe_v[S26.ul.index(k), 0:8 * NPAIR], rhs, None)):
                    e_v[(v // 4) * 16:(v // 4 + 1) * 16, s0 + v % 4] = _pack(t).reshape(16, 8, DH)
            return carry

        lax.fori_loop(0, NPRE, pre, 0)

        wait("wo")
        mem_v[...] = mem0_ref[...].astype(f32)

        def slab(w, h):
            return (h // G) * SPG + w * G + h % G

        def step(j, hx, odd, late, allow, fill):
            qs, ks, vs, ps = {}, {}, {}, {}
            wload = lambda w, h: pltpu.bitcast(wqkv_v[slab(w, h)], bf16)
            eload = lambda w, h: pltpu.bitcast(e_v[j, slab(w, h)], bf16)

            def proj(g):
                part = {}
                if late and g == 0:
                    for h in range(2):
                        for w in range(3):
                            part[w, h] = _dot(hx[:, :DH2], wload(w, h)[:DH2])
                for h in range(g * G, (g + 1) * G):
                    q, k, v = [(_dot(hx[:, DH2:], wload(w, h)[DH2:]) + part[w, h] if (w, h) in part
                                else _dot(hx, wload(w, h))).astype(bf16) for w in range(3)]
                    if odd:
                        q = jnp.concatenate([q, eload(0, h)], axis=0)
                        k = jnp.concatenate([pltpu.bitcast(ke_v[h], bf16), eload(1, h), k], axis=0)
                        v = jnp.concatenate([pltpu.bitcast(ve_v[h], bf16), eload(2, h), v], axis=0)
                    else:
                        ke_v[h] = pltpu.bitcast(k, u32)
                        ve_v[h] = pltpu.bitcast(v, u32)
                        k = jnp.concatenate([k, eload(1, h)], axis=0)
                        v = jnp.concatenate([v, eload(2, h)], axis=0)
                    qs[h], ks[h], vs[h] = q, k, v

            def score(g):
                for h in range(g * G, (g + 1) * G):
                    s = lax.dot_general(qs.pop(h), ks.pop(h), (((1,), (1,)), ((), ())),
                                        preferred_element_type=f32)
                    ps[h] = _softmax(s, allow, fill)

            def pv(g):
                os_ = []
                for h in range(g * G, (g + 1) * G):
                    o = _dot(ps.pop(h), vs.pop(h))
                    o_v[:, h * 128:(h + 1) * 128] = _pack(o[:32])
                    os_.append(o)
                if odd:
                    quads = [jnp.concatenate([os_[2 * kk][r:r + 8], os_[2 * kk + 1][r:r + 8]], axis=1)
                             for r in (32, 40) for kk in range(2)]
                    for k, t in enumerate(_lcombos(*quads)):
                        oe_v[k, pl.ds(pl.multiple_of(j * 8, 8), 8), g * 256:(g + 1) * 256] = t.astype(bf16)

            acc = [None] * NT

            def wo(h0, h1, j0, j1):
                o = pltpu.bitcast(o_v[:, h0 * 128:h1 * 128], bf16)
                for n in range(j0, j1):
                    y = _dot(o, pltpu.bitcast(wo_v[n, h0 * 64:h1 * 64, :], bf16))
                    acc[n] = y if acc[n] is None else y + acc[n]

            for t in range(NG):
                proj(t)
                if t >= 2:
                    pv(t - 2)
                if t >= 1:
                    score(t - 1)
            wo(0, 16, 0, 4)
            pv(NG - 2)
            score(NG - 1)
            wo(0, 16, 4, 8)
            pv(NG - 1)
            wo(16, 24, 0, 8)
            wo(24, 32, 0, 8)
            return jnp.concatenate(acc, axis=1)

        def emit(j, r0, o0, a):
            rs = pl.ds(r0 + o0, 24)
            g = jnp.concatenate([g_v[rs, :]] * NT, axis=1)
            out_v[j, o0:o0 + 24, :] = (g * a + b_v[rs, :]).astype(bf16)

        def pair(j, mem, late):
            r0 = pl.multiple_of(j * 64, 64)
            allow_e, fill_e, allow_o, fill_o = _masks()
            xa = x_v[pl.ds(r0 + 16, 8), :].astype(f32)
            xb = x_v[pl.ds(r0 + 40, 8), :].astype(f32)
            hx = jnp.concatenate([x_v[pl.ds(r0, 16), :], jnp.concatenate([xa, mem], 0).astype(bf16)], 0)
            oe = step(j, hx, False, late, allow_e, fill_e)
            emit(j, r0, 0, oe[:24])
            hx = jnp.concatenate([jnp.concatenate([oe[24:32], xb], 0).astype(bf16), x_v[pl.ds(r0 + 48, 16), :]], 0)
            oo = step(j, hx, True, True, allow_o, fill_o)
            emit(j, r0, 40, oo[8:])
            return oo[:8]

        def a_iter(it, carry):
            mem = mem_v[...]
            for t in range(PPI):
                mem = pair(it * PPI + t, mem, t > 0)
            mem_v[...] = mem
            for t in range(PPI):
                for o0 in (0, 40):
                    idx = (it * PPI + t, pl.ds(o0, 24))
                    pltpu.make_async_copy(out_v.at[idx], out_hbm.at[idx], sem_out).start()
            return carry

        lax.fori_loop(0, NPAIR // PPI, a_iter, 0)

        @once
        def _post():
            hist.clear()
            for n in range(NT // 2):
                quad = [lambda k, t=2 * n + q % 2, o=(q // 2) * 128: jnp.concatenate(
                    [wo_v[t + zero_s[k], g * 256 + o:g * 256 + o + 128, :] for g in range(NG)], axis=0) for q in range(4)]
                cs = strassen(lambda k: oe_v[k], lambda k: _rcombo(k, *quad), None)
                cols = slice(n * 256, (n + 1) * 256)
                for half in (1, 0):
                    t = jnp.concatenate(cs[2 * half:2 * half + 2], axis=1)
                    o0 = 24 + half * 8
                    for jj in range(NPAIR):
                        rs = slice(jj * 64 + o0, jj * 64 + o0 + 8)
                        g = jnp.concatenate([g_v[rs, :]] * 2, axis=1)
                        out_v[jj, o0:o0 + 8, cols] = (g * t[jj * 8:jj * 8 + 8] + b_v[rs, cols]).astype(bf16)
                    idx = (slice(None), pl.ds(o0, 8), pl.ds(n * 256, 256))
                    pltpu.make_async_copy(out_v.at[idx], out_hbm.at[idx], sem_out).start()

        pltpu.make_async_copy(out_v, out_hbm, sem_out).wait()

    pl.run_scoped(
        phase_a,
        pltpu.VMEM((NPAIR, 64, D), bf16),
        pltpu.VMEM((NPAIR, 3 * H, 8, DH), u32),
        pltpu.VMEM((7, 8 * NPAIR, H * DH // 2), bf16),
        pltpu.VMEM((H, 16, 128), u32),
        pltpu.VMEM((H, 16, 128), u32),
        pltpu.VMEM((16, H * DH), u32),
    )


@jax.jit
def pallas_gated_mix__memory_aug_recurrent_mem_tr__mixer_s_mlp__prompt_kernel(
    A_x, A_mem0, A_Wq, A_Wk, A_Wv, A_Wo, A_seg_len, B_x, B_w1, B_w2, B_w3, B_w4, gate_w,
):
    assert A_x.shape == (1, S, D) and A_mem0.shape == (1, M, D)
    any_spec = pl.BlockSpec(memory_space=pl.ANY)
    out = pl.pallas_call(
        _kernel,
        out_shape=jax.ShapeDtypeStruct((NPAIR, 64, D), bf16),
        in_specs=[any_spec] * 11,
        out_specs=any_spec,
        scratch_shapes=[
            pltpu.VMEM((S, D), bf16),
            pltpu.VMEM((3 * H, D // 2, DH), u32),
            pltpu.VMEM((NT, H * DH // 2 + 8, 128), u32),
            pltpu.VMEM((S, D), f32),
            pltpu.VMEM((S, 128), f32),
            pltpu.VMEM((len(S26.ul), 8 * NPAIR + 8, D4), bf16),
            pltpu.VMEM((M, D), f32),
            pltpu.VMEM((M, D), bf16),
            pltpu.VMEM((64, 128), bf16),
            pltpu.SMEM((S26.rank,), jnp.int32),
            pltpu.SemaphoreType.DMA((NLOAD,)),
            pltpu.SemaphoreType.DMA((NG,)),
            pltpu.SemaphoreType.DMA,
        ],
        compiler_params=pltpu.CompilerParams(vmem_limit_bytes=127 * 1024 * 1024,
                                             disable_bounds_checks=True),
    )(
        A_x.reshape(S, D), A_mem0.reshape(M, D),
        A_Wq.reshape(D // 2, 2 * H, DH), A_Wk.reshape(D // 2, 2 * H, DH), A_Wv.reshape(D // 2, 2 * H, DH),
        A_Wo.reshape(H * DH, D), B_w1, B_w2, B_w3, B_w4, gate_w.reshape(NT, 128),
    )
    return out.reshape(1, S, D)
```

```python
import functools

import jax
import jax.numpy as jnp
from jax import lax
import jax.experimental.pallas as pl
import jax.experimental.pallas.tpu as pltpu

f32, bf16, u32 = jnp.float32, jnp.bfloat16, jnp.uint32

S, D, H, DH, M, SEG, F = 2048, 1024, 32, 128, 8, 32, 3584
SCALE = DH ** -0.5
NEG = -1000000000.0
EPS = 1e-05

TM = 256
NB = S // TM
HM = TM // 2
DH2 = D // 2
D4, F4 = D // 4, F // 4
FCH = ((0, 128), (128, 384), (384, 640), (640, 896))
NC1 = 128
NPAIR = S // (2 * SEG)
PPI = 2
NPRE = 3
G = 4
NG = H // G
PAD = 8
NT = D // 128
TIEP = 2
W3A = 208
NLOAD = 11
assert NB == NG

_dot = functools.partial(jnp.dot, preferred_element_type=f32)

def _run(prog, blocks):
    vals = list(blocks)
    for a, sa, b, sb in prog:
        vals.append(vals[a] + vals[b] if sa > 0 and sb > 0 else
                    vals[a] - vals[b] if sa > 0 else vals[b] - vals[a])
    return vals


def _terms(prog, nin, node):
    if node < nin:
        return {node: 1}
    a, sa, b, sb = prog[node - nin]
    out = {k: sa * v for k, v in _terms(prog, nin, a).items()}
    out.update({k: sb * v for k, v in _terms(prog, nin, b).items()})
    return out


class _Scheme:
    def __init__(self, ms, up, vp, wp, un, vn, wn):
        self.ms, self.nb, self.rank = ms, 4 * ms, len(un)
        self.up, self.vp, self.wp, self.un, self.vn, self.wn = up, vp, wp, un, vn, wn
        self.ul = tuple(sorted(set(un)))
        t = {}
        for r in range(self.rank):
            for a, ca in _terms(up, self.nb, un[r]).items():
                for b, cb in _terms(vp, 16, vn[r]).items():
                    for c, cc in _terms(wp, self.nb, wn[r]).items():
                        t[a, b, c] = t.get((a, b, c), 0) + ca * cb * cc
        assert {k: v for k, v in t.items() if v} == {
            (4 * i + j, 4 * j + l, 4 * i + l): 1 for i in range(ms) for j in range(4) for l in range(4)}
        free = iter(r for r in range(self.rank) if vn[r] >= 16)
        self.raw = tuple(vn.index(q) if q in vn else next(free) for q in range(16))
        self.par = {n: [] for n in range(self.nb + len(wp))}
        for k, (a, sa, b, sb) in enumerate(wp):
            self.par[a].append((self.nb + k, sa))
            self.par[b].append((self.nb + k, sb))
        self.order = order = []

        def closure(n, acc):
            if n not in acc and n not in order:
                acc.add(n)
                for q, _ in self.par[n]:
                    closure(q, acc)
            return acc

        def visit(n):
            if n not in order:
                for q, _ in self.par[n]:
                    visit(q)
                order.append(n)
        while len([v for v in range(self.nb) if v not in order]):
            visit(min((v for v in range(self.nb) if v not in order), key=lambda v: len(closure(v, set()))))


UP = ((4, 1, 5, 1), (6, 1, 8, 1), (0, 1, 3, 1), (2, -1, 9, 1), (4, -1, 10, 1), (0, 1, 1, 1), (2, 1, 12, 1),
      (5, 1, 7, -1), (7, 1, 12, -1), (11, -1, 13, 1), (10, -1, 11, 1), (2, 1, 7, 1), (0, -1, 4, 1),
      (6, 1, 7, 1), (1, -1, 5, 1), (3, 1, 7, -1), (1, 1, 4, 1), (2, 1, 3, 1), (1, -1, 3, 1), (1, 1, 7, -1),
      (2, 1, 6, -1))
WP = ((0, -1, 3, 1), (4, 1, 6, -1), (1, 1, 8, 1), (5, 1, 10, 1), (4, -1, 7, 1), (0, -1, 9, -1),
      (11, 1, 12, 1), (6, 1, 7, -1), (2, 1, 5, -1), (0, -1, 7, -1), (9, 1, 11, -1), (2, 1, 13, 1),
      (5, 1, 13, 1), (2, -1, 3, 1), (5, 1, 6, 1), (0, 1, 4, 1), (2, 1, 7, 1), (1, 1, 2, 1), (1, 1, 5, 1),
      (3, 1, 7, 1), (2, 1, 6, 1))
VP = ((1, 1, 5, -1), (8, 1, 11, 1), (10, 1, 17, 1), (13, 1, 16, -1), (0, 1, 4, -1), (0, 1, 3, 1),
      (14, 1, 18, -1), (0, 1, 11, 1), (14, 1, 19, -1), (0, 1, 5, 1), (12, 1, 15, 1), (2, 1, 21, 1),
      (10, 1, 14, -1), (4, 1, 7, 1), (11, 1, 19, 1), (12, -1, 20, 1), (13, 1, 14, -1), (9, 1, 30, -1),
      (3, -1, 15, 1), (6, 1, 23, 1), (24, 1, 27, -1), (9, -1, 18, 1), (7, 1, 34, 1), (2, 1, 6, -1),
      (0, 1, 8, -1), (6, 1, 21, 1), (22, 1, 31, -1), (6, 1, 29, 1), (0, 1, 1, 1), (15, 1, 25, 1),
      (5, 1, 37, 1), (15, 1, 20, 1))
UN = (7, 27, 24, 17, 9, 22, 21, 2, 15, 11, 8, 25, 19, 28, 2, 23, 26, 20, 1, 18, 10, 28, 4, 13, 14, 16)
WN = (23, 17, 24, 10, 14, 7, 22, 19, 12, 18, 15, 25, 20, 5, 26, 0, 8, 2, 27, 11, 26, 9, 28, 21, 16, 5)
VN = (42, 47, 41, 5, 11, 43, 18, 28, 20, 23, 35, 19, 22, 46, 33, 26, 45, 36, 38, 25, 44, 40, 39, 21, 24, 32)
S26 = _Scheme(2, UP, VP, WP, UN, VN, WN)


def _twice(forms):
    prog, nodes = [], []

    def apply(f, quad):
        if len(f) == 1:
            return quad[f[0]]
        prog.append((quad[f[0]], f[1], quad[f[2]], f[3]))
        return 15 + len(prog)
    for f1 in forms:
        inner = [apply(f1, [4 * (2 * (q // 2) + p // 2) + 2 * (q % 2) + p % 2 for q in range(4)]) for p in range(4)]
        nodes += [apply(f2, inner) for f2 in forms]
    return tuple(prog), tuple(nodes)


_U2 = _twice(((0, 1, 3, 1), (2, 1, 3, 1), (0,), (3,), (0, 1, 1, 1), (2, 1, 0, -1), (1, 1, 3, -1)))
_V2 = _twice(((0, 1, 3, 1), (0,), (1, 1, 3, -1), (2, 1, 0, -1), (3,), (0, 1, 1, 1), (2, 1, 3, 1)))
_W2 = _twice(((0, 1, 3, 1), (2, 1, 3, -1), (1, 1, 3, 1), (0, 1, 2, 1), (1, 1, 0, -1), (3,), (0,)))
S49 = _Scheme(4, _U2[0], _V2[0], _W2[0], _U2[1], _V2[1], _W2[1])
VSTAGES = (((2, 5), (2, 7)), ((3, 6), (8, 13)), ((0, 1, 4), (0, 5, 10, 15)))
S49.raw = tuple(7 * (1, 2, 3, 4)[2 * (q // 8) + q % 4 // 2] + (1, 2, 3, 4)[2 * (q // 4 % 2) + q % 2] for q in range(16))
assert all(S49.raw[S49.vn[r]] == r for r in range(49) if S49.vn[r] < 16)


def _outer_major(n):
    rs = [r for r in range(49) if S49.wn[r] == n]
    return max(rs + [-1] + [_outer_major(q) + 0.01 for q, _ in S49.par[n]])


S49N = _Scheme(4, _U2[0], _V2[0], _W2[0], _U2[1], _V2[1], _W2[1])
S49N.order.sort(key=_outer_major)
UPARTS = [[S49.un[r] for k in ks for r in range(7 * k, 7 * k + 7)] for ks in ((0, 2, 3), (4, 6), (1, 5))]
SF = S49
QM = TM // SF.ms


def _ln(x):
    m = jnp.mean(x, axis=-1, keepdims=True)
    xc = x - m
    v = jnp.mean(xc * xc, axis=-1, keepdims=True)
    return xc * lax.rsqrt(v + EPS)


_GC = 0.7978845608028654


def _gelu(x):
    h = 0.5 * x
    return h + h * jnp.tanh(x * (_GC + (_GC * 0.044715) * (x * x)))


def _unpack(u):
    return pltpu.bitcast(u, bf16).astype(f32)


def _pack(x):
    return pltpu.bitcast(x.astype(bf16), u32)


def _cat(xs, axis):
    xs = [x for x in xs if x.shape[axis]]
    return xs[0] if len(xs) == 1 else jnp.concatenate(xs, axis=axis)


def _as(x, dtype):
    return x if x.dtype == dtype else pltpu.bitcast(x, dtype)


def _lcombos(a11, a12, a21, a22):
    return [a11 + a22, a21 + a22, a11, a22, a11 + a12, a21 - a11, a12 - a22]


def _merge(*lists):
    keyed = [((j + 0.5) / len(l), n, j, v) for n, l in enumerate(lists) for j, v in enumerate(l)]
    return [v for _, _, _, v in sorted(keyed, key=lambda t: t[:3])]


def _masks():
    r = lax.broadcasted_iota(jnp.int32, (32, 48), 0)
    c = lax.broadcasted_iota(jnp.int32, (32, 48), 1)
    exist_e = c < 40
    allow_e = exist_e & ((r >= 24) | ((c >= 24) & (c < 32)) | (c <= r))
    fill_e = jnp.where(exist_e, NEG, -jnp.inf).astype(f32)
    r = lax.broadcasted_iota(jnp.int32, (48, 80), 0)
    c = lax.broadcasted_iota(jnp.int32, (48, 80), 1)
    q_even = (r >= 32) & (r < 40)
    exist_o = (q_even & (c < 40)) | (~q_even & (c >= 40))
    ktok = jnp.where(c < 24, c, jnp.where(c < 48, c - 8, c - 16))
    qtok = jnp.where(r < 32, r + 32, r - 8)
    is_mem_key = ((c >= 24) & (c < 32)) | ((c >= 48) & (c < 56))
    allow_o = exist_o & (is_mem_key | (r < 8) | (ktok <= qtok))
    fill_o = jnp.where(exist_o, NEG, -jnp.inf).astype(f32)
    return allow_e, fill_e, allow_o, fill_o


def _rcombo(k, b11, b12, b21, b22):
    if k in (1, 4):
        return (b11 if k == 1 else b22)(k)
    a, b, sign = {0: (b11, b22, 1), 2: (b12, b22, -1), 3: (b21, b11, -1), 5: (b11, b12, 1), 6: (b21, b22, 1)}[k]
    a, b = _unpack(a(k)), _unpack(b(k))
    return (a + b if sign > 0 else a - b).astype(bf16)


def _softmax(s, allow, fill):
    s = jnp.where(allow, s * SCALE, fill)
    m = jnp.max(s, axis=-1, keepdims=True)
    e = jnp.exp(s - m)
    l = jnp.sum(e, axis=-1, keepdims=True)
    r = pl.reciprocal(l, approx=True)
    r = r * (2.0 - l * r)
    return (e * r).astype(bf16)


def _kernel(x_hbm, mem0_hbm, wq_hbm, wk_hbm, wv_hbm, wo_hbm, w1_hbm, w2_hbm, w3_hbm, w4_hbm,
            gw_hbm, out_hbm,
            x_v, wqkv_v, wo_v, b_v, g_v, xe_v, mem_v, mem0_ref, gw_ref, zero_s,
            sem, sem_qkv, sem_out):
    RAW = (1, 2, 3, 4)
    RAW1 = (1, 7, 8, 4)

    loads = []

    def rows_load(name, r0, r1):
        loads.append((name, x_hbm.at[pl.ds(r0, r1 - r0)], x_v.at[pl.ds(r0, r1 - r0)]))

    def quad_load(name, w_hbm, s_v, raw, q, c0=0, c1=None):
        k4, n2 = s_v.shape[1], s_v.shape[2]
        c1 = n2 if c1 is None else c1
        src = w_hbm.bitcast(u32).at[pl.ds((q // 2) * k4, k4), pl.ds((q % 2) * n2 + c0, c1 - c0)]
        loads.append((name, src, s_v.at[raw[q], :, pl.ds(c0, c1 - c0)]))

    for j in range(NT):
        loads.append(("wo", wo_hbm.bitcast(u32).at[:, pl.ds(j * 128, 128)], wo_v.at[j, pl.ds(0, H * DH // 2)]))
    groups = []

    def start(*names, priority=0):
        for name, src, dst in loads:
            if name in names:
                pltpu.make_async_copy(src, dst, sem.at[groups.index(name)]).start(priority=priority)

    def wait(*names):
        for name, src, dst in loads:
            if name in names:
                pltpu.make_async_copy(src, dst, sem.at[groups.index(name)]).wait()

    SPG = 3 * G

    def qkv_start(g):
        for w, w_hbm in enumerate((wq_hbm, wk_hbm, wv_hbm)):
            wu = w_hbm.bitcast(u32)
            for k in range(G // 2):
                for par in range(2):
                    pltpu.make_async_copy(
                        wu.at[:, par * (H // 2) + g * (G // 2) + k, :],
                        wqkv_v.at[g * SPG + w * G + 2 * k + par], sem_qkv.at[g]).start(priority=1)

    def qkv_wait(g):
        grp = wqkv_v.at[pl.ds(g * SPG, SPG)]
        pltpu.make_async_copy(grp, grp, sem_qkv.at[g]).wait()

    def once(fn):
        def body(_, carry):
            fn()
            return carry
        lax.fori_loop(0, 1 + zero_s[1], body, 0)

    def tile_idx(ref, cols=128):
        z = zero_s[0]
        n = 16 if ref.dtype == bf16 and cols == 128 else 8
        return (z,) * (len(ref.shape) - 2) + (pl.ds(pl.multiple_of(z, n), n), slice(0, cols))

    hist = []

    def mm(lhs, rhs, side=None, acc=None):
        if side is not None:
            lhs = side(lhs)
        lhs = pltpu.bitcast(lhs, bf16) if lhs.dtype == u32 else lhs.astype(bf16)
        y = _dot(lhs, pltpu.bitcast(rhs, bf16) if rhs.dtype == u32 else rhs)
        if acc is not None:
            y = y + acc
        hist.append(y)
        return y

    class Side:
        def __init__(self, pieces, n, skip=0):
            cap = [0] * skip + [1] * n
            tot = sum(p[4] for p in pieces)
            self.plan = [[] for _ in cap]
            done = 0
            for p in pieces:
                done += p[4]
                x, d = done / tot * sum(cap), 0
                while x > cap[d] + 1e-9:
                    x -= cap[d]
                    d += 1
                self.plan[d].append((p, x / cap[d]))
            self.pieces = len(pieces)

        def __call__(self, val):
            todo = self.plan.pop(0) if self.plan else []
            if not todo:
                return val
            self.pieces -= len(todo)
            never = zero_s[0] > 0
            if val.dtype == bf16:
                val = pltpu.bitcast(val, u32)
            rg = 8 if val.dtype == u32 else 16
            ng = val.shape[0] // rg
            tied = {}
            for (fn, rd, wr, lag, _), pos in todo:
                m = min(max(-int(-pos * ng // 1) - 1, 0), ng - 1)
                pin = lambda v, w=128: v
                if lag is not None and len(hist) >= lag:
                    r0 = (16 * m) % hist[-lag].shape[0]
                    a = hist[-lag][r0:r0 + 8, :128]
                    if rd is None:
                        def pin(v, w=128, a=a):
                            if v.dtype == bf16:
                                return lax.select(never, _cat([a] * (v.shape[1] // 128), 1).astype(bf16), v)
                            a = _cat([_cat([_as(a, v.dtype)] * (v.shape[0] // 8), 0)] * (w // 128), 1)
                            if v.shape[1] == w:
                                return lax.select(never, a, v)
                            return _cat([lax.select(never, a, v[:, :w]), v[:, w:]], 1)
                    elif rd.dtype == bf16:
                        idx = tile_idx(rd, 256)
                        rd[idx] = lax.select(never, _cat([a, a], 1).astype(bf16), rd[idx])
                    else:
                        idx = tile_idx(rd)
                        rd[idx] = lax.select(never, _as(a, rd.dtype), rd[idx])
                u = fn(pin)
                if wr is False:
                    continue
                if wr is not None:
                    u = wr[tile_idx(wr)]
                t, n = tied.get(m * rg) or (val[m * rg:m * rg + 8, -128:], 0)
                tied[m * rg] = (lax.select(zero_s[n] > 0, _as(u, val.dtype), t), n + 1)
            if not tied:
                return val
            col, r = [], 0
            for r0 in sorted(tied):
                col += ([val[r:r0, -128:]] if r0 > r else []) + [tied[r0][0]]
                r = r0 + 8
            col += [val[r:, -128:]] if r < val.shape[0] else []
            return _cat([val[:, :-128], _cat(col, 0)], 1) if val.shape[1] > 128 else _cat(col, 0)

    def strassen(lhs, rhs, side, init=(None, None, None, None)):
        def add(a, b):
            return a if b is None else a + b
        p = [mm(lhs(k), rhs(k), side) for k in range(5)]
        c12 = add(p[2] + p[4], init[1])
        c21 = add(p[1] + p[3], init[2])
        c22 = mm(lhs(5), rhs(5), side, add(p[0] - p[1] + p[2], init[3]))
        c11 = mm(lhs(6), rhs(6), side, add(p[0] + p[3] - p[4], init[0]))
        return c11, c12, c21, c22

    def fmm(sc, lhs, rhs, side, extra=lambda n: None, emit=None):
        val = {}
        for n in sc.order:
            t = extra(n)
            for q, sg in sorted(sc.par[n], key=lambda e: -e[1]):
                t = val[q] if t is None else (t + val[q] if sg > 0 else t - val[q])
            for r in range(sc.rank):
                if sc.wn[r] == n:
                    t = mm(lhs(sc.un[r]), rhs(r), side, t)
            val[n] = t
            if n < sc.nb and emit is not None:
                emit(n, t)
        return [val[v] for v in range(sc.nb)]

    def phase_b(s1_v, s2_v, s3_v, s4_v, h_v, c0_v, l_v, lf_v, n_v, gb_v):
        def w1_load(name, half, c0, c1):
            quad_load(name, w1_hbm, s1_v, RAW1, half, c0, c1)
            quad_load(name, w1_hbm, s1_v, RAW1, 2 + half, c0, c1)

        def block_load(name, w_hbm, s_v, r0, r1):
            kb, nb = s_v.shape[1] // 128 * 128, s_v.shape[2]
            for q in range(16):
                loads.append((name, w_hbm.at[pl.ds((q // 4) * kb + r0, r1 - r0), pl.ds((q % 4) * nb, nb)],
                              s_v.at[SF.raw[q], pl.ds(r0, r1 - r0)]))

        rows_load("x0", 0, TM)
        w1_load("w1a", 0, 0, 256)
        rows_load("x1", TM, 2 * TM)
        w1_load("w1b", 0, 256, 512)
        w1_load("w1cd", 1, 0, 512)
        rows_load("x23", 2 * TM, 4 * TM)
        rows_load("x4567", 4 * TM, S)
        for q in range(4):
            quad_load("w2", w2_hbm, s2_v, RAW, q)
        block_load("w2", w3_hbm, s3_v, 0, W3A)
        block_load("w4", w3_hbm, s3_v, W3A, D4)
        block_load("w4", w4_hbm, s4_v, 0, F4)
        loads.append(("small", mem0_hbm, mem0_ref))
        loads.append(("small", gw_hbm, gw_ref.at[pl.ds(0, NT)]))
        groups.extend(dict.fromkeys(name for name, _, _ in loads))
        assert len(groups) == NLOAD

        start("x0", "w1a", "w1b", "x1", "w1cd", "x23", "x4567", "w2", "w4", "small")

        def zero(k, carry):
            zero_s[k] = 0
            return carry
        lax.fori_loop(0, S26.rank, zero, 0)

        def prepf_pieces(s_v, lag):
            def piece(rs, cs, st, pin):
                z = 4 * zero_s[st]

                @functools.lru_cache(None)
                def node(n):
                    if n < 16:
                        t = s_v[z + SF.raw[n], rs, cs]
                        return (pin(t) if n in VSTAGES[st][1] else t).astype(f32)
                    a, sa, b, sb = SF.vp[n - 16]
                    return _run([(0, sa, 1, sb)], [node(a), node(b)])[-1]
                rr = [r for k in VSTAGES[st][0] for r in range(7 * k, 7 * k + 7) if SF.raw.count(r) == 0 or SF.vn[r] >= 16]
                vals = [node(SF.vn[r]).astype(bf16) for r in rr]
                for r, t in zip(rr, vals):
                    s_v[z + r, rs, cs] = t
            kb, nb = s_v.shape[1] // 128 * 128, s_v.shape[2]
            out = []
            for r in range(0, kb, 16):
                out += [(slice(rr, rr + 8), slice(c, c + 256)) for c in range(0, nb - 255, 256) for rr in (r, r + 8)]
                out += [(slice(rr, rr + 8), slice(nb - 128, nb)) for rr in (r, r + 8)] if nb % 256 else []
            return [(functools.partial(piece, rs, cs, st), None, s_v if n % TIEP == TIEP - 1 else False, lag,
                     80 if cs.stop - cs.start == 256 else 60)
                    for g in range(0, len(out), 8) for st in range(3) for n, (rs, cs) in enumerate(out[g:g + 8])]

        def prep_pieces(s_v, raw, lag, width=256):
            def piece(r, c, pin):
                idx = (slice(r, r + 8), slice(c, c + width))
                b11, b12, b21, b22 = [_unpack(pin(s_v[(q,) + idx], width) if n in (0, 3) else s_v[(q,) + idx])
                                      for n, q in enumerate(raw)]
                for k, t in ((0, b11 + b22), (2, b12 - b22), (3, b21 - b11), (5, b11 + b12), (6, b21 + b22)):
                    s_v[(k,) + idx] = _pack(t)
            return [(functools.partial(piece, r, c), None, s_v, lag, 80)
                    for c in range(0, s_v.shape[2], width) for r in range(0, s_v.shape[1], 8)]

        def store_l(slot, q, c, quads):
            for k, t in enumerate(_lcombos(*quads)):
                l_v[slot, k, q // 2:q // 2 + 8, c:c + t.shape[1]] = _pack(t)

        def ln_pieces(src, r0, slot, lag, width=256, staged=False, clag=None):
            def stats(q, pin):
                x = pin(src[pl.ds(r0 + q, 16), :].astype(f32))
                xs = [x[:, j * 128:(j + 1) * 128] for j in range(NT)]
                m = functools.reduce(lambda a, b: a + b, xs) * (1.0 / NT)
                w = functools.reduce(lambda a, b: a + b, [(t - m) * (t - m) for t in xs])
                mean = jnp.mean(m, axis=-1, keepdims=True)
                var = jnp.sum(w + NT * ((m - mean) * (m - mean)), axis=-1, keepdims=True) * (1.0 / D)
                n_v[0, q:q + 16, :] = jnp.broadcast_to(mean, (16, 128))
                n_v[1, q:q + 16, :] = jnp.broadcast_to(lax.rsqrt(var + EPS), (16, 128))

            def comb(q, c, pin):
                quads = []
                for rr in (0, HM):
                    rs = pl.ds(pl.multiple_of(r0 + rr + q + zero_s[0], 16), 16)
                    mean, rstd = [jnp.concatenate([n_v[t, rr + q:rr + q + 16, :]] * (width // 128), axis=1)
                                  for t in range(2)]
                    quads += [(src[rs, cc + c:cc + c + width].astype(f32) - mean) * rstd for cc in (0, DH2)]
                store_l(slot, q, c, quads)

            def normf(q, pin):
                mean, rstd = [_cat([n_v[t, q:q + 16, :]] * NT, 1) for t in range(2)]
                c0_v[q:q + 16, :] = (src[pl.ds(pl.multiple_of(r0 + q + zero_s[0], 8), 16), :] - mean) * rstd

            def combf(q, us, pin):
                @functools.lru_cache(None)
                def node(n):
                    if n < SF.nb:
                        return c0_v[(n // 4) * QM + q:(n // 4) * QM + q + 8, (n % 4) * D4:(n % 4 + 1) * D4]
                    a, sa, b, sb = SF.up[n - SF.nb]
                    return _run([(0, sa, 1, sb)], [node(a), node(b)])[-1]
                for u in us:
                    lf_v[SF.ul.index(u), q:q + 8, :] = node(u).astype(bf16)
            dense = slot is not None or src is b_v
            norms = [[(functools.partial(stats, rr + q), None, n_v if dense else False, lag, 90) for rr in (0, HM)]
                     for q in range(0, HM, 16)]
            if slot is None:
                parts = [[SF.un[r] for k in ks for r in range(7 * k, 7 * k + 7)] for ks in ((0, 2, 3), (4, 6), (1, 5))]
                combs = [[(functools.partial(combf, q, us), c0_v, lf_v if dense or us is parts[-1] else False, clag, 55)
                          for us in parts] for q in range(0, QM, 8)]
            else:
                combs = [[(functools.partial(comb, q, c), n_v, l_v, clag, 125) for c in range(0, DH2, width)]
                         for q in range(0, HM, 16)]
            if staged:
                return (sum(norms, []) + [(functools.partial(normf, q), n_v, c0_v, clag, 40) for q in range(0, TM, 16)],
                        sum(combs, []))
            out = list(norms[0])
            for a, b in zip(norms[1:] + [[]], combs):
                out += _merge(a, b) if a else b
            return out

        shifts = (1, 1, -1, -1, 2, 2, -2, -2)

        def shift_pieces(r0, slot, lag, by_value=True):
            def piece(q, j, pin):
                a = [h_v[jj, pl.ds(PAD + r0 + rr + q - shifts[jj], 16), :]
                     for rr in (0, HM) for jj in (j, j + NT // 2)]
                store_l(slot, q, j * 128, [pin(a[0]), a[1], a[2], pin(a[3])])
            return [(functools.partial(piece, q, j), None if by_value else h_v,
                     l_v if j % 2 else False, lag, 50)
                    for q in range(0, HM, 16) for j in range(NT // 2)]

        def lhs_of(slot):
            return lambda k: l_v[slot, k]

        xe_v[0, 0:16, :] = jnp.zeros((16, D4), bf16)
        h_v[:, 0:PAD, :] = jnp.zeros((NT, PAD, 128), f32)
        h_v[:, PAD + S:PAD + S + PAD, :] = jnp.zeros((NT, PAD, 128), f32)

        def store_h(r0, c0, h):
            for j in range(h.shape[1] // 128):
                h_v[c0 // 128 + j, PAD + r0:PAD + r0 + h.shape[0], :] = h[:, j * 128:(j + 1) * 128]

        def h_pieces(r0, c0, t, lag, n=4):
            def piece(r, pin):
                store_h(r0 + r, c0, _gelu(pin(t[r:r + 8 * n])))
            return [(functools.partial(piece, r), None, h_v, lag, 10 * n) for r in range(0, t.shape[0], 8 * n)]

        def flush(pieces):
            for p in pieces:
                p[0](lambda v, w=128: v)

        def w1_cols(c, step):
            half, cc = c // DH2, c % DH2
            return jnp.concatenate([s1_v[RAW1[half], :, cc:cc + step], s1_v[RAW1[2 + half], :, cc:cc + step]], axis=0)

        def d1_plain(xn, r0, c0, c1, step):
            for c in range(c0, c1, step):
                store_h(r0, c, _gelu(mm(xn, w1_cols(c, step))))

        def d1_fine(lhs, r0, nrb, cols, pieces, carry, skip=0):
            tiles = [(rb, c) for c in cols for rb in range(nrb)]
            rounds = [tiles[i:i + 4] for i in range(0, len(tiles), 4)]
            for n, (rnd, part) in enumerate(zip(rounds, split(pieces, len(rounds)))):
                sk = skip if n == 0 else 0
                side = Side(_merge(carry, part) if carry else part, 8 - sk, sk)
                carry = []
                for rb, c in rnd:
                    half, cc = c // DH2, c % DH2
                    t = mm(lhs(rb, 0), s1_v[RAW1[half], :, cc:cc + 128], side)
                    t = mm(lhs(rb, 1), s1_v[RAW1[2 + half], :, cc:cc + 128], side, t)
                    carry += h_pieces(r0 + rb * HM, c, t, LS)
            return carry

        def d1_s(b, slot, pieces, carry, early=()):
            for c, part, e in zip(range(0, DH2, NC1), split(pieces, DH2 // NC1), split(early, 2) + [[], []]):
                side = Side(merge(carry, part, e), *((7,) if hist else (5, 2)))
                cs = strassen(lhs_of(slot), lambda k: s1_v[k, :, c:c + NC1], side)
                carry = sum([h_pieces(b * TM + (q // 2) * HM, (q % 2) * DH2 + c, cs[q], LS) for q in (1, 2, 3, 0)], [])
            return carry

        def d2_s(b, slot, pieces, carry=(), early=(), late=()):
            for c, part, e in zip(range(0, DH2, NC1), split(pieces, DH2 // NC1), split(early, 2) + split(late, 2)):
                side = Side(merge(carry, part, e), *((7,) if hist else (5, 2)))
                carry = ()
                idx = [(slice(b * TM + (q // 2) * HM, b * TM + (q // 2 + 1) * HM),
                        slice((q % 2) * DH2 + c, (q % 2) * DH2 + c + NC1)) for q in range(4)]
                cs = strassen(lhs_of(slot), lambda k: s2_v[k, :, c:c + NC1], side,
                              [x_v[i].astype(f32) for i in idx])
                for i, t in zip(idx, cs):
                    b_v[i] = t
                    if b == 0:
                        c0_v[i] = t

        def split(l, n):
            w = [1.0 if hist else 0.6] + [1.0] * (n - 1)
            cut = [int(round(len(l) * sum(w[:i]) / sum(w))) for i in range(n + 1)]
            return [l[cut[i]:cut[i + 1]] for i in range(n)]

        def merge(*ls):
            ls = [l for l in ls if l]
            return _merge(*ls) if ls else []

        NW1, NW3, N30 = 52, 32, 48
        LS, LL = 3, 5

        p3 = prepf_pieces(s3_v, LS)
        n3 = len(p3) * W3A // D4

        @once
        def _phase1a():
            wait("x0")
            xn0 = _pack(_ln(x_v[0:TM, :].astype(f32)))
            wait("w1a")
            d1_plain(xn0, 0, 0, 256, 256)
            wait("x1")
            xn1 = [_pack(_ln(x_v[r:r + HM, :].astype(f32))) for r in (TM, TM + HM)]
            for n in range(2):
                d1_plain(xn1[n], TM + n * HM, 0, 256, 256)
            wait("w1b")
            d1_plain(jnp.concatenate([xn0] + xn1, axis=0), 0, 256, 512, 256)
            wait("w1cd")
            hist.clear()
            xn01 = jnp.concatenate([xn0] + xn1, axis=0)
            l01 = lambda rb, kh: xn01[rb * 64:(rb + 1) * 64, kh * DH2:(kh + 1) * DH2]
            pw = prep_pieces(s1_v, RAW1, LS)
            flush(d1_fine(l01, 0, 4, (512, 640), pw[:NW1], [], 1))
            carry = []
            wait("x23")
            hist.clear()
            carry = d1_fine(l01, 0, 4, (768, 896), ln_pieces(x_v, 2 * TM, 0, LL), carry, 3)
            carry = d1_s(2, 0, ln_pieces(x_v, 3 * TM, 1, LL), carry, pw[NW1:])
            wait("x4567")
            qkv_start(0)
            qkv_start(1)
            hist.clear()
            for b in range(3, NB - 1):
                carry = d1_s(b, b % 2, ln_pieces(x_v, (b + 1) * TM, (b + 1) % 2, LL), carry)
            wait("w2")
            hist.clear()
            pw = prep_pieces(s2_v, RAW, LS)
            carry = d1_s(7, 1, _merge(pw[:NW3], shift_pieces(0, 0, LS, True)), carry)
            d2_s(0, 0, shift_pieces(TM, 1, LS, True), carry, pw[NW3:], p3[:N30])
            pw = split(_merge(p3[N30:n3], sum(ln_pieces(c0_v, 0, None, LL, clag=LS, staged=True), [])), 3)
            for b in range(1, 4):
                d2_s(b, b % 2, _merge(pw[b - 1], shift_pieces((b + 1) * TM, (b + 1) % 2, LS)))
            wait("w4", "small")

        hist.clear()
        pw = p3[n3:] + prepf_pieces(s4_v, LS)
        cut = (0, 93, 192, 291) + (len(pw),)
        for b in range(4, NB):
            d2_s(b, b % 2, merge(pw[cut[b - 4]:cut[b - 3]],
                                 shift_pieces((b + 1) * TM, (b + 1) % 2, LS) if b + 1 < NB else ()))
        start("wo", priority=1)
        gw = gw_ref[0:NT, :].astype(f32)
        gb_v[...] = _cat([jnp.broadcast_to(gw[j:j + 1, :], (8, 128)) for j in range(NT)], 1)

        def ffn(i, carry):
            qkv_wait(i)
            r0 = pl.multiple_of(i * TM, TM)
            rn = pl.multiple_of(jnp.minimum(i + 1, NB - 1) * TM, TM)
            acc = {}
            hist.clear()
            LG = 5

            def relayout(p, r0_, r1_, pin):
                s0 = i * SPG + 2 * p
                e = wqkv_v[s0, r0_:r1_, :]
                o = wqkv_v[s0 + 1, r0_:r1_, :]
                wqkv_v[s0, r0_:r1_, :] = (e & jnp.uint32(0xFFFF)) | (o << 16)
                wqkv_v[s0 + 1, r0_:r1_, :] = (e >> 16) | (o & jnp.uint32(0xFFFF0000))

            relays = [(functools.partial(relayout, p, r, r + 32), wqkv_v, wqkv_v, LG, 35)
                      for p in range(SPG // 2) for r in range(0, D // 2, 32)]
            norms, combs = ln_pieces(b_v, rn, None, 10, staged=True, clag=LG)

            def gate(q, pin):
                x = pin(x_v[pl.ds(r0 + q, 16), :].astype(f32)) * _cat([gb_v[...]] * 2, 0)
                t = functools.reduce(lambda a, b: a + b, [x[:, j * 128:(j + 1) * 128] for j in range(NT)])
                g = jax.nn.sigmoid(jnp.sum(t, axis=-1, keepdims=True))
                g_v[pl.ds(r0 + q, 16), :] = jnp.broadcast_to(g, (16, 128))

            gates = [(functools.partial(gate, q), None, g_v, 10, 90) for q in range(0, TM, 16)]

            def extras(t, us, pin):
                @functools.lru_cache(None)
                def node(n):
                    if n < 16:
                        rs = pl.ds(pl.multiple_of((i + 4 * zero_s[us[0] % 3]) * 64, 64) + (n // 4) * 512 + 24 + 8 * t, 8)
                        x = x_v[rs, (n % 4) * D4:(n % 4 + 1) * D4]
                        return (pin(x) if n in (0, 5, 10, 15) else x).astype(f32)
                    a, sa, b, sb = S49.up[n - 16]
                    return _run([(0, sa, 1, sb)], [node(a), node(b)])[-1]
                for u in us:
                    xe_v[S49.ul.index(u), pl.ds(pl.multiple_of(i * 16, 16) + t * 8, 8), :] = node(u).astype(bf16)

            xes = [(functools.partial(extras, t, us), None, xe_v, LG, 80) for t in range(2) for us in UPARTS]
            hs = {}

            def gelu_pieces(c, cs):
                def piece(r, cc, vs, pin):
                    t = _gelu(pin(_cat([cs[v][r:r + 8, cc:cc + 128] for v in vs], 0)))
                    ts = [t[8 * n:8 * n + 8] for n in range(len(vs))]
                    hs.update({(c, v, r, cc): u for v, u in zip(vs, ts)})
                    return functools.reduce(lambda a, b: a + b, ts)
                return [(functools.partial(piece, r, cc, range(v, v + 4)), None, None, LG, 40) for r in range(0, QM, 8)
                        for cc in range(0, cs[0].shape[1], 128) for v in range(0, SF.nb, 4)]

            def d3(c, side):
                c0, c1 = FCH[c]
                cs = fmm(SF, lambda u: lf_v[SF.ul.index(u), 0:QM], lambda r: s3_v[r, 0:D4, c0:c1], side)
                assert not side.pieces
                return gelu_pieces(c, cs)

            def d4(c, side):
                c0, c1 = FCH[c]
                lh = _run(SF.up, [_cat([_cat([hs.pop((c, v, r, cc)) for r in range(0, QM, 8)], 0)
                                        for cc in range(0, c1 - c0, 128)], 1) for v in range(SF.nb)])
                rhs = lambda r: s4_v[r, c0:c1, :]
                if c + 1 < len(FCH):
                    for n in SF.order:
                        for r in range(SF.rank):
                            if SF.wn[r] == n:
                                acc[n] = mm(lh[SF.un[r]], rhs(r), side, acc.get(n))
                else:
                    idx = lambda v: (pl.ds(r0 + (v // 4) * QM, QM), slice((v % 4) * D4, (v % 4 + 1) * D4))

                    def extra(n):
                        if n >= SF.nb:
                            return acc.get(n)
                        return b_v[idx(n)] + acc[n] if n in acc else b_v[idx(n)]

                    def emit_b(v, t):
                        b_v[idx(v)] = jnp.concatenate([1.0 - g_v[idx(v)[0], :]] * 2, axis=1) * t
                    fmm(SF, lambda u: lh[u], rhs, side, extra, emit_b)
                assert not side.pieces

            g0 = d3(0, Side(relays[:16], 43, 6))
            g1 = d3(1, Side(_merge(g0, gates[:8], xes), 43, 4))
            d4(0, Side(g1[:22], 41, 8))
            g2 = d3(2, Side(_merge(g1[22:], relays[16:32]), 47))
            d4(1, Side(_merge(g2, relays[32:60]), 43, 4))
            g3 = d3(3, Side(_merge(gates[8:], norms), 49))
            d4(2, Side(_merge(g3, combs), 43, 4))
            d4(3, Side(relays[60:], 44))

            @pl.when(i + 2 < NG)
            def _():
                qkv_start(i + 2)

            return carry

        lax.fori_loop(0, NB, ffn, 0)

    pl.run_scoped(
        phase_b,
        pltpu.VMEM((9, D // 4, D // 2), u32),
        pltpu.VMEM((7, D // 4, D // 2), u32),
        pltpu.VMEM((52, D4 + 16, F4), bf16),
        pltpu.VMEM((52, F4 + 8, D4), bf16),
        pltpu.VMEM((NT, S + 2 * PAD, 128), f32),
        pltpu.VMEM((TM, D), f32),
        pltpu.VMEM((2, 7, HM // 2, D // 2), u32),
        pltpu.VMEM((52, QM + 8, D4), bf16),
        pltpu.VMEM((2, TM, 128), f32),
        pltpu.VMEM((8, D), f32),
    )

    def phase_a(out_v, e_v, oe_v, ke_v, ve_v, o_v):
        def pre(it, carry):
            hist.clear()
            for u in range(3 * NG // NPRE):
                s0 = (it * (3 * NG // NPRE) + u) * G

                @functools.lru_cache(None)
                def node(k, n):
                    if n < 16:
                        return _unpack(wqkv_v[s0 + zero_s[k] + n % 4, (n // 4) * (D // 8):(n // 4 + 1) * (D // 8), :])
                    a, sa, b, sb = S49.vp[n - 16]
                    return _run([(0, sa, 1, sb)], [node(k, a), node(k, b)])[-1]

                def rhs(r):
                    n = S49.vn[r]
                    if n < 16:
                        return wqkv_v[s0 + n % 4, (n // 4) * (D // 8):(n // 4 + 1) * (D // 8), :]
                    return node(r // 7, n).astype(bf16)

                def emit_e(v, t):
                    e_v[(v // 4) * 8:(v // 4 + 1) * 8, s0 + v % 4] = _pack(t).reshape(8, 8, DH)
                fmm(S49N, lambda k: xe_v[S49.ul.index(k), 0:4 * NPAIR], rhs, None, emit=emit_e)
            return carry

        lax.fori_loop(0, NPRE, pre, 0)

        wait("wo")
        mem_v[...] = mem0_ref[...].astype(f32)

        def slab(w, h):
            return (h // G) * SPG + w * G + h % G

        def step(j, hx, odd, late, allow, fill):
            qs, ks, vs, ps = {}, {}, {}, {}
            wload = lambda w, h: pltpu.bitcast(wqkv_v[slab(w, h)], bf16)
            eload = lambda w, h: pltpu.bitcast(e_v[j, slab(w, h)], bf16)

            def proj(g):
                part = {}
                if late and g == 0:
                    for h in range(2):
                        for w in range(3):
                            part[w, h] = _dot(hx[:, :DH2], wload(w, h)[:DH2])
                for h in range(g * G, (g + 1) * G):
                    q, k, v = [(_dot(hx[:, DH2:], wload(w, h)[DH2:]) + part[w, h] if (w, h) in part
                                else _dot(hx, wload(w, h))).astype(bf16) for w in range(3)]
                    if odd:
                        q = jnp.concatenate([q, eload(0, h)], axis=0)
                        k = jnp.concatenate([pltpu.bitcast(ke_v[h], bf16), eload(1, h), k], axis=0)
                        v = jnp.concatenate([pltpu.bitcast(ve_v[h], bf16), eload(2, h), v], axis=0)
                    else:
                        ke_v[h] = pltpu.bitcast(k, u32)
                        ve_v[h] = pltpu.bitcast(v, u32)
                        k = jnp.concatenate([k, eload(1, h)], axis=0)
                        v = jnp.concatenate([v, eload(2, h)], axis=0)
                    qs[h], ks[h], vs[h] = q, k, v

            def score(g):
                for h in range(g * G, (g + 1) * G):
                    s = lax.dot_general(qs.pop(h), ks.pop(h), (((1,), (1,)), ((), ())),
                                        preferred_element_type=f32)
                    ps[h] = _softmax(s, allow, fill)

            def pv(g):
                os_ = []
                for h in range(g * G, (g + 1) * G):
                    o = _dot(ps.pop(h), vs.pop(h))
                    o_v[:, h * 128:(h + 1) * 128] = _pack(o[:32])
                    os_.append(o)
                if odd:
                    quads = [jnp.concatenate([os_[2 * kk][r:r + 8], os_[2 * kk + 1][r:r + 8]], axis=1)
                             for r in (32, 40) for kk in range(2)]
                    for k, t in enumerate(_lcombos(*quads)):
                        oe_v[k, pl.ds(pl.multiple_of(j * 8, 8), 8), g * 256:(g + 1) * 256] = t.astype(bf16)

            acc = [None] * NT

            def wo(h0, h1, j0, j1):
                o = pltpu.bitcast(o_v[:, h0 * 128:h1 * 128], bf16)
                for n in range(j0, j1):
                    y = _dot(o, pltpu.bitcast(wo_v[n, h0 * 64:h1 * 64, :], bf16))
                    acc[n] = y if acc[n] is None else y + acc[n]

            for t in range(NG):
                proj(t)
                if t >= 2:
                    pv(t - 2)
                if t >= 1:
                    score(t - 1)
            wo(0, 16, 0, 4)
            pv(NG - 2)
            score(NG - 1)
            wo(0, 16, 4, 8)
            pv(NG - 1)
            wo(16, 24, 0, 8)
            wo(24, 32, 0, 8)
            return jnp.concatenate(acc, axis=1)

        def emit(j, r0, o0, a):
            rs = pl.ds(r0 + o0, 24)
            g = jnp.concatenate([g_v[rs, :]] * NT, axis=1)
            out_v[j, o0:o0 + 24, :] = (g * a + b_v[rs, :]).astype(bf16)

        def pair(j, mem, late):
            r0 = pl.multiple_of(j * 64, 64)
            allow_e, fill_e, allow_o, fill_o = _masks()
            xa = x_v[pl.ds(r0 + 16, 8), :].astype(f32)
            xb = x_v[pl.ds(r0 + 40, 8), :].astype(f32)
            hx = jnp.concatenate([x_v[pl.ds(r0, 16), :], jnp.concatenate([xa, mem], 0).astype(bf16)], 0)
            oe = step(j, hx, False, late, allow_e, fill_e)
            emit(j, r0, 0, oe[:24])
            hx = jnp.concatenate([jnp.concatenate([oe[24:32], xb], 0).astype(bf16), x_v[pl.ds(r0 + 48, 16), :]], 0)
            oo = step(j, hx, True, True, allow_o, fill_o)
            emit(j, r0, 40, oo[8:])
            return oo[:8]

        def a_iter(it, carry):
            mem = mem_v[...]
            for t in range(PPI):
                mem = pair(it * PPI + t, mem, t > 0)
            mem_v[...] = mem
            for t in range(PPI):
                for o0 in (0, 40):
                    idx = (it * PPI + t, pl.ds(o0, 24))
                    pltpu.make_async_copy(out_v.at[idx], out_hbm.at[idx], sem_out).start()
            return carry

        lax.fori_loop(0, NPAIR // PPI, a_iter, 0)

        @once
        def _post():
            hist.clear()
            for n in range(NT // 2):
                quad = [lambda k, t=2 * n + q % 2, o=(q // 2) * 128: jnp.concatenate(
                    [wo_v[t + zero_s[k], g * 256 + o:g * 256 + o + 128, :] for g in range(NG)], axis=0) for q in range(4)]
                cs = strassen(lambda k: oe_v[k], lambda k: _rcombo(k, *quad), None)
                cols = slice(n * 256, (n + 1) * 256)
                for half in (1, 0):
                    t = jnp.concatenate(cs[2 * half:2 * half + 2], axis=1)
                    o0 = 24 + half * 8
                    for jj in range(NPAIR):
                        rs = slice(jj * 64 + o0, jj * 64 + o0 + 8)
                        g = jnp.concatenate([g_v[rs, :]] * 2, axis=1)
                        out_v[jj, o0:o0 + 8, cols] = (g * t[jj * 8:jj * 8 + 8] + b_v[rs, cols]).astype(bf16)
                    idx = (slice(None), pl.ds(o0, 8), pl.ds(n * 256, 256))
                    pltpu.make_async_copy(out_v.at[idx], out_hbm.at[idx], sem_out).start()

        pltpu.make_async_copy(out_v, out_hbm, sem_out).wait()

    pl.run_scoped(
        phase_a,
        pltpu.VMEM((NPAIR, 64, D), bf16),
        pltpu.VMEM((NPAIR, 3 * H, 8, DH), u32),
        pltpu.VMEM((7, 8 * NPAIR, H * DH // 2), bf16),
        pltpu.VMEM((H, 16, 128), u32),
        pltpu.VMEM((H, 16, 128), u32),
        pltpu.VMEM((16, H * DH), u32),
    )


@jax.jit
def pallas_gated_mix__memory_aug_recurrent_mem_tr__mixer_s_mlp__prompt_kernel(
    A_x, A_mem0, A_Wq, A_Wk, A_Wv, A_Wo, A_seg_len, B_x, B_w1, B_w2, B_w3, B_w4, gate_w,
):
    assert A_x.shape == (1, S, D) and A_mem0.shape == (1, M, D)
    any_spec = pl.BlockSpec(memory_space=pl.ANY)
    out = pl.pallas_call(
        _kernel,
        out_shape=jax.ShapeDtypeStruct((NPAIR, 64, D), bf16),
        in_specs=[any_spec] * 11,
        out_specs=any_spec,
        scratch_shapes=[
            pltpu.VMEM((S, D), bf16),
            pltpu.VMEM((3 * H, D // 2, DH), u32),
            pltpu.VMEM((NT, H * DH // 2 + 8, 128), u32),
            pltpu.VMEM((S, D), f32),
            pltpu.VMEM((S, 128), f32),
            pltpu.VMEM((52, 4 * NPAIR + 8, D4), bf16),
            pltpu.VMEM((M, D), f32),
            pltpu.VMEM((M, D), bf16),
            pltpu.VMEM((64, 128), bf16),
            pltpu.SMEM((S26.rank,), jnp.int32),
            pltpu.SemaphoreType.DMA((NLOAD,)),
            pltpu.SemaphoreType.DMA((NG,)),
            pltpu.SemaphoreType.DMA,
        ],
        compiler_params=pltpu.CompilerParams(vmem_limit_bytes=127 * 1024 * 1024,
                                             disable_bounds_checks=True),
    )(
        A_x.reshape(S, D), A_mem0.reshape(M, D),
        A_Wq.reshape(D // 2, 2 * H, DH), A_Wk.reshape(D // 2, 2 * H, DH), A_Wv.reshape(D // 2, 2 * H, DH),
        A_Wo.reshape(H * DH, D), B_w1, B_w2, B_w3, B_w4, gate_w.reshape(NT, 128),
    )
    return out.reshape(1, S, D)
```

```python
import functools

import jax
import jax.numpy as jnp
from jax import lax
import jax.experimental.pallas as pl
import jax.experimental.pallas.tpu as pltpu

f32, bf16, u32 = jnp.float32, jnp.bfloat16, jnp.uint32

S, D, H, DH, M, SEG, F = 2048, 1024, 32, 128, 8, 32, 3584
SCALE = DH ** -0.5
NEG = -1000000000.0
EPS = 1e-05

TM = 256
NB = S // TM
HM = TM // 2
DH2 = D // 2
D4, F4 = D // 4, F // 4
FCH = ((0, 128), (128, 384), (384, 640), (640, 896))
NC1 = 128
NPAIR = S // (2 * SEG)
PPI = 2
NPRE = 3
G = 4
NG = H // G
PAD = 8
NT = D // 128
TIEP = 2
W3A = 208
NLOAD = 11
assert NB == NG

_dot = functools.partial(jnp.dot, preferred_element_type=f32)

def _run(prog, blocks):
    vals = list(blocks)
    for a, sa, b, sb in prog:
        vals.append(vals[a] + vals[b] if sa > 0 and sb > 0 else
                    vals[a] - vals[b] if sa > 0 else vals[b] - vals[a])
    return vals


def _terms(prog, nin, node):
    if node < nin:
        return {node: 1}
    a, sa, b, sb = prog[node - nin]
    out = {k: sa * v for k, v in _terms(prog, nin, a).items()}
    out.update({k: sb * v for k, v in _terms(prog, nin, b).items()})
    return out


class _Scheme:
    def __init__(self, ms, up, vp, wp, un, vn, wn):
        self.ms, self.nb, self.rank = ms, 4 * ms, len(un)
        self.up, self.vp, self.wp, self.un, self.vn, self.wn = up, vp, wp, un, vn, wn
        self.ul = tuple(sorted(set(un)))
        t = {}
        for r in range(self.rank):
            for a, ca in _terms(up, self.nb, un[r]).items():
                for b, cb in _terms(vp, 16, vn[r]).items():
                    for c, cc in _terms(wp, self.nb, wn[r]).items():
                        t[a, b, c] = t.get((a, b, c), 0) + ca * cb * cc
        assert {k: v for k, v in t.items() if v} == {
            (4 * i + j, 4 * j + l, 4 * i + l): 1 for i in range(ms) for j in range(4) for l in range(4)}
        free = iter(r for r in range(self.rank) if vn[r] >= 16)
        self.raw = tuple(vn.index(q) if q in vn else next(free) for q in range(16))
        self.par = {n: [] for n in range(self.nb + len(wp))}
        for k, (a, sa, b, sb) in enumerate(wp):
            self.par[a].append((self.nb + k, sa))
            self.par[b].append((self.nb + k, sb))
        self.order = order = []

        def closure(n, acc):
            if n not in acc and n not in order:
                acc.add(n)
                for q, _ in self.par[n]:
                    closure(q, acc)
            return acc

        def visit(n):
            if n not in order:
                for q, _ in self.par[n]:
                    visit(q)
                order.append(n)
        while len([v for v in range(self.nb) if v not in order]):
            visit(min((v for v in range(self.nb) if v not in order), key=lambda v: len(closure(v, set()))))


UP = ((4, 1, 5, 1), (6, 1, 8, 1), (0, 1, 3, 1), (2, -1, 9, 1), (4, -1, 10, 1), (0, 1, 1, 1), (2, 1, 12, 1),
      (5, 1, 7, -1), (7, 1, 12, -1), (11, -1, 13, 1), (10, -1, 11, 1), (2, 1, 7, 1), (0, -1, 4, 1),
      (6, 1, 7, 1), (1, -1, 5, 1), (3, 1, 7, -1), (1, 1, 4, 1), (2, 1, 3, 1), (1, -1, 3, 1), (1, 1, 7, -1),
      (2, 1, 6, -1))
WP = ((0, -1, 3, 1), (4, 1, 6, -1), (1, 1, 8, 1), (5, 1, 10, 1), (4, -1, 7, 1), (0, -1, 9, -1),
      (11, 1, 12, 1), (6, 1, 7, -1), (2, 1, 5, -1), (0, -1, 7, -1), (9, 1, 11, -1), (2, 1, 13, 1),
      (5, 1, 13, 1), (2, -1, 3, 1), (5, 1, 6, 1), (0, 1, 4, 1), (2, 1, 7, 1), (1, 1, 2, 1), (1, 1, 5, 1),
      (3, 1, 7, 1), (2, 1, 6, 1))
VP = ((1, 1, 5, -1), (8, 1, 11, 1), (10, 1, 17, 1), (13, 1, 16, -1), (0, 1, 4, -1), (0, 1, 3, 1),
      (14, 1, 18, -1), (0, 1, 11, 1), (14, 1, 19, -1), (0, 1, 5, 1), (12, 1, 15, 1), (2, 1, 21, 1),
      (10, 1, 14, -1), (4, 1, 7, 1), (11, 1, 19, 1), (12, -1, 20, 1), (13, 1, 14, -1), (9, 1, 30, -1),
      (3, -1, 15, 1), (6, 1, 23, 1), (24, 1, 27, -1), (9, -1, 18, 1), (7, 1, 34, 1), (2, 1, 6, -1),
      (0, 1, 8, -1), (6, 1, 21, 1), (22, 1, 31, -1), (6, 1, 29, 1), (0, 1, 1, 1), (15, 1, 25, 1),
      (5, 1, 37, 1), (15, 1, 20, 1))
UN = (7, 27, 24, 17, 9, 22, 21, 2, 15, 11, 8, 25, 19, 28, 2, 23, 26, 20, 1, 18, 10, 28, 4, 13, 14, 16)
WN = (23, 17, 24, 10, 14, 7, 22, 19, 12, 18, 15, 25, 20, 5, 26, 0, 8, 2, 27, 11, 26, 9, 28, 21, 16, 5)
VN = (42, 47, 41, 5, 11, 43, 18, 28, 20, 23, 35, 19, 22, 46, 33, 26, 45, 36, 38, 25, 44, 40, 39, 21, 24, 32)
S26 = _Scheme(2, UP, VP, WP, UN, VN, WN)


def _twice(forms):
    prog, nodes = [], []

    def apply(f, quad):
        if len(f) == 1:
            return quad[f[0]]
        prog.append((quad[f[0]], f[1], quad[f[2]], f[3]))
        return 15 + len(prog)
    for f1 in forms:
        inner = [apply(f1, [4 * (2 * (q // 2) + p // 2) + 2 * (q % 2) + p % 2 for q in range(4)]) for p in range(4)]
        nodes += [apply(f2, inner) for f2 in forms]
    return tuple(prog), tuple(nodes)


_U2 = _twice(((0, 1, 3, 1), (2, 1, 3, 1), (0,), (3,), (0, 1, 1, 1), (2, 1, 0, -1), (1, 1, 3, -1)))
_V2 = _twice(((0, 1, 3, 1), (0,), (1, 1, 3, -1), (2, 1, 0, -1), (3,), (0, 1, 1, 1), (2, 1, 3, 1)))
_W2 = _twice(((0, 1, 3, 1), (2, 1, 3, -1), (1, 1, 3, 1), (0, 1, 2, 1), (1, 1, 0, -1), (3,), (0,)))
S49 = _Scheme(4, _U2[0], _V2[0], _W2[0], _U2[1], _V2[1], _W2[1])
VSTAGES = (((2, 5), (2, 7)), ((3, 6), (8, 13)), ((0, 1, 4), (0, 5, 10, 15)))
S49.raw = tuple(7 * (1, 2, 3, 4)[2 * (q // 8) + q % 4 // 2] + (1, 2, 3, 4)[2 * (q // 4 % 2) + q % 2] for q in range(16))
assert all(S49.raw[S49.vn[r]] == r for r in range(49) if S49.vn[r] < 16)


def _outer_major(n):
    seq = (1, 3, 4, 2, 0, 5, 6)
    rs = [7 * seq.index(r // 7) + seq.index(r % 7) for r in range(49) if S49.wn[r] == n]
    return max(rs + [-1] + [_outer_major(q) + 0.01 for q, _ in S49.par[n]])


S49N = _Scheme(4, _U2[0], _V2[0], _W2[0], _U2[1], _V2[1], _W2[1])
S49N.order.sort(key=_outer_major)
UPARTS = [[S49.un[r] for k in ks for r in range(7 * k, 7 * k + 7)] for ks in ((0, 2, 3), (4, 6), (1, 5))]
SF = S49
QM = TM // SF.ms


def _ln(x):
    m = jnp.mean(x, axis=-1, keepdims=True)
    xc = x - m
    v = jnp.mean(xc * xc, axis=-1, keepdims=True)
    return xc * lax.rsqrt(v + EPS)


_GC = 0.7978845608028654


def _gelu(x):
    h = 0.5 * x
    return h + h * jnp.tanh(x * (_GC + (_GC * 0.044715) * (x * x)))


def _unpack(u):
    return pltpu.bitcast(u, bf16).astype(f32)


def _pack(x):
    return pltpu.bitcast(x.astype(bf16), u32)


def _cat(xs, axis):
    xs = [x for x in xs if x.shape[axis]]
    return xs[0] if len(xs) == 1 else jnp.concatenate(xs, axis=axis)


def _as(x, dtype):
    return x if x.dtype == dtype else pltpu.bitcast(x, dtype)


def _lcombos(a11, a12, a21, a22):
    return [a11 + a22, a21 + a22, a11, a22, a11 + a12, a21 - a11, a12 - a22]


def _merge(*lists):
    keyed = [((j + 0.5) / len(l), n, j, v) for n, l in enumerate(lists) for j, v in enumerate(l)]
    return [v for _, _, _, v in sorted(keyed, key=lambda t: t[:3])]


def _masks():
    r = lax.broadcasted_iota(jnp.int32, (32, 48), 0)
    c = lax.broadcasted_iota(jnp.int32, (32, 48), 1)
    exist_e = c < 40
    allow_e = exist_e & ((r >= 24) | ((c >= 24) & (c < 32)) | (c <= r))
    fill_e = jnp.where(exist_e, NEG, -jnp.inf).astype(f32)
    r = lax.broadcasted_iota(jnp.int32, (48, 80), 0)
    c = lax.broadcasted_iota(jnp.int32, (48, 80), 1)
    q_even = (r >= 32) & (r < 40)
    exist_o = (q_even & (c < 40)) | (~q_even & (c >= 40))
    ktok = jnp.where(c < 24, c, jnp.where(c < 48, c - 8, c - 16))
    qtok = jnp.where(r < 32, r + 32, r - 8)
    is_mem_key = ((c >= 24) & (c < 32)) | ((c >= 48) & (c < 56))
    allow_o = exist_o & (is_mem_key | (r < 8) | (ktok <= qtok))
    fill_o = jnp.where(exist_o, NEG, -jnp.inf).astype(f32)
    return allow_e, fill_e, allow_o, fill_o


def _rcombo(k, b11, b12, b21, b22):
    if k in (1, 4):
        return (b11 if k == 1 else b22)(k)
    a, b, sign = {0: (b11, b22, 1), 2: (b12, b22, -1), 3: (b21, b11, -1), 5: (b11, b12, 1), 6: (b21, b22, 1)}[k]
    a, b = _unpack(a(k)), _unpack(b(k))
    return (a + b if sign > 0 else a - b).astype(bf16)


def _softmax(s, allow, fill):
    s = jnp.where(allow, s * SCALE, fill)
    m = jnp.max(s, axis=-1, keepdims=True)
    e = jnp.exp(s - m)
    l = jnp.sum(e, axis=-1, keepdims=True)
    r = pl.reciprocal(l, approx=True)
    r = r * (2.0 - l * r)
    return (e * r).astype(bf16)


def _kernel(x_hbm, mem0_hbm, wq_hbm, wk_hbm, wv_hbm, wo_hbm, w1_hbm, w2_hbm, w3_hbm, w4_hbm,
            gw_hbm, out_hbm,
            x_v, wqkv_v, wo_v, b_v, g_v, xe_v, mem_v, mem0_ref, gw_ref, zero_s,
            sem, sem_qkv, sem_out):
    RAW = (1, 2, 3, 4)
    RAW1 = (1, 7, 8, 4)

    loads = []

    def rows_load(name, r0, r1):
        loads.append((name, x_hbm.at[pl.ds(r0, r1 - r0)], x_v.at[pl.ds(r0, r1 - r0)]))

    def quad_load(name, w_hbm, s_v, raw, q, c0=0, c1=None):
        k4, n2 = s_v.shape[1], s_v.shape[2]
        c1 = n2 if c1 is None else c1
        src = w_hbm.bitcast(u32).at[pl.ds((q // 2) * k4, k4), pl.ds((q % 2) * n2 + c0, c1 - c0)]
        loads.append((name, src, s_v.at[raw[q], :, pl.ds(c0, c1 - c0)]))

    for j in range(NT):
        loads.append(("wo", wo_hbm.bitcast(u32).at[:, pl.ds(j * 128, 128)], wo_v.at[j, pl.ds(0, H * DH // 2)]))
    groups = []

    def start(*names, priority=0):
        for name, src, dst in loads:
            if name in names:
                pltpu.make_async_copy(src, dst, sem.at[groups.index(name)]).start(priority=priority)

    def wait(*names):
        for name, src, dst in loads:
            if name in names:
                pltpu.make_async_copy(src, dst, sem.at[groups.index(name)]).wait()

    SPG = 3 * G

    def qkv_start(g):
        for w, w_hbm in enumerate((wq_hbm, wk_hbm, wv_hbm)):
            wu = w_hbm.bitcast(u32)
            for k in range(G // 2):
                for par in range(2):
                    pltpu.make_async_copy(
                        wu.at[:, par * (H // 2) + g * (G // 2) + k, :],
                        wqkv_v.at[g * SPG + w * G + 2 * k + par], sem_qkv.at[g]).start(priority=1)

    def qkv_wait(g):
        grp = wqkv_v.at[pl.ds(g * SPG, SPG)]
        pltpu.make_async_copy(grp, grp, sem_qkv.at[g]).wait()

    def once(fn):
        def body(_, carry):
            fn()
            return carry
        lax.fori_loop(0, 1 + zero_s[1], body, 0)

    def tile_idx(ref, cols=128):
        z = zero_s[0]
        n = 16 if ref.dtype == bf16 and cols == 128 else 8
        return (z,) * (len(ref.shape) - 2) + (pl.ds(pl.multiple_of(z, n), n), slice(0, cols))

    hist = []

    def mm(lhs, rhs, side=None, acc=None):
        if side is not None:
            lhs = side(lhs)
        lhs = pltpu.bitcast(lhs, bf16) if lhs.dtype == u32 else lhs.astype(bf16)
        y = _dot(lhs, pltpu.bitcast(rhs, bf16) if rhs.dtype == u32 else rhs)
        if acc is not None:
            y = y + acc
        hist.append(y)
        return y

    class Side:
        def __init__(self, pieces, n, skip=0):
            cap = [0] * skip + [1] * n
            tot = sum(p[4] for p in pieces)
            self.plan = [[] for _ in cap]
            done = 0
            for p in pieces:
                done += p[4]
                x, d = done / tot * sum(cap), 0
                while x > cap[d] + 1e-9:
                    x -= cap[d]
                    d += 1
                self.plan[d].append((p, x / cap[d]))
            self.pieces = len(pieces)

        def __call__(self, val):
            todo = self.plan.pop(0) if self.plan else []
            if not todo:
                return val
            self.pieces -= len(todo)
            never = zero_s[0] > 0
            if val.dtype == bf16:
                val = pltpu.bitcast(val, u32)
            rg = 8 if val.dtype == u32 else 16
            ng = val.shape[0] // rg
            tied = {}
            for (fn, rd, wr, lag, _), pos in todo:
                m = min(max(-int(-pos * ng // 1) - 1, 0), ng - 1)
                pin = lambda v, w=128: v
                if lag is not None and len(hist) >= lag:
                    r0 = (16 * m) % hist[-lag].shape[0]
                    a = hist[-lag][r0:r0 + 8, :128]
                    if rd is None:
                        def pin(v, w=128, a=a):
                            if v.dtype == bf16:
                                return lax.select(never, _cat([a] * (v.shape[1] // 128), 1).astype(bf16), v)
                            a = _cat([_cat([_as(a, v.dtype)] * (v.shape[0] // 8), 0)] * (w // 128), 1)
                            if v.shape[1] == w:
                                return lax.select(never, a, v)
                            return _cat([lax.select(never, a, v[:, :w]), v[:, w:]], 1)
                    elif rd.dtype == bf16:
                        idx = tile_idx(rd, 256)
                        rd[idx] = lax.select(never, _cat([a, a], 1).astype(bf16), rd[idx])
                    else:
                        idx = tile_idx(rd)
                        rd[idx] = lax.select(never, _as(a, rd.dtype), rd[idx])
                u = fn(pin)
                if wr is False:
                    continue
                if wr is not None:
                    u = wr[tile_idx(wr)]
                t, n = tied.get(m * rg) or (val[m * rg:m * rg + 8, -128:], 0)
                tied[m * rg] = (lax.select(zero_s[n] > 0, _as(u, val.dtype), t), n + 1)
            if not tied:
                return val
            col, r = [], 0
            for r0 in sorted(tied):
                col += ([val[r:r0, -128:]] if r0 > r else []) + [tied[r0][0]]
                r = r0 + 8
            col += [val[r:, -128:]] if r < val.shape[0] else []
            return _cat([val[:, :-128], _cat(col, 0)], 1) if val.shape[1] > 128 else _cat(col, 0)

    def strassen(lhs, rhs, side, init=(None, None, None, None)):
        def add(a, b):
            return a if b is None else a + b
        p = [mm(lhs(k), rhs(k), side) for k in range(5)]
        c12 = add(p[2] + p[4], init[1])
        c21 = add(p[1] + p[3], init[2])
        c22 = mm(lhs(5), rhs(5), side, add(p[0] - p[1] + p[2], init[3]))
        c11 = mm(lhs(6), rhs(6), side, add(p[0] + p[3] - p[4], init[0]))
        return c11, c12, c21, c22

    def fmm(sc, lhs, rhs, side, extra=lambda n: None, emit=None):
        val = {}
        for n in sc.order:
            t = extra(n)
            for q, sg in sorted(sc.par[n], key=lambda e: -e[1]):
                t = val[q] if t is None else (t + val[q] if sg > 0 else t - val[q])
            for r in range(sc.rank):
                if sc.wn[r] == n:
                    t = mm(lhs(sc.un[r]), rhs(r), side, t)
            val[n] = t
            if n < sc.nb and emit is not None:
                emit(n, t)
        return [val[v] for v in range(sc.nb)]

    def phase_b(s1_v, s2_v, s3_v, s4_v, h_v, c0_v, l_v, lf_v, n_v, gb_v):
        def w1_load(name, half, c0, c1):
            quad_load(name, w1_hbm, s1_v, RAW1, half, c0, c1)
            quad_load(name, w1_hbm, s1_v, RAW1, 2 + half, c0, c1)

        def block_load(name, w_hbm, s_v, r0, r1):
            kb, nb = s_v.shape[1] // 128 * 128, s_v.shape[2]
            for q in range(16):
                loads.append((name, w_hbm.at[pl.ds((q // 4) * kb + r0, r1 - r0), pl.ds((q % 4) * nb, nb)],
                              s_v.at[SF.raw[q], pl.ds(r0, r1 - r0)]))

        rows_load("x0", 0, TM)
        w1_load("w1a", 0, 0, 256)
        rows_load("x1", TM, 2 * TM)
        w1_load("w1b", 0, 256, 512)
        w1_load("w1cd", 1, 0, 512)
        rows_load("x23", 2 * TM, 4 * TM)
        rows_load("x4567", 4 * TM, S)
        for q in range(4):
            quad_load("w2", w2_hbm, s2_v, RAW, q)
        block_load("w2", w3_hbm, s3_v, 0, W3A)
        block_load("w4", w3_hbm, s3_v, W3A, D4)
        block_load("w4", w4_hbm, s4_v, 0, F4)
        loads.append(("small", mem0_hbm, mem0_ref))
        loads.append(("small", gw_hbm, gw_ref.at[pl.ds(0, NT)]))
        groups.extend(dict.fromkeys(name for name, _, _ in loads))
        assert len(groups) == NLOAD

        start("x0", "w1a", "w1b", "x1", "w1cd", "x23", "x4567", "w2", "w4", "small")

        def zero(k, carry):
            zero_s[k] = 0
            return carry
        lax.fori_loop(0, S26.rank, zero, 0)

        def prepf_pieces(s_v, lag):
            def piece(rs, cs, st, pin):
                z = 4 * zero_s[st]

                @functools.lru_cache(None)
                def node(n):
                    if n < 16:
                        t = s_v[z + SF.raw[n], rs, cs]
                        return (pin(t) if n in VSTAGES[st][1] else t).astype(f32)
                    a, sa, b, sb = SF.vp[n - 16]
                    return _run([(0, sa, 1, sb)], [node(a), node(b)])[-1]
                rr = [r for k in VSTAGES[st][0] for r in range(7 * k, 7 * k + 7) if SF.raw.count(r) == 0 or SF.vn[r] >= 16]
                vals = [node(SF.vn[r]).astype(bf16) for r in rr]
                for r, t in zip(rr, vals):
                    s_v[z + r, rs, cs] = t
            kb, nb = s_v.shape[1] // 128 * 128, s_v.shape[2]
            out = []
            for r in range(0, kb, 16):
                out += [(slice(rr, rr + 8), slice(c, c + 256)) for c in range(0, nb - 255, 256) for rr in (r, r + 8)]
                out += [(slice(rr, rr + 8), slice(nb - 128, nb)) for rr in (r, r + 8)] if nb % 256 else []
            return [(functools.partial(piece, rs, cs, st), None, s_v if n % TIEP == TIEP - 1 else False, lag,
                     80 if cs.stop - cs.start == 256 else 60)
                    for g in range(0, len(out), 8) for st in range(3) for n, (rs, cs) in enumerate(out[g:g + 8])]

        def prep_pieces(s_v, raw, lag, width=256):
            def piece(r, c, pin):
                idx = (slice(r, r + 8), slice(c, c + width))
                b11, b12, b21, b22 = [_unpack(pin(s_v[(q,) + idx], width) if n in (0, 3) else s_v[(q,) + idx])
                                      for n, q in enumerate(raw)]
                for k, t in ((0, b11 + b22), (2, b12 - b22), (3, b21 - b11), (5, b11 + b12), (6, b21 + b22)):
                    s_v[(k,) + idx] = _pack(t)
            return [(functools.partial(piece, r, c), None, s_v, lag, 80)
                    for c in range(0, s_v.shape[2], width) for r in range(0, s_v.shape[1], 8)]

        def store_l(slot, q, c, quads):
            for k, t in enumerate(_lcombos(*quads)):
                l_v[slot, k, q // 2:q // 2 + 8, c:c + t.shape[1]] = _pack(t)

        def ln_pieces(src, r0, slot, lag, width=256, staged=False, clag=None):
            def stats(q, pin):
                x = pin(src[pl.ds(r0 + q, 16), :].astype(f32))
                xs = [x[:, j * 128:(j + 1) * 128] for j in range(NT)]
                m = functools.reduce(lambda a, b: a + b, xs) * (1.0 / NT)
                w = functools.reduce(lambda a, b: a + b, [(t - m) * (t - m) for t in xs])
                mean = jnp.mean(m, axis=-1, keepdims=True)
                var = jnp.sum(w + NT * ((m - mean) * (m - mean)), axis=-1, keepdims=True) * (1.0 / D)
                n_v[0, q:q + 16, :] = jnp.broadcast_to(mean, (16, 128))
                n_v[1, q:q + 16, :] = jnp.broadcast_to(lax.rsqrt(var + EPS), (16, 128))

            def comb(q, c, pin):
                quads = []
                for rr in (0, HM):
                    rs = pl.ds(pl.multiple_of(r0 + rr + q + zero_s[0], 16), 16)
                    mean, rstd = [jnp.concatenate([n_v[t, rr + q:rr + q + 16, :]] * (width // 128), axis=1)
                                  for t in range(2)]
                    quads += [(src[rs, cc + c:cc + c + width].astype(f32) - mean) * rstd for cc in (0, DH2)]
                store_l(slot, q, c, quads)

            def normf(q, pin):
                mean, rstd = [_cat([n_v[t, q:q + 16, :]] * NT, 1) for t in range(2)]
                c0_v[q:q + 16, :] = (src[pl.ds(pl.multiple_of(r0 + q + zero_s[0], 8), 16), :] - mean) * rstd

            def combf(q, us, pin):
                @functools.lru_cache(None)
                def node(n):
                    if n < SF.nb:
                        return c0_v[(n // 4) * QM + q:(n // 4) * QM + q + 8, (n % 4) * D4:(n % 4 + 1) * D4]
                    a, sa, b, sb = SF.up[n - SF.nb]
                    return _run([(0, sa, 1, sb)], [node(a), node(b)])[-1]
                for u in us:
                    lf_v[SF.ul.index(u), q:q + 8, :] = node(u).astype(bf16)
            dense = slot is not None or src is b_v
            norms = [[(functools.partial(stats, rr + q), None, n_v if dense else False, lag, 90) for rr in (0, HM)]
                     for q in range(0, HM, 16)]
            if slot is None:
                parts = [[SF.un[r] for k in ks for r in range(7 * k, 7 * k + 7)] for ks in ((0, 2, 3), (4, 6), (1, 5))]
                combs = [[(functools.partial(combf, q, us), c0_v, lf_v if dense or us is parts[-1] else False, clag, 55)
                          for us in parts] for q in range(0, QM, 8)]
            else:
                combs = [[(functools.partial(comb, q, c), n_v, l_v, clag, 125) for c in range(0, DH2, width)]
                         for q in range(0, HM, 16)]
            if staged:
                return (sum(norms, []) + [(functools.partial(normf, q), n_v, c0_v, clag, 40) for q in range(0, TM, 16)],
                        sum(combs, []))
            out = list(norms[0])
            for a, b in zip(norms[1:] + [[]], combs):
                out += _merge(a, b) if a else b
            return out

        shifts = (1, 1, -1, -1, 2, 2, -2, -2)

        def shift_pieces(r0, slot, lag, by_value=True):
            def piece(q, j, pin):
                a = [h_v[jj, pl.ds(PAD + r0 + rr + q - shifts[jj], 16), :]
                     for rr in (0, HM) for jj in (j, j + NT // 2)]
                store_l(slot, q, j * 128, [pin(a[0]), a[1], a[2], pin(a[3])])
            return [(functools.partial(piece, q, j), None if by_value else h_v,
                     l_v if j % 2 else False, lag, 50)
                    for q in range(0, HM, 16) for j in range(NT // 2)]

        def lhs_of(slot):
            return lambda k: l_v[slot, k]

        xe_v[0, 0:16, :] = jnp.zeros((16, D4), bf16)
        h_v[:, 0:PAD, :] = jnp.zeros((NT, PAD, 128), f32)
        h_v[:, PAD + S:PAD + S + PAD, :] = jnp.zeros((NT, PAD, 128), f32)

        def store_h(r0, c0, h):
            for j in range(h.shape[1] // 128):
                h_v[c0 // 128 + j, PAD + r0:PAD + r0 + h.shape[0], :] = h[:, j * 128:(j + 1) * 128]

        def h_pieces(r0, c0, t, lag, n=4):
            def piece(r, pin):
                store_h(r0 + r, c0, _gelu(pin(t[r:r + 8 * n])))
            return [(functools.partial(piece, r), None, h_v, lag, 10 * n) for r in range(0, t.shape[0], 8 * n)]

        def flush(pieces):
            for p in pieces:
                p[0](lambda v, w=128: v)

        def w1_cols(c, step):
            half, cc = c // DH2, c % DH2
            return jnp.concatenate([s1_v[RAW1[half], :, cc:cc + step], s1_v[RAW1[2 + half], :, cc:cc + step]], axis=0)

        def d1_plain(xn, r0, c0, c1, step):
            for c in range(c0, c1, step):
                store_h(r0, c, _gelu(mm(xn, w1_cols(c, step))))

        def d1_fine(lhs, r0, nrb, cols, pieces, carry, skip=0):
            tiles = [(rb, c) for c in cols for rb in range(nrb)]
            rounds = [tiles[i:i + 4] for i in range(0, len(tiles), 4)]
            for n, (rnd, part) in enumerate(zip(rounds, split(pieces, len(rounds)))):
                sk = skip if n == 0 else 0
                side = Side(_merge(carry, part) if carry else part, 8 - sk, sk)
                carry = []
                for rb, c in rnd:
                    half, cc = c // DH2, c % DH2
                    t = mm(lhs(rb, 0), s1_v[RAW1[half], :, cc:cc + 128], side)
                    t = mm(lhs(rb, 1), s1_v[RAW1[2 + half], :, cc:cc + 128], side, t)
                    carry += h_pieces(r0 + rb * HM, c, t, LS)
            return carry

        def d1_s(b, slot, pieces, carry, early=()):
            for c, part, e in zip(range(0, DH2, NC1), split(pieces, DH2 // NC1), split(early, 2) + [[], []]):
                side = Side(merge(carry, part, e), *((7,) if hist else (5, 2)))
                cs = strassen(lhs_of(slot), lambda k: s1_v[k, :, c:c + NC1], side)
                carry = sum([h_pieces(b * TM + (q // 2) * HM, (q % 2) * DH2 + c, cs[q], LS) for q in (1, 2, 3, 0)], [])
            return carry

        def d2_s(b, slot, pieces, carry=(), early=(), late=()):
            for c, part, e in zip(range(0, DH2, NC1), split(pieces, DH2 // NC1), split(early, 2) + split(late, 2)):
                side = Side(merge(carry, part, e), *((7,) if hist else (5, 2)))
                carry = ()
                idx = [(slice(b * TM + (q // 2) * HM, b * TM + (q // 2 + 1) * HM),
                        slice((q % 2) * DH2 + c, (q % 2) * DH2 + c + NC1)) for q in range(4)]
                cs = strassen(lhs_of(slot), lambda k: s2_v[k, :, c:c + NC1], side,
                              [x_v[i].astype(f32) for i in idx])
                for i, t in zip(idx, cs):
                    b_v[i] = t
                    if b == 0:
                        c0_v[i] = t

        def split(l, n):
            w = [1.0 if hist else 0.6] + [1.0] * (n - 1)
            cut = [int(round(len(l) * sum(w[:i]) / sum(w))) for i in range(n + 1)]
            return [l[cut[i]:cut[i + 1]] for i in range(n)]

        def merge(*ls):
            ls = [l for l in ls if l]
            return _merge(*ls) if ls else []

        NW1, NW3, N30 = 52, 32, 48
        LS, LL = 3, 5

        p3 = prepf_pieces(s3_v, LS)
        n3 = len(p3) * W3A // D4

        @once
        def _phase1a():
            wait("x0")
            xn0 = _pack(_ln(x_v[0:TM, :].astype(f32)))
            wait("w1a")
            d1_plain(xn0, 0, 0, 256, 256)
            wait("x1")
            xn1 = [_pack(_ln(x_v[r:r + HM, :].astype(f32))) for r in (TM, TM + HM)]
            for n in range(2):
                d1_plain(xn1[n], TM + n * HM, 0, 256, 256)
            wait("w1b")
            d1_plain(jnp.concatenate([xn0] + xn1, axis=0), 0, 256, 512, 256)
            wait("w1cd")
            hist.clear()
            xn01 = jnp.concatenate([xn0] + xn1, axis=0)
            l01 = lambda rb, kh: xn01[rb * 64:(rb + 1) * 64, kh * DH2:(kh + 1) * DH2]
            pw = prep_pieces(s1_v, RAW1, LS)
            flush(d1_fine(l01, 0, 4, (512, 640), pw[:NW1], [], 1))
            carry = []
            wait("x23")
            hist.clear()
            carry = d1_fine(l01, 0, 4, (768, 896), ln_pieces(x_v, 2 * TM, 0, LL), carry, 3)
            carry = d1_s(2, 0, ln_pieces(x_v, 3 * TM, 1, LL), carry, pw[NW1:])
            wait("x4567")
            qkv_start(0)
            qkv_start(1)
            hist.clear()
            for b in range(3, NB - 1):
                carry = d1_s(b, b % 2, ln_pieces(x_v, (b + 1) * TM, (b + 1) % 2, LL), carry)
            wait("w2")
            hist.clear()
            pw = prep_pieces(s2_v, RAW, LS)
            carry = d1_s(7, 1, _merge(pw[:NW3], shift_pieces(0, 0, LS, True)), carry)
            d2_s(0, 0, shift_pieces(TM, 1, LS, True), carry, pw[NW3:], p3[:N30])
            pw = split(_merge(p3[N30:n3], sum(ln_pieces(c0_v, 0, None, LL, clag=LS, staged=True), [])), 3)
            for b in range(1, 4):
                d2_s(b, b % 2, _merge(pw[b - 1], shift_pieces((b + 1) * TM, (b + 1) % 2, LS)))
            wait("w4", "small")

        hist.clear()
        pw = p3[n3:] + prepf_pieces(s4_v, LS)
        cut = (0, 93, 192, 291) + (len(pw),)
        for b in range(4, NB):
            d2_s(b, b % 2, merge(pw[cut[b - 4]:cut[b - 3]],
                                 shift_pieces((b + 1) * TM, (b + 1) % 2, LS) if b + 1 < NB else ()))
        start("wo", priority=1)
        gw = gw_ref[0:NT, :].astype(f32)
        gb_v[...] = _cat([jnp.broadcast_to(gw[j:j + 1, :], (8, 128)) for j in range(NT)], 1)

        def ffn(i, carry):
            qkv_wait(i)
            r0 = pl.multiple_of(i * TM, TM)
            rn = pl.multiple_of(jnp.minimum(i + 1, NB - 1) * TM, TM)
            acc = {}
            hist.clear()
            LG = 5

            def relayout(p, r0_, r1_, pin):
                s0 = i * SPG + 2 * p
                e = wqkv_v[s0, r0_:r1_, :]
                o = wqkv_v[s0 + 1, r0_:r1_, :]
                wqkv_v[s0, r0_:r1_, :] = (e & jnp.uint32(0xFFFF)) | (o << 16)
                wqkv_v[s0 + 1, r0_:r1_, :] = (e >> 16) | (o & jnp.uint32(0xFFFF0000))

            relays = [(functools.partial(relayout, p, r, r + 32), wqkv_v, wqkv_v, LG, 35)
                      for p in range(SPG // 2) for r in range(0, D // 2, 32)]
            norms, combs = ln_pieces(b_v, rn, None, 10, staged=True, clag=LG)

            def gate(q, pin):
                x = pin(x_v[pl.ds(r0 + q, 16), :].astype(f32)) * _cat([gb_v[...]] * 2, 0)
                t = functools.reduce(lambda a, b: a + b, [x[:, j * 128:(j + 1) * 128] for j in range(NT)])
                g = jax.nn.sigmoid(jnp.sum(t, axis=-1, keepdims=True))
                g_v[pl.ds(r0 + q, 16), :] = jnp.broadcast_to(g, (16, 128))

            gates = [(functools.partial(gate, q), None, g_v, 10, 90) for q in range(0, TM, 16)]

            def extras(t, us, pin):
                @functools.lru_cache(None)
                def node(n):
                    if n < 16:
                        rs = pl.ds(pl.multiple_of((i + 4 * zero_s[us[0] % 3]) * 64, 64) + (n // 4) * 512 + 24 + 8 * t, 8)
                        x = x_v[rs, (n % 4) * D4:(n % 4 + 1) * D4]
                        return (pin(x) if n in (0, 5, 10, 15) else x).astype(f32)
                    a, sa, b, sb = S49.up[n - 16]
                    return _run([(0, sa, 1, sb)], [node(a), node(b)])[-1]
                for u in us:
                    xe_v[S49.ul.index(u), pl.ds(pl.multiple_of(i * 16, 16) + t * 8, 8), :] = node(u).astype(bf16)

            xes = [(functools.partial(extras, t, us), None, xe_v, LG, 80) for t in range(2) for us in UPARTS]
            hs = {}

            def gelu_pieces(c, cs):
                def piece(r, cc, vs, pin):
                    t = _gelu(pin(_cat([cs[v][r:r + 8, cc:cc + 128] for v in vs], 0)))
                    ts = [t[8 * n:8 * n + 8] for n in range(len(vs))]
                    hs.update({(c, v, r, cc): u for v, u in zip(vs, ts)})
                    return functools.reduce(lambda a, b: a + b, ts)
                return [(functools.partial(piece, r, cc, range(v, v + 4)), None, None, LG, 40) for r in range(0, QM, 8)
                        for cc in range(0, cs[0].shape[1], 128) for v in range(0, SF.nb, 4)]

            def d3(c, side):
                c0, c1 = FCH[c]
                cs = fmm(SF, lambda u: lf_v[SF.ul.index(u), 0:QM], lambda r: s3_v[r, 0:D4, c0:c1], side)
                assert not side.pieces
                return gelu_pieces(c, cs)

            def d4(c, side):
                c0, c1 = FCH[c]
                lh = _run(SF.up, [_cat([_cat([hs.pop((c, v, r, cc)) for r in range(0, QM, 8)], 0)
                                        for cc in range(0, c1 - c0, 128)], 1) for v in range(SF.nb)])
                rhs = lambda r: s4_v[r, c0:c1, :]
                if c + 1 < len(FCH):
                    for n in SF.order:
                        for r in range(SF.rank):
                            if SF.wn[r] == n:
                                acc[n] = mm(lh[SF.un[r]], rhs(r), side, acc.get(n))
                else:
                    idx = lambda v: (pl.ds(r0 + (v // 4) * QM, QM), slice((v % 4) * D4, (v % 4 + 1) * D4))

                    def extra(n):
                        if n >= SF.nb:
                            return acc.get(n)
                        return b_v[idx(n)] + acc[n] if n in acc else b_v[idx(n)]

                    def emit_b(v, t):
                        b_v[idx(v)] = jnp.concatenate([1.0 - g_v[idx(v)[0], :]] * 2, axis=1) * t
                    fmm(SF, lambda u: lh[u], rhs, side, extra, emit_b)
                assert not side.pieces

            g0 = d3(0, Side(relays[:16], 43, 6))
            g1 = d3(1, Side(_merge(g0, gates[:12]), 43, 4))
            d4(0, Side(g1[:22], 41, 8))
            g2 = d3(2, Side(_merge(g1[22:], relays[16:32]), 47))
            d4(1, Side(_merge(g2, relays[32:60]), 43, 4))
            g3 = d3(3, Side(_merge(gates[12:], xes, norms), 49))
            d4(2, Side(_merge(g3, combs), 43, 4))
            d4(3, Side(relays[60:], 44))

            @pl.when(i + 2 < NG)
            def _():
                qkv_start(i + 2)

            return carry

        lax.fori_loop(0, NB, ffn, 0)

    pl.run_scoped(
        phase_b,
        pltpu.VMEM((9, D // 4, D // 2), u32),
        pltpu.VMEM((7, D // 4, D // 2), u32),
        pltpu.VMEM((52, D4 + 16, F4), bf16),
        pltpu.VMEM((52, F4 + 8, D4), bf16),
        pltpu.VMEM((NT, S + 2 * PAD, 128), f32),
        pltpu.VMEM((TM, D), f32),
        pltpu.VMEM((2, 7, HM // 2, D // 2), u32),
        pltpu.VMEM((52, QM + 8, D4), bf16),
        pltpu.VMEM((2, TM, 128), f32),
        pltpu.VMEM((8, D), f32),
    )

    def phase_a(out_v, e_v, oe_v, ke_v, ve_v, o_v):
        def pre(it, carry):
            hist.clear()
            for u in range(3 * NG // NPRE):
                s0 = (it * (3 * NG // NPRE) + u) * G

                @functools.lru_cache(None)
                def node(k, n):
                    if n < 16:
                        return _unpack(wqkv_v[s0 + zero_s[k] + n % 4, (n // 4) * (D // 8):(n // 4 + 1) * (D // 8), :])
                    a, sa, b, sb = S49.vp[n - 16]
                    return _run([(0, sa, 1, sb)], [node(k, a), node(k, b)])[-1]

                def rhs(r):
                    n = S49.vn[r]
                    if n < 16:
                        return wqkv_v[s0 + n % 4, (n // 4) * (D // 8):(n // 4 + 1) * (D // 8), :]
                    return node(r // 7, n).astype(bf16)

                def emit_e(v, t):
                    e_v[(v // 4) * 8:(v // 4 + 1) * 8, s0 + v % 4] = _pack(t).reshape(8, 8, DH)
                fmm(S49N, lambda k: xe_v[S49.ul.index(k), 0:4 * NPAIR], rhs, None, emit=emit_e)
            return carry

        lax.fori_loop(0, NPRE, pre, 0)

        wait("wo")
        mem_v[...] = mem0_ref[...].astype(f32)

        def slab(w, h):
            return (h // G) * SPG + w * G + h % G

        def step(j, hx, odd, late, allow, fill):
            qs, ks, vs, ps = {}, {}, {}, {}
            wload = lambda w, h: pltpu.bitcast(wqkv_v[slab(w, h)], bf16)
            eload = lambda w, h: pltpu.bitcast(e_v[j, slab(w, h)], bf16)

            def proj(g):
                part = {}
                if late and g == 0:
                    for h in range(2):
                        for w in range(3):
                            part[w, h] = _dot(hx[:, :DH2], wload(w, h)[:DH2])
                for h in range(g * G, (g + 1) * G):
                    q, k, v = [(_dot(hx[:, DH2:], wload(w, h)[DH2:]) + part[w, h] if (w, h) in part
                                else _dot(hx, wload(w, h))).astype(bf16) for w in range(3)]
                    if odd:
                        q = jnp.concatenate([q, eload(0, h)], axis=0)
                        k = jnp.concatenate([pltpu.bitcast(ke_v[h], bf16), eload(1, h), k], axis=0)
                        v = jnp.concatenate([pltpu.bitcast(ve_v[h], bf16), eload(2, h), v], axis=0)
                    else:
                        ke_v[h] = pltpu.bitcast(k, u32)
                        ve_v[h] = pltpu.bitcast(v, u32)
                        k = jnp.concatenate([k, eload(1, h)], axis=0)
                        v = jnp.concatenate([v, eload(2, h)], axis=0)
                    qs[h], ks[h], vs[h] = q, k, v

            def score(g):
                for h in range(g * G, (g + 1) * G):
                    s = lax.dot_general(qs.pop(h), ks.pop(h), (((1,), (1,)), ((), ())),
                                        preferred_element_type=f32)
                    ps[h] = _softmax(s, allow, fill)

            def pv(g):
                os_ = []
                for h in range(g * G, (g + 1) * G):
                    o = _dot(ps.pop(h), vs.pop(h))
                    o_v[:, h * 128:(h + 1) * 128] = _pack(o[:32])
                    os_.append(o)
                if odd:
                    quads = [jnp.concatenate([os_[2 * kk][r:r + 8], os_[2 * kk + 1][r:r + 8]], axis=1)
                             for r in (32, 40) for kk in range(2)]
                    for k, t in enumerate(_lcombos(*quads)):
                        oe_v[k, pl.ds(pl.multiple_of(j * 8, 8), 8), g * 256:(g + 1) * 256] = t.astype(bf16)

            acc = [None] * NT

            def wo(h0, h1, j0, j1):
                o = pltpu.bitcast(o_v[:, h0 * 128:h1 * 128], bf16)
                for n in range(j0, j1):
                    y = _dot(o, pltpu.bitcast(wo_v[n, h0 * 64:h1 * 64, :], bf16))
                    acc[n] = y if acc[n] is None else y + acc[n]

            for t in range(NG):
                proj(t)
                if t >= 2:
                    pv(t - 2)
                if t >= 1:
                    score(t - 1)
            wo(0, 16, 0, 4)
            pv(NG - 2)
            score(NG - 1)
            wo(0, 16, 4, 8)
            pv(NG - 1)
            wo(16, 24, 0, 8)
            wo(24, 32, 0, 8)
            return jnp.concatenate(acc, axis=1)

        def emit(j, r0, o0, a):
            rs = pl.ds(r0 + o0, 24)
            g = jnp.concatenate([g_v[rs, :]] * NT, axis=1)
            out_v[j, o0:o0 + 24, :] = (g * a + b_v[rs, :]).astype(bf16)

        def pair(j, mem, late):
            r0 = pl.multiple_of(j * 64, 64)
            allow_e, fill_e, allow_o, fill_o = _masks()
            xa = x_v[pl.ds(r0 + 16, 8), :].astype(f32)
            xb = x_v[pl.ds(r0 + 40, 8), :].astype(f32)
            hx = jnp.concatenate([x_v[pl.ds(r0, 16), :], jnp.concatenate([xa, mem], 0).astype(bf16)], 0)
            oe = step(j, hx, False, late, allow_e, fill_e)
            emit(j, r0, 0, oe[:24])
            hx = jnp.concatenate([jnp.concatenate([oe[24:32], xb], 0).astype(bf16), x_v[pl.ds(r0 + 48, 16), :]], 0)
            oo = step(j, hx, True, True, allow_o, fill_o)
            emit(j, r0, 40, oo[8:])
            return oo[:8]

        def a_iter(it, carry):
            mem = mem_v[...]
            for t in range(PPI):
                mem = pair(it * PPI + t, mem, t > 0)
            mem_v[...] = mem
            for t in range(PPI):
                for o0 in (0, 40):
                    idx = (it * PPI + t, pl.ds(o0, 24))
                    pltpu.make_async_copy(out_v.at[idx], out_hbm.at[idx], sem_out).start()
            return carry

        lax.fori_loop(0, NPAIR // PPI, a_iter, 0)

        @once
        def _post():
            hist.clear()
            for n in range(NT // 2):
                quad = [lambda k, t=2 * n + q % 2, o=(q // 2) * 128: jnp.concatenate(
                    [wo_v[t + zero_s[k], g * 256 + o:g * 256 + o + 128, :] for g in range(NG)], axis=0) for q in range(4)]
                cs = strassen(lambda k: oe_v[k], lambda k: _rcombo(k, *quad), None)
                cols = slice(n * 256, (n + 1) * 256)
                for half in (1, 0):
                    t = jnp.concatenate(cs[2 * half:2 * half + 2], axis=1)
                    o0 = 24 + half * 8
                    for jj in range(NPAIR):
                        rs = slice(jj * 64 + o0, jj * 64 + o0 + 8)
                        g = jnp.concatenate([g_v[rs, :]] * 2, axis=1)
                        out_v[jj, o0:o0 + 8, cols] = (g * t[jj * 8:jj * 8 + 8] + b_v[rs, cols]).astype(bf16)
                    idx = (slice(None), pl.ds(o0, 8), pl.ds(n * 256, 256))
                    pltpu.make_async_copy(out_v.at[idx], out_hbm.at[idx], sem_out).start()

        pltpu.make_async_copy(out_v, out_hbm, sem_out).wait()

    pl.run_scoped(
        phase_a,
        pltpu.VMEM((NPAIR, 64, D), bf16),
        pltpu.VMEM((NPAIR, 3 * H, 8, DH), u32),
        pltpu.VMEM((7, 8 * NPAIR, H * DH // 2), bf16),
        pltpu.VMEM((H, 16, 128), u32),
        pltpu.VMEM((H, 16, 128), u32),
        pltpu.VMEM((16, H * DH), u32),
    )


@jax.jit
def pallas_gated_mix__memory_aug_recurrent_mem_tr__mixer_s_mlp__prompt_kernel(
    A_x, A_mem0, A_Wq, A_Wk, A_Wv, A_Wo, A_seg_len, B_x, B_w1, B_w2, B_w3, B_w4, gate_w,
):
    assert A_x.shape == (1, S, D) and A_mem0.shape == (1, M, D)
    any_spec = pl.BlockSpec(memory_space=pl.ANY)
    out = pl.pallas_call(
        _kernel,
        out_shape=jax.ShapeDtypeStruct((NPAIR, 64, D), bf16),
        in_specs=[any_spec] * 11,
        out_specs=any_spec,
        scratch_shapes=[
            pltpu.VMEM((S, D), bf16),
            pltpu.VMEM((3 * H, D // 2, DH), u32),
            pltpu.VMEM((NT, H * DH // 2 + 8, 128), u32),
            pltpu.VMEM((S, D), f32),
            pltpu.VMEM((S, 128), f32),
            pltpu.VMEM((52, 4 * NPAIR + 8, D4), bf16),
            pltpu.VMEM((M, D), f32),
            pltpu.VMEM((M, D), bf16),
            pltpu.VMEM((64, 128), bf16),
            pltpu.SMEM((S26.rank,), jnp.int32),
            pltpu.SemaphoreType.DMA((NLOAD,)),
            pltpu.SemaphoreType.DMA((NG,)),
            pltpu.SemaphoreType.DMA,
        ],
        compiler_params=pltpu.CompilerParams(vmem_limit_bytes=127 * 1024 * 1024,
                                             disable_bounds_checks=True),
    )(
        A_x.reshape(S, D), A_mem0.reshape(M, D),
        A_Wq.reshape(D // 2, 2 * H, DH), A_Wk.reshape(D // 2, 2 * H, DH), A_Wv.reshape(D // 2, 2 * H, DH),
        A_Wo.reshape(H * DH, D), B_w1, B_w2, B_w3, B_w4, gate_w.reshape(NT, 128),
    )
    return out.reshape(1, S, D)
```

```python
import functools

import jax
import jax.numpy as jnp
from jax import lax
import jax.experimental.pallas as pl
import jax.experimental.pallas.tpu as pltpu

f32, bf16, u32 = jnp.float32, jnp.bfloat16, jnp.uint32

S, D, H, DH, M, SEG, F = 2048, 1024, 32, 128, 8, 32, 3584
SCALE = DH ** -0.5
NEG = -1000000000.0
EPS = 1e-05

TM = 256
NB = S // TM
HM = TM // 2
DH2 = D // 2
D4, F4 = D // 4, F // 4
FCH = ((0, 128), (128, 384), (384, 640), (640, 896))
NC1 = 128
NPAIR = S // (2 * SEG)
PPI = 2
NPRE = 3
G = 4
NG = H // G
PAD = 8
NT = D // 128
TIEP = 2
W3A = 208
NZ = 16
NLOAD = 11
assert NB == NG

_dot = functools.partial(jnp.dot, preferred_element_type=f32)

def _run(prog, blocks):
    vals = list(blocks)
    for a, sa, b, sb in prog:
        vals.append(vals[a] + vals[b] if sa > 0 and sb > 0 else
                    vals[a] - vals[b] if sa > 0 else vals[b] - vals[a])
    return vals


def _terms(prog, nin, node):
    if node < nin:
        return {node: 1}
    a, sa, b, sb = prog[node - nin]
    out = {k: sa * v for k, v in _terms(prog, nin, a).items()}
    out.update({k: sb * v for k, v in _terms(prog, nin, b).items()})
    return out


class _Scheme:
    def __init__(self, ms, up, vp, wp, un, vn, wn):
        self.ms, self.nb, self.rank = ms, 4 * ms, len(un)
        self.up, self.vp, self.wp, self.un, self.vn, self.wn = up, vp, wp, un, vn, wn
        self.ul = tuple(sorted(set(un)))
        t = {}
        for r in range(self.rank):
            for a, ca in _terms(up, self.nb, un[r]).items():
                for b, cb in _terms(vp, 16, vn[r]).items():
                    for c, cc in _terms(wp, self.nb, wn[r]).items():
                        t[a, b, c] = t.get((a, b, c), 0) + ca * cb * cc
        assert {k: v for k, v in t.items() if v} == {
            (4 * i + j, 4 * j + l, 4 * i + l): 1 for i in range(ms) for j in range(4) for l in range(4)}
        self.par = {n: [] for n in range(self.nb + len(wp))}
        for k, (a, sa, b, sb) in enumerate(wp):
            self.par[a].append((self.nb + k, sa))
            self.par[b].append((self.nb + k, sb))
        self.order = order = []

        def closure(n, acc):
            if n not in acc and n not in order:
                acc.add(n)
                for q, _ in self.par[n]:
                    closure(q, acc)
            return acc

        def visit(n):
            if n not in order:
                for q, _ in self.par[n]:
                    visit(q)
                order.append(n)
        while len([v for v in range(self.nb) if v not in order]):
            visit(min((v for v in range(self.nb) if v not in order), key=lambda v: len(closure(v, set()))))


def _twice(forms):
    prog, nodes = [], []

    def apply(f, quad):
        if len(f) == 1:
            return quad[f[0]]
        prog.append((quad[f[0]], f[1], quad[f[2]], f[3]))
        return 15 + len(prog)
    for f1 in forms:
        inner = [apply(f1, [4 * (2 * (q // 2) + p // 2) + 2 * (q % 2) + p % 2 for q in range(4)]) for p in range(4)]
        nodes += [apply(f2, inner) for f2 in forms]
    return tuple(prog), tuple(nodes)


UFORMS = ((0, 1, 3, 1), (2, 1, 3, 1), (0,), (3,), (0, 1, 1, 1), (2, 1, 0, -1), (1, 1, 3, -1))
UQ = [f[::2] for f in UFORMS]
SEQ = (1, 3, 4, 2, 0, 5, 6)
_U2 = _twice(UFORMS)
_V2 = _twice(((0, 1, 3, 1), (0,), (1, 1, 3, -1), (2, 1, 0, -1), (3,), (0, 1, 1, 1), (2, 1, 3, 1)))
_W2 = _twice(((0, 1, 3, 1), (2, 1, 3, -1), (1, 1, 3, 1), (0, 1, 2, 1), (1, 1, 0, -1), (3,), (0,)))
S49 = _Scheme(4, _U2[0], _V2[0], _W2[0], _U2[1], _V2[1], _W2[1])
VSTAGES = (((2, 5), (2, 7)), ((3, 6), (8, 13)), ((0, 1, 4), (0, 5, 10, 15)))
S49.raw = tuple(7 * (1, 2, 3, 4)[2 * (q // 8) + q % 4 // 2] + (1, 2, 3, 4)[2 * (q // 4 % 2) + q % 2] for q in range(16))
assert all(S49.raw[S49.vn[r]] == r for r in range(49) if S49.vn[r] < 16)


def _outer_major(n):
    rs = [7 * SEQ.index(r // 7) + SEQ.index(r % 7) for r in range(49) if S49.wn[r] == n]
    return max(rs + [-1] + [_outer_major(q) + 0.01 for q, _ in S49.par[n]])


S49N = _Scheme(4, _U2[0], _V2[0], _W2[0], _U2[1], _V2[1], _W2[1])
S49N.order.sort(key=_outer_major)
UPARTS = [[S49.un[r] for k in ks for r in range(7 * k, 7 * k + 7)] for ks in ((0, 2, 3), (4, 6), (1, 5))]
SF = S49
QM = TM // SF.ms


def _ln(x):
    m = jnp.mean(x, axis=-1, keepdims=True)
    xc = x - m
    v = jnp.mean(xc * xc, axis=-1, keepdims=True)
    return xc * lax.rsqrt(v + EPS)


_GC = 0.7978845608028654


def _gelu(x):
    h = 0.5 * x
    return h + h * jnp.tanh(x * (_GC + (_GC * 0.044715) * (x * x)))


def _unpack(u):
    return pltpu.bitcast(u, bf16).astype(f32)


def _pack(x):
    return pltpu.bitcast(x.astype(bf16), u32)


def _cat(xs, axis):
    xs = [x for x in xs if x.shape[axis]]
    return xs[0] if len(xs) == 1 else jnp.concatenate(xs, axis=axis)


def _as(x, dtype):
    return x if x.dtype == dtype else pltpu.bitcast(x, dtype)


def _lcombos(a11, a12, a21, a22):
    return [a11 + a22, a21 + a22, a11, a22, a11 + a12, a21 - a11, a12 - a22]


def _merge(*lists):
    keyed = [((j + 0.5) / len(l), n, j, v) for n, l in enumerate(lists) for j, v in enumerate(l)]
    return [v for _, _, _, v in sorted(keyed, key=lambda t: t[:3])]


def _masks():
    r = lax.broadcasted_iota(jnp.int32, (32, 48), 0)
    c = lax.broadcasted_iota(jnp.int32, (32, 48), 1)
    exist_e = c < 40
    allow_e = exist_e & ((r >= 24) | ((c >= 24) & (c < 32)) | (c <= r))
    fill_e = jnp.where(exist_e, NEG, -jnp.inf).astype(f32)
    r = lax.broadcasted_iota(jnp.int32, (48, 80), 0)
    c = lax.broadcasted_iota(jnp.int32, (48, 80), 1)
    q_even = (r >= 32) & (r < 40)
    exist_o = (q_even & (c < 40)) | (~q_even & (c >= 40))
    ktok = jnp.where(c < 24, c, jnp.where(c < 48, c - 8, c - 16))
    qtok = jnp.where(r < 32, r + 32, r - 8)
    is_mem_key = ((c >= 24) & (c < 32)) | ((c >= 48) & (c < 56))
    allow_o = exist_o & (is_mem_key | (r < 8) | (ktok <= qtok))
    fill_o = jnp.where(exist_o, NEG, -jnp.inf).astype(f32)
    return allow_e, fill_e, allow_o, fill_o


def _softmax(s, allow, fill):
    s = jnp.where(allow, s * SCALE, fill)
    m = jnp.max(s, axis=-1, keepdims=True)
    e = jnp.exp(s - m)
    l = jnp.sum(e, axis=-1, keepdims=True)
    r = pl.reciprocal(l, approx=True)
    r = r * (2.0 - l * r)
    return (e * r).astype(bf16)


def _kernel(x_hbm, mem0_hbm, wq_hbm, wk_hbm, wv_hbm, wo_hbm, w1_hbm, w2_hbm, w3_hbm, w4_hbm,
            gw_hbm, out_hbm,
            x_v, wqkv_v, wo_v, b_v, g_v, xe_v, mem_v, mem0_ref, gw_ref, zero_s,
            sem, sem_qkv, sem_out):
    RAW = (1, 2, 3, 4)
    RAW1 = (1, 7, 8, 4)

    loads = []

    def rows_load(name, r0, r1):
        loads.append((name, x_hbm.at[pl.ds(r0, r1 - r0)], x_v.at[pl.ds(r0, r1 - r0)]))

    def quad_load(name, w_hbm, s_v, raw, q, c0=0, c1=None):
        k4, n2 = s_v.shape[1], s_v.shape[2]
        c1 = n2 if c1 is None else c1
        src = w_hbm.bitcast(u32).at[pl.ds((q // 2) * k4, k4), pl.ds((q % 2) * n2 + c0, c1 - c0)]
        loads.append((name, src, s_v.at[raw[q], :, pl.ds(c0, c1 - c0)]))

    for j in range(NT):
        loads.append(("wo", wo_hbm.bitcast(u32).at[:, pl.ds(j * 128, 128)], wo_v.at[j, pl.ds(0, H * DH // 2)]))
    groups = []

    def start(*names, priority=0):
        for name, src, dst in loads:
            if name in names:
                pltpu.make_async_copy(src, dst, sem.at[groups.index(name)]).start(priority=priority)

    def wait(*names):
        for name, src, dst in loads:
            if name in names:
                pltpu.make_async_copy(src, dst, sem.at[groups.index(name)]).wait()

    SPG = 3 * G

    def qkv_start(g):
        for w, w_hbm in enumerate((wq_hbm, wk_hbm, wv_hbm)):
            wu = w_hbm.bitcast(u32)
            for k in range(G // 2):
                for par in range(2):
                    pltpu.make_async_copy(
                        wu.at[:, par * (H // 2) + g * (G // 2) + k, :],
                        wqkv_v.at[g * SPG + w * G + 2 * k + par], sem_qkv.at[g]).start(priority=1)

    def qkv_wait(g):
        grp = wqkv_v.at[pl.ds(g * SPG, SPG)]
        pltpu.make_async_copy(grp, grp, sem_qkv.at[g]).wait()

    def once(fn):
        def body(_, carry):
            fn()
            return carry
        lax.fori_loop(0, 1 + zero_s[1], body, 0)

    def tile_idx(ref, cols=128):
        z = zero_s[0]
        n = 16 if ref.dtype == bf16 and cols == 128 else 8
        return (z,) * (len(ref.shape) - 2) + (pl.ds(pl.multiple_of(z, n), n), slice(0, cols))

    hist = []

    def mm(lhs, rhs, side=None, acc=None):
        if side is not None:
            lhs = side(lhs)
        lhs = pltpu.bitcast(lhs, bf16) if lhs.dtype == u32 else lhs.astype(bf16)
        y = _dot(lhs, pltpu.bitcast(rhs, bf16) if rhs.dtype == u32 else rhs)
        if acc is not None:
            y = y + acc
        hist.append(y)
        return y

    class Side:
        def __init__(self, pieces, n, skip=0):
            cap = [0] * skip + [1] * n
            tot = sum(p[4] for p in pieces)
            self.plan = [[] for _ in cap]
            done = 0
            for p in pieces:
                done += p[4]
                x, d = done / tot * sum(cap), 0
                while x > cap[d] + 1e-9:
                    x -= cap[d]
                    d += 1
                self.plan[d].append((p, x / cap[d]))
            self.pieces = len(pieces)

        def __call__(self, val):
            todo = self.plan.pop(0) if self.plan else []
            if not todo:
                return val
            self.pieces -= len(todo)
            never = zero_s[0] > 0
            if val.dtype == bf16:
                val = pltpu.bitcast(val, u32)
            rg = 8 if val.dtype == u32 else 16
            ng = val.shape[0] // rg
            tied = {}
            for (fn, rd, wr, lag, _), pos in todo:
                m = min(max(-int(-pos * ng // 1) - 1, 0), ng - 1)
                pin = lambda v, w=128: v
                if lag is not None and len(hist) >= lag:
                    r0 = (16 * m) % hist[-lag].shape[0]
                    a = hist[-lag][r0:r0 + 8, :128]
                    if rd is None:
                        def pin(v, w=128, a=a):
                            if v.dtype == bf16:
                                return lax.select(never, _cat([a] * (v.shape[1] // 128), 1).astype(bf16), v)
                            a = _cat([_cat([_as(a, v.dtype)] * (v.shape[0] // 8), 0)] * (w // 128), 1)
                            if v.shape[1] == w:
                                return lax.select(never, a, v)
                            return _cat([lax.select(never, a, v[:, :w]), v[:, w:]], 1)
                    elif rd.dtype == bf16:
                        idx = tile_idx(rd, 256)
                        rd[idx] = lax.select(never, _cat([a, a], 1).astype(bf16), rd[idx])
                    else:
                        idx = tile_idx(rd)
                        rd[idx] = lax.select(never, _as(a, rd.dtype), rd[idx])
                u = fn(pin)
                if wr is False:
                    continue
                if wr is not None:
                    u = wr[tile_idx(wr)]
                t, n = tied.get(m * rg) or (val[m * rg:m * rg + 8, -128:], 0)
                tied[m * rg] = (lax.select(zero_s[n] > 0, _as(u, val.dtype), t), n + 1)
            if not tied:
                return val
            col, r = [], 0
            for r0 in sorted(tied):
                col += ([val[r:r0, -128:]] if r0 > r else []) + [tied[r0][0]]
                r = r0 + 8
            col += [val[r:, -128:]] if r < val.shape[0] else []
            return _cat([val[:, :-128], _cat(col, 0)], 1) if val.shape[1] > 128 else _cat(col, 0)

    def strassen(lhs, rhs, side, init=(None, None, None, None)):
        def add(a, b):
            return a if b is None else a + b
        p = [mm(lhs(k), rhs(k), side) for k in range(5)]
        c12 = add(p[2] + p[4], init[1])
        c21 = add(p[1] + p[3], init[2])
        c22 = mm(lhs(5), rhs(5), side, add(p[0] - p[1] + p[2], init[3]))
        c11 = mm(lhs(6), rhs(6), side, add(p[0] + p[3] - p[4], init[0]))
        return c11, c12, c21, c22

    def fmm(sc, lhs, rhs, side, extra=lambda n: None, emit=None):
        val = {}
        for n in sc.order:
            t = extra(n)
            for q, sg in sorted(sc.par[n], key=lambda e: -e[1]):
                t = val[q] if t is None else (t + val[q] if sg > 0 else t - val[q])
            for r in range(sc.rank):
                if sc.wn[r] == n:
                    t = mm(lhs(sc.un[r]), rhs(r), side, t)
            val[n] = t
            if n < sc.nb and emit is not None:
                emit(n, t)
        return [val[v] for v in range(sc.nb)]

    def phase_b(s1_v, s2_v, s3_v, s4_v, h_v, c0_v, l_v, lf_v, n_v, gb_v):
        def w1_load(name, half, c0, c1):
            quad_load(name, w1_hbm, s1_v, RAW1, half, c0, c1)
            quad_load(name, w1_hbm, s1_v, RAW1, 2 + half, c0, c1)

        def block_load(name, w_hbm, s_v, r0, r1):
            kb, nb = s_v.shape[1] // 128 * 128, s_v.shape[2]
            for q in range(16):
                loads.append((name, w_hbm.at[pl.ds((q // 4) * kb + r0, r1 - r0), pl.ds((q % 4) * nb, nb)],
                              s_v.at[SF.raw[q], pl.ds(r0, r1 - r0)]))

        rows_load("x0", 0, TM)
        w1_load("w1a", 0, 0, 256)
        rows_load("x1", TM, 2 * TM)
        w1_load("w1b", 0, 256, 512)
        w1_load("w1cd", 1, 0, 512)
        rows_load("x23", 2 * TM, 4 * TM)
        rows_load("x4567", 4 * TM, S)
        for q in range(4):
            quad_load("w2", w2_hbm, s2_v, RAW, q)
        block_load("w2", w3_hbm, s3_v, 0, W3A)
        block_load("w4", w3_hbm, s3_v, W3A, D4)
        block_load("w4", w4_hbm, s4_v, 0, F4)
        loads.append(("small", mem0_hbm, mem0_ref))
        loads.append(("small", gw_hbm, gw_ref.at[pl.ds(0, NT)]))
        groups.extend(dict.fromkeys(name for name, _, _ in loads))
        assert len(groups) == NLOAD

        start("x0", "w1a", "w1b", "x1", "w1cd", "x23", "x4567", "w2", "w4", "small")

        def zero(k, carry):
            zero_s[k] = 0
            return carry
        lax.fori_loop(0, NZ, zero, 0)

        def prepf_pieces(s_v, lag):
            def piece(rs, cs, st, pin):
                z = 4 * zero_s[st]

                @functools.lru_cache(None)
                def node(n):
                    if n < 16:
                        t = s_v[z + SF.raw[n], rs, cs]
                        return (pin(t) if n in VSTAGES[st][1] else t).astype(f32)
                    a, sa, b, sb = SF.vp[n - 16]
                    return _run([(0, sa, 1, sb)], [node(a), node(b)])[-1]
                rr = [r for k in VSTAGES[st][0] for r in range(7 * k, 7 * k + 7) if SF.raw.count(r) == 0 or SF.vn[r] >= 16]
                vals = [node(SF.vn[r]).astype(bf16) for r in rr]
                for r, t in zip(rr, vals):
                    s_v[z + r, rs, cs] = t
            kb, nb = s_v.shape[1] // 128 * 128, s_v.shape[2]
            out = []
            for r in range(0, kb, 16):
                out += [(slice(rr, rr + 8), slice(c, c + 256)) for c in range(0, nb - 255, 256) for rr in (r, r + 8)]
                out += [(slice(rr, rr + 8), slice(nb - 128, nb)) for rr in (r, r + 8)] if nb % 256 else []
            return [(functools.partial(piece, rs, cs, st), None, s_v if n % TIEP == TIEP - 1 else False, lag,
                     80 if cs.stop - cs.start == 256 else 60)
                    for g in range(0, len(out), 8) for st in range(3) for n, (rs, cs) in enumerate(out[g:g + 8])]

        def prep_pieces(s_v, raw, lag, width=256):
            def piece(r, c, pin):
                idx = (slice(r, r + 8), slice(c, c + width))
                b11, b12, b21, b22 = [_unpack(pin(s_v[(q,) + idx], width) if n in (0, 3) else s_v[(q,) + idx])
                                      for n, q in enumerate(raw)]
                for k, t in ((0, b11 + b22), (2, b12 - b22), (3, b21 - b11), (5, b11 + b12), (6, b21 + b22)):
                    s_v[(k,) + idx] = _pack(t)
            return [(functools.partial(piece, r, c), None, s_v, lag, 80)
                    for c in range(0, s_v.shape[2], width) for r in range(0, s_v.shape[1], 8)]

        def store_l(slot, q, c, quads):
            for k, t in enumerate(_lcombos(*quads)):
                l_v[slot, k, q // 2:q // 2 + 8, c:c + t.shape[1]] = _pack(t)

        def ln_pieces(src, r0, slot, lag, width=256, staged=False, clag=None):
            def stats(q, pin):
                x = pin(src[pl.ds(r0 + q, 16), :].astype(f32))
                xs = [x[:, j * 128:(j + 1) * 128] for j in range(NT)]
                m = functools.reduce(lambda a, b: a + b, xs) * (1.0 / NT)
                w = functools.reduce(lambda a, b: a + b, [(t - m) * (t - m) for t in xs])
                mean = jnp.mean(m, axis=-1, keepdims=True)
                var = jnp.sum(w + NT * ((m - mean) * (m - mean)), axis=-1, keepdims=True) * (1.0 / D)
                n_v[0, q:q + 16, :] = jnp.broadcast_to(mean, (16, 128))
                n_v[1, q:q + 16, :] = jnp.broadcast_to(lax.rsqrt(var + EPS), (16, 128))

            def comb(q, c, pin):
                quads = []
                for rr in (0, HM):
                    rs = pl.ds(pl.multiple_of(r0 + rr + q + zero_s[0], 16), 16)
                    mean, rstd = [jnp.concatenate([n_v[t, rr + q:rr + q + 16, :]] * (width // 128), axis=1)
                                  for t in range(2)]
                    quads += [(src[rs, cc + c:cc + c + width].astype(f32) - mean) * rstd for cc in (0, DH2)]
                store_l(slot, q, c, quads)

            def normf(q, pin):
                mean, rstd = [_cat([n_v[t, q:q + 16, :]] * NT, 1) for t in range(2)]
                c0_v[q:q + 16, :] = (src[pl.ds(pl.multiple_of(r0 + q + zero_s[0], 8), 16), :] - mean) * rstd

            def combf(q, us, pin):
                @functools.lru_cache(None)
                def node(n):
                    if n < SF.nb:
                        return c0_v[(n // 4) * QM + q:(n // 4) * QM + q + 8, (n % 4) * D4:(n % 4 + 1) * D4]
                    a, sa, b, sb = SF.up[n - SF.nb]
                    return _run([(0, sa, 1, sb)], [node(a), node(b)])[-1]
                for u in us:
                    lf_v[SF.ul.index(u), q:q + 8, :] = node(u).astype(bf16)
            dense = slot is not None or src is b_v
            norms = [[(functools.partial(stats, rr + q), None, n_v if dense else False, lag, 90) for rr in (0, HM)]
                     for q in range(0, HM, 16)]
            if slot is None:
                combs = [[(functools.partial(combf, q, us), c0_v, lf_v if dense or us is UPARTS[-1] else False, clag, 55)
                          for us in UPARTS] for q in range(0, QM, 8)]
            else:
                combs = [[(functools.partial(comb, q, c), n_v, l_v, clag, 125) for c in range(0, DH2, width)]
                         for q in range(0, HM, 16)]
            if staged:
                return (sum(norms, []) + [(functools.partial(normf, q), n_v, c0_v, clag, 40) for q in range(0, TM, 16)],
                        sum(combs, []))
            out = list(norms[0])
            for a, b in zip(norms[1:] + [[]], combs):
                out += _merge(a, b) if a else b
            return out

        shifts = (1, 1, -1, -1, 2, 2, -2, -2)

        def shift_pieces(r0, slot, lag, by_value=True):
            def piece(q, j, pin):
                a = [h_v[jj, pl.ds(PAD + r0 + rr + q - shifts[jj], 16), :]
                     for rr in (0, HM) for jj in (j, j + NT // 2)]
                store_l(slot, q, j * 128, [pin(a[0]), a[1], a[2], pin(a[3])])
            return [(functools.partial(piece, q, j), None if by_value else h_v,
                     l_v if j % 2 else False, lag, 50)
                    for q in range(0, HM, 16) for j in range(NT // 2)]

        def lhs_of(slot):
            return lambda k: l_v[slot, k]

        for ref in (xe_v, lf_v, s3_v, s4_v):
            ref[0, 0:16, 0:D4] = jnp.zeros((16, D4), bf16)
        h_v[:, 0:PAD, :] = jnp.zeros((NT, PAD, 128), f32)
        h_v[:, PAD + S:PAD + S + PAD, :] = jnp.zeros((NT, PAD, 128), f32)

        def store_h(r0, c0, h):
            for j in range(h.shape[1] // 128):
                h_v[c0 // 128 + j, PAD + r0:PAD + r0 + h.shape[0], :] = h[:, j * 128:(j + 1) * 128]

        def h_pieces(r0, c0, t, lag, n=4):
            def piece(r, pin):
                store_h(r0 + r, c0, _gelu(pin(t[r:r + 8 * n])))
            return [(functools.partial(piece, r), None, h_v, lag, 10 * n) for r in range(0, t.shape[0], 8 * n)]

        def flush(pieces):
            for p in pieces:
                p[0](lambda v, w=128: v)

        def w1_cols(c, step):
            half, cc = c // DH2, c % DH2
            return jnp.concatenate([s1_v[RAW1[half], :, cc:cc + step], s1_v[RAW1[2 + half], :, cc:cc + step]], axis=0)

        def d1_plain(xn, r0, c0, c1, step):
            for c in range(c0, c1, step):
                store_h(r0, c, _gelu(mm(xn, w1_cols(c, step))))

        def d1_fine(lhs, r0, nrb, cols, pieces, carry, skip=0):
            tiles = [(rb, c) for c in cols for rb in range(nrb)]
            rounds = [tiles[i:i + 4] for i in range(0, len(tiles), 4)]
            for n, (rnd, part) in enumerate(zip(rounds, split(pieces, len(rounds)))):
                sk = skip if n == 0 else 0
                side = Side(_merge(carry, part) if carry else part, 8 - sk, sk)
                carry = []
                for rb, c in rnd:
                    half, cc = c // DH2, c % DH2
                    t = mm(lhs(rb, 0), s1_v[RAW1[half], :, cc:cc + 128], side)
                    t = mm(lhs(rb, 1), s1_v[RAW1[2 + half], :, cc:cc + 128], side, t)
                    carry += h_pieces(r0 + rb * HM, c, t, LS)
            return carry

        def d1_s(b, slot, pieces, carry, early=()):
            for c, part, e in zip(range(0, DH2, NC1), split(pieces, DH2 // NC1), split(early, 2) + [[], []]):
                side = Side(merge(carry, part, e), *((7,) if hist else (5, 2)))
                cs = strassen(lhs_of(slot), lambda k: s1_v[k, :, c:c + NC1], side)
                carry = sum([h_pieces(b * TM + (q // 2) * HM, (q % 2) * DH2 + c, cs[q], LS) for q in (1, 2, 3, 0)], [])
            return carry

        def d2_s(b, slot, pieces, carry=(), early=(), late=()):
            for c, part, e in zip(range(0, DH2, NC1), split(pieces, DH2 // NC1), split(early, 2) + split(late, 2)):
                side = Side(merge(carry, part, e), *((7,) if hist else (5, 2)))
                carry = ()
                idx = [(slice(b * TM + (q // 2) * HM, b * TM + (q // 2 + 1) * HM),
                        slice((q % 2) * DH2 + c, (q % 2) * DH2 + c + NC1)) for q in range(4)]
                cs = strassen(lhs_of(slot), lambda k: s2_v[k, :, c:c + NC1], side,
                              [x_v[i].astype(f32) for i in idx])
                for i, t in zip(idx, cs):
                    b_v[i] = t
                    if b == 0:
                        c0_v[i] = t

        def split(l, n):
            w = [1.0 if hist else 0.6] + [1.0] * (n - 1)
            cut = [int(round(len(l) * sum(w[:i]) / sum(w))) for i in range(n + 1)]
            return [l[cut[i]:cut[i + 1]] for i in range(n)]

        def merge(*ls):
            ls = [l for l in ls if l]
            return _merge(*ls) if ls else []

        NW1, NW3, N30 = 52, 32, 48
        LS, LL = 3, 5

        p3 = prepf_pieces(s3_v, LS)
        n3 = len(p3) * W3A // D4

        @once
        def _phase1a():
            wait("x0")
            xn0 = _pack(_ln(x_v[0:TM, :].astype(f32)))
            wait("w1a")
            d1_plain(xn0, 0, 0, 256, 256)
            wait("x1")
            xn1 = [_pack(_ln(x_v[r:r + HM, :].astype(f32))) for r in (TM, TM + HM)]
            for n in range(2):
                d1_plain(xn1[n], TM + n * HM, 0, 256, 256)
            wait("w1b")
            d1_plain(jnp.concatenate([xn0] + xn1, axis=0), 0, 256, 512, 256)
            wait("w1cd")
            hist.clear()
            xn01 = jnp.concatenate([xn0] + xn1, axis=0)
            l01 = lambda rb, kh: xn01[rb * 64:(rb + 1) * 64, kh * DH2:(kh + 1) * DH2]
            pw = prep_pieces(s1_v, RAW1, LS)
            flush(d1_fine(l01, 0, 4, (512, 640), pw[:NW1], [], 1))
            carry = []
            wait("x23")
            hist.clear()
            carry = d1_fine(l01, 0, 4, (768, 896), ln_pieces(x_v, 2 * TM, 0, LL), carry, 3)
            carry = d1_s(2, 0, ln_pieces(x_v, 3 * TM, 1, LL), carry, pw[NW1:])
            wait("x4567")
            qkv_start(0)
            qkv_start(1)
            hist.clear()
            for b in range(3, NB - 1):
                carry = d1_s(b, b % 2, ln_pieces(x_v, (b + 1) * TM, (b + 1) % 2, LL), carry)
            wait("w2")
            hist.clear()
            pw = prep_pieces(s2_v, RAW, LS)
            carry = d1_s(7, 1, _merge(pw[:NW3], shift_pieces(0, 0, LS, True)), carry)
            d2_s(0, 0, shift_pieces(TM, 1, LS, True), carry, pw[NW3:], p3[:N30])
            pw = split(_merge(p3[N30:n3], sum(ln_pieces(c0_v, 0, None, LL, clag=LS, staged=True), [])), 3)
            for b in range(1, 4):
                d2_s(b, b % 2, _merge(pw[b - 1], shift_pieces((b + 1) * TM, (b + 1) % 2, LS)))
            wait("w4", "small")

        hist.clear()
        pw = p3[n3:] + prepf_pieces(s4_v, LS)
        cut = (0, 93, 192, 291) + (len(pw),)
        for b in range(4, NB):
            d2_s(b, b % 2, merge(pw[cut[b - 4]:cut[b - 3]],
                                 shift_pieces((b + 1) * TM, (b + 1) % 2, LS) if b + 1 < NB else ()))
        start("wo", priority=1)
        gw = gw_ref[0:NT, :].astype(f32)
        gb_v[...] = _cat([jnp.broadcast_to(gw[j:j + 1, :], (8, 128)) for j in range(NT)], 1)

        def ffn(i, carry):
            qkv_wait(i)
            r0 = pl.multiple_of(i * TM, TM)
            rn = pl.multiple_of(jnp.minimum(i + 1, NB - 1) * TM, TM)
            acc = {}
            hist.clear()
            LG = 5

            def relayout(p, r0_, r1_, pin):
                s0 = i * SPG + 2 * p
                e = wqkv_v[s0, r0_:r1_, :]
                o = wqkv_v[s0 + 1, r0_:r1_, :]
                wqkv_v[s0, r0_:r1_, :] = (e & jnp.uint32(0xFFFF)) | (o << 16)
                wqkv_v[s0 + 1, r0_:r1_, :] = (e >> 16) | (o & jnp.uint32(0xFFFF0000))

            relays = [(functools.partial(relayout, p, r, r + 32), wqkv_v, wqkv_v, LG, 35)
                      for p in range(SPG // 2) for r in range(0, D // 2, 32)]
            norms, combs = ln_pieces(b_v, rn, None, 10, staged=True, clag=LG)

            def gate(q, pin):
                x = pin(x_v[pl.ds(r0 + q, 16), :].astype(f32)) * _cat([gb_v[...]] * 2, 0)
                t = functools.reduce(lambda a, b: a + b, [x[:, j * 128:(j + 1) * 128] for j in range(NT)])
                g = jax.nn.sigmoid(jnp.sum(t, axis=-1, keepdims=True))
                g_v[pl.ds(r0 + q, 16), :] = jnp.broadcast_to(g, (16, 128))

            gates = [(functools.partial(gate, q), None, g_v, 10, 90) for q in range(0, TM, 16)]

            def extras(t, us, pin):
                @functools.lru_cache(None)
                def node(n):
                    if n < 16:
                        rs = pl.ds(pl.multiple_of((i + 4 * zero_s[UPARTS.index(us)]) * 64, 64) + (n // 4) * 512 + 24 + 8 * t, 8)
                        x = x_v[rs, (n % 4) * D4:(n % 4 + 1) * D4]
                        return (pin(x) if n in (0, 5, 10, 15) else x).astype(f32)
                    a, sa, b, sb = S49.up[n - 16]
                    return _run([(0, sa, 1, sb)], [node(a), node(b)])[-1]
                for u in us:
                    xe_v[S49.ul.index(u), pl.ds(pl.multiple_of(i * 16, 16) + t * 8, 8), :] = node(u).astype(bf16)

            xes = [(functools.partial(extras, t, us), None, xe_v, LG, 80) for t in range(2) for us in UPARTS]
            hs = {}

            def gelu_pieces(c, cs):
                def piece(r, cc, vs, pin):
                    t = _gelu(pin(_cat([cs[v][r:r + 8, cc:cc + 128] for v in vs], 0)))
                    ts = [t[8 * n:8 * n + 8] for n in range(len(vs))]
                    hs.update({(c, v, r, cc): u for v, u in zip(vs, ts)})
                    return functools.reduce(lambda a, b: a + b, ts)
                return [(functools.partial(piece, r, cc, range(v, v + 4)), None, None, LG, 40) for r in range(0, QM, 8)
                        for cc in range(0, cs[0].shape[1], 128) for v in range(0, SF.nb, 4)]

            def d3(c, side):
                c0, c1 = FCH[c]
                cs = fmm(SF, lambda u: lf_v[SF.ul.index(u), 0:QM], lambda r: s3_v[r, 0:D4, c0:c1], side)
                assert not side.pieces
                return gelu_pieces(c, cs)

            def d4(c, side):
                c0, c1 = FCH[c]
                lh = _run(SF.up, [_cat([_cat([hs.pop((c, v, r, cc)) for r in range(0, QM, 8)], 0)
                                        for cc in range(0, c1 - c0, 128)], 1) for v in range(SF.nb)])
                rhs = lambda r: s4_v[r, c0:c1, :]
                if c + 1 < len(FCH):
                    for n in SF.order:
                        for r in range(SF.rank):
                            if SF.wn[r] == n:
                                acc[n] = mm(lh[SF.un[r]], rhs(r), side, acc.get(n))
                else:
                    idx = lambda v: (pl.ds(r0 + (v // 4) * QM, QM), slice((v % 4) * D4, (v % 4 + 1) * D4))

                    def extra(n):
                        if n >= SF.nb:
                            return acc.get(n)
                        return b_v[idx(n)] + acc[n] if n in acc else b_v[idx(n)]

                    def emit_b(v, t):
                        b_v[idx(v)] = jnp.concatenate([1.0 - g_v[idx(v)[0], :]] * 2, axis=1) * t
                    fmm(SF, lambda u: lh[u], rhs, side, extra, emit_b)
                assert not side.pieces

            g0 = d3(0, Side(relays[:16], 43, 6))
            g1 = d3(1, Side(_merge(g0, gates[:12]), 43, 4))
            d4(0, Side(g1[:22], 41, 8))
            g2 = d3(2, Side(_merge(g1[22:], relays[16:32]), 47))
            d4(1, Side(_merge(g2, relays[32:60]), 43, 4))
            g3 = d3(3, Side(_merge(gates[12:], xes, norms), 49))
            d4(2, Side(_merge(g3, combs), 43, 4))
            d4(3, Side(relays[60:], 44))

            @pl.when(i + 2 < NG)
            def _():
                qkv_start(i + 2)

            return carry

        lax.fori_loop(0, NB, ffn, 0)

    pl.run_scoped(
        phase_b,
        pltpu.VMEM((9, D // 4, D // 2), u32),
        pltpu.VMEM((7, D // 4, D // 2), u32),
        pltpu.VMEM((52, D4 + 16, F4), bf16),
        pltpu.VMEM((52, F4 + 8, D4), bf16),
        pltpu.VMEM((NT, S + 2 * PAD, 128), f32),
        pltpu.VMEM((TM, D), f32),
        pltpu.VMEM((2, 7, HM // 2, D // 2), u32),
        pltpu.VMEM((52, QM + 8, D4), bf16),
        pltpu.VMEM((2, TM, 128), f32),
        pltpu.VMEM((8, D), f32),
    )

    def phase_a(out_v, e_v, oe_v, ke_v, ve_v, o_v):
        def pre(it, carry):
            hist.clear()
            for u in range(3 * NG // NPRE):
                s0 = (it * (3 * NG // NPRE) + u) * G

                @functools.lru_cache(None)
                def node(k, n):
                    if n < 16:
                        return _unpack(wqkv_v[s0 + zero_s[k] + n % 4, (n // 4) * (D // 8):(n // 4 + 1) * (D // 8), :])
                    a, sa, b, sb = S49.vp[n - 16]
                    return _run([(0, sa, 1, sb)], [node(k, a), node(k, b)])[-1]

                def rhs(r):
                    n = S49.vn[r]
                    if n < 16:
                        return wqkv_v[s0 + n % 4, (n // 4) * (D // 8):(n // 4 + 1) * (D // 8), :]
                    return node(r // 7, n).astype(bf16)

                def emit_e(v, t):
                    e_v[(v // 4) * 8:(v // 4 + 1) * 8, s0 + v % 4] = _pack(t).reshape(8, 8, DH)
                fmm(S49N, lambda k: xe_v[S49.ul.index(k), 0:4 * NPAIR], rhs, None, emit=emit_e)
            return carry

        lax.fori_loop(0, NPRE, pre, 0)

        wait("wo")
        mem_v[...] = mem0_ref[...].astype(f32)

        def slab(w, h):
            return (h // G) * SPG + w * G + h % G

        def step(j, hx, odd, late, allow, fill):
            qs, ks, vs, ps = {}, {}, {}, {}
            wload = lambda w, h: pltpu.bitcast(wqkv_v[slab(w, h)], bf16)
            eload = lambda w, h: pltpu.bitcast(e_v[j, slab(w, h)], bf16)

            def proj(g):
                part = {}
                if late and g == 0:
                    for h in range(2):
                        for w in range(3):
                            part[w, h] = _dot(hx[:, :DH2], wload(w, h)[:DH2])
                for h in range(g * G, (g + 1) * G):
                    q, k, v = [(_dot(hx[:, DH2:], wload(w, h)[DH2:]) + part[w, h] if (w, h) in part
                                else _dot(hx, wload(w, h))).astype(bf16) for w in range(3)]
                    if odd:
                        q = jnp.concatenate([q, eload(0, h)], axis=0)
                        k = jnp.concatenate([pltpu.bitcast(ke_v[h], bf16), eload(1, h), k], axis=0)
                        v = jnp.concatenate([pltpu.bitcast(ve_v[h], bf16), eload(2, h), v], axis=0)
                    else:
                        ke_v[h] = pltpu.bitcast(k, u32)
                        ve_v[h] = pltpu.bitcast(v, u32)
                        k = jnp.concatenate([k, eload(1, h)], axis=0)
                        v = jnp.concatenate([v, eload(2, h)], axis=0)
                    qs[h], ks[h], vs[h] = q, k, v

            def score(g):
                for h in range(g * G, (g + 1) * G):
                    s = lax.dot_general(qs.pop(h), ks.pop(h), (((1,), (1,)), ((), ())),
                                        preferred_element_type=f32)
                    ps[h] = _softmax(s, allow, fill)

            def pv(g):
                os_ = []
                for h in range(g * G, (g + 1) * G):
                    o = _dot(ps.pop(h), vs.pop(h))
                    o_v[:, h * 128:(h + 1) * 128] = _pack(o[:32])
                    os_.append(o)
                if odd:
                    quads = [jnp.concatenate([os_[2 * kk][r:r + 8], os_[2 * kk + 1][r:r + 8]], axis=1)
                             for r in (32, 40) for kk in range(2)]
                    for k, t in enumerate(_lcombos(*quads)):
                        oe_v[k, pl.ds(pl.multiple_of(j * 8, 8), 8), g * 256:(g + 1) * 256] = t

            acc = [None] * NT

            def wo(h0, h1, j0, j1):
                o = pltpu.bitcast(o_v[:, h0 * 128:h1 * 128], bf16)
                for n in range(j0, j1):
                    y = _dot(o, pltpu.bitcast(wo_v[n, h0 * 64:h1 * 64, :], bf16))
                    acc[n] = y if acc[n] is None else y + acc[n]

            for t in range(NG):
                proj(t)
                if t >= 2:
                    pv(t - 2)
                if t >= 1:
                    score(t - 1)
            wo(0, 16, 0, 4)
            pv(NG - 2)
            score(NG - 1)
            wo(0, 16, 4, 8)
            pv(NG - 1)
            wo(16, 24, 0, 8)
            wo(24, 32, 0, 8)
            return jnp.concatenate(acc, axis=1)

        def emit(j, r0, o0, a):
            rs = pl.ds(r0 + o0, 24)
            g = jnp.concatenate([g_v[rs, :]] * NT, axis=1)
            out_v[j, o0:o0 + 24, :] = (g * a + b_v[rs, :]).astype(bf16)

        def pair(j, mem, late):
            r0 = pl.multiple_of(j * 64, 64)
            allow_e, fill_e, allow_o, fill_o = _masks()
            xa = x_v[pl.ds(r0 + 16, 8), :].astype(f32)
            xb = x_v[pl.ds(r0 + 40, 8), :].astype(f32)
            hx = jnp.concatenate([x_v[pl.ds(r0, 16), :], jnp.concatenate([xa, mem], 0).astype(bf16)], 0)
            oe = step(j, hx, False, late, allow_e, fill_e)
            emit(j, r0, 0, oe[:24])
            hx = jnp.concatenate([jnp.concatenate([oe[24:32], xb], 0).astype(bf16), x_v[pl.ds(r0 + 48, 16), :]], 0)
            oo = step(j, hx, True, True, allow_o, fill_o)
            emit(j, r0, 40, oo[8:])
            return oo[:8]

        def a_iter(it, carry):
            mem = mem_v[...]
            for t in range(PPI):
                mem = pair(it * PPI + t, mem, t > 0)
            mem_v[...] = mem
            for t in range(PPI):
                for o0 in (0, 40):
                    idx = (it * PPI + t, pl.ds(o0, 24))
                    pltpu.make_async_copy(out_v.at[idx], out_hbm.at[idx], sem_out).start()
            return carry

        lax.fori_loop(0, NPAIR // PPI, a_iter, 0)

        @once
        def _post():
            hist.clear()
            NK, NW = 2, 128
            for n in range(D // (4 * NW)):
                @functools.lru_cache(None)
                def node(k, kc, q):
                    if q < 16:
                        return _unpack(raw(kc, q, 4 * zero_s[k]))
                    a, sa, b, sb = S49.vp[q - 16]
                    return _run([(0, sa, 1, sb)], [node(k, kc, a), node(k, kc, b)])[-1]

                def raw(kc, q, z=0):
                    return _cat([_cat([wo_v[z + (4 * n + q % 4) * (NW // 128) + c, (4 * g + q // 4) * 64:(4 * g + q // 4 + 1) * 64, :]
                                       for c in range(NW // 128)], 1)
                                 for g in range(kc * NG // NK, (kc + 1) * NG // NK)], 0)

                def prod(r, kc, acc):
                    z = zero_s[7 + r % 7]
                    quad = [_cat([oe_v[z + r // 7, (q // 2) * 128:(q // 2 + 1) * 128, (2 * g + q % 2) * 128:(2 * g + q % 2 + 1) * 128]
                                  for g in range(kc * NG // NK, (kc + 1) * NG // NK)], 1) if q in UQ[r % 7] else None
                            for q in range(4)]
                    f = UFORMS[r % 7]
                    lhs = quad[f[0]] if len(f) == 1 else _run([(0, f[1], 1, f[3])], [quad[f[0]], quad[f[2]]])[-1]
                    q = S49.vn[r]
                    return mm(lhs, raw(kc, q) if q < 16 else node(r // 7, kc, q).astype(bf16), None, acc)

                val, part = {}, {}
                for nd in S49N.order:
                    rs = [r for r in range(49) if S49.wn[r] == nd]
                    for r in rs:
                        if r not in part:
                            for kc in range(NK - 1):
                                for k2 in SEQ:
                                    part[r // 7 * 7 + k2] = prod(r // 7 * 7 + k2, kc, part.get(r // 7 * 7 + k2))
                    t = part[rs[0]] if rs else None
                    for q, sg in sorted(S49.par[nd], key=lambda e: -e[1]):
                        t = val[q] if t is None else (t + val[q] if sg > 0 else t - val[q])
                    if rs:
                        t = prod(rs[0], NK - 1, t)
                    val[nd] = t
                    if nd < 16:
                        o0, j0 = 24 + (nd // 8) * 8, (nd // 4 % 2) * 16
                        c0 = (4 * n + nd % 4) * NW
                        for jj in range(16):
                            rr = slice((j0 + jj) * 64 + o0, (j0 + jj) * 64 + o0 + 8)
                            out_v[j0 + jj, o0:o0 + 8, c0:c0 + NW] = (
                                _cat([g_v[rr, :]] * (NW // 128), 1) * t[jj * 8:jj * 8 + 8] + b_v[rr, c0:c0 + NW]).astype(bf16)
                        idx = (pl.ds(j0, 16), pl.ds(o0, 8), pl.ds(c0, NW))
                        pltpu.make_async_copy(out_v.at[idx], out_hbm.at[idx], sem_out).start()

        pltpu.make_async_copy(out_v, out_hbm, sem_out).wait()

    pl.run_scoped(
        phase_a,
        pltpu.VMEM((NPAIR, 64, D), bf16),
        pltpu.VMEM((NPAIR, 3 * H, 8, DH), u32),
        pltpu.VMEM((7, 8 * NPAIR, H * DH // 2), f32),
        pltpu.VMEM((H, 16, 128), u32),
        pltpu.VMEM((H, 16, 128), u32),
        pltpu.VMEM((16, H * DH), u32),
    )


@jax.jit
def pallas_gated_mix__memory_aug_recurrent_mem_tr__mixer_s_mlp__prompt_kernel(
    A_x, A_mem0, A_Wq, A_Wk, A_Wv, A_Wo, A_seg_len, B_x, B_w1, B_w2, B_w3, B_w4, gate_w,
):
    assert A_x.shape == (1, S, D) and A_mem0.shape == (1, M, D)
    any_spec = pl.BlockSpec(memory_space=pl.ANY)
    out = pl.pallas_call(
        _kernel,
        out_shape=jax.ShapeDtypeStruct((NPAIR, 64, D), bf16),
        in_specs=[any_spec] * 11,
        out_specs=any_spec,
        scratch_shapes=[
            pltpu.VMEM((S, D), bf16),
            pltpu.VMEM((3 * H, D // 2, DH), u32),
            pltpu.VMEM((NT, H * DH // 2 + 8, 128), u32),
            pltpu.VMEM((S, D), f32),
            pltpu.VMEM((S, 128), f32),
            pltpu.VMEM((52, 4 * NPAIR + 8, D4), bf16),
            pltpu.VMEM((M, D), f32),
            pltpu.VMEM((M, D), bf16),
            pltpu.VMEM((64, 128), bf16),
            pltpu.SMEM((NZ,), jnp.int32),
            pltpu.SemaphoreType.DMA((NLOAD,)),
            pltpu.SemaphoreType.DMA((NG,)),
            pltpu.SemaphoreType.DMA,
        ],
        compiler_params=pltpu.CompilerParams(vmem_limit_bytes=127 * 1024 * 1024,
                                             disable_bounds_checks=True),
    )(
        A_x.reshape(S, D), A_mem0.reshape(M, D),
        A_Wq.reshape(D // 2, 2 * H, DH), A_Wk.reshape(D // 2, 2 * H, DH), A_Wv.reshape(D // 2, 2 * H, DH),
        A_Wo.reshape(H * DH, D), B_w1, B_w2, B_w3, B_w4, gate_w.reshape(NT, 128),
    )
    return out.reshape(1, S, D)
```

```python
import functools

import jax
import jax.numpy as jnp
from jax import lax
import jax.experimental.pallas as pl
import jax.experimental.pallas.tpu as pltpu

f32, bf16, u32 = jnp.float32, jnp.bfloat16, jnp.uint32

S, D, H, DH, M, SEG, F = 2048, 1024, 32, 128, 8, 32, 3584
SCALE = DH ** -0.5
NEG = -1000000000.0
EPS = 1e-05

TM = 256
NB = S // TM
HM = TM // 2
DH2 = D // 2
D4, F4 = D // 4, F // 4
FCH = ((0, 128), (128, 384), (384, 640), (640, 896))
NC1 = 128
NPAIR = S // (2 * SEG)
PPI = 2
NPRE = 3
G = 4
NG = H // G
PAD = 8
NT = D // 128
TIEP = 2
W3A = 208
NZ = 16
NLOAD = 11
assert NB == NG

_dot = functools.partial(jnp.dot, preferred_element_type=f32)

def _run(prog, blocks):
    vals = list(blocks)
    for a, sa, b, sb in prog:
        vals.append(vals[a] + vals[b] if sa > 0 and sb > 0 else
                    vals[a] - vals[b] if sa > 0 else vals[b] - vals[a])
    return vals


def _form(f, get):
    return get(f[0]) if len(f) == 1 else get(f[0]) + get(f[2]) if f[3] > 0 else get(f[0]) - get(f[2])


def _terms(prog, nin, node):
    if node < nin:
        return {node: 1}
    a, sa, b, sb = prog[node - nin]
    out = {k: sa * v for k, v in _terms(prog, nin, a).items()}
    out.update({k: sb * v for k, v in _terms(prog, nin, b).items()})
    return out


class _Scheme:
    def __init__(self, ms, up, vp, wp, un, vn, wn):
        self.ms, self.nb, self.rank = ms, 4 * ms, len(un)
        self.up, self.vp, self.wp, self.un, self.vn, self.wn = up, vp, wp, un, vn, wn
        self.ul = tuple(sorted(set(un)))
        t = {}
        for r in range(self.rank):
            for a, ca in _terms(up, self.nb, un[r]).items():
                for b, cb in _terms(vp, 16, vn[r]).items():
                    for c, cc in _terms(wp, self.nb, wn[r]).items():
                        t[a, b, c] = t.get((a, b, c), 0) + ca * cb * cc
        assert {k: v for k, v in t.items() if v} == {
            (4 * i + j, 4 * j + l, 4 * i + l): 1 for i in range(ms) for j in range(4) for l in range(4)}
        self.par = {n: [] for n in range(self.nb + len(wp))}
        for k, (a, sa, b, sb) in enumerate(wp):
            self.par[a].append((self.nb + k, sa))
            self.par[b].append((self.nb + k, sb))
        self.order = order = []

        def closure(n, acc):
            if n not in acc and n not in order:
                acc.add(n)
                for q, _ in self.par[n]:
                    closure(q, acc)
            return acc

        def visit(n):
            if n not in order:
                for q, _ in self.par[n]:
                    visit(q)
                order.append(n)
        while len([v for v in range(self.nb) if v not in order]):
            visit(min((v for v in range(self.nb) if v not in order), key=lambda v: len(closure(v, set()))))


def _twice(forms):
    prog, nodes = [], []

    def apply(f, quad):
        if len(f) == 1:
            return quad[f[0]]
        prog.append((quad[f[0]], f[1], quad[f[2]], f[3]))
        return 15 + len(prog)
    for f1 in forms:
        inner = [apply(f1, [4 * (2 * (q // 2) + p // 2) + 2 * (q % 2) + p % 2 for q in range(4)]) for p in range(4)]
        nodes += [apply(f2, inner) for f2 in forms]
    return tuple(prog), tuple(nodes)


UFORMS = ((0, 1, 3, 1), (2, 1, 3, 1), (0,), (3,), (0, 1, 1, 1), (2, 1, 0, -1), (1, 1, 3, -1))
UQ = [f[::2] for f in UFORMS]
SEQ = (1, 3, 4, 2, 0, 5, 6)
_U2 = _twice(UFORMS)
VFORMS = ((0, 1, 3, 1), (0,), (1, 1, 3, -1), (2, 1, 0, -1), (3,), (0, 1, 1, 1), (2, 1, 3, 1))
_V2 = _twice(VFORMS)
_W2 = _twice(((0, 1, 3, 1), (2, 1, 3, -1), (1, 1, 3, 1), (0, 1, 2, 1), (1, 1, 0, -1), (3,), (0,)))
S49 = _Scheme(4, _U2[0], _V2[0], _W2[0], _U2[1], _V2[1], _W2[1])
VSTAGES = (((2, 5), (1,)), ((3, 6), (2,)), ((0, 1, 4), (0, 3)))
S49.raw = tuple(7 * (1, 2, 3, 4)[2 * (q // 8) + q % 4 // 2] + (1, 2, 3, 4)[2 * (q // 4 % 2) + q % 2] for q in range(16))
assert all(S49.raw[S49.vn[r]] == r for r in range(49) if S49.vn[r] < 16)


def _outer_major(n):
    rs = [7 * SEQ.index(r // 7) + SEQ.index(r % 7) for r in range(49) if S49.wn[r] == n]
    return max(rs + [-1] + [_outer_major(q) + 0.01 for q, _ in S49.par[n]])


S49N = _Scheme(4, _U2[0], _V2[0], _W2[0], _U2[1], _V2[1], _W2[1])
S49N.order.sort(key=_outer_major)
UPARTS = [[S49.un[r] for k in ks for r in range(7 * k, 7 * k + 7)] for ks in ((0, 2, 3), (4, 6), (1, 5))]
SF = S49
QM = TM // SF.ms


def _ln(x):
    m = jnp.mean(x, axis=-1, keepdims=True)
    xc = x - m
    v = jnp.mean(xc * xc, axis=-1, keepdims=True)
    return xc * lax.rsqrt(v + EPS)


_GC = 0.7978845608028654


def _gelu(x):
    h = 0.5 * x
    return h + h * jnp.tanh(x * (_GC + (_GC * 0.044715) * (x * x)))


def _unpack(u):
    return pltpu.bitcast(u, bf16).astype(f32)


def _pack(x):
    return pltpu.bitcast(x.astype(bf16), u32)


def _cat(xs, axis):
    xs = [x for x in xs if x.shape[axis]]
    return xs[0] if len(xs) == 1 else jnp.concatenate(xs, axis=axis)


def _as(x, dtype):
    return x if x.dtype == dtype else pltpu.bitcast(x, dtype)


def _lcombos(a11, a12, a21, a22):
    return [a11 + a22, a21 + a22, a11, a22, a11 + a12, a21 - a11, a12 - a22]


def _merge(*lists):
    keyed = [((j + 0.5) / len(l), n, j, v) for n, l in enumerate(lists) for j, v in enumerate(l)]
    return [v for _, _, _, v in sorted(keyed, key=lambda t: t[:3])]


def _masks():
    r = lax.broadcasted_iota(jnp.int32, (32, 48), 0)
    c = lax.broadcasted_iota(jnp.int32, (32, 48), 1)
    exist_e = c < 40
    allow_e = exist_e & ((r >= 24) | ((c >= 24) & (c < 32)) | (c <= r))
    fill_e = jnp.where(exist_e, NEG, -jnp.inf).astype(f32)
    r = lax.broadcasted_iota(jnp.int32, (48, 80), 0)
    c = lax.broadcasted_iota(jnp.int32, (48, 80), 1)
    q_even = (r >= 32) & (r < 40)
    exist_o = (q_even & (c < 40)) | (~q_even & (c >= 40))
    ktok = jnp.where(c < 24, c, jnp.where(c < 48, c - 8, c - 16))
    qtok = jnp.where(r < 32, r + 32, r - 8)
    is_mem_key = ((c >= 24) & (c < 32)) | ((c >= 48) & (c < 56))
    allow_o = exist_o & (is_mem_key | (r < 8) | (ktok <= qtok))
    fill_o = jnp.where(exist_o, NEG, -jnp.inf).astype(f32)
    return allow_e, fill_e, allow_o, fill_o


def _softmax(s, allow, fill):
    s = jnp.where(allow, s * SCALE, fill)
    m = jnp.max(s, axis=-1, keepdims=True)
    e = jnp.exp(s - m)
    l = jnp.sum(e, axis=-1, keepdims=True)
    r = pl.reciprocal(l, approx=True)
    r = r * (2.0 - l * r)
    return (e * r).astype(bf16)


def _kernel(x_hbm, mem0_hbm, wq_hbm, wk_hbm, wv_hbm, wo_hbm, w1_hbm, w2_hbm, w3_hbm, w4_hbm,
            gw_hbm, out_hbm,
            x_v, wqkv_v, wo_v, b_v, g_v, xe_v, mem_v, mem0_ref, gw_ref, zero_s,
            sem, sem_qkv, sem_out):
    RAW = (1, 2, 3, 4)
    RAW1 = (1, 7, 8, 4)

    loads = []

    def rows_load(name, r0, r1):
        loads.append((name, x_hbm.at[pl.ds(r0, r1 - r0)], x_v.at[pl.ds(r0, r1 - r0)]))

    def quad_load(name, w_hbm, s_v, raw, q, c0=0, c1=None):
        k4, n2 = s_v.shape[1], s_v.shape[2]
        c1 = n2 if c1 is None else c1
        src = w_hbm.bitcast(u32).at[pl.ds((q // 2) * k4, k4), pl.ds((q % 2) * n2 + c0, c1 - c0)]
        loads.append((name, src, s_v.at[raw[q], :, pl.ds(c0, c1 - c0)]))

    for j in range(NT):
        loads.append(("wo", wo_hbm.bitcast(u32).at[:, pl.ds(j * 128, 128)], wo_v.at[j, pl.ds(0, H * DH // 2)]))
    groups = []

    def start(*names, priority=0):
        for name, src, dst in loads:
            if name in names:
                pltpu.make_async_copy(src, dst, sem.at[groups.index(name)]).start(priority=priority)

    def wait(*names):
        for name, src, dst in loads:
            if name in names:
                pltpu.make_async_copy(src, dst, sem.at[groups.index(name)]).wait()

    SPG = 3 * G

    def qkv_start(g):
        for w, w_hbm in enumerate((wq_hbm, wk_hbm, wv_hbm)):
            wu = w_hbm.bitcast(u32)
            for k in range(G // 2):
                for par in range(2):
                    pltpu.make_async_copy(
                        wu.at[:, par * (H // 2) + g * (G // 2) + k, :],
                        wqkv_v.at[g * SPG + w * G + 2 * k + par], sem_qkv.at[g]).start(priority=1)

    def qkv_wait(g):
        grp = wqkv_v.at[pl.ds(g * SPG, SPG)]
        pltpu.make_async_copy(grp, grp, sem_qkv.at[g]).wait()

    def once(fn):
        def body(_, carry):
            fn()
            return carry
        lax.fori_loop(0, 1 + zero_s[1], body, 0)

    def tile_idx(ref, cols=128):
        z = zero_s[0]
        n = 16 if ref.dtype == bf16 and cols == 128 else 8
        return (z,) * (len(ref.shape) - 2) + (pl.ds(pl.multiple_of(z, n), n), slice(0, cols))

    hist = []

    def mm(lhs, rhs, side=None, acc=None):
        if side is not None:
            lhs = side(lhs)
        lhs = pltpu.bitcast(lhs, bf16) if lhs.dtype == u32 else lhs.astype(bf16)
        y = _dot(lhs, pltpu.bitcast(rhs, bf16) if rhs.dtype == u32 else rhs)
        if acc is not None:
            y = y + acc
        hist.append(y)
        return y

    class Side:
        def __init__(self, pieces, n, skip=0):
            cap = [0] * skip + [1] * n
            tot = sum(p[4] for p in pieces)
            self.plan = [[] for _ in cap]
            done = 0
            for p in pieces:
                done += p[4]
                x, d = done / tot * sum(cap), 0
                while x > cap[d] + 1e-9:
                    x -= cap[d]
                    d += 1
                self.plan[d].append((p, x / cap[d]))
            self.pieces = len(pieces)

        def __call__(self, val):
            todo = self.plan.pop(0) if self.plan else []
            if not todo:
                return val
            self.pieces -= len(todo)
            never = zero_s[0] > 0
            if val.dtype == bf16:
                val = pltpu.bitcast(val, u32)
            rg = 8 if val.dtype == u32 else 16
            ng = val.shape[0] // rg
            tied = {}
            for (fn, rd, wr, lag, _), pos in todo:
                m = min(max(-int(-pos * ng // 1) - 1, 0), ng - 1)
                pin = lambda v, w=128: v
                if lag is not None and len(hist) >= lag:
                    r0 = (16 * m) % hist[-lag].shape[0]
                    a = hist[-lag][r0:r0 + 8, :128]
                    if rd is None:
                        def pin(v, w=128, a=a):
                            if v.dtype == bf16:
                                a = _cat([a] * (v.shape[-1] // 128), 1).astype(bf16)
                                return lax.select(never, a.reshape(v.shape), v)
                            a = _cat([_cat([_as(a, v.dtype)] * (v.shape[0] // 8), 0)] * (w // 128), 1)
                            if v.shape[1] == w:
                                return lax.select(never, a, v)
                            return _cat([lax.select(never, a, v[:, :w]), v[:, w:]], 1)
                    elif rd.dtype == bf16:
                        idx = tile_idx(rd, 256)
                        rd[idx] = lax.select(never, _cat([a, a], 1).astype(bf16), rd[idx])
                    else:
                        idx = tile_idx(rd)
                        rd[idx] = lax.select(never, _as(a, rd.dtype), rd[idx])
                u = fn(pin)
                if wr is False:
                    continue
                if wr is not None:
                    u = wr[tile_idx(wr)]
                t, n = tied.get(m * rg) or (val[m * rg:m * rg + 8, -128:], 0)
                tied[m * rg] = (lax.select(zero_s[n] > 0, _as(u, val.dtype), t), n + 1)
            if not tied:
                return val
            col, r = [], 0
            for r0 in sorted(tied):
                col += ([val[r:r0, -128:]] if r0 > r else []) + [tied[r0][0]]
                r = r0 + 8
            col += [val[r:, -128:]] if r < val.shape[0] else []
            return _cat([val[:, :-128], _cat(col, 0)], 1) if val.shape[1] > 128 else _cat(col, 0)

    def strassen(lhs, rhs, side, init=(None, None, None, None)):
        def add(a, b):
            return a if b is None else a + b
        p = [mm(lhs(k), rhs(k), side) for k in range(5)]
        c12 = add(p[2] + p[4], init[1])
        c21 = add(p[1] + p[3], init[2])
        c22 = mm(lhs(5), rhs(5), side, add(p[0] - p[1] + p[2], init[3]))
        c11 = mm(lhs(6), rhs(6), side, add(p[0] + p[3] - p[4], init[0]))
        return c11, c12, c21, c22

    def fmm(sc, lhs, rhs, side, extra=lambda n: None, emit=None):
        val = {}
        for n in sc.order:
            t = extra(n)
            for q, sg in sorted(sc.par[n], key=lambda e: -e[1]):
                t = val[q] if t is None else (t + val[q] if sg > 0 else t - val[q])
            for r in range(sc.rank):
                if sc.wn[r] == n:
                    t = mm(lhs(sc.un[r]), rhs(r), side, t)
            val[n] = t
            if n < sc.nb and emit is not None:
                emit(n, t)
        return [val[v] for v in range(sc.nb)]

    def phase_b(s1_v, s2_v, s3_v, s4_v, h_v, c0_v, l_v, lf_v, n_v, gb_v):
        def w1_load(name, half, c0, c1):
            quad_load(name, w1_hbm, s1_v, RAW1, half, c0, c1)
            quad_load(name, w1_hbm, s1_v, RAW1, 2 + half, c0, c1)

        def block_load(name, w_hbm, s_v, r0, r1):
            kb, nb = s_v.shape[1] // 128 * 128, s_v.shape[2]
            for q in range(16):
                loads.append((name, w_hbm.at[pl.ds((q // 4) * kb + r0, r1 - r0), pl.ds((q % 4) * nb, nb)],
                              s_v.at[SF.raw[q], pl.ds(r0, r1 - r0)]))

        rows_load("x0", 0, TM)
        w1_load("w1a", 0, 0, 256)
        rows_load("x1", TM, 2 * TM)
        w1_load("w1b", 0, 256, 512)
        w1_load("w1cd", 1, 0, 512)
        rows_load("x23", 2 * TM, 4 * TM)
        rows_load("x4567", 4 * TM, S)
        for q in range(4):
            quad_load("w2", w2_hbm, s2_v, RAW, q)
        block_load("w2", w3_hbm, s3_v, 0, W3A)
        block_load("w4", w3_hbm, s3_v, W3A, D4)
        block_load("w4", w4_hbm, s4_v, 0, F4)
        loads.append(("small", mem0_hbm, mem0_ref))
        loads.append(("small", gw_hbm, gw_ref.at[pl.ds(0, NT)]))
        groups.extend(dict.fromkeys(name for name, _, _ in loads))
        assert len(groups) == NLOAD

        start("x0", "w1a", "w1b", "x1", "w1cd", "x23", "x4567", "w2", "w4", "small")

        def zero(k, carry):
            zero_s[k] = 0
            return carry
        lax.fori_loop(0, NZ, zero, 0)

        def prepf_pieces(s_v, lag):
            def piece(rs, cs, st, pin):
                z = 4 * zero_s[st]

                @functools.lru_cache(None)
                def quad(q):
                    t = s_v[pl.ds(z + 7 * q + 8, 4), rs, cs]
                    if q in VSTAGES[st][1]:
                        t = _cat([pin(t[0:1]), t[1:3], pin(t[3:4])], 0)
                    return t.astype(f32)
                done = []
                for k in VSTAGES[st][0]:
                    t = _form(VFORMS[k], quad)
                    t = [t[q:q + 1] for q in range(4)]
                    ts = [_form(f, lambda q: t[q]) for f in VFORMS]
                    for a, b in ((0, 7),) if len(VFORMS[k]) > 1 else ((0, 1), (2, 4), (5, 7)):
                        done.append((7 * k + a, _cat(ts[a:b], 0).astype(bf16)))
                for r, t in done:
                    s_v[pl.ds(z + r, t.shape[0]), rs, cs] = t
            kb, nb = s_v.shape[1] // 128 * 128, s_v.shape[2]
            out = []
            for r in range(0, kb, 16):
                out += [(slice(rr, rr + 8), slice(c, c + 256)) for c in range(0, nb - 255, 256) for rr in (r, r + 8)]
                out += [(slice(rr, rr + 8), slice(nb - 128, nb)) for rr in (r, r + 8)] if nb % 256 else []
            return [(functools.partial(piece, rs, cs, st), None, s_v if n % TIEP == TIEP - 1 else False, lag,
                     80 if cs.stop - cs.start == 256 else 60)
                    for g in range(0, len(out), 8) for st in range(3) for n, (rs, cs) in enumerate(out[g:g + 8])]

        def prep_pieces(s_v, raw, lag, width=256):
            def piece(r, c, pin):
                idx = (slice(r, r + 8), slice(c, c + width))
                b11, b12, b21, b22 = [_unpack(pin(s_v[(q,) + idx], width) if n in (0, 3) else s_v[(q,) + idx])
                                      for n, q in enumerate(raw)]
                for k, t in ((0, b11 + b22), (2, b12 - b22), (3, b21 - b11), (5, b11 + b12), (6, b21 + b22)):
                    s_v[(k,) + idx] = _pack(t)
            return [(functools.partial(piece, r, c), None, s_v, lag, 80)
                    for c in range(0, s_v.shape[2], width) for r in range(0, s_v.shape[1], 8)]

        def store_l(slot, q, c, quads):
            for k, t in enumerate(_lcombos(*quads)):
                l_v[slot, k, q // 2:q // 2 + 8, c:c + t.shape[1]] = _pack(t)

        def ln_pieces(src, r0, slot, lag, width=256, staged=False, clag=None):
            def stats(q, pin):
                x = pin(src[pl.ds(r0 + q, 16), :].astype(f32))
                xs = [x[:, j * 128:(j + 1) * 128] for j in range(NT)]
                m = functools.reduce(lambda a, b: a + b, xs) * (1.0 / NT)
                w = functools.reduce(lambda a, b: a + b, [(t - m) * (t - m) for t in xs])
                mean = jnp.mean(m, axis=-1, keepdims=True)
                var = jnp.sum(w + NT * ((m - mean) * (m - mean)), axis=-1, keepdims=True) * (1.0 / D)
                n_v[0, q:q + 16, :] = jnp.broadcast_to(mean, (16, 128))
                n_v[1, q:q + 16, :] = jnp.broadcast_to(lax.rsqrt(var + EPS), (16, 128))

            def comb(q, c, pin):
                quads = []
                for rr in (0, HM):
                    rs = pl.ds(pl.multiple_of(r0 + rr + q + zero_s[0], 16), 16)
                    mean, rstd = [jnp.concatenate([n_v[t, rr + q:rr + q + 16, :]] * (width // 128), axis=1)
                                  for t in range(2)]
                    quads += [(src[rs, cc + c:cc + c + width].astype(f32) - mean) * rstd for cc in (0, DH2)]
                store_l(slot, q, c, quads)

            def normf(q, pin):
                mean, rstd = [_cat([n_v[t, q:q + 16, :]] * NT, 1) for t in range(2)]
                c0_v[q:q + 16, :] = (src[pl.ds(pl.multiple_of(r0 + q + zero_s[0], 8), 16), :] - mean) * rstd

            def combf(q, us, pin):
                @functools.lru_cache(None)
                def node(n):
                    if n < SF.nb:
                        return c0_v[(n // 4) * QM + q:(n // 4) * QM + q + 8, (n % 4) * D4:(n % 4 + 1) * D4]
                    a, sa, b, sb = SF.up[n - SF.nb]
                    return _run([(0, sa, 1, sb)], [node(a), node(b)])[-1]
                for u in us:
                    lf_v[SF.ul.index(u), q:q + 8, :] = node(u).astype(bf16)
            dense = slot is not None or src is b_v
            norms = [[(functools.partial(stats, rr + q), None, n_v if dense else False, lag, 90) for rr in (0, HM)]
                     for q in range(0, HM, 16)]
            if slot is None:
                combs = [[(functools.partial(combf, q, us), c0_v, lf_v if dense or us is UPARTS[-1] else False, clag, 55)
                          for us in UPARTS] for q in range(0, QM, 8)]
            else:
                combs = [[(functools.partial(comb, q, c), n_v, l_v, clag, 125) for c in range(0, DH2, width)]
                         for q in range(0, HM, 16)]
            if staged:
                return (sum(norms, []) + [(functools.partial(normf, q), n_v, c0_v, clag, 40) for q in range(0, TM, 16)],
                        sum(combs, []))
            out = list(norms[0])
            for a, b in zip(norms[1:] + [[]], combs):
                out += _merge(a, b) if a else b
            return out

        shifts = (1, 1, -1, -1, 2, 2, -2, -2)

        def shift_pieces(r0, slot, lag, by_value=True):
            def piece(q, j, pin):
                a = [h_v[jj, pl.ds(PAD + r0 + rr + q - shifts[jj], 16), :]
                     for rr in (0, HM) for jj in (j, j + NT // 2)]
                store_l(slot, q, j * 128, [pin(a[0]), a[1], a[2], pin(a[3])])
            return [(functools.partial(piece, q, j), None if by_value else h_v,
                     l_v if j % 2 else False, lag, 50)
                    for q in range(0, HM, 16) for j in range(NT // 2)]

        def lhs_of(slot):
            return lambda k: l_v[slot, k]

        for ref in (xe_v, lf_v, s3_v, s4_v):
            ref[0, 0:16, 0:D4] = jnp.zeros((16, D4), bf16)
        h_v[:, 0:PAD, :] = jnp.zeros((NT, PAD, 128), f32)
        h_v[:, PAD + S:PAD + S + PAD, :] = jnp.zeros((NT, PAD, 128), f32)

        def store_h(r0, c0, h):
            for j in range(h.shape[1] // 128):
                h_v[c0 // 128 + j, PAD + r0:PAD + r0 + h.shape[0], :] = h[:, j * 128:(j + 1) * 128]

        def h_pieces(r0, c0, t, lag, n=4):
            def piece(r, pin):
                store_h(r0 + r, c0, _gelu(pin(t[r:r + 8 * n])))
            return [(functools.partial(piece, r), None, h_v, lag, 10 * n) for r in range(0, t.shape[0], 8 * n)]

        def flush(pieces):
            for p in pieces:
                p[0](lambda v, w=128: v)

        def w1_cols(c, step):
            half, cc = c // DH2, c % DH2
            return jnp.concatenate([s1_v[RAW1[half], :, cc:cc + step], s1_v[RAW1[2 + half], :, cc:cc + step]], axis=0)

        def d1_plain(xn, r0, c0, c1, step):
            for c in range(c0, c1, step):
                store_h(r0, c, _gelu(mm(xn, w1_cols(c, step))))

        def d1_fine(lhs, r0, nrb, cols, pieces, carry, skip=0):
            tiles = [(rb, c) for c in cols for rb in range(nrb)]
            rounds = [tiles[i:i + 4] for i in range(0, len(tiles), 4)]
            for n, (rnd, part) in enumerate(zip(rounds, split(pieces, len(rounds)))):
                sk = skip if n == 0 else 0
                side = Side(_merge(carry, part) if carry else part, 8 - sk, sk)
                carry = []
                for rb, c in rnd:
                    half, cc = c // DH2, c % DH2
                    t = mm(lhs(rb, 0), s1_v[RAW1[half], :, cc:cc + 128], side)
                    t = mm(lhs(rb, 1), s1_v[RAW1[2 + half], :, cc:cc + 128], side, t)
                    carry += h_pieces(r0 + rb * HM, c, t, LS)
            return carry

        def d1_s(b, slot, pieces, carry, early=()):
            for c, part, e in zip(range(0, DH2, NC1), split(pieces, DH2 // NC1), split(early, 2) + [[], []]):
                side = Side(merge(carry, part, e), *((7,) if hist else (5, 2)))
                cs = strassen(lhs_of(slot), lambda k: s1_v[k, :, c:c + NC1], side)
                carry = sum([h_pieces(b * TM + (q // 2) * HM, (q % 2) * DH2 + c, cs[q], LS) for q in (1, 2, 3, 0)], [])
            return carry

        def d2_s(b, slot, pieces, carry=(), early=(), late=()):
            for c, part, e in zip(range(0, DH2, NC1), split(pieces, DH2 // NC1), split(early, 2) + split(late, 2)):
                side = Side(merge(carry, part, e), *((7,) if hist else (5, 2)))
                carry = ()
                idx = [(slice(b * TM + (q // 2) * HM, b * TM + (q // 2 + 1) * HM),
                        slice((q % 2) * DH2 + c, (q % 2) * DH2 + c + NC1)) for q in range(4)]
                cs = strassen(lhs_of(slot), lambda k: s2_v[k, :, c:c + NC1], side,
                              [x_v[i].astype(f32) for i in idx])
                for i, t in zip(idx, cs):
                    b_v[i] = t
                    if b == 0:
                        c0_v[i] = t

        def split(l, n):
            w = [1.0 if hist else 0.6] + [1.0] * (n - 1)
            cut = [int(round(len(l) * sum(w[:i]) / sum(w))) for i in range(n + 1)]
            return [l[cut[i]:cut[i + 1]] for i in range(n)]

        def merge(*ls):
            ls = [l for l in ls if l]
            return _merge(*ls) if ls else []

        NW1, NW3, N30 = 52, 32, 48
        LS, LL = 3, 5

        p3 = prepf_pieces(s3_v, LS)
        n3 = len(p3) * W3A // D4

        @once
        def _phase1a():
            wait("x0")
            xn0 = _pack(_ln(x_v[0:TM, :].astype(f32)))
            wait("w1a")
            d1_plain(xn0, 0, 0, 256, 256)
            wait("x1")
            xn1 = [_pack(_ln(x_v[r:r + HM, :].astype(f32))) for r in (TM, TM + HM)]
            for n in range(2):
                d1_plain(xn1[n], TM + n * HM, 0, 256, 256)
            wait("w1b")
            d1_plain(jnp.concatenate([xn0] + xn1, axis=0), 0, 256, 512, 256)
            wait("w1cd")
            hist.clear()
            xn01 = jnp.concatenate([xn0] + xn1, axis=0)
            l01 = lambda rb, kh: xn01[rb * 64:(rb + 1) * 64, kh * DH2:(kh + 1) * DH2]
            pw = prep_pieces(s1_v, RAW1, LS)
            flush(d1_fine(l01, 0, 4, (512, 640), pw[:NW1], [], 1))
            carry = []
            wait("x23")
            hist.clear()
            carry = d1_fine(l01, 0, 4, (768, 896), ln_pieces(x_v, 2 * TM, 0, LL), carry, 3)
            carry = d1_s(2, 0, ln_pieces(x_v, 3 * TM, 1, LL), carry, pw[NW1:])
            wait("x4567")
            qkv_start(0)
            qkv_start(1)
            hist.clear()
            for b in range(3, NB - 1):
                carry = d1_s(b, b % 2, ln_pieces(x_v, (b + 1) * TM, (b + 1) % 2, LL), carry)
            wait("w2")
            hist.clear()
            pw = prep_pieces(s2_v, RAW, LS)
            carry = d1_s(7, 1, _merge(pw[:NW3], shift_pieces(0, 0, LS, True)), carry)
            d2_s(0, 0, shift_pieces(TM, 1, LS, True), carry, pw[NW3:], p3[:N30])
            pw = split(_merge(p3[N30:n3], sum(ln_pieces(c0_v, 0, None, LL, clag=LS, staged=True), [])), 3)
            for b in range(1, 4):
                d2_s(b, b % 2, _merge(pw[b - 1], shift_pieces((b + 1) * TM, (b + 1) % 2, LS)))
            wait("w4", "small")

        hist.clear()
        pw = p3[n3:] + prepf_pieces(s4_v, LS)
        cut = (0, 93, 192, 291) + (len(pw),)
        for b in range(4, NB):
            d2_s(b, b % 2, merge(pw[cut[b - 4]:cut[b - 3]],
                                 shift_pieces((b + 1) * TM, (b + 1) % 2, LS) if b + 1 < NB else ()))
        start("wo", priority=1)
        gw = gw_ref[0:NT, :].astype(f32)
        gb_v[...] = _cat([jnp.broadcast_to(gw[j:j + 1, :], (8, 128)) for j in range(NT)], 1)

        def ffn(i, carry):
            qkv_wait(i)
            r0 = pl.multiple_of(i * TM, TM)
            rn = pl.multiple_of(jnp.minimum(i + 1, NB - 1) * TM, TM)
            acc = {}
            hist.clear()
            LG = 5

            def relayout(p, r0_, r1_, pin):
                s0 = i * SPG + 2 * p
                e = wqkv_v[s0, r0_:r1_, :]
                o = wqkv_v[s0 + 1, r0_:r1_, :]
                wqkv_v[s0, r0_:r1_, :] = (e & jnp.uint32(0xFFFF)) | (o << 16)
                wqkv_v[s0 + 1, r0_:r1_, :] = (e >> 16) | (o & jnp.uint32(0xFFFF0000))

            relays = [(functools.partial(relayout, p, r, r + 32), wqkv_v, wqkv_v, LG, 35)
                      for p in range(SPG // 2) for r in range(0, D // 2, 32)]
            norms, combs = ln_pieces(b_v, rn, None, 10, staged=True, clag=LG)

            def gate(q, pin):
                x = pin(x_v[pl.ds(r0 + q, 16), :].astype(f32)) * _cat([gb_v[...]] * 2, 0)
                t = functools.reduce(lambda a, b: a + b, [x[:, j * 128:(j + 1) * 128] for j in range(NT)])
                g = jax.nn.sigmoid(jnp.sum(t, axis=-1, keepdims=True))
                g_v[pl.ds(r0 + q, 16), :] = jnp.broadcast_to(g, (16, 128))

            gates = [(functools.partial(gate, q), None, g_v, 10, 90) for q in range(0, TM, 16)]

            def extras(t, us, pin):
                @functools.lru_cache(None)
                def node(n):
                    if n < 16:
                        rs = pl.ds(pl.multiple_of((i + 4 * zero_s[UPARTS.index(us)]) * 64, 64) + (n // 4) * 512 + 24 + 8 * t, 8)
                        x = x_v[rs, (n % 4) * D4:(n % 4 + 1) * D4]
                        return (pin(x) if n in (0, 5, 10, 15) else x).astype(f32)
                    a, sa, b, sb = S49.up[n - 16]
                    return _run([(0, sa, 1, sb)], [node(a), node(b)])[-1]
                for u in us:
                    xe_v[S49.ul.index(u), pl.ds(pl.multiple_of(i * 16, 16) + t * 8, 8), :] = node(u).astype(bf16)

            xes = [(functools.partial(extras, t, us), None, xe_v, LG, 80) for t in range(2) for us in UPARTS]
            hs = {}

            def gelu_pieces(c, cs):
                def piece(r, cc, vs, pin):
                    t = _gelu(pin(_cat([cs[v][r:r + 8, cc:cc + 128] for v in vs], 0)))
                    ts = [t[8 * n:8 * n + 8] for n in range(len(vs))]
                    hs.update({(c, v, r, cc): u for v, u in zip(vs, ts)})
                    return functools.reduce(lambda a, b: a + b, ts)
                return [(functools.partial(piece, r, cc, range(v, v + 4)), None, None, LG, 40) for r in range(0, QM, 8)
                        for cc in range(0, cs[0].shape[1], 128) for v in range(0, SF.nb, 4)]

            def d3(c, side):
                c0, c1 = FCH[c]
                cs = fmm(SF, lambda u: lf_v[SF.ul.index(u), 0:QM], lambda r: s3_v[r, 0:D4, c0:c1], side)
                assert not side.pieces
                return gelu_pieces(c, cs)

            def d4(c, side):
                c0, c1 = FCH[c]
                lh = _run(SF.up, [_cat([_cat([hs.pop((c, v, r, cc)) for r in range(0, QM, 8)], 0)
                                        for cc in range(0, c1 - c0, 128)], 1) for v in range(SF.nb)])
                rhs = lambda r: s4_v[r, c0:c1, :]
                if c + 1 < len(FCH):
                    for n in SF.order:
                        for r in range(SF.rank):
                            if SF.wn[r] == n:
                                acc[n] = mm(lh[SF.un[r]], rhs(r), side, acc.get(n))
                else:
                    idx = lambda v: (pl.ds(r0 + (v // 4) * QM, QM), slice((v % 4) * D4, (v % 4 + 1) * D4))

                    def extra(n):
                        if n >= SF.nb:
                            return acc.get(n)
                        return b_v[idx(n)] + acc[n] if n in acc else b_v[idx(n)]

                    def emit_b(v, t):
                        b_v[idx(v)] = jnp.concatenate([1.0 - g_v[idx(v)[0], :]] * 2, axis=1) * t
                    fmm(SF, lambda u: lh[u], rhs, side, extra, emit_b)
                assert not side.pieces

            g0 = d3(0, Side(relays[:16], 43, 6))
            g1 = d3(1, Side(_merge(g0, gates[:12]), 43, 4))
            d4(0, Side(g1[:22], 41, 8))
            g2 = d3(2, Side(_merge(g1[22:], relays[16:32]), 47))
            d4(1, Side(_merge(g2, relays[32:60]), 43, 4))
            g3 = d3(3, Side(_merge(gates[12:], xes, norms), 49))
            d4(2, Side(_merge(g3, combs), 43, 4))
            d4(3, Side(relays[60:], 44))

            @pl.when(i + 2 < NG)
            def _():
                qkv_start(i + 2)

            return carry

        lax.fori_loop(0, NB, ffn, 0)

    pl.run_scoped(
        phase_b,
        pltpu.VMEM((9, D // 4, D // 2), u32),
        pltpu.VMEM((7, D // 4, D // 2), u32),
        pltpu.VMEM((52, D4 + 16, F4), bf16),
        pltpu.VMEM((52, F4 + 8, D4), bf16),
        pltpu.VMEM((NT, S + 2 * PAD, 128), f32),
        pltpu.VMEM((TM, D), f32),
        pltpu.VMEM((2, 7, HM // 2, D // 2), u32),
        pltpu.VMEM((52, QM + 8, D4), bf16),
        pltpu.VMEM((2, TM, 128), f32),
        pltpu.VMEM((8, D), f32),
    )

    def phase_a(out_v, e_v, oe_v, ke_v, ve_v, o_v):
        def pre(it, carry):
            hist.clear()
            for u in range(3 * NG // NPRE):
                s0 = (it * (3 * NG // NPRE) + u) * G

                @functools.lru_cache(None)
                def node(k, n):
                    if n < 16:
                        return _unpack(wqkv_v[s0 + zero_s[k] + n % 4, (n // 4) * (D // 8):(n // 4 + 1) * (D // 8), :])
                    a, sa, b, sb = S49.vp[n - 16]
                    return _run([(0, sa, 1, sb)], [node(k, a), node(k, b)])[-1]

                def rhs(r):
                    n = S49.vn[r]
                    if n < 16:
                        return wqkv_v[s0 + n % 4, (n // 4) * (D // 8):(n // 4 + 1) * (D // 8), :]
                    return node(r // 7, n).astype(bf16)

                def emit_e(v, t):
                    e_v[(v // 4) * 8:(v // 4 + 1) * 8, s0 + v % 4] = _pack(t).reshape(8, 8, DH)
                fmm(S49N, lambda k: xe_v[S49.ul.index(k), 0:4 * NPAIR], rhs, None, emit=emit_e)
            return carry

        lax.fori_loop(0, NPRE, pre, 0)

        wait("wo")
        mem_v[...] = mem0_ref[...].astype(f32)

        def slab(w, h):
            return (h // G) * SPG + w * G + h % G

        def step(j, hx, odd, late, allow, fill):
            qs, ks, vs, ps = {}, {}, {}, {}
            wload = lambda w, h: pltpu.bitcast(wqkv_v[slab(w, h)], bf16)
            eload = lambda w, h: pltpu.bitcast(e_v[j, slab(w, h)], bf16)

            def proj(g):
                part = {}
                if late and g == 0:
                    for h in range(2):
                        for w in range(3):
                            part[w, h] = _dot(hx[:, :DH2], wload(w, h)[:DH2])
                for h in range(g * G, (g + 1) * G):
                    q, k, v = [(_dot(hx[:, DH2:], wload(w, h)[DH2:]) + part[w, h] if (w, h) in part
                                else _dot(hx, wload(w, h))).astype(bf16) for w in range(3)]
                    if odd:
                        q = jnp.concatenate([q, eload(0, h)], axis=0)
                        k = jnp.concatenate([pltpu.bitcast(ke_v[h], bf16), eload(1, h), k], axis=0)
                        v = jnp.concatenate([pltpu.bitcast(ve_v[h], bf16), eload(2, h), v], axis=0)
                    else:
                        ke_v[h] = pltpu.bitcast(k, u32)
                        ve_v[h] = pltpu.bitcast(v, u32)
                        k = jnp.concatenate([k, eload(1, h)], axis=0)
                        v = jnp.concatenate([v, eload(2, h)], axis=0)
                    qs[h], ks[h], vs[h] = q, k, v

            def score(g):
                for h in range(g * G, (g + 1) * G):
                    s = lax.dot_general(qs.pop(h), ks.pop(h), (((1,), (1,)), ((), ())),
                                        preferred_element_type=f32)
                    ps[h] = _softmax(s, allow, fill)

            def pv(g):
                os_ = []
                for h in range(g * G, (g + 1) * G):
                    o = _dot(ps.pop(h), vs.pop(h))
                    o_v[:, h * 128:(h + 1) * 128] = _pack(o[:32])
                    os_.append(o)
                if odd:
                    quads = [jnp.concatenate([os_[2 * kk][r:r + 8], os_[2 * kk + 1][r:r + 8]], axis=1)
                             for r in (32, 40) for kk in range(2)]
                    for k, t in enumerate(_lcombos(*quads)):
                        oe_v[k, pl.ds(pl.multiple_of(j * 8, 8), 8), g * 256:(g + 1) * 256] = t

            acc = [None] * NT

            def wo(h0, h1, j0, j1):
                o = pltpu.bitcast(o_v[:, h0 * 128:h1 * 128], bf16)
                for n in range(j0, j1):
                    y = _dot(o, pltpu.bitcast(wo_v[n, h0 * 64:h1 * 64, :], bf16))
                    acc[n] = y if acc[n] is None else y + acc[n]

            for t in range(NG):
                proj(t)
                if t >= 2:
                    pv(t - 2)
                if t >= 1:
                    score(t - 1)
            wo(0, 16, 0, 4)
            pv(NG - 2)
            score(NG - 1)
            wo(0, 16, 4, 8)
            pv(NG - 1)
            wo(16, 24, 0, 8)
            wo(24, 32, 0, 8)
            return jnp.concatenate(acc, axis=1)

        def emit(j, r0, o0, a):
            rs = pl.ds(r0 + o0, 24)
            g = jnp.concatenate([g_v[rs, :]] * NT, axis=1)
            out_v[j, o0:o0 + 24, :] = (g * a + b_v[rs, :]).astype(bf16)

        def pair(j, mem, late):
            r0 = pl.multiple_of(j * 64, 64)
            allow_e, fill_e, allow_o, fill_o = _masks()
            xa = x_v[pl.ds(r0 + 16, 8), :].astype(f32)
            xb = x_v[pl.ds(r0 + 40, 8), :].astype(f32)
            hx = jnp.concatenate([x_v[pl.ds(r0, 16), :], jnp.concatenate([xa, mem], 0).astype(bf16)], 0)
            oe = step(j, hx, False, late, allow_e, fill_e)
            emit(j, r0, 0, oe[:24])
            hx = jnp.concatenate([jnp.concatenate([oe[24:32], xb], 0).astype(bf16), x_v[pl.ds(r0 + 48, 16), :]], 0)
            oo = step(j, hx, True, True, allow_o, fill_o)
            emit(j, r0, 40, oo[8:])
            return oo[:8]

        def a_iter(it, carry):
            mem = mem_v[...]
            for t in range(PPI):
                mem = pair(it * PPI + t, mem, t > 0)
            mem_v[...] = mem
            for t in range(PPI):
                for o0 in (0, 40):
                    idx = (it * PPI + t, pl.ds(o0, 24))
                    pltpu.make_async_copy(out_v.at[idx], out_hbm.at[idx], sem_out).start()
            return carry

        lax.fori_loop(0, NPAIR // PPI, a_iter, 0)

        @once
        def _post():
            hist.clear()
            NK, NW = 2, 128
            for n in range(D // (4 * NW)):
                @functools.lru_cache(None)
                def node(k, kc, q):
                    if q < 16:
                        return _unpack(raw(kc, q, 4 * zero_s[k]))
                    a, sa, b, sb = S49.vp[q - 16]
                    return _run([(0, sa, 1, sb)], [node(k, kc, a), node(k, kc, b)])[-1]

                def raw(kc, q, z=0):
                    return _cat([_cat([wo_v[z + (4 * n + q % 4) * (NW // 128) + c, (4 * g + q // 4) * 64:(4 * g + q // 4 + 1) * 64, :]
                                       for c in range(NW // 128)], 1)
                                 for g in range(kc * NG // NK, (kc + 1) * NG // NK)], 0)

                def prod(r, kc, acc):
                    z = zero_s[7 + r % 7]
                    quad = [_cat([oe_v[z + r // 7, (q // 2) * 128:(q // 2 + 1) * 128, (2 * g + q % 2) * 128:(2 * g + q % 2 + 1) * 128]
                                  for g in range(kc * NG // NK, (kc + 1) * NG // NK)], 1) if q in UQ[r % 7] else None
                            for q in range(4)]
                    f = UFORMS[r % 7]
                    lhs = quad[f[0]] if len(f) == 1 else _run([(0, f[1], 1, f[3])], [quad[f[0]], quad[f[2]]])[-1]
                    q = S49.vn[r]
                    return mm(lhs, raw(kc, q) if q < 16 else node(r // 7, kc, q).astype(bf16), None, acc)

                val, part = {}, {}
                for nd in S49N.order:
                    rs = [r for r in range(49) if S49.wn[r] == nd]
                    for r in rs:
                        if r not in part:
                            for kc in range(NK - 1):
                                for k2 in SEQ:
                                    part[r // 7 * 7 + k2] = prod(r // 7 * 7 + k2, kc, part.get(r // 7 * 7 + k2))
                    t = part[rs[0]] if rs else None
                    for q, sg in sorted(S49.par[nd], key=lambda e: -e[1]):
                        t = val[q] if t is None else (t + val[q] if sg > 0 else t - val[q])
                    if rs:
                        t = prod(rs[0], NK - 1, t)
                    val[nd] = t
                    if nd < 16:
                        o0, j0 = 24 + (nd // 8) * 8, (nd // 4 % 2) * 16
                        c0 = (4 * n + nd % 4) * NW
                        for jj in range(16):
                            rr = slice((j0 + jj) * 64 + o0, (j0 + jj) * 64 + o0 + 8)
                            out_v[j0 + jj, o0:o0 + 8, c0:c0 + NW] = (
                                _cat([g_v[rr, :]] * (NW // 128), 1) * t[jj * 8:jj * 8 + 8] + b_v[rr, c0:c0 + NW]).astype(bf16)
                        idx = (pl.ds(j0, 16), pl.ds(o0, 8), pl.ds(c0, NW))
                        pltpu.make_async_copy(out_v.at[idx], out_hbm.at[idx], sem_out).start()

        pltpu.make_async_copy(out_v, out_hbm, sem_out).wait()

    pl.run_scoped(
        phase_a,
        pltpu.VMEM((NPAIR, 64, D), bf16),
        pltpu.VMEM((NPAIR, 3 * H, 8, DH), u32),
        pltpu.VMEM((7, 8 * NPAIR, H * DH // 2), f32),
        pltpu.VMEM((H, 16, 128), u32),
        pltpu.VMEM((H, 16, 128), u32),
        pltpu.VMEM((16, H * DH), u32),
    )


@jax.jit
def pallas_gated_mix__memory_aug_recurrent_mem_tr__mixer_s_mlp__prompt_kernel(
    A_x, A_mem0, A_Wq, A_Wk, A_Wv, A_Wo, A_seg_len, B_x, B_w1, B_w2, B_w3, B_w4, gate_w,
):
    assert A_x.shape == (1, S, D) and A_mem0.shape == (1, M, D)
    any_spec = pl.BlockSpec(memory_space=pl.ANY)
    out = pl.pallas_call(
        _kernel,
        out_shape=jax.ShapeDtypeStruct((NPAIR, 64, D), bf16),
        in_specs=[any_spec] * 11,
        out_specs=any_spec,
        scratch_shapes=[
            pltpu.VMEM((S, D), bf16),
            pltpu.VMEM((3 * H, D // 2, DH), u32),
            pltpu.VMEM((NT, H * DH // 2 + 8, 128), u32),
            pltpu.VMEM((S, D), f32),
            pltpu.VMEM((S, 128), f32),
            pltpu.VMEM((52, 4 * NPAIR + 8, D4), bf16),
            pltpu.VMEM((M, D), f32),
            pltpu.VMEM((M, D), bf16),
            pltpu.VMEM((64, 128), bf16),
            pltpu.SMEM((NZ,), jnp.int32),
            pltpu.SemaphoreType.DMA((NLOAD,)),
            pltpu.SemaphoreType.DMA((NG,)),
            pltpu.SemaphoreType.DMA,
        ],
        compiler_params=pltpu.CompilerParams(vmem_limit_bytes=127 * 1024 * 1024,
                                             disable_bounds_checks=True),
    )(
        A_x.reshape(S, D), A_mem0.reshape(M, D),
        A_Wq.reshape(D // 2, 2 * H, DH), A_Wk.reshape(D // 2, 2 * H, DH), A_Wv.reshape(D // 2, 2 * H, DH),
        A_Wo.reshape(H * DH, D), B_w1, B_w2, B_w3, B_w4, gate_w.reshape(NT, 128),
    )
    return out.reshape(1, S, D)
```

```python
import functools

import jax
import jax.numpy as jnp
from jax import lax
import jax.experimental.pallas as pl
import jax.experimental.pallas.tpu as pltpu

f32, bf16, u32 = jnp.float32, jnp.bfloat16, jnp.uint32

S, D, H, DH, M, SEG, F = 2048, 1024, 32, 128, 8, 32, 3584
SCALE = DH ** -0.5
NEG = -1000000000.0
EPS = 1e-05

TM = 256
NB = S // TM
HM = TM // 2
DH2 = D // 2
D4, F4 = D // 4, F // 4
FCH = ((0, 128), (128, 384), (384, 640), (640, 896))
NC1 = 128
NPAIR = S // (2 * SEG)
PPI = 2
NPRE = 3
G = 4
NG = H // G
PAD = 8
NT = D // 128
TIEP = 2
W3A = 224
NZ = 16
NLOAD = 11
assert NB == NG

_dot = functools.partial(jnp.dot, preferred_element_type=f32)

def _run(prog, blocks):
    vals = list(blocks)
    for a, sa, b, sb in prog:
        vals.append(vals[a] + vals[b] if sa > 0 and sb > 0 else
                    vals[a] - vals[b] if sa > 0 else vals[b] - vals[a])
    return vals


def _form(f, get):
    return get(f[0]) if len(f) == 1 else get(f[0]) + get(f[2]) if f[3] > 0 else get(f[0]) - get(f[2])


def _terms(prog, nin, node):
    if node < nin:
        return {node: 1}
    a, sa, b, sb = prog[node - nin]
    out = {k: sa * v for k, v in _terms(prog, nin, a).items()}
    out.update({k: sb * v for k, v in _terms(prog, nin, b).items()})
    return out


class _Scheme:
    def __init__(self, ms, up, vp, wp, un, vn, wn):
        self.ms, self.nb, self.rank = ms, 4 * ms, len(un)
        self.up, self.vp, self.wp, self.un, self.vn, self.wn = up, vp, wp, un, vn, wn
        self.ul = tuple(sorted(set(un)))
        t = {}
        for r in range(self.rank):
            for a, ca in _terms(up, self.nb, un[r]).items():
                for b, cb in _terms(vp, 16, vn[r]).items():
                    for c, cc in _terms(wp, self.nb, wn[r]).items():
                        t[a, b, c] = t.get((a, b, c), 0) + ca * cb * cc
        assert {k: v for k, v in t.items() if v} == {
            (4 * i + j, 4 * j + l, 4 * i + l): 1 for i in range(ms) for j in range(4) for l in range(4)}
        self.par = {n: [] for n in range(self.nb + len(wp))}
        for k, (a, sa, b, sb) in enumerate(wp):
            self.par[a].append((self.nb + k, sa))
            self.par[b].append((self.nb + k, sb))
        self.order = order = []

        def closure(n, acc):
            if n not in acc and n not in order:
                acc.add(n)
                for q, _ in self.par[n]:
                    closure(q, acc)
            return acc

        def visit(n):
            if n not in order:
                for q, _ in self.par[n]:
                    visit(q)
                order.append(n)
        while len([v for v in range(self.nb) if v not in order]):
            visit(min((v for v in range(self.nb) if v not in order), key=lambda v: len(closure(v, set()))))


def _twice(forms):
    prog, nodes = [], []

    def apply(f, quad):
        if len(f) == 1:
            return quad[f[0]]
        prog.append((quad[f[0]], f[1], quad[f[2]], f[3]))
        return 15 + len(prog)
    for f1 in forms:
        inner = [apply(f1, [4 * (2 * (q // 2) + p // 2) + 2 * (q % 2) + p % 2 for q in range(4)]) for p in range(4)]
        nodes += [apply(f2, inner) for f2 in forms]
    return tuple(prog), tuple(nodes)


UFORMS = ((0, 1, 3, 1), (2, 1, 3, 1), (0,), (3,), (0, 1, 1, 1), (2, 1, 0, -1), (1, 1, 3, -1))
UQ = [f[::2] for f in UFORMS]
SEQ = (1, 3, 4, 2, 0, 5, 6)
_U2 = _twice(UFORMS)
VFORMS = ((0, 1, 3, 1), (0,), (1, 1, 3, -1), (2, 1, 0, -1), (3,), (0, 1, 1, 1), (2, 1, 3, 1))
_V2 = _twice(VFORMS)
_W2 = _twice(((0, 1, 3, 1), (2, 1, 3, -1), (1, 1, 3, 1), (0, 1, 2, 1), (1, 1, 0, -1), (3,), (0,)))
S49 = _Scheme(4, _U2[0], _V2[0], _W2[0], _U2[1], _V2[1], _W2[1])
VSTAGES = (((2, 5), (1,)), ((3, 6), (2,)), ((0, 1, 4), (0, 3)))
S49.raw = tuple(7 * (1, 2, 3, 4)[2 * (q // 8) + q % 4 // 2] + (1, 2, 3, 4)[2 * (q // 4 % 2) + q % 2] for q in range(16))
assert all(S49.raw[S49.vn[r]] == r for r in range(49) if S49.vn[r] < 16)


def _outer_major(n):
    rs = [7 * SEQ.index(r // 7) + SEQ.index(r % 7) for r in range(49) if S49.wn[r] == n]
    return max(rs + [-1] + [_outer_major(q) + 0.01 for q, _ in S49.par[n]])


S49N = _Scheme(4, _U2[0], _V2[0], _W2[0], _U2[1], _V2[1], _W2[1])
S49N.order.sort(key=_outer_major)
UPARTS = [[S49.un[r] for k in ks for r in range(7 * k, 7 * k + 7)] for ks in ((0, 2, 3), (4, 6), (1, 5))]
SF = S49
QM = TM // SF.ms


def _ln(x):
    m = jnp.mean(x, axis=-1, keepdims=True)
    xc = x - m
    v = jnp.mean(xc * xc, axis=-1, keepdims=True)
    return xc * lax.rsqrt(v + EPS)


_GC = 0.7978845608028654


def _gelu(x):
    h = 0.5 * x
    return h + h * jnp.tanh(x * (_GC + (_GC * 0.044715) * (x * x)))


def _unpack(u):
    return pltpu.bitcast(u, bf16).astype(f32)


def _pack(x):
    return pltpu.bitcast(x.astype(bf16), u32)


def _split(u):
    return jnp.concatenate([pltpu.bitcast(u << 16, f32), pltpu.bitcast(u & jnp.uint32(0xFFFF0000), f32)], axis=-1)


def _join(x):
    return pltpu.bitcast(x.astype(bf16).reshape(x.shape[:-2] + (2 * x.shape[-2], 128)), u32)


def _cat(xs, axis):
    xs = [x for x in xs if x.shape[axis]]
    return xs[0] if len(xs) == 1 else jnp.concatenate(xs, axis=axis)


def _as(x, dtype):
    return x if x.dtype == dtype else pltpu.bitcast(x, dtype)


def _lcombos(a11, a12, a21, a22):
    return [a11 + a22, a21 + a22, a11, a22, a11 + a12, a21 - a11, a12 - a22]


def _merge(*lists):
    keyed = [((j + 0.5) / len(l), n, j, v) for n, l in enumerate(lists) for j, v in enumerate(l)]
    return [v for _, _, _, v in sorted(keyed, key=lambda t: t[:3])]


def _masks():
    r = lax.broadcasted_iota(jnp.int32, (32, 48), 0)
    c = lax.broadcasted_iota(jnp.int32, (32, 48), 1)
    exist_e = c < 40
    allow_e = exist_e & ((r >= 24) | ((c >= 24) & (c < 32)) | (c <= r))
    fill_e = jnp.where(exist_e, NEG, -jnp.inf).astype(f32)
    r = lax.broadcasted_iota(jnp.int32, (48, 80), 0)
    c = lax.broadcasted_iota(jnp.int32, (48, 80), 1)
    q_even = (r >= 32) & (r < 40)
    exist_o = (q_even & (c < 40)) | (~q_even & (c >= 40))
    ktok = jnp.where(c < 24, c, jnp.where(c < 48, c - 8, c - 16))
    qtok = jnp.where(r < 32, r + 32, r - 8)
    is_mem_key = ((c >= 24) & (c < 32)) | ((c >= 48) & (c < 56))
    allow_o = exist_o & (is_mem_key | (r < 8) | (ktok <= qtok))
    fill_o = jnp.where(exist_o, NEG, -jnp.inf).astype(f32)
    return allow_e, fill_e, allow_o, fill_o


def _softmax(s, allow, fill):
    s = jnp.where(allow, s * SCALE, fill)
    m = jnp.max(s, axis=-1, keepdims=True)
    e = jnp.exp(s - m)
    l = jnp.sum(e, axis=-1, keepdims=True)
    r = pl.reciprocal(l, approx=True)
    r = r * (2.0 - l * r)
    return (e * r).astype(bf16)


def _kernel(x_hbm, mem0_hbm, wq_hbm, wk_hbm, wv_hbm, wo_hbm, w1_hbm, w2_hbm, w3_hbm, w4_hbm,
            gw_hbm, out_hbm,
            x_v, wqkv_v, wo_v, b_v, g_v, xe_v, mem_v, mem0_ref, gw_ref, zero_s,
            sem, sem_qkv, sem_out):
    RAW = (1, 2, 3, 4)
    RAW1 = (1, 7, 8, 4)

    loads = []

    def rows_load(name, r0, r1):
        loads.append((name, x_hbm.at[pl.ds(r0, r1 - r0)], x_v.at[pl.ds(r0, r1 - r0)]))

    def quad_load(name, w_hbm, s_v, raw, q, c0=0, c1=None):
        k4, n2 = s_v.shape[1], s_v.shape[2]
        c1 = n2 if c1 is None else c1
        src = w_hbm.bitcast(u32).at[pl.ds((q // 2) * k4, k4), pl.ds((q % 2) * n2 + c0, c1 - c0)]
        loads.append((name, src, s_v.at[raw[q], :, pl.ds(c0, c1 - c0)]))

    for j in range(NT):
        loads.append(("wo", wo_hbm.bitcast(u32).at[:, pl.ds(j * 128, 128)], wo_v.at[j, pl.ds(0, H * DH // 2)]))
    groups = []

    def start(*names, priority=0):
        for name, src, dst in loads:
            if name in names:
                pltpu.make_async_copy(src, dst, sem.at[groups.index(name)]).start(priority=priority)

    def wait(*names):
        for name, src, dst in loads:
            if name in names:
                pltpu.make_async_copy(src, dst, sem.at[groups.index(name)]).wait()

    SPG = 3 * G

    def qkv_start(g):
        for w, w_hbm in enumerate((wq_hbm, wk_hbm, wv_hbm)):
            wu = w_hbm.bitcast(u32)
            for k in range(G // 2):
                for par in range(2):
                    pltpu.make_async_copy(
                        wu.at[:, par * (H // 2) + g * (G // 2) + k, :],
                        wqkv_v.at[g * SPG + w * G + 2 * k + par], sem_qkv.at[g]).start(priority=1)

    def qkv_wait(g):
        grp = wqkv_v.at[pl.ds(g * SPG, SPG)]
        pltpu.make_async_copy(grp, grp, sem_qkv.at[g]).wait()

    def once(fn):
        def body(_, carry):
            fn()
            return carry
        lax.fori_loop(0, 1 + zero_s[1], body, 0)

    def tile_idx(ref, cols=128):
        z = zero_s[0]
        n = 16 if ref.dtype == bf16 and cols == 128 else 8
        return (z,) * (len(ref.shape) - 2) + (pl.ds(pl.multiple_of(z, n), n), slice(0, cols))

    hist = []

    def mm(lhs, rhs, side=None, acc=None):
        if side is not None:
            lhs = side(lhs)
        lhs = pltpu.bitcast(lhs, bf16) if lhs.dtype == u32 else lhs.astype(bf16)
        y = _dot(lhs, pltpu.bitcast(rhs, bf16) if rhs.dtype == u32 else rhs)
        if acc is not None:
            y = y + acc
        hist.append(y)
        return y

    class Side:
        def __init__(self, pieces, n, skip=0):
            cap = [0] * skip + [1] * n
            tot = sum(p[4] for p in pieces)
            self.plan = [[] for _ in cap]
            done = 0
            for p in pieces:
                done += p[4]
                x, d = done / tot * sum(cap), 0
                while x > cap[d] + 1e-9:
                    x -= cap[d]
                    d += 1
                self.plan[d].append((p, x / cap[d]))
            self.pieces = len(pieces)

        def __call__(self, val):
            todo = self.plan.pop(0) if self.plan else []
            if not todo:
                return val
            self.pieces -= len(todo)
            never = zero_s[0] > 0
            if val.dtype == bf16:
                val = pltpu.bitcast(val, u32)
            rg = 8 if val.dtype == u32 else 16
            ng = val.shape[0] // rg
            tied = {}
            for (fn, rd, wr, lag, _), pos in todo:
                m = min(max(-int(-pos * ng // 1) - 1, 0), ng - 1)
                pin = lambda v, w=128: v
                if lag is not None and len(hist) >= lag:
                    r0 = (16 * m) % hist[-lag].shape[0]
                    a = hist[-lag][r0:r0 + 8, :128]
                    if rd is None:
                        def pin(v, w=128, a=a):
                            if v.ndim == 3:
                                return lax.select(never, _as(a, v.dtype).reshape(v.shape), v)
                            if v.dtype == bf16:
                                a = _cat([a] * (v.shape[-1] // 128), 1).astype(bf16)
                                return lax.select(never, a.reshape(v.shape), v)
                            a = _cat([_cat([_as(a, v.dtype)] * (v.shape[0] // 8), 0)] * (w // 128), 1)
                            if v.shape[1] == w:
                                return lax.select(never, a, v)
                            return _cat([lax.select(never, a, v[:, :w]), v[:, w:]], 1)
                    elif rd.dtype == bf16:
                        idx = tile_idx(rd, 256)
                        rd[idx] = lax.select(never, _cat([a, a], 1).astype(bf16), rd[idx])
                    else:
                        idx = tile_idx(rd)
                        rd[idx] = lax.select(never, _as(a, rd.dtype), rd[idx])
                u = fn(pin)
                if wr is False:
                    continue
                if wr is not None:
                    u = wr[tile_idx(wr)]
                t, n = tied.get(m * rg) or (val[m * rg:m * rg + 8, -128:], 0)
                tied[m * rg] = (lax.select(zero_s[n] > 0, _as(u, val.dtype), t), n + 1)
            if not tied:
                return val
            col, r = [], 0
            for r0 in sorted(tied):
                col += ([val[r:r0, -128:]] if r0 > r else []) + [tied[r0][0]]
                r = r0 + 8
            col += [val[r:, -128:]] if r < val.shape[0] else []
            return _cat([val[:, :-128], _cat(col, 0)], 1) if val.shape[1] > 128 else _cat(col, 0)

    def strassen(lhs, rhs, side, init=(None, None, None, None)):
        def add(a, b):
            return a if b is None else a + b
        p = [mm(lhs(k), rhs(k), side) for k in range(5)]
        c12 = add(p[2] + p[4], init[1])
        c21 = add(p[1] + p[3], init[2])
        c22 = mm(lhs(5), rhs(5), side, add(p[0] - p[1] + p[2], init[3]))
        c11 = mm(lhs(6), rhs(6), side, add(p[0] + p[3] - p[4], init[0]))
        return c11, c12, c21, c22

    def fmm(sc, lhs, rhs, side, extra=lambda n: None, emit=None):
        val = {}
        for n in sc.order:
            t = extra(n)
            for q, sg in sorted(sc.par[n], key=lambda e: -e[1]):
                t = val[q] if t is None else (t + val[q] if sg > 0 else t - val[q])
            for r in range(sc.rank):
                if sc.wn[r] == n:
                    t = mm(lhs(sc.un[r]), rhs(r), side, t)
            val[n] = t
            if n < sc.nb and emit is not None:
                emit(n, t)
        return [val[v] for v in range(sc.nb)]

    def phase_b(s1_v, s2_v, s3_v, s4_v, h_v, c0_v, l_v, lf_v, n_v, gb_v):
        def w1_load(name, half, c0, c1):
            quad_load(name, w1_hbm, s1_v, RAW1, half, c0, c1)
            quad_load(name, w1_hbm, s1_v, RAW1, 2 + half, c0, c1)

        def block_load(name, w_hbm, s_v, r0, r1):
            kb, nb = s_v.shape[1] - 8, s_v.shape[2]
            for q in range(16):
                loads.append((name, w_hbm.bitcast(u32).at[pl.ds((q // 4) * kb + r0, r1 - r0), pl.ds((q % 4) * nb, nb)],
                              s_v.at[SF.raw[q], pl.ds(r0, r1 - r0)]))

        rows_load("x0", 0, TM)
        w1_load("w1a", 0, 0, 256)
        rows_load("x1", TM, 2 * TM)
        w1_load("w1b", 0, 256, 512)
        w1_load("w1cd", 1, 0, 512)
        rows_load("x23", 2 * TM, 4 * TM)
        rows_load("x4567", 4 * TM, S)
        for q in range(4):
            quad_load("w2", w2_hbm, s2_v, RAW, q)
        block_load("w2", w3_hbm, s3_v, 0, W3A // 2)
        block_load("w4", w3_hbm, s3_v, W3A // 2, D4 // 2)
        block_load("w4", w4_hbm, s4_v, 0, F4 // 2)
        loads.append(("small", mem0_hbm, mem0_ref))
        loads.append(("small", gw_hbm, gw_ref.at[pl.ds(0, NT)]))
        groups.extend(dict.fromkeys(name for name, _, _ in loads))
        assert len(groups) == NLOAD

        start("x0", "w1a", "w1b", "x1", "w1cd", "x23", "x4567", "w2", "w4", "small")

        def zero(k, carry):
            zero_s[k] = 0
            return carry
        lax.fori_loop(0, NZ, zero, 0)

        def prepf_pieces(s_v, lag):
            def piece(rs, cs, st, pin):
                z = 4 * zero_s[st]

                @functools.lru_cache(None)
                def quad(q):
                    t = s_v[pl.ds(z + 7 * q + 8, 4), rs, cs]
                    if q in VSTAGES[st][1]:
                        t = _cat([pin(t[0:1]), t[1:3], pin(t[3:4])], 0)
                    return _split(t)
                done = []
                for k in VSTAGES[st][0]:
                    t = _form(VFORMS[k], quad)
                    t = [t[q:q + 1] for q in range(4)]
                    ts = [_form(f, lambda q: t[q]) for f in VFORMS]
                    for a, b in ((0, 7),) if len(VFORMS[k]) > 1 else ((0, 1), (2, 4), (5, 7)):
                        done.append((7 * k + a, _join(_cat(ts[a:b], 0))))
                for r, t in done:
                    s_v[pl.ds(z + r, t.shape[0]), rs, cs] = t
            out = [(slice(r, r + 8), slice(c, c + 128))
                   for r in range(0, s_v.shape[1] - 8, 8) for c in range(0, s_v.shape[2], 128)]
            return [(functools.partial(piece, rs, cs, st), None, s_v if n % TIEP == 0 else False, lag, 80)
                    for g in range(0, len(out), 7) for st in range(3) for n, (rs, cs) in enumerate(out[g:g + 7])]

        def prep_pieces(s_v, raw, lag):
            def piece(r, c, pin):
                idx = (slice(r, r + 16), slice(c, c + 128))
                b = [_split(pin(s_v[(q,) + idx]) if n in (0, 3) else s_v[(q,) + idx]) for n, q in enumerate(raw)]
                for k in (0, 2, 3, 5, 6):
                    s_v[(k,) + idx] = _join(_form(VFORMS[k], lambda q: b[q]))
            return [(functools.partial(piece, r, c), None, s_v, lag, 50)
                    for c in range(0, s_v.shape[2], 128) for r in range(0, s_v.shape[1], 16)]

        def store_l(slot, q, c, quads):
            for k, t in enumerate(_lcombos(*quads)):
                l_v[slot, k, q // 2:q // 2 + 8, c:c + t.shape[1]] = _pack(t)

        def ln_pieces(src, r0, slot, lag, width=256, staged=False, clag=None):
            def stats(q, pin):
                x = pin(src[pl.ds(r0 + q, 16), :].astype(f32))
                xs = [x[:, j * 128:(j + 1) * 128] for j in range(NT)]
                m = functools.reduce(lambda a, b: a + b, xs) * (1.0 / NT)
                w = functools.reduce(lambda a, b: a + b, [(t - m) * (t - m) for t in xs])
                mean = jnp.mean(m, axis=-1, keepdims=True)
                var = jnp.sum(w + NT * ((m - mean) * (m - mean)), axis=-1, keepdims=True) * (1.0 / D)
                n_v[0, q:q + 16, :] = jnp.broadcast_to(mean, (16, 128))
                n_v[1, q:q + 16, :] = jnp.broadcast_to(lax.rsqrt(var + EPS), (16, 128))

            def comb(q, c, pin):
                quads = []
                for rr in (0, HM):
                    rs = pl.ds(pl.multiple_of(r0 + rr + q + zero_s[0], 16), 16)
                    mean, rstd = [jnp.concatenate([n_v[t, rr + q:rr + q + 16, :]] * (width // 128), axis=1)
                                  for t in range(2)]
                    quads += [(src[rs, cc + c:cc + c + width].astype(f32) - mean) * rstd for cc in (0, DH2)]
                store_l(slot, q, c, quads)

            def normf(q, pin):
                mean, rstd = [_cat([n_v[t, q:q + 16, :]] * NT, 1) for t in range(2)]
                c0_v[q:q + 16, :] = (src[pl.ds(pl.multiple_of(r0 + q + zero_s[0], 8), 16), :] - mean) * rstd

            def combf(q, us, pin):
                @functools.lru_cache(None)
                def node(n):
                    if n < SF.nb:
                        return c0_v[(n // 4) * QM + q:(n // 4) * QM + q + 8, (n % 4) * D4:(n % 4 + 1) * D4]
                    a, sa, b, sb = SF.up[n - SF.nb]
                    return _run([(0, sa, 1, sb)], [node(a), node(b)])[-1]
                for u in us:
                    lf_v[SF.ul.index(u), q:q + 8, :] = node(u).astype(bf16)
            dense = slot is not None or src is b_v
            norms = [[(functools.partial(stats, rr + q), None, n_v if dense else False, lag, 90) for rr in (0, HM)]
                     for q in range(0, HM, 16)]
            if slot is None:
                combs = [[(functools.partial(combf, q, us), c0_v, lf_v if dense or us is UPARTS[-1] else False, clag, 55)
                          for us in UPARTS] for q in range(0, QM, 8)]
            else:
                combs = [[(functools.partial(comb, q, c), n_v, l_v, clag, 125) for c in range(0, DH2, width)]
                         for q in range(0, HM, 16)]
            if staged:
                return (sum(norms, []) + [(functools.partial(normf, q), n_v, c0_v, clag, 40) for q in range(0, TM, 16)],
                        sum(combs, []))
            out = list(norms[0])
            for a, b in zip(norms[1:] + [[]], combs):
                out += _merge(a, b) if a else b
            return out

        shifts = (1, 1, -1, -1, 2, 2, -2, -2)

        def shift_pieces(r0, slot, lag, by_value=True):
            def piece(q, j, pin):
                a = [_cat([h_v[jj, pl.ds(PAD + r0 + rr + q - shifts[jj] + par, 8, stride=2), :] for par in range(2)], 1)
                     for rr in (0, HM) for jj in (j, j + NT // 2)]
                for k, t in enumerate(_lcombos(pin(a[0]), a[1], a[2], pin(a[3]))):
                    l_v[slot, k, q // 2:q // 2 + 8, j * 128:(j + 1) * 128] = _join(t)
            return [(functools.partial(piece, q, j), None if by_value else h_v,
                     l_v if j % 2 else False, lag, 25)
                    for q in range(0, HM, 16) for j in range(NT // 2)]

        def lhs_of(slot):
            return lambda k: l_v[slot, k]

        for ref in (xe_v, lf_v, s3_v, s4_v):
            ref[0, 0:16, 0:D4] = jnp.zeros((16, D4), ref.dtype)
        h_v[:, 0:PAD, :] = jnp.zeros((NT, PAD, 128), f32)
        h_v[:, PAD + S:PAD + S + PAD, :] = jnp.zeros((NT, PAD, 128), f32)

        def store_h(r0, c0, h):
            for j in range(h.shape[1] // 128):
                h_v[c0 // 128 + j, PAD + r0:PAD + r0 + h.shape[0], :] = h[:, j * 128:(j + 1) * 128]

        def h_pieces(r0, c0, t, lag, n=4):
            def piece(r, pin):
                store_h(r0 + r, c0, _gelu(pin(t[r:r + 8 * n])))
            return [(functools.partial(piece, r), None, h_v, lag, 10 * n) for r in range(0, t.shape[0], 8 * n)]

        def flush(pieces):
            for p in pieces:
                p[0](lambda v, w=128: v)

        def w1_cols(c, step):
            half, cc = c // DH2, c % DH2
            return jnp.concatenate([s1_v[RAW1[half], :, cc:cc + step], s1_v[RAW1[2 + half], :, cc:cc + step]], axis=0)

        def d1_plain(xn, r0, c0, c1, step):
            for c in range(c0, c1, step):
                store_h(r0, c, _gelu(mm(xn, w1_cols(c, step))))

        def d1_fine(lhs, r0, nrb, cols, pieces, carry, skip=0):
            tiles = [(rb, c) for c in cols for rb in range(nrb)]
            rounds = [tiles[i:i + 4] for i in range(0, len(tiles), 4)]
            for n, (rnd, part) in enumerate(zip(rounds, split(pieces, len(rounds)))):
                sk = skip if n == 0 else 0
                side = Side(_merge(carry, part) if carry else part, 8 - sk, sk)
                carry = []
                for rb, c in rnd:
                    half, cc = c // DH2, c % DH2
                    t = mm(lhs(rb, 0), s1_v[RAW1[half], :, cc:cc + 128], side)
                    t = mm(lhs(rb, 1), s1_v[RAW1[2 + half], :, cc:cc + 128], side, t)
                    carry += h_pieces(r0 + rb * HM, c, t, LS)
            return carry

        def d1_s(b, slot, pieces, carry, early=()):
            for c, part, e in zip(range(0, DH2, NC1), split(pieces, DH2 // NC1), split(early, 2) + [[], []]):
                side = Side(merge(carry, part, e), *((7,) if hist else (5, 2)))
                cs = strassen(lhs_of(slot), lambda k: s1_v[k, :, c:c + NC1], side)
                carry = sum([h_pieces(b * TM + (q // 2) * HM, (q % 2) * DH2 + c, cs[q], LS) for q in (1, 2, 3, 0)], [])
            return carry

        def d2_s(b, slot, pieces, carry=(), early=(), late=()):
            for c, part, e in zip(range(0, DH2, NC1), split(pieces, DH2 // NC1), split(early, 2) + split(late, 2)):
                side = Side(merge(carry, part, e), *((7,) if hist else (5, 2)))
                carry = ()
                idx = [(slice(b * TM + (q // 2) * HM, b * TM + (q // 2 + 1) * HM),
                        slice((q % 2) * DH2 + c, (q % 2) * DH2 + c + NC1)) for q in range(4)]
                cs = strassen(lhs_of(slot), lambda k: s2_v[k, :, c:c + NC1], side,
                              [x_v[i].astype(f32) for i in idx])
                for i, t in zip(idx, cs):
                    b_v[i] = t
                    if b == 0:
                        c0_v[i] = t

        def split(l, n):
            w = [1.0 if hist else 0.6] + [1.0] * (n - 1)
            cut = [int(round(len(l) * sum(w[:i]) / sum(w))) for i in range(n + 1)]
            return [l[cut[i]:cut[i + 1]] for i in range(n)]

        def merge(*ls):
            ls = [l for l in ls if l]
            return _merge(*ls) if ls else []

        NW1, NW3, NA, NB2, N30 = 56, 32, 40, 56, 98
        LS, LL = 3, 5

        p3 = prepf_pieces(s3_v, LS)
        n3 = len(p3) * W3A // D4

        @once
        def _phase1a():
            wait("x0")
            xn0 = _pack(_ln(x_v[0:TM, :].astype(f32)))
            wait("w1a")
            d1_plain(xn0, 0, 0, 256, 256)
            wait("x1")
            xn1 = [_pack(_ln(x_v[r:r + HM, :].astype(f32))) for r in (TM, TM + HM)]
            for n in range(2):
                d1_plain(xn1[n], TM + n * HM, 0, 256, 256)
            wait("w1b")
            d1_plain(jnp.concatenate([xn0] + xn1, axis=0), 0, 256, 512, 256)
            wait("w1cd")
            hist.clear()
            xn01 = jnp.concatenate([xn0] + xn1, axis=0)
            l01 = lambda rb, kh: xn01[rb * 64:(rb + 1) * 64, kh * DH2:(kh + 1) * DH2]
            pw = prep_pieces(s1_v, RAW1, LS)
            flush(d1_fine(l01, 0, 4, (512, 640), pw[:NW1], [], 1))
            carry = []
            wait("x23")
            hist.clear()
            carry = d1_fine(l01, 0, 4, (768, 896), ln_pieces(x_v, 2 * TM, 0, LL), carry, 3)
            carry = d1_s(2, 0, ln_pieces(x_v, 3 * TM, 1, LL), carry, pw[NW1:])
            wait("x4567")
            qkv_start(0)
            qkv_start(1)
            hist.clear()
            for b in range(3, NB - 1):
                carry = d1_s(b, b % 2, ln_pieces(x_v, (b + 1) * TM, (b + 1) % 2, LL), carry)
            wait("w2")
            hist.clear()
            pw = prep_pieces(s2_v, RAW, LS)
            carry = d1_s(7, 1, _merge(pw[:NW3], shift_pieces(0, 0, LS, True), p3[:NA]), carry)
            d2_s(0, 0, shift_pieces(TM, 1, LS, True), carry, _merge(pw[NW3:], p3[NA:NB2]), p3[NB2:N30])
            pw = split(_merge(p3[N30:n3], sum(ln_pieces(c0_v, 0, None, LL, clag=LS, staged=True), [])), 3)
            for b in range(1, 4):
                d2_s(b, b % 2, _merge(pw[b - 1], shift_pieces((b + 1) * TM, (b + 1) % 2, LS)))
            wait("w4", "small")

        hist.clear()
        pw = p3[n3:] + prepf_pieces(s4_v, LS)
        cut = (0, 90, 184, 278) + (len(pw),)
        for b in range(4, NB):
            d2_s(b, b % 2, merge(pw[cut[b - 4]:cut[b - 3]],
                                 shift_pieces((b + 1) * TM, (b + 1) % 2, LS) if b + 1 < NB else ()))
        start("wo", priority=1)
        gw = gw_ref[0:NT, :].astype(f32)
        gb_v[...] = _cat([jnp.broadcast_to(gw[j:j + 1, :], (8, 128)) for j in range(NT)], 1)

        def ffn(i, carry):
            qkv_wait(i)
            r0 = pl.multiple_of(i * TM, TM)
            rn = pl.multiple_of(jnp.minimum(i + 1, NB - 1) * TM, TM)
            acc = {}
            hist.clear()
            LG = 6

            def relayout(p, r0_, r1_, pin):
                s0 = i * SPG + 2 * p
                e = wqkv_v[s0, r0_:r1_, :]
                o = wqkv_v[s0 + 1, r0_:r1_, :]
                wqkv_v[s0, r0_:r1_, :] = (e & jnp.uint32(0xFFFF)) | (o << 16)
                wqkv_v[s0 + 1, r0_:r1_, :] = (e >> 16) | (o & jnp.uint32(0xFFFF0000))

            relays = [(functools.partial(relayout, p, r, r + 32), wqkv_v, wqkv_v, LG, 35)
                      for p in range(SPG // 2) for r in range(0, D // 2, 32)]
            norms, combs = ln_pieces(b_v, rn, None, 10, staged=True, clag=LG)

            def gate(q, pin):
                x = pin(x_v[pl.ds(r0 + q, 16), :].astype(f32)) * _cat([gb_v[...]] * 2, 0)
                t = functools.reduce(lambda a, b: a + b, [x[:, j * 128:(j + 1) * 128] for j in range(NT)])
                g = jax.nn.sigmoid(jnp.sum(t, axis=-1, keepdims=True))
                g_v[pl.ds(r0 + q, 16), :] = jnp.broadcast_to(g, (16, 128))

            gates = [(functools.partial(gate, q), None, g_v, 10, 90) for q in range(0, TM, 16)]

            def extras(t, us, pin):
                @functools.lru_cache(None)
                def node(n):
                    if n < 16:
                        rs = pl.ds(pl.multiple_of((i + 4 * zero_s[UPARTS.index(us)]) * 64, 64) + (n // 4) * 512 + 24 + 8 * t, 8)
                        x = x_v[rs, (n % 4) * D4:(n % 4 + 1) * D4]
                        return (pin(x) if n in (0, 5, 10, 15) else x).astype(f32)
                    a, sa, b, sb = S49.up[n - 16]
                    return _run([(0, sa, 1, sb)], [node(a), node(b)])[-1]
                for u in us:
                    xe_v[S49.ul.index(u), pl.ds(pl.multiple_of(i * 16, 16) + t * 8, 8), :] = node(u).astype(bf16)

            xes = [(functools.partial(extras, t, us), None, xe_v, LG, 80) for t in range(2) for us in UPARTS]
            hs = {}

            def gelu_pieces(c, cs):
                def piece(r, cc, vs, pin):
                    t = _gelu(pin(_cat([cs[v][r:r + 8, cc:cc + 128] for v in vs], 0)))
                    ts = [t[8 * n:8 * n + 8] for n in range(len(vs))]
                    hs.update({(c, v, r, cc): u for v, u in zip(vs, ts)})
                    return functools.reduce(lambda a, b: a + b, ts)
                return [(functools.partial(piece, r, cc, range(v, v + 4)), None, None, LG, 40) for r in range(0, QM, 8)
                        for cc in range(0, cs[0].shape[1], 128) for v in range(0, SF.nb, 4)]

            def d3(c, side):
                c0, c1 = FCH[c]
                cs = fmm(SF, lambda u: lf_v[SF.ul.index(u), 0:QM], lambda r: s3_v[r, 0:D4 // 2, c0:c1], side)
                assert not side.pieces
                return gelu_pieces(c, cs)

            def d4(c, side):
                c0, c1 = FCH[c]
                lh = _run(SF.up, [_cat([_cat([hs.pop((c, v, r, cc)) for r in range(0, QM, 8)], 0)
                                        for cc in range(0, c1 - c0, 128)], 1) for v in range(SF.nb)])
                rhs = lambda r: s4_v[r, c0 // 2:c1 // 2, :]
                if c + 1 < len(FCH):
                    for n in SF.order:
                        for r in range(SF.rank):
                            if SF.wn[r] == n:
                                acc[n] = mm(lh[SF.un[r]], rhs(r), side, acc.get(n))
                else:
                    idx = lambda v: (pl.ds(r0 + (v // 4) * QM, QM), slice((v % 4) * D4, (v % 4 + 1) * D4))

                    def extra(n):
                        if n >= SF.nb:
                            return acc.get(n)
                        return b_v[idx(n)] + acc[n] if n in acc else b_v[idx(n)]

                    def emit_b(v, t):
                        b_v[idx(v)] = jnp.concatenate([1.0 - g_v[idx(v)[0], :]] * 2, axis=1) * t
                    fmm(SF, lambda u: lh[u], rhs, side, extra, emit_b)
                assert not side.pieces

            g0 = d3(0, Side(relays[:16], 43, 6))
            g1 = d3(1, Side(_merge(g0, gates[:12]), 43, 4))
            d4(0, Side(g1[:22], 41, 8))
            g2 = d3(2, Side(_merge(g1[22:], relays[16:32]), 47))
            d4(1, Side(_merge(g2, relays[32:60]), 43, 4))
            g3 = d3(3, Side(_merge(gates[12:], xes, norms), 49))
            d4(2, Side(_merge(g3, combs), 43, 4))
            d4(3, Side(relays[60:], 44))

            @pl.when(i + 2 < NG)
            def _():
                qkv_start(i + 2)

            return carry

        lax.fori_loop(0, NB, ffn, 0)

    pl.run_scoped(
        phase_b,
        pltpu.VMEM((9, D // 4, D // 2), u32),
        pltpu.VMEM((7, D // 4, D // 2), u32),
        pltpu.VMEM((52, D4 // 2 + 8, F4), u32),
        pltpu.VMEM((50, F4 // 2 + 8, D4), u32),
        pltpu.VMEM((NT, S + 2 * PAD, 128), f32),
        pltpu.VMEM((TM, D), f32),
        pltpu.VMEM((2, 7, HM // 2, D // 2), u32),
        pltpu.VMEM((52, QM + 8, D4), bf16),
        pltpu.VMEM((2, TM, 128), f32),
        pltpu.VMEM((8, D), f32),
    )

    def phase_a(out_v, e_v, oe_v, ke_v, ve_v, o_v):
        def pre(it, carry):
            hist.clear()
            for u in range(3 * NG // NPRE):
                s0 = (it * (3 * NG // NPRE) + u) * G

                @functools.lru_cache(None)
                def node(k, n):
                    if n < 16:
                        return _unpack(wqkv_v[s0 + zero_s[k] + n % 4, (n // 4) * (D // 8):(n // 4 + 1) * (D // 8), :])
                    a, sa, b, sb = S49.vp[n - 16]
                    return _run([(0, sa, 1, sb)], [node(k, a), node(k, b)])[-1]

                def rhs(r):
                    n = S49.vn[r]
                    if n < 16:
                        return wqkv_v[s0 + n % 4, (n // 4) * (D // 8):(n // 4 + 1) * (D // 8), :]
                    return node(r // 7, n).astype(bf16)

                def emit_e(v, t):
                    e_v[(v // 4) * 8:(v // 4 + 1) * 8, s0 + v % 4] = _pack(t).reshape(8, 8, DH)
                fmm(S49N, lambda k: xe_v[S49.ul.index(k), 0:4 * NPAIR], rhs, None, emit=emit_e)
            return carry

        lax.fori_loop(0, NPRE, pre, 0)

        wait("wo")
        mem_v[...] = mem0_ref[...].astype(f32)

        def slab(w, h):
            return (h // G) * SPG + w * G + h % G

        def step(j, hx, odd, late, allow, fill):
            qs, ks, vs, ps = {}, {}, {}, {}
            wload = lambda w, h: pltpu.bitcast(wqkv_v[slab(w, h)], bf16)
            eload = lambda w, h: pltpu.bitcast(e_v[j, slab(w, h)], bf16)

            def proj(g):
                part = {}
                if late and g == 0:
                    for h in range(2):
                        for w in range(3):
                            part[w, h] = _dot(hx[:, :DH2], wload(w, h)[:DH2])
                for h in range(g * G, (g + 1) * G):
                    q, k, v = [(_dot(hx[:, DH2:], wload(w, h)[DH2:]) + part[w, h] if (w, h) in part
                                else _dot(hx, wload(w, h))).astype(bf16) for w in range(3)]
                    if odd:
                        q = jnp.concatenate([q, eload(0, h)], axis=0)
                        k = jnp.concatenate([pltpu.bitcast(ke_v[h], bf16), eload(1, h), k], axis=0)
                        v = jnp.concatenate([pltpu.bitcast(ve_v[h], bf16), eload(2, h), v], axis=0)
                    else:
                        ke_v[h] = pltpu.bitcast(k, u32)
                        ve_v[h] = pltpu.bitcast(v, u32)
                        k = jnp.concatenate([k, eload(1, h)], axis=0)
                        v = jnp.concatenate([v, eload(2, h)], axis=0)
                    qs[h], ks[h], vs[h] = q, k, v

            def score(g):
                for h in range(g * G, (g + 1) * G):
                    s = lax.dot_general(qs.pop(h), ks.pop(h), (((1,), (1,)), ((), ())),
                                        preferred_element_type=f32)
                    ps[h] = _softmax(s, allow, fill)

            def pv(g):
                os_ = []
                for h in range(g * G, (g + 1) * G):
                    o = _dot(ps.pop(h), vs.pop(h))
                    o_v[:, h * 128:(h + 1) * 128] = _pack(o[:32])
                    os_.append(o)
                if odd:
                    quads = [jnp.concatenate([os_[2 * kk][r:r + 8], os_[2 * kk + 1][r:r + 8]], axis=1)
                             for r in (32, 40) for kk in range(2)]
                    for k, t in enumerate(_lcombos(*quads)):
                        oe_v[k, pl.ds(pl.multiple_of(j * 8, 8), 8), g * 256:(g + 1) * 256] = t

            acc = [None] * NT

            def wo(h0, h1, j0, j1):
                o = pltpu.bitcast(o_v[:, h0 * 128:h1 * 128], bf16)
                for n in range(j0, j1):
                    y = _dot(o, pltpu.bitcast(wo_v[n, h0 * 64:h1 * 64, :], bf16))
                    acc[n] = y if acc[n] is None else y + acc[n]

            for t in range(NG):
                proj(t)
                if t >= 2:
                    pv(t - 2)
                if t >= 1:
                    score(t - 1)
            wo(0, 16, 0, 4)
            pv(NG - 2)
            score(NG - 1)
            wo(0, 16, 4, 8)
            pv(NG - 1)
            wo(16, 24, 0, 8)
            wo(24, 32, 0, 8)
            return jnp.concatenate(acc, axis=1)

        def emit(j, r0, o0, a):
            rs = pl.ds(r0 + o0, 24)
            g = jnp.concatenate([g_v[rs, :]] * NT, axis=1)
            out_v[j, o0:o0 + 24, :] = (g * a + b_v[rs, :]).astype(bf16)

        def pair(j, mem, late):
            r0 = pl.multiple_of(j * 64, 64)
            allow_e, fill_e, allow_o, fill_o = _masks()
            xa = x_v[pl.ds(r0 + 16, 8), :].astype(f32)
            xb = x_v[pl.ds(r0 + 40, 8), :].astype(f32)
            hx = jnp.concatenate([x_v[pl.ds(r0, 16), :], jnp.concatenate([xa, mem], 0).astype(bf16)], 0)
            oe = step(j, hx, False, late, allow_e, fill_e)
            emit(j, r0, 0, oe[:24])
            hx = jnp.concatenate([jnp.concatenate([oe[24:32], xb], 0).astype(bf16), x_v[pl.ds(r0 + 48, 16), :]], 0)
            oo = step(j, hx, True, True, allow_o, fill_o)
            emit(j, r0, 40, oo[8:])
            return oo[:8]

        def a_iter(it, carry):
            mem = mem_v[...]
            for t in range(PPI):
                mem = pair(it * PPI + t, mem, t > 0)
            mem_v[...] = mem
            for t in range(PPI):
                for o0 in (0, 40):
                    idx = (it * PPI + t, pl.ds(o0, 24))
                    pltpu.make_async_copy(out_v.at[idx], out_hbm.at[idx], sem_out).start()
            return carry

        lax.fori_loop(0, NPAIR // PPI, a_iter, 0)

        @once
        def _post():
            hist.clear()
            NK, NW = 2, 128
            for n in range(D // (4 * NW)):
                @functools.lru_cache(None)
                def node(k, kc, q):
                    if q < 16:
                        return _unpack(raw(kc, q, 4 * zero_s[k]))
                    a, sa, b, sb = S49.vp[q - 16]
                    return _run([(0, sa, 1, sb)], [node(k, kc, a), node(k, kc, b)])[-1]

                def raw(kc, q, z=0):
                    return _cat([_cat([wo_v[z + (4 * n + q % 4) * (NW // 128) + c, (4 * g + q // 4) * 64:(4 * g + q // 4 + 1) * 64, :]
                                       for c in range(NW // 128)], 1)
                                 for g in range(kc * NG // NK, (kc + 1) * NG // NK)], 0)

                def prod(r, kc, acc):
                    z = zero_s[7 + r % 7]
                    quad = [_cat([oe_v[z + r // 7, (q // 2) * 128:(q // 2 + 1) * 128, (2 * g + q % 2) * 128:(2 * g + q % 2 + 1) * 128]
                                  for g in range(kc * NG // NK, (kc + 1) * NG // NK)], 1) if q in UQ[r % 7] else None
                            for q in range(4)]
                    f = UFORMS[r % 7]
                    lhs = quad[f[0]] if len(f) == 1 else _run([(0, f[1], 1, f[3])], [quad[f[0]], quad[f[2]]])[-1]
                    q = S49.vn[r]
                    return mm(lhs, raw(kc, q) if q < 16 else node(r // 7, kc, q).astype(bf16), None, acc)

                val, part = {}, {}
                for nd in S49N.order:
                    rs = [r for r in range(49) if S49.wn[r] == nd]
                    for r in rs:
                        if r not in part:
                            for kc in range(NK - 1):
                                for k2 in SEQ:
                                    part[r // 7 * 7 + k2] = prod(r // 7 * 7 + k2, kc, part.get(r // 7 * 7 + k2))
                    t = part[rs[0]] if rs else None
                    for q, sg in sorted(S49.par[nd], key=lambda e: -e[1]):
                        t = val[q] if t is None else (t + val[q] if sg > 0 else t - val[q])
                    if rs:
                        t = prod(rs[0], NK - 1, t)
                    val[nd] = t
                    if nd < 16:
                        o0, j0 = 24 + (nd // 8) * 8, (nd // 4 % 2) * 16
                        c0 = (4 * n + nd % 4) * NW
                        for jj in range(16):
                            rr = slice((j0 + jj) * 64 + o0, (j0 + jj) * 64 + o0 + 8)
                            out_v[j0 + jj, o0:o0 + 8, c0:c0 + NW] = (
                                _cat([g_v[rr, :]] * (NW // 128), 1) * t[jj * 8:jj * 8 + 8] + b_v[rr, c0:c0 + NW]).astype(bf16)
                        idx = (pl.ds(j0, 16), pl.ds(o0, 8), pl.ds(c0, NW))
                        pltpu.make_async_copy(out_v.at[idx], out_hbm.at[idx], sem_out).start()

        pltpu.make_async_copy(out_v, out_hbm, sem_out).wait()

    pl.run_scoped(
        phase_a,
        pltpu.VMEM((NPAIR, 64, D), bf16),
        pltpu.VMEM((NPAIR, 3 * H, 8, DH), u32),
        pltpu.VMEM((7, 8 * NPAIR, H * DH // 2), f32),
        pltpu.VMEM((H, 16, 128), u32),
        pltpu.VMEM((H, 16, 128), u32),
        pltpu.VMEM((16, H * DH), u32),
    )


@jax.jit
def pallas_gated_mix__memory_aug_recurrent_mem_tr__mixer_s_mlp__prompt_kernel(
    A_x, A_mem0, A_Wq, A_Wk, A_Wv, A_Wo, A_seg_len, B_x, B_w1, B_w2, B_w3, B_w4, gate_w,
):
    assert A_x.shape == (1, S, D) and A_mem0.shape == (1, M, D)
    any_spec = pl.BlockSpec(memory_space=pl.ANY)
    out = pl.pallas_call(
        _kernel,
        out_shape=jax.ShapeDtypeStruct((NPAIR, 64, D), bf16),
        in_specs=[any_spec] * 11,
        out_specs=any_spec,
        scratch_shapes=[
            pltpu.VMEM((S, D), bf16),
            pltpu.VMEM((3 * H, D // 2, DH), u32),
            pltpu.VMEM((NT, H * DH // 2 + 8, 128), u32),
            pltpu.VMEM((S, D), f32),
            pltpu.VMEM((S, 128), f32),
            pltpu.VMEM((52, 4 * NPAIR + 8, D4), bf16),
            pltpu.VMEM((M, D), f32),
            pltpu.VMEM((M, D), bf16),
            pltpu.VMEM((64, 128), bf16),
            pltpu.SMEM((NZ,), jnp.int32),
            pltpu.SemaphoreType.DMA((NLOAD,)),
            pltpu.SemaphoreType.DMA((NG,)),
            pltpu.SemaphoreType.DMA,
        ],
        compiler_params=pltpu.CompilerParams(vmem_limit_bytes=127 * 1024 * 1024,
                                             disable_bounds_checks=True),
    )(
        A_x.reshape(S, D), A_mem0.reshape(M, D),
        A_Wq.reshape(D // 2, 2 * H, DH), A_Wk.reshape(D // 2, 2 * H, DH), A_Wv.reshape(D // 2, 2 * H, DH),
        A_Wo.reshape(H * DH, D), B_w1, B_w2, B_w3, B_w4, gate_w.reshape(NT, 128),
    )
    return out.reshape(1, S, D)
```
